```python
import jax
import jax.numpy as jnp

def _softmax(x, axis=-1):
    return jax.nn.softmax(x, axis=axis)
def _gelu(x):
    return jax.nn.gelu(x, approximate=True)
def _silu(x):
    return jax.nn.silu(x)
def _sigmoid(x):
    return jax.nn.sigmoid(x)
def _layernorm(x, axis=-1, eps=1e-5):
    m = jnp.mean(x, axis=axis, keepdims=True)
    v = jnp.var(x, axis=axis, keepdims=True)
    return (x - m) / jnp.sqrt(v + eps)
def _scatter_add(tgt, idx, src, axis=0):
    return tgt.at[idx].add(src)
def _segment_sum(src, seg, n):
    return jax.ops.segment_sum(src, seg, n)
class _Rng:
    def __init__(self, key):
        self._k = key
    def _next(self):
        self._k, sub = jax.random.split(self._k)
        return sub
    def normal(self, shape):
        return jax.random.normal(self._next(), shape, dtype=jnp.bfloat16)
    def randint(self, lo, hi, shape):
        return jax.random.randint(self._next(), shape, lo, hi, dtype=jnp.int32)
    def uniform(self, shape, lo=0.0, hi=1.0):
        return jax.random.uniform(self._next(), shape, jnp.bfloat16, lo, hi)
    def permutation(self, n):
        return jax.random.permutation(self._next(), n)


kernel_name = 'concat_heads__ssm_conv_s5__ssm_conv_h3__prompt'

def setup_inputs():
    _rng = _Rng(jax.random.key(int.from_bytes(__import__("os").urandom(4), "little")))
    _w = (lambda a: (lambda t: t.astype(jnp.bfloat16) if jnp.issubdtype(t.dtype, jnp.floating) else t)(jnp.asarray(a)))
    def _A_setup():
        B, S, D = 1, 2048, 640
        P = D
        Lambda_re = -0.5 * jnp.exp((lambda *s: _rng.normal(s) * 0.05)(P))
        Lambda_im = (lambda *s: _rng.normal(s) * 0.05)(P) * 1.0
        B_re = (lambda *s: _rng.normal(s) * 0.05)(P, D) * (D ** -0.5)
        B_im = (lambda *s: _rng.normal(s) * 0.05)(P, D) * (D ** -0.5)
        C_re = (lambda *s: _rng.normal(s) * 0.05)(D, P) * (P ** -0.5)
        C_im = (lambda *s: _rng.normal(s) * 0.05)(D, P) * (P ** -0.5)
        log_dt = (lambda *s: _rng.normal(s) * 0.05)(P) * 0.3 - 2.0
        Dskip = (lambda *s: _rng.normal(s) * 0.05)(D)
        return {
            "x": _w((lambda *s: _rng.normal(s) * 0.05)(B, S, D)),
            "Lambda_re": _w(Lambda_re),
            "Lambda_im": _w(Lambda_im),
            "B_re": _w(B_re),
            "B_im": _w(B_im),
            "C_re": _w(C_re),
            "C_im": _w(C_im),
            "log_dt": _w(log_dt),
            "Dskip": _w(Dskip),
        }
    _A_in = _A_setup()

    def _B_setup():
        B, S, D = 1, 2048, 640
        ks = 4
        return {
            "q": _w((lambda *s: _rng.normal(s) * 0.05)(B, S, D)),
            "k": _w((lambda *s: _rng.normal(s) * 0.05)(B, S, D)),
            "v": _w((lambda *s: _rng.normal(s) * 0.05)(B, S, D)),
            "shift_k": _w((lambda *s: _rng.normal(s) * 0.05)(D, ks) * 0.5),
            "ssm_k": _w((lambda *s: _rng.normal(s) * 0.05)(D, S) * (1.0 / S ** 0.5)),
            "ssm_D": _w((lambda *s: _rng.normal(s) * 0.05)(D)),
        }
    _B_in = _B_setup()

    return {
        "A_x": _A_in["x"],
        "A_Lambda_re": _A_in["Lambda_re"],
        "A_Lambda_im": _A_in["Lambda_im"],
        "A_B_re": _A_in["B_re"],
        "A_B_im": _A_in["B_im"],
        "A_C_re": _A_in["C_re"],
        "A_C_im": _A_in["C_im"],
        "A_log_dt": _A_in["log_dt"],
        "A_Dskip": _A_in["Dskip"],
        "B_q": _B_in["q"],
        "B_k": _B_in["k"],
        "B_v": _B_in["v"],
        "B_shift_k": _B_in["shift_k"],
        "B_ssm_k": _B_in["ssm_k"],
        "B_ssm_D": _B_in["ssm_D"],
    }

def reference(A_x, A_Lambda_re, A_Lambda_im, A_B_re, A_B_im, A_C_re, A_C_im, A_log_dt, A_Dskip, B_q, B_k, B_v, B_shift_k, B_ssm_k, B_ssm_D):
    def _A_ref(x, Lambda_re, Lambda_im, B_re, B_im, C_re, C_im, log_dt, Dskip):
        Bsz, L, H = x.shape
        Lam = Lambda_re + 1j * Lambda_im
        Bmat = B_re + 1j * B_im
        Cmat = C_re + 1j * C_im
        dt = jnp.exp(log_dt)
        Lam_bar = jnp.exp(dt * Lam)
        B_bar = ((Lam_bar - 1.0) / Lam)[:, None] * Bmat
        Bu = jnp.einsum("bld,pd->blp", x + 0j, B_bar)
        h = jnp.zeros_like(Bu[:, 0, :])
        hs = []
        for t in range(L):
            h = Lam_bar[None, :] * h + Bu[:, t, :]
            hs.append(h)
        hseq = jnp.stack(hs, 1)
        y = 2.0 * jnp.einsum("blp,dp->bld", hseq, Cmat).real + x * Dskip[None, None, :]
        return y

    def _B_ref(q, k, v, shift_k, ssm_k, ssm_D):
        B, S, D = q.shape
        ks = shift_k.shape[-1]
        k_pad = jnp.pad(k, ((0, 0), (ks - 1, 0), (0, 0)))
        k_shift = jnp.zeros_like(k)
        for t in range(ks):
            k_shift = k_shift + k_pad[:, t:t + S, :] * shift_k[:, ks - 1 - t][None, None, :]
        kv = k_shift * v
        L = 2 * S
        kv_pad = jnp.pad(kv, ((0, 0), (0, S), (0, 0)))
        kf_pad = jnp.pad(ssm_k, ((0, 0), (0, S)))
        kv_f = (lambda x, axes=(-2,-1): jnp.fft.rfft2(x.astype(jnp.float32), axes=axes))(kv_pad[:, None, :, :], axes=(1, 2))
        kf_f = (lambda x, axes=(-2,-1): jnp.fft.rfft2(x.astype(jnp.float32), axes=axes))(kf_pad[:, None, :], axes=(1, 2))
        kf_f = (lambda x, *d: x.transpose(*d))(kf_f, 1, 2, 0)
        y_f = kv_f * kf_f[None, :, :, :]
        y = (lambda x, s, axes=(-2,-1): jnp.fft.irfft2(x, s=s, axes=axes).astype(jnp.bfloat16))(y_f, (1, L), axes=(1, 2))[:, 0, :S, :]
        y = y + kv * ssm_D[None, None, :]
        return q * y

    a = _A_ref(A_x, A_Lambda_re, A_Lambda_im, A_B_re, A_B_im, A_C_re, A_C_im, A_log_dt, A_Dskip)
    b = _B_ref(B_q, B_k, B_v, B_shift_k, B_ssm_k, B_ssm_D)
    return jnp.concatenate([a, b], axis=-1)
```

```python
import math

import jax
import jax.numpy as jnp
import numpy as np
from jax import lax
from jax.experimental import pallas as pl
from jax.experimental.pallas import tpu as pltpu

F32, BF16, I32 = jnp.float32, jnp.bfloat16, jnp.int32

L = 2048
D = 640
NG = D // 128
UNIT = 256
R = UNIT // 8
LEAD = L // UNIT - NG
MM = 64
BU_PART = 9 * R
YS_ROWS = 8 * (R + 1)
KF_PAD = 8


class _Signed:
    def __init__(self, v, neg=False):
        self.v, self.neg = v, neg

    def __neg__(self):
        return _Signed(self.v, not self.neg)

    def __add__(self, o):
        if self.neg == o.neg:
            return _Signed(self.v + o.v, self.neg)
        return _Signed(o.v - self.v if self.neg else self.v - o.v)

    def __sub__(self, o):
        return self + (-o)

    def __mul__(self, c):
        return _Signed(self.v * np.float32(-c if self.neg else c))

    def get(self):
        return -self.v if self.neg else self.v


def _rot(re, im, num, den):
    num %= den
    h = math.sqrt(0.5)
    if num == 0:
        return re, im
    if 4 * num == den:
        return -im, re
    if 4 * num == 3 * den:
        return im, -re
    if 8 * num == den:
        return (re - im) * h, (re + im) * h
    if 8 * num == 3 * den:
        return (re + im) * (-h), (re - im) * h
    if 8 * num == 5 * den:
        return (im - re) * h, (re + im) * (-h)
    if 8 * num == 7 * den:
        return (re + im) * h, (im - re) * h
    c = math.cos(2 * math.pi * num / den)
    s = math.sin(2 * math.pi * num / den)
    return re * c - im * s, re * s + im * c


def _dft4(z, sign):
    (r0, i0), (r1, i1), (r2, i2), (r3, i3) = z
    ar, ai, br, bi = r0 + r2, i0 + i2, r0 - r2, i0 - i2
    cr, ci, dr, di = r1 + r3, i1 + i3, r1 - r3, i1 - i3
    plus, minus = (br - di, bi + dr), (br + di, bi - dr)
    if sign < 0:
        plus, minus = minus, plus
    return [(ar + cr, ai + ci), plus, (ar - cr, ai - ci), minus]


def _fwd1(n0, u):
    a, b = u[:4], u[4:]
    z = _dft4([_rot(a[m], b[m], n0 + 4 * m, 64) for m in range(4)], 1)
    out = [_rot(*z[k], n0 * k, 16) for k in range(4)]
    s2 = [a[m] + b[m] for m in range(4)]
    d2 = [a[m] - b[m] for m in range(4)]
    p = _rot(d2[0], d2[2], n0, 32)
    q = _rot(d2[1], d2[3], n0 + 4, 32)
    out.append((p[0] + q[0], p[1] + q[1]))
    out.append(_rot(p[0] - q[0], p[1] - q[1], n0, 8))
    s3 = [s2[0] + s2[2], s2[1] + s2[3]]
    d3 = [s2[0] - s2[2], s2[1] - s2[3]]
    out.append(_rot(d3[0], d3[1], n0, 16))
    out.append((s3[0] + s3[1], s3[0] - s3[1]))
    return out


def _fwd2(grp, z):
    if grp < 7:
        return _dft4(z, 1)
    s4 = [t[0] for t in z]
    d4 = [t[1] for t in z]
    p = (d4[0], d4[2])
    q = _rot(d4[1], d4[3], 1, 8)
    s5 = [s4[0] + s4[2], s4[1] + s4[3]]
    return [
        (s5[0] + s5[1], s5[0] - s5[1]),
        (s4[0] - s4[2], s4[1] - s4[3]),
        (p[0] + q[0], p[1] + q[1]),
        (p[0] - q[0], p[1] - q[1]),
    ]


def _inv2(grp, w):
    if grp < 7:
        return _dft4(w, -1)
    s5 = [w[0][0] + w[0][1], w[0][0] - w[0][1]]
    s4 = [s5[0] + w[1][0], s5[1] + w[1][1], s5[0] - w[1][0], s5[1] - w[1][1]]
    p = (w[2][0] + w[3][0], w[2][1] + w[3][1])
    q = _rot(w[2][0] - w[3][0], w[2][1] - w[3][1], -1, 8)
    d4 = [p[0], q[0], p[1], q[1]]
    return [(s4[n], d4[n]) for n in range(4)]


def _inv1(n0, z):
    t = _dft4([_rot(*z[k], -n0 * k, 16) for k in range(4)], -1)
    ab = [_rot(*t[m], -(n0 + 4 * m), 64) for m in range(4)]
    e = _rot(*z[5], -n0, 8)
    p = _rot(z[4][0] + e[0], z[4][1] + e[1], -n0, 32)
    q = _rot(z[4][0] - e[0], z[4][1] - e[1], -(n0 + 4), 32)
    d2 = [p[0], q[0], p[1], q[1]]
    d3 = _rot(*z[6], -n0, 16)
    s3 = [z[7][0] + z[7][1], z[7][0] - z[7][1]]
    s2 = [s3[0] + d3[0], s3[1] + d3[1], s3[0] - d3[0], s3[1] - d3[1]]
    a = [ab[m][0] + (s2[m] + d2[m]) for m in range(4)]
    b = [ab[m][1] + (s2[m] - d2[m]) for m in range(4)]
    return a + b


_F1 = [4 * (g + 4 * k) + 1 for g in range(4) for k in range(4)]
_F1 += [2 * (4 * (g + 2 * k) + 1) for g in range(2) for k in range(4)]
_F1 += [4 * (4 * k + 1) for k in range(4)]
_F1 += [0, 16, 8, 40]
_REAL_SLOT = 28


def _dft_tables():
    kap = np.arange(128)
    j = 8 * (kap // 16) + kap % 8
    part = (kap // 8) % 2
    pr, pc, jr, jc = part[:, None], part[None, :], j[:, None], j[None, :]
    lo = 2 * np.pi * jr * jc / 64
    base = np.where(pr == pc, np.cos(lo), np.where(pr == 0, -np.sin(lo), np.sin(lo)))
    hi = 2 * np.pi * (32 + 64 * (jr - 32)) * jc / 4096
    v0 = np.where(pr == 0, np.cos(lo), np.where(jr == 0, np.cos(np.pi * jc), np.sin(lo)))
    v32 = np.where(pr == 0, np.cos(hi), np.sin(hi))
    real = np.where(jr < 32, np.where(pc == 0, v0, 0.0), np.where(pc == 1, v32, 0.0))
    th = 2 * np.pi * np.outer(np.array(_F1), j) / 4096
    return np.concatenate([base, real, np.cos(th), np.sin(th)]).astype(np.float32)


_TABLES = _dft_tables()
_ZERO = np.zeros((1,), np.int32)
_FFT_SCALE = 2.0 ** -11

(P_MU, P_RHO1, P_RHO2, P_RHO4, P_TAP, P_SSMD, P_DSKIP, P_ROWS) = (0, 2, 4, 6, 8, 12, 13, 14)


def _cmul(a, b):
    return a[0] * b[0] - a[1] * b[1], a[0] * b[1] + a[1] * b[0]


def _pack(lo, hi):
    return pltpu.bitcast(jnp.concatenate([lo, hi], axis=0).astype(BF16), I32)


def _unpack(w):
    v = pltpu.bitcast(w, BF16).astype(F32)
    return v[:8], v[8:]


def _weave(passes, tasks, pred):
    total = sum(c for c, _ in tasks)
    at, done = [[] for _ in passes], 0.0
    for cost, fn in tasks:
        at[int((done + 0.5 * cost) / total * len(passes))].append(fn)
        done += cost
    for (lhs, rhs, consume), fns in zip(passes, at):
        w = rhs()
        for fn in fns:
            w[-1] = jnp.where(pred, w[-1], fn())
        a = pltpu.bitcast(jnp.concatenate(lhs(), axis=0), BF16)
        b = pltpu.bitcast(jnp.concatenate(w, axis=0), BF16)
        consume(jnp.dot(a, b, preferred_element_type=F32))


def _kernel(zero_hbm, tab_hbm, x_hbm, lre_hbm, lim_hbm, bre_hbm, bim_hbm, cre_hbm, cim_hbm,
            ldt_hbm, dsk_hbm, q_hbm, k_hbm, v_hbm, tap_hbm, sk_hbm, sd_hbm,
            o_hbm,
            zero_s, tab, lre_v, lim_v, ldt_v, dsk_v, sd_v, tap_v,
            xb, braw, craw, qb, kb, vb, skb,
            par, wb, wc, mf, mi, bu, hb, carry, ys, oa,
            kt, kf, st_u, st_k, st_i, vu, vk, pb, ob,
            sem_p, sem_x, sem_b, sem_c, sem_g, sem_oa, sem_ob):
    x32, q32, k32, v32 = (r.bitcast(I32) for r in (xb, qb, kb, vb))

    def rows(ref, start, n=8):
        return ref[pl.ds(start, n), :]

    def hint(v, n):
        return v if isinstance(v, int) else pl.multiple_of(v, n)

    small = [pltpu.make_async_copy(s, d, sem_p.at[n]) for n, (s, d) in enumerate((
        (zero_hbm, zero_s), (lre_hbm, lre_v), (lim_hbm, lim_v), (ldt_hbm, ldt_v),
        (dsk_hbm, dsk_v), (sd_hbm, sd_v), (tap_hbm, tap_v), (tab_hbm, tab)))]

    def x_dma(u):
        t = hint(u * UNIT, UNIT)
        return [pltpu.make_async_copy(
            x_hbm.at[pl.ds(t, UNIT), pl.ds(128 * n, 128)],
            xb.at[pl.ds(hint(n * L + t, UNIT), UNIT), :], sem_x.at[u, n]) for n in range(NG)]

    def b_dma(p):
        return [pltpu.make_async_copy(
            src.at[pl.ds(128 * p, 128), :], braw.at[pl.ds(D * c + 128 * p, 128), :],
            sem_b.at[2 * p + c]) for c, src in enumerate((bre_hbm, bim_hbm))]

    c_dma = [pltpu.make_async_copy(
        src.at[:, pl.ds(128 * p, 128)], craw.at[pl.ds(D * (NG * c + p), D), :],
        sem_c.at[NG * c + p]) for c, src in enumerate((cre_hbm, cim_hbm)) for p in range(NG)]

    def col_dma(which, g):
        src, dst = ((k_hbm, kb), (v_hbm, vb), (q_hbm, qb))[which]
        return pltpu.make_async_copy(
            src.at[:, pl.ds(hint(128 * g, 128), 128)],
            dst.at[pl.ds(hint(L * g, L), L), :], sem_g.at[which, g])

    def sk_dma(g):
        t = hint(128 * g, 128)
        return pltpu.make_async_copy(
            sk_hbm.at[pl.ds(t, 128), :], skb.at[pl.ds(t, 128), :], sem_g.at[3, g])

    def oa_dma(u):
        t = hint(u * UNIT, UNIT)
        return pltpu.make_async_copy(
            oa.at[pl.ds(t, UNIT), :], o_hbm.at[pl.ds(t, UNIT), pl.ds(0, D)], sem_oa.at[u])

    def ob_dma(g):
        return pltpu.make_async_copy(
            ob.at[pl.ds(hint(L * g, L), L), :],
            o_hbm.at[:, pl.ds(hint(D + 128 * g, 128), 128)], sem_ob.at[g])

    def start(ds):
        for d in ds:
            d.start()

    def wait(ds):
        for d in ds:
            d.wait()

    def prm(g, row):
        return rows(par, hint((g * P_ROWS + row) * 8, 8))

    def bu_passes(u, slot):
        out = []
        for m in range(UNIT // MM):
            for n in range(2 * NG):
                acc = []
                for kk in range(NG):
                    def lhs(m=m, kk=kk):
                        t = hint((kk * L + u * UNIT + m * MM) // 2, 8)
                        return [rows(x32, t + 8 * i) for i in range(MM // 16)]

                    def rhs(n=n, kk=kk):
                        return [rows(wb, (n * NG + kk) * 64 + 8 * i) for i in range(8)]

                    def consume(d, m=m, n=n, kk=kk, acc=acc):
                        acc.append(d if kk == 0 else acc[-1] + d)
                        if kk == NG - 1:
                            for i in range(MM // 8):
                                s, r = divmod(m * MM + 8 * i, R)
                                bu[pl.ds((slot * 2 * NG + n) * BU_PART + 9 * r + s, 8, stride=9), :] = (
                                    acc[-1][8 * i:8 * i + 8])
                    out.append((lhs, rhs, consume))
        return out

    def scan_tasks(u, slot, z, steps=4):
        state = {}

        def b(p, r):
            return tuple(rows(bu, z + (slot * 2 * NG + c * NG + p) * BU_PART + 9 * r) for c in range(2))

        def step(mu, h, br):
            return (mu[0] * h[0] + br[0]) - mu[1] * h[1], (mu[0] * h[1] + br[1]) + mu[1] * h[0]

        def ends(r0):
            for p in range(NG):
                mu = (prm(p, P_MU), prm(p, P_MU + 1))
                h = state.get(p)
                for r in range(r0, r0 + steps):
                    h = b(p, r) if r == 0 else step(mu, h, b(p, r))
                state[p] = h
            for p in range(NG):
                carry[pl.ds((2 * NG + p) * 8, 8), :] = state[p][0] + state[p][1]
            return pltpu.bitcast(rows(carry, z + 2 * NG * 8), I32)

        def starts():
            last = lax.broadcasted_iota(I32, (8, 128), 0) == 7
            for p in range(NG):
                a = tuple(pltpu.roll(jnp.where(last, rows(carry, (2 * p + c) * 8), state[p][c]), 1, 0)
                          for c in range(2))
                for sh, row in ((1, P_RHO1), (2, P_RHO2), (4, P_RHO4)):
                    t = _cmul((prm(p, row), prm(p, row + 1)),
                              tuple(pltpu.roll(c, sh, 0) for c in a))
                    a = (a[0] + t[0], a[1] + t[1])
                state[p] = a
            for p in range(NG):
                carry[pl.ds((2 * NG + p) * 8, 8), :] = state[p][0] + state[p][1]
            return pltpu.bitcast(rows(carry, z + 2 * NG * 8), I32)

        def run(r0):
            for p in range(NG):
                mu = (prm(p, P_MU), prm(p, P_MU + 1))
                h = state[p]
                for r in range(r0, r0 + steps, 2):
                    h0 = step(mu, h, b(p, r))
                    h = step(mu, h0, b(p, r + 1))
                    for c in range(2):
                        at = hint((c * NG + p) * (L // 2) + u * (UNIT // 2) + 4 * r, 8)
                        hb[pl.ds(at, 8), :] = _pack(h0[c], h[c])
                state[p] = h
                if r0 + steps == R:
                    for c in range(2):
                        carry[pl.ds((2 * p + c) * 8, 8), :] = h[c]
            return rows(hb, z + hint(u * (UNIT // 2), 8))

        tasks = [(8 * NG * steps, lambda r0=r0: ends(r0)) for r0 in range(0, R, steps)]
        tasks.append((34 * NG, starts))
        tasks += [(9 * NG * steps, lambda r0=r0: run(r0)) for r0 in range(0, R, steps)]
        return tasks

    def y_passes(u, ns):
        out = []
        for n in ns:
            for m in range(UNIT // MM):
                acc = []
                for kk in range(2 * NG):
                    def lhs(m=m, kk=kk):
                        t = hint(kk * (L // 2) + u * (UNIT // 2) + m * (MM // 2), 8)
                        return [rows(hb, t + 8 * i) for i in range(MM // 16)]

                    def rhs(n=n, kk=kk):
                        return [rows(wc, (kk * NG + n) * 64 + 8 * i) for i in range(8)]

                    def consume(d, m=m, n=n, kk=kk, acc=acc):
                        acc.append(d if kk == 0 else acc[-1] + d)
                        if kk == 2 * NG - 1:
                            for i in range(MM // 8):
                                r = m * (MM // 8) + i
                                ys[pl.ds(n * YS_ROWS + r, 8, stride=R + 1), :] = acc[-1][8 * i:8 * i + 8]
                    out.append((lhs, rhs, consume))
        return out

    def skip_task(u, n, z):
        def fn():
            dsk = prm(n, P_DSKIP)
            for i in range(UNIT // 16):
                xs = _unpack(rows(x32, hint((n * L + u * UNIT) // 2 + 8 * i, 8)))
                for c in range(2):
                    t = 16 * i + 8 * c
                    y = rows(ys, z + n * YS_ROWS + (t // R) * (R + 1) + t % R)
                    oa[pl.ds(hint(u * UNIT + t, 8), 8), pl.ds(128 * n, 128)] = y + xs[c] * dsk
            return pltpu.bitcast(oa[pl.ds(z + hint(u * UNIT, 8), 8), pl.ds(128 * n, 128)], I32)
        return (3 * UNIT // 8, fn)

    def widen_tasks(g, z, pieces=2):
        def fn(i0, i1):
            for i in range(i0, i1):
                lo, hi = _unpack(rows(k32, hint(g * (L // 2) + 8 * i, 8)))
                kf[pl.ds(KF_PAD + 16 * i, 8), :] = lo
                kf[pl.ds(KF_PAD + 16 * i + 8, 8), :] = hi
            return pltpu.bitcast(rows(kf, z + 16 * i0 + KF_PAD), I32)
        n = L // 16 // pieces
        return [(2 * n, lambda i=i: fn(i * n, (i + 1) * n)) for i in range(pieces)]

    def transpose_tasks(g, z, pieces=4):
        def fn(c0, c1):
            for c in range(c0, c1):
                t = skb[pl.ds(hint(128 * g, 128), 128), pl.ds(128 * c, 128)]
                kt[pl.ds(64 * c, 64), :] = pltpu.bitcast(t.T, I32)
            return rows(kt, z + 64 * c0)
        n = L // 128 // pieces
        return [(8 * n, lambda i=i: fn(i * n, (i + 1) * n)) for i in range(pieces)]

    def pass1(st, s, n0, u, z):
        for grp, pair in enumerate(_fwd1(n0, [_Signed(v) for v in u])):
            for c in range(2):
                st[pl.ds(((s * 4 + n0) * 8 + grp) * 16 + 8 * c, 8), :] = pair[c].get()
        return pltpu.bitcast(rows(st, z + (s * 4 + n0) * 128), I32)

    def u1_task(g, s, n0, z):
        def fn():
            taps = [prm(g, P_TAP + t) for t in range(4)]
            u = []
            for m in range(8):
                t = 64 * (n0 + 4 * m) + 8 * s
                ks = rows(kf, z + KF_PAD + t) * taps[0]
                for lag in range(1, 4):
                    ks = ks + rows(kf, z + KF_PAD + t - lag) * taps[lag]
                v = _unpack(rows(v32, hint(g * (L // 2) + (t // 16) * 8, 8)))[s % 2]
                u.append(ks * v)
            return pass1(st_u, s, n0, u, z)
        return (72 + (54, 96, 80, 96)[n0], fn)

    def k1_task(g, s, n0, z):
        def fn():
            u = [_unpack(rows(kt, z + 32 * (n0 + 4 * m) + 8 * (s // 2)))[s % 2] for m in range(8)]
            if s == 0 and n0 == 0:
                first = lax.broadcasted_iota(I32, (8, 128), 0) == 0
                u[0] = u[0] + jnp.where(first, prm(g, P_SSMD), 0.0)
            return pass1(st_k, s, n0, u, z)
        return (8 + (54, 96, 80, 96)[n0], fn)

    def pass2_task(st, dst, s, grps, z):
        def fn():
            for grp in grps:
                zs = [tuple(_Signed(rows(st, z + ((s * 4 + n0) * 8 + grp) * 16 + 8 * c)) for c in range(2))
                      for n0 in range(4)]
                for k, pair in enumerate(_fwd2(grp, zs)):
                    dst[pl.ds((4 * grp + k) * 64 + 8 * s, 8), :] = _pack(pair[0].get(), pair[1].get())
            return rows(dst, z + 4 * grps[0] * 64 + 8 * s)
        return (20 * len(grps), fn)

    def pass2_tasks(st, dst, s, z):
        return [pass2_task(st, dst, s, g, z) for g in ((0, 1, 2, 3), (4, 5, 6, 7))]

    def fwd_passes(grp, z):
        out = []
        for slot in range(4 * grp, 4 * grp + 4):
            got = {}
            for half in range(2):
                for which, src in enumerate((vu, vk)):
                    def lhs(slot=slot, half=half):
                        return [rows(mf, slot * 64 + 32 * half + 8 * i) for i in range(4)]

                    def rhs(slot=slot, src=src):
                        return [rows(src, z + slot * 64 + 8 * i) for i in range(8)]

                    def consume(d, slot=slot, half=half, which=which, got=got):
                        got[which] = d
                        if which == 0:
                            return
                        for i in range(4):
                            a = (got[0][16 * i:16 * i + 8], got[0][16 * i + 8:16 * i + 16])
                            b = (d[16 * i:16 * i + 8], d[16 * i + 8:16 * i + 16])
                            re, im = _cmul(a, b)
                            if slot == _REAL_SLOT and half == 0 and i == 0:
                                first = lax.broadcasted_iota(I32, (8, 128), 0) == 0
                                re = jnp.where(first, 0.5 * (a[0] * b[0]), re)
                                im = jnp.where(first, 0.5 * (a[1] * b[1]), im)
                            pb[pl.ds(slot * 64 + 32 * half + 8 * i, 8), :] = _pack(re, im)
                    out.append((lhs, rhs, consume))
        return out

    def inv_passes(grp, z):
        out = []
        for half in range(2):
            got = []
            for slot in range(4 * grp, 4 * grp + 4):
                def lhs(slot=slot, half=half):
                    return [rows(mi, slot * 64 + 32 * half + 8 * i) for i in range(4)]

                def rhs(slot=slot):
                    return [rows(pb, z + slot * 64 + 8 * i) for i in range(8)]

                def consume(d, half=half, got=got):
                    got.append(d)
                    if len(got) < 4:
                        return
                    for i in range(4):
                        w = [(_Signed(t[16 * i:16 * i + 8]), _Signed(t[16 * i + 8:16 * i + 16])) for t in got]
                        for n0, pair in enumerate(_inv2(grp, w)):
                            for c in range(2):
                                at = (((4 * half + i) * 4 + n0) * 8 + grp) * 16 + 8 * c
                                st_i[pl.ds(at, 8), :] = pair[c].get()
                out.append((lhs, rhs, consume))
        return out

    def inv1_task(g, s, n0, z):
        def fn():
            zs = [tuple(_Signed(rows(st_i, z + ((s * 4 + n0) * 8 + grp) * 16 + 8 * c)) for c in range(2))
                  for grp in range(8)]
            for m, y in enumerate(_inv1(n0, zs)):
                t = 64 * (n0 + 4 * m) + 8 * s
                qv = _unpack(rows(q32, hint(g * (L // 2) + (t // 16) * 8, 8)))[s % 2]
                ob[pl.ds(hint(g * L + t, 8), 8), :] = qv * y.get()
            return pltpu.bitcast(rows(ob, z + hint(g * L + 64 * n0 + 8 * s, 8)), I32)
        return (16 + (62, 104, 88, 104)[n0], fn)

    start(small)
    start(x_dma(0))
    start(b_dma(0))
    start(b_dma(1))
    wait(small)
    z = zero_s[0]
    z8 = pl.multiple_of(z, 8)
    sub = lax.broadcasted_iota(I32, (8, 128), 0)
    pred = sub + z >= 0

    def stack(ref):
        v = ref[...].astype(F32).reshape(1, D)
        return jnp.concatenate([v[:, 128 * g:128 * (g + 1)] for g in range(NG)]
                               + [v[:, :128]] * (8 - NG), axis=0)

    lre, lim = stack(lre_v), stack(lim_v)
    dt = jnp.exp(stack(ldt_v)).astype(BF16).astype(F32)
    mag, ang = jnp.exp(dt * lre), dt * lim
    lam = (mag * jnp.cos(ang), mag * jnp.sin(ang))
    scale = jnp.maximum(jnp.abs(lre), jnp.abs(lim))
    nre, nim = lre / scale, lim / scale
    den = (nre * nre + nim * nim) * scale
    coef = _cmul(((lam[0] - 1.0) / den, lam[1] / den), (nre, -nim))
    mu = (lam[0], -lam[1])
    rho = [mu]
    for _ in range(R.bit_length() + 1):
        rho.append(_cmul(rho[-1], rho[-1]))
    dsk, ssd = stack(dsk_v), stack(sd_v)
    taps = tap_v[...].astype(F32) * _FFT_SCALE
    for g in range(NG):
        def put(row, v):
            par[pl.ds((g * P_ROWS + row) * 8, 8), :] = v

        def lanes(v):
            return jnp.broadcast_to(v[g:g + 1], (8, 128))
        for c in range(2):
            put(P_MU + c, lanes(mu[c]))
            for n, row in enumerate((P_RHO1, P_RHO2, P_RHO4)):
                put(row + c, jnp.where(sub >= 1 << n, lanes(rho[n - 3][c]), 0.0))
        for t in range(4):
            put(P_TAP + t, jnp.broadcast_to(taps[t:t + 1, 128 * g:128 * (g + 1)], (8, 128)))
        put(P_SSMD, lanes(ssd))
        put(P_DSKIP, lanes(dsk))
    for i in range(2 * NG):
        carry[pl.ds(8 * i, 8), :] = jnp.zeros((8, 128), F32)
    kf[pl.ds(0, KF_PAD), :] = jnp.zeros((KF_PAD, 128), F32)

    def matrix_task(slot):
        def fn():
            if slot != _REAL_SLOT:
                c, s = tab[pl.ds(256 + slot, 1), :], tab[pl.ds(288 + slot, 1), :]
            for a in range(8):
                if slot == _REAL_SLOT:
                    re, im = rows(tab, 128 + 16 * a), rows(tab, 128 + 16 * a + 8)
                else:
                    br, bi = rows(tab, 16 * a), rows(tab, 16 * a + 8)
                    re, im = c * br - s * bi, s * br + c * bi
                mf[pl.ds(slot * 64 + 8 * a, 8), :] = _pack(re, im)
            m = pltpu.bitcast(rows(mf, z8 + slot * 64, 64), BF16)
            mi[pl.ds(slot * 64, 64), :] = pltpu.bitcast(m.T, I32)
            return rows(mi, z8 + slot * 64)
        return (56, fn)

    def scale_b(p):
        cr = jnp.broadcast_to(2.0 * coef[0][p:p + 1], (128, 128))
        ci = jnp.broadcast_to(2.0 * coef[1][p:p + 1], (128, 128))
        for kk in range(NG):
            br, bi = (braw[pl.ds(D * c + 128 * p, 128), pl.ds(128 * kk, 128)].T.astype(F32) for c in range(2))
            wb[pl.ds((p * NG + kk) * 64, 64), :] = pltpu.bitcast((cr * br - ci * bi).astype(BF16), I32)
            wb[pl.ds(((NG + p) * NG + kk) * 64, 64), :] = pltpu.bitcast(
                (-(cr * bi + ci * br)).astype(BF16), I32)

    def c_task(kk):
        def fn():
            for n in range(NG):
                t = craw[pl.ds(kk * D + 128 * n, 128), :]
                wc[pl.ds((kk * NG + n) * 64, 64), :] = pltpu.bitcast(t.T, I32)
            return rows(wc, z8 + kk * NG * 64)
        return (40, fn)

    first = bu_passes(0, 0)
    per_tile = NG
    mats = [matrix_task(slot) for slot in range(32)]
    wait(x_dma(0))
    for p in range(NG):
        if p + 2 < NG:
            start(b_dma(p + 2))
        elif p + 2 == NG:
            start(x_dma(1) + x_dma(2))
        else:
            start([sk_dma(0)] + c_dma)
        wait(b_dma(p))
        scale_b(p)
        mine = [q for i, q in enumerate(first) if (i // per_tile) % NG == p]
        _weave(mine, mats[4 * p:4 * p + 4], pred)
    start([col_dma(0, 0), col_dma(1, 0)] + x_dma(LEAD) + [col_dma(2, 0)])
    wait(x_dma(1) + x_dma(2))
    _weave(bu_passes(1, 1), mats[20:] + scan_tasks(0, 0, z8), pred)
    wait([sk_dma(0)] + c_dma)
    k_tasks = transpose_tasks(0, z8) + [c_task(kk) for kk in range(2 * NG)]
    for s in range(8):
        k_tasks += [k1_task(0, s, n0, z8) for n0 in range(4)] + pass2_tasks(st_k, vk, s, z8)
    passes = bu_passes(2, 0)
    sc = scan_tasks(1, 1, z8)
    _weave(passes, sc + k_tasks, pred)
    for _, fn in scan_tasks(2, 0, z8):
        fn()

    def body(i, _):
        nxt = jnp.minimum(i + 1, NG - 1)
        wait([col_dma(0, i), col_dma(1, i), col_dma(2, i)] + x_dma(i + LEAD))

        @pl.when(i + 1 < NG)
        def _():
            start([col_dma(0, i + 1), col_dma(1, i + 1), col_dma(2, i + 1)] + x_dma(i + 1 + LEAD))

        @pl.when(i + 2 < NG)
        def _():
            start([sk_dma(i + 2)])

        @pl.when(i + 1 < NG)
        def _():
            wait([sk_dma(i + 1)])

        u_tasks = widen_tasks(i, z8)
        k1 = transpose_tasks(nxt, z8)
        k2 = []
        for s in range(8):
            u_tasks += [u1_task(i, s, n0, z8) for n0 in range(4)] + pass2_tasks(st_u, vu, s, z8)
            k1 += [k1_task(nxt, s, n0, z8) for n0 in range(4)]
            k2 += pass2_tasks(st_k, vk, s, z8)
        bup = bu_passes(i + LEAD, 0)
        yp = y_passes(i, range(NG))
        per_n = len(yp) // NG
        _weave(bup, u_tasks, pred)
        _weave(yp[:8], k1[:4], pred)
        conv = fwd_passes(0, z8)
        for grp in range(1, 8):
            conv += fwd_passes(grp, z8) + inv_passes(grp - 1, z8)
        conv += yp[8:16] + inv_passes(7, z8)
        _weave(conv, scan_tasks(i + LEAD, 0, z8) + k1[4:22], pred)
        _weave(yp[16:24], k1[22:25], pred)
        inv = [inv1_task(i, s, n0, z8) for s in range(8) for n0 in range(4)]
        rest = k1[25:] + k2
        _weave(yp[24:2 * per_n + 8], inv[:8] + rest[:5], pred)
        _weave(yp[2 * per_n + 8:3 * per_n + 8],
               [skip_task(i, 0, z8), skip_task(i, 1, z8)] + inv[8:16] + rest[5:11], pred)
        _weave(yp[3 * per_n + 8:4 * per_n + 8], [skip_task(i, 2, z8)] + inv[16:25] + rest[11:17], pred)
        _weave(yp[4 * per_n + 8:], [skip_task(i, 3, z8)] + inv[25:] + rest[17:], pred)
        skip_task(i, 4, z8)[1]()
        start([oa_dma(i), ob_dma(i)])
        return 0

    start([sk_dma(1)])
    lax.fori_loop(0, NG, body, 0)

    for u in range(NG, NG + LEAD):
        yp = y_passes(u, range(NG))
        per_n = len(yp) // NG
        _weave(yp[:per_n + 8], [skip_task(u, 0, z8)][:0] + [(1, lambda: rows(hb, z8))], pred)
        for n in range(1, NG):
            _weave(yp[n * per_n + 8:(n + 1) * per_n + 8], [skip_task(u, n - 1, z8)], pred)
        skip_task(u, NG - 1, z8)[1]()
        start([oa_dma(u)])
    wait([oa_dma(u) for u in range(NG + LEAD)] + [ob_dma(g) for g in range(NG)])


@jax.jit
def pallas_concat_heads__ssm_conv_s5__ssm_conv_h3__prompt_kernel(
    A_x: jax.Array,
    A_Lambda_re: jax.Array,
    A_Lambda_im: jax.Array,
    A_B_re: jax.Array,
    A_B_im: jax.Array,
    A_C_re: jax.Array,
    A_C_im: jax.Array,
    A_log_dt: jax.Array,
    A_Dskip: jax.Array,
    B_q: jax.Array,
    B_k: jax.Array,
    B_v: jax.Array,
    B_shift_k: jax.Array,
    B_ssm_k: jax.Array,
    B_ssm_D: jax.Array,
):
    assert A_x.shape == (1, L, D) and B_shift_k.shape == (D, 4)
    vmem = pltpu.VMEM
    dma = pltpu.SemaphoreType.DMA
    scratch = [
        pltpu.SMEM((1,), I32),
        vmem(_TABLES.shape, F32),
        vmem((D,), BF16), vmem((D,), BF16), vmem((D,), BF16), vmem((D,), BF16), vmem((D,), BF16),
        vmem((4, D), BF16),
        vmem((NG * L, 128), BF16),
        vmem((2 * D, D), BF16),
        vmem((2 * NG * D, 128), BF16),
        vmem((NG * L, 128), BF16),
        vmem((NG * L, 128), BF16),
        vmem((NG * L, 128), BF16),
        vmem((D, L), BF16),
        vmem((NG * P_ROWS * 8, 128), F32),
        vmem((2 * NG * NG * 64, 128), I32),
        vmem((2 * NG * NG * 64, 128), I32),
        vmem((32 * 64, 128), I32),
        vmem((32 * 64, 128), I32),
        vmem((2 * 2 * NG * BU_PART, 128), F32),
        vmem((2 * NG * L // 2, 128), I32),
        vmem((3 * NG * 8, 128), F32),
        vmem((NG * YS_ROWS, 128), F32),
        vmem((L, D), F32),
        vmem((L // 2, 128), I32),
        vmem((KF_PAD + L, 128), F32),
        vmem((2 * L, 128), F32),
        vmem((2 * L, 128), F32),
        vmem((2 * L, 128), F32),
        vmem((32 * 64, 128), I32),
        vmem((32 * 64, 128), I32),
        vmem((32 * 64, 128), I32),
        vmem((NG * L, 128), F32),
        dma((8,)), dma((L // UNIT, NG)), dma((2 * NG,)), dma((2 * NG,)), dma((4, NG)),
        dma((L // UNIT,)), dma((NG,)),
    ]
    out = pl.pallas_call(
        _kernel,
        out_shape=jax.ShapeDtypeStruct((L, 2 * D), F32),
        in_specs=[pl.BlockSpec(memory_space=pl.ANY)] * 17,
        out_specs=pl.BlockSpec(memory_space=pl.ANY),
        scratch_shapes=scratch,
        compiler_params=pltpu.CompilerParams(vmem_limit_bytes=100 * 1024 * 1024),
        name="s5_h3",
    )(_ZERO, _TABLES, A_x.reshape(L, D), A_Lambda_re, A_Lambda_im, A_B_re, A_B_im, A_C_re, A_C_im,
      A_log_dt, A_Dskip, B_q.reshape(L, D), B_k.reshape(L, D), B_v.reshape(L, D),
      B_shift_k.T, B_ssm_k, B_ssm_D)
    return out.reshape(1, L, 2 * D)
```

```python
import math

import jax
import jax.numpy as jnp
import numpy as np
from jax import lax
from jax.experimental import pallas as pl
from jax.experimental.pallas import tpu as pltpu

F32, BF16, I32 = jnp.float32, jnp.bfloat16, jnp.int32

L = 2048
D = 640
NG = D // 128
UNIT = 256
SEG = 16
R = UNIT // SEG
LEAD = L // UNIT - NG
MM = 64
BU_PART = 9 * 2 * R
YS_ROWS = SEG * (R + 1)
KF_PAD = 8


class _Signed:
    def __init__(self, v, neg=False):
        self.v, self.neg = v, neg

    def __neg__(self):
        return _Signed(self.v, not self.neg)

    def __add__(self, o):
        if self.neg == o.neg:
            return _Signed(self.v + o.v, self.neg)
        return _Signed(o.v - self.v if self.neg else self.v - o.v)

    def __sub__(self, o):
        return self + (-o)

    def __mul__(self, c):
        return _Signed(self.v * np.float32(-c if self.neg else c))

    def get(self):
        return -self.v if self.neg else self.v


def _rot(re, im, num, den):
    num %= den
    h = math.sqrt(0.5)
    if num == 0:
        return re, im
    if 4 * num == den:
        return -im, re
    if 4 * num == 3 * den:
        return im, -re
    if 8 * num == den:
        return (re - im) * h, (re + im) * h
    if 8 * num == 3 * den:
        return (re + im) * (-h), (re - im) * h
    if 8 * num == 5 * den:
        return (im - re) * h, (re + im) * (-h)
    if 8 * num == 7 * den:
        return (re + im) * h, (im - re) * h
    c = math.cos(2 * math.pi * num / den)
    s = math.sin(2 * math.pi * num / den)
    return re * c - im * s, re * s + im * c


def _dft4(z, sign):
    (r0, i0), (r1, i1), (r2, i2), (r3, i3) = z
    ar, ai, br, bi = r0 + r2, i0 + i2, r0 - r2, i0 - i2
    cr, ci, dr, di = r1 + r3, i1 + i3, r1 - r3, i1 - i3
    plus, minus = (br - di, bi + dr), (br + di, bi - dr)
    if sign < 0:
        plus, minus = minus, plus
    return [(ar + cr, ai + ci), plus, (ar - cr, ai - ci), minus]


def _fwd1(n0, u):
    a, b = u[:4], u[4:]
    z = _dft4([_rot(a[m], b[m], n0 + 4 * m, 64) for m in range(4)], 1)
    out = [_rot(*z[k], n0 * k, 16) for k in range(4)]
    s2 = [a[m] + b[m] for m in range(4)]
    d2 = [a[m] - b[m] for m in range(4)]
    p = _rot(d2[0], d2[2], n0, 32)
    q = _rot(d2[1], d2[3], n0 + 4, 32)
    out.append((p[0] + q[0], p[1] + q[1]))
    out.append(_rot(p[0] - q[0], p[1] - q[1], n0, 8))
    s3 = [s2[0] + s2[2], s2[1] + s2[3]]
    d3 = [s2[0] - s2[2], s2[1] - s2[3]]
    out.append(_rot(d3[0], d3[1], n0, 16))
    out.append((s3[0] + s3[1], s3[0] - s3[1]))
    return out


def _fwd2(grp, z):
    if grp < 7:
        return _dft4(z, 1)
    s4 = [t[0] for t in z]
    d4 = [t[1] for t in z]
    p = (d4[0], d4[2])
    q = _rot(d4[1], d4[3], 1, 8)
    s5 = [s4[0] + s4[2], s4[1] + s4[3]]
    return [
        (s5[0] + s5[1], s5[0] - s5[1]),
        (s4[0] - s4[2], s4[1] - s4[3]),
        (p[0] + q[0], p[1] + q[1]),
        (p[0] - q[0], p[1] - q[1]),
    ]


def _inv2(grp, w):
    if grp < 7:
        return _dft4(w, -1)
    s5 = [w[0][0] + w[0][1], w[0][0] - w[0][1]]
    s4 = [s5[0] + w[1][0], s5[1] + w[1][1], s5[0] - w[1][0], s5[1] - w[1][1]]
    p = (w[2][0] + w[3][0], w[2][1] + w[3][1])
    q = _rot(w[2][0] - w[3][0], w[2][1] - w[3][1], -1, 8)
    d4 = [p[0], q[0], p[1], q[1]]
    return [(s4[n], d4[n]) for n in range(4)]


def _inv1(n0, z):
    t = _dft4([_rot(*z[k], -n0 * k, 16) for k in range(4)], -1)
    ab = [_rot(*t[m], -(n0 + 4 * m), 64) for m in range(4)]
    e = _rot(*z[5], -n0, 8)
    p = _rot(z[4][0] + e[0], z[4][1] + e[1], -n0, 32)
    q = _rot(z[4][0] - e[0], z[4][1] - e[1], -(n0 + 4), 32)
    d2 = [p[0], q[0], p[1], q[1]]
    d3 = _rot(*z[6], -n0, 16)
    s3 = [z[7][0] + z[7][1], z[7][0] - z[7][1]]
    s2 = [s3[0] + d3[0], s3[1] + d3[1], s3[0] - d3[0], s3[1] - d3[1]]
    a = [ab[m][0] + (s2[m] + d2[m]) for m in range(4)]
    b = [ab[m][1] + (s2[m] - d2[m]) for m in range(4)]
    return a + b


_F1 = [4 * (g + 4 * k) + 1 for g in range(4) for k in range(4)]
_F1 += [2 * (4 * (g + 2 * k) + 1) for g in range(2) for k in range(4)]
_F1 += [4 * (4 * k + 1) for k in range(4)]
_F1 += [0, 16, 8, 40]
_REAL_SLOT = 28


def _dft_tables():
    kap = np.arange(128)
    j = 8 * (kap // 16) + kap % 8
    part = (kap // 8) % 2
    pr, pc, jr, jc = part[:, None], part[None, :], j[:, None], j[None, :]
    lo = 2 * np.pi * jr * jc / 64
    base = np.where(pr == pc, np.cos(lo), np.where(pr == 0, -np.sin(lo), np.sin(lo)))
    hi = 2 * np.pi * (32 + 64 * (jr - 32)) * jc / 4096
    v0 = np.where(pr == 0, np.cos(lo), np.where(jr == 0, np.cos(np.pi * jc), np.sin(lo)))
    v32 = np.where(pr == 0, np.cos(hi), np.sin(hi))
    real = np.where(jr < 32, np.where(pc == 0, v0, 0.0), np.where(pc == 1, v32, 0.0))
    th = 2 * np.pi * np.outer(np.array(_F1), j) / 4096
    return np.concatenate([base, real, np.cos(th), np.sin(th)]).astype(np.float32)


_TABLES = _dft_tables()
_ZERO = np.zeros((1,), np.int32)
_FFT_SCALE = 2.0 ** -11

(P_MU, P_RHO, P_RHO1, P_RHO2, P_RHO4, P_TAP, P_SSMD, P_DSKIP, P_COEF, P_ROWS) = (
    0, 2, 4, 6, 8, 10, 14, 15, 16, 20)


def _cmul(a, b):
    return a[0] * b[0] - a[1] * b[1], a[0] * b[1] + a[1] * b[0]


def _pack(lo, hi):
    return jnp.concatenate([lo, hi], axis=0).astype(BF16)


def _unpack(w):
    v = pltpu.bitcast(w, BF16).astype(F32)
    return v[:8], v[8:]


def _mix(a, b):
    keyed = []
    for which, tasks in enumerate((a, b)):
        total, done = sum(c for c, _ in tasks), 0.0
        for task in tasks:
            keyed.append(((done + 0.5 * task[0]) / total, which, len(keyed), task))
            done += task[0]
    return [k[-1] for k in sorted(keyed, key=lambda k: k[:3])]


def _weave(passes, tasks, pred, lag=24):
    total = sum(c for c, _ in tasks)
    at, done = [[] for _ in passes], 0.0
    for cost, fn in tasks:
        at[int((done + 0.5 * cost) / total * len(passes))].append(fn)
        done += cost
    seen = []
    for (lhs, rhs, consume), fns in zip(passes, at):
        def gate(v):
            return jnp.where(pred, v, seen[-lag]) if len(seen) >= lag else v
        w = rhs()
        for fn in fns:
            w[-1] = jnp.where(pred, w[-1], fn(gate))
        a = pltpu.bitcast(jnp.concatenate(lhs(), axis=0), BF16)
        b = pltpu.bitcast(jnp.concatenate(w, axis=0), BF16)
        d = jnp.dot(a, b, preferred_element_type=F32)
        seen.append(d[-8:])
        consume(d)


def _spread(tasks, where, extra):
    total, done, out, todo = sum(c for c, _ in tasks + extra), 0.0, [], list(zip(where, extra))
    for task in tasks:
        while todo and done >= todo[0][0] * total:
            done += todo[0][1][0]
            out.append(todo.pop(0)[1])
        out.append(task)
        done += task[0]
    return out + [t for _, t in todo]


def _now(task):
    task[1](lambda v: v)


def _kernel(zero_hbm, tab_hbm, x_hbm, lre_hbm, lim_hbm, bre_hbm, bim_hbm, cre_hbm, cim_hbm,
            ldt_hbm, dsk_hbm, q_hbm, k_hbm, v_hbm, tap_hbm, sk_hbm, sd_hbm,
            o_hbm,
            zero_s, tab, lre_v, lim_v, ldt_v, dsk_v, sd_v, tap_v,
            xb, braw, craw, qb, kb, vb, skb,
            par, wb16, wc, mf16, mi, bu, hb16, carry, ys, oa,
            kt, kf, st_u, st_k, st_i, vu16, vk16, pb0, pb1, ob,
            sem_p, sem_x, sem_b, sem_c, sem_g, sem_oa, sem_ob):
    x32, q32, k32, v32, wb, mf, hb, vu, vk = (
        r.bitcast(I32) for r in (xb, qb, kb, vb, wb16, mf16, hb16, vu16, vk16))
    pb16 = (pb0, pb1)
    pb = (pb0.bitcast(I32), pb1.bitcast(I32))

    def rows(ref, start, n=8):
        return ref[pl.ds(start, n), :]

    def hint(v, n):
        return v if isinstance(v, int) else pl.multiple_of(v, n)

    def view(ref, start, n=None):
        return ref.at[pl.ds(hint(start, 16), n or ref.shape[0]), :]

    small = [pltpu.make_async_copy(s, d, sem_p.at[n]) for n, (s, d) in enumerate((
        (zero_hbm, zero_s), (lre_hbm, lre_v), (lim_hbm, lim_v), (ldt_hbm, ldt_v),
        (dsk_hbm, dsk_v), (sd_hbm, sd_v), (tap_hbm, tap_v), (tab_hbm, tab)))]

    def x_dma(t, size):
        return [pltpu.make_async_copy(
            x_hbm.at[pl.ds(t, size), pl.ds(128 * n, 128)],
            xb.at[pl.ds(n * L + t, size), :], sem_x.at[t // UNIT, n]) for n in range(NG)]

    def b_dma(p):
        return [pltpu.make_async_copy(
            src.at[pl.ds(128 * p, 128), :], braw.at[pl.ds(D * c + 128 * p, 128), :],
            sem_b.at[2 * p + c]) for c, src in enumerate((bre_hbm, bim_hbm))]

    c_dma = [pltpu.make_async_copy(
        src.at[:, pl.ds(128 * p, 128)], craw.at[pl.ds(D * (NG * c + p), D), :],
        sem_c.at[NG * c + p]) for c, src in enumerate((cre_hbm, cim_hbm)) for p in range(NG)]

    def clamp(g):
        return min(g, NG - 1) if isinstance(g, int) else jnp.minimum(g, NG - 1)

    def col_dma(which, g):
        src, dst = ((k_hbm, kb), (v_hbm, vb), (q_hbm, qb))[which]
        return pltpu.make_async_copy(
            src.at[:, pl.ds(hint(128 * clamp(g), 128), 128)],
            dst.at[pl.ds(hint(L * g, L), L), :], sem_g.at[which, g])

    def sk_dma(g):
        t = hint(128 * g, 128)
        return pltpu.make_async_copy(
            sk_hbm.at[pl.ds(hint(128 * clamp(g), 128), 128), :], skb.at[pl.ds(t, 128), :],
            sem_g.at[3, g])

    def oa_dma(u):
        t = hint(u * UNIT, UNIT)
        return pltpu.make_async_copy(
            oa.at[pl.ds(t, UNIT), :], o_hbm.at[pl.ds(t, UNIT), pl.ds(0, D)], sem_oa.at[u])

    def ob_dma(g):
        return pltpu.make_async_copy(
            ob.at[pl.ds(hint(L * g, L), L), :],
            o_hbm.at[:, pl.ds(hint(D + 128 * g, 128), 128)], sem_ob.at[g])

    def start(ds):
        for d in ds:
            d.start()

    def wait(ds):
        for d in ds:
            d.wait()

    def prm(g, row):
        return rows(view(par, g * (P_ROWS * 8), P_ROWS * 8), row * 8)

    def bu_passes(u, slot, z=0):
        out = []
        xu, w = view(x32, u * (UNIT // 2), ((NG - 1) * L + UNIT) // 2), view(wb, z)
        for m in range(UNIT // MM):
            for n in range(2 * NG):
                acc = []
                for kk in range(NG):
                    def lhs(m=m, kk=kk):
                        t = (kk * L + m * MM) // 2
                        return [rows(xu, t + 8 * i) for i in range(MM // 16)]

                    def rhs(n=n, kk=kk):
                        return [rows(w, (n * NG + kk) * 64 + 8 * i) for i in range(8)]

                    def consume(d, m=m, n=n, kk=kk, acc=acc):
                        acc.append(d if kk == 0 else acc[-1] + d)
                        if kk == NG - 1:
                            for i in range(MM // 8):
                                seg, r = divmod(m * MM + 8 * i, R)
                                row = 9 * (seg % 2 * R + r) + seg // 2
                                bu[pl.ds((slot * 2 * NG + n) * BU_PART + row, 8, stride=9), :] = (
                                    acc[-1][8 * i:8 * i + 8])
                    out.append((lhs, rhs, consume))
        return out

    def scan_tasks(u, slot, z, steps=8):
        state = {}
        hu, cz = view(hb16, u * UNIT, (2 * NG - 1) * L + UNIT), view(carry, z)

        def b(p, ch, r):
            return tuple(rows(bu, (slot * 2 * NG + c * NG + p) * BU_PART + 9 * (ch * R + r))
                         for c in range(2))

        def step(mu, h, br):
            return (mu[0] * h[0] + br[0]) - mu[1] * h[1], (mu[0] * h[1] + br[1]) + mu[1] * h[0]

        def ends(p, r0, gate):
            mu, h = (gate(prm(p, P_MU)), prm(p, P_MU + 1)), state.get(p)
            for r in range(r0, r0 + steps):
                h = [b(p, ch, r) if r == 0 else step(mu, h[ch], b(p, ch, r)) for ch in range(2)]
            if r0 + steps == R:
                h = starts(p, h)
            state[p] = h
            carry[pl.ds(2 * NG * 8, 8), :] = (h[0][0] + h[0][1]) + (h[1][0] + h[1][1])
            return pltpu.bitcast(rows(cz, 2 * NG * 8), I32)

        def starts(p, e):
            last = lax.broadcasted_iota(I32, (8, 128), 0) == 7
            rho = (prm(p, P_RHO), prm(p, P_RHO + 1))
            pair = step(rho, e[0], e[1])
            a = tuple(pltpu.roll(jnp.where(last, rows(carry, (2 * p + c) * 8), pair[c]), 1, 0)
                      for c in range(2))
            for sh, row in ((1, P_RHO1), (2, P_RHO2), (4, P_RHO4)):
                a = step((prm(p, row), prm(p, row + 1)), tuple(pltpu.roll(c, sh, 0) for c in a), a)
            return [a, step(rho, a, e[0])]

        def run(p, r0, gate):
            mu, h = (gate(prm(p, P_MU)), prm(p, P_MU + 1)), state[p]
            for r in range(r0, r0 + steps):
                h = [step(mu, h[ch], b(p, ch, r)) for ch in range(2)]
                for c in range(2):
                    hu[pl.ds((c * NG + p) * L + 16 * r, 16), :] = _pack(h[0][c], h[1][c])
            state[p] = h
            if r0 + steps == R:
                for c in range(2):
                    carry[pl.ds((2 * p + c) * 8, 8), :] = h[1][c]
            return rows(view(hb, z, 8), 0)

        tasks = []
        for p in range(NG):
            tasks += [(16 * steps + (46 if r0 + steps == R else 0), lambda gate, p=p, r0=r0: ends(p, r0, gate))
                      for r0 in range(0, R, steps)]
            tasks += [(18 * steps, lambda gate, p=p, r0=r0: run(p, r0, gate)) for r0 in range(0, R, steps)]
        return tasks

    def y_passes(u, ns):
        out = []
        hu = view(hb, u * (UNIT // 2), ((2 * NG - 1) * L + UNIT) // 2)
        for n in ns:
            for m in range(UNIT // MM):
                acc = []
                for kk in range(2 * NG):
                    def lhs(m=m, kk=kk):
                        t = kk * (L // 2) + m * (MM // 2)
                        return [rows(hu, t + 8 * i) for i in range(MM // 16)]

                    def rhs(n=n, kk=kk):
                        return [rows(wc, (kk * NG + n) * 64 + 8 * i) for i in range(8)]

                    def consume(d, m=m, n=n, kk=kk, acc=acc):
                        acc.append(d if kk == 0 else acc[-1] + d)
                        if kk == 2 * NG - 1:
                            for i in range(MM // 8):
                                r, ch = divmod(m * (MM // 8) + i, 2)
                                ys[pl.ds(n * YS_ROWS + ch * (R + 1) + r, 8, stride=2 * (R + 1)), :] = (
                                    acc[-1][8 * i:8 * i + 8])
                    out.append((lhs, rhs, consume))
        return out

    def skip_task(u, n, z):
        def fn(gate):
            dsk = gate(prm(n, P_DSKIP))
            xu, ou = view(x32, u * (UNIT // 2) + n * (L // 2), UNIT // 2), view(oa, u * UNIT, UNIT)
            for i in range(UNIT // 16):
                xs = _unpack(rows(xu, 8 * i))
                for c in range(2):
                    t = 16 * i + 8 * c
                    y = rows(ys, n * YS_ROWS + (t // R) * (R + 1) + t % R)
                    ou[pl.ds(t, 8), pl.ds(128 * n, 128)] = y + xs[c] * dsk
            return pltpu.bitcast(view(oa, z + u * UNIT, 8)[:, pl.ds(128 * n, 128)], I32)
        return (3 * UNIT // 8, fn)

    def widen_tasks(g, z, pieces=2):
        def fn(i0, i1):
            kg = view(k32, g * (L // 2), L // 2)
            for i in range(i0, i1):
                lo, hi = _unpack(rows(kg, 8 * i))
                kf[pl.ds(KF_PAD + 16 * i, 8), :] = lo
                kf[pl.ds(KF_PAD + 16 * i + 8, 8), :] = hi
            return pltpu.bitcast(rows(view(kf, z), 16 * i0 + KF_PAD), I32)
        n = L // 16 // pieces
        return [(2 * n, lambda gate, i=i: fn(i * n, (i + 1) * n)) for i in range(pieces)]

    def transpose_tasks(g, z, pieces=4):
        def fn(c0, c1):
            for c in range(c0, c1):
                t = skb[pl.ds(hint(128 * g, 128), 128), pl.ds(128 * c, 128)]
                kt[pl.ds(64 * c, 64), :] = pltpu.bitcast(t.T, I32)
            return rows(view(kt, z), 64 * c0)
        n = L // 128 // pieces
        return [(8 * n, lambda gate, i=i: fn(i * n, (i + 1) * n)) for i in range(pieces)]

    def pass1(st, s, n0, u, z):
        for grp, pair in enumerate(_fwd1(n0, [_Signed(v) for v in u])):
            for c in range(2):
                st[pl.ds(((s * 4 + n0) * 8 + grp) * 16 + 8 * c, 8), :] = pair[c].get()
        return pltpu.bitcast(rows(view(st, z), (s * 4 + n0) * 128), I32)

    def u1_task(g, s, n0, z):
        def fn(gate):
            taps = [prm(g, P_TAP + t) for t in range(4)]
            taps[0] = gate(taps[0])
            u, kz, vg = [], view(kf, z), view(v32, g * (L // 2), L // 2)
            for m in range(8):
                t = 64 * (n0 + 4 * m) + 8 * s
                ks = rows(kz, KF_PAD + t) * taps[0]
                for lag in range(1, 4):
                    ks = ks + rows(kz, KF_PAD + t - lag) * taps[lag]
                v = _unpack(rows(vg, (t // 16) * 8))[s % 2]
                u.append(ks * v)
            return pass1(st_u, s, n0, u, z)
        return (72 + (54, 96, 80, 96)[n0], fn)

    def k1_task(g, s, n0, z):
        def fn(gate):
            u = [_unpack(rows(view(kt, z), 32 * (n0 + 4 * m) + 8 * (s // 2)))[s % 2] for m in range(8)]
            if s == 0 and n0 == 0:
                first = lax.broadcasted_iota(I32, (8, 128), 0) == 0
                u[0] = u[0] + jnp.where(first, prm(g, P_SSMD), 0.0)
            return pass1(st_k, s, n0, u, z)
        return (8 + (54, 96, 80, 96)[n0], fn)

    def pass2_task(st, dst16, dst, s, grps, z):
        def fn(gate):
            for grp in grps:
                zs = [tuple(_Signed(rows(view(st, z), ((s * 4 + n0) * 8 + grp) * 16 + 8 * c)) for c in range(2))
                      for n0 in range(4)]
                for k, pair in enumerate(_fwd2(grp, zs)):
                    dst16[pl.ds((4 * grp + k) * 128 + 16 * s, 16), :] = _pack(pair[0].get(), pair[1].get())
            return rows(view(dst, z), 4 * grps[0] * 64 + 8 * s)
        return (20 * len(grps), fn)

    def pass2_tasks(st, s, z):
        dst = (vu16, vu) if st is st_u else (vk16, vk)
        return [pass2_task(st, *dst, s, g, z) for g in ((0, 1, 2, 3), (4, 5, 6, 7))]

    def fwd_passes(grp, z):
        out = []
        for slot in range(4 * grp, 4 * grp + 4):
            got = {}
            for half in range(2):
                for which, src in enumerate((vu, vk)):
                    def lhs(slot=slot, half=half):
                        return [rows(mf, slot * 64 + 32 * half + 8 * i) for i in range(4)]

                    def rhs(slot=slot, src=src):
                        return [rows(view(src, z), slot * 64 + 8 * i) for i in range(8)]

                    def consume(d, slot=slot, half=half, which=which, got=got):
                        got[which] = d
                        if which == 0:
                            return
                        for i in range(4):
                            a = (got[0][16 * i:16 * i + 8], got[0][16 * i + 8:16 * i + 16])
                            b = (d[16 * i:16 * i + 8], d[16 * i + 8:16 * i + 16])
                            re, im = _cmul(a, b)
                            if slot == _REAL_SLOT and half == 0 and i == 0:
                                first = lax.broadcasted_iota(I32, (8, 128), 0) == 0
                                re = jnp.where(first, 0.5 * (a[0] * b[0]), re)
                                im = jnp.where(first, 0.5 * (a[1] * b[1]), im)
                            pb16[grp % 2][pl.ds(slot % 4 * 128 + 64 * half + 16 * i, 16), :] = _pack(re, im)
                    out.append((lhs, rhs, consume))
        return out

    def inv_passes(grp, z):
        out = []
        for half in range(2):
            got = []
            for slot in range(4 * grp, 4 * grp + 4):
                def lhs(slot=slot, half=half):
                    return [rows(mi, slot * 64 + 32 * half + 8 * i) for i in range(4)]

                def rhs(slot=slot):
                    return [rows(view(pb[grp % 2], z), slot % 4 * 64 + 8 * i) for i in range(8)]

                def consume(d, half=half, got=got):
                    got.append(d)
                    if len(got) < 4:
                        return
                    for i in range(4):
                        w = [(_Signed(t[16 * i:16 * i + 8]), _Signed(t[16 * i + 8:16 * i + 16])) for t in got]
                        for n0, pair in enumerate(_inv2(grp, w)):
                            for c in range(2):
                                at = (((4 * half + i) * 4 + n0) * 8 + grp) * 16 + 8 * c
                                st_i[pl.ds(at, 8), :] = pair[c].get()
                out.append((lhs, rhs, consume))
        return out

    def inv1_task(g, s, n0, z):
        def fn(gate):
            zs = [tuple(_Signed(rows(view(st_i, z), ((s * 4 + n0) * 8 + grp) * 16 + 8 * c)) for c in range(2))
                  for grp in range(8)]
            qg, og = view(q32, g * (L // 2), L // 2), view(ob, g * L, L)
            for m, y in enumerate(_inv1(n0, zs)):
                t = 64 * (n0 + 4 * m) + 8 * s
                qv = _unpack(rows(qg, (t // 16) * 8))[s % 2]
                og[pl.ds(t, 8), :] = qv * y.get()
            return pltpu.bitcast(rows(view(ob, z + g * L, L), 64 * n0 + 8 * s), I32)
        return (16 + (62, 104, 88, 104)[n0], fn)

    start(small)
    start(x_dma(0, UNIT))
    for p in range(NG):
        start(b_dma(p))
    start(x_dma(UNIT, UNIT) + x_dma(2 * UNIT, UNIT) + [sk_dma(0)] + c_dma)
    start([col_dma(0, 0)] + x_dma(LEAD * UNIT, L - LEAD * UNIT))
    for g in range(NG):
        start([col_dma(1, g), col_dma(2, g), sk_dma(g + 1), col_dma(0, g + 1)])
    wait(small)
    z = zero_s[0]
    z8 = pl.multiple_of(z, 16)
    sub = lax.broadcasted_iota(I32, (8, 128), 0)
    pred = sub + z >= 0

    def stack(ref):
        v = ref[...].astype(F32).reshape(1, D)
        return jnp.concatenate([v[:, 128 * g:128 * (g + 1)] for g in range(NG)]
                               + [v[:, :128]] * (8 - NG), axis=0)

    lre, lim = stack(lre_v), stack(lim_v)
    dt = jnp.exp(stack(ldt_v)).astype(BF16).astype(F32)
    mag, ang = jnp.exp(dt * lre), dt * lim
    lam = (mag * jnp.cos(ang), mag * jnp.sin(ang))
    scale = jnp.maximum(jnp.abs(lre), jnp.abs(lim))
    nre, nim = lre / scale, lim / scale
    den = (nre * nre + nim * nim) * scale
    coef = _cmul(((lam[0] - 1.0) / den, lam[1] / den), (nre, -nim))
    mu = (lam[0], -lam[1])
    rho = [mu]
    for _ in range(R.bit_length() + 2):
        rho.append(_cmul(rho[-1], rho[-1]))
    dsk, ssd = stack(dsk_v), stack(sd_v)
    taps = tap_v[...].astype(F32) * _FFT_SCALE
    for g in range(NG):
        def put(row, v):
            par[pl.ds((g * P_ROWS + row) * 8, 8), :] = v

        def lanes(v):
            return jnp.broadcast_to(v[g:g + 1], (8, 128))
        for c in range(2):
            put(P_MU + c, lanes(mu[c]))
            put(P_RHO + c, lanes(rho[-4][c]))
            for n, row in enumerate((P_RHO1, P_RHO2, P_RHO4)):
                put(row + c, jnp.where(sub >= 1 << n, lanes(rho[n - 3][c]), 0.0))
        for t in range(4):
            put(P_TAP + t, jnp.broadcast_to(taps[t:t + 1, 128 * g:128 * (g + 1)], (8, 128)))
        put(P_COEF, lanes(2.0 * coef[0]))
        put(P_COEF + 1, lanes(-2.0 * coef[0]))
        put(P_COEF + 2, lanes(2.0 * coef[1]))
        put(P_SSMD, lanes(ssd))
        put(P_DSKIP, lanes(dsk))
    for i in range(2 * NG):
        carry[pl.ds(8 * i, 8), :] = jnp.zeros((8, 128), F32)
    kf[pl.ds(0, KF_PAD), :] = jnp.zeros((KF_PAD, 128), F32)

    def matrix_task(slot):
        def fn(gate):
            if slot != _REAL_SLOT:
                c, s = tab[pl.ds(256 + slot, 1), :], tab[pl.ds(288 + slot, 1), :]
            for a in range(8):
                if slot == _REAL_SLOT:
                    re, im = rows(tab, 128 + 16 * a), rows(tab, 128 + 16 * a + 8)
                else:
                    br, bi = rows(tab, 16 * a), rows(tab, 16 * a + 8)
                    re, im = c * br - s * bi, s * br + c * bi
                mf16[pl.ds(slot * 128 + 16 * a, 16), :] = _pack(re, im)
            m = pltpu.bitcast(rows(view(mf, z8), slot * 64, 64), BF16)
            mi[pl.ds(slot * 64, 64), :] = pltpu.bitcast(m.T, I32)
            return rows(view(mi, z8), slot * 64)
        return (56, fn)

    def scale_b(p, kk):
        cr, ncr, ci = prm(p, P_COEF), prm(p, P_COEF + 1), prm(p, P_COEF + 2)
        br, bi = (braw[pl.ds(D * c + 128 * p, 128), pl.ds(128 * kk, 128)].T.astype(F32)
                  for c in range(2))
        for i in range(8):
            r0, r1 = br[16 * i:16 * i + 8], br[16 * i + 8:16 * i + 16]
            i0, i1 = bi[16 * i:16 * i + 8], bi[16 * i + 8:16 * i + 16]
            wb16[pl.ds((p * NG + kk) * 128 + 16 * i, 16), :] = _pack(
                cr * r0 - ci * i0, cr * r1 - ci * i1)
            wb16[pl.ds(((NG + p) * NG + kk) * 128 + 16 * i, 16), :] = _pack(
                ncr * i0 - ci * r0, ncr * i1 - ci * r1)
        return rows(view(wb, z8), ((NG + p) * NG + kk) * 64)

    def c_task(kk):
        def fn(gate):
            for n in range(NG):
                t = craw[pl.ds(kk * D + 128 * n, 128), :]
                wc[pl.ds((kk * NG + n) * 64, 64), :] = pltpu.bitcast(t.T, I32)
            return rows(view(wc, z8), kk * NG * 64)
        return (40, fn)

    first = bu_passes(0, 0, z8)
    first = [[q for i, q in enumerate(first) if (i // NG) % NG == p] for p in range(NG)]
    mats = [matrix_task(slot) for slot in range(32)]

    def scale_tasks(p):
        return [(144, lambda gate, kk=kk: scale_b(p, kk)) for kk in range(NG)]

    wait(x_dma(0, UNIT) + b_dma(0) + b_dma(1))
    for task in scale_tasks(0):
        _now(task)
    _weave(first[0], scale_tasks(1), pred)
    wait(b_dma(2) + b_dma(3))
    _weave(first[1] + first[2], scale_tasks(2) + scale_tasks(3), pred)
    wait(b_dma(4) + x_dma(UNIT, UNIT))
    _weave(first[3], scale_tasks(4), pred)
    second = bu_passes(1, 1)
    _weave(first[4] + second[:40], mats[:12], pred)
    _weave(second[40:], _mix(scan_tasks(0, 0, z8), mats[12:24]), pred)
    wait(x_dma(2 * UNIT, UNIT) + [sk_dma(0)] + c_dma)
    k_tasks = transpose_tasks(0, z8)
    for s in range(8):
        k_tasks += [k1_task(0, s, n0, z8) for n0 in range(4)] + pass2_tasks(st_k, s, z8)
    third = bu_passes(2, 0)
    _weave(third[:16], mats[24:28] + k_tasks[:4], pred)
    _weave(third[16:], _mix(_mix(scan_tasks(1, 1, z8), k_tasks[4:]),
                            mats[28:] + [c_task(kk) for kk in range(2 * NG)]), pred)
    wait([col_dma(0, 0)] + x_dma(LEAD * UNIT, L - LEAD * UNIT))
    for task in widen_tasks(0, z8):
        _now(task)

    def body(i, _):
        nxt = jnp.minimum(i + 1, NG - 1)
        wait([col_dma(1, i), col_dma(2, i), sk_dma(i + 1), col_dma(0, i + 1)])

        u_tasks, k1, k2 = [], transpose_tasks(i + 1, z8), []
        for s in range(8):
            u_tasks += [u1_task(i, s, n0, z8) for n0 in range(4)] + pass2_tasks(st_u, s, z8)
            k1 += [k1_task(nxt, s, n0, z8) for n0 in range(4)]
            k2 += pass2_tasks(st_k, s, z8)
        yp, bup = y_passes(i, range(NG)), bu_passes(i + LEAD, 0)
        skips = [skip_task(i, n, z8) for n in range(NG)]
        per_n = len(yp) // NG

        span = len(yp) - 8
        _weave(yp[:span], _spread(u_tasks, [(per_n * (n + 1) + 16) / span for n in range(NG - 1)],
                                  skips[:-1]), pred)
        _weave(yp[span:], k1[:2], pred)
        conv = fwd_passes(0, z8)
        for grp in range(1, 8):
            conv += fwd_passes(grp, z8) + inv_passes(grp - 1, z8)
        conv += bup[:8] + inv_passes(7, z8)
        _weave(conv[:16], k1[2:5] + skips[-1:], pred)
        start([oa_dma(i)])
        _weave(conv[16:184], _mix(scan_tasks(i + LEAD - 1, 0, z8), k1[5:16]), pred)
        _weave(conv[184:], k1[16:19], pred)
        _weave(bup[8:24], k1[19:22], pred)
        inv = [inv1_task(i, s, n0, z8) for s in range(8) for n0 in range(4)]
        _weave(bup[24:140], _mix(inv, k1[22:]), pred)
        start([ob_dma(i)])
        _weave(bup[140:], _mix(k2, widen_tasks(i + 1, z8, 8)), pred)
        return 0

    lax.fori_loop(0, NG, body, 0)

    yp = [q for u in range(NG, NG + LEAD) for q in y_passes(u, range(NG))]
    per_n = len(yp) // (NG * LEAD)
    skips = [skip_task(u, n, z8) for u in range(NG, NG + LEAD) for n in range(NG)]
    scan = scan_tasks(L // UNIT - 1, 0, z8)
    _weave(yp[:per_n + 16], scan[:8], pred)
    for n in range(1, NG * LEAD):
        extra = scan[8 + 3 * (n - 1):8 + 3 * n] if n < 5 else []
        _weave(yp[n * per_n + 16:(n + 1) * per_n + 16], skips[n - 1:n] + extra, pred)
        if n % NG == 0:
            start([oa_dma(NG + n // NG - 1)])
    _now(skips[-1])
    start([oa_dma(L // UNIT - 1)])
    wait([oa_dma(u) for u in range(NG + LEAD)] + [ob_dma(g) for g in range(NG)])


@jax.jit
def pallas_concat_heads__ssm_conv_s5__ssm_conv_h3__prompt_kernel(
    A_x: jax.Array,
    A_Lambda_re: jax.Array,
    A_Lambda_im: jax.Array,
    A_B_re: jax.Array,
    A_B_im: jax.Array,
    A_C_re: jax.Array,
    A_C_im: jax.Array,
    A_log_dt: jax.Array,
    A_Dskip: jax.Array,
    B_q: jax.Array,
    B_k: jax.Array,
    B_v: jax.Array,
    B_shift_k: jax.Array,
    B_ssm_k: jax.Array,
    B_ssm_D: jax.Array,
):
    assert A_x.shape == (1, L, D) and B_shift_k.shape == (D, 4)
    vmem = pltpu.VMEM
    dma = pltpu.SemaphoreType.DMA
    scratch = [
        pltpu.SMEM((1,), I32),
        vmem(_TABLES.shape, F32),
        vmem((D,), BF16), vmem((D,), BF16), vmem((D,), BF16), vmem((D,), BF16), vmem((D,), BF16),
        vmem((4, D), BF16),
        vmem((NG * L, 128), BF16),
        vmem((2 * D, D), BF16),
        vmem((2 * NG * D, 128), BF16),
        vmem((NG * L, 128), BF16),
        vmem(((NG + 1) * L, 128), BF16),
        vmem((NG * L, 128), BF16),
        vmem((D + 128, L), BF16),
        vmem((NG * P_ROWS * 8, 128), F32),
        vmem((2 * NG * D, 128), BF16),
        vmem((2 * NG * NG * 64, 128), I32),
        vmem((32 * 128, 128), BF16),
        vmem((32 * 64, 128), I32),
        vmem((2 * 2 * NG * BU_PART, 128), F32),
        vmem((2 * NG * L, 128), BF16),
        vmem((3 * NG * 8, 128), F32),
        vmem((NG * YS_ROWS, 128), F32),
        vmem((L, D), F32),
        vmem((L // 2, 128), I32),
        vmem((KF_PAD + L, 128), F32),
        vmem((2 * L, 128), F32),
        vmem((2 * L, 128), F32),
        vmem((2 * L, 128), F32),
        vmem((32 * 128, 128), BF16),
        vmem((32 * 128, 128), BF16),
        vmem((4 * 128, 128), BF16),
        vmem((4 * 128, 128), BF16),
        vmem((NG * L, 128), F32),
        dma((8,)), dma((L // UNIT, NG)), dma((2 * NG,)), dma((2 * NG,)), dma((4, NG + 1)),
        dma((L // UNIT,)), dma((NG,)),
    ]
    out = pl.pallas_call(
        _kernel,
        out_shape=jax.ShapeDtypeStruct((L, 2 * D), F32),
        in_specs=[pl.BlockSpec(memory_space=pl.ANY)] * 17,
        out_specs=pl.BlockSpec(memory_space=pl.ANY),
        scratch_shapes=scratch,
        compiler_params=pltpu.CompilerParams(vmem_limit_bytes=100 * 1024 * 1024),
        name="s5_h3",
    )(_ZERO, _TABLES, A_x.reshape(L, D), A_Lambda_re, A_Lambda_im, A_B_re, A_B_im, A_C_re, A_C_im,
      A_log_dt, A_Dskip, B_q.reshape(L, D), B_k.reshape(L, D), B_v.reshape(L, D),
      B_shift_k.T, B_ssm_k, B_ssm_D)
    return out.reshape(1, L, 2 * D)
```

```python
import math

import jax
import jax.numpy as jnp
import numpy as np
from jax import lax
from jax.experimental import pallas as pl
from jax.experimental.pallas import tpu as pltpu

F32, BF16, I32 = jnp.float32, jnp.bfloat16, jnp.int32

L = 2048
D = 640
NG = D // 128
UNIT = 256
SEG = 16
R = UNIT // SEG
LEAD = L // UNIT - NG
MM = 64
BU_PART = 9 * 2 * R
YS_ROWS = SEG * (R + 1)
KF_PAD = 8


class _Signed:
    def __init__(self, v, neg=False):
        self.v, self.neg = v, neg

    def __neg__(self):
        return _Signed(self.v, not self.neg)

    def __add__(self, o):
        if self.neg == o.neg:
            return _Signed(self.v + o.v, self.neg)
        return _Signed(o.v - self.v if self.neg else self.v - o.v)

    def __sub__(self, o):
        return self + (-o)

    def __mul__(self, c):
        return _Signed(self.v * np.float32(-c if self.neg else c))

    def get(self):
        return -self.v if self.neg else self.v


def _rot(re, im, num, den):
    num %= den
    h = math.sqrt(0.5)
    if num == 0:
        return re, im
    if 4 * num == den:
        return -im, re
    if 4 * num == 3 * den:
        return im, -re
    if 8 * num == den:
        return (re - im) * h, (re + im) * h
    if 8 * num == 3 * den:
        return (re + im) * (-h), (re - im) * h
    if 8 * num == 5 * den:
        return (im - re) * h, (re + im) * (-h)
    if 8 * num == 7 * den:
        return (re + im) * h, (im - re) * h
    c = math.cos(2 * math.pi * num / den)
    s = math.sin(2 * math.pi * num / den)
    return re * c - im * s, re * s + im * c


def _dft4(z, sign):
    (r0, i0), (r1, i1), (r2, i2), (r3, i3) = z
    ar, ai, br, bi = r0 + r2, i0 + i2, r0 - r2, i0 - i2
    cr, ci, dr, di = r1 + r3, i1 + i3, r1 - r3, i1 - i3
    plus, minus = (br - di, bi + dr), (br + di, bi - dr)
    if sign < 0:
        plus, minus = minus, plus
    return [(ar + cr, ai + ci), plus, (ar - cr, ai - ci), minus], [ai.v, ci.v]


def _fwd1(n0, u):
    a, b = u[:4], u[4:]
    r = [_rot(a[m], b[m], n0 + 4 * m, 64) for m in range(4)]
    z, halves = _dft4(r, 1)
    out = [_rot(*z[k], n0 * k, 16) for k in range(4)]
    s2 = [a[m] + b[m] for m in range(4)]
    d2 = [a[m] - b[m] for m in range(4)]
    p = _rot(d2[0], d2[2], n0, 32)
    q = _rot(d2[1], d2[3], n0 + 4, 32)
    out.append((p[0] + q[0], p[1] + q[1]))
    out.append(_rot(p[0] - q[0], p[1] - q[1], n0, 8))
    s3 = [s2[0] + s2[2], s2[1] + s2[3]]
    d3 = [s2[0] - s2[2], s2[1] - s2[3]]
    out.append(_rot(d3[0], d3[1], n0, 16))
    out.append((s3[0] + s3[1], s3[0] - s3[1]))
    return out, halves


def _fwd2(grp, z):
    if grp < 7:
        return _dft4(z, 1)[0]
    s4 = [t[0] for t in z]
    d4 = [t[1] for t in z]
    p = (d4[0], d4[2])
    q = _rot(d4[1], d4[3], 1, 8)
    s5 = [s4[0] + s4[2], s4[1] + s4[3]]
    return [
        (s5[0] + s5[1], s5[0] - s5[1]),
        (s4[0] - s4[2], s4[1] - s4[3]),
        (p[0] + q[0], p[1] + q[1]),
        (p[0] - q[0], p[1] - q[1]),
    ]


def _inv2(grp, w):
    if grp < 7:
        return _dft4(w, -1)[0]
    s5 = [w[0][0] + w[0][1], w[0][0] - w[0][1]]
    s4 = [s5[0] + w[1][0], s5[1] + w[1][1], s5[0] - w[1][0], s5[1] - w[1][1]]
    p = (w[2][0] + w[3][0], w[2][1] + w[3][1])
    q = _rot(w[2][0] - w[3][0], w[2][1] - w[3][1], -1, 8)
    d4 = [p[0], q[0], p[1], q[1]]
    return [(s4[n], d4[n]) for n in range(4)]


def _inv1(n0, z):
    t, _ = _dft4([_rot(*z[k], -n0 * k, 16) for k in range(4)], -1)
    ab = [_rot(*t[m], -(n0 + 4 * m), 64) for m in range(4)]
    e = _rot(*z[5], -n0, 8)
    p = _rot(z[4][0] + e[0], z[4][1] + e[1], -n0, 32)
    q = _rot(z[4][0] - e[0], z[4][1] - e[1], -(n0 + 4), 32)
    d2 = [p[0], q[0], p[1], q[1]]
    d3 = _rot(*z[6], -n0, 16)
    s3 = [z[7][0] + z[7][1], z[7][0] - z[7][1]]
    s2 = [s3[0] + d3[0], s3[1] + d3[1], s3[0] - d3[0], s3[1] - d3[1]]
    e2 = [s2[m] + d2[m] for m in range(4)]
    a = [ab[m][0] + e2[m] for m in range(4)]
    b = [ab[m][1] + (s2[m] - d2[m]) for m in range(4)]
    return a + b, [t[0][0].v + t[1][1].v, e2[0].v]


_F1 = [4 * (g + 4 * k) + 1 for g in range(4) for k in range(4)]
_F1 += [2 * (4 * (g + 2 * k) + 1) for g in range(2) for k in range(4)]
_F1 += [4 * (4 * k + 1) for k in range(4)]
_F1 += [0, 16, 8, 40]
_REAL_SLOT = 28


def _dft_tables():
    kap = np.arange(128)
    j = 8 * (kap // 16) + kap % 8
    part = (kap // 8) % 2
    pr, pc, jr, jc = part[:, None], part[None, :], j[:, None], j[None, :]
    lo = 2 * np.pi * jr * jc / 64
    base = np.where(pr == pc, np.cos(lo), np.where(pr == 0, -np.sin(lo), np.sin(lo)))
    hi = 2 * np.pi * (32 + 64 * (jr - 32)) * jc / 4096
    v0 = np.where(pr == 0, np.cos(lo), np.where(jr == 0, np.cos(np.pi * jc), np.sin(lo)))
    v32 = np.where(pr == 0, np.cos(hi), np.sin(hi))
    real = np.where(jr < 32, np.where(pc == 0, v0, 0.0), np.where(pc == 1, v32, 0.0))
    th = 2 * np.pi * np.outer(np.array(_F1), j) / 4096
    zeros = np.zeros((8, 128))
    return np.concatenate([base, real, np.cos(th), np.sin(th), zeros]).astype(np.float32)


_TABLES = _dft_tables()
_FFT_SCALE = 2.0 ** -11

(P_MU, P_RHO, P_RHO1, P_RHO2, P_RHO4, P_TAP, P_SSMD, P_DSKIP, P_COEF, P_ROWS) = (
    0, 2, 4, 6, 8, 10, 14, 15, 16, 20)
S_SMALL, S_B, S_C, S_COL = 0, 7, 7 + 2 * NG, 7 + 4 * NG
S_X = S_COL + 4 * (NG + 1)
S_END = S_X + L // UNIT * NG


def _cmul(a, b):
    return a[0] * b[0] - a[1] * b[1], a[0] * b[1] + a[1] * b[0]


def _pack(lo, hi):
    return jnp.concatenate([lo, hi], axis=0).astype(BF16)


def _unpack(w):
    v = pltpu.bitcast(w, BF16).astype(F32)
    return v[:8], v[8:]


CFG = dict(scan=24, u=24, k1=0, p2=0, inv=0, skip=24, tail=3, kconv=10, steps=2, p2n=4, wid=(216, 340),
           early=30, pos=1.0, kwin=(100, 216), tr=(40, 88), scanw=(0, 184))


class _Gate:
    def __init__(self, pred=None, seen=()):
        self.pred, self.seen = pred, seen

    def value(self, v, lag):
        return jnp.where(self.pred, v, self.seen[-lag]) if 0 < lag <= len(self.seen) else v

    def loads(self, ref, lag):
        if 0 < lag <= len(self.seen):
            v = self.seen[-lag] if ref.dtype == F32 else pltpu.bitcast(self.seen[-lag], I32)
            ref[pl.ds(ref.shape[0] - 8, 8), :] = v


def _weave(passes, plan, pred):
    at = [[] for _ in range(len(passes) + 1)]
    for tasks, lo, hi in plan:
        total, done = sum(sum(c) for c, _ in tasks) or 1, 0.0
        for costs, fn in tasks:
            where = []
            for cost in costs:
                where.append(int(lo + (done + CFG["pos"] * cost) / total * (hi - lo)))
                done += cost
            at[where[0]].append((fn, where))
    seen, ties = [], [[] for _ in at]
    for i, fns in enumerate(at):
        for fn, where in fns:
            for w, tie in zip(where, fn(_Gate(pred, seen)) or ()):
                ties[w].append(tie)
        if i == len(passes):
            break
        lhs, rhs, consume = passes[i]
        w = rhs()
        for tie in ties[i]:
            w[-1] = jnp.where(pred, w[-1], tie if tie.dtype == I32 else pltpu.bitcast(tie, I32))
        a = pltpu.bitcast(jnp.concatenate(lhs(), axis=0), BF16)
        b = pltpu.bitcast(jnp.concatenate(w, axis=0), BF16)
        d = jnp.dot(a, b, preferred_element_type=F32)
        seen.append(d[-8:])
        consume(d)


def _now(tasks):
    for _, fn in tasks:
        fn(_Gate())


def _kernel(tab_hbm, x_hbm, lre_hbm, lim_hbm, bre_hbm, bim_hbm, cre_hbm, cim_hbm,
            ldt_hbm, dsk_hbm, q_hbm, k_hbm, v_hbm, tap_hbm, sk_hbm, sd_hbm,
            o_hbm,
            tab, lre_v, lim_v, ldt_v, dsk_v, sd_v, tap_v,
            xb, braw, craw, qb, kb, vb, skb,
            par, wb16, wc, mf16, mi, bu, hb16, carry, ys, oa,
            kt, kf, st_u, st_k, st_i, vu16, vk16, pb0, pb1, ob,
            sem, sem_oa, sem_ob):
    x32, q32, k32, v32, wb, mf, hb, vu, vk = (
        r.bitcast(I32) for r in (xb, qb, kb, vb, wb16, mf16, hb16, vu16, vk16))
    pb16 = (pb0, pb1)
    pb = (pb0.bitcast(I32), pb1.bitcast(I32))

    def rows(ref, start, n=8):
        return ref[pl.ds(start, n), :]

    def hint(v, n):
        return v if isinstance(v, int) else pl.multiple_of(v, n)

    def view(ref, start, n=None):
        return ref.at[pl.ds(hint(start, 16), n or ref.shape[0]), :]

    small = [pltpu.make_async_copy(s, d, sem.at[S_SMALL + n]) for n, (s, d) in enumerate((
        (lre_hbm, lre_v), (lim_hbm, lim_v), (ldt_hbm, ldt_v),
        (dsk_hbm, dsk_v), (sd_hbm, sd_v), (tap_hbm, tap_v), (tab_hbm, tab)))]

    def x_dma(u):
        return [pltpu.make_async_copy(
            x_hbm.at[pl.ds(hint(u * UNIT, UNIT), UNIT), pl.ds(128 * n, 128)],
            xb.at[pl.ds(hint(n * L + u * UNIT, UNIT), UNIT), :], sem.at[S_X + u * NG + n])
            for n in range(NG)]

    def b_dma(p):
        return [pltpu.make_async_copy(
            src.at[pl.ds(128 * p, 128), :], braw.at[pl.ds(D * c + 128 * p, 128), :],
            sem.at[S_B + 2 * p + c]) for c, src in enumerate((bre_hbm, bim_hbm))]

    c_dma = [pltpu.make_async_copy(
        src.at[:, pl.ds(128 * p, 128)], craw.at[pl.ds(D * (NG * c + p), D), :],
        sem.at[S_C + NG * c + p]) for c, src in enumerate((cre_hbm, cim_hbm)) for p in range(NG)]

    def clamp(g):
        return min(g, NG - 1) if isinstance(g, int) else jnp.minimum(g, NG - 1)

    def col_dma(which, g):
        src, dst = ((k_hbm, kb), (v_hbm, vb), (q_hbm, qb))[which]
        return pltpu.make_async_copy(
            src.at[:, pl.ds(hint(128 * clamp(g), 128), 128)],
            dst.at[pl.ds(hint(L * g, L), L), :], sem.at[S_COL + which * (NG + 1) + g])

    def sk_dma(g):
        t = hint(128 * g, 128)
        return pltpu.make_async_copy(
            sk_hbm.at[pl.ds(hint(128 * clamp(g), 128), 128), :], skb.at[pl.ds(t, 128), :],
            sem.at[S_COL + 3 * (NG + 1) + g])

    def oa_dma(u):
        t = hint(u * UNIT, UNIT)
        return pltpu.make_async_copy(
            oa.at[pl.ds(t, UNIT), :], o_hbm.at[pl.ds(t, UNIT), pl.ds(0, D)], sem_oa.at[u])

    def ob_dma(g):
        return pltpu.make_async_copy(
            ob.at[pl.ds(hint(L * g, L), L), :],
            o_hbm.at[:, pl.ds(hint(D + 128 * g, 128), 128)], sem_ob.at[g])

    def start(ds):
        for d in ds:
            d.start()

    def wait(ds):
        for d in ds:
            d.wait()

    def prm(g, row):
        return rows(view(par, g * (P_ROWS * 8), P_ROWS * 8), row * 8)

    def bu_passes(u, slot, z=0):
        out = []
        xu, w = view(x32, u * (UNIT // 2), ((NG - 1) * L + UNIT) // 2), view(wb, z)
        for m in range(UNIT // MM):
            for n in range(2 * NG):
                acc = []
                for kk in range(NG):
                    def lhs(m=m, kk=kk):
                        t = (kk * L + m * MM) // 2
                        return [rows(xu, t + 8 * i) for i in range(MM // 16)]

                    def rhs(n=n, kk=kk):
                        return [rows(w, (n * NG + kk) * 64 + 8 * i) for i in range(8)]

                    def consume(d, m=m, n=n, kk=kk, acc=acc):
                        acc.append(d if kk == 0 else acc[-1] + d)
                        if kk == NG - 1:
                            for i in range(MM // 8):
                                seg, r = divmod(m * MM + 8 * i, R)
                                row = 9 * (seg % 2 * R + r) + seg // 2
                                bu[pl.ds((slot * 2 * NG + n) * BU_PART + row, 8, stride=9), :] = (
                                    acc[-1][8 * i:8 * i + 8])
                    out.append((lhs, rhs, consume))
        return out

    def scan_tasks(u, slot, z):
        steps = CFG["steps"]
        state = {}
        hu = view(hb16, u * UNIT, (2 * NG - 1) * L + UNIT)

        def b(p, ch, r):
            return tuple(rows(bu, (slot * 2 * NG + c * NG + p) * BU_PART + 9 * (ch * R + r))
                         for c in range(2))

        def step(mu, h, br):
            return (mu[0] * h[0] + br[0]) - mu[1] * h[1], (mu[0] * h[1] + br[1]) + mu[1] * h[0]

        def ends(p, gate):
            mu, ties = (gate.value(prm(p, P_MU), CFG["scan"]), prm(p, P_MU + 1)), []
            h = [b(p, ch, 0) for ch in range(2)]
            for r in range(1, R):
                h = [step(mu, h[ch], b(p, ch, r)) for ch in range(2)]
                if r % steps == 0:
                    ties.append(h[r // steps % 2][0])
            state[p] = starts(p, h)
            return ties + [state[p][1][0]]

        def starts(p, e):
            last = lax.broadcasted_iota(I32, (8, 128), 0) == 7
            rho = (prm(p, P_RHO), prm(p, P_RHO + 1))
            pair = step(rho, e[0], e[1])
            a = tuple(pltpu.roll(jnp.where(last, rows(carry, (2 * p + c) * 8), pair[c]), 1, 0)
                      for c in range(2))
            for sh, row in ((1, P_RHO1), (2, P_RHO2), (4, P_RHO4)):
                a = step((prm(p, row), prm(p, row + 1)), tuple(pltpu.roll(c, sh, 0) for c in a), a)
            return [a, step(rho, a, e[0])]

        def run(p, r0, gate):
            if r0 == 0:
                state["mu"] = (prm(p, P_MU), prm(p, P_MU + 1))
            mu, h = (gate.value(state["mu"][0], CFG["scan"]), state["mu"][1]), state[p]
            for r in range(r0, r0 + steps):
                h = [step(mu, h[ch], b(p, ch, r)) for ch in range(2)]
                for c in range(2):
                    hu[pl.ds((c * NG + p) * L + 16 * r, 16), :] = _pack(h[0][c], h[1][c])
            state[p] = h
            if r0 + steps == R:
                for c in range(2):
                    carry[pl.ds((2 * p + c) * 8, 8), :] = h[1][c]
            return [rows(view(hb, z, 8), 0)]

        tasks = []
        for p in range(NG):
            tasks.append(([16 * steps] * ((R - 1) // steps) + [46 + 16 * steps],
                          lambda gate, p=p: ends(p, gate)))
            tasks += [([18 * steps], lambda gate, p=p, r0=r0: run(p, r0, gate))
                      for r0 in range(0, R, steps)]
        return tasks

    def y_passes(u, ns):
        out = []
        hu = view(hb, u * (UNIT // 2), ((2 * NG - 1) * L + UNIT) // 2)
        for n in ns:
            for m in range(UNIT // MM):
                acc = []
                for kk in range(2 * NG):
                    def lhs(m=m, kk=kk):
                        t = kk * (L // 2) + m * (MM // 2)
                        return [rows(hu, t + 8 * i) for i in range(MM // 16)]

                    def rhs(n=n, kk=kk):
                        return [rows(wc, (kk * NG + n) * 64 + 8 * i) for i in range(8)]

                    def consume(d, m=m, n=n, kk=kk, acc=acc):
                        acc.append(d if kk == 0 else acc[-1] + d)
                        if kk == 2 * NG - 1:
                            for i in range(MM // 8):
                                r, ch = divmod(m * (MM // 8) + i, 2)
                                ys[pl.ds(n * YS_ROWS + ch * (R + 1) + r, 8, stride=2 * (R + 1)), :] = (
                                    acc[-1][8 * i:8 * i + 8])
                    out.append((lhs, rhs, consume))
        return out

    def skip_task(u, n, z):
        def fn(gate):
            dsk = gate.value(prm(n, P_DSKIP), CFG["skip"])
            xu, ou = view(x32, u * (UNIT // 2) + n * (L // 2), UNIT // 2), view(oa, u * UNIT, UNIT)
            ties = []
            for i in range(UNIT // 16):
                xs = _unpack(rows(xu, 8 * i))
                for c in range(2):
                    t = 16 * i + 8 * c
                    y = rows(ys, n * YS_ROWS + (t // R) * (R + 1) + t % R)
                    ou[pl.ds(t, 8), pl.ds(128 * n, 128)] = y + xs[c] * dsk
                if i % 4 == 3:
                    ties.append(view(oa, z + u * UNIT, 8)[:, pl.ds(128 * n, 128)])
            return ties
        return ([24] * (UNIT // 64), fn)

    def widen_tasks(g, z, pieces=2):
        def fn(i0, i1):
            kg = view(k32, g * (L // 2), L // 2)
            for i in range(i0, i1):
                lo, hi = _unpack(rows(kg, 8 * i))
                kf[pl.ds(KF_PAD + 16 * i, 8), :] = lo
                kf[pl.ds(KF_PAD + 16 * i + 8, 8), :] = hi
            return [rows(view(kf, z), 16 * i0 + KF_PAD)]
        n = L // 16 // pieces
        return [([2 * n], lambda gate, i=i: fn(i * n, (i + 1) * n)) for i in range(pieces)]

    def transpose_tasks(g, z, pieces=8):
        def fn(c0, c1):
            for c in range(c0, c1):
                t = skb[pl.ds(hint(128 * g, 128), 128), pl.ds(128 * c, 128)]
                kt[pl.ds(64 * c, 64), :] = pltpu.bitcast(t.T, I32)
            return [rows(view(kt, z), 64 * c0)]
        n = L // 128 // pieces
        return [([8 * n], lambda gate, i=i: fn(i * n, (i + 1) * n)) for i in range(pieces)]

    def pass1(st, s, n0, u, z):
        pairs, ties = _fwd1(n0, [_Signed(v) for v in u])
        for grp, pair in enumerate(pairs):
            for c in range(2):
                st[pl.ds(((s * 4 + n0) * 8 + grp) * 16 + 8 * c, 8), :] = pair[c].get()
            if grp % 4 == 3:
                ties.append(rows(view(st, z), (s * 4 + n0) * 128))
        return ties

    def u1_task(g, s, n0, z):
        def fn(gate):
            taps = [prm(g, P_TAP + t) for t in range(4)]
            taps[0] = gate.value(taps[0], CFG["u"])
            u, kz, vg = [], view(kf, z), view(v32, g * (L // 2), L // 2)
            for m in range(8):
                t = 64 * (n0 + 4 * m) + 8 * s
                ks = rows(kz, KF_PAD + t) * taps[0]
                for lag in range(1, 4):
                    ks = ks + rows(kz, KF_PAD + t - lag) * taps[lag]
                v = _unpack(rows(vg, (t // 16) * 8))[s % 2]
                u.append(ks * v)
            return pass1(st_u, s, n0, u, z)
        rest = ((54, 96, 80, 96)[n0] - 8) // 2
        return ([40, 40, rest, rest], fn)

    def k1_task(g, s, n0, z):
        def fn(gate):
            gate.loads(kt, CFG["k1"])
            u = [_unpack(rows(view(kt, z), 32 * (n0 + 4 * m) + 8 * (s // 2)))[s % 2] for m in range(8)]
            if s == 0 and n0 == 0:
                first = lax.broadcasted_iota(I32, (8, 128), 0) == 0
                u[0] = u[0] + jnp.where(first, prm(g, P_SSMD), 0.0)
            return pass1(st_k, s, n0, u, z)[2:]
        half = (54, 96, 80, 96)[n0] // 2
        return ([half + 12, half - 4], fn)

    def pass2_task(st, dst16, dst, s, grps, z):
        def fn(gate):
            gate.loads(st, CFG["p2"])
            for grp in grps:
                zs = [tuple(_Signed(rows(view(st, z), ((s * 4 + n0) * 8 + grp) * 16 + 8 * c)) for c in range(2))
                      for n0 in range(4)]
                for k, pair in enumerate(_fwd2(grp, zs)):
                    dst16[pl.ds((4 * grp + k) * 128 + 16 * s, 16), :] = _pack(pair[0].get(), pair[1].get())
            return [rows(view(dst, z), 4 * grps[0] * 64 + 8 * s)]
        return ([20 * len(grps)], fn)

    def pass2_tasks(st, s, z):
        dst = (vu16, vu) if st is st_u else (vk16, vk)
        return [pass2_task(st, *dst, s, g, z) for g in np.arange(8).reshape(CFG["p2n"], -1).tolist()]

    def fwd_passes(grp, z):
        out = []
        for slot in range(4 * grp, 4 * grp + 4):
            got = {}
            for half in range(2):
                for which, src in enumerate((vu, vk)):
                    def lhs(slot=slot, half=half):
                        return [rows(mf, slot * 64 + 32 * half + 8 * i) for i in range(4)]

                    def rhs(slot=slot, src=src):
                        return [rows(view(src, z), slot * 64 + 8 * i) for i in range(8)]

                    def consume(d, slot=slot, half=half, which=which, got=got):
                        got[which] = d
                        if which == 0:
                            return
                        for i in range(4):
                            a = (got[0][16 * i:16 * i + 8], got[0][16 * i + 8:16 * i + 16])
                            b = (d[16 * i:16 * i + 8], d[16 * i + 8:16 * i + 16])
                            re, im = _cmul(a, b)
                            if slot == _REAL_SLOT and half == 0 and i == 0:
                                first = lax.broadcasted_iota(I32, (8, 128), 0) == 0
                                re = jnp.where(first, 0.5 * (a[0] * b[0]), re)
                                im = jnp.where(first, 0.5 * (a[1] * b[1]), im)
                            pb16[grp % 2][pl.ds(slot % 4 * 128 + 64 * half + 16 * i, 16), :] = _pack(re, im)
                    out.append((lhs, rhs, consume))
        return out

    def inv_passes(grp, z):
        out = []
        for half in range(2):
            got = []
            for slot in range(4 * grp, 4 * grp + 4):
                def lhs(slot=slot, half=half):
                    return [rows(mi, slot * 64 + 32 * half + 8 * i) for i in range(4)]

                def rhs(slot=slot):
                    return [rows(view(pb[grp % 2], z), slot % 4 * 64 + 8 * i) for i in range(8)]

                def consume(d, half=half, got=got):
                    got.append(d)
                    if len(got) < 4:
                        return
                    for i in range(4):
                        w = [(_Signed(t[16 * i:16 * i + 8]), _Signed(t[16 * i + 8:16 * i + 16])) for t in got]
                        for n0, pair in enumerate(_inv2(grp, w)):
                            for c in range(2):
                                at = (((4 * half + i) * 4 + n0) * 8 + grp) * 16 + 8 * c
                                st_i[pl.ds(at, 8), :] = pair[c].get()
                out.append((lhs, rhs, consume))
        return out

    def inv1_task(g, s, n0, z):
        def fn(gate):
            gate.loads(st_i, CFG["inv"])
            zs = [tuple(_Signed(rows(view(st_i, z), ((s * 4 + n0) * 8 + grp) * 16 + 8 * c)) for c in range(2))
                  for grp in range(8)]
            qg, og = view(q32, g * (L // 2), L // 2), view(ob, g * L, L)
            ys8, ties = _inv1(n0, zs)
            for m in (0, 4, 2, 6, 1, 5, 3, 7):
                t = 64 * (n0 + 4 * m) + 8 * s
                qv = _unpack(rows(qg, (t // 16) * 8))[s % 2]
                og[pl.ds(t, 8), :] = qv * ys8[m].get()
                if m in (6, 7):
                    ties.append(rows(view(ob, z + g * L, L), 64 * n0 + 8 * s))
            return ties
        quarter = (16 + (62, 104, 88, 104)[n0]) // 4
        return ([quarter, quarter - 8, quarter + 4, quarter + 4], fn)

    start(small)
    start(x_dma(0))
    for p in range(NG):
        start(b_dma(p))
    start(x_dma(1) + x_dma(2) + [sk_dma(0)] + c_dma)
    start([col_dma(0, 0), col_dma(1, 0)])
    for g in range(NG):
        start([col_dma(2, g), sk_dma(g + 1), col_dma(0, g + 1), col_dma(1, g + 1)] + x_dma(g + LEAD))
    wait(small)
    zeros = rows(tab, 320).astype(I32)
    z8 = pl.multiple_of(zeros[0, 0], 16)
    sub = lax.broadcasted_iota(I32, (8, 128), 0)
    pred = zeros == 0

    def stack(ref):
        v = ref[...].astype(F32).reshape(1, D)
        return jnp.concatenate([v[:, 128 * g:128 * (g + 1)] for g in range(NG)]
                               + [v[:, :128]] * (8 - NG), axis=0)

    lre, lim = stack(lre_v), stack(lim_v)
    dt = jnp.exp(stack(ldt_v)).astype(BF16).astype(F32)
    mag, ang = jnp.exp(dt * lre), dt * lim
    lam = (mag * jnp.cos(ang), mag * jnp.sin(ang))
    scale = jnp.maximum(jnp.abs(lre), jnp.abs(lim))
    nre, nim = lre / scale, lim / scale
    den = (nre * nre + nim * nim) * scale
    coef = _cmul(((lam[0] - 1.0) / den, lam[1] / den), (nre, -nim))
    mu = (lam[0], -lam[1])
    rho = [mu]
    for _ in range(R.bit_length() + 2):
        rho.append(_cmul(rho[-1], rho[-1]))
    dsk, ssd = stack(dsk_v), stack(sd_v)
    taps = tap_v[...].astype(F32) * _FFT_SCALE
    for g in range(NG):
        def put(row, v):
            par[pl.ds((g * P_ROWS + row) * 8, 8), :] = v

        def lanes(v):
            return jnp.broadcast_to(v[g:g + 1], (8, 128))
        for c in range(2):
            put(P_MU + c, lanes(mu[c]))
            put(P_RHO + c, lanes(rho[-4][c]))
            for n, row in enumerate((P_RHO1, P_RHO2, P_RHO4)):
                put(row + c, jnp.where(sub >= 1 << n, lanes(rho[n - 3][c]), 0.0))
        for t in range(4):
            put(P_TAP + t, jnp.broadcast_to(taps[t:t + 1, 128 * g:128 * (g + 1)], (8, 128)))
        put(P_COEF, lanes(2.0 * coef[0]))
        put(P_COEF + 1, lanes(-2.0 * coef[0]))
        put(P_COEF + 2, lanes(2.0 * coef[1]))
        put(P_SSMD, lanes(ssd))
        put(P_DSKIP, lanes(dsk))
    for i in range(2 * NG):
        carry[pl.ds(8 * i, 8), :] = jnp.zeros((8, 128), F32)
    kf[pl.ds(0, KF_PAD), :] = jnp.zeros((KF_PAD, 128), F32)

    def matrix_task(slot):
        def fn(gate):
            if slot != _REAL_SLOT:
                c, s = tab[pl.ds(256 + slot, 1), :], tab[pl.ds(288 + slot, 1), :]
            for a in range(8):
                if slot == _REAL_SLOT:
                    re, im = rows(tab, 128 + 16 * a), rows(tab, 128 + 16 * a + 8)
                else:
                    br, bi = rows(tab, 16 * a), rows(tab, 16 * a + 8)
                    re, im = c * br - s * bi, s * br + c * bi
                mf16[pl.ds(slot * 128 + 16 * a, 16), :] = _pack(re, im)
            m = pltpu.bitcast(rows(view(mf, z8), slot * 64, 64), BF16)
            mi[pl.ds(slot * 64, 64), :] = pltpu.bitcast(m.T, I32)
            return [rows(view(mf, z8), 0), rows(view(mi, z8), slot * 64)]
        return ([48, 8], fn)

    def scale_b(p, kk):
        cr, ncr, ci = prm(p, P_COEF), prm(p, P_COEF + 1), prm(p, P_COEF + 2)
        br, bi = (braw[pl.ds(D * c + 128 * p, 128), pl.ds(128 * kk, 128)].T.astype(F32)
                  for c in range(2))
        ties = []
        for i in range(8):
            r0, r1 = br[16 * i:16 * i + 8], br[16 * i + 8:16 * i + 16]
            i0, i1 = bi[16 * i:16 * i + 8], bi[16 * i + 8:16 * i + 16]
            wb16[pl.ds((p * NG + kk) * 128 + 16 * i, 16), :] = _pack(
                cr * r0 - ci * i0, cr * r1 - ci * i1)
            wb16[pl.ds(((NG + p) * NG + kk) * 128 + 16 * i, 16), :] = _pack(
                ncr * i0 - ci * r0, ncr * i1 - ci * r1)
            if i % 2:
                ties.append(rows(view(wb, z8), ((NG + p) * NG + kk) * 64))
        return ties

    def c_task(kk):
        def fn(gate):
            for n in range(NG):
                t = craw[pl.ds(kk * D + 128 * n, 128), :]
                wc[pl.ds((kk * NG + n) * 64, 64), :] = pltpu.bitcast(t.T, I32)
            return [rows(view(wc, z8), kk * NG * 64)]
        return ([40], fn)

    first = bu_passes(0, 0, z8)
    first = [[q for i, q in enumerate(first) if (i // NG) % NG == p] for p in range(NG)]
    mats = [matrix_task(slot) for slot in range(32)]

    def scale_tasks(p):
        return [([36] * 4, lambda gate, kk=kk: scale_b(p, kk)) for kk in range(NG)]

    def dma_task(ds):
        return ([1], lambda gate: start(ds))

    def filter_tasks(g, slot):
        k1, k2 = [], []
        for s in range(8):
            k1 += [k1_task(g, s, n0, z8) for n0 in range(4)]
            k2 += pass2_tasks(st_k, s, z8)
        return transpose_tasks(slot, z8), k1, k2

    def forward_tasks(u, g):
        tasks = []
        for s in range(8):
            tasks += [u1_task(g, s, n0, z8) for n0 in range(4)] + pass2_tasks(st_u, s, z8)
        return tasks, [skip_task(u, n, z8) for n in range(NG)]

    per_n = 2 * NG * UNIT // MM
    total = NG * per_n

    wait(x_dma(0) + b_dma(0) + b_dma(1))
    _now(scale_tasks(0))
    _weave(first[0], [(scale_tasks(1), 0, 40)], pred)
    wait(b_dma(2) + b_dma(3))
    _weave(first[1] + first[2], [(scale_tasks(2), 0, 40), (scale_tasks(3), 40, 80)], pred)
    wait(b_dma(4) + x_dma(1))
    _weave(first[3] + first[4] + bu_passes(1, 1),
           [(scale_tasks(4), 0, 40), (mats, 40, 80 + total), (scan_tasks(0, 0, z8), 92, 80 + total)], pred)
    wait(x_dma(2) + [sk_dma(0)] + c_dma + [col_dma(0, 0), col_dma(1, 0)])
    tr, k1, k2 = filter_tasks(0, 0)
    fwd, skips = forward_tasks(0, 0)
    _weave(bu_passes(2, 0) + y_passes(0, range(NG)), [
        (scan_tasks(1, 1, z8), 0, 180), (tr, 8, 24), (k1, 24, 250),
        ([c_task(kk) for kk in range(2 * NG)], 24, 180), (widen_tasks(0, z8, 8), 0, total),
        (fwd, total, 2 * total), (k2, 250, 2 * total)]
        + [(skips[n:n + 1], total + per_n * (n + 1) + 16, total + per_n * (n + 1) + 16)
           for n in range(NG - 1)], pred)

    def body(i, _):
        wait([col_dma(2, i), sk_dma(i + 1), col_dma(0, i + 1), col_dma(1, i + 1)] + x_dma(i + LEAD))
        bup, yp = bu_passes(i + LEAD, 0), y_passes(i + 1, range(NG))
        passes = fwd_passes(0, z8)
        for grp in range(1, 8):
            passes += fwd_passes(grp, z8) + inv_passes(grp - 1, z8)
        passes += bup[:8] + inv_passes(7, z8) + bup[8:] + yp
        y0 = len(passes) - total
        tr, k1, k2 = filter_tasks(clamp(i + 1), i + 1)
        fwd, skips = forward_tasks(i + 1, clamp(i + 1))
        inv = [inv1_task(i, s, n0, z8) for s in range(8) for n0 in range(4)]
        nk, tail = CFG["kconv"], CFG["tail"]
        _weave(passes, [
            (scan_tasks(i + LEAD - 1, 0, z8), *CFG["scanw"]), (tr, *CFG["tr"]),
            ([skip_task(i, NG - 1, z8), dma_task([oa_dma(i)])], 12, 12),
            (widen_tasks(i + 1, z8, 16), *CFG["wid"]), (k1[:nk], *CFG["kwin"]),
            (inv, 216, y0 - 8), (k1[nk:] + k2, 216, y0), ([dma_task([ob_dma(i)])], y0, y0),
            (fwd[:-tail], y0 - CFG["early"], y0 + total), (fwd[-tail:], y0 + total, y0 + total)]
            + [(skips[n:n + 1], y0 + per_n * (n + 1) + 16, y0 + per_n * (n + 1) + 16)
               for n in range(NG - 1)], pred)
        return 0

    lax.fori_loop(0, NG, body, 0)

    units = range(NG + 1, NG + LEAD)
    yp = [q for u in units for q in y_passes(u, range(NG))]
    plan = [(scan_tasks(L // UNIT - 1, 0, z8), 0, total - 8),
            ([skip_task(NG, NG - 1, z8), dma_task([oa_dma(NG)])], 8, 8)]
    for j, u in enumerate(units):
        for n in range(NG):
            where = min(j * total + per_n * (n + 1) + 16, len(yp))
            plan.append(([skip_task(u, n, z8)] + [dma_task([oa_dma(u)])] * (n == NG - 1), where, where))
    _weave(yp, plan, pred)
    wait([oa_dma(u) for u in range(NG + LEAD)] + [ob_dma(g) for g in range(NG)])


@jax.jit
def pallas_concat_heads__ssm_conv_s5__ssm_conv_h3__prompt_kernel(
    A_x: jax.Array,
    A_Lambda_re: jax.Array,
    A_Lambda_im: jax.Array,
    A_B_re: jax.Array,
    A_B_im: jax.Array,
    A_C_re: jax.Array,
    A_C_im: jax.Array,
    A_log_dt: jax.Array,
    A_Dskip: jax.Array,
    B_q: jax.Array,
    B_k: jax.Array,
    B_v: jax.Array,
    B_shift_k: jax.Array,
    B_ssm_k: jax.Array,
    B_ssm_D: jax.Array,
):
    assert A_x.shape == (1, L, D) and B_shift_k.shape == (D, 4)
    vmem = pltpu.VMEM
    dma = pltpu.SemaphoreType.DMA
    scratch = [
        vmem(_TABLES.shape, F32),
        vmem((D,), BF16), vmem((D,), BF16), vmem((D,), BF16), vmem((D,), BF16), vmem((D,), BF16),
        vmem((4, D), BF16),
        vmem((NG * L, 128), BF16),
        vmem((2 * D, D), BF16),
        vmem((2 * NG * D, 128), BF16),
        vmem((NG * L, 128), BF16),
        vmem(((NG + 1) * L, 128), BF16),
        vmem(((NG + 1) * L, 128), BF16),
        vmem((D + 128, L), BF16),
        vmem((NG * P_ROWS * 8, 128), F32),
        vmem((2 * NG * D, 128), BF16),
        vmem((2 * NG * NG * 64, 128), I32),
        vmem((32 * 128, 128), BF16),
        vmem((32 * 64, 128), I32),
        vmem((2 * 2 * NG * BU_PART, 128), F32),
        vmem((2 * NG * L, 128), BF16),
        vmem((3 * NG * 8, 128), F32),
        vmem((NG * YS_ROWS, 128), F32),
        vmem((L, D), F32),
        vmem((L // 2 + 8, 128), I32),
        vmem((KF_PAD + L, 128), F32),
        vmem((2 * L + 8, 128), F32),
        vmem((2 * L + 8, 128), F32),
        vmem((2 * L + 8, 128), F32),
        vmem((32 * 128, 128), BF16),
        vmem((32 * 128, 128), BF16),
        vmem((4 * 128, 128), BF16),
        vmem((4 * 128, 128), BF16),
        vmem((NG * L, 128), F32),
        dma((S_END,)), dma((L // UNIT,)), dma((NG,)),
    ]
    out = pl.pallas_call(
        _kernel,
        out_shape=jax.ShapeDtypeStruct((L, 2 * D), F32),
        in_specs=[pl.BlockSpec(memory_space=pl.ANY)] * 16,
        out_specs=pl.BlockSpec(memory_space=pl.ANY),
        scratch_shapes=scratch,
        compiler_params=pltpu.CompilerParams(vmem_limit_bytes=100 * 1024 * 1024),
        name="s5_h3",
    )(_TABLES, A_x.reshape(L, D), A_Lambda_re, A_Lambda_im, A_B_re, A_B_im, A_C_re, A_C_im,
      A_log_dt, A_Dskip, B_q.reshape(L, D), B_k.reshape(L, D), B_v.reshape(L, D),
      B_shift_k.T, B_ssm_k, B_ssm_D)
    return out.reshape(1, L, 2 * D)
```

```python
import math

import jax
import jax.numpy as jnp
import numpy as np
from jax import lax
from jax.experimental import pallas as pl
from jax.experimental.pallas import tpu as pltpu

F32, BF16, I32 = jnp.float32, jnp.bfloat16, jnp.int32

L = 2048
D = 640
NG = D // 128
UNIT = 256
SEG = 16
R = UNIT // SEG
LEAD = L // UNIT - NG
BU_PART = 9 * 2 * R
YS_ROWS = SEG * (R + 1)
KF_PAD = 8


class _Signed:
    def __init__(self, v, neg=False):
        self.v, self.neg = v, neg

    def __neg__(self):
        return _Signed(self.v, not self.neg)

    def __add__(self, o):
        if self.neg == o.neg:
            return _Signed(self.v + o.v, self.neg)
        return _Signed(o.v - self.v if self.neg else self.v - o.v)

    def __sub__(self, o):
        return self + (-o)

    def __mul__(self, c):
        return _Signed(self.v * np.float32(-c if self.neg else c))

    def get(self):
        return -self.v if self.neg else self.v


def _rot(re, im, num, den):
    num %= den
    h = math.sqrt(0.5)
    if num == 0:
        return re, im
    if 4 * num == den:
        return -im, re
    if 4 * num == 3 * den:
        return im, -re
    if 8 * num == den:
        return (re - im) * h, (re + im) * h
    if 8 * num == 3 * den:
        return (re + im) * (-h), (re - im) * h
    if 8 * num == 5 * den:
        return (im - re) * h, (re + im) * (-h)
    if 8 * num == 7 * den:
        return (re + im) * h, (im - re) * h
    c = math.cos(2 * math.pi * num / den)
    s = math.sin(2 * math.pi * num / den)
    return re * c - im * s, re * s + im * c


def _dft4(z, sign):
    (r0, i0), (r1, i1), (r2, i2), (r3, i3) = z
    ar, ai, br, bi = r0 + r2, i0 + i2, r0 - r2, i0 - i2
    cr, ci, dr, di = r1 + r3, i1 + i3, r1 - r3, i1 - i3
    plus, minus = (br - di, bi + dr), (br + di, bi - dr)
    if sign < 0:
        plus, minus = minus, plus
    return [(ar + cr, ai + ci), plus, (ar - cr, ai - ci), minus], [ai.v, ci.v]


def _fwd1(n0, u):
    a, b = u[:4], u[4:]
    r = [_rot(a[m], b[m], n0 + 4 * m, 64) for m in range(4)]
    z, halves = _dft4(r, 1)
    out = [_rot(*z[k], n0 * k, 16) for k in range(4)]
    s2 = [a[m] + b[m] for m in range(4)]
    d2 = [a[m] - b[m] for m in range(4)]
    p = _rot(d2[0], d2[2], n0, 32)
    q = _rot(d2[1], d2[3], n0 + 4, 32)
    out.append((p[0] + q[0], p[1] + q[1]))
    out.append(_rot(p[0] - q[0], p[1] - q[1], n0, 8))
    s3 = [s2[0] + s2[2], s2[1] + s2[3]]
    d3 = [s2[0] - s2[2], s2[1] - s2[3]]
    out.append(_rot(d3[0], d3[1], n0, 16))
    out.append((s3[0] + s3[1], s3[0] - s3[1]))
    return out, halves


def _fwd2(grp, z):
    if grp < 7:
        return _dft4(z, 1)[0]
    s4 = [t[0] for t in z]
    d4 = [t[1] for t in z]
    p = (d4[0], d4[2])
    q = _rot(d4[1], d4[3], 1, 8)
    s5 = [s4[0] + s4[2], s4[1] + s4[3]]
    return [
        (s5[0] + s5[1], s5[0] - s5[1]),
        (s4[0] - s4[2], s4[1] - s4[3]),
        (p[0] + q[0], p[1] + q[1]),
        (p[0] - q[0], p[1] - q[1]),
    ]


def _inv2(grp, w):
    if grp < 7:
        return _dft4(w, -1)[0]
    s5 = [w[0][0] + w[0][1], w[0][0] - w[0][1]]
    s4 = [s5[0] + w[1][0], s5[1] + w[1][1], s5[0] - w[1][0], s5[1] - w[1][1]]
    p = (w[2][0] + w[3][0], w[2][1] + w[3][1])
    q = _rot(w[2][0] - w[3][0], w[2][1] - w[3][1], -1, 8)
    d4 = [p[0], q[0], p[1], q[1]]
    return [(s4[n], d4[n]) for n in range(4)]


def _inv1(n0, z):
    t, _ = _dft4([_rot(*z[k], -n0 * k, 16) for k in range(4)], -1)
    ab = [_rot(*t[m], -(n0 + 4 * m), 64) for m in range(4)]
    e = _rot(*z[5], -n0, 8)
    p = _rot(z[4][0] + e[0], z[4][1] + e[1], -n0, 32)
    q = _rot(z[4][0] - e[0], z[4][1] - e[1], -(n0 + 4), 32)
    d2 = [p[0], q[0], p[1], q[1]]
    d3 = _rot(*z[6], -n0, 16)
    s3 = [z[7][0] + z[7][1], z[7][0] - z[7][1]]
    s2 = [s3[0] + d3[0], s3[1] + d3[1], s3[0] - d3[0], s3[1] - d3[1]]
    e2 = [s2[m] + d2[m] for m in range(4)]
    a = [ab[m][0] + e2[m] for m in range(4)]
    b = [ab[m][1] + (s2[m] - d2[m]) for m in range(4)]
    return a + b, [t[0][0].v + t[1][1].v, e2[0].v]


_F1 = [4 * (g + 4 * k) + 1 for g in range(4) for k in range(4)]
_F1 += [2 * (4 * (g + 2 * k) + 1) for g in range(2) for k in range(4)]
_F1 += [4 * (4 * k + 1) for k in range(4)]
_F1 += [0, 16, 8, 40]
_REAL_SLOT = 28


def _dft_tables():
    kap = np.arange(128)
    j = 8 * (kap // 16) + kap % 8
    part = (kap // 8) % 2
    pr, pc, jr, jc = part[:, None], part[None, :], j[:, None], j[None, :]
    lo = 2 * np.pi * jr * jc / 64
    base = np.where(pr == pc, np.cos(lo), np.where(pr == 0, -np.sin(lo), np.sin(lo)))
    hi = 2 * np.pi * (32 + 64 * (jr - 32)) * jc / 4096
    v0 = np.where(pr == 0, np.cos(lo), np.where(jr == 0, np.cos(np.pi * jc), np.sin(lo)))
    v32 = np.where(pr == 0, np.cos(hi), np.sin(hi))
    real = np.where(jr < 32, np.where(pc == 0, v0, 0.0), np.where(pc == 1, v32, 0.0))
    th = 2 * np.pi * np.outer(np.array(_F1), j) / 4096
    zeros = np.zeros((8, 128))
    return np.concatenate([base, real, np.cos(th), np.sin(th), zeros]).astype(np.float32)


_TABLES = _dft_tables()
_FFT_SCALE = 2.0 ** -11

(P_MU, P_RHO, P_RHO1, P_RHO2, P_RHO4, P_TAP, P_SSMD, P_DSKIP, P_COEF, P_ROWS) = (
    0, 2, 4, 6, 8, 10, 14, 15, 16, 20)
S_SMALL, S_C, S_K0, S_B, S_COL, S_X = 0, 1, 2, 3, 3 + NG, 3 + 2 * NG
S_END = S_X + L // UNIT


Y128 = [(0, 128, 128)] + [(n, t, 128) for n in range(1, 4) for t in (0, 128)] + [
    (4, 0, 128), (4, 128, 96), (4, 224, 32)]
Y96 = [(0, 64, 96), (0, 160, 96)] + [(n, t, m) for n in range(1, 5) for t, m in ((0, 96), (96, 96), (192, 64))]


def _cmul(a, b):
    return a[0] * b[0] - a[1] * b[1], a[0] * b[1] + a[1] * b[0]


def _pack(lo, hi):
    return jnp.concatenate([lo, hi], axis=0).astype(BF16)


def _unpack(w):
    v = pltpu.bitcast(w, BF16).astype(F32)
    return v[:8], v[8:]


CFG = dict(scan=22, u=28, k1=24, p2=0, inv=0, skip=28, tail=3, kconv=16, steps=2, p2n=4,
           early=40, kwin=(44, 216), tr=(20, 40), wid=(16, 200), scanw=(0, 350), invw=(230, 400),
           k2w=(230, 400), s1=45, k0=24, mf=128, mi=128, bsz=[128, 128],
           ylead=[(0, 0, 32), (0, 32, 96)], ylead_slots=20, yt=Y128, p1ties=(3, 7), kskip=1)


class _Gate:
    def __init__(self, pred=None, seen=()):
        self.pred, self.seen = pred, seen

    def early(self, lag):
        old = [e for e in self.seen if e[0] <= -lag]
        return max(old, key=lambda e: e[0])[1] if lag and old else None

    def value(self, v, lag):
        early = self.early(lag)
        return v if early is None else jnp.where(self.pred, v, early)

    def loads(self, ref, lag):
        early = self.early(lag)
        if early is not None:
            ref[pl.ds(ref.shape[0] - 8, 8), :] = (
                early if ref.dtype == F32 else pltpu.bitcast(early, I32))


def _weave(passes, plan, pred):
    begin, clock = [], [0] * 4
    for i, (n, *_) in enumerate(passes):
        begin.append(clock[i % 4] / 16)
        clock[i % 4] += n

    def index(t):
        later = [i for i, b in enumerate(begin) if b >= t - 3.999]
        if not later:
            return len(passes)
        same = [i for i in later if begin[i] == min(begin[j] for j in later)]
        return same[min(max(int((t - begin[same[0]]) / 4 * len(same)), 0), len(same) - 1)]

    at = [[] for _ in range(len(passes) + 1)]
    for tasks, lo, hi in plan:
        total, done = sum(sum(c) for c, _ in tasks) or 1, 0.0
        for costs, fn in tasks:
            where = []
            for cost in costs:
                done += cost
                where.append(index(lo + done / total * (hi - lo)))
            at[min(where)].append((fn, where))
    seen, ties = [], [[] for _ in at]
    for i, fns in enumerate(at):
        now = (begin[i] + i % 4) if i < len(begin) else clock[0] / 16
        early = [(t - now, v) for t, v in seen]
        for fn, where in fns:
            for w, tie in zip(where, fn(_Gate(pred, early)) or ()):
                ties[w].append(tie)
        if i == len(passes):
            break
        n, lhs, rhs, consume = passes[i]
        w = rhs()
        for tie in ties[i]:
            w[-1] = jnp.where(pred, w[-1], tie if tie.dtype == I32 else pltpu.bitcast(tie, I32))
        d = jnp.dot(pltpu.bitcast(jnp.concatenate(lhs(), axis=0), BF16),
                    pltpu.bitcast(jnp.concatenate(w, axis=0), BF16), preferred_element_type=F32)
        seen += [(begin[i] + i % 4 + j // 16 - 4, d[j - 8:j]) for j in range(64, n + 1, 64)]
        consume(d)


def _now(tasks):
    for _, fn in tasks:
        fn(_Gate())


def _kernel(tab_hbm, x_hbm, lre_hbm, lim_hbm, bre_hbm, bim_hbm, cre_hbm, cim_hbm,
            ldt_hbm, dsk_hbm, q_hbm, k_hbm, v_hbm, tap_hbm, sk_hbm, sd_hbm,
            o_hbm,
            tab, lre_v, lim_v, ldt_v, dsk_v, sd_v, tap_v,
            xb, braw, craw, qb, kb, vb, skb,
            par, wb16, wc, mf16, mi, bu, hb16, carry, ys, oa,
            kt, kf, st_u, st_k, st_i, vu16, vk16, pb0, pb1, ob,
            sem, sem_oa, sem_ob):
    x32, q32, k32, v32, wb, mf, hb, vu, vk = (
        r.bitcast(I32) for r in (xb, qb, kb, vb, wb16, mf16, hb16, vu16, vk16))
    pb16 = (pb0, pb1)
    pb = (pb0.bitcast(I32), pb1.bitcast(I32))

    def rows(ref, start, n=8):
        return ref[pl.ds(start, n), :]

    def hint(v, n):
        return v if isinstance(v, int) else pl.multiple_of(v, n)

    def view(ref, start, n=None):
        return ref.at[pl.ds(hint(start, 16), n or ref.shape[0]), :]

    small = [pltpu.make_async_copy(s, d, sem.at[S_SMALL]) for s, d in (
        (lre_hbm, lre_v), (lim_hbm, lim_v), (ldt_hbm, ldt_v),
        (dsk_hbm, dsk_v), (sd_hbm, sd_v), (tap_hbm, tap_v), (tab_hbm, tab))]

    def x_dma(u):
        return [pltpu.make_async_copy(
            x_hbm.at[pl.ds(hint(u * UNIT, UNIT), UNIT), pl.ds(128 * n, 128)],
            xb.at[pl.ds(hint(n * L + u * UNIT, UNIT), UNIT), :], sem.at[S_X + u])
            for n in range(NG)]

    def b_dma(p):
        return [pltpu.make_async_copy(
            src.at[pl.ds(128 * p, 128), :], braw.at[pl.ds(D * c + 128 * p, 128), :],
            sem.at[S_B + p]) for c, src in enumerate((bre_hbm, bim_hbm))]

    c_dma = [pltpu.make_async_copy(
        src.at[:, pl.ds(128 * p, 128)], craw.at[pl.ds(D * (NG * c + p), D), :],
        sem.at[S_C]) for c, src in enumerate((cre_hbm, cim_hbm)) for p in range(NG)]

    def clamp(g):
        return min(g, NG - 1) if isinstance(g, int) else jnp.minimum(g, NG - 1)

    def col_dma(which, g, first=False):
        src, dst = ((k_hbm, kb), (v_hbm, vb), (q_hbm, qb))[which]
        return pltpu.make_async_copy(
            src.at[:, pl.ds(hint(128 * clamp(g), 128), 128)],
            dst.at[pl.ds(hint(L * g, L), L), :], sem.at[S_K0 if first else S_COL + g])

    def sk_dma(g, sem_at):
        t = hint(128 * g, 128)
        return pltpu.make_async_copy(
            sk_hbm.at[pl.ds(hint(128 * clamp(g), 128), 128), :], skb.at[pl.ds(t, 128), :],
            sem.at[sem_at])

    def oa_dma(u):
        t = hint(u * UNIT, UNIT)
        return pltpu.make_async_copy(
            oa.at[pl.ds(t, UNIT), :], o_hbm.at[pl.ds(t, UNIT), pl.ds(0, D)], sem_oa.at[u])

    def ob_dma(g):
        return pltpu.make_async_copy(
            ob.at[pl.ds(hint(L * g, L), L), :],
            o_hbm.at[:, pl.ds(hint(D + 128 * g, 128), 128)], sem_ob.at[g])

    def start(ds):
        for d in ds:
            d.start()

    def wait(ds):
        for d in ds:
            d.wait()

    def prm(g, row):
        return rows(view(par, g * (P_ROWS * 8), P_ROWS * 8), row * 8)

    def bu_passes(u, slot, z=0, sizes=None):
        out = []
        xu, w = view(x32, u * (UNIT // 2), ((NG - 1) * L + UNIT) // 2), view(wb, z)
        sizes = sizes or [64] * (UNIT // 64)
        for n in (p + c * NG for p in range(NG) for c in range(2)):
            for m, MM in zip(np.cumsum([0] + sizes).tolist(), sizes):
                acc = []
                for kk in range(NG):
                    def lhs(m=m, kk=kk, MM=MM):
                        t = (kk * L + m) // 2
                        return [rows(xu, t + 8 * i) for i in range(MM // 16)]

                    def rhs(n=n, kk=kk):
                        return [rows(w, (n * NG + kk) * 64 + 8 * i) for i in range(8)]

                    def consume(d, m=m, n=n, kk=kk, acc=acc, MM=MM):
                        acc.append(d if kk == 0 else acc[-1] + d)
                        if kk == NG - 1:
                            for i in range(MM // 8):
                                seg, r = divmod(m + 8 * i, R)
                                row = 9 * (seg % 2 * R + r) + seg // 2
                                bu[pl.ds((slot * 2 * NG + n) * BU_PART + row, 8, stride=9), :] = (
                                    acc[-1][8 * i:8 * i + 8])
                    out.append((MM, lhs, rhs, consume))
        return out

    def scan_tasks(u, slot, z):
        steps = CFG["steps"]
        state = {}
        hu = view(hb16, u * UNIT, (2 * NG - 1) * L + UNIT)

        def b(p, ch, r):
            return tuple(rows(bu, (slot * 2 * NG + c * NG + p) * BU_PART + 9 * (ch * R + r))
                         for c in range(2))

        def step(mu, h, br):
            return (mu[0] * h[0] + br[0]) - mu[1] * h[1], (mu[0] * h[1] + br[1]) + mu[1] * h[0]

        def ends(p, gate):
            mu, ties = (gate.value(prm(p, P_MU), CFG["scan"]), prm(p, P_MU + 1)), []
            h = [b(p, ch, 0) for ch in range(2)]
            for r in range(1, R):
                h = [step(mu, h[ch], b(p, ch, r)) for ch in range(2)]
                if r % steps == 0:
                    ties.append(h[r // steps % 2][0])
            state[p] = starts(p, h)
            return ties + [state[p][1][0]]

        def starts(p, e):
            last = lax.broadcasted_iota(I32, (8, 128), 0) == 7
            rho = (prm(p, P_RHO), prm(p, P_RHO + 1))
            pair = step(rho, e[0], e[1])
            a = tuple(pltpu.roll(jnp.where(last, rows(carry, (2 * p + c) * 8), pair[c]), 1, 0)
                      for c in range(2))
            for sh, row in ((1, P_RHO1), (2, P_RHO2), (4, P_RHO4)):
                a = step((prm(p, row), prm(p, row + 1)), tuple(pltpu.roll(c, sh, 0) for c in a), a)
            return [a, step(rho, a, e[0])]

        def run(p, r0, gate):
            if r0 == 0:
                state["mu"] = (prm(p, P_MU), prm(p, P_MU + 1))
            mu, h = (gate.value(state["mu"][0], CFG["scan"]), state["mu"][1]), state[p]
            for r in range(r0, r0 + steps):
                h = [step(mu, h[ch], b(p, ch, r)) for ch in range(2)]
                for c in range(2):
                    hu[pl.ds((c * NG + p) * L + 16 * r, 16), :] = _pack(h[0][c], h[1][c])
            state[p] = h
            if r0 + steps == R:
                for c in range(2):
                    carry[pl.ds((2 * p + c) * 8, 8), :] = h[1][c]
            return [rows(view(hb, z, 8), 0)]

        tasks = []
        for p in range(NG):
            tasks.append(([16 * steps] * ((R - 1) // steps) + [46 + 16 * steps],
                          lambda gate, p=p: ends(p, gate)))
            tasks += [([18 * steps], lambda gate, p=p, r0=r0: run(p, r0, gate))
                      for r0 in range(0, R, steps)]
        return tasks

    def y_tiles(MM):
        return [(n, t, MM) for n in range(NG) for t in range(0, UNIT, MM)]

    def y_passes(u, tiles):
        out = []
        hu = view(hb, u * (UNIT // 2), ((2 * NG - 1) * L + UNIT) // 2)
        if True:
            for n, t0, MM in tiles:
                acc = []
                for kk in range(2 * NG):
                    def lhs(t0=t0, kk=kk, MM=MM):
                        t = kk * (L // 2) + t0 // 2
                        return [rows(hu, t + 8 * i) for i in range(MM // 16)]

                    def rhs(n=n, kk=kk):
                        return [rows(wc, (kk * NG + n) * 64 + 8 * i) for i in range(8)]

                    def consume(d, t0=t0, n=n, kk=kk, acc=acc, MM=MM):
                        acc.append(d if kk == 0 else acc[-1] + d)
                        if kk == 2 * NG - 1:
                            for i in range(MM // 8):
                                r, ch = divmod(t0 // 8 + i, 2)
                                ys[pl.ds(n * YS_ROWS + ch * (R + 1) + r, 8, stride=2 * (R + 1)), :] = (
                                    acc[-1][8 * i:8 * i + 8])
                    out.append((MM, lhs, rhs, consume))
        return out

    def skip_task(u, n, z):
        def fn(gate):
            dsk = gate.value(prm(n, P_DSKIP), CFG["skip"])
            xu, ou = view(x32, u * (UNIT // 2) + n * (L // 2), UNIT // 2), view(oa, u * UNIT, UNIT)
            ties = []
            for i in range(UNIT // 16):
                xs = _unpack(rows(xu, 8 * i))
                for c in range(2):
                    t = 16 * i + 8 * c
                    y = rows(ys, n * YS_ROWS + (t // R) * (R + 1) + t % R)
                    ou[pl.ds(t, 8), pl.ds(128 * n, 128)] = y + xs[c] * dsk
                if i % 4 == 3:
                    ties.append(view(oa, z + u * UNIT, 8)[:, pl.ds(128 * n, 128)])
            return ties
        return ([24] * (UNIT // 64), fn)

    def widen_tasks(g, z, pieces=2):
        def fn(i0, i1):
            kg = view(k32, g * (L // 2), L // 2)
            for i in range(i0, i1):
                lo, hi = _unpack(rows(kg, 8 * i))
                kf[pl.ds(KF_PAD + 16 * i, 8), :] = lo
                kf[pl.ds(KF_PAD + 16 * i + 8, 8), :] = hi
            return [rows(view(kf, z), 16 * i0 + KF_PAD)]
        n = L // 16 // pieces
        return [([2 * n], lambda gate, i=i: fn(i * n, (i + 1) * n)) for i in range(pieces)]

    def transpose_tasks(g, z, pieces=8):
        def fn(c0, c1):
            for c in range(c0, c1):
                t = skb[pl.ds(hint(128 * g, 128), 128), pl.ds(128 * c, 128)]
                kt[pl.ds(64 * c, 64), :] = pltpu.bitcast(t.T, I32)
            return [rows(view(kt, z), 64 * c0)]
        n = L // 128 // pieces
        return [([8 * n], lambda gate, i=i: fn(i * n, (i + 1) * n)) for i in range(pieces)]

    def pass1(st, s, n0, u, z):
        pairs, ties = _fwd1(n0, [_Signed(v) for v in u])
        for grp, pair in enumerate(pairs):
            for c in range(2):
                st[pl.ds(((s * 4 + n0) * 8 + grp) * 16 + 8 * c, 8), :] = pair[c].get()
            if grp in CFG["p1ties"]:
                ties.append(rows(view(st, z), (s * 4 + n0) * 128))
        return ties

    def rest_costs(n0):
        each = np.array([14, 14, 14, 14, 30, 8, 12, 4]) * ((54, 96, 80, 96)[n0] - 16) / 110
        cut = np.cumsum(each)[list(CFG["p1ties"])]
        return np.diff(cut, prepend=0).tolist()

    def u1_task(g, s, n0, z):
        def fn(gate):
            taps = [prm(g, P_TAP + t) for t in range(4)]
            taps[0] = gate.value(taps[0], CFG["u"])
            u, kz, vg = [], view(kf, z), view(v32, g * (L // 2), L // 2)
            for m in range(8):
                t = 64 * (n0 + 4 * m) + 8 * s
                ks = rows(kz, KF_PAD + t) * taps[0]
                for lag in range(1, 4):
                    ks = ks + rows(kz, KF_PAD + t - lag) * taps[lag]
                v = _unpack(rows(vg, (t // 16) * 8))[s % 2]
                u.append(ks * v)
            return pass1(st_u, s, n0, u, z)
        return ([40, 40] + rest_costs(n0), fn)

    def k1_task(g, s, n0, z):
        def fn(gate):
            gate.loads(kt, CFG["k1"])
            u = [_unpack(rows(view(kt, z), 32 * (n0 + 4 * m) + 8 * (s // 2)))[s % 2] for m in range(8)]
            if s == 0 and n0 == 0:
                first = lax.broadcasted_iota(I32, (8, 128), 0) == 0
                u[0] = u[0] + jnp.where(first, prm(g, P_SSMD), 0.0)
            return pass1(st_k, s, n0, u, z)[CFG["kskip"]:]
        costs = [11, 11] + rest_costs(n0)
        return ([sum(costs[:CFG["kskip"] + 1])] + costs[CFG["kskip"] + 1:], fn)

    def pass2_task(st, dst16, dst, s, grps, z):
        def fn(gate):
            gate.loads(st, CFG["p2"])
            for grp in grps:
                zs = [tuple(_Signed(rows(view(st, z), ((s * 4 + n0) * 8 + grp) * 16 + 8 * c)) for c in range(2))
                      for n0 in range(4)]
                for k, pair in enumerate(_fwd2(grp, zs)):
                    dst16[pl.ds((4 * grp + k) * 128 + 16 * s, 16), :] = _pack(pair[0].get(), pair[1].get())
            return [rows(view(dst, z), 4 * grps[0] * 64 + 8 * s)]
        return ([20 * len(grps)], fn)

    def pass2_tasks(st, s, z):
        dst = (vu16, vu) if st is st_u else (vk16, vk)
        return [pass2_task(st, *dst, s, g, z) for g in np.arange(8).reshape(CFG["p2n"], -1).tolist()]

    def fwd_passes(grp, z):
        out, MM = [], CFG["mf"]
        for slot in range(4 * grp, 4 * grp + 4):
            got = {}
            for half in range(128 // MM):
                for which, src in enumerate((vu, vk)):
                    def lhs(slot=slot, half=half):
                        return [rows(mf, slot * 64 + MM // 2 * half + 8 * i) for i in range(MM // 16)]

                    def rhs(slot=slot, src=src):
                        return [rows(view(src, z), slot * 64 + 8 * i) for i in range(8)]

                    def consume(d, slot=slot, half=half, which=which, got=got):
                        got[which] = d
                        if which == 0:
                            return
                        for i in range(MM // 16):
                            a = (got[0][16 * i:16 * i + 8], got[0][16 * i + 8:16 * i + 16])
                            b = (d[16 * i:16 * i + 8], d[16 * i + 8:16 * i + 16])
                            re, im = _cmul(a, b)
                            if slot == _REAL_SLOT and half == 0 and i == 0:
                                first = lax.broadcasted_iota(I32, (8, 128), 0) == 0
                                re = jnp.where(first, 0.5 * (a[0] * b[0]), re)
                                im = jnp.where(first, 0.5 * (a[1] * b[1]), im)
                            pb16[grp % 2][pl.ds(slot % 4 * 128 + MM * half + 16 * i, 16), :] = (
                                _pack(re, im))
                    out.append((MM, lhs, rhs, consume))
        return out

    def inv_passes(grp, z):
        out, MM = [], CFG["mi"]
        for half in range(128 // MM):
            got = []
            for slot in range(4 * grp, 4 * grp + 4):
                def lhs(slot=slot, half=half):
                    return [rows(mi, slot * 64 + MM // 2 * half + 8 * i) for i in range(MM // 16)]

                def rhs(slot=slot):
                    return [rows(view(pb[grp % 2], z), slot % 4 * 64 + 8 * i) for i in range(8)]

                def consume(d, half=half, got=got):
                    got.append(d)
                    if len(got) < 4:
                        return
                    for i in range(MM // 16):
                        w = [(_Signed(t[16 * i:16 * i + 8]), _Signed(t[16 * i + 8:16 * i + 16]))
                             for t in got]
                        for n0, pair in enumerate(_inv2(grp, w)):
                            for c in range(2):
                                at = (((MM // 16 * half + i) * 4 + n0) * 8 + grp) * 16 + 8 * c
                                st_i[pl.ds(at, 8), :] = pair[c].get()
                out.append((MM, lhs, rhs, consume))
        return out

    def inv1_task(g, s, n0, z):
        def fn(gate):
            gate.loads(st_i, CFG["inv"])
            zs = [tuple(_Signed(rows(view(st_i, z), ((s * 4 + n0) * 8 + grp) * 16 + 8 * c)) for c in range(2))
                  for grp in range(8)]
            qg, og = view(q32, g * (L // 2), L // 2), view(ob, g * L, L)
            ys8, ties = _inv1(n0, zs)
            for m in (0, 4, 2, 6, 1, 5, 3, 7):
                t = 64 * (n0 + 4 * m) + 8 * s
                qv = _unpack(rows(qg, (t // 16) * 8))[s % 2]
                og[pl.ds(t, 8), :] = qv * ys8[m].get()
                if m in (6, 7):
                    ties.append(rows(view(ob, z + g * L, L), 64 * n0 + 8 * s))
            return ties
        quarter = (16 + (62, 104, 88, 104)[n0]) // 4
        return ([quarter, quarter - 8, quarter + 4, quarter + 4], fn)

    start(small)
    start(x_dma(0))
    start(b_dma(0) + b_dma(1))
    filter0 = [sk_dma(0, S_C)] + c_dma
    data0 = [col_dma(0, 0, True), col_dma(1, 0, True)]

    def group_dma(g):
        return [col_dma(2, g), sk_dma(g + 1, S_COL + g), col_dma(0, g + 1), col_dma(1, g + 1)]

    wait(small)
    zeros = rows(tab, 320).astype(I32)
    z8 = pl.multiple_of(zeros[0, 0], 16)
    sub = lax.broadcasted_iota(I32, (8, 128), 0)
    pred = zeros == 0

    def stack(ref):
        v = ref[...].astype(F32).reshape(1, D)
        return jnp.concatenate([v[:, 128 * g:128 * (g + 1)] for g in range(NG)]
                               + [v[:, :128]] * (8 - NG), axis=0)

    lre, lim = stack(lre_v), stack(lim_v)
    dt = jnp.exp(stack(ldt_v)).astype(BF16).astype(F32)
    mag, ang = jnp.exp(dt * lre), dt * lim
    lam = (mag * jnp.cos(ang), mag * jnp.sin(ang))
    scale = jnp.maximum(jnp.abs(lre), jnp.abs(lim))
    nre, nim = lre / scale, lim / scale
    den = (nre * nre + nim * nim) * scale
    coef = _cmul(((lam[0] - 1.0) / den, lam[1] / den), (nre, -nim))
    mu = (lam[0], -lam[1])
    rho = [mu]
    for _ in range(R.bit_length() + 2):
        rho.append(_cmul(rho[-1], rho[-1]))
    dsk, ssd = stack(dsk_v), stack(sd_v)
    taps = tap_v[...].astype(F32) * _FFT_SCALE
    for g in range(NG):
        def put(row, v):
            par[pl.ds((g * P_ROWS + row) * 8, 8), :] = v

        def lanes(v):
            return jnp.broadcast_to(v[g:g + 1], (8, 128))
        for c in range(2):
            put(P_MU + c, lanes(mu[c]))
            put(P_RHO + c, lanes(rho[-4][c]))
            for n, row in enumerate((P_RHO1, P_RHO2, P_RHO4)):
                put(row + c, jnp.where(sub >= 1 << n, lanes(rho[n - 3][c]), 0.0))
        for t in range(4):
            put(P_TAP + t, jnp.broadcast_to(taps[t:t + 1, 128 * g:128 * (g + 1)], (8, 128)))
        put(P_COEF, lanes(2.0 * coef[0]))
        put(P_COEF + 1, lanes(-2.0 * coef[0]))
        put(P_COEF + 2, lanes(2.0 * coef[1]))
        put(P_SSMD, lanes(ssd))
        put(P_DSKIP, lanes(dsk))
    for i in range(2 * NG):
        carry[pl.ds(8 * i, 8), :] = jnp.zeros((8, 128), F32)
    kf[pl.ds(0, KF_PAD), :] = jnp.zeros((KF_PAD, 128), F32)

    def matrix_task(slot):
        def fn(gate):
            if slot != _REAL_SLOT:
                c, s = tab[pl.ds(256 + slot, 1), :], tab[pl.ds(288 + slot, 1), :]
            for a in range(8):
                if slot == _REAL_SLOT:
                    re, im = rows(tab, 128 + 16 * a), rows(tab, 128 + 16 * a + 8)
                else:
                    br, bi = rows(tab, 16 * a), rows(tab, 16 * a + 8)
                    re, im = c * br - s * bi, s * br + c * bi
                mf16[pl.ds(slot * 128 + 16 * a, 16), :] = _pack(re, im)
            m = pltpu.bitcast(rows(view(mf, z8), slot * 64, 64), BF16)
            mi[pl.ds(slot * 64, 64), :] = pltpu.bitcast(m.T, I32)
            return [rows(view(mf, z8), 0), rows(view(mi, z8), slot * 64)]
        return ([48, 8], fn)

    def scale_b(p, kk):
        cr, ncr, ci = prm(p, P_COEF), prm(p, P_COEF + 1), prm(p, P_COEF + 2)
        br, bi = (braw[pl.ds(D * c + 128 * p, 128), pl.ds(128 * kk, 128)].T.astype(F32)
                  for c in range(2))
        ties = []
        for i in range(8):
            r0, r1 = br[16 * i:16 * i + 8], br[16 * i + 8:16 * i + 16]
            i0, i1 = bi[16 * i:16 * i + 8], bi[16 * i + 8:16 * i + 16]
            wb16[pl.ds((p * NG + kk) * 128 + 16 * i, 16), :] = _pack(
                cr * r0 - ci * i0, cr * r1 - ci * i1)
            wb16[pl.ds(((NG + p) * NG + kk) * 128 + 16 * i, 16), :] = _pack(
                ncr * i0 - ci * r0, ncr * i1 - ci * r1)
            if i % 2:
                ties.append(rows(view(wb, z8), ((NG + p) * NG + kk) * 64))
        return ties

    def c_task(kk):
        def fn(gate):
            for n in range(NG):
                t = craw[pl.ds(kk * D + 128 * n, 128), :]
                wc[pl.ds((kk * NG + n) * 64, 64), :] = pltpu.bitcast(t.T, I32)
            return [rows(view(wc, z8), kk * NG * 64)]
        return ([40], fn)

    first = bu_passes(0, 0, z8)
    first = [first[40 * p:40 * (p + 1)] for p in range(NG)]

    mats = [matrix_task(slot) for slot in range(32)]

    def scale_tasks(p):
        return [([36] * 4, lambda gate, kk=kk: scale_b(p, kk)) for kk in range(NG)]

    def dma_task(ds):
        return ([1], lambda gate: start(ds))

    def filter_tasks(g, slot):
        k1, k2 = [], []
        for s in range(8):
            k1 += [k1_task(g, s, n0, z8) for n0 in range(4)]
            k2 += pass2_tasks(st_k, s, z8)
        return transpose_tasks(slot, z8), k1, k2

    def forward_tasks(u, g):
        tasks = []
        for s in range(8):
            tasks += [u1_task(g, s, n0, z8) for n0 in range(4)] + pass2_tasks(st_u, s, z8)
        return tasks, [skip_task(u, n, z8) for n in range(NG)]

    per_n = 2 * NG * UNIT // 64
    total = NG * per_n

    start(b_dma(2) + b_dma(3))
    wait(x_dma(0) + b_dma(0) + b_dma(1))
    start(b_dma(4) + x_dma(1) + x_dma(2))
    _now(scale_tasks(0))
    _weave(first[0], [(scale_tasks(1), 0, 40)], pred)
    start(filter0)
    wait(b_dma(2) + b_dma(3))
    _weave(first[1] + first[2], [(scale_tasks(2), 0, 40), (scale_tasks(3), 40, 80)], pred)
    start(data0 + group_dma(0) + x_dma(LEAD))
    wait(b_dma(4) + x_dma(1))
    _weave(first[3] + first[4] + bu_passes(1, 1),
           [(scale_tasks(4), 0, 40), (mats, 40, 80 + total), (scan_tasks(0, 0, z8), 92, 80 + total)],
           pred)
    start(group_dma(1) + x_dma(LEAD + 1))
    wait(x_dma(2) + filter0)
    tr, k1, k2 = filter_tasks(0, 0)
    fwd, skips = forward_tasks(0, 0)
    scan = scan_tasks(1, 1, z8)
    _weave(bu_passes(2, 0), [
        (scan[:CFG["s1"]], 0, 150), (tr, 16, 40), (k1[:CFG["k0"]], 40, total),
        ([c_task(kk) for kk in range(2 * NG)], 8, total - 8)], pred)
    for g in range(2, NG):
        start(group_dma(g) + x_dma(LEAD + g))
    wait(data0)
    _weave(y_passes(0, y_tiles(64)), [
        (widen_tasks(0, z8, 8), 0, 20), (fwd[:-3], 20, total), (fwd[-3:], total, total),
        (scan[CFG["s1"]:] + k1[CFG["k0"]:] + k2, 0, total)]
        + [(skips[n:n + 1], per_n * (n + 1) + 16, per_n * (n + 1) + 16) for n in range(NG - 1)], pred)

    def body(i, _):
        wait(group_dma(i) + x_dma(i + LEAD))
        bup = bu_passes(i + LEAD, 0, sizes=CFG["bsz"])
        yp = y_passes(i + 1, CFG["yt"] or y_tiles(64))
        passes = fwd_passes(0, z8)
        for grp in range(1, 8):
            passes += fwd_passes(grp, z8) + inv_passes(grp - 1, z8)
        lead = y_passes(i + 1, CFG["ylead"])
        passes += lead[:8] + inv_passes(7, z8) + lead[8:] + bup + yp
        y0 = 192 + total + CFG["ylead_slots"]
        tr, k1, k2 = filter_tasks(clamp(i + 1), i + 1)
        fwd, skips = forward_tasks(i + 1, clamp(i + 1))
        inv = [inv1_task(i, s, n0, z8) for s in range(8) for n0 in range(4)]
        nk, tail, end = CFG["kconv"], CFG["tail"], 192 + 2 * total
        _weave(passes, [
            (scan_tasks(i + LEAD - 1, 0, z8), *CFG["scanw"]), (tr, *CFG["tr"]),
            ([skip_task(i, NG - 1, z8), dma_task([oa_dma(i)])], 12, 12),
            (widen_tasks(i + 1, z8, 16), *CFG["wid"]), (k1[:nk], *CFG["kwin"]),
            (inv + [dma_task([ob_dma(i)])], *CFG["invw"]), (k1[nk:] + k2, *CFG["k2w"]),
            (fwd[:-tail], y0 - CFG["early"], end), (fwd[-tail:], end, end)]
            + [(skips[n:n + 1], end - per_n * (NG - 1 - n) + 16, end - per_n * (NG - 1 - n) + 24)
               for n in range(NG - 1)], pred)
        return 0

    lax.fori_loop(0, NG, body, 0)

    units = range(NG + 1, NG + LEAD)
    yp = [q for u in units for q in y_passes(u, y_tiles(64))]
    plan = [(scan_tasks(L // UNIT - 1, 0, z8), 0, total - 8),
            ([skip_task(NG, NG - 1, z8), dma_task([oa_dma(NG)])], 8, 8)]
    for j, u in enumerate(units):
        for n in range(NG):
            where = min(j * total + per_n * (n + 1) + 16, len(units) * total)
            plan.append(([skip_task(u, n, z8)] + [dma_task([oa_dma(u)])] * (n == NG - 1), where, where))
    _weave(yp, plan, pred)
    wait([oa_dma(u) for u in range(NG + LEAD)] + [ob_dma(g) for g in range(NG)])


@jax.jit
def pallas_concat_heads__ssm_conv_s5__ssm_conv_h3__prompt_kernel(
    A_x: jax.Array,
    A_Lambda_re: jax.Array,
    A_Lambda_im: jax.Array,
    A_B_re: jax.Array,
    A_B_im: jax.Array,
    A_C_re: jax.Array,
    A_C_im: jax.Array,
    A_log_dt: jax.Array,
    A_Dskip: jax.Array,
    B_q: jax.Array,
    B_k: jax.Array,
    B_v: jax.Array,
    B_shift_k: jax.Array,
    B_ssm_k: jax.Array,
    B_ssm_D: jax.Array,
):
    assert A_x.shape == (1, L, D) and B_shift_k.shape == (D, 4)
    vmem = pltpu.VMEM
    dma = pltpu.SemaphoreType.DMA
    scratch = [
        vmem(_TABLES.shape, F32),
        vmem((D,), BF16), vmem((D,), BF16), vmem((D,), BF16), vmem((D,), BF16), vmem((D,), BF16),
        vmem((4, D), BF16),
        vmem((NG * L, 128), BF16),
        vmem((2 * D, D), BF16),
        vmem((2 * NG * D, 128), BF16),
        vmem((NG * L, 128), BF16),
        vmem(((NG + 1) * L, 128), BF16),
        vmem(((NG + 1) * L, 128), BF16),
        vmem((D + 128, L), BF16),
        vmem((NG * P_ROWS * 8, 128), F32),
        vmem((2 * NG * D, 128), BF16),
        vmem((2 * NG * NG * 64, 128), I32),
        vmem((32 * 128, 128), BF16),
        vmem((32 * 64, 128), I32),
        vmem((2 * 2 * NG * BU_PART, 128), F32),
        vmem((2 * NG * L, 128), BF16),
        vmem((3 * NG * 8, 128), F32),
        vmem((NG * YS_ROWS, 128), F32),
        vmem((L, D), F32),
        vmem((L // 2 + 8, 128), I32),
        vmem((KF_PAD + L, 128), F32),
        vmem((2 * L + 8, 128), F32),
        vmem((2 * L + 8, 128), F32),
        vmem((2 * L + 8, 128), F32),
        vmem((32 * 128, 128), BF16),
        vmem((32 * 128, 128), BF16),
        vmem((4 * 128, 128), BF16),
        vmem((4 * 128, 128), BF16),
        vmem((NG * L, 128), F32),
        dma((S_END,)), dma((L // UNIT,)), dma((NG,)),
    ]
    out = pl.pallas_call(
        _kernel,
        out_shape=jax.ShapeDtypeStruct((L, 2 * D), F32),
        in_specs=[pl.BlockSpec(memory_space=pl.ANY)] * 16,
        out_specs=pl.BlockSpec(memory_space=pl.ANY),
        scratch_shapes=scratch,
        compiler_params=pltpu.CompilerParams(vmem_limit_bytes=100 * 1024 * 1024),
        name="s5_h3",
    )(_TABLES, A_x.reshape(L, D), A_Lambda_re, A_Lambda_im, A_B_re, A_B_im, A_C_re, A_C_im,
      A_log_dt, A_Dskip, B_q.reshape(L, D), B_k.reshape(L, D), B_v.reshape(L, D),
      B_shift_k.T, B_ssm_k, B_ssm_D)
    return out.reshape(1, L, 2 * D)
```

```python
import math

import jax
import jax.numpy as jnp
import numpy as np
from jax import lax
from jax.experimental import pallas as pl
from jax.experimental.pallas import tpu as pltpu

F32, BF16, I32 = jnp.float32, jnp.bfloat16, jnp.int32

L = 2048
D = 640
NG = D // 128
UNIT = 256
SEG = 16
R = UNIT // SEG
LEAD = L // UNIT - NG
BU_PART = 9 * 2 * R
YS_ROWS = SEG * (R + 1)
KF_PAD = 8


class _Signed:
    def __init__(self, v, neg=False):
        self.v, self.neg = v, neg

    def __neg__(self):
        return _Signed(self.v, not self.neg)

    def __add__(self, o):
        if self.neg == o.neg:
            return _Signed(self.v + o.v, self.neg)
        return _Signed(o.v - self.v if self.neg else self.v - o.v)

    def __sub__(self, o):
        return self + (-o)

    def __mul__(self, c):
        return _Signed(self.v * np.float32(-c if self.neg else c))

    def get(self):
        return -self.v if self.neg else self.v


def _rot(re, im, num, den):
    num %= den
    h = math.sqrt(0.5)
    if num == 0:
        return re, im
    if 4 * num == den:
        return -im, re
    if 4 * num == 3 * den:
        return im, -re
    if 8 * num == den:
        return (re - im) * h, (re + im) * h
    if 8 * num == 3 * den:
        return (re + im) * (-h), (re - im) * h
    if 8 * num == 5 * den:
        return (im - re) * h, (re + im) * (-h)
    if 8 * num == 7 * den:
        return (re + im) * h, (im - re) * h
    c = math.cos(2 * math.pi * num / den)
    s = math.sin(2 * math.pi * num / den)
    return re * c - im * s, re * s + im * c


def _dft4(z, sign):
    (r0, i0), (r1, i1), (r2, i2), (r3, i3) = z
    ar, ai, br, bi = r0 + r2, i0 + i2, r0 - r2, i0 - i2
    cr, ci, dr, di = r1 + r3, i1 + i3, r1 - r3, i1 - i3
    plus, minus = (br - di, bi + dr), (br + di, bi - dr)
    if sign < 0:
        plus, minus = minus, plus
    return [(ar + cr, ai + ci), plus, (ar - cr, ai - ci), minus], [ai.v, ci.v]


def _fwd1(n0, u):
    a, b = u[:4], u[4:]
    r = [_rot(a[m], b[m], n0 + 4 * m, 64) for m in range(4)]
    z, halves = _dft4(r, 1)
    out = [_rot(*z[k], n0 * k, 16) for k in range(4)]
    s2 = [a[m] + b[m] for m in range(4)]
    d2 = [a[m] - b[m] for m in range(4)]
    p = _rot(d2[0], d2[2], n0, 32)
    q = _rot(d2[1], d2[3], n0 + 4, 32)
    out.append((p[0] + q[0], p[1] + q[1]))
    out.append(_rot(p[0] - q[0], p[1] - q[1], n0, 8))
    s3 = [s2[0] + s2[2], s2[1] + s2[3]]
    d3 = [s2[0] - s2[2], s2[1] - s2[3]]
    out.append(_rot(d3[0], d3[1], n0, 16))
    out.append((s3[0] + s3[1], s3[0] - s3[1]))
    return out, halves


def _fwd2(grp, z):
    if grp < 7:
        return _dft4(z, 1)[0]
    s4 = [t[0] for t in z]
    d4 = [t[1] for t in z]
    p = (d4[0], d4[2])
    q = _rot(d4[1], d4[3], 1, 8)
    s5 = [s4[0] + s4[2], s4[1] + s4[3]]
    return [
        (s5[0] + s5[1], s5[0] - s5[1]),
        (s4[0] - s4[2], s4[1] - s4[3]),
        (p[0] + q[0], p[1] + q[1]),
        (p[0] - q[0], p[1] - q[1]),
    ]


def _inv2(grp, w):
    if grp < 7:
        return _dft4(w, -1)[0]
    s5 = [w[0][0] + w[0][1], w[0][0] - w[0][1]]
    s4 = [s5[0] + w[1][0], s5[1] + w[1][1], s5[0] - w[1][0], s5[1] - w[1][1]]
    p = (w[2][0] + w[3][0], w[2][1] + w[3][1])
    q = _rot(w[2][0] - w[3][0], w[2][1] - w[3][1], -1, 8)
    d4 = [p[0], q[0], p[1], q[1]]
    return [(s4[n], d4[n]) for n in range(4)]


def _inv1(n0, z):
    t, _ = _dft4([_rot(*z[k], -n0 * k, 16) for k in range(4)], -1)
    ab = [_rot(*t[m], -(n0 + 4 * m), 64) for m in range(4)]
    e = _rot(*z[5], -n0, 8)
    p = _rot(z[4][0] + e[0], z[4][1] + e[1], -n0, 32)
    q = _rot(z[4][0] - e[0], z[4][1] - e[1], -(n0 + 4), 32)
    d2 = [p[0], q[0], p[1], q[1]]
    d3 = _rot(*z[6], -n0, 16)
    s3 = [z[7][0] + z[7][1], z[7][0] - z[7][1]]
    s2 = [s3[0] + d3[0], s3[1] + d3[1], s3[0] - d3[0], s3[1] - d3[1]]
    e2 = [s2[m] + d2[m] for m in range(4)]
    a = [ab[m][0] + e2[m] for m in range(4)]
    b = [ab[m][1] + (s2[m] - d2[m]) for m in range(4)]
    return a + b, [t[0][0].v + t[1][1].v, e2[0].v]


_F1 = [4 * (g + 4 * k) + 1 for g in range(4) for k in range(4)]
_F1 += [2 * (4 * (g + 2 * k) + 1) for g in range(2) for k in range(4)]
_F1 += [4 * (4 * k + 1) for k in range(4)]
_F1 += [0, 16, 8, 40]
_REAL_SLOT = 28


def _dft_tables():
    kap = np.arange(128)
    j = 8 * (kap // 16) + kap % 8
    part = (kap // 8) % 2
    pr, pc, jr, jc = part[:, None], part[None, :], j[:, None], j[None, :]
    lo = 2 * np.pi * jr * jc / 64
    base = np.where(pr == pc, np.cos(lo), np.where(pr == 0, -np.sin(lo), np.sin(lo)))
    hi = 2 * np.pi * (32 + 64 * (jr - 32)) * jc / 4096
    v0 = np.where(pr == 0, np.cos(lo), np.where(jr == 0, np.cos(np.pi * jc), np.sin(lo)))
    v32 = np.where(pr == 0, np.cos(hi), np.sin(hi))
    real = np.where(jr < 32, np.where(pc == 0, v0, 0.0), np.where(pc == 1, v32, 0.0))
    th = 2 * np.pi * np.outer(np.array(_F1), j) / 4096
    zeros = np.zeros((8, 128))
    return np.concatenate([base, real, np.cos(th), np.sin(th), zeros]).astype(np.float32)


_TABLES = _dft_tables()
_FFT_SCALE = 2.0 ** -11

(P_MU, P_RHO, P_RHO1, P_RHO2, P_RHO4, P_TAP, P_SSMD, P_DSKIP, P_COEF, P_ROWS) = (
    0, 2, 4, 6, 8, 10, 14, 15, 16, 20)
S_SMALL, S_F0, S_K0, S_C, S_OUT, S_B, S_COL, S_END = 0, 1, 2, 3, 4, 5, 8, 8 + NG - 1


Y128 = [(0, 128, 128)] + [(n, t, 128) for n in range(1, 4) for t in (0, 128)] + [
    (4, 0, 128), (4, 128, 96), (4, 224, 32)]
Y_LAST = [(n, t, 128) for n in range(4) for t in (0, 128)] + [(4, 0, 128), (4, 128, 96), (4, 224, 32)]


def _cmul(a, b):
    return a[0] * b[0] - a[1] * b[1], a[0] * b[1] + a[1] * b[0]


def _pack(lo, hi):
    return jnp.concatenate([lo, hi], axis=0).astype(BF16)


def _unpack(w):
    v = pltpu.bitcast(w, BF16).astype(F32)
    return v[:8], v[8:]


CFG = dict(scan=22, u=28, k1=24, p2=0, inv=44, skip=28, tail=5, kconv=28, steps=2, p2n=8,
           early=60, kwin=(44, 230), tr=(20, 40), wid=(16, 200), scanw=(0, 250), invw=(230, 400),
           k2w=(230, 400), mf=128, mi=128, bsz0=[64] * 4, bsz1=[64] * 4, m0=14,
           p1ties=(3, 7), kskip=1, skipme=lambda n, rows: False)


class _Gate:
    def __init__(self, pred=None, seen=()):
        self.pred, self.seen = pred, seen

    def early(self, lag):
        old = [e for e in self.seen if e[0] <= -lag]
        return max(old, key=lambda e: e[0])[1] if lag and old else None

    def value(self, v, lag):
        early = self.early(lag)
        return v if early is None else jnp.where(self.pred, v, early)

    def loads(self, ref, lag):
        early = self.early(lag)
        if early is not None:
            ref[pl.ds(ref.shape[0] - 8, 8), :] = (
                early if ref.dtype == F32 else pltpu.bitcast(early, I32))


def _weave(passes, plan, pred):
    if CFG["skipme"](len(passes), sum(q[0] for q in passes)):
        return
    begin, clock = [], [0] * 4
    for i, (n, *_) in enumerate(passes):
        begin.append(clock[i % 4] / 16)
        clock[i % 4] += n

    def index(t):
        later = [i for i, b in enumerate(begin) if b >= t - 3.999]
        if not later:
            return len(passes)
        same = [i for i in later if begin[i] == min(begin[j] for j in later)]
        return same[min(max(int((t - begin[same[0]]) / 4 * len(same)), 0), len(same) - 1)]

    at = [[] for _ in range(len(passes) + 1)]
    for tasks, lo, hi in plan:
        total, done = sum(sum(c) for c, _ in tasks) or 1, 0.0
        for costs, fn in tasks:
            where = []
            for cost in costs:
                done += cost
                where.append(index(lo + done / total * (hi - lo)))
            at[min(where)].append((fn, where))
    seen, ties = [], [[] for _ in at]
    for i, fns in enumerate(at):
        now = (begin[i] + i % 4) if i < len(begin) else clock[0] / 16
        early = [(t - now, v) for t, v in seen]
        for fn, where in fns:
            for w, tie in zip(where, fn(_Gate(pred, early)) or ()):
                ties[w].append(tie)
        if i == len(passes):
            break
        n, lhs, rhs, consume = passes[i]
        w = rhs()
        for tie in ties[i]:
            w[-1] = jnp.where(pred, w[-1], tie if tie.dtype == I32 else pltpu.bitcast(tie, I32))
        d = jnp.dot(pltpu.bitcast(jnp.concatenate(lhs(), axis=0), BF16),
                    pltpu.bitcast(jnp.concatenate(w, axis=0), BF16), preferred_element_type=F32)
        seen += [(begin[i] + i % 4 + j // 16 - 4, d[j - 8:j]) for j in range(64, n + 1, 64)]
        consume(d)


def _now(tasks):
    for _, fn in tasks:
        fn(_Gate())


def _kernel(tab_hbm, x_hbm, lre_hbm, lim_hbm, bre_hbm, bim_hbm, cre_hbm, cim_hbm,
            ldt_hbm, dsk_hbm, q_hbm, k_hbm, v_hbm, tap_hbm, sk_hbm, sd_hbm,
            o_hbm,
            tab, lre_v, lim_v, ldt_v, dsk_v, sd_v, tap_v,
            xb, braw, craw, qb, kb, vb, skb,
            par, wb16, wc, mf16, mi, bu, hb16, carry, ys, oa,
            kt, kf, st_u, st_k, st_i, vu16, vk16, pb0, pb1, ob,
            sem):
    x32, q32, k32, v32, wb, mf, hb, vu, vk = (
        r.bitcast(I32) for r in (xb, qb, kb, vb, wb16, mf16, hb16, vu16, vk16))
    pb16 = (pb0, pb1)
    pb = (pb0.bitcast(I32), pb1.bitcast(I32))

    def rows(ref, start, n=8):
        return ref[pl.ds(start, n), :]

    def hint(v, n):
        return v if isinstance(v, int) else pl.multiple_of(v, n)

    def view(ref, start, n=None):
        return ref.at[pl.ds(hint(start, 16), n or ref.shape[0]), :]

    small = [pltpu.make_async_copy(s, d, sem.at[S_SMALL]) for s, d in (
        (lre_hbm, lre_v), (lim_hbm, lim_v), (ldt_hbm, ldt_v),
        (dsk_hbm, dsk_v), (sd_hbm, sd_v), (tap_hbm, tap_v),
        (tab_hbm.at[pl.ds(320, 8), :], tab.at[pl.ds(320, 8), :]))]
    tab_dma = pltpu.make_async_copy(
        tab_hbm.at[pl.ds(0, 320), :], tab.at[pl.ds(0, 320), :], sem.at[S_F0])

    def x_dma(u):
        return [pltpu.make_async_copy(
            x_hbm.at[pl.ds(hint(u * UNIT, UNIT), UNIT), pl.ds(128 * n, 128)],
            xb.at[pl.ds(hint(n * L + u * UNIT, UNIT), UNIT), :], sem.at[(S_B, S_F0, S_K0)[u] if isinstance(u, int) and u < LEAD
                                                     else S_COL + u - LEAD])
            for n in range(NG)]

    def b_dma(p):
        return [pltpu.make_async_copy(
            src.at[pl.ds(128 * p, 128), :], braw.at[pl.ds(D * c + 128 * p, 128), :],
            sem.at[S_B + (p + 1) // 2]) for c, src in enumerate((bre_hbm, bim_hbm))]

    c_dma = [pltpu.make_async_copy(
        src.at[:, pl.ds(128 * p, 128)], craw.at[pl.ds(D * (NG * c + p), D), :],
        sem.at[S_C]) for c, src in enumerate((cre_hbm, cim_hbm)) for p in range(NG)]

    def col_dma(which, g, sem_at):
        src, dst = ((k_hbm, kb), (v_hbm, vb), (q_hbm, qb))[which]
        return pltpu.make_async_copy(
            src.at[:, pl.ds(hint(128 * g, 128), 128)],
            dst.at[pl.ds(hint(L * g, L), L), :], sem.at[sem_at])

    def sk_dma(g, sem_at):
        t = hint(128 * g, 128)
        return pltpu.make_async_copy(
            sk_hbm.at[pl.ds(hint(128 * g, 128), 128), :], skb.at[pl.ds(t, 128), :],
            sem.at[sem_at])

    def oa_dma(u, n):
        t = hint(u * UNIT, UNIT)
        return pltpu.make_async_copy(
            oa.at[pl.ds(t, UNIT), pl.ds(128 * n, 128)],
            o_hbm.at[pl.ds(t, UNIT), pl.ds(128 * n, 128)], sem.at[S_OUT])

    def oa_unit_dma(u):
        t = hint(u * UNIT, UNIT)
        return pltpu.make_async_copy(
            oa.at[pl.ds(t, UNIT), :], o_hbm.at[pl.ds(t, UNIT), pl.ds(0, D)], sem.at[S_OUT])

    def ob_dma(g):
        return pltpu.make_async_copy(
            ob.at[pl.ds(hint(L * g, L), L), :],
            o_hbm.at[:, pl.ds(hint(D + 128 * g, 128), 128)], sem.at[S_OUT])

    def start(ds):
        for d in ds:
            d.start()

    def wait(ds):
        for d in ds:
            d.wait()

    def prm(g, row):
        return rows(view(par, g * (P_ROWS * 8), P_ROWS * 8), row * 8)

    def bu_passes(u, slot, z=0, sizes=None):
        out = []
        xu, w = view(x32, u * (UNIT // 2), ((NG - 1) * L + UNIT) // 2), view(wb, z)
        sizes = sizes or [64] * (UNIT // 64)
        for n in (p + c * NG for p in range(NG) for c in range(2)):
            for m, MM in zip(np.cumsum([0] + sizes).tolist(), sizes):
                acc = []
                for kk in range(NG):
                    def lhs(m=m, kk=kk, MM=MM):
                        t = (kk * L + m) // 2
                        return [rows(xu, t + 8 * i) for i in range(MM // 16)]

                    def rhs(n=n, kk=kk):
                        return [rows(w, (n * NG + kk) * 64 + 8 * i) for i in range(8)]

                    def consume(d, m=m, n=n, kk=kk, acc=acc, MM=MM):
                        acc.append(d if kk == 0 else acc[-1] + d)
                        if kk == NG - 1:
                            for i in range(MM // 8):
                                seg, r = divmod(m + 8 * i, R)
                                row = 9 * (seg % 2 * R + r) + seg // 2
                                bu[pl.ds((slot * 2 * NG + n) * BU_PART + row, 8, stride=9), :] = (
                                    acc[-1][8 * i:8 * i + 8])
                    out.append((MM, lhs, rhs, consume))
        return out

    def scan_tasks(u, slot, z):
        steps = CFG["steps"]
        state = {}
        hu = view(hb16, u * UNIT, (2 * NG - 1) * L + UNIT)

        def b(p, ch, r):
            return tuple(rows(bu, (slot * 2 * NG + c * NG + p) * BU_PART + 9 * (ch * R + r))
                         for c in range(2))

        def step(mu, h, br):
            return (mu[0] * h[0] + br[0]) - mu[1] * h[1], (mu[0] * h[1] + br[1]) + mu[1] * h[0]

        def ends(p, gate):
            mu, ties = (gate.value(prm(p, P_MU), CFG["scan"]), prm(p, P_MU + 1)), []
            h = [b(p, ch, 0) for ch in range(2)]
            for r in range(1, R):
                h = [step(mu, h[ch], b(p, ch, r)) for ch in range(2)]
                if r % steps == 0:
                    ties.append(h[r // steps % 2][0])
            state[p] = starts(p, h)
            return ties + [state[p][1][0]]

        def starts(p, e):
            last = lax.broadcasted_iota(I32, (8, 128), 0) == 7
            rho = (prm(p, P_RHO), prm(p, P_RHO + 1))
            pair = step(rho, e[0], e[1])
            a = tuple(pltpu.roll(jnp.where(last, rows(carry, (2 * p + c) * 8), pair[c]), 1, 0)
                      for c in range(2))
            for sh, row in ((1, P_RHO1), (2, P_RHO2), (4, P_RHO4)):
                a = step((prm(p, row), prm(p, row + 1)), tuple(pltpu.roll(c, sh, 0) for c in a), a)
            return [a, step(rho, a, e[0])]

        def run(p, r0, gate):
            if r0 == 0:
                state["mu"] = (prm(p, P_MU), prm(p, P_MU + 1))
            mu, h = (gate.value(state["mu"][0], CFG["scan"]), state["mu"][1]), state[p]
            for r in range(r0, r0 + steps):
                h = [step(mu, h[ch], b(p, ch, r)) for ch in range(2)]
                for c in range(2):
                    hu[pl.ds((c * NG + p) * L + 16 * r, 16), :] = _pack(h[0][c], h[1][c])
            state[p] = h
            if r0 + steps == R:
                for c in range(2):
                    carry[pl.ds((2 * p + c) * 8, 8), :] = h[1][c]
            return [rows(view(hb, z, 8), 0)]

        tasks = []
        for p in range(NG):
            tasks.append(([16 * steps] * ((R - 1) // steps) + [46 + 16 * steps],
                          lambda gate, p=p: ends(p, gate)))
            tasks += [([18 * steps], lambda gate, p=p, r0=r0: run(p, r0, gate))
                      for r0 in range(0, R, steps)]
        return tasks

    def y_tiles(MM):
        return [(n, t, MM) for n in range(NG) for t in range(0, UNIT, MM)]

    def y_passes(u, tiles, z=0):
        out, w = [], view(wc, z)
        hu = view(hb, u * (UNIT // 2), ((2 * NG - 1) * L + UNIT) // 2)
        if True:
            for n, t0, MM in tiles:
                acc = []
                for kk in range(2 * NG):
                    def lhs(t0=t0, kk=kk, MM=MM):
                        t = kk * (L // 2) + t0 // 2
                        return [rows(hu, t + 8 * i) for i in range(MM // 16)]

                    def rhs(n=n, kk=kk):
                        return [rows(w, (kk * NG + n) * 64 + 8 * i) for i in range(8)]

                    def consume(d, t0=t0, n=n, kk=kk, acc=acc, MM=MM):
                        acc.append(d if kk == 0 else acc[-1] + d)
                        if kk == 2 * NG - 1:
                            for i in range(MM // 8):
                                r, ch = divmod(t0 // 8 + i, 2)
                                ys[pl.ds(n * YS_ROWS + ch * (R + 1) + r, 8, stride=2 * (R + 1)), :] = (
                                    acc[-1][8 * i:8 * i + 8])
                    out.append((MM, lhs, rhs, consume))
        return out

    def skip_task(u, n, z):
        def fn(gate):
            dsk = gate.value(prm(n, P_DSKIP), CFG["skip"])
            xu, ou = view(x32, u * (UNIT // 2) + n * (L // 2), UNIT // 2), view(oa, u * UNIT, UNIT)
            ties = []
            for i in range(UNIT // 16):
                xs = _unpack(rows(xu, 8 * i))
                for c in range(2):
                    t = 16 * i + 8 * c
                    y = rows(ys, n * YS_ROWS + (t // R) * (R + 1) + t % R)
                    ou[pl.ds(t, 8), pl.ds(128 * n, 128)] = y + xs[c] * dsk
                if i % 4 == 3:
                    ties.append(view(oa, z + u * UNIT, 8)[:, pl.ds(128 * n, 128)])
            return ties
        return ([24] * (UNIT // 64), fn)

    def widen_tasks(g, z, pieces=2):
        def fn(i0, i1):
            kg = view(k32, g * (L // 2), L // 2)
            for i in range(i0, i1):
                lo, hi = _unpack(rows(kg, 8 * i))
                kf[pl.ds(KF_PAD + 16 * i, 8), :] = lo
                kf[pl.ds(KF_PAD + 16 * i + 8, 8), :] = hi
            return [rows(view(kf, z), 16 * i0 + KF_PAD)]
        n = L // 16 // pieces
        return [([2 * n], lambda gate, i=i: fn(i * n, (i + 1) * n)) for i in range(pieces)]

    def transpose_tasks(g, z, pieces=8):
        def fn(c0, c1):
            for c in range(c0, c1):
                t = skb[pl.ds(hint(128 * g, 128), 128), pl.ds(128 * c, 128)]
                kt[pl.ds(64 * c, 64), :] = pltpu.bitcast(t.T, I32)
            return [rows(view(kt, z), 64 * c0)]
        n = L // 128 // pieces
        return [([8 * n], lambda gate, i=i: fn(i * n, (i + 1) * n)) for i in range(pieces)]

    def pass1(st, s, n0, u, z):
        pairs, ties = _fwd1(n0, [_Signed(v) for v in u])
        for grp, pair in enumerate(pairs):
            for c in range(2):
                st[pl.ds(((s * 4 + n0) * 8 + grp) * 16 + 8 * c, 8), :] = pair[c].get()
            if grp in CFG["p1ties"]:
                ties.append(rows(view(st, z), (s * 4 + n0) * 128))
        return ties

    def rest_costs(n0):
        each = np.array([14, 14, 14, 14, 30, 8, 12, 4]) * ((54, 96, 80, 96)[n0] - 16) / 110
        cut = np.cumsum(each)[list(CFG["p1ties"])]
        return np.diff(cut, prepend=0).tolist()

    def u1_task(g, s, n0, z):
        def fn(gate):
            taps = [prm(g, P_TAP + t) for t in range(4)]
            taps[0] = gate.value(taps[0], CFG["u"])
            u, kz, vg = [], view(kf, z), view(v32, g * (L // 2), L // 2)
            for m in range(8):
                t = 64 * (n0 + 4 * m) + 8 * s
                ks = rows(kz, KF_PAD + t) * taps[0]
                for lag in range(1, 4):
                    ks = ks + rows(kz, KF_PAD + t - lag) * taps[lag]
                v = _unpack(rows(vg, (t // 16) * 8))[s % 2]
                u.append(ks * v)
            return pass1(st_u, s, n0, u, z)
        return ([40, 40] + rest_costs(n0), fn)

    def k1_task(g, s, n0, z):
        def fn(gate):
            gate.loads(kt, CFG["k1"])
            u = [_unpack(rows(view(kt, z), 32 * (n0 + 4 * m) + 8 * (s // 2)))[s % 2] for m in range(8)]
            if s == 0 and n0 == 0:
                first = lax.broadcasted_iota(I32, (8, 128), 0) == 0
                u[0] = u[0] + jnp.where(first, prm(g, P_SSMD), 0.0)
            return pass1(st_k, s, n0, u, z)[CFG["kskip"]:]
        costs = [11, 11] + rest_costs(n0)
        return ([sum(costs[:CFG["kskip"] + 1])] + costs[CFG["kskip"] + 1:], fn)

    def pass2_task(st, dst16, dst, s, grps, z):
        def fn(gate):
            gate.loads(st, CFG["p2"])
            for grp in grps:
                zs = [tuple(_Signed(rows(view(st, z), ((s * 4 + n0) * 8 + grp) * 16 + 8 * c)) for c in range(2))
                      for n0 in range(4)]
                for k, pair in enumerate(_fwd2(grp, zs)):
                    dst16[pl.ds((4 * grp + k) * 128 + 16 * s, 16), :] = _pack(pair[0].get(), pair[1].get())
            return [rows(view(dst, z), 4 * grps[0] * 64 + 8 * s)]
        return ([20 * len(grps)], fn)

    def pass2_tasks(st, s, z):
        dst = (vu16, vu) if st is st_u else (vk16, vk)
        return [pass2_task(st, *dst, s, g, z) for g in np.arange(8).reshape(CFG["p2n"], -1).tolist()]

    def fwd_passes(grp, z):
        out, MM = [], CFG["mf"]
        for slot in range(4 * grp, 4 * grp + 4):
            got = {}
            for half in range(128 // MM):
                for which, src in enumerate((vu, vk)):
                    def lhs(slot=slot, half=half):
                        return [rows(mf, slot * 64 + MM // 2 * half + 8 * i) for i in range(MM // 16)]

                    def rhs(slot=slot, src=src):
                        return [rows(view(src, z), slot * 64 + 8 * i) for i in range(8)]

                    def consume(d, slot=slot, half=half, which=which, got=got):
                        got[which] = d
                        if which == 0:
                            return
                        for i in range(MM // 16):
                            a = (got[0][16 * i:16 * i + 8], got[0][16 * i + 8:16 * i + 16])
                            b = (d[16 * i:16 * i + 8], d[16 * i + 8:16 * i + 16])
                            re, im = _cmul(a, b)
                            if slot == _REAL_SLOT and half == 0 and i == 0:
                                first = lax.broadcasted_iota(I32, (8, 128), 0) == 0
                                re = jnp.where(first, 0.5 * (a[0] * b[0]), re)
                                im = jnp.where(first, 0.5 * (a[1] * b[1]), im)
                            pb16[grp % 2][pl.ds(slot % 4 * 128 + MM * half + 16 * i, 16), :] = (
                                _pack(re, im))
                    out.append((MM, lhs, rhs, consume))
        return out

    def inv_passes(grp, z):
        out, MM = [], CFG["mi"]
        for half in range(128 // MM):
            got = []
            for slot in range(4 * grp, 4 * grp + 4):
                def lhs(slot=slot, half=half):
                    return [rows(mi, slot * 64 + MM // 2 * half + 8 * i) for i in range(MM // 16)]

                def rhs(slot=slot):
                    return [rows(view(pb[grp % 2], z), slot % 4 * 64 + 8 * i) for i in range(8)]

                def consume(d, half=half, got=got):
                    got.append(d)
                    if len(got) < 4:
                        return
                    for i in range(MM // 16):
                        w = [(_Signed(t[16 * i:16 * i + 8]), _Signed(t[16 * i + 8:16 * i + 16]))
                             for t in got]
                        for n0, pair in enumerate(_inv2(grp, w)):
                            for c in range(2):
                                at = (((MM // 16 * half + i) * 4 + n0) * 8 + grp) * 16 + 8 * c
                                st_i[pl.ds(at, 8), :] = pair[c].get()
                out.append((MM, lhs, rhs, consume))
        return out

    def inv1_task(g, s, n0, z):
        def fn(gate):
            gate.loads(st_i, CFG["inv"])
            zs = [tuple(_Signed(rows(view(st_i, z), ((s * 4 + n0) * 8 + grp) * 16 + 8 * c)) for c in range(2))
                  for grp in range(8)]
            qg, og = view(q32, g * (L // 2), L // 2), view(ob, g * L, L)
            ys8, ties = _inv1(n0, zs)
            for m in (0, 4, 2, 6, 1, 5, 3, 7):
                t = 64 * (n0 + 4 * m) + 8 * s
                qv = _unpack(rows(qg, (t // 16) * 8))[s % 2]
                og[pl.ds(t, 8), :] = qv * ys8[m].get()
                if m in (6, 7):
                    ties.append(rows(view(ob, z + g * L, L), 64 * n0 + 8 * s))
            return ties
        quarter = (16 + (62, 104, 88, 104)[n0]) // 4
        return ([quarter, quarter - 8, quarter + 4, quarter + 4], fn)

    filter0 = x_dma(1) + [sk_dma(0, S_F0), tab_dma]
    data0 = x_dma(2) + [col_dma(0, 0, S_K0), col_dma(1, 0, S_K0)]

    def group_dma(g):
        at = S_COL + g
        return [col_dma(2, g, at), sk_dma(g + 1, at), col_dma(0, g + 1, at),
                col_dma(1, g + 1, at)] + x_dma(g + LEAD)

    last_dma = [col_dma(2, NG - 1, S_SMALL)] + [pltpu.make_async_copy(
        x_hbm.at[pl.ds(L - UNIT, UNIT), pl.ds(128 * n, 128)],
        xb.at[pl.ds(n * L + L - UNIT, UNIT), :], sem.at[S_SMALL]) for n in range(NG)]

    start(small + x_dma(0) + b_dma(0))
    wait(small)
    zeros = rows(tab, 320).astype(I32)
    z8 = pl.multiple_of(zeros[0, 0], 16)
    sub = lax.broadcasted_iota(I32, (8, 128), 0)
    pred = zeros == 0

    def stack(ref):
        v = ref[...].astype(F32).reshape(1, D)
        return jnp.concatenate([v[:, 128 * g:128 * (g + 1)] for g in range(NG)]
                               + [v[:, :128]] * (8 - NG), axis=0)

    lre, lim = stack(lre_v), stack(lim_v)
    dt = jnp.exp(stack(ldt_v)).astype(BF16).astype(F32)
    mag, ang = jnp.exp(dt * lre), dt * lim
    lam = (mag * jnp.cos(ang), mag * jnp.sin(ang))
    scale = jnp.maximum(jnp.abs(lre), jnp.abs(lim))
    nre, nim = lre / scale, lim / scale
    den = (nre * nre + nim * nim) * scale
    coef = _cmul(((lam[0] - 1.0) / den, lam[1] / den), (nre, -nim))
    mu = (lam[0], -lam[1])
    rho = [mu]
    for _ in range(R.bit_length() + 2):
        rho.append(_cmul(rho[-1], rho[-1]))
    dsk, ssd = stack(dsk_v), stack(sd_v)
    taps = tap_v[...].astype(F32) * _FFT_SCALE
    for g in range(NG):
        def put(row, v):
            par[pl.ds((g * P_ROWS + row) * 8, 8), :] = v

        def lanes(v):
            return jnp.broadcast_to(v[g:g + 1], (8, 128))
        for c in range(2):
            put(P_MU + c, lanes(mu[c]))
            put(P_RHO + c, lanes(rho[-4][c]))
            for n, row in enumerate((P_RHO1, P_RHO2, P_RHO4)):
                put(row + c, jnp.where(sub >= 1 << n, lanes(rho[n - 3][c]), 0.0))
        for t in range(4):
            put(P_TAP + t, jnp.broadcast_to(taps[t:t + 1, 128 * g:128 * (g + 1)], (8, 128)))
        put(P_COEF, lanes(2.0 * coef[0]))
        put(P_COEF + 1, lanes(-2.0 * coef[0]))
        put(P_COEF + 2, lanes(2.0 * coef[1]))
        put(P_SSMD, lanes(ssd))
        put(P_DSKIP, lanes(dsk))
    for i in range(2 * NG):
        carry[pl.ds(8 * i, 8), :] = jnp.zeros((8, 128), F32)
    kf[pl.ds(0, KF_PAD), :] = jnp.zeros((KF_PAD, 128), F32)

    def matrix_task(slot):
        def fn(gate):
            if slot != _REAL_SLOT:
                c, s = tab[pl.ds(256 + slot, 1), :], tab[pl.ds(288 + slot, 1), :]
            for a in range(8):
                if slot == _REAL_SLOT:
                    re, im = rows(tab, 128 + 16 * a), rows(tab, 128 + 16 * a + 8)
                else:
                    br, bi = rows(tab, 16 * a), rows(tab, 16 * a + 8)
                    re, im = c * br - s * bi, s * br + c * bi
                mf16[pl.ds(slot * 128 + 16 * a, 16), :] = _pack(re, im)
            m = pltpu.bitcast(rows(view(mf, z8), slot * 64, 64), BF16)
            mi[pl.ds(slot * 64, 64), :] = pltpu.bitcast(m.T, I32)
            return [rows(view(mf, z8), 0), rows(view(mi, z8), slot * 64)]
        return ([48, 8], fn)

    def scale_b(p, kk):
        cr, ncr, ci = prm(p, P_COEF), prm(p, P_COEF + 1), prm(p, P_COEF + 2)
        br, bi = (braw[pl.ds(D * c + 128 * p, 128), pl.ds(128 * kk, 128)].T.astype(F32)
                  for c in range(2))
        ties = []
        for i in range(8):
            r0, r1 = br[16 * i:16 * i + 8], br[16 * i + 8:16 * i + 16]
            i0, i1 = bi[16 * i:16 * i + 8], bi[16 * i + 8:16 * i + 16]
            wb16[pl.ds((p * NG + kk) * 128 + 16 * i, 16), :] = _pack(
                cr * r0 - ci * i0, cr * r1 - ci * i1)
            wb16[pl.ds(((NG + p) * NG + kk) * 128 + 16 * i, 16), :] = _pack(
                ncr * i0 - ci * r0, ncr * i1 - ci * r1)
            if i % 2:
                ties.append(rows(view(wb, z8), ((NG + p) * NG + kk) * 64))
        return ties

    def c_task(n, k0, k1):
        def fn(gate):
            for kk in range(k0, k1):
                t = craw[pl.ds(kk * D + 128 * n, 128), :]
                wc[pl.ds((kk * NG + n) * 64, 64), :] = pltpu.bitcast(t.T, I32)
            return [rows(view(wc, z8), ((k1 - 1) * NG + n) * 64)]
        return ([16], fn)

    first = bu_passes(0, 0, z8, CFG["bsz0"])
    first = [first[len(first) // NG * p:len(first) // NG * (p + 1)] for p in range(NG)]

    mats = [matrix_task(slot) for slot in range(32)]

    def scale_tasks(p):
        return [([36] * 4, lambda gate, kk=kk: scale_b(p, kk)) for kk in range(NG)]

    def dma_task(ds):
        return ([1], lambda gate: start(ds))

    def filter_tasks(g, slot):
        k1, k2 = [], []
        for s in range(8):
            k1 += [k1_task(g, s, n0, z8) for n0 in range(4)]
            k2 += pass2_tasks(st_k, s, z8)
        return transpose_tasks(slot, z8), k1, k2

    def forward_tasks(u, g):
        tasks = []
        for s in range(8):
            tasks += [u1_task(g, s, n0, z8) for n0 in range(4)] + pass2_tasks(st_u, s, z8)
        return tasks, [skip_task(u, n, z8) for n in range(NG)]

    per_n = 2 * NG * UNIT // 64
    total = NG * per_n

    start(b_dma(1) + b_dma(2))
    wait(x_dma(0) + b_dma(0))
    start(b_dma(3) + b_dma(4) + filter0)
    _now(scale_tasks(0))
    _weave(first[0], [], pred)
    start(data0)
    wait(b_dma(1) + b_dma(2))
    _now(scale_tasks(1))
    _weave(first[1] + first[2], [(scale_tasks(2), 0, 40)], pred)
    start(c_dma)
    wait(b_dma(3) + b_dma(4))
    _now(scale_tasks(3))
    _weave(first[3] + first[4], [(scale_tasks(4), 0, 40)], pred)
    start(group_dma(0))
    wait(filter0)
    tr, k1, k2 = filter_tasks(0, 0)
    nm = CFG["m0"]
    _weave(bu_passes(1, 1, 0, CFG["bsz1"]), [
        (scan_tasks(0, 0, z8), 0, total), (mats[:nm], 0, total), (tr, 8, 32),
        (k1, 36, total)], pred)
    start(group_dma(1))
    wait(data0)
    fwd, skips = forward_tasks(0, 0)
    _weave(bu_passes(2, 0, 0, CFG["bsz1"]), [
        (widen_tasks(0, z8, 8), 0, 20), (fwd[:-3], 20, total), (fwd[-3:], total, total)], pred)
    start(group_dma(2))
    wait(c_dma)
    cs = [c_task(n, k, k + 2) for n in range(NG) for k in range(0, 2 * NG, 2)]
    _now(cs[:NG])
    _weave(y_passes(0, y_tiles(64), z8), [
        (cs[n * NG:(n + 1) * NG], max(per_n * (n - 1) - 8, 0), per_n * n - 8) for n in range(1, NG)] + [
        (scan_tasks(1, 1, z8), 0, total), (k2, 0, total), (mats[nm:], 0, total)]
        + [(skips[n:n + 1], per_n * (n + 1) + 16, per_n * (n + 1) + 24) for n in range(NG - 1)], pred)
    start(group_dma(3) + last_dma)

    def conv_passes(lead):
        passes = fwd_passes(0, z8)
        for grp in range(1, 8):
            passes += fwd_passes(grp, z8) + inv_passes(grp - 1, z8)
        return passes + lead[:8] + inv_passes(7, z8) + lead[8:]

    def body(i, _):
        wait(group_dma(i))
        passes = (conv_passes(y_passes(i + 1, [(0, 0, 32), (0, 32, 96)]))
                  + bu_passes(i + LEAD, 0, 0, [128, 128]) + y_passes(i + 1, Y128))
        y0, end = 192 + total + 20, 192 + 2 * total
        tr, k1, k2 = filter_tasks(i + 1, i + 1)
        fwd, skips = forward_tasks(i + 1, i + 1)
        inv = [inv1_task(i, s, n0, z8) for s in range(8) for n0 in range(4)]
        nk, tail = CFG["kconv"], CFG["tail"]
        _weave(passes, [
            (scan_tasks(i + LEAD - 1, 0, z8), *CFG["scanw"]), (tr, *CFG["tr"]),
            ([skip_task(i, NG - 1, z8), dma_task([oa_unit_dma(i)])], 12, 12),
            (widen_tasks(i + 1, z8, 16), *CFG["wid"]), (k1[:nk], *CFG["kwin"]),
            (inv + [dma_task([ob_dma(i)])], *CFG["invw"]), (k1[nk:] + k2, *CFG["k2w"]),
            (fwd[:-tail], y0 - CFG["early"], end), (fwd[-tail:], end, end)]
            + [(skips[n:n + 1], end - per_n * (NG - 1 - n) + 16, end - per_n * (NG - 1 - n) + 24)
               for n in range(NG - 1)], pred)
        return 0

    lax.fori_loop(0, NG - 1, body, 0)

    wait(last_dma)
    g, u0, last = NG - 1, NG, L // UNIT - 1
    passes = (conv_passes(y_passes(u0, [(0, 0, 32), (0, 32, 96)])) + bu_passes(last, 1, 0, [128, 128])
              + y_passes(u0, [(0, 128, 128)] + y_tiles(128)[2:]) + y_passes(u0 + 1, y_tiles(128))
              + y_passes(last, Y_LAST))
    y0 = 192 + total + 20
    plan = [(scan_tasks(last - 1, 0, z8), 0, 192),
            ([skip_task(g, NG - 1, z8), dma_task([oa_unit_dma(g)])], 12, 12),
            ([inv1_task(g, s, n0, z8) for s in range(8) for n0 in range(4)]
             + [dma_task([ob_dma(g)])], 230, y0 + total),
            (scan_tasks(last, 1, z8), y0 + 16, y0 + 2 * total - 40)]
    out = [oa_unit_dma(u) for u in range(u0)] + [ob_dma(n) for n in range(NG)]
    for u in range(u0, last + 1):
        for n in range(NG):
            where = y0 + (u - u0) * total + per_n * (n + 1)
            plan.append(([skip_task(u, n, z8), dma_task([oa_dma(u, n)])], where, where))
            out.append(oa_dma(u, n))
    _weave(passes, plan, pred)
    wait(out)


@jax.jit
def pallas_concat_heads__ssm_conv_s5__ssm_conv_h3__prompt_kernel(
    A_x: jax.Array,
    A_Lambda_re: jax.Array,
    A_Lambda_im: jax.Array,
    A_B_re: jax.Array,
    A_B_im: jax.Array,
    A_C_re: jax.Array,
    A_C_im: jax.Array,
    A_log_dt: jax.Array,
    A_Dskip: jax.Array,
    B_q: jax.Array,
    B_k: jax.Array,
    B_v: jax.Array,
    B_shift_k: jax.Array,
    B_ssm_k: jax.Array,
    B_ssm_D: jax.Array,
):
    assert A_x.shape == (1, L, D) and B_shift_k.shape == (D, 4)
    vmem = pltpu.VMEM
    dma = pltpu.SemaphoreType.DMA
    scratch = [
        vmem(_TABLES.shape, F32),
        vmem((D,), BF16), vmem((D,), BF16), vmem((D,), BF16), vmem((D,), BF16), vmem((D,), BF16),
        vmem((4, D), BF16),
        vmem((NG * L, 128), BF16),
        vmem((2 * D, D), BF16),
        vmem((2 * NG * D, 128), BF16),
        vmem((NG * L, 128), BF16),
        vmem((NG * L, 128), BF16),
        vmem((NG * L, 128), BF16),
        vmem((D, L), BF16),
        vmem((NG * P_ROWS * 8, 128), F32),
        vmem((2 * NG * D, 128), BF16),
        vmem((2 * NG * NG * 64, 128), I32),
        vmem((32 * 128, 128), BF16),
        vmem((32 * 64, 128), I32),
        vmem((2 * 2 * NG * BU_PART, 128), F32),
        vmem((2 * NG * L, 128), BF16),
        vmem((3 * NG * 8, 128), F32),
        vmem((NG * YS_ROWS, 128), F32),
        vmem((L, D), F32),
        vmem((L // 2 + 8, 128), I32),
        vmem((KF_PAD + L, 128), F32),
        vmem((2 * L + 8, 128), F32),
        vmem((2 * L + 8, 128), F32),
        vmem((2 * L + 8, 128), F32),
        vmem((32 * 128, 128), BF16),
        vmem((32 * 128, 128), BF16),
        vmem((4 * 128, 128), BF16),
        vmem((4 * 128, 128), BF16),
        vmem((NG * L, 128), F32),
        dma((S_END,)),
    ]
    out = pl.pallas_call(
        _kernel,
        out_shape=jax.ShapeDtypeStruct((L, 2 * D), F32),
        in_specs=[pl.BlockSpec(memory_space=pl.ANY)] * 16,
        out_specs=pl.BlockSpec(memory_space=pl.ANY),
        scratch_shapes=scratch,
        compiler_params=pltpu.CompilerParams(vmem_limit_bytes=100 * 1024 * 1024),
        name="s5_h3",
    )(_TABLES, A_x.reshape(L, D), A_Lambda_re, A_Lambda_im, A_B_re, A_B_im, A_C_re, A_C_im,
      A_log_dt, A_Dskip, B_q.reshape(L, D), B_k.reshape(L, D), B_v.reshape(L, D),
      B_shift_k.T, B_ssm_k, B_ssm_D)
    return out.reshape(1, L, 2 * D)
```

```python
import math

import jax
import jax.numpy as jnp
import numpy as np
from jax import lax
from jax.experimental import pallas as pl
from jax.experimental.pallas import tpu as pltpu

F32, BF16, I32 = jnp.float32, jnp.bfloat16, jnp.int32

L = 2048
D = 640
NG = D // 128
UNIT = 256
SEG = 16
R = UNIT // SEG
LEAD = L // UNIT - NG
BU_PART = 9 * 2 * R
YS_ROWS = SEG * (R + 1)
KF_PAD = 8


class _Signed:
    def __init__(self, v, neg=False):
        self.v, self.neg = v, neg

    def __neg__(self):
        return _Signed(self.v, not self.neg)

    def __add__(self, o):
        if self.neg == o.neg:
            return _Signed(self.v + o.v, self.neg)
        return _Signed(o.v - self.v if self.neg else self.v - o.v)

    def __sub__(self, o):
        return self + (-o)

    def __mul__(self, c):
        return _Signed(self.v * np.float32(-c if self.neg else c))

    def get(self):
        return -self.v if self.neg else self.v


def _rot(re, im, num, den):
    num %= den
    h = math.sqrt(0.5)
    if num == 0:
        return re, im
    if 4 * num == den:
        return -im, re
    if 4 * num == 3 * den:
        return im, -re
    if 8 * num == den:
        return (re - im) * h, (re + im) * h
    if 8 * num == 3 * den:
        return (re + im) * (-h), (re - im) * h
    if 8 * num == 5 * den:
        return (im - re) * h, (re + im) * (-h)
    if 8 * num == 7 * den:
        return (re + im) * h, (im - re) * h
    c = math.cos(2 * math.pi * num / den)
    s = math.sin(2 * math.pi * num / den)
    return re * c - im * s, re * s + im * c


def _dft4(z, sign):
    (r0, i0), (r1, i1), (r2, i2), (r3, i3) = z
    ar, ai, br, bi = r0 + r2, i0 + i2, r0 - r2, i0 - i2
    cr, ci, dr, di = r1 + r3, i1 + i3, r1 - r3, i1 - i3
    plus, minus = (br - di, bi + dr), (br + di, bi - dr)
    if sign < 0:
        plus, minus = minus, plus
    return [(ar + cr, ai + ci), plus, (ar - cr, ai - ci), minus]


def _fwd1(n, u):
    a0, a1, b0, b1 = u
    p, q = _rot(a0, b0, n, 32), _rot(a1, b1, n + 4, 32)
    s0, s1 = a0 + b0, a1 + b1
    return [(p[0] + q[0], p[1] + q[1]), _rot(p[0] - q[0], p[1] - q[1], n, 8),
            _rot(a0 - b0, a1 - b1, n, 16), (s0 + s1, s0 - s1)]


def _fwd2(grp, z):
    if grp < 3:
        return _dft4(z, 1)
    s4 = [t[0] for t in z]
    d4 = [t[1] for t in z]
    p = (d4[0], d4[2])
    q = _rot(d4[1], d4[3], 1, 8)
    s5 = [s4[0] + s4[2], s4[1] + s4[3]]
    return [
        (s5[0] + s5[1], s5[0] - s5[1]),
        (s4[0] - s4[2], s4[1] - s4[3]),
        (p[0] + q[0], p[1] + q[1]),
        (p[0] - q[0], p[1] - q[1]),
    ]


def _inv2(grp, w):
    if grp < 3:
        return _dft4(w, -1)
    s5 = [w[0][0] + w[0][1], w[0][0] - w[0][1]]
    s4 = [s5[0] + w[1][0], s5[1] + w[1][1], s5[0] - w[1][0], s5[1] - w[1][1]]
    p = (w[2][0] + w[3][0], w[2][1] + w[3][1])
    q = _rot(w[2][0] - w[3][0], w[2][1] - w[3][1], -1, 8)
    d4 = [p[0], q[0], p[1], q[1]]
    return [(s4[n], d4[n]) for n in range(4)]


def _inv1(n, z):
    e = _rot(*z[1], -n, 8)
    p = _rot(z[0][0] + e[0], z[0][1] + e[1], -n, 32)
    q = _rot(z[0][0] - e[0], z[0][1] - e[1], -(n + 4), 32)
    d0, d1 = _rot(*z[2], -n, 16)
    s0, s1 = z[3][0] + z[3][1], z[3][0] - z[3][1]
    return [p[0] + (s0 + d0), q[0] + (s1 + d1), p[1] + (s0 - d0), q[1] + (s1 - d1)]


_F1 = [4 * (g + 2 * k) + 1 for g in range(2) for k in range(4)]
_F1 += [2 * (4 * k + 1) for k in range(4)] + [0, 8, 4, 20]
_REAL_SLOT = 12
SLOTS = len(_F1)


def _dft_tables():
    kap = np.arange(128)
    j = 8 * (kap // 16) + kap % 8
    part = (kap // 8) % 2
    pr, pc, jr, jc = part[:, None], part[None, :], j[:, None], j[None, :]
    lo = 2 * np.pi * jr * jc / 64
    base = np.where(pr == pc, np.cos(lo), np.where(pr == 0, -np.sin(lo), np.sin(lo)))
    hi = 2 * np.pi * (16 + 32 * (jr - 32)) * jc / 2048
    v0 = np.where(pr == 0, np.cos(lo), np.where(jr == 0, np.cos(np.pi * jc), np.sin(lo)))
    v32 = np.where(pr == 0, np.cos(hi), np.sin(hi))
    real = np.where(jr < 32, np.where(pc == 0, v0, 0.0), np.where(pc == 1, v32, 0.0))
    th = 2 * np.pi * np.outer(np.array(_F1), j) / 2048
    zeros = np.zeros((8, 128))
    return np.concatenate([base, real, np.cos(th), np.sin(th), zeros]).astype(np.float32)


_TABLES = _dft_tables()
_FFT_SCALE = 2.0 ** -10

(P_MU, P_RHO, P_RHO1, P_RHO2, P_RHO4, P_TAP, P_SSMD, P_DSKIP, P_COEF, P_ROWS) = (
    0, 2, 4, 6, 8, 10, 14, 15, 16, 20)
S_SMALL, S_F0, S_K0, S_C, S_OUT, S_X0, S_B, S_COL, S_END = 0, 1, 2, 3, 4, 5, 6, 9, 9 + NG - 1


Y128 = [(0, 128, 128)] + [(n, t, 128) for n in range(1, 4) for t in (0, 128)] + [
    (4, 0, 128), (4, 128, 96), (4, 224, 32)]
Y_BOTH = [(0, 0, 32), (0, 32, 96), (0, 128, 128)] + [
    (n, t, 128) for n in range(1, 4) for t in (0, 128)] + [(4, 0, 128), (4, 128, 96), (4, 224, 32)]
Y_LAST = [(n, t, 128) for n in range(4) for t in (0, 128)] + [(4, 0, 128), (4, 128, 96), (4, 224, 32)]


def _cmul(a, b):
    return a[0] * b[0] - a[1] * b[1], a[0] * b[1] + a[1] * b[0]


def _pack(lo, hi):
    return jnp.concatenate([lo, hi], axis=0).astype(BF16)


def _unpack(w):
    v = pltpu.bitcast(w, BF16).astype(F32)
    return v[:8], v[8:]


CFG = dict(scan=22, u=28, k1=24, p2=0, inv=36, skip=28, tail=3, kconv=14, steps=2, p2n=2,
           early=60, kwin=(44, 230), tr=(20, 40), wid=(16, 200), scanw=(0, 250), invw=(230, 400),
           k2w=(230, 400), mf=128, mi=128, sh1=True, sh2=True, y0=True, m0=8,
           flags=None, nosem=False, skipme=lambda n, rows: False)


class _Gate:
    def __init__(self, pred=None, seen=()):
        self.pred, self.seen = pred, seen

    def early(self, lag):
        old = [e for e in self.seen if e[0] <= -lag]
        return max(old, key=lambda e: e[0])[1] if lag and old else None

    def value(self, v, lag):
        early = self.early(lag)
        return v if early is None else jnp.where(self.pred, v, early)

    def loads(self, ref, lag):
        early = self.early(lag)
        if early is not None:
            ref[pl.ds(ref.shape[0] - 8, 8), :] = (
                early if ref.dtype == F32 else pltpu.bitcast(early, I32))


def _weave(passes, plan, pred):
    if CFG["skipme"](len(passes), sum(q[0] for q in passes)):
        return
    begin, clock = [], [0] * 4
    for i, (n, *_) in enumerate(passes):
        begin.append(clock[i % 4] / 16)
        clock[i % 4] += n

    def index(t):
        later = [i for i, b in enumerate(begin) if b >= t - 3.999]
        if not later:
            return len(passes)
        same = [i for i in later if begin[i] == min(begin[j] for j in later)]
        return same[min(max(int((t - begin[same[0]]) / 4 * len(same)), 0), len(same) - 1)]

    at = [[] for _ in range(len(passes) + 1)]
    for tasks, lo, hi in plan:
        total, done = sum(sum(c) for c, _ in tasks) or 1, 0.0
        for costs, fn in tasks:
            where = []
            for cost in costs:
                done += cost
                where.append(index(lo + done / total * (hi - lo)))
            at[min(where)].append((fn, where))
    seen, ties = [], [[] for _ in at]
    for i, fns in enumerate(at):
        now = (begin[i] + i % 4) if i < len(begin) else clock[0] / 16
        early = [(t - now, v) for t, v in seen]
        for fn, where in fns:
            for w, tie in zip(where, fn(_Gate(pred, early)) or ()):
                ties[w].append(tie)
        if i == len(passes):
            break
        n, lhs, rhs, consume = passes[i]
        w = rhs()
        for tie in ties[i]:
            w[-1] = jnp.where(pred, w[-1], tie if tie.dtype == I32 else pltpu.bitcast(tie, I32))
        d = jnp.dot(pltpu.bitcast(jnp.concatenate(lhs(), axis=0), BF16),
                    pltpu.bitcast(jnp.concatenate(w, axis=0), BF16), preferred_element_type=F32)
        seen += [(begin[i] + i % 4 + j // 16 - 4, d[j - 8:j]) for j in range(64, n + 1, 64)]
        consume(d)


def _now(tasks):
    for _, fn in tasks:
        fn(_Gate())


def _kernel(tab_hbm, x_hbm, lre_hbm, lim_hbm, bre_hbm, bim_hbm, cre_hbm, cim_hbm,
            ldt_hbm, dsk_hbm, q_hbm, k_hbm, v_hbm, tap_hbm, sk_hbm, sd_hbm,
            o_hbm,
            tab, lre_v, lim_v, ldt_v, dsk_v, sd_v, tap_v,
            xb, braw, craw, qb, kb, vb, skb,
            par, wb16, wc, mf16, mi, bu, hb16, carry, ys, oa,
            kt, kf, st_u, st_k, st_i, vu16, vk16, pb0, pb1, ob,
            sem):
    x32, q32, k32, v32, wb, mf, hb, vu, vk = (
        r.bitcast(I32) for r in (xb, qb, kb, vb, wb16, mf16, hb16, vu16, vk16))
    pb16 = (pb0, pb1)
    pb = (pb0.bitcast(I32), pb1.bitcast(I32))

    def rows(ref, start, n=8):
        return ref[pl.ds(start, n), :]

    def hint(v, n):
        return v if isinstance(v, int) else pl.multiple_of(v, n)

    def view(ref, start, n=None):
        return ref.at[pl.ds(hint(start, 16), n or ref.shape[0]), :]

    small = [pltpu.make_async_copy(s, d, sem.at[S_SMALL]) for s, d in (
        (lre_hbm, lre_v), (lim_hbm, lim_v), (ldt_hbm, ldt_v),
        (dsk_hbm, dsk_v), (sd_hbm, sd_v), (tap_hbm, tap_v),
        (tab_hbm.at[pl.ds(288, 8), :], tab.at[pl.ds(288, 8), :]))]
    tab_dma = pltpu.make_async_copy(
        tab_hbm.at[pl.ds(0, 288), :], tab.at[pl.ds(0, 288), :], sem.at[S_F0])

    def x_dma(u):
        return [pltpu.make_async_copy(
            x_hbm.at[pl.ds(hint(u * UNIT, UNIT), UNIT), pl.ds(128 * n, 128)],
            xb.at[pl.ds(hint(n * L + u * UNIT, UNIT), UNIT), :], sem.at[(S_X0, S_F0, S_K0)[u] if isinstance(u, int) and u < LEAD
                                                     else S_COL + u - LEAD])
            for n in range(NG)]

    def b_dma(p):
        return [pltpu.make_async_copy(
            src.at[pl.ds(128 * p, 128), :], braw.at[pl.ds(D * c + 128 * p, 128), :],
            sem.at[S_B + (p + 1) // 2]) for c, src in enumerate((bre_hbm, bim_hbm))]

    c_dma = [pltpu.make_async_copy(
        src.at[:, pl.ds(128 * p, 128)], craw.at[pl.ds(D * (NG * c + p), D), :],
        sem.at[S_C]) for c, src in enumerate((cre_hbm, cim_hbm)) for p in range(NG)]

    def col_dma(which, g, sem_at):
        src, dst = ((k_hbm, kb), (v_hbm, vb), (q_hbm, qb))[which]
        return pltpu.make_async_copy(
            src.at[:, pl.ds(hint(128 * g, 128), 128)],
            dst.at[pl.ds(hint(L * g, L), L), :], sem.at[sem_at])

    def sk_dma(g, sem_at):
        t = hint(128 * g, 128)
        return pltpu.make_async_copy(
            sk_hbm.at[pl.ds(hint(128 * g, 128), 128), :], skb.at[pl.ds(t, 128), :],
            sem.at[sem_at])

    def oa_dma(u, n):
        t = hint(u * UNIT, UNIT)
        return pltpu.make_async_copy(
            oa.at[pl.ds(t, UNIT), pl.ds(128 * n, 128)],
            o_hbm.at[pl.ds(t, UNIT), pl.ds(128 * n, 128)], sem.at[S_OUT])

    def oa_unit_dma(u):
        t = hint(u * UNIT, UNIT)
        return pltpu.make_async_copy(
            oa.at[pl.ds(t, UNIT), :], o_hbm.at[pl.ds(t, UNIT), pl.ds(0, D)], sem.at[S_OUT])

    def ob_dma(g):
        return pltpu.make_async_copy(
            ob.at[pl.ds(hint(L * g, L), L), :],
            o_hbm.at[:, pl.ds(hint(D + 128 * g, 128), 128)], sem.at[S_OUT])

    def start(ds):
        for d in ds:
            d.start()

    def wait(ds):
        for d in ds:
            d.wait()

    def prm(g, row):
        return rows(view(par, g * (P_ROWS * 8), P_ROWS * 8), row * 8)

    def bu_passes(u, slot, z, shift):
        out = []
        xu, w = view(x32, u * (UNIT // 2), ((NG - 1) * L + UNIT) // 2), view(wb, z)
        order = [p + c * NG for p in range(NG) for c in range(2)]
        for n in order:
            sizes = [128, 128]
            if shift and n == order[0]:
                sizes = [32, 32, 96, 96]
            if shift and n == order[-1]:
                sizes = [96, 96, 32, 32]
            if shift is None:
                sizes = [64] * 4
            for m, MM in zip(np.cumsum([0] + sizes).tolist(), sizes):
                acc = []
                for kk in range(NG):
                    def lhs(m=m, kk=kk, MM=MM):
                        t = (kk * L + m) // 2
                        return [rows(xu, t + 8 * i) for i in range(MM // 16)]

                    def rhs(n=n, kk=kk):
                        return [rows(w, (n * NG + kk) * 64 + 8 * i) for i in range(8)]

                    def consume(d, m=m, n=n, kk=kk, acc=acc, MM=MM):
                        acc.append(d if kk == 0 else acc[-1] + d)
                        if kk == NG - 1:
                            for i in range(MM // 8):
                                seg, r = divmod(m + 8 * i, R)
                                row = 9 * (seg % 2 * R + r) + seg // 2
                                bu[pl.ds((slot * 2 * NG + n) * BU_PART + row, 8, stride=9), :] = (
                                    acc[-1][8 * i:8 * i + 8])
                    out.append((MM, lhs, rhs, consume))
        return out

    def scan_tasks(u, slot, z):
        steps = CFG["steps"]
        state = {}
        hu = view(hb16, u * UNIT, (2 * NG - 1) * L + UNIT)

        def b(p, ch, r):
            return tuple(rows(bu, (slot * 2 * NG + c * NG + p) * BU_PART + 9 * (ch * R + r))
                         for c in range(2))

        def step(mu, h, br):
            return (mu[0] * h[0] + br[0]) - mu[1] * h[1], (mu[0] * h[1] + br[1]) + mu[1] * h[0]

        def ends(p, gate):
            mu, ties = (gate.value(prm(p, P_MU), CFG["scan"]), prm(p, P_MU + 1)), []
            h = [b(p, ch, 0) for ch in range(2)]
            for r in range(1, R):
                h = [step(mu, h[ch], b(p, ch, r)) for ch in range(2)]
                if r % steps == 0:
                    ties.append(h[r // steps % 2][0])
            state[p] = starts(p, h)
            return ties + [state[p][1][0]]

        def starts(p, e):
            last = lax.broadcasted_iota(I32, (8, 128), 0) == 7
            rho = (prm(p, P_RHO), prm(p, P_RHO + 1))
            pair = step(rho, e[0], e[1])
            a = tuple(pltpu.roll(jnp.where(last, rows(carry, (2 * p + c) * 8), pair[c]), 1, 0)
                      for c in range(2))
            for sh, row in ((1, P_RHO1), (2, P_RHO2), (4, P_RHO4)):
                a = step((prm(p, row), prm(p, row + 1)), tuple(pltpu.roll(c, sh, 0) for c in a), a)
            return [a, step(rho, a, e[0])]

        def run(p, r0, gate):
            if r0 == 0:
                state["mu"] = (prm(p, P_MU), prm(p, P_MU + 1))
            mu, h = (gate.value(state["mu"][0], CFG["scan"]), state["mu"][1]), state[p]
            for r in range(r0, r0 + steps):
                h = [step(mu, h[ch], b(p, ch, r)) for ch in range(2)]
                for c in range(2):
                    hu[pl.ds((c * NG + p) * L + 16 * r, 16), :] = _pack(h[0][c], h[1][c])
            state[p] = h
            if r0 + steps == R:
                for c in range(2):
                    carry[pl.ds((2 * p + c) * 8, 8), :] = h[1][c]
            return [rows(view(hb, z, 8), 0)]

        tasks = []
        for p in range(NG):
            tasks.append(([16 * steps] * ((R - 1) // steps) + [46 + 16 * steps],
                          lambda gate, p=p: ends(p, gate)))
            tasks += [([18 * steps], lambda gate, p=p, r0=r0: run(p, r0, gate))
                      for r0 in range(0, R, steps)]
        return tasks

    def y_tiles(MM):
        return [(n, t, MM) for n in range(NG) for t in range(0, UNIT, MM)]

    def y_passes(u, tiles, z=0):
        out, w = [], view(wc, z)
        hu = view(hb, u * (UNIT // 2), ((2 * NG - 1) * L + UNIT) // 2)
        if True:
            for n, t0, MM in tiles:
                acc = []
                for kk in range(2 * NG):
                    def lhs(t0=t0, kk=kk, MM=MM):
                        t = kk * (L // 2) + t0 // 2
                        return [rows(hu, t + 8 * i) for i in range(MM // 16)]

                    def rhs(n=n, kk=kk):
                        return [rows(w, (kk * NG + n) * 64 + 8 * i) for i in range(8)]

                    def consume(d, t0=t0, n=n, kk=kk, acc=acc, MM=MM):
                        acc.append(d if kk == 0 else acc[-1] + d)
                        if kk == 2 * NG - 1:
                            for i in range(MM // 8):
                                r, ch = divmod(t0 // 8 + i, 2)
                                ys[pl.ds(n * YS_ROWS + ch * (R + 1) + r, 8, stride=2 * (R + 1)), :] = (
                                    acc[-1][8 * i:8 * i + 8])
                    out.append((MM, lhs, rhs, consume))
        return out

    def skip_task(u, n, z):
        def fn(gate):
            dsk = gate.value(prm(n, P_DSKIP), CFG["skip"])
            xu, ou = view(x32, u * (UNIT // 2) + n * (L // 2), UNIT // 2), view(oa, u * UNIT, UNIT)
            ties = []
            for i in range(UNIT // 16):
                xs = _unpack(rows(xu, 8 * i))
                for c in range(2):
                    t = 16 * i + 8 * c
                    y = rows(ys, n * YS_ROWS + (t // R) * (R + 1) + t % R)
                    ou[pl.ds(t, 8), pl.ds(128 * n, 128)] = y + xs[c] * dsk
                if i % 4 == 3:
                    ties.append(view(oa, z + u * UNIT, 8)[:, pl.ds(128 * n, 128)])
            return ties
        return ([24] * (UNIT // 64), fn)

    def widen_tasks(g, z, pieces=2):
        def fn(i0, i1):
            kg = view(k32, g * (L // 2), L // 2)
            for i in range(i0, i1):
                lo, hi = _unpack(rows(kg, 8 * i))
                kf[pl.ds(KF_PAD + 16 * i, 8), :] = lo
                kf[pl.ds(KF_PAD + 16 * i + 8, 8), :] = hi
            return [rows(view(kf, z), 16 * i0 + KF_PAD)]
        n = L // 16 // pieces
        return [([2 * n], lambda gate, i=i: fn(i * n, (i + 1) * n)) for i in range(pieces)]

    def transpose_tasks(g, z, pieces=8):
        def fn(c0, c1):
            for c in range(c0, c1):
                t = skb[pl.ds(hint(128 * g, 128), 128), pl.ds(128 * c, 128)]
                kt[pl.ds(64 * c, 64), :] = pltpu.bitcast(t.T, I32)
            return [rows(view(kt, z), 64 * c0)]
        n = L // 128 // pieces
        return [([8 * n], lambda gate, i=i: fn(i * n, (i + 1) * n)) for i in range(pieces)]

    def staged(s, half, n, grp, c):
        return (((s * 2 + half) * 4 + n) * 4 + grp) * 16 + 8 * c

    def pass1(st, s, half, n, u, z):
        for grp, pair in enumerate(_fwd1(n, [_Signed(v) for v in u])):
            for c in range(2):
                st[pl.ds(staged(s, half, n, grp, c), 8), :] = pair[c].get()
        return rows(view(st, z), staged(s, half, n, 0, 0))

    ops1 = (18, 36, 30, 36)

    def u1_task(g, s, half, n, z):
        def fn(gate):
            taps = [prm(g, P_TAP + t) for t in range(4)]
            taps[0] = gate.value(taps[0], CFG["u"])
            u, kz, vg = [], view(kf, z), view(v32, g * (L // 2), L // 2)
            for m in range(4):
                t = 64 * (16 * half + n + 4 * m) + 8 * s
                ks = rows(kz, KF_PAD + t) * taps[0]
                for lag in range(1, 4):
                    ks = ks + rows(kz, KF_PAD + t - lag) * taps[lag]
                u.append(ks * _unpack(rows(vg, (t // 16) * 8))[s % 2])
            return [u[0] + u[2], pass1(st_u, s, half, n, u, z)]
        return ([19, 17 + ops1[n]], fn)

    def k1_task(g, s, half, z):
        def fn(gate):
            gate.loads(kt, CFG["k1"])
            ties = []
            for n in range(4):
                u = [_unpack(rows(view(kt, z), 32 * (16 * half + n + 4 * m) + 8 * (s // 2)))[s % 2]
                     for m in range(4)]
                if s == 0 and half == 0 and n == 0:
                    first = lax.broadcasted_iota(I32, (8, 128), 0) == 0
                    u[0] = u[0] + jnp.where(first, prm(g, P_SSMD), 0.0)
                ties.append(pass1(st_k, s, half, n, u, z))
            return ties
        return ([4 + n for n in ops1], fn)

    def pass2_tasks(st, s, half, z):
        dst16, dst = (vu16, vu) if st is st_u else (vk16, vk)

        def fn(gate, grps):
            gate.loads(st, CFG["p2"])
            for grp in grps:
                zs = [tuple(_Signed(rows(view(st, z), staged(s, half, n, grp, c))) for c in range(2))
                      for n in range(4)]
                for k, pair in enumerate(_fwd2(grp, zs)):
                    dst16[pl.ds(((4 * grp + k) * 2 + half) * 128 + 16 * s, 16), :] = (
                        _pack(pair[0].get(), pair[1].get()))
            return [rows(view(dst, z), (8 * grps[0] + half) * 64 + 8 * s)]
        return [([20 * len(g)], lambda gate, g=g: fn(gate, g))
                for g in np.arange(4).reshape(CFG["p2n"], -1).tolist()]

    def fwd_passes(grp, z):
        out, MM = [], CFG["mf"]
        for slot in range(4 * grp, 4 * grp + 4):
            for part in range(128 // MM):
                got = []
                for src, half in ((vu, 0), (vk, 0), (vu, 1), (vk, 1)):
                    def lhs(slot=slot, part=part):
                        return [rows(mf, slot * 64 + MM // 2 * part + 8 * i) for i in range(MM // 16)]

                    def rhs(slot=slot, src=src, half=half):
                        return [rows(view(src, z), (2 * slot + half) * 64 + 8 * i) for i in range(8)]

                    def consume(d, slot=slot, part=part, got=got):
                        got.append(d)
                        if len(got) < 4:
                            return
                        for i in range(MM // 16):
                            u0, k0, u1, k1 = ((t[16 * i:16 * i + 8], t[16 * i + 8:16 * i + 16]) for t in got)
                            lo, a, b = _cmul(u0, k0), _cmul(u0, k1), _cmul(u1, k0)
                            if slot == _REAL_SLOT and part == 0 and i == 0:
                                first = lax.broadcasted_iota(I32, (8, 128), 0) == 0
                                lo, a, b = (tuple(jnp.where(first, 0.5 * (x[c] * y[c]), p[c]) for c in range(2))
                                            for p, x, y in ((lo, u0, k0), (a, u0, k1), (b, u1, k0)))
                            if _F1[slot] % 2:
                                hi = ((a[0] + b[0]) - lo[0], (a[1] + b[1]) - lo[1])
                            else:
                                hi = ((a[0] + b[0]) + lo[0], (a[1] + b[1]) + lo[1])
                            for half, p in enumerate((lo, hi)):
                                at = (slot % 4 * 2 + half) * 128 + MM * part + 16 * i
                                pb16[grp % 2][pl.ds(at, 16), :] = _pack(*p)
                    out.append((MM, lhs, rhs, consume))
        return out

    def inv_passes(grp, half, z):
        out, MM = [], CFG["mi"]
        for part in range(128 // MM):
            got = []
            for slot in range(4 * grp, 4 * grp + 4):
                def lhs(slot=slot, part=part):
                    return [rows(mi, slot * 64 + MM // 2 * part + 8 * i) for i in range(MM // 16)]

                def rhs(slot=slot):
                    return [rows(view(pb[grp % 2], z), (slot % 4 * 2 + half) * 64 + 8 * i)
                            for i in range(8)]

                def consume(d, part=part, got=got):
                    got.append(d)
                    if len(got) < 4:
                        return
                    for i in range(MM // 16):
                        w = [(_Signed(t[16 * i:16 * i + 8]), _Signed(t[16 * i + 8:16 * i + 16]))
                             for t in got]
                        for n, pair in enumerate(_inv2(grp, w)):
                            for c in range(2):
                                at = staged(MM // 16 * part + i, half, n, grp, c)
                                st_i[pl.ds(at, 8), :] = pair[c].get()
                out.append((MM, lhs, rhs, consume))
        return out

    def inv1_task(g, s, half, z):
        def fn(gate):
            gate.loads(st_i, CFG["inv"])
            qg, og, ties = view(q32, g * (L // 2), L // 2), view(ob, g * L, L), []
            for n in range(4):
                zs = [tuple(_Signed(rows(view(st_i, z), staged(s, half, n, grp, c))) for c in range(2))
                      for grp in range(4)]
                for m, y in enumerate(_inv1(n, zs)):
                    t = 64 * (16 * half + n + 4 * m) + 8 * s
                    og[pl.ds(t, 8), :] = _unpack(rows(qg, (t // 16) * 8))[s % 2] * y.get()
                ties.append(rows(view(ob, z + g * L, L), 64 * (16 * half + n) + 8 * s))
            return ties
        return ([12 + n for n in ops1], fn)

    filter0 = x_dma(1) + [sk_dma(0, S_F0), tab_dma]
    data0 = x_dma(2) + [col_dma(0, 0, S_K0), col_dma(1, 0, S_K0)]

    def group_dma(g):
        at = S_COL + g
        return [col_dma(2, g, at), sk_dma(g + 1, at), col_dma(0, g + 1, at),
                col_dma(1, g + 1, at)] + x_dma(g + LEAD)

    last_dma = [col_dma(2, NG - 1, S_SMALL)] + [pltpu.make_async_copy(
        x_hbm.at[pl.ds(L - UNIT, UNIT), pl.ds(128 * n, 128)],
        xb.at[pl.ds(n * L + L - UNIT, UNIT), :], sem.at[S_SMALL]) for n in range(NG)]

    start(b_dma(0) + small + x_dma(0))
    start(b_dma(1) + b_dma(2))
    wait(small)
    zeros = rows(tab, 288).astype(I32)
    z8 = pl.multiple_of(zeros[0, 0], 16)
    sub = lax.broadcasted_iota(I32, (8, 128), 0)
    pred = zeros == 0

    def stack(ref):
        v = ref[...].astype(F32).reshape(1, D)
        return jnp.concatenate([v[:, 128 * g:128 * (g + 1)] for g in range(NG)]
                               + [v[:, :128]] * (8 - NG), axis=0)

    lre, lim = stack(lre_v), stack(lim_v)
    dt = jnp.exp(stack(ldt_v)).astype(BF16).astype(F32)
    mag, ang = jnp.exp(dt * lre), dt * lim
    lam = (mag * jnp.cos(ang), mag * jnp.sin(ang))
    scale = jnp.maximum(jnp.abs(lre), jnp.abs(lim))
    nre, nim = lre / scale, lim / scale
    den = (nre * nre + nim * nim) * scale
    coef = _cmul(((lam[0] - 1.0) / den, lam[1] / den), (nre, -nim))
    mu = (lam[0], -lam[1])
    rho = [mu]
    for _ in range(R.bit_length() + 2):
        rho.append(_cmul(rho[-1], rho[-1]))
    dsk, ssd = stack(dsk_v), stack(sd_v)
    taps = tap_v[...].astype(F32) * _FFT_SCALE
    for g in range(NG):
        def put(row, v):
            par[pl.ds((g * P_ROWS + row) * 8, 8), :] = v

        def lanes(v):
            return jnp.broadcast_to(v[g:g + 1], (8, 128))
        for c in range(2):
            put(P_MU + c, lanes(mu[c]))
            put(P_RHO + c, lanes(rho[-4][c]))
            for n, row in enumerate((P_RHO1, P_RHO2, P_RHO4)):
                put(row + c, jnp.where(sub >= 1 << n, lanes(rho[n - 3][c]), 0.0))
        for t in range(4):
            put(P_TAP + t, jnp.broadcast_to(taps[t:t + 1, 128 * g:128 * (g + 1)], (8, 128)))
        put(P_COEF, lanes(2.0 * coef[0]))
        put(P_COEF + 1, lanes(-2.0 * coef[0]))
        put(P_COEF + 2, lanes(2.0 * coef[1]))
        put(P_SSMD, lanes(ssd))
        put(P_DSKIP, lanes(dsk))
    for i in range(2 * NG):
        carry[pl.ds(8 * i, 8), :] = jnp.zeros((8, 128), F32)
    kf[pl.ds(0, KF_PAD), :] = jnp.zeros((KF_PAD, 128), F32)

    def matrix_task(slot):
        def fn(gate):
            if slot != _REAL_SLOT:
                c, s = tab[pl.ds(256 + slot, 1), :], tab[pl.ds(272 + slot, 1), :]
            for a in range(8):
                if slot == _REAL_SLOT:
                    re, im = rows(tab, 128 + 16 * a), rows(tab, 128 + 16 * a + 8)
                else:
                    br, bi = rows(tab, 16 * a), rows(tab, 16 * a + 8)
                    re, im = c * br - s * bi, s * br + c * bi
                mf16[pl.ds(slot * 128 + 16 * a, 16), :] = _pack(re, im)
            m = pltpu.bitcast(rows(view(mf, z8), slot * 64, 64), BF16)
            mi[pl.ds(slot * 64, 64), :] = pltpu.bitcast(m.T, I32)
            return [rows(view(mf, z8), 0), rows(view(mi, z8), slot * 64)]
        return ([48, 8], fn)

    def scale_b(p, kk):
        cr, ncr, ci = prm(p, P_COEF), prm(p, P_COEF + 1), prm(p, P_COEF + 2)
        br, bi = (braw[pl.ds(D * c + 128 * p, 128), pl.ds(128 * kk, 128)].T.astype(F32)
                  for c in range(2))
        ties = []
        for i in range(8):
            r0, r1 = br[16 * i:16 * i + 8], br[16 * i + 8:16 * i + 16]
            i0, i1 = bi[16 * i:16 * i + 8], bi[16 * i + 8:16 * i + 16]
            wb16[pl.ds((p * NG + kk) * 128 + 16 * i, 16), :] = _pack(
                cr * r0 - ci * i0, cr * r1 - ci * i1)
            wb16[pl.ds(((NG + p) * NG + kk) * 128 + 16 * i, 16), :] = _pack(
                ncr * i0 - ci * r0, ncr * i1 - ci * r1)
            if i % 2:
                ties.append(rows(view(wb, z8), ((NG + p) * NG + kk) * 64))
        return ties

    def c_task(n, k0, k1):
        def fn(gate):
            for kk in range(k0, k1):
                t = craw[pl.ds(kk * D + 128 * n, 128), :]
                wc[pl.ds((kk * NG + n) * 64, 64), :] = pltpu.bitcast(t.T, I32)
            return [rows(view(wc, z8), ((k1 - 1) * NG + n) * 64)]
        return ([16], fn)

    first = bu_passes(0, 0, z8, None)
    first = [first[len(first) // NG * p:len(first) // NG * (p + 1)] for p in range(NG)]

    mats = [matrix_task(slot) for slot in range(SLOTS)]

    def scale_tasks(p):
        return [([36] * 4, lambda gate, kk=kk: scale_b(p, kk)) for kk in range(NG)]

    def dma_task(ds):
        return ([1], lambda gate: start(ds))

    def filter_tasks(g, slot):
        k1, k2 = [], []
        for s in range(8):
            for half in range(2):
                k1.append(k1_task(g, s, half, z8))
                k2 += pass2_tasks(st_k, s, half, z8)
        return transpose_tasks(slot, z8), k1, k2

    def forward_tasks(u, g):
        tasks = []
        for s in range(8):
            for half in range(2):
                tasks += [u1_task(g, s, half, n, z8) for n in range(4)] + pass2_tasks(st_u, s, half, z8)
        return tasks, [skip_task(u, n, z8) for n in range(NG)]

    per_n = 2 * NG * UNIT // 64
    total = NG * per_n

    wait(b_dma(0))
    _now(scale_tasks(0))
    start(b_dma(3) + b_dma(4) + filter0)
    wait(x_dma(0))
    _weave(first[0], [], pred)
    start(data0)
    wait(b_dma(1) + b_dma(2))
    _now(scale_tasks(1))
    _weave(first[1] + first[2], [(scale_tasks(2), 0, 40)], pred)
    start(c_dma)
    wait(b_dma(3) + b_dma(4))
    _now(scale_tasks(3))
    _weave(first[3] + first[4], [(scale_tasks(4), 0, 40)], pred)
    start(group_dma(0))
    wait(filter0)
    tr, k1, k2 = filter_tasks(0, 0)
    nm = CFG["m0"]
    _weave(bu_passes(1, 1, 0, CFG["sh1"]), [
        (scan_tasks(0, 0, z8), 0, total), (mats[:nm], 0, total), (tr, 8, 32),
        (k1, 36, total)], pred)
    start(group_dma(1))
    wait(data0)
    fwd, skips = forward_tasks(0, 0)
    _weave(bu_passes(2, 0, 0, CFG["sh2"]), [
        (widen_tasks(0, z8, 8), 0, 20), (fwd[:-3], 20, total), (fwd[-3:], total, total)], pred)
    start(group_dma(2))
    wait(c_dma)
    cs = [c_task(n, k, k + 2) for n in range(NG) for k in range(0, 2 * NG, 2)]
    _now(cs[:NG])
    _weave(y_passes(0, Y_BOTH if CFG["y0"] else y_tiles(64), z8), [
        (cs[n * NG:(n + 1) * NG], max(per_n * (n - 1) - 8, 0), per_n * n - 8) for n in range(1, NG)] + [
        (scan_tasks(1, 1, z8), 0, total), (k2, 0, total), (mats[nm:], 0, total)]
        + [(skips[n:n + 1], per_n * (n + 1) + 16, per_n * (n + 1) + 24) for n in range(NG - 1)], pred)
    start(group_dma(3) + last_dma)

    def conv_passes(lead):
        passes = fwd_passes(0, z8)
        for grp in range(1, 4):
            f, n = fwd_passes(grp, z8), 4 * 128 // CFG["mf"]
            passes += f[:n] + inv_passes(grp - 1, 0, z8) + f[n:3 * n] + inv_passes(grp - 1, 1, z8) + f[3 * n:]
        return passes + lead[:8] + inv_passes(3, 0, z8) + inv_passes(3, 1, z8) + lead[8:]

    def inverse_tasks(g):
        return [inv1_task(g, s, half, z8) for s in range(8) for half in range(2)]

    def body(i, _):
        wait(group_dma(i))
        passes = (conv_passes(y_passes(i + 1, [(0, 0, 32), (0, 32, 96)]))
                  + bu_passes(i + LEAD, 0, 0, False) + y_passes(i + 1, Y128))
        y0, end = 192 + total + 20, 192 + 2 * total
        tr, k1, k2 = filter_tasks(i + 1, i + 1)
        fwd, skips = forward_tasks(i + 1, i + 1)
        inv = inverse_tasks(i)
        nk, tail = CFG["kconv"], CFG["tail"]
        _weave(passes, [
            (scan_tasks(i + LEAD - 1, 0, z8), *CFG["scanw"]), (tr, *CFG["tr"]),
            ([skip_task(i, NG - 1, z8), dma_task([oa_unit_dma(i)])], 12, 12),
            (widen_tasks(i + 1, z8, 16), *CFG["wid"]), (k1[:nk], *CFG["kwin"]),
            (inv + [dma_task([ob_dma(i)])], *CFG["invw"]), (k1[nk:] + k2, *CFG["k2w"]),
            (fwd[:-tail], y0 - CFG["early"], end), (fwd[-tail:], end, end)]
            + [(skips[n:n + 1], end - per_n * (NG - 1 - n) + 16, end - per_n * (NG - 1 - n) + 24)
               for n in range(NG - 1)], pred)
        return 0

    lax.fori_loop(0, NG - 1, body, 0)

    wait(last_dma)
    g, u0, last = NG - 1, NG, L // UNIT - 1
    passes = (conv_passes(y_passes(u0, [(0, 0, 32), (0, 32, 96)])) + bu_passes(last, 1, 0, False)
              + y_passes(u0, [(0, 128, 128)] + y_tiles(128)[2:]) + y_passes(u0 + 1, y_tiles(128))
              + y_passes(last, Y_LAST))
    y0 = 192 + total + 20
    plan = [(scan_tasks(last - 1, 0, z8), 0, 192),
            ([skip_task(g, NG - 1, z8), dma_task([oa_unit_dma(g)])], 12, 12),
            (inverse_tasks(g) + [dma_task([ob_dma(g)])], 230, y0 + total),
            (scan_tasks(last, 1, z8), y0 + 16, y0 + 2 * total - 40)]
    out = [oa_unit_dma(u) for u in range(u0)] + [ob_dma(n) for n in range(NG)]
    for u in range(u0, last + 1):
        for n in range(NG):
            where = y0 + (u - u0) * total + per_n * (n + 1)
            plan.append(([skip_task(u, n, z8), dma_task([oa_dma(u, n)])], where, where))
            out.append(oa_dma(u, n))
    _weave(passes, plan, pred)
    wait(out)


@jax.jit
def pallas_concat_heads__ssm_conv_s5__ssm_conv_h3__prompt_kernel(
    A_x: jax.Array,
    A_Lambda_re: jax.Array,
    A_Lambda_im: jax.Array,
    A_B_re: jax.Array,
    A_B_im: jax.Array,
    A_C_re: jax.Array,
    A_C_im: jax.Array,
    A_log_dt: jax.Array,
    A_Dskip: jax.Array,
    B_q: jax.Array,
    B_k: jax.Array,
    B_v: jax.Array,
    B_shift_k: jax.Array,
    B_ssm_k: jax.Array,
    B_ssm_D: jax.Array,
):
    assert A_x.shape == (1, L, D) and B_shift_k.shape == (D, 4)
    vmem = pltpu.VMEM
    dma = pltpu.SemaphoreType.DMA
    scratch = [
        vmem(_TABLES.shape, F32),
        vmem((D,), BF16), vmem((D,), BF16), vmem((D,), BF16), vmem((D,), BF16), vmem((D,), BF16),
        vmem((4, D), BF16),
        vmem((NG * L, 128), BF16),
        vmem((2 * D, D), BF16),
        vmem((2 * NG * D, 128), BF16),
        vmem((NG * L, 128), BF16),
        vmem((NG * L, 128), BF16),
        vmem((NG * L, 128), BF16),
        vmem((D, L), BF16),
        vmem((NG * P_ROWS * 8, 128), F32),
        vmem((2 * NG * D, 128), BF16),
        vmem((2 * NG * NG * 64, 128), I32),
        vmem((SLOTS * 128, 128), BF16),
        vmem((SLOTS * 64, 128), I32),
        vmem((2 * 2 * NG * BU_PART, 128), F32),
        vmem((2 * NG * L, 128), BF16),
        vmem((3 * NG * 8, 128), F32),
        vmem((NG * YS_ROWS, 128), F32),
        vmem((L, D), F32),
        vmem((L // 2 + 8, 128), I32),
        vmem((KF_PAD + L, 128), F32),
        vmem((2 * L + 8, 128), F32),
        vmem((2 * L + 8, 128), F32),
        vmem((2 * L + 8, 128), F32),
        vmem((32 * 128, 128), BF16),
        vmem((32 * 128, 128), BF16),
        vmem((8 * 128, 128), BF16),
        vmem((8 * 128, 128), BF16),
        vmem((NG * L, 128), F32),
        dma((S_END,)),
    ]
    out = pl.pallas_call(
        _kernel,
        out_shape=jax.ShapeDtypeStruct((L, 2 * D), F32),
        in_specs=[pl.BlockSpec(memory_space=pl.ANY)] * 16,
        out_specs=pl.BlockSpec(memory_space=pl.ANY),
        scratch_shapes=scratch,
        compiler_params=pltpu.CompilerParams(vmem_limit_bytes=100 * 1024 * 1024, flags=CFG["flags"], disable_semaphore_checks=CFG["nosem"]),
        name="s5_h3",
    )(_TABLES, A_x.reshape(L, D), A_Lambda_re, A_Lambda_im, A_B_re, A_B_im, A_C_re, A_C_im,
      A_log_dt, A_Dskip, B_q.reshape(L, D), B_k.reshape(L, D), B_v.reshape(L, D),
      B_shift_k.T, B_ssm_k, B_ssm_D)
    return out.reshape(1, L, 2 * D)
```

```python
import math

import jax
import jax.numpy as jnp
import numpy as np
from jax import lax
from jax.experimental import pallas as pl
from jax.experimental.pallas import tpu as pltpu

F32, BF16, I32 = jnp.float32, jnp.bfloat16, jnp.int32

L = 2048
D = 640
NG = D // 128
UNIT = 256
SEG = 16
R = UNIT // SEG
LEAD = L // UNIT - NG
BU_PART = 9 * 2 * R
YS_ROWS = SEG * (R + 1)
KF_PAD = 8


class _Signed:
    def __init__(self, v, neg=False):
        self.v, self.neg = v, neg

    def __neg__(self):
        return _Signed(self.v, not self.neg)

    def __add__(self, o):
        if self.neg == o.neg:
            return _Signed(self.v + o.v, self.neg)
        return _Signed(o.v - self.v if self.neg else self.v - o.v)

    def __sub__(self, o):
        return self + (-o)

    def __mul__(self, c):
        return _Signed(self.v * np.float32(-c if self.neg else c))

    def get(self):
        return -self.v if self.neg else self.v


def _rot(re, im, num, den):
    num %= den
    h = math.sqrt(0.5)
    if num == 0:
        return re, im
    if 4 * num == den:
        return -im, re
    if 4 * num == 3 * den:
        return im, -re
    if 8 * num == den:
        return (re - im) * h, (re + im) * h
    if 8 * num == 3 * den:
        return (re + im) * (-h), (re - im) * h
    if 8 * num == 5 * den:
        return (im - re) * h, (re + im) * (-h)
    if 8 * num == 7 * den:
        return (re + im) * h, (im - re) * h
    c = math.cos(2 * math.pi * num / den)
    s = math.sin(2 * math.pi * num / den)
    return re * c - im * s, re * s + im * c


def _dft4(z, sign):
    (r0, i0), (r1, i1), (r2, i2), (r3, i3) = z
    ar, ai, br, bi = r0 + r2, i0 + i2, r0 - r2, i0 - i2
    cr, ci, dr, di = r1 + r3, i1 + i3, r1 - r3, i1 - i3
    plus, minus = (br - di, bi + dr), (br + di, bi - dr)
    if sign < 0:
        plus, minus = minus, plus
    return [(ar + cr, ai + ci), plus, (ar - cr, ai - ci), minus]


def _fwd1(n, u):
    a0, a1, b0, b1 = u
    p, q = _rot(a0, b0, n, 32), _rot(a1, b1, n + 4, 32)
    s0, s1 = a0 + b0, a1 + b1
    return [(p[0] + q[0], p[1] + q[1]), _rot(p[0] - q[0], p[1] - q[1], n, 8),
            _rot(a0 - b0, a1 - b1, n, 16), (s0 + s1, s0 - s1)]


def _fwd2(grp, z):
    if grp < 3:
        return _dft4(z, 1)
    s4 = [t[0] for t in z]
    d4 = [t[1] for t in z]
    p = (d4[0], d4[2])
    q = _rot(d4[1], d4[3], 1, 8)
    s5 = [s4[0] + s4[2], s4[1] + s4[3]]
    return [
        (s5[0] + s5[1], s5[0] - s5[1]),
        (s4[0] - s4[2], s4[1] - s4[3]),
        (p[0] + q[0], p[1] + q[1]),
        (p[0] - q[0], p[1] - q[1]),
    ]


def _inv2(grp, w):
    if grp < 3:
        return _dft4(w, -1)
    s5 = [w[0][0] + w[0][1], w[0][0] - w[0][1]]
    s4 = [s5[0] + w[1][0], s5[1] + w[1][1], s5[0] - w[1][0], s5[1] - w[1][1]]
    p = (w[2][0] + w[3][0], w[2][1] + w[3][1])
    q = _rot(w[2][0] - w[3][0], w[2][1] - w[3][1], -1, 8)
    d4 = [p[0], q[0], p[1], q[1]]
    return [(s4[n], d4[n]) for n in range(4)]


def _inv1(n, z):
    e = _rot(*z[1], -n, 8)
    p = _rot(z[0][0] + e[0], z[0][1] + e[1], -n, 32)
    q = _rot(z[0][0] - e[0], z[0][1] - e[1], -(n + 4), 32)
    d0, d1 = _rot(*z[2], -n, 16)
    s0, s1 = z[3][0] + z[3][1], z[3][0] - z[3][1]
    return [p[0] + (s0 + d0), q[0] + (s1 + d1), p[1] + (s0 - d0), q[1] + (s1 - d1)]


_F1 = [4 * (g + 2 * k) + 1 for g in range(2) for k in range(4)]
_F1 += [2 * (4 * k + 1) for k in range(4)] + [0, 8, 4, 20]
_REAL_SLOT = 12
SLOTS = len(_F1)


def _dft_tables():
    kap = np.arange(128)
    j = 8 * (kap // 16) + kap % 8
    part = (kap // 8) % 2
    pr, pc, jr, jc = part[:, None], part[None, :], j[:, None], j[None, :]
    lo = 2 * np.pi * jr * jc / 64
    base = np.where(pr == pc, np.cos(lo), np.where(pr == 0, -np.sin(lo), np.sin(lo)))
    hi = 2 * np.pi * (16 + 32 * (jr - 32)) * jc / 2048
    v0 = np.where(pr == 0, np.cos(lo), np.where(jr == 0, np.cos(np.pi * jc), np.sin(lo)))
    v32 = np.where(pr == 0, np.cos(hi), np.sin(hi))
    real = np.where(jr < 32, np.where(pc == 0, v0, 0.0), np.where(pc == 1, v32, 0.0))
    th = 2 * np.pi * np.outer(np.array(_F1), j) / 2048
    zeros = np.zeros((8, 128))
    return np.concatenate([base, real, np.cos(th), np.sin(th), zeros]).astype(np.float32)


_TABLES = _dft_tables()
_FFT_SCALE = 2.0 ** -10

(P_MU, P_RHO, P_RHO1, P_RHO2, P_RHO4, P_TAP, P_SSMD, P_DSKIP, P_COEF, P_ROWS) = (
    0, 2, 4, 6, 8, 10, 14, 15, 16, 20)
S_SMALL, S_F0, S_K0, S_C, S_OUT, S_X0, S_B, S_COL, S_END = 0, 1, 2, 3, 4, 5, 6, 9, 9 + NG - 1


Y128 = [(0, 128, 128)] + [(n, t, 128) for n in range(1, 4) for t in (0, 128)] + [
    (4, 0, 128), (4, 128, 96), (4, 224, 32)]
Y_BOTH = [(0, 0, 32), (0, 32, 96), (0, 128, 128)] + [
    (n, t, 128) for n in range(1, 4) for t in (0, 128)] + [(4, 0, 128), (4, 128, 96), (4, 224, 32)]
Y_LAST = [(n, t, 128) for n in range(4) for t in (0, 128)] + [(4, 0, 128), (4, 128, 96), (4, 224, 32)]


def _cmul(a, b):
    return a[0] * b[0] - a[1] * b[1], a[0] * b[1] + a[1] * b[0]


def _pack(lo, hi):
    return jnp.concatenate([lo, hi], axis=0).astype(BF16)


def _unpack(w):
    v = pltpu.bitcast(w, BF16).astype(F32)
    return v[:8], v[8:]


CFG = dict(scan=22, u=24, k1=24, p2=0, inv=36, skip=36, tail=4, kconv=8, steps=4, p2n=2,
           early=60, kwin=(44, 216), tr=(20, 40), wid=(16, 200), scanw=(0, 330), invw=(220, 380),
           k2w=(230, 400), mf=128, mi=128, sh1=True, sh2=True, y0=True, ord=(3, 4), late=False,
           m0=8, Q=1, invsplit=False, kg=1, k0=0.75, udir=True, kdir=True,
           flags=None, nosem=False, skipme=lambda n, rows: False)


class _Gate:
    def __init__(self, pred=None, seen=()):
        self.pred, self.seen = pred, seen

    def early(self, lag):
        old = [e for e in self.seen if e[0] <= -lag]
        return max(old, key=lambda e: e[0])[1] if lag and old else None

    def value(self, v, lag):
        early = self.early(lag)
        return v if early is None else jnp.where(self.pred, v, early)

    def loads(self, ref, lag):
        early = self.early(lag)
        if early is not None:
            ref[pl.ds(ref.shape[0] - 8, 8), :] = (
                early if ref.dtype == F32 else pltpu.bitcast(early, I32))


def _weave(passes, plan, pred):
    if CFG["skipme"](len(passes), sum(q[0] for q in passes)):
        return
    begin, clock = [], [0] * 4
    for i, (n, *_) in enumerate(passes):
        begin.append(clock[i % 4] / 16)
        clock[i % 4] += n

    def index(t):
        later = [i for i, b in enumerate(begin) if b >= t - 3.999]
        if not later:
            return len(passes)
        same = [i for i in later if begin[i] == min(begin[j] for j in later)]
        return same[min(max(int((t - begin[same[0]]) / 4 * len(same)), 0), len(same) - 1)]

    at = [[] for _ in range(len(passes) + 1)]
    for tasks, lo, hi in plan:
        total, done = sum(sum(c) for c, _ in tasks) or 1, 0.0
        for costs, fn in tasks:
            where = []
            for cost in costs:
                done += cost
                where.append(index(lo + done / total * (hi - lo)))
            at[min(where)].append((fn, where))
    seen, ties = [], [[] for _ in at]
    for i, fns in enumerate(at):
        now = (begin[i] + i % 4) if i < len(begin) else clock[0] / 16
        early = [(t - now, v) for t, v in seen if t % CFG["Q"] < 1 or CFG["Q"] == 1]
        for fn, where in fns:
            for w, tie in zip(where, fn(_Gate(pred, early)) or ()):
                ties[w].append(tie)
        if i == len(passes):
            break
        n, lhs, rhs, consume = passes[i]
        w = rhs()
        for tie in ties[i]:
            w[-1] = jnp.where(pred, w[-1], tie if tie.dtype == I32 else pltpu.bitcast(tie, I32))
        d = jnp.dot(pltpu.bitcast(jnp.concatenate(lhs(), axis=0), BF16),
                    pltpu.bitcast(jnp.concatenate(w, axis=0), BF16), preferred_element_type=F32)
        seen += [(begin[i] + i % 4 + j // 16 - 4, d[j - 8:j]) for j in range(64, n + 1, 64)]
        consume(d)


def _now(tasks):
    for _, fn in tasks:
        fn(_Gate())


def _kernel(tab_hbm, x_hbm, lre_hbm, lim_hbm, bre_hbm, bim_hbm, cre_hbm, cim_hbm,
            ldt_hbm, dsk_hbm, q_hbm, k_hbm, v_hbm, tap_hbm, sk_hbm, sd_hbm,
            o_hbm,
            tab, lre_v, lim_v, ldt_v, dsk_v, sd_v, tap_v,
            xb, braw, craw, qb, kb, vb, skb,
            par, wb16, wc, mf16, mi, bu, hb16, carry, ys, oa,
            kt, kf, st_u, st_k, st_i, vu16, vk16, pb0, pb1, ob,
            sem):
    x32, q32, k32, v32, wb, mf, hb, vu, vk = (
        r.bitcast(I32) for r in (xb, qb, kb, vb, wb16, mf16, hb16, vu16, vk16))
    pb16 = (pb0, pb1)
    pb = (pb0.bitcast(I32), pb1.bitcast(I32))

    def rows(ref, start, n=8):
        return ref[pl.ds(start, n), :]

    def hint(v, n):
        return v if isinstance(v, int) else pl.multiple_of(v, n)

    def view(ref, start, n=None):
        return ref.at[pl.ds(hint(start, 16), n or ref.shape[0]), :]

    small = [pltpu.make_async_copy(s, d, sem.at[S_SMALL]) for s, d in (
        (lre_hbm, lre_v), (lim_hbm, lim_v), (ldt_hbm, ldt_v),
        (dsk_hbm, dsk_v), (sd_hbm, sd_v), (tap_hbm, tap_v),
        (tab_hbm.at[pl.ds(288, 8), :], tab.at[pl.ds(288, 8), :]))]
    tab_dma = pltpu.make_async_copy(
        tab_hbm.at[pl.ds(0, 288), :], tab.at[pl.ds(0, 288), :], sem.at[S_F0])

    def x_dma(u):
        return [pltpu.make_async_copy(
            x_hbm.at[pl.ds(hint(u * UNIT, UNIT), UNIT), pl.ds(128 * n, 128)],
            xb.at[pl.ds(hint(n * L + u * UNIT, UNIT), UNIT), :], sem.at[(S_X0, S_F0, S_K0)[u] if isinstance(u, int) and u < LEAD
                                                     else S_COL + u - LEAD])
            for n in range(NG)]

    def b_dma(p):
        return [pltpu.make_async_copy(
            src.at[pl.ds(128 * p, 128), :], braw.at[pl.ds(D * c + 128 * p, 128), :],
            sem.at[S_B + (p + 1) // 2]) for c, src in enumerate((bre_hbm, bim_hbm))]

    c_dma = [pltpu.make_async_copy(
        src.at[:, pl.ds(128 * p, 128)], craw.at[pl.ds(D * (NG * c + p), D), :],
        sem.at[S_C]) for c, src in enumerate((cre_hbm, cim_hbm)) for p in range(NG)]

    def col_dma(which, g, sem_at):
        src, dst = ((k_hbm, kb), (v_hbm, vb), (q_hbm, qb))[which]
        return pltpu.make_async_copy(
            src.at[:, pl.ds(hint(128 * g, 128), 128)],
            dst.at[pl.ds(hint(L * g, L), L), :], sem.at[sem_at])

    def sk_dma(g, sem_at):
        t = hint(128 * g, 128)
        return pltpu.make_async_copy(
            sk_hbm.at[pl.ds(hint(128 * g, 128), 128), :], skb.at[pl.ds(t, 128), :],
            sem.at[sem_at])

    def oa_dma(u, n):
        t = hint(u * UNIT, UNIT)
        return pltpu.make_async_copy(
            oa.at[pl.ds(t, UNIT), pl.ds(128 * n, 128)],
            o_hbm.at[pl.ds(t, UNIT), pl.ds(128 * n, 128)], sem.at[S_OUT])

    def oa_unit_dma(u):
        t = hint(u * UNIT, UNIT)
        return pltpu.make_async_copy(
            oa.at[pl.ds(t, UNIT), :], o_hbm.at[pl.ds(t, UNIT), pl.ds(0, D)], sem.at[S_OUT])

    def ob_dma(g):
        return pltpu.make_async_copy(
            ob.at[pl.ds(hint(L * g, L), L), :],
            o_hbm.at[:, pl.ds(hint(D + 128 * g, 128), 128)], sem.at[S_OUT])

    def start(ds):
        for d in ds:
            d.start()

    def wait(ds):
        for d in ds:
            d.wait()

    def prm(g, row):
        return rows(view(par, g * (P_ROWS * 8), P_ROWS * 8), row * 8)

    def bu_passes(u, slot, z, shift):
        out = []
        xu, w = view(x32, u * (UNIT // 2), ((NG - 1) * L + UNIT) // 2), view(wb, z)
        order = [p + c * NG for p in range(NG) for c in range(2)]
        for n in order:
            sizes = [128, 128]
            if shift and n == order[0]:
                sizes = [32, 32, 96, 96]
            if shift and n == order[-1]:
                sizes = [96, 96, 32, 32]
            if shift is None:
                sizes = [64] * 4
            for m, MM in zip(np.cumsum([0] + sizes).tolist(), sizes):
                acc = []
                for kk in range(NG):
                    def lhs(m=m, kk=kk, MM=MM):
                        t = (kk * L + m) // 2
                        return [rows(xu, t + 8 * i) for i in range(MM // 16)]

                    def rhs(n=n, kk=kk):
                        return [rows(w, (n * NG + kk) * 64 + 8 * i) for i in range(8)]

                    def consume(d, m=m, n=n, kk=kk, acc=acc, MM=MM):
                        acc.append(d if kk == 0 else acc[-1] + d)
                        if kk == NG - 1:
                            for i in range(MM // 8):
                                seg, r = divmod(m + 8 * i, R)
                                row = 9 * (seg % 2 * R + r) + seg // 2
                                bu[pl.ds((slot * 2 * NG + n) * BU_PART + row, 8, stride=9), :] = (
                                    acc[-1][8 * i:8 * i + 8])
                    out.append((MM, lhs, rhs, consume))
        return out

    def scan_tasks(u, slot, z):
        steps = CFG["steps"]
        state = {}
        hu = view(hb16, u * UNIT, (2 * NG - 1) * L + UNIT)

        def b(p, ch, r):
            return tuple(rows(bu, (slot * 2 * NG + c * NG + p) * BU_PART + 9 * (ch * R + r))
                         for c in range(2))

        def step(mu, h, br):
            return (mu[0] * h[0] + br[0]) - mu[1] * h[1], (mu[0] * h[1] + br[1]) + mu[1] * h[0]

        def ends(p, gate):
            mu, ties = (gate.value(prm(p, P_MU), CFG["scan"]), prm(p, P_MU + 1)), []
            h = [b(p, ch, 0) for ch in range(2)]
            for r in range(1, R):
                h = [step(mu, h[ch], b(p, ch, r)) for ch in range(2)]
                if r % steps == 0:
                    ties.append(h[r // steps % 2][0])
            state[p] = starts(p, h)
            return ties + [state[p][1][0]]

        def starts(p, e):
            last = lax.broadcasted_iota(I32, (8, 128), 0) == 7
            rho = (prm(p, P_RHO), prm(p, P_RHO + 1))
            pair = step(rho, e[0], e[1])
            a = tuple(pltpu.roll(jnp.where(last, rows(carry, (2 * p + c) * 8), pair[c]), 1, 0)
                      for c in range(2))
            for sh, row in ((1, P_RHO1), (2, P_RHO2), (4, P_RHO4)):
                a = step((prm(p, row), prm(p, row + 1)), tuple(pltpu.roll(c, sh, 0) for c in a), a)
            return [a, step(rho, a, e[0])]

        def run(p, r0, gate):
            if r0 == 0:
                state["mu"] = (prm(p, P_MU), prm(p, P_MU + 1))
            mu, h = (gate.value(state["mu"][0], CFG["scan"]), state["mu"][1]), state[p]
            for r in range(r0, r0 + steps):
                h = [step(mu, h[ch], b(p, ch, r)) for ch in range(2)]
                for c in range(2):
                    hu[pl.ds((c * NG + p) * L + 16 * r, 16), :] = _pack(h[0][c], h[1][c])
            state[p] = h
            if r0 + steps == R:
                for c in range(2):
                    carry[pl.ds((2 * p + c) * 8, 8), :] = h[1][c]
            return [rows(view(hb, z, 8), 0)]

        tasks = []
        for p in range(NG):
            tasks.append(([16 * steps] * ((R - 1) // steps) + [46 + 16 * steps],
                          lambda gate, p=p: ends(p, gate)))
            tasks += [([18 * steps], lambda gate, p=p, r0=r0: run(p, r0, gate))
                      for r0 in range(0, R, steps)]
        return tasks

    def y_tiles(MM):
        return [(n, t, MM) for n in range(NG) for t in range(0, UNIT, MM)]

    def y_passes(u, tiles, z=0):
        out, w = [], view(wc, z)
        hu = view(hb, u * (UNIT // 2), ((2 * NG - 1) * L + UNIT) // 2)
        if True:
            for n, t0, MM in tiles:
                acc = []
                for kk in range(2 * NG):
                    def lhs(t0=t0, kk=kk, MM=MM):
                        t = kk * (L // 2) + t0 // 2
                        return [rows(hu, t + 8 * i) for i in range(MM // 16)]

                    def rhs(n=n, kk=kk):
                        return [rows(w, (kk * NG + n) * 64 + 8 * i) for i in range(8)]

                    def consume(d, t0=t0, n=n, kk=kk, acc=acc, MM=MM):
                        acc.append(d if kk == 0 else acc[-1] + d)
                        if kk == 2 * NG - 1:
                            for i in range(MM // 8):
                                r, ch = divmod(t0 // 8 + i, 2)
                                ys[pl.ds(n * YS_ROWS + ch * (R + 1) + r, 8, stride=2 * (R + 1)), :] = (
                                    acc[-1][8 * i:8 * i + 8])
                    out.append((MM, lhs, rhs, consume))
        return out

    def skip_task(u, n, z):
        def fn(gate):
            dsk = gate.value(prm(n, P_DSKIP), CFG["skip"])
            xu, ou = view(x32, u * (UNIT // 2) + n * (L // 2), UNIT // 2), view(oa, u * UNIT, UNIT)
            ties = []
            for i in range(UNIT // 16):
                xs = _unpack(rows(xu, 8 * i))
                for c in range(2):
                    t = 16 * i + 8 * c
                    y = rows(ys, n * YS_ROWS + (t // R) * (R + 1) + t % R)
                    ou[pl.ds(t, 8), pl.ds(128 * n, 128)] = y + xs[c] * dsk
                if i % 4 == 3:
                    ties.append(view(oa, z + u * UNIT, 8)[:, pl.ds(128 * n, 128)])
            return ties
        return ([24] * (UNIT // 64), fn)

    def widen_tasks(g, z, pieces=2):
        def fn(i0, i1):
            kg = view(k32, g * (L // 2), L // 2)
            for i in range(i0, i1):
                lo, hi = _unpack(rows(kg, 8 * i))
                kf[pl.ds(KF_PAD + 16 * i, 8), :] = lo
                kf[pl.ds(KF_PAD + 16 * i + 8, 8), :] = hi
            return [rows(view(kf, z), 16 * i0 + KF_PAD)]
        n = L // 16 // pieces
        return [([2 * n], lambda gate, i=i: fn(i * n, (i + 1) * n)) for i in range(pieces)]

    def transpose_tasks(g, z, pieces=8):
        def fn(c0, c1):
            for c in range(c0, c1):
                t = skb[pl.ds(hint(128 * g, 128), 128), pl.ds(128 * c, 128)]
                kt[pl.ds(64 * c, 64), :] = pltpu.bitcast(t.T, I32)
            return [rows(view(kt, z), 64 * c0)]
        n = L // 128 // pieces
        return [([8 * n], lambda gate, i=i: fn(i * n, (i + 1) * n)) for i in range(pieces)]

    def staged(s, half, n, grp, c):
        return (((s * 2 + half) * 4 + n) * 4 + grp) * 16 + 8 * c

    ops1 = (18, 36, 30, 36)

    def forward_tasks_of(st, s, half, z, chunk, chunk_cost, direct):
        dst16, dst = (vu16, vu) if st is st_u else (vk16, vk)

        def second(grp, zs):
            for k, pair in enumerate(_fwd2(grp, zs)):
                dst16[pl.ds(((4 * grp + k) * 2 + half) * 128 + 16 * s, 16), :] = (
                    _pack(pair[0].get(), pair[1].get()))
            return rows(view(dst, z), (8 * grp + half) * 64 + 8 * s)

        kept = []

        def first(gate, n):
            load = chunk(gate, n)
            u = [load(16 * half + n + 4 * m) for m in range(4)]
            pairs = _fwd1(n, [_Signed(v) for v in u])
            kept.append(pairs)
            for grp in range(2 * direct, 4):
                for c in range(2):
                    st[pl.ds(staged(s, half, n, grp, c), 8), :] = pairs[grp][c].get()
            return [u[0] + u[2]] * (chunk_cost > 4) + [rows(view(st, z), staged(s, half, n, 3, 0))]

        def rest(grp):
            if direct and grp < 2:
                return [second(grp, [t[grp] for t in kept])]
            return [second(grp, [tuple(_Signed(rows(view(st, z), staged(s, half, n, grp, c)))
                                       for c in range(2)) for n in range(4)])]

        split = (chunk_cost > 4) * (chunk_cost // 2 + 1)
        one = [([split] * (split > 0) + [chunk_cost + ops1[n] - split], lambda gate, n=n: first(gate, n))
               for n in range(4)]
        if CFG["p2n"] == 4:
            two = [([20], lambda gate, grp=grp: rest(grp)) for grp in range(4)]
        else:
            two = [([40], lambda gate, grp=grp: rest(grp) and rest(grp + 1)) for grp in (0, 2)]
        h = len(two) // 2
        return (one + two[:h], two[h:]) if direct else (one, two)

    def u_tasks(g, s, half, z):
        def chunk(gate, n):
            taps = [prm(g, P_TAP + t) for t in range(4)]
            taps[0] = gate.value(taps[0], CFG["u"])
            kz, vg = view(kf, z), view(v32, g * (L // 2), L // 2)

            def load(c):
                t = 64 * c + 8 * s
                ks = rows(kz, KF_PAD + t) * taps[0]
                for lag in range(1, 4):
                    ks = ks + rows(kz, KF_PAD + t - lag) * taps[lag]
                return ks * _unpack(rows(vg, (t // 16) * 8))[s % 2]
            return load
        return forward_tasks_of(st_u, s, half, z, chunk, 36, CFG["udir"])

    def k_tasks(g, s, half, z, direct):
        def chunk(gate, n):
            if n % CFG["kg"] == 0:
                gate.loads(kt, CFG["k1"])

            def load(c):
                v = _unpack(rows(view(kt, z), 32 * c + 8 * (s // 2)))[s % 2]
                if s == 0 and c == 0:
                    first = lax.broadcasted_iota(I32, (8, 128), 0) == 0
                    v = v + jnp.where(first, prm(g, P_SSMD), 0.0)
                return v
            return load
        return forward_tasks_of(st_k, s, half, z, chunk, 4, direct)

    def fwd_passes(grp, z):
        out, MM = [], CFG["mf"]
        for slot in range(4 * grp, 4 * grp + 4):
            for part in range(128 // MM):
                got = []
                for src, half in ((vu, 0), (vk, 0), (vu, 1), (vk, 1)):
                    def lhs(slot=slot, part=part):
                        return [rows(mf, slot * 64 + MM // 2 * part + 8 * i) for i in range(MM // 16)]

                    def rhs(slot=slot, src=src, half=half):
                        return [rows(view(src, z), (2 * slot + half) * 64 + 8 * i) for i in range(8)]

                    def consume(d, slot=slot, part=part, got=got):
                        got.append(d)
                        if len(got) < 4:
                            return
                        for i in range(MM // 16):
                            u0, k0, u1, k1 = ((t[16 * i:16 * i + 8], t[16 * i + 8:16 * i + 16]) for t in got)
                            lo, a, b = _cmul(u0, k0), _cmul(u0, k1), _cmul(u1, k0)
                            if slot == _REAL_SLOT and part == 0 and i == 0:
                                first = lax.broadcasted_iota(I32, (8, 128), 0) == 0
                                lo, a, b = (tuple(jnp.where(first, 0.5 * (x[c] * y[c]), p[c]) for c in range(2))
                                            for p, x, y in ((lo, u0, k0), (a, u0, k1), (b, u1, k0)))
                            if _F1[slot] % 2:
                                hi = ((a[0] + b[0]) - lo[0], (a[1] + b[1]) - lo[1])
                            else:
                                hi = ((a[0] + b[0]) + lo[0], (a[1] + b[1]) + lo[1])
                            for half, p in enumerate((lo, hi)):
                                at = (slot % 4 * 2 + half) * 128 + MM * part + 16 * i
                                pb16[grp % 2][pl.ds(at, 16), :] = _pack(*p)
                    out.append((MM, lhs, rhs, consume))
        return out

    def inv_passes(grp, half, z):
        out, MM = [], CFG["mi"]
        for part in range(128 // MM):
            got = []
            for slot in range(4 * grp, 4 * grp + 4):
                def lhs(slot=slot, part=part):
                    return [rows(mi, slot * 64 + MM // 2 * part + 8 * i) for i in range(MM // 16)]

                def rhs(slot=slot):
                    return [rows(view(pb[grp % 2], z), (slot % 4 * 2 + half) * 64 + 8 * i)
                            for i in range(8)]

                def consume(d, part=part, got=got):
                    got.append(d)
                    if len(got) < 4:
                        return
                    for i in range(MM // 16):
                        w = [(_Signed(t[16 * i:16 * i + 8]), _Signed(t[16 * i + 8:16 * i + 16]))
                             for t in got]
                        for n, pair in enumerate(_inv2(grp, w)):
                            for c in range(2):
                                at = staged(MM // 16 * part + i, half, n, grp, c)
                                st_i[pl.ds(at, 8), :] = pair[c].get()
                out.append((MM, lhs, rhs, consume))
        return out

    def inv1_task(g, s, half, z):
        def fn(gate, ns):
            gate.loads(st_i, CFG["inv"])
            qg, og, ties = view(q32, g * (L // 2), L // 2), view(ob, g * L, L), []
            for n in ns:
                zs = [tuple(_Signed(rows(view(st_i, z), staged(s, half, n, grp, c))) for c in range(2))
                      for grp in range(4)]
                for m, y in enumerate(_inv1(n, zs)):
                    t = 64 * (16 * half + n + 4 * m) + 8 * s
                    og[pl.ds(t, 8), :] = _unpack(rows(qg, (t // 16) * 8))[s % 2] * y.get()
                ties.append(rows(view(ob, z + g * L, L), 64 * (16 * half + n) + 8 * s))
            return ties
        if CFG["invsplit"]:
            return [([12 + ops1[n]], lambda gate, n=n: fn(gate, [n])) for n in range(4)]
        return [([12 + n for n in ops1], lambda gate: fn(gate, range(4)))]

    filter0 = x_dma(1) + [sk_dma(0, S_F0), tab_dma]
    data0 = x_dma(2) + [col_dma(0, 0, S_K0), col_dma(1, 0, S_K0)]

    def group_dma(g):
        at = S_COL + g
        return [col_dma(2, g, at), sk_dma(g + 1, at), col_dma(0, g + 1, at),
                col_dma(1, g + 1, at)] + x_dma(g + LEAD)

    last_dma = [col_dma(2, NG - 1, S_SMALL)] + [pltpu.make_async_copy(
        x_hbm.at[pl.ds(L - UNIT, UNIT), pl.ds(128 * n, 128)],
        xb.at[pl.ds(n * L + L - UNIT, UNIT), :], sem.at[S_SMALL]) for n in range(NG)]

    start(b_dma(0) + small + x_dma(0))
    start(b_dma(1) + b_dma(2))
    wait(small)
    zeros = rows(tab, 288).astype(I32)
    z8 = pl.multiple_of(zeros[0, 0], 16)
    sub = lax.broadcasted_iota(I32, (8, 128), 0)
    pred = zeros == 0

    def stack(ref):
        v = ref[...].astype(F32).reshape(1, D)
        return jnp.concatenate([v[:, 128 * g:128 * (g + 1)] for g in range(NG)]
                               + [v[:, :128]] * (8 - NG), axis=0)

    lre, lim = stack(lre_v), stack(lim_v)
    dt = jnp.exp(stack(ldt_v)).astype(BF16).astype(F32)
    mag, ang = jnp.exp(dt * lre), dt * lim
    lam = (mag * jnp.cos(ang), mag * jnp.sin(ang))
    scale = jnp.maximum(jnp.abs(lre), jnp.abs(lim))
    nre, nim = lre / scale, lim / scale
    den = (nre * nre + nim * nim) * scale
    coef = _cmul(((lam[0] - 1.0) / den, lam[1] / den), (nre, -nim))
    mu = (lam[0], -lam[1])
    rho = [mu]
    for _ in range(R.bit_length() + 2):
        rho.append(_cmul(rho[-1], rho[-1]))
    dsk, ssd = stack(dsk_v), stack(sd_v)
    taps = tap_v[...].astype(F32) * _FFT_SCALE
    for g in range(NG):
        def put(row, v):
            par[pl.ds((g * P_ROWS + row) * 8, 8), :] = v

        def lanes(v):
            return jnp.broadcast_to(v[g:g + 1], (8, 128))
        for c in range(2):
            put(P_MU + c, lanes(mu[c]))
            put(P_RHO + c, lanes(rho[-4][c]))
            for n, row in enumerate((P_RHO1, P_RHO2, P_RHO4)):
                put(row + c, jnp.where(sub >= 1 << n, lanes(rho[n - 3][c]), 0.0))
        for t in range(4):
            put(P_TAP + t, jnp.broadcast_to(taps[t:t + 1, 128 * g:128 * (g + 1)], (8, 128)))
        put(P_COEF, lanes(2.0 * coef[0]))
        put(P_COEF + 1, lanes(-2.0 * coef[0]))
        put(P_COEF + 2, lanes(2.0 * coef[1]))
        put(P_SSMD, lanes(ssd))
        put(P_DSKIP, lanes(dsk))
    for i in range(2 * NG):
        carry[pl.ds(8 * i, 8), :] = jnp.zeros((8, 128), F32)
    kf[pl.ds(0, KF_PAD), :] = jnp.zeros((KF_PAD, 128), F32)

    def matrix_task(slot):
        def fn(gate):
            if slot != _REAL_SLOT:
                c, s = tab[pl.ds(256 + slot, 1), :], tab[pl.ds(272 + slot, 1), :]
            for a in range(8):
                if slot == _REAL_SLOT:
                    re, im = rows(tab, 128 + 16 * a), rows(tab, 128 + 16 * a + 8)
                else:
                    br, bi = rows(tab, 16 * a), rows(tab, 16 * a + 8)
                    re, im = c * br - s * bi, s * br + c * bi
                mf16[pl.ds(slot * 128 + 16 * a, 16), :] = _pack(re, im)
            m = pltpu.bitcast(rows(view(mf, z8), slot * 64, 64), BF16)
            mi[pl.ds(slot * 64, 64), :] = pltpu.bitcast(m.T, I32)
            return [rows(view(mf, z8), 0), rows(view(mi, z8), slot * 64)]
        return ([48, 8], fn)

    def scale_b(p, kk):
        cr, ncr, ci = prm(p, P_COEF), prm(p, P_COEF + 1), prm(p, P_COEF + 2)
        br, bi = (braw[pl.ds(D * c + 128 * p, 128), pl.ds(128 * kk, 128)].T.astype(F32)
                  for c in range(2))
        ties = []
        for i in range(8):
            r0, r1 = br[16 * i:16 * i + 8], br[16 * i + 8:16 * i + 16]
            i0, i1 = bi[16 * i:16 * i + 8], bi[16 * i + 8:16 * i + 16]
            wb16[pl.ds((p * NG + kk) * 128 + 16 * i, 16), :] = _pack(
                cr * r0 - ci * i0, cr * r1 - ci * i1)
            wb16[pl.ds(((NG + p) * NG + kk) * 128 + 16 * i, 16), :] = _pack(
                ncr * i0 - ci * r0, ncr * i1 - ci * r1)
            if i % 2:
                ties.append(rows(view(wb, z8), ((NG + p) * NG + kk) * 64))
        return ties

    def c_task(n, k0, k1):
        def fn(gate):
            for kk in range(k0, k1):
                t = craw[pl.ds(kk * D + 128 * n, 128), :]
                wc[pl.ds((kk * NG + n) * 64, 64), :] = pltpu.bitcast(t.T, I32)
            return [rows(view(wc, z8), ((k1 - 1) * NG + n) * 64)]
        return ([16], fn)

    first = bu_passes(0, 0, z8, None)
    first = [first[len(first) // NG * p:len(first) // NG * (p + 1)] for p in range(NG)]

    mats = [matrix_task(slot) for slot in range(SLOTS)]

    def scale_tasks(p):
        return [([36] * 4, lambda gate, kk=kk: scale_b(p, kk)) for kk in range(NG)]

    def dma_task(ds):
        return ([1], lambda gate: start(ds))

    def filter_tasks(g, early):
        ts = [k_tasks(g, j // 2, j % 2, z8, j >= early and CFG["kdir"]) for j in range(16)]
        return (transpose_tasks(g, z8), [q for t in ts[:early] for q in t[0]],
                [q for t in ts[:early] for q in t[1]] + [q for t in ts[early:] for q in t[0] + t[1]])

    def forward_tasks(u, g):
        tasks = []
        for s in range(8):
            for half in range(2):
                tasks += sum(u_tasks(g, s, half, z8), [])
        return tasks, [skip_task(u, n, z8) for n in range(NG)]

    per_n = 2 * NG * UNIT // 64
    total = NG * per_n

    wait(b_dma(0))
    _now(scale_tasks(0))
    start(b_dma(3) + b_dma(4) + filter0)
    wait(x_dma(0))
    _weave(first[0], [], pred)
    start(data0)
    wait(b_dma(1) + b_dma(2))
    _now(scale_tasks(1))
    _weave(first[1] + first[2], [(scale_tasks(2), 0, 40)], pred)
    start(c_dma)
    wait(b_dma(3) + b_dma(4))
    _now(scale_tasks(3))
    _weave(first[3] + first[4], [(scale_tasks(4), 0, 40)], pred)
    start(group_dma(0))
    wait(filter0)
    tr, _, k1 = filter_tasks(0, 0)
    nm = CFG["m0"]
    _weave(bu_passes(1, 1, 0, CFG["sh1"]), [
        (scan_tasks(0, 0, z8), 0, total), (mats[:nm], 0, total), (tr, 8, 32),
        (k1[:int(CFG["k0"] * len(k1))], 36, total)], pred)
    start(group_dma(1))
    wait(data0)
    fwd, skips = forward_tasks(0, 0)
    _weave(bu_passes(2, 0, 0, CFG["sh2"]), [
        (widen_tasks(0, z8, 8), 0, 20), (fwd[:-3], 20, total), (fwd[-3:], total, total)], pred)
    start(group_dma(2))
    wait(c_dma)
    cs = [c_task(n, k, k + 2) for n in range(NG) for k in range(0, 2 * NG, 2)]
    _now(cs[:NG])
    _weave(y_passes(0, Y_BOTH if CFG["y0"] else y_tiles(64), z8), [
        (cs[n * NG:(n + 1) * NG], max(per_n * (n - 1) - 8, 0), per_n * n - 8) for n in range(1, NG)] + [
        (scan_tasks(1, 1, z8), 0, total), (k1[int(CFG["k0"] * len(k1)):], 0, total), (mats[nm:], 0, total)]
        + [(skips[n:n + 1], per_n * (n + 1) + 16, per_n * (n + 1) + 24) for n in range(NG - 1)], pred)
    start(group_dma(3) + last_dma)

    def conv_passes(lead, extra=[]):
        passes = fwd_passes(0, z8)
        for grp in range(1, 4):
            f, n = fwd_passes(grp, z8), 4 * 128 // CFG["mf"]
            a, b = (n * j for j in CFG["ord"])
            passes += f[:a] + inv_passes(grp - 1, 0, z8) + f[a:b] + inv_passes(grp - 1, 1, z8) + f[b:]
        if CFG["late"]:
            return passes + lead + extra + inv_passes(3, 0, z8) + inv_passes(3, 1, z8)
        return passes + lead[:8] + inv_passes(3, 0, z8) + inv_passes(3, 1, z8) + lead[8:]

    def inverse_tasks(g):
        return [t for s in range(8) for half in range(2) for t in inv1_task(g, s, half, z8)]

    def body(i, _):
        wait(group_dma(i))
        passes = (conv_passes(y_passes(i + 1, [(0, 0, 32), (0, 32, 96)]))
                  + bu_passes(i + LEAD, 0, 0, False) + y_passes(i + 1, Y128))
        y0, end = 192 + total + 20, 192 + 2 * total
        tr, k1, k2 = filter_tasks(i + 1, CFG["kconv"])
        fwd, skips = forward_tasks(i + 1, i + 1)
        inv = inverse_tasks(i)
        tail = CFG["tail"]
        _weave(passes, [
            (scan_tasks(i + LEAD - 1, 0, z8), *CFG["scanw"]), (tr, *CFG["tr"]),
            ([skip_task(i, NG - 1, z8), dma_task([oa_unit_dma(i)])], 12, 12),
            (widen_tasks(i + 1, z8, 16), *CFG["wid"]), (k1, *CFG["kwin"]),
            (inv + [dma_task([ob_dma(i)])], *CFG["invw"]), (k2, *CFG["k2w"]),
            (fwd[:-tail], y0 - CFG["early"], end), (fwd[-tail:], end, end)]
            + [(skips[n:n + 1], end - per_n * (NG - 1 - n) + 16, end - per_n * (NG - 1 - n) + 24)
               for n in range(NG - 1)], pred)
        return 0

    lax.fori_loop(0, NG - 1, body, 0)

    wait(last_dma)
    g, u0, last = NG - 1, NG, L // UNIT - 1
    passes = (conv_passes(y_passes(u0, [(0, 0, 32), (0, 32, 96)])) + bu_passes(last, 1, 0, False)
              + y_passes(u0, [(0, 128, 128)] + y_tiles(128)[2:]) + y_passes(u0 + 1, y_tiles(128))
              + y_passes(last, Y_LAST))
    y0 = 192 + total + 20
    plan = [(scan_tasks(last - 1, 0, z8), 0, 192),
            ([skip_task(g, NG - 1, z8), dma_task([oa_unit_dma(g)])], 12, 12),
            (inverse_tasks(g) + [dma_task([ob_dma(g)])], 230, y0 + total),
            (scan_tasks(last, 1, z8), y0 + 16, y0 + 2 * total - 40)]
    out = [oa_unit_dma(u) for u in range(u0)] + [ob_dma(n) for n in range(NG)]
    for u in range(u0, last + 1):
        for n in range(NG):
            where = y0 + (u - u0) * total + per_n * (n + 1)
            plan.append(([skip_task(u, n, z8), dma_task([oa_dma(u, n)])], where, where))
            out.append(oa_dma(u, n))
    _weave(passes, plan, pred)
    wait(out)


@jax.jit
def pallas_concat_heads__ssm_conv_s5__ssm_conv_h3__prompt_kernel(
    A_x: jax.Array,
    A_Lambda_re: jax.Array,
    A_Lambda_im: jax.Array,
    A_B_re: jax.Array,
    A_B_im: jax.Array,
    A_C_re: jax.Array,
    A_C_im: jax.Array,
    A_log_dt: jax.Array,
    A_Dskip: jax.Array,
    B_q: jax.Array,
    B_k: jax.Array,
    B_v: jax.Array,
    B_shift_k: jax.Array,
    B_ssm_k: jax.Array,
    B_ssm_D: jax.Array,
):
    assert A_x.shape == (1, L, D) and B_shift_k.shape == (D, 4)
    vmem = pltpu.VMEM
    dma = pltpu.SemaphoreType.DMA
    scratch = [
        vmem(_TABLES.shape, F32),
        vmem((D,), BF16), vmem((D,), BF16), vmem((D,), BF16), vmem((D,), BF16), vmem((D,), BF16),
        vmem((4, D), BF16),
        vmem((NG * L, 128), BF16),
        vmem((2 * D, D), BF16),
        vmem((2 * NG * D, 128), BF16),
        vmem((NG * L, 128), BF16),
        vmem((NG * L, 128), BF16),
        vmem((NG * L, 128), BF16),
        vmem((D, L), BF16),
        vmem((NG * P_ROWS * 8, 128), F32),
        vmem((2 * NG * D, 128), BF16),
        vmem((2 * NG * NG * 64, 128), I32),
        vmem((SLOTS * 128, 128), BF16),
        vmem((SLOTS * 64, 128), I32),
        vmem((2 * 2 * NG * BU_PART, 128), F32),
        vmem((2 * NG * L, 128), BF16),
        vmem((3 * NG * 8, 128), F32),
        vmem((NG * YS_ROWS, 128), F32),
        vmem((L, D), F32),
        vmem((L // 2 + 8, 128), I32),
        vmem((KF_PAD + L, 128), F32),
        vmem((2 * L + 8, 128), F32),
        vmem((2 * L + 8, 128), F32),
        vmem((2 * L + 8, 128), F32),
        vmem((32 * 128, 128), BF16),
        vmem((32 * 128, 128), BF16),
        vmem((8 * 128, 128), BF16),
        vmem((8 * 128, 128), BF16),
        vmem((NG * L, 128), F32),
        dma((S_END,)),
    ]
    out = pl.pallas_call(
        _kernel,
        out_shape=jax.ShapeDtypeStruct((L, 2 * D), F32),
        in_specs=[pl.BlockSpec(memory_space=pl.ANY)] * 16,
        out_specs=pl.BlockSpec(memory_space=pl.ANY),
        scratch_shapes=scratch,
        compiler_params=pltpu.CompilerParams(vmem_limit_bytes=100 * 1024 * 1024, flags=CFG["flags"], disable_semaphore_checks=CFG["nosem"]),
        name="s5_h3",
    )(_TABLES, A_x.reshape(L, D), A_Lambda_re, A_Lambda_im, A_B_re, A_B_im, A_C_re, A_C_im,
      A_log_dt, A_Dskip, B_q.reshape(L, D), B_k.reshape(L, D), B_v.reshape(L, D),
      B_shift_k.T, B_ssm_k, B_ssm_D)
    return out.reshape(1, L, 2 * D)
```

```python
import math

import jax
import jax.numpy as jnp
import numpy as np
from jax import lax
from jax.experimental import pallas as pl
from jax.experimental.pallas import tpu as pltpu

F32, BF16, I32 = jnp.float32, jnp.bfloat16, jnp.int32

L = 2048
D = 640
NG = D // 128
UNIT = 256
SEG = 16
R = UNIT // SEG
LEAD = 4
HALF = UNIT // 2
BU_PART = 9 * 2 * R
YS_ROWS = SEG * (R // 2 + 1)
KF_PAD = 8


class _Signed:
    def __init__(self, v, neg=False):
        self.v, self.neg = v, neg

    def __neg__(self):
        return _Signed(self.v, not self.neg)

    def __add__(self, o):
        if self.neg == o.neg:
            return _Signed(self.v + o.v, self.neg)
        return _Signed(o.v - self.v if self.neg else self.v - o.v)

    def __sub__(self, o):
        return self + (-o)

    def __mul__(self, c):
        return _Signed(self.v * np.float32(-c if self.neg else c))

    def get(self):
        return -self.v if self.neg else self.v


def _rot(re, im, num, den):
    num %= den
    h = math.sqrt(0.5)
    if num == 0:
        return re, im
    if 4 * num == den:
        return -im, re
    if 4 * num == 3 * den:
        return im, -re
    if 8 * num == den:
        return (re - im) * h, (re + im) * h
    if 8 * num == 3 * den:
        return (re + im) * (-h), (re - im) * h
    if 8 * num == 5 * den:
        return (im - re) * h, (re + im) * (-h)
    if 8 * num == 7 * den:
        return (re + im) * h, (im - re) * h
    c = math.cos(2 * math.pi * num / den)
    s = math.sin(2 * math.pi * num / den)
    return re * c - im * s, re * s + im * c


def _dft4(z, sign):
    (r0, i0), (r1, i1), (r2, i2), (r3, i3) = z
    ar, ai, br, bi = r0 + r2, i0 + i2, r0 - r2, i0 - i2
    cr, ci, dr, di = r1 + r3, i1 + i3, r1 - r3, i1 - i3
    plus, minus = (br - di, bi + dr), (br + di, bi - dr)
    if sign < 0:
        plus, minus = minus, plus
    return [(ar + cr, ai + ci), plus, (ar - cr, ai - ci), minus]


def _fwd1(n, u):
    a0, a1, b0, b1 = u
    p, q = _rot(a0, b0, n, 32), _rot(a1, b1, n + 4, 32)
    s0, s1 = a0 + b0, a1 + b1
    return [(p[0] + q[0], p[1] + q[1]), _rot(p[0] - q[0], p[1] - q[1], n, 8),
            _rot(a0 - b0, a1 - b1, n, 16), (s0 + s1, s0 - s1)]


def _fwd2(grp, z):
    if grp < 3:
        return _dft4(z, 1)
    s4 = [t[0] for t in z]
    d4 = [t[1] for t in z]
    p = (d4[0], d4[2])
    q = _rot(d4[1], d4[3], 1, 8)
    s5 = [s4[0] + s4[2], s4[1] + s4[3]]
    return [
        (s5[0] + s5[1], s5[0] - s5[1]),
        (s4[0] - s4[2], s4[1] - s4[3]),
        (p[0] + q[0], p[1] + q[1]),
        (p[0] - q[0], p[1] - q[1]),
    ]


def _inv2(grp, w):
    if grp < 3:
        return _dft4(w, -1)
    s5 = [w[0][0] + w[0][1], w[0][0] - w[0][1]]
    s4 = [s5[0] + w[1][0], s5[1] + w[1][1], s5[0] - w[1][0], s5[1] - w[1][1]]
    p = (w[2][0] + w[3][0], w[2][1] + w[3][1])
    q = _rot(w[2][0] - w[3][0], w[2][1] - w[3][1], -1, 8)
    d4 = [p[0], q[0], p[1], q[1]]
    return [(s4[n], d4[n]) for n in range(4)]


def _inv1(n, z):
    e = _rot(*z[1], -n, 8)
    p = _rot(z[0][0] + e[0], z[0][1] + e[1], -n, 32)
    q = _rot(z[0][0] - e[0], z[0][1] - e[1], -(n + 4), 32)
    d0, d1 = _rot(*z[2], -n, 16)
    s0, s1 = z[3][0] + z[3][1], z[3][0] - z[3][1]
    return [p[0] + (s0 + d0), q[0] + (s1 + d1), p[1] + (s0 - d0), q[1] + (s1 - d1)]


_F1 = [4 * (g + 2 * k) + 1 for g in range(2) for k in range(4)]
_F1 += [2 * (4 * k + 1) for k in range(4)] + [0, 8, 4, 20]
_REAL_SLOT = 12
SLOTS = len(_F1)


def _dft_tables():
    kap = np.arange(128)
    j = 8 * (kap // 16) + kap % 8
    part = (kap // 8) % 2
    pr, pc, jr, jc = part[:, None], part[None, :], j[:, None], j[None, :]
    lo = 2 * np.pi * jr * jc / 64
    base = np.where(pr == pc, np.cos(lo), np.where(pr == 0, -np.sin(lo), np.sin(lo)))
    hi = 2 * np.pi * (16 + 32 * (jr - 32)) * jc / 2048
    v0 = np.where(pr == 0, np.cos(lo), np.where(jr == 0, np.cos(np.pi * jc), np.sin(lo)))
    v32 = np.where(pr == 0, np.cos(hi), np.sin(hi))
    real = np.where(jr < 32, np.where(pc == 0, v0, 0.0), np.where(pc == 1, v32, 0.0))
    th = 2 * np.pi * np.outer(np.array(_F1), j) / 2048
    zeros = np.zeros((8, 128))
    return np.concatenate([base, real, np.cos(th), np.sin(th), zeros]).astype(np.float32)


_TABLES = _dft_tables()
_FFT_SCALE = 2.0 ** -10

(P_MU, P_RHO, P_RHO1, P_RHO2, P_RHO4, P_TAP, P_SSMD, P_DSKIP, P_COEF, P_ROWS) = (
    0, 2, 4, 6, 8, 10, 14, 15, 16, 20)
S_SMALL, S_F0, S_K0, S_C, S_OUT, S_X0, S_B, S_COL, S_END = 0, 1, 2, 3, 4, 5, 6, 9, 9 + NG - 1


def _cmul(a, b):
    return a[0] * b[0] - a[1] * b[1], a[0] * b[1] + a[1] * b[0]


def _pack(lo, hi):
    return jnp.concatenate([lo, hi], axis=0).astype(BF16)


def _unpack(w):
    v = pltpu.bitcast(w, BF16).astype(F32)
    return v[:8], v[8:]


CFG = dict(scan=22, u=24, k1=24, p2=0, inv=36, skip=30, tail=4, kconv=4, steps=2, p2n=2,
           u0w=350, kwin=(100, 216), tr=(60, 90), wid=(100, 300), scanw=(0, 250), invw=(220, 420),
           k2w=(230, 480), mf=128, mi=128, ord=(3, 4), sk0=12, invend=290,
           Q=1, invsplit=False, kg=1, k0=0.5, u0=0.35, udir=True, kdir=True,
           flags=None, nosem=False, skipme=lambda n, rows: False)


class _Gate:
    def __init__(self, pred=None, seen=()):
        self.pred, self.seen = pred, seen

    def early(self, lag):
        old = [e for e in self.seen if e[0] <= -lag]
        return max(old, key=lambda e: e[0])[1] if lag and old else None

    def value(self, v, lag):
        early = self.early(lag)
        return v if early is None else jnp.where(self.pred, v, early)

    def loads(self, ref, lag):
        early = self.early(lag)
        if early is not None:
            ref[pl.ds(ref.shape[0] - 8, 8), :] = (
                early if ref.dtype == F32 else pltpu.bitcast(early, I32))


def _weave(passes, plan, pred):
    if CFG["skipme"](len(passes), sum(q[0] for q in passes)):
        return
    begin, clock = [], [0] * 4
    for i, (n, *_) in enumerate(passes):
        begin.append(clock[i % 4] / 16)
        clock[i % 4] += n

    def index(t):
        later = [i for i, b in enumerate(begin) if b >= t - 3.999]
        if not later:
            return len(passes)
        same = [i for i in later if begin[i] == min(begin[j] for j in later)]
        return same[min(max(int((t - begin[same[0]]) / 4 * len(same)), 0), len(same) - 1)]

    at = [[] for _ in range(len(passes) + 1)]
    for tasks, lo, hi in plan:
        total, done = sum(sum(c) for c, _ in tasks) or 1, 0.0
        for costs, fn in tasks:
            where = []
            for cost in costs:
                done += cost
                where.append(index(lo + done / total * (hi - lo)))
            at[min(where)].append((fn, where))
    seen, ties = [], [[] for _ in at]
    for i, fns in enumerate(at):
        now = (begin[i] + i % 4) if i < len(begin) else clock[0] / 16
        early = [(t - now, v) for t, v in seen if t % CFG["Q"] < 1 or CFG["Q"] == 1]
        for fn, where in fns:
            for w, tie in zip(where, fn(_Gate(pred, early)) or ()):
                ties[w].append(tie)
        if i == len(passes):
            break
        n, lhs, rhs, consume = passes[i]
        w = rhs()
        for tie in ties[i]:
            w[-1] = jnp.where(pred, w[-1], tie if tie.dtype == I32 else pltpu.bitcast(tie, I32))
        d = jnp.dot(pltpu.bitcast(jnp.concatenate(lhs(), axis=0), BF16),
                    pltpu.bitcast(jnp.concatenate(w, axis=0), BF16), preferred_element_type=F32)
        seen += [(begin[i] + i % 4 + j // 16 - 4, d[j - 8:j]) for j in range(64, n + 1, 64)]
        consume(d)


def _now(tasks):
    for _, fn in tasks:
        fn(_Gate())


def _kernel(tab_hbm, x_hbm, lre_hbm, lim_hbm, bre_hbm, bim_hbm, cre_hbm, cim_hbm,
            ldt_hbm, dsk_hbm, q_hbm, k_hbm, v_hbm, tap_hbm, sk_hbm, sd_hbm,
            o_hbm,
            tab, lre_v, lim_v, ldt_v, dsk_v, sd_v, tap_v,
            xb, braw, craw, qb, kb, vb, skb,
            par, wb16, wc, mf16, mi, bu, hb16, carry, ys, oa,
            kt, kf, st_u, st_k, st_i, vu16, vk16, pb0, pb1, ob,
            sem):
    x32, q32, k32, v32, wb, mf, hb, vu, vk = (
        r.bitcast(I32) for r in (xb, qb, kb, vb, wb16, mf16, hb16, vu16, vk16))
    pb16 = (pb0, pb1)
    pb = (pb0.bitcast(I32), pb1.bitcast(I32))

    def rows(ref, start, n=8):
        return ref[pl.ds(start, n), :]

    def hint(v, n):
        return v if isinstance(v, int) or n == 1 else pl.multiple_of(v, n)

    def view(ref, start, n=None):
        return ref.at[pl.ds(hint(start, 16), n or ref.shape[0]), :]

    small = [pltpu.make_async_copy(s, d, sem.at[S_SMALL]) for s, d in (
        (lre_hbm, lre_v), (lim_hbm, lim_v), (ldt_hbm, ldt_v),
        (dsk_hbm, dsk_v), (sd_hbm, sd_v), (tap_hbm, tap_v),
        (tab_hbm.at[pl.ds(288, 8), :], tab.at[pl.ds(288, 8), :]))]
    tab_dma = pltpu.make_async_copy(
        tab_hbm.at[pl.ds(0, 288), :], tab.at[pl.ds(0, 288), :], sem.at[S_F0])

    def x_dma(u):
        return [pltpu.make_async_copy(
            x_hbm.at[pl.ds(hint(u * UNIT, UNIT), UNIT), pl.ds(128 * n, 128)],
            xb.at[pl.ds(hint(n * L + u * UNIT, UNIT), UNIT), :], sem.at[(S_X0, S_F0, S_K0, S_K0)[u] if isinstance(u, int) and u < LEAD
                                                     else S_COL + u - LEAD])
            for n in range(NG)]

    def b_dma(p):
        return [pltpu.make_async_copy(
            src.at[pl.ds(128 * p, 128), :], braw.at[pl.ds(D * c + 128 * p, 128), :],
            sem.at[S_B + (p + 1) // 2]) for c, src in enumerate((bre_hbm, bim_hbm))]

    c_dma = [pltpu.make_async_copy(
        src.at[:, pl.ds(128 * p, 128)], craw.at[pl.ds(D * (NG * c + p), D), :],
        sem.at[S_C]) for c, src in enumerate((cre_hbm, cim_hbm)) for p in range(NG)]

    def col_dma(which, g, sem_at):
        src, dst = ((k_hbm, kb), (v_hbm, vb), (q_hbm, qb))[which]
        return pltpu.make_async_copy(
            src.at[:, pl.ds(hint(128 * g, 128), 128)],
            dst.at[pl.ds(hint(L * g, L), L), :], sem.at[sem_at])

    def sk_dma(g, sem_at):
        t = hint(128 * g, 128)
        return pltpu.make_async_copy(
            sk_hbm.at[pl.ds(hint(128 * g, 128), 128), :], skb.at[pl.ds(t, 128), :],
            sem.at[sem_at])

    def oa_dma(u, n):
        t = hint(u * UNIT, UNIT)
        return pltpu.make_async_copy(
            oa.at[pl.ds(t, UNIT), pl.ds(128 * n, 128)],
            o_hbm.at[pl.ds(t, UNIT), pl.ds(128 * n, 128)], sem.at[S_OUT])

    def oa_unit_dma(u):
        t = hint(u * UNIT, UNIT)
        return pltpu.make_async_copy(
            oa.at[pl.ds(t, UNIT), :], o_hbm.at[pl.ds(t, UNIT), pl.ds(0, D)], sem.at[S_OUT])

    def ob_dma(g, half):
        h = L // 2
        return pltpu.make_async_copy(
            ob.at[pl.ds(hint(L * g + h * half, h), h), :],
            o_hbm.at[pl.ds(h * half, h), pl.ds(hint(D + 128 * g, 128), 128)], sem.at[S_OUT])

    def start(ds):
        for d in ds:
            d.start()

    def wait(ds):
        for d in ds:
            d.wait()

    def prm(g, row):
        return rows(view(par, g * (P_ROWS * 8), P_ROWS * 8), row * 8)

    def bu_passes(u, slot, z, shift):
        out = []
        xu, w = view(x32, u * (UNIT // 2), ((NG - 1) * L + UNIT) // 2), view(wb, z)
        order = [p + c * NG for p in range(NG) for c in range(2)]
        for n in order:
            sizes = [128, 128]
            if shift and n == order[0]:
                sizes = [32, 32, 96, 96]
            if shift and n == order[-1]:
                sizes = [96, 96, 32, 32]
            if shift is None:
                sizes = [64] * 4
            for m, MM in zip(np.cumsum([0] + sizes).tolist(), sizes):
                acc = []
                for kk in range(NG):
                    def lhs(m=m, kk=kk, MM=MM):
                        t = (kk * L + m) // 2
                        return [rows(xu, t + 8 * i) for i in range(MM // 16)]

                    def rhs(n=n, kk=kk):
                        return [rows(w, (n * NG + kk) * 64 + 8 * i) for i in range(8)]

                    def consume(d, m=m, n=n, kk=kk, acc=acc, MM=MM):
                        acc.append(d if kk == 0 else acc[-1] + d)
                        if kk == NG - 1:
                            for i in range(MM // 8):
                                seg, r = divmod(m + 8 * i, R)
                                row = 9 * (seg % 2 * R + r) + seg // 2
                                bu[pl.ds((slot * 2 * NG + n) * BU_PART + row, 8, stride=9), :] = (
                                    acc[-1][8 * i:8 * i + 8])
                    out.append((MM, lhs, rhs, consume))
        return out

    def scan_tasks(u, slot, z):
        steps = CFG["steps"]
        state = {}
        hu = view(hb16, u * UNIT, (2 * NG - 1) * L + UNIT)

        def b(p, ch, r):
            return tuple(rows(bu, (slot * 2 * NG + c * NG + p) * BU_PART + 9 * (ch * R + r))
                         for c in range(2))

        def step(mu, h, br):
            return (mu[0] * h[0] + br[0]) - mu[1] * h[1], (mu[0] * h[1] + br[1]) + mu[1] * h[0]

        def ends(p, gate):
            mu, ties = (gate.value(prm(p, P_MU), CFG["scan"]), prm(p, P_MU + 1)), []
            h = [b(p, ch, 0) for ch in range(2)]
            for r in range(1, R):
                h = [step(mu, h[ch], b(p, ch, r)) for ch in range(2)]
                if r % steps == 0:
                    ties.append(h[r // steps % 2][0])
            state[p] = starts(p, h)
            return ties + [state[p][1][0]]

        def starts(p, e):
            last = lax.broadcasted_iota(I32, (8, 128), 0) == 7
            rho = (prm(p, P_RHO), prm(p, P_RHO + 1))
            pair = step(rho, e[0], e[1])
            a = tuple(pltpu.roll(jnp.where(last, rows(carry, (2 * p + c) * 8), pair[c]), 1, 0)
                      for c in range(2))
            for sh, row in ((1, P_RHO1), (2, P_RHO2), (4, P_RHO4)):
                a = step((prm(p, row), prm(p, row + 1)), tuple(pltpu.roll(c, sh, 0) for c in a), a)
            return [a, step(rho, a, e[0])]

        def run(p, r0, gate):
            if r0 == 0:
                state["mu"] = (prm(p, P_MU), prm(p, P_MU + 1))
            mu, h = (gate.value(state["mu"][0], CFG["scan"]), state["mu"][1]), state[p]
            for r in range(r0, r0 + steps):
                h = [step(mu, h[ch], b(p, ch, r)) for ch in range(2)]
                for c in range(2):
                    hu[pl.ds((c * NG + p) * L + 16 * r, 16), :] = _pack(h[0][c], h[1][c])
            state[p] = h
            if r0 + steps == R:
                for c in range(2):
                    carry[pl.ds((2 * p + c) * 8, 8), :] = h[1][c]
            return [rows(view(hb, z, 8), 0)]

        tasks = []
        for p in range(NG):
            tasks.append(([16 * steps] * ((R - 1) // steps) + [46 + 16 * steps],
                          lambda gate, p=p: ends(p, gate)))
            tasks += [([18 * steps], lambda gate, p=p, r0=r0: run(p, r0, gate))
                      for r0 in range(0, R, steps)]
        return tasks

    def y_passes(h, n, sizes=(HALF,), z=0):
        out, w, hu = [], view(wc, z), view(hb, h * (HALF // 2), ((2 * NG - 1) * L + HALF) // 2)
        for t0, MM in zip(np.cumsum((0,) + sizes).tolist(), sizes):
            acc = []
            for kk in range(2 * NG):
                def lhs(t0=t0, kk=kk, MM=MM):
                    return [rows(hu, (kk * L + t0) // 2 + 8 * i) for i in range(MM // 16)]

                def rhs(kk=kk):
                    return [rows(w, (kk * NG + n) * 64 + 8 * i) for i in range(8)]

                def consume(d, t0=t0, kk=kk, acc=acc, MM=MM):
                    acc.append(d if kk == 0 else acc[-1] + d)
                    if kk == 2 * NG - 1:
                        for i in range(MM // 8):
                            r, ch = divmod(t0 // 8 + i, 2)
                            ys[pl.ds(n * YS_ROWS + ch * (R // 2 + 1) + r, 8, stride=R + 2), :] = (
                                acc[-1][8 * i:8 * i + 8])
                out.append((MM, lhs, rhs, consume))
        return out

    def skip_task(h, n):
        def fn(gate):
            dsk, ties = gate.value(prm(n, P_DSKIP), CFG["skip"]), []
            t = h // 2 * UNIT + h % 2 * (R // 2)
            xu = x32.at[pl.ds(hint(t // 2 + n * (L // 2), 4), UNIT // 2 - 4 + 8 * (n < NG - 1 or not isinstance(h, int))), :]
            ou = oa.at[pl.ds(hint(t, 8), UNIT - R // 2), :]
            for g in range(SEG):
                if g == SEG - 1 and n == NG - 1 and isinstance(h, int):
                    xs = _unpack(rows(xu, 8 * g - 4))[1]
                else:
                    xs = _unpack(rows(xu, 8 * g))[0]
                y = rows(ys, n * YS_ROWS + g * (R // 2 + 1))
                ou[pl.ds(R * g, 8), pl.ds(128 * n, 128)] = y + xs * dsk
                if g % 8 == 7:
                    ties.append(oa[pl.ds(hint(z8 + t, 8), 8), pl.ds(128 * n, 128)])
            return ties
        return ([24, 24], fn)

    def widen_tasks(g, z, pieces=2):
        def fn(i0, i1):
            kg = view(k32, g * (L // 2), L // 2)
            for i in range(i0, i1):
                lo, hi = _unpack(rows(kg, 8 * i))
                kf[pl.ds(KF_PAD + 16 * i, 8), :] = lo
                kf[pl.ds(KF_PAD + 16 * i + 8, 8), :] = hi
            return [rows(view(kf, z), 16 * i0 + KF_PAD)]
        n = L // 16 // pieces
        return [([2 * n], lambda gate, i=i: fn(i * n, (i + 1) * n)) for i in range(pieces)]

    def transpose_tasks(g, z, pieces=8):
        def fn(c0, c1):
            for c in range(c0, c1):
                t = skb[pl.ds(hint(128 * g, 128), 128), pl.ds(128 * c, 128)]
                kt[pl.ds(64 * c, 64), :] = pltpu.bitcast(t.T, I32)
            return [rows(view(kt, z), 64 * c0)]
        n = L // 128 // pieces
        return [([8 * n], lambda gate, i=i: fn(i * n, (i + 1) * n)) for i in range(pieces)]

    def staged(s, half, n, grp, c):
        return (((s * 2 + half) * 4 + n) * 4 + grp) * 16 + 8 * c

    ops1 = (18, 36, 30, 36)

    def forward_tasks_of(st, s, half, z, chunk, chunk_cost, direct):
        dst16, dst = (vu16, vu) if st is st_u else (vk16, vk)

        def second(grp, zs):
            for k, pair in enumerate(_fwd2(grp, zs)):
                dst16[pl.ds(((4 * grp + k) * 2 + half) * 128 + 16 * s, 16), :] = (
                    _pack(pair[0].get(), pair[1].get()))
            return rows(view(dst, z), (8 * grp + half) * 64 + 8 * s)

        kept = []

        def first(gate, n):
            load = chunk(gate, n)
            u = [load(16 * half + n + 4 * m) for m in range(4)]
            pairs = _fwd1(n, [_Signed(v) for v in u])
            kept.append(pairs)
            for grp in range(2 * direct, 4):
                for c in range(2):
                    st[pl.ds(staged(s, half, n, grp, c), 8), :] = pairs[grp][c].get()
            return [u[0] + u[2]] * (chunk_cost > 4) + [rows(view(st, z), staged(s, half, n, 3, 0))]

        def rest(grp):
            if direct and grp < 2:
                return [second(grp, [t[grp] for t in kept])]
            return [second(grp, [tuple(_Signed(rows(view(st, z), staged(s, half, n, grp, c)))
                                       for c in range(2)) for n in range(4)])]

        split = (chunk_cost > 4) * (chunk_cost // 2 + 1)
        one = [([split] * (split > 0) + [chunk_cost + ops1[n] - split], lambda gate, n=n: first(gate, n))
               for n in range(4)]
        if CFG["p2n"] == 4:
            two = [([20], lambda gate, grp=grp: rest(grp)) for grp in range(4)]
        else:
            two = [([40], lambda gate, grp=grp: rest(grp) and rest(grp + 1)) for grp in (0, 2)]
        h = len(two) // 2
        return (one + two[:h], two[h:]) if direct else (one, two)

    def u_tasks(g, s, half, z):
        def chunk(gate, n):
            taps = [prm(g, P_TAP + t) for t in range(4)]
            taps[0] = gate.value(taps[0], CFG["u"])
            kz, vg = view(kf, z), view(v32, g * (L // 2), L // 2)

            def load(c):
                t = 64 * c + 8 * s
                ks = rows(kz, KF_PAD + t) * taps[0]
                for lag in range(1, 4):
                    ks = ks + rows(kz, KF_PAD + t - lag) * taps[lag]
                return ks * _unpack(rows(vg, (t // 16) * 8))[s % 2]
            return load
        return forward_tasks_of(st_u, s, half, z, chunk, 36, CFG["udir"])

    def k_tasks(g, s, half, z, direct):
        def chunk(gate, n):
            if n % CFG["kg"] == 0:
                gate.loads(kt, CFG["k1"])

            def load(c):
                v = _unpack(rows(view(kt, z), 32 * c + 8 * (s // 2)))[s % 2]
                if s == 0 and c == 0:
                    first = lax.broadcasted_iota(I32, (8, 128), 0) == 0
                    v = v + jnp.where(first, prm(g, P_SSMD), 0.0)
                return v
            return load
        return forward_tasks_of(st_k, s, half, z, chunk, 4, direct)

    def fwd_passes(grp, z):
        out, MM = [], CFG["mf"]
        for slot in range(4 * grp, 4 * grp + 4):
            for part in range(128 // MM):
                got = []
                for src, half in ((vu, 0), (vk, 0), (vu, 1), (vk, 1)):
                    def lhs(slot=slot, part=part):
                        return [rows(mf, slot * 64 + MM // 2 * part + 8 * i) for i in range(MM // 16)]

                    def rhs(slot=slot, src=src, half=half):
                        return [rows(view(src, z), (2 * slot + half) * 64 + 8 * i) for i in range(8)]

                    def consume(d, slot=slot, part=part, got=got):
                        got.append(d)
                        if len(got) < 4:
                            return
                        for i in range(MM // 16):
                            u0, k0, u1, k1 = ((t[16 * i:16 * i + 8], t[16 * i + 8:16 * i + 16]) for t in got)
                            lo, a, b = _cmul(u0, k0), _cmul(u0, k1), _cmul(u1, k0)
                            if slot == _REAL_SLOT and part == 0 and i == 0:
                                first = lax.broadcasted_iota(I32, (8, 128), 0) == 0
                                lo, a, b = (tuple(jnp.where(first, 0.5 * (x[c] * y[c]), p[c]) for c in range(2))
                                            for p, x, y in ((lo, u0, k0), (a, u0, k1), (b, u1, k0)))
                            if _F1[slot] % 2:
                                hi = ((a[0] + b[0]) - lo[0], (a[1] + b[1]) - lo[1])
                            else:
                                hi = ((a[0] + b[0]) + lo[0], (a[1] + b[1]) + lo[1])
                            for half, p in enumerate((lo, hi)):
                                at = (slot % 4 * 2 + half) * 128 + MM * part + 16 * i
                                pb16[grp % 2][pl.ds(at, 16), :] = _pack(*p)
                    out.append((MM, lhs, rhs, consume))
        return out

    def inv_passes(grp, half, z):
        out, MM = [], CFG["mi"]
        for part in range(128 // MM):
            got = []
            for slot in range(4 * grp, 4 * grp + 4):
                def lhs(slot=slot, part=part):
                    return [rows(mi, slot * 64 + MM // 2 * part + 8 * i) for i in range(MM // 16)]

                def rhs(slot=slot):
                    return [rows(view(pb[grp % 2], z), (slot % 4 * 2 + half) * 64 + 8 * i)
                            for i in range(8)]

                def consume(d, part=part, got=got):
                    got.append(d)
                    if len(got) < 4:
                        return
                    for i in range(MM // 16):
                        w = [(_Signed(t[16 * i:16 * i + 8]), _Signed(t[16 * i + 8:16 * i + 16]))
                             for t in got]
                        for n, pair in enumerate(_inv2(grp, w)):
                            for c in range(2):
                                at = staged(MM // 16 * part + i, half, n, grp, c)
                                st_i[pl.ds(at, 8), :] = pair[c].get()
                out.append((MM, lhs, rhs, consume))
        return out

    def inv1_task(g, s, half, z):
        def fn(gate, ns):
            gate.loads(st_i, CFG["inv"])
            qg, og, ties = view(q32, g * (L // 2), L // 2), view(ob, g * L, L), []
            for n in ns:
                zs = [tuple(_Signed(rows(view(st_i, z), staged(s, half, n, grp, c))) for c in range(2))
                      for grp in range(4)]
                for m, y in enumerate(_inv1(n, zs)):
                    t = 64 * (16 * half + n + 4 * m) + 8 * s
                    og[pl.ds(t, 8), :] = _unpack(rows(qg, (t // 16) * 8))[s % 2] * y.get()
                ties.append(rows(view(ob, z + g * L, L), 64 * (16 * half + n) + 8 * s))
            return ties
        if CFG["invsplit"]:
            return [([12 + ops1[n]], lambda gate, n=n: fn(gate, [n])) for n in range(4)]
        return [([12 + n for n in ops1], lambda gate: fn(gate, range(4)))]

    filter0 = x_dma(1) + [sk_dma(0, S_F0), tab_dma]
    data0 = x_dma(2) + x_dma(3) + [col_dma(0, 0, S_K0), col_dma(1, 0, S_K0)]

    def group_dma(g):
        at = S_COL + g
        return [col_dma(2, g, at), sk_dma(g + 1, at), col_dma(0, g + 1, at),
                col_dma(1, g + 1, at)] + x_dma(g + LEAD)

    last_dma = col_dma(2, NG - 1, S_SMALL)

    start(b_dma(0) + small + x_dma(0))
    start(b_dma(1) + b_dma(2))
    wait(small)
    zeros = rows(tab, 288).astype(I32)
    z8 = pl.multiple_of(zeros[0, 0], 16)
    sub = lax.broadcasted_iota(I32, (8, 128), 0)
    pred = zeros == 0

    def stack(ref):
        v = ref[...].astype(F32).reshape(1, D)
        return jnp.concatenate([v[:, 128 * g:128 * (g + 1)] for g in range(NG)]
                               + [v[:, :128]] * (8 - NG), axis=0)

    lre, lim = stack(lre_v), stack(lim_v)
    dt = jnp.exp(stack(ldt_v)).astype(BF16).astype(F32)
    mag, ang = jnp.exp(dt * lre), dt * lim
    lam = (mag * jnp.cos(ang), mag * jnp.sin(ang))
    scale = jnp.maximum(jnp.abs(lre), jnp.abs(lim))
    nre, nim = lre / scale, lim / scale
    den = (nre * nre + nim * nim) * scale
    coef = _cmul(((lam[0] - 1.0) / den, lam[1] / den), (nre, -nim))
    mu = (lam[0], -lam[1])
    rho = [mu]
    for _ in range(R.bit_length() + 2):
        rho.append(_cmul(rho[-1], rho[-1]))
    dsk, ssd = stack(dsk_v), stack(sd_v)
    taps = tap_v[...].astype(F32) * _FFT_SCALE
    for g in range(NG):
        def put(row, v):
            par[pl.ds((g * P_ROWS + row) * 8, 8), :] = v

        def lanes(v):
            return jnp.broadcast_to(v[g:g + 1], (8, 128))
        for c in range(2):
            put(P_MU + c, lanes(mu[c]))
            put(P_RHO + c, lanes(rho[-4][c]))
            for n, row in enumerate((P_RHO1, P_RHO2, P_RHO4)):
                put(row + c, jnp.where(sub >= 1 << n, lanes(rho[n - 3][c]), 0.0))
        for t in range(4):
            put(P_TAP + t, jnp.broadcast_to(taps[t:t + 1, 128 * g:128 * (g + 1)], (8, 128)))
        put(P_COEF, lanes(2.0 * coef[0]))
        put(P_COEF + 1, lanes(-2.0 * coef[0]))
        put(P_COEF + 2, lanes(2.0 * coef[1]))
        put(P_SSMD, lanes(ssd))
        put(P_DSKIP, lanes(dsk))
    for i in range(2 * NG):
        carry[pl.ds(8 * i, 8), :] = jnp.zeros((8, 128), F32)
    kf[pl.ds(0, KF_PAD), :] = jnp.zeros((KF_PAD, 128), F32)

    def matrix_task(slot):
        def fn(gate):
            if slot != _REAL_SLOT:
                c, s = tab[pl.ds(256 + slot, 1), :], tab[pl.ds(272 + slot, 1), :]
            for a in range(8):
                if slot == _REAL_SLOT:
                    re, im = rows(tab, 128 + 16 * a), rows(tab, 128 + 16 * a + 8)
                else:
                    br, bi = rows(tab, 16 * a), rows(tab, 16 * a + 8)
                    re, im = c * br - s * bi, s * br + c * bi
                mf16[pl.ds(slot * 128 + 16 * a, 16), :] = _pack(re, im)
            m = pltpu.bitcast(rows(view(mf, z8), slot * 64, 64), BF16)
            mi[pl.ds(slot * 64, 64), :] = pltpu.bitcast(m.T, I32)
            return [rows(view(mf, z8), 0), rows(view(mi, z8), slot * 64)]
        return ([48, 8], fn)

    def scale_b(p, kk):
        cr, ncr, ci = prm(p, P_COEF), prm(p, P_COEF + 1), prm(p, P_COEF + 2)
        br, bi = (braw[pl.ds(D * c + 128 * p, 128), pl.ds(128 * kk, 128)].T.astype(F32)
                  for c in range(2))
        ties = []
        for i in range(8):
            r0, r1 = br[16 * i:16 * i + 8], br[16 * i + 8:16 * i + 16]
            i0, i1 = bi[16 * i:16 * i + 8], bi[16 * i + 8:16 * i + 16]
            wb16[pl.ds((p * NG + kk) * 128 + 16 * i, 16), :] = _pack(
                cr * r0 - ci * i0, cr * r1 - ci * i1)
            wb16[pl.ds(((NG + p) * NG + kk) * 128 + 16 * i, 16), :] = _pack(
                ncr * i0 - ci * r0, ncr * i1 - ci * r1)
            if i % 2:
                ties.append(rows(view(wb, z8), ((NG + p) * NG + kk) * 64))
        return ties

    def c_task(n, k0, k1):
        def fn(gate):
            for kk in range(k0, k1):
                t = craw[pl.ds(kk * D + 128 * n, 128), :]
                wc[pl.ds((kk * NG + n) * 64, 64), :] = pltpu.bitcast(t.T, I32)
            return [rows(view(wc, z8), ((k1 - 1) * NG + n) * 64)]
        return ([16], fn)

    first = bu_passes(0, 1, z8, None)
    first = [first[len(first) // NG * p:len(first) // NG * (p + 1)] for p in range(NG)]

    mats = [matrix_task(slot) for slot in range(SLOTS)]

    def scale_tasks(p):
        return [([36] * 4, lambda gate, kk=kk: scale_b(p, kk)) for kk in range(NG)]

    def dma_task(ds):
        return ([1], lambda gate: start(ds))

    def filter_tasks(g, early):
        ts = [k_tasks(g, j // 2, j % 2, z8, j >= early and CFG["kdir"]) for j in range(16)]
        return (transpose_tasks(g, z8), [q for t in ts[:early] for q in t[0]],
                [q for t in ts[:early] for q in t[1]] + [q for t in ts[early:] for q in t[0] + t[1]])

    def forward_tasks(g):
        return [t for s in range(8) for half in range(2) for t in sum(u_tasks(g, s, half, z8), [])]

    def y_block(halves, t0, z=0, lead=True, even=None):
        tiles = [(h, n) for h in halves for n in range(NG)]
        passes, plan = [], []
        for j, (h, n) in enumerate(tiles):
            sizes = (HALF,)
            if j == 0:
                if not lead:
                    continue
                sizes = (32, 96)
            if j == even:
                sizes = (64, 64)
            if j == len(tiles) - 1:
                sizes = (96, 32)
            passes += y_passes(h, n, sizes, z)
            t0 += 20
            plan.append(([skip_task(h, n)], t0 + CFG["sk0"], t0 + CFG["sk0"] + 6))
        return passes, plan

    total = 2 * NG * NG * UNIT // 64

    wait(b_dma(0))
    _now(scale_tasks(0))
    start(b_dma(3) + b_dma(4) + filter0)
    wait(x_dma(0))
    _weave(first[0], [], pred)
    start(data0)
    wait(b_dma(1) + b_dma(2))
    _now(scale_tasks(1))
    _weave(first[1] + first[2], [(scale_tasks(2), 0, 40)], pred)
    start(c_dma)
    wait(b_dma(3) + b_dma(4))
    _now(scale_tasks(3))
    _weave(first[3] + first[4], [(scale_tasks(4), 0, 40)], pred)
    start(group_dma(0))
    wait(filter0)
    tr, _, k1 = filter_tasks(0, 0)
    nk, fwd = int(CFG["k0"] * len(k1)), forward_tasks(0)
    nu = int(CFG["u0"] * len(fwd))
    _weave(bu_passes(1, 0, 0, True), [
        (scan_tasks(0, 1, z8), 0, total), (tr, 8, 32), (k1[:nk], 36, total)], pred)
    start(group_dma(1))
    wait(data0)
    _weave(bu_passes(2, 1, 0, True)[:-20] + bu_passes(3, 0, 0, True)[20:] if False else
           bu_passes(2, 1, 0, True) + bu_passes(3, 0, 0, True), [
        (scan_tasks(1, 0, z8), 0, total), (scan_tasks(2, 1, z8), total + 16, 2 * total),
        (k1[nk:], 0, total), (widen_tasks(0, z8, 16), 0, total // 2),
        (fwd[:nu], total // 2, 2 * total)], pred)
    start(group_dma(2))
    wait(c_dma)
    cs = [c_task(n, k, k + 2) for n in range(NG) for k in range(0, 2 * NG, 2)]
    _now(cs[:NG])
    yp, plan = y_block((0, 1), 0, z8, even=2)
    _weave(yp, plan + [
        (cs[n * NG:(n + 1) * NG], max(20 * (n - 1) - 8, 0), 20 * n - 8) for n in range(1, NG)] + [
        (fwd[nu:-2], 0, total), (fwd[-2:], total, total), (mats, 0, total)], pred)
    start(group_dma(3) + [last_dma, oa_unit_dma(0)])

    def conv_passes():
        passes = fwd_passes(0, z8)
        for grp in range(1, 4):
            f, n = fwd_passes(grp, z8), 4 * 128 // CFG["mf"]
            a, b = (n * j for j in CFG["ord"])
            passes += f[:a] + inv_passes(grp - 1, 0, z8) + f[a:b] + inv_passes(grp - 1, 1, z8) + f[b:]
        return passes

    def inverse_tasks(g):
        tasks = []
        for half in range(2):
            for s in range(8):
                tasks += inv1_task(g, s, half, z8)
            tasks.append(dma_task([ob_dma(g, half)]))
        return tasks

    def body(i, _):
        wait(group_dma(i))
        halves = [2 + 3 * i + j for j in range(3)]
        lead = y_passes(halves[0], 0, (32, 96))
        y0 = 192 + 20 + total
        yp, plan = y_block(halves, y0, lead=False, even=7)
        passes = (conv_passes() + lead[:8] + inv_passes(3, 0, z8) + inv_passes(3, 1, z8) + lead[8:]
                  + bu_passes(i + LEAD, 0, 0, False) + yp)
        tr, k1, k2 = filter_tasks(i + 1, CFG["kconv"])
        fwd, tail, end = forward_tasks(i + 1), CFG["tail"], y0 + 280
        done = (3 * i + 2) // 2
        _weave(passes, plan + [
            ([dma_task([oa_unit_dma(done)])], y0 + 210, y0 + 210),
            (scan_tasks(i + LEAD - 1, 0, z8), *CFG["scanw"]), (tr, *CFG["tr"]),
            ([skip_task(halves[0], 0)], 232, 238),
            (widen_tasks(i + 1, z8, 16), *CFG["wid"]), (k1, *CFG["kwin"]),
            (inverse_tasks(i), *CFG["invw"]), (k2, *CFG["k2w"]),
            (fwd[:-tail], CFG["u0w"], end), (fwd[-tail:], end, end)], pred)
        pl.when(i % 2 == 1)(lambda: start([oa_unit_dma(done + 1)]))
        return 0

    lax.fori_loop(0, NG - 1, body, 0)

    wait([last_dma])
    g, last = NG - 1, L // UNIT - 1
    yp, plan = y_block((2 * last, 2 * last + 1), 192, even=2)
    ends = [[dma_task([oa_dma(last, n)])] for n in range(NG)]
    plan += [(ends[n], t + 6, t + 6) for n, (_, _, t) in enumerate(plan[NG:])]
    _weave(conv_passes() + yp[:8] + inv_passes(3, 0, z8) + inv_passes(3, 1, z8) + yp[8:], plan + [
        (scan_tasks(last, 0, z8), 0, 170),
        (inverse_tasks(g), 216, CFG["invend"])], pred)
    wait([oa_unit_dma(u) for u in range(last)] + [oa_dma(last, n) for n in range(NG)]
         + [ob_dma(n, half) for n in range(NG) for half in range(2)])


@jax.jit
def pallas_concat_heads__ssm_conv_s5__ssm_conv_h3__prompt_kernel(
    A_x: jax.Array,
    A_Lambda_re: jax.Array,
    A_Lambda_im: jax.Array,
    A_B_re: jax.Array,
    A_B_im: jax.Array,
    A_C_re: jax.Array,
    A_C_im: jax.Array,
    A_log_dt: jax.Array,
    A_Dskip: jax.Array,
    B_q: jax.Array,
    B_k: jax.Array,
    B_v: jax.Array,
    B_shift_k: jax.Array,
    B_ssm_k: jax.Array,
    B_ssm_D: jax.Array,
):
    assert A_x.shape == (1, L, D) and B_shift_k.shape == (D, 4)
    vmem = pltpu.VMEM
    dma = pltpu.SemaphoreType.DMA
    scratch = [
        vmem(_TABLES.shape, F32),
        vmem((D,), BF16), vmem((D,), BF16), vmem((D,), BF16), vmem((D,), BF16), vmem((D,), BF16),
        vmem((4, D), BF16),
        vmem((NG * L, 128), BF16),
        vmem((2 * D, D), BF16),
        vmem((2 * NG * D, 128), BF16),
        vmem((NG * L, 128), BF16),
        vmem((NG * L, 128), BF16),
        vmem((NG * L, 128), BF16),
        vmem((D, L), BF16),
        vmem((NG * P_ROWS * 8, 128), F32),
        vmem((2 * NG * D, 128), BF16),
        vmem((2 * NG * NG * 64, 128), I32),
        vmem((SLOTS * 128, 128), BF16),
        vmem((SLOTS * 64, 128), I32),
        vmem((2 * 2 * NG * BU_PART, 128), F32),
        vmem((2 * NG * L, 128), BF16),
        vmem((3 * NG * 8, 128), F32),
        vmem((NG * YS_ROWS, 128), F32),
        vmem((L, D), F32),
        vmem((L // 2 + 8, 128), I32),
        vmem((KF_PAD + L, 128), F32),
        vmem((2 * L + 8, 128), F32),
        vmem((2 * L + 8, 128), F32),
        vmem((2 * L + 8, 128), F32),
        vmem((32 * 128, 128), BF16),
        vmem((32 * 128, 128), BF16),
        vmem((8 * 128, 128), BF16),
        vmem((8 * 128, 128), BF16),
        vmem((NG * L, 128), F32),
        dma((S_END,)),
    ]
    out = pl.pallas_call(
        _kernel,
        out_shape=jax.ShapeDtypeStruct((L, 2 * D), F32),
        in_specs=[pl.BlockSpec(memory_space=pl.ANY)] * 16,
        out_specs=pl.BlockSpec(memory_space=pl.ANY),
        scratch_shapes=scratch,
        compiler_params=pltpu.CompilerParams(vmem_limit_bytes=100 * 1024 * 1024, flags=CFG["flags"], disable_semaphore_checks=CFG["nosem"]),
        name="s5_h3",
    )(_TABLES, A_x.reshape(L, D), A_Lambda_re, A_Lambda_im, A_B_re, A_B_im, A_C_re, A_C_im,
      A_log_dt, A_Dskip, B_q.reshape(L, D), B_k.reshape(L, D), B_v.reshape(L, D),
      B_shift_k.T, B_ssm_k, B_ssm_D)
    return out.reshape(1, L, 2 * D)
```

```python
import math

import jax
import jax.numpy as jnp
import numpy as np
from jax import lax
from jax.experimental import pallas as pl
from jax.experimental.pallas import tpu as pltpu

F32, BF16, I32 = jnp.float32, jnp.bfloat16, jnp.int32

L = 2048
D = 640
NG = D // 128
UNIT = 256
SEG = 16
R = UNIT // SEG
LEAD = 4
HALF = UNIT // 2
BU_PART = 9 * 2 * R
YS_ROWS = SEG * (R // 2 + 1)
KF_PAD = 8


class _Signed:
    def __init__(self, v, neg=False):
        self.v, self.neg = v, neg

    def __neg__(self):
        return _Signed(self.v, not self.neg)

    def __add__(self, o):
        if self.neg == o.neg:
            return _Signed(self.v + o.v, self.neg)
        return _Signed(o.v - self.v if self.neg else self.v - o.v)

    def __sub__(self, o):
        return self + (-o)

    def __mul__(self, c):
        return _Signed(self.v * np.float32(-c if self.neg else c))

    def get(self):
        return -self.v if self.neg else self.v


def _rot(re, im, num, den):
    num %= den
    h = math.sqrt(0.5)
    if num == 0:
        return re, im
    if 4 * num == den:
        return -im, re
    if 4 * num == 3 * den:
        return im, -re
    if 8 * num == den:
        return (re - im) * h, (re + im) * h
    if 8 * num == 3 * den:
        return (re + im) * (-h), (re - im) * h
    if 8 * num == 5 * den:
        return (im - re) * h, (re + im) * (-h)
    if 8 * num == 7 * den:
        return (re + im) * h, (im - re) * h
    c = math.cos(2 * math.pi * num / den)
    s = math.sin(2 * math.pi * num / den)
    return re * c - im * s, re * s + im * c


def _dft4(z, sign):
    (r0, i0), (r1, i1), (r2, i2), (r3, i3) = z
    ar, ai, br, bi = r0 + r2, i0 + i2, r0 - r2, i0 - i2
    cr, ci, dr, di = r1 + r3, i1 + i3, r1 - r3, i1 - i3
    plus, minus = (br - di, bi + dr), (br + di, bi - dr)
    if sign < 0:
        plus, minus = minus, plus
    return [(ar + cr, ai + ci), plus, (ar - cr, ai - ci), minus]


def _fwd1(n, u):
    a0, a1, b0, b1 = u
    p, q = _rot(a0, b0, n, 32), _rot(a1, b1, n + 4, 32)
    s0, s1 = a0 + b0, a1 + b1
    return [(p[0] + q[0], p[1] + q[1]), _rot(p[0] - q[0], p[1] - q[1], n, 8),
            _rot(a0 - b0, a1 - b1, n, 16), (s0 + s1, s0 - s1)]


def _fwd2(grp, z):
    if grp < 3:
        return _dft4(z, 1)
    s4 = [t[0] for t in z]
    d4 = [t[1] for t in z]
    p = (d4[0], d4[2])
    q = _rot(d4[1], d4[3], 1, 8)
    s5 = [s4[0] + s4[2], s4[1] + s4[3]]
    return [
        (s5[0] + s5[1], s5[0] - s5[1]),
        (s4[0] - s4[2], s4[1] - s4[3]),
        (p[0] + q[0], p[1] + q[1]),
        (p[0] - q[0], p[1] - q[1]),
    ]


def _inv2(grp, w):
    if grp < 3:
        return _dft4(w, -1)
    s5 = [w[0][0] + w[0][1], w[0][0] - w[0][1]]
    s4 = [s5[0] + w[1][0], s5[1] + w[1][1], s5[0] - w[1][0], s5[1] - w[1][1]]
    p = (w[2][0] + w[3][0], w[2][1] + w[3][1])
    q = _rot(w[2][0] - w[3][0], w[2][1] - w[3][1], -1, 8)
    d4 = [p[0], q[0], p[1], q[1]]
    return [(s4[n], d4[n]) for n in range(4)]


def _inv1(n, z):
    e = _rot(*z[1], -n, 8)
    p = _rot(z[0][0] + e[0], z[0][1] + e[1], -n, 32)
    q = _rot(z[0][0] - e[0], z[0][1] - e[1], -(n + 4), 32)
    d0, d1 = _rot(*z[2], -n, 16)
    s0, s1 = z[3][0] + z[3][1], z[3][0] - z[3][1]
    return [p[0] + (s0 + d0), q[0] + (s1 + d1), p[1] + (s0 - d0), q[1] + (s1 - d1)]


_F1 = [4 * (g + 2 * k) + 1 for g in range(2) for k in range(4)]
_F1 += [2 * (4 * k + 1) for k in range(4)] + [0, 8, 4, 20]
_REAL_SLOT = 12
SLOTS = len(_F1)


def _dft_tables():
    kap = np.arange(128)
    j = 8 * (kap // 16) + kap % 8
    part = (kap // 8) % 2
    pr, pc, jr, jc = part[:, None], part[None, :], j[:, None], j[None, :]
    lo = 2 * np.pi * jr * jc / 64
    base = np.where(pr == pc, np.cos(lo), np.where(pr == 0, -np.sin(lo), np.sin(lo)))
    hi = 2 * np.pi * (16 + 32 * (jr - 32)) * jc / 2048
    v0 = np.where(pr == 0, np.cos(lo), np.where(jr == 0, np.cos(np.pi * jc), np.sin(lo)))
    v32 = np.where(pr == 0, np.cos(hi), np.sin(hi))
    real = np.where(jr < 32, np.where(pc == 0, v0, 0.0), np.where(pc == 1, v32, 0.0))
    th = 2 * np.pi * np.outer(np.array(_F1), j) / 2048
    zeros = np.zeros((8, 128))
    return np.concatenate([base, real, np.cos(th), np.sin(th), zeros]).astype(np.float32)


_TABLES = _dft_tables()
_FFT_SCALE = 2.0 ** -10

(P_MU, P_RHO, P_RHO1, P_RHO2, P_RHO4, P_TAP, P_SSMD, P_DSKIP, P_COEF, P_ROWS) = (
    0, 2, 4, 6, 8, 10, 14, 15, 16, 20)
S_SMALL, S_F0, S_K0, S_C, S_OUT, S_B = range(6)
S_COL = S_B + NG
S_END = S_COL + NG - 1


def _cmul(a, b):
    return a[0] * b[0] - a[1] * b[1], a[0] * b[1] + a[1] * b[0]


def _pack(lo, hi):
    return jnp.concatenate([lo, hi], axis=0).astype(BF16)


def _unpack(w):
    v = pltpu.bitcast(w, BF16).astype(F32)
    return v[:8], v[8:]


CFG = dict(scan=22, u=24, k1=0, p2=0, inv=36, skip=30, tail=4, kconv=4, steps=2, p2n=2,
           u0w=350, kwin=(100, 216), tr=(60, 90), wid=(100, 300), scanw=(0, 250), invw=(220, 420),
           k2w=(230, 480), mf=128, mi=128, ord=(3, 4), sk0=12, invend=290,
           Q=1, invsplit=False, kg=1, k0=0.7, u0=0.25, udir=True, kdir=True,
           flags=None, nosem=False, skipme=lambda n, rows: False)


class _Zeros:
    def __init__(self, v):
        self.v = v


class _Gate:
    def __init__(self, pred=None, seen=()):
        self.pred, self.seen = pred, seen

    def early(self, lag):
        old = [e for e in self.seen if e[0] <= -lag]
        return max(old, key=lambda e: e[0])[1] if lag and old else None

    def value(self, v, lag):
        early = self.early(lag)
        return v if early is None else jnp.where(self.pred, v, early)

    def loads(self, ref, lag):
        early = self.early(lag)
        if early is not None:
            ref[pl.ds(ref.shape[0] - 8, 8), :] = (
                early if ref.dtype == F32 else pltpu.bitcast(early, I32))


def _weave(passes, plan, pred):
    if CFG["skipme"](len(passes), sum(q[0] for q in passes)):
        return
    begin, clock = [], [0] * 4
    for i, (n, *_) in enumerate(passes):
        begin.append(clock[i % 4] / 16)
        clock[i % 4] += n

    def index(t):
        later = [i for i, b in enumerate(begin) if b >= t - 3.999]
        if not later:
            return len(passes)
        same = [i for i in later if begin[i] == min(begin[j] for j in later)]
        return same[min(max(int((t - begin[same[0]]) / 4 * len(same)), 0), len(same) - 1)]

    at = [[] for _ in range(len(passes) + 1)]
    for tasks, lo, hi in plan:
        total, done = sum(sum(c) for c, _ in tasks) or 1, 0.0
        for costs, fn in tasks:
            where = []
            for cost in costs:
                done += cost
                where.append(index(lo + done / total * (hi - lo)))
            at[min(where)].append((fn, where))
    seen, ties = [], [[] for _ in at]
    for i, fns in enumerate(at):
        now = (begin[i] + i % 4) if i < len(begin) else clock[0] / 16
        early = [(t - now, v) for t, v in seen if t % CFG["Q"] < 1 or CFG["Q"] == 1]
        for fn, where in fns:
            for w, tie in zip(where, fn(_Gate(pred, early)) or ()):
                ties[w].append(tie)
        if i == len(passes):
            break
        n, lhs, rhs, consume = passes[i]
        w = rhs()
        for tie in ties[i]:
            if isinstance(tie, _Zeros):
                v = tie.v
                w[-1] = w[-1] | (v if v.dtype == I32 else pltpu.bitcast(v, I32))
            else:
                w[-1] = jnp.where(pred, w[-1], pltpu.bitcast(tie, I32))
        d = jnp.dot(pltpu.bitcast(jnp.concatenate(lhs(), axis=0), BF16),
                    pltpu.bitcast(jnp.concatenate(w, axis=0), BF16), preferred_element_type=F32)
        seen += [(begin[i] + i % 4 + j // 16 - 4, d[j - 8:j]) for j in range(64, n + 1, 64)]
        consume(d)


def _now(tasks):
    for _, fn in tasks:
        fn(_Gate())


def _kernel(tab_hbm, x_hbm, lre_hbm, lim_hbm, bre_hbm, bim_hbm, cre_hbm, cim_hbm,
            ldt_hbm, dsk_hbm, q_hbm, k_hbm, v_hbm, tap_hbm, sk_hbm, sd_hbm,
            o_hbm,
            tab, lre_v, lim_v, ldt_v, dsk_v, sd_v, tap_v,
            xb, braw, craw, qb, kb, vb, skb,
            par, wb16, wc, mf16, mi, bu, hb16, carry, ys, oa,
            kt, kf, st_u, st_k, st_i, vu16, vk16, pb0, pb1, ob,
            sem):
    x32, q32, k32, v32, wb, mf, hb, vu, vk = (
        r.bitcast(I32) for r in (xb, qb, kb, vb, wb16, mf16, hb16, vu16, vk16))
    pb16 = (pb0, pb1)
    pb = (pb0.bitcast(I32), pb1.bitcast(I32))

    def rows(ref, start, n=8):
        return ref[pl.ds(start, n), :]

    def hint(v, n):
        return v if isinstance(v, int) or n == 1 else pl.multiple_of(v, n)

    def view(ref, start, n=None):
        return ref.at[pl.ds(hint(start, 16), n or ref.shape[0]), :]

    def after(ref):
        return _Zeros(view(ref, z8)[ref.shape[0] - 16:ref.shape[0] - 8, 0:128])

    small = [pltpu.make_async_copy(s, d, sem.at[S_SMALL]) for s, d in (
        (lre_hbm, lre_v), (lim_hbm, lim_v), (ldt_hbm, ldt_v),
        (dsk_hbm, dsk_v), (sd_hbm, sd_v), (tap_hbm, tap_v),
        (tab_hbm.at[pl.ds(288, 8), :], tab.at[pl.ds(288, 8), :]))]
    tab_dma = pltpu.make_async_copy(
        tab_hbm.at[pl.ds(0, 288), :], tab.at[pl.ds(0, 288), :], sem.at[S_C])

    def x_dma(u):
        return [pltpu.make_async_copy(
            x_hbm.at[pl.ds(hint(u * UNIT, UNIT), UNIT), pl.ds(128 * n, 128)],
            xb.at[pl.ds(hint(n * L + u * UNIT, UNIT), UNIT), :], sem.at[(S_B + 1, S_B + 4, S_F0, S_K0)[u] if isinstance(u, int) and u < LEAD
                                                     else S_COL + u - LEAD])
            for n in range(NG)]

    def b_dma(p):
        return [pltpu.make_async_copy(
            src.at[pl.ds(128 * p, 128), :], braw.at[pl.ds(D * c + 128 * p, 128), :],
            sem.at[S_B + p]) for c, src in enumerate((bre_hbm, bim_hbm))]

    c_dma = [pltpu.make_async_copy(
        src.at[:, pl.ds(128 * p, 128)], craw.at[pl.ds(D * (NG * c + p), D), :],
        sem.at[S_C]) for c, src in enumerate((cre_hbm, cim_hbm)) for p in range(NG)]

    def col_dma(which, g, sem_at):
        src, dst = ((k_hbm, kb), (v_hbm, vb), (q_hbm, qb))[which]
        return pltpu.make_async_copy(
            src.at[:, pl.ds(hint(128 * g, 128), 128)],
            dst.at[pl.ds(hint(L * g, L), L), :], sem.at[sem_at])

    def sk_dma(g, sem_at):
        t = hint(128 * g, 128)
        return pltpu.make_async_copy(
            sk_hbm.at[pl.ds(hint(128 * g, 128), 128), :], skb.at[pl.ds(t, 128), :],
            sem.at[sem_at])

    def oa_dma(u, n):
        t = hint(u * UNIT, UNIT)
        return pltpu.make_async_copy(
            oa.at[pl.ds(t, UNIT), pl.ds(128 * n, 128)],
            o_hbm.at[pl.ds(t, UNIT), pl.ds(128 * n, 128)], sem.at[S_OUT])

    def oa_unit_dma(u):
        t = hint(u * UNIT, UNIT)
        return pltpu.make_async_copy(
            oa.at[pl.ds(t, UNIT), :], o_hbm.at[pl.ds(t, UNIT), pl.ds(0, D)], sem.at[S_OUT])

    def ob_dma(g, half):
        h = L // 2
        return pltpu.make_async_copy(
            ob.at[pl.ds(hint(L * g + h * half, h), h), :],
            o_hbm.at[pl.ds(h * half, h), pl.ds(hint(D + 128 * g, 128), 128)], sem.at[S_OUT])

    def start(ds):
        for d in ds:
            d.start()

    def wait(ds):
        for d in ds:
            d.wait()

    def prm(g, row):
        return rows(view(par, g * (P_ROWS * 8), P_ROWS * 8), row * 8)

    def bu_passes(u, slot, z, shift):
        out = []
        xu, w = view(x32, u * (UNIT // 2), ((NG - 1) * L + UNIT) // 2), view(wb, z)
        order = [p + c * NG for p in range(NG) for c in range(2)]
        for n in order:
            sizes = [128, 128]
            if shift and n == order[0]:
                sizes = [32, 32, 96, 96]
            if shift and n == order[-1]:
                sizes = [96, 96, 32, 32]
            if shift is None:
                sizes = [64] * 4
            for m, MM in zip(np.cumsum([0] + sizes).tolist(), sizes):
                acc = []
                for kk in range(NG):
                    def lhs(m=m, kk=kk, MM=MM):
                        t = (kk * L + m) // 2
                        return [rows(xu, t + 8 * i) for i in range(MM // 16)]

                    def rhs(n=n, kk=kk):
                        return [rows(w, (n * NG + kk) * 64 + 8 * i) for i in range(8)]

                    def consume(d, m=m, n=n, kk=kk, acc=acc, MM=MM):
                        acc.append(d if kk == 0 else acc[-1] + d)
                        if kk == NG - 1:
                            for i in range(MM // 8):
                                seg, r = divmod(m + 8 * i, R)
                                row = 9 * (seg % 2 * R + r) + seg // 2
                                bu[pl.ds((slot * 2 * NG + n) * BU_PART + row, 8, stride=9), :] = (
                                    acc[-1][8 * i:8 * i + 8])
                    out.append((MM, lhs, rhs, consume))
        return out

    def scan_tasks(u, slot, z):
        steps = CFG["steps"]
        state = {}
        hu = view(hb16, u * UNIT, (2 * NG - 1) * L + UNIT)

        def b(p, ch, r):
            return tuple(rows(bu, (slot * 2 * NG + c * NG + p) * BU_PART + 9 * (ch * R + r))
                         for c in range(2))

        def step(mu, h, br):
            return (mu[0] * h[0] + br[0]) - mu[1] * h[1], (mu[0] * h[1] + br[1]) + mu[1] * h[0]

        def ends(p, gate):
            mu, ties = (gate.value(prm(p, P_MU), CFG["scan"]), prm(p, P_MU + 1)), []
            h = [b(p, ch, 0) for ch in range(2)]
            for r in range(1, R):
                h = [step(mu, h[ch], b(p, ch, r)) for ch in range(2)]
                if r % steps == 0:
                    ties.append(h[r // steps % 2][0])
            state[p] = starts(p, h)
            return ties + [state[p][1][0]]

        def starts(p, e):
            last = lax.broadcasted_iota(I32, (8, 128), 0) == 7
            rho = (prm(p, P_RHO), prm(p, P_RHO + 1))
            pair = step(rho, e[0], e[1])
            a = tuple(pltpu.roll(jnp.where(last, rows(carry, (2 * p + c) * 8), pair[c]), 1, 0)
                      for c in range(2))
            for sh, row in ((1, P_RHO1), (2, P_RHO2), (4, P_RHO4)):
                a = step((prm(p, row), prm(p, row + 1)), tuple(pltpu.roll(c, sh, 0) for c in a), a)
            return [a, step(rho, a, e[0])]

        def run(p, r0, gate):
            if r0 == 0:
                state["mu"] = (prm(p, P_MU), prm(p, P_MU + 1))
            mu, h = (gate.value(state["mu"][0], CFG["scan"]), state["mu"][1]), state[p]
            for r in range(r0, r0 + steps):
                h = [step(mu, h[ch], b(p, ch, r)) for ch in range(2)]
                for c in range(2):
                    hu[pl.ds((c * NG + p) * L + 16 * r, 16), :] = _pack(h[0][c], h[1][c])
            state[p] = h
            if r0 + steps == R:
                for c in range(2):
                    carry[pl.ds((2 * p + c) * 8, 8), :] = h[1][c]
            return [after(hb)]

        tasks = []
        for p in range(NG):
            tasks.append(([16 * steps] * ((R - 1) // steps) + [46 + 16 * steps],
                          lambda gate, p=p: ends(p, gate)))
            tasks += [([18 * steps], lambda gate, p=p, r0=r0: run(p, r0, gate))
                      for r0 in range(0, R, steps)]
        return tasks

    def y_passes(h, n, sizes=(HALF,), z=0):
        out, w, hu = [], view(wc, z), view(hb, h * (HALF // 2), ((2 * NG - 1) * L + HALF) // 2)
        for t0, MM in zip(np.cumsum((0,) + sizes).tolist(), sizes):
            acc = []
            for kk in range(2 * NG):
                def lhs(t0=t0, kk=kk, MM=MM):
                    return [rows(hu, (kk * L + t0) // 2 + 8 * i) for i in range(MM // 16)]

                def rhs(kk=kk):
                    return [rows(w, (kk * NG + n) * 64 + 8 * i) for i in range(8)]

                def consume(d, t0=t0, kk=kk, acc=acc, MM=MM):
                    acc.append(d if kk == 0 else acc[-1] + d)
                    if kk == 2 * NG - 1:
                        for i in range(MM // 8):
                            r, ch = divmod(t0 // 8 + i, 2)
                            ys[pl.ds(n * YS_ROWS + ch * (R // 2 + 1) + r, 8, stride=R + 2), :] = (
                                acc[-1][8 * i:8 * i + 8])
                out.append((MM, lhs, rhs, consume))
        return out

    def skip_task(h, n):
        def fn(gate):
            dsk, ties = gate.value(prm(n, P_DSKIP), CFG["skip"]), []
            t = h // 2 * UNIT + h % 2 * (R // 2)
            xu = x32.at[pl.ds(hint(t // 2 + n * (L // 2), 4), UNIT // 2 - 4 + 8 * (n < NG - 1 or not isinstance(h, int))), :]
            ou = oa.at[pl.ds(hint(t, 8), UNIT - R // 2), :]
            for g in range(SEG):
                if g == SEG - 1 and n == NG - 1 and isinstance(h, int):
                    xs = _unpack(rows(xu, 8 * g - 4))[1]
                else:
                    xs = _unpack(rows(xu, 8 * g))[0]
                y = rows(ys, n * YS_ROWS + g * (R // 2 + 1))
                ou[pl.ds(R * g, 8), pl.ds(128 * n, 128)] = y + xs * dsk
                if g % 8 == 7:
                    ties.append(after(oa))
            return ties
        return ([24, 24], fn)

    def widen_tasks(g, z, pieces=2):
        def fn(i0, i1):
            kg = view(k32, g * (L // 2), L // 2)
            for i in range(i0, i1):
                lo, hi = _unpack(rows(kg, 8 * i))
                kf[pl.ds(KF_PAD + 16 * i, 8), :] = lo
                kf[pl.ds(KF_PAD + 16 * i + 8, 8), :] = hi
            return [after(kf)]
        n = L // 16 // pieces
        return [([2 * n], lambda gate, i=i: fn(i * n, (i + 1) * n)) for i in range(pieces)]

    def transpose_tasks(g, z, pieces=8):
        def fn(c0, c1):
            for c in range(c0, c1):
                t = skb[pl.ds(hint(128 * g, 128), 128), pl.ds(128 * c, 128)]
                kt[pl.ds(64 * c, 64), :] = pltpu.bitcast(t.T, I32)
            return [after(kt)]
        n = L // 128 // pieces
        return [([8 * n], lambda gate, i=i: fn(i * n, (i + 1) * n)) for i in range(pieces)]

    def staged(s, half, n, grp, c):
        return (((s * 2 + half) * 4 + n) * 4 + grp) * 16 + 8 * c

    ops1 = (18, 36, 30, 36)

    def forward_tasks_of(st, s, half, z, chunk, chunk_cost, direct):
        dst16, dst = (vu16, vu) if st is st_u else (vk16, vk)

        def second(grp, zs):
            for k, pair in enumerate(_fwd2(grp, zs)):
                dst16[pl.ds(((4 * grp + k) * 2 + half) * 128 + 16 * s, 16), :] = (
                    _pack(pair[0].get(), pair[1].get()))
            return after(dst)

        kept = []

        def first(gate, n):
            load = chunk(gate, n)
            u = [load(16 * half + n + 4 * m) for m in range(4)]
            pairs = _fwd1(n, [_Signed(v) for v in u])
            kept.append(pairs)
            for grp in range(2 * direct, 4):
                for c in range(2):
                    st[pl.ds(staged(s, half, n, grp, c), 8), :] = pairs[grp][c].get()
            return [u[0] + u[2]] * (chunk_cost > 4) + [after(st)]

        def rest(grp):
            if direct and grp < 2:
                return [second(grp, [t[grp] for t in kept])]
            return [second(grp, [tuple(_Signed(rows(view(st, z), staged(s, half, n, grp, c)))
                                       for c in range(2)) for n in range(4)])]

        split = (chunk_cost > 4) * (chunk_cost // 2 + 1)
        one = [([split] * (split > 0) + [chunk_cost + ops1[n] - split], lambda gate, n=n: first(gate, n))
               for n in range(4)]
        if CFG["p2n"] == 4:
            two = [([20], lambda gate, grp=grp: rest(grp)) for grp in range(4)]
        else:
            two = [([40], lambda gate, grp=grp: rest(grp) and rest(grp + 1)) for grp in (0, 2)]
        h = len(two) // 2
        return (one + two[:h], two[h:]) if direct else (one, two)

    def u_tasks(g, s, half, z):
        def chunk(gate, n):
            taps = [prm(g, P_TAP + t) for t in range(4)]
            taps[0] = gate.value(taps[0], CFG["u"])
            kz, vg = view(kf, z), view(v32, g * (L // 2), L // 2)

            def load(c):
                t = 64 * c + 8 * s
                ks = rows(kz, KF_PAD + t) * taps[0]
                for lag in range(1, 4):
                    ks = ks + rows(kz, KF_PAD + t - lag) * taps[lag]
                return ks * _unpack(rows(vg, (t // 16) * 8))[s % 2]
            return load
        return forward_tasks_of(st_u, s, half, z, chunk, 36, CFG["udir"])

    def k_tasks(g, s, half, z, direct):
        def chunk(gate, n):
            if n % CFG["kg"] == 0:
                gate.loads(kt, CFG["k1"])

            def load(c):
                v = _unpack(rows(view(kt, z), 32 * c + 8 * (s // 2)))[s % 2]
                if s == 0 and c == 0:
                    first = lax.broadcasted_iota(I32, (8, 128), 0) == 0
                    v = v + jnp.where(first, prm(g, P_SSMD), 0.0)
                return v
            return load
        return forward_tasks_of(st_k, s, half, z, chunk, 4, direct)

    def fwd_passes(grp, z):
        out, MM = [], CFG["mf"]
        for slot in range(4 * grp, 4 * grp + 4):
            for part in range(128 // MM):
                got = []
                for src, half in ((vu, 0), (vk, 0), (vu, 1), (vk, 1)):
                    def lhs(slot=slot, part=part):
                        return [rows(mf, slot * 64 + MM // 2 * part + 8 * i) for i in range(MM // 16)]

                    def rhs(slot=slot, src=src, half=half):
                        return [rows(view(src, z), (2 * slot + half) * 64 + 8 * i) for i in range(8)]

                    def consume(d, slot=slot, part=part, got=got):
                        got.append(d)
                        if len(got) < 4:
                            return
                        for i in range(MM // 16):
                            u0, k0, u1, k1 = ((t[16 * i:16 * i + 8], t[16 * i + 8:16 * i + 16]) for t in got)
                            lo, a, b = _cmul(u0, k0), _cmul(u0, k1), _cmul(u1, k0)
                            if slot == _REAL_SLOT and part == 0 and i == 0:
                                first = lax.broadcasted_iota(I32, (8, 128), 0) == 0
                                lo, a, b = (tuple(jnp.where(first, 0.5 * (x[c] * y[c]), p[c]) for c in range(2))
                                            for p, x, y in ((lo, u0, k0), (a, u0, k1), (b, u1, k0)))
                            if _F1[slot] % 2:
                                hi = ((a[0] + b[0]) - lo[0], (a[1] + b[1]) - lo[1])
                            else:
                                hi = ((a[0] + b[0]) + lo[0], (a[1] + b[1]) + lo[1])
                            for half, p in enumerate((lo, hi)):
                                at = (slot % 4 * 2 + half) * 128 + MM * part + 16 * i
                                pb16[grp % 2][pl.ds(at, 16), :] = _pack(*p)
                    out.append((MM, lhs, rhs, consume))
        return out

    def inv_passes(grp, half, z):
        out, MM = [], CFG["mi"]
        for part in range(128 // MM):
            got = []
            for slot in range(4 * grp, 4 * grp + 4):
                def lhs(slot=slot, part=part):
                    return [rows(mi, slot * 64 + MM // 2 * part + 8 * i) for i in range(MM // 16)]

                def rhs(slot=slot):
                    return [rows(view(pb[grp % 2], z), (slot % 4 * 2 + half) * 64 + 8 * i)
                            for i in range(8)]

                def consume(d, part=part, got=got):
                    got.append(d)
                    if len(got) < 4:
                        return
                    for i in range(MM // 16):
                        w = [(_Signed(t[16 * i:16 * i + 8]), _Signed(t[16 * i + 8:16 * i + 16]))
                             for t in got]
                        for n, pair in enumerate(_inv2(grp, w)):
                            for c in range(2):
                                at = staged(MM // 16 * part + i, half, n, grp, c)
                                st_i[pl.ds(at, 8), :] = pair[c].get()
                out.append((MM, lhs, rhs, consume))
        return out

    def inv1_task(g, s, half, z):
        def fn(gate, ns):
            gate.loads(st_i, CFG["inv"])
            qg, og, ties = view(q32, g * (L // 2), L // 2), view(ob, g * L, L), []
            for n in ns:
                zs = [tuple(_Signed(rows(view(st_i, z), staged(s, half, n, grp, c))) for c in range(2))
                      for grp in range(4)]
                for m, y in enumerate(_inv1(n, zs)):
                    t = 64 * (16 * half + n + 4 * m) + 8 * s
                    og[pl.ds(t, 8), :] = _unpack(rows(qg, (t // 16) * 8))[s % 2] * y.get()
                ties.append(after(ob))
            return ties
        if CFG["invsplit"]:
            return [([12 + ops1[n]], lambda gate, n=n: fn(gate, [n])) for n in range(4)]
        return [([12 + n for n in ops1], lambda gate: fn(gate, range(4)))]

    filter0 = x_dma(2) + [sk_dma(0, S_F0)]
    data0 = x_dma(3) + [col_dma(0, 0, S_K0), col_dma(1, 0, S_K0)]

    def group_dma(g):
        at = S_COL + g
        return [col_dma(2, g, at), sk_dma(g + 1, at), col_dma(0, g + 1, at),
                col_dma(1, g + 1, at)] + x_dma(g + LEAD)

    last_dma = col_dma(2, NG - 1, S_SMALL)

    start(small + b_dma(0) + x_dma(0) + b_dma(1) + b_dma(2))
    wait(small)
    zeros = rows(tab, 288).astype(I32)
    z8 = pl.multiple_of(zeros[0, 0], 16)
    sub = lax.broadcasted_iota(I32, (8, 128), 0)
    pred = zeros == 0

    def stack(ref):
        v = ref[...].astype(F32).reshape(1, D)
        return jnp.concatenate([v[:, 128 * g:128 * (g + 1)] for g in range(NG)]
                               + [v[:, :128]] * (8 - NG), axis=0)

    lre, lim = stack(lre_v), stack(lim_v)
    dt = jnp.exp(stack(ldt_v)).astype(BF16).astype(F32)
    mag, ang = jnp.exp(dt * lre), dt * lim
    lam = (mag * jnp.cos(ang), mag * jnp.sin(ang))
    scale = jnp.maximum(jnp.abs(lre), jnp.abs(lim))
    nre, nim = lre / scale, lim / scale
    den = (nre * nre + nim * nim) * scale
    coef = _cmul(((lam[0] - 1.0) / den, lam[1] / den), (nre, -nim))
    mu = (lam[0], -lam[1])
    rho = [mu]
    for _ in range(R.bit_length() + 2):
        rho.append(_cmul(rho[-1], rho[-1]))
    dsk, ssd = stack(dsk_v), stack(sd_v)
    taps = tap_v[...].astype(F32) * _FFT_SCALE
    for g in range(NG):
        def put(row, v):
            par[pl.ds((g * P_ROWS + row) * 8, 8), :] = v

        def lanes(v):
            return jnp.broadcast_to(v[g:g + 1], (8, 128))
        for c in range(2):
            put(P_MU + c, lanes(mu[c]))
            put(P_RHO + c, lanes(rho[-4][c]))
            for n, row in enumerate((P_RHO1, P_RHO2, P_RHO4)):
                put(row + c, jnp.where(sub >= 1 << n, lanes(rho[n - 3][c]), 0.0))
        for t in range(4):
            put(P_TAP + t, jnp.broadcast_to(taps[t:t + 1, 128 * g:128 * (g + 1)], (8, 128)))
        put(P_COEF, lanes(2.0 * coef[0]))
        put(P_COEF + 1, lanes(-2.0 * coef[0]))
        put(P_COEF + 2, lanes(2.0 * coef[1]))
        put(P_SSMD, lanes(ssd))
        put(P_DSKIP, lanes(dsk))
    for ref in (hb, oa, kf, kt, vu, vk, st_u, st_k, ob, mf, mi, wb, wc):
        ref[pl.ds(ref.shape[0] - 16, 8), pl.ds(0, 128)] = jnp.zeros((8, 128), ref.dtype)
    for i in range(2 * NG):
        carry[pl.ds(8 * i, 8), :] = jnp.zeros((8, 128), F32)
    kf[pl.ds(0, KF_PAD), :] = jnp.zeros((KF_PAD, 128), F32)

    def matrix_task(slot):
        def fn(gate):
            if slot != _REAL_SLOT:
                c, s = tab[pl.ds(256 + slot, 1), :], tab[pl.ds(272 + slot, 1), :]
            for a in range(8):
                if slot == _REAL_SLOT:
                    re, im = rows(tab, 128 + 16 * a), rows(tab, 128 + 16 * a + 8)
                else:
                    br, bi = rows(tab, 16 * a), rows(tab, 16 * a + 8)
                    re, im = c * br - s * bi, s * br + c * bi
                mf16[pl.ds(slot * 128 + 16 * a, 16), :] = _pack(re, im)
            m = pltpu.bitcast(rows(view(mf, z8), slot * 64, 64), BF16)
            mi[pl.ds(slot * 64, 64), :] = pltpu.bitcast(m.T, I32)
            return [after(mf), after(mi)]
        return ([48, 8], fn)

    def scale_b(p, kk):
        cr, ncr, ci = prm(p, P_COEF), prm(p, P_COEF + 1), prm(p, P_COEF + 2)
        br, bi = (braw[pl.ds(D * c + 128 * p, 128), pl.ds(128 * kk, 128)].T.astype(F32)
                  for c in range(2))
        ties = []
        for i in range(8):
            r0, r1 = br[16 * i:16 * i + 8], br[16 * i + 8:16 * i + 16]
            i0, i1 = bi[16 * i:16 * i + 8], bi[16 * i + 8:16 * i + 16]
            wb16[pl.ds((p * NG + kk) * 128 + 16 * i, 16), :] = _pack(
                cr * r0 - ci * i0, cr * r1 - ci * i1)
            wb16[pl.ds(((NG + p) * NG + kk) * 128 + 16 * i, 16), :] = _pack(
                ncr * i0 - ci * r0, ncr * i1 - ci * r1)
            if i % 2:
                ties.append(after(wb))
        return ties

    def c_task(n, k0, k1):
        def fn(gate):
            for kk in range(k0, k1):
                t = craw[pl.ds(kk * D + 128 * n, 128), :]
                wc[pl.ds((kk * NG + n) * 64, 64), :] = pltpu.bitcast(t.T, I32)
            return [after(wc)]
        return ([16], fn)

    first = bu_passes(0, 1, z8, None)
    first = [first[len(first) // NG * p:len(first) // NG * (p + 1)] for p in range(NG)]

    mats = [matrix_task(slot) for slot in range(SLOTS)]

    def scale_tasks(p):
        return [([36] * 4, lambda gate, kk=kk: scale_b(p, kk)) for kk in range(NG)]

    def dma_task(ds):
        return ([1], lambda gate: start(ds))

    def filter_tasks(g, early):
        ts = [k_tasks(g, j // 2, j % 2, z8, j >= early and CFG["kdir"]) for j in range(16)]
        return (transpose_tasks(g, z8), [q for t in ts[:early] for q in t[0]],
                [q for t in ts[:early] for q in t[1]] + [q for t in ts[early:] for q in t[0] + t[1]])

    def forward_tasks(g):
        return [t for s in range(8) for half in range(2) for t in sum(u_tasks(g, s, half, z8), [])]

    def y_block(halves, t0, z=0, lead=True, even=None):
        tiles = [(h, n) for h in halves for n in range(NG)]
        passes, plan = [], []
        for j, (h, n) in enumerate(tiles):
            sizes = (HALF,)
            if j == 0:
                if not lead:
                    continue
                sizes = (32, 96)
            if j == even:
                sizes = (64, 64)
            if j == len(tiles) - 1:
                sizes = (96, 32)
            passes += y_passes(h, n, sizes, z)
            t0 += 20
            plan.append(([skip_task(h, n)], t0 + CFG["sk0"], t0 + CFG["sk0"] + 6))
        return passes, plan

    total = 2 * NG * NG * UNIT // 64

    wait(b_dma(0))
    start(b_dma(3) + b_dma(4) + x_dma(1))
    _now(scale_tasks(0))
    wait(x_dma(0) + b_dma(1))
    start(filter0 + data0)
    _weave(first[0], [(scale_tasks(1), 0, 32)], pred)
    wait(b_dma(2))
    start(c_dma + [tab_dma])
    _weave(first[1], [(scale_tasks(2), 0, 32)], pred)
    wait(b_dma(3))
    _weave(first[2], [(scale_tasks(3), 0, 32)], pred)
    start(group_dma(0))
    wait(b_dma(4) + x_dma(1))
    _weave(first[3] + first[4] + bu_passes(1, 0, 0, True), [
        (scale_tasks(4), 0, 32), (scan_tasks(0, 1, z8), 80, 80 + total)], pred)
    wait(filter0)
    tr, _, k1 = filter_tasks(0, 0)
    nk, fwd = int(CFG["k0"] * len(k1)), forward_tasks(0)
    nu = int(CFG["u0"] * len(fwd))
    _weave(bu_passes(2, 1, 0, True), [
        (scan_tasks(1, 0, z8), 0, total), (tr, 8, 32), (k1[:nk], 36, total)], pred)
    start(group_dma(1))
    wait(data0)
    _weave(bu_passes(3, 0, 0, True), [
        (scan_tasks(2, 1, z8), 0, total), (k1[nk:], 0, total), (widen_tasks(0, z8, 16), 0, 40),
        (fwd[:nu], 40, total)], pred)
    start(group_dma(2))
    wait(c_dma + [tab_dma])
    cs = [c_task(n, k, k + 2) for n in range(NG) for k in range(0, 2 * NG, 2)]
    _now(cs[:NG])
    yp, plan = y_block((0, 1), 0, z8, even=2)
    _weave(yp, plan + [
        (cs[n * NG:(n + 1) * NG], max(20 * (n - 1) - 8, 0), 20 * n - 8) for n in range(1, NG)] + [
        (fwd[nu:-2], 0, total), (fwd[-2:], total, total), (mats, 0, total)], pred)
    start(group_dma(3) + [last_dma, oa_unit_dma(0)])

    def conv_passes():
        passes = fwd_passes(0, z8)
        for grp in range(1, 4):
            f, n = fwd_passes(grp, z8), 4 * 128 // CFG["mf"]
            a, b = (n * j for j in CFG["ord"])
            passes += f[:a] + inv_passes(grp - 1, 0, z8) + f[a:b] + inv_passes(grp - 1, 1, z8) + f[b:]
        return passes

    def inverse_tasks(g):
        tasks = []
        for half in range(2):
            for s in range(8):
                tasks += inv1_task(g, s, half, z8)
            tasks.append(dma_task([ob_dma(g, half)]))
        return tasks

    def body(i, _):
        wait(group_dma(i))
        halves = [2 + 3 * i + j for j in range(3)]
        lead = y_passes(halves[0], 0, (32, 96))
        y0 = 192 + 20 + total
        yp, plan = y_block(halves, y0, lead=False, even=7)
        passes = (conv_passes() + lead[:8] + inv_passes(3, 0, z8) + inv_passes(3, 1, z8) + lead[8:]
                  + bu_passes(i + LEAD, 0, 0, False) + yp)
        tr, k1, k2 = filter_tasks(i + 1, CFG["kconv"])
        fwd, tail, end = forward_tasks(i + 1), CFG["tail"], y0 + 280
        done = (3 * i + 2) // 2
        _weave(passes, plan + [
            ([dma_task([oa_unit_dma(done)])], y0 + 210, y0 + 210),
            (scan_tasks(i + LEAD - 1, 0, z8), *CFG["scanw"]), (tr, *CFG["tr"]),
            ([skip_task(halves[0], 0)], 232, 238),
            (widen_tasks(i + 1, z8, 16), *CFG["wid"]), (k1, *CFG["kwin"]),
            (inverse_tasks(i), *CFG["invw"]), (k2, *CFG["k2w"]),
            (fwd[:-tail], CFG["u0w"], end), (fwd[-tail:], end, end)], pred)
        pl.when(i % 2 == 1)(lambda: start([oa_unit_dma(done + 1)]))
        return 0

    lax.fori_loop(0, NG - 1, body, 0)

    wait([last_dma])
    g, last = NG - 1, L // UNIT - 1
    yp, plan = y_block((2 * last, 2 * last + 1), 192, even=2)
    ends = [[dma_task([oa_dma(last, n)])] for n in range(NG)]
    plan += [(ends[n], t + 6, t + 6) for n, (_, _, t) in enumerate(plan[NG:])]
    _weave(conv_passes() + yp[:8] + inv_passes(3, 0, z8) + inv_passes(3, 1, z8) + yp[8:], plan + [
        (scan_tasks(last, 0, z8), 0, 170),
        (inverse_tasks(g), 216, CFG["invend"])], pred)
    wait([oa_unit_dma(u) for u in range(last)] + [oa_dma(last, n) for n in range(NG)]
         + [ob_dma(n, half) for n in range(NG) for half in range(2)])


@jax.jit
def pallas_concat_heads__ssm_conv_s5__ssm_conv_h3__prompt_kernel(
    A_x: jax.Array,
    A_Lambda_re: jax.Array,
    A_Lambda_im: jax.Array,
    A_B_re: jax.Array,
    A_B_im: jax.Array,
    A_C_re: jax.Array,
    A_C_im: jax.Array,
    A_log_dt: jax.Array,
    A_Dskip: jax.Array,
    B_q: jax.Array,
    B_k: jax.Array,
    B_v: jax.Array,
    B_shift_k: jax.Array,
    B_ssm_k: jax.Array,
    B_ssm_D: jax.Array,
):
    assert A_x.shape == (1, L, D) and B_shift_k.shape == (D, 4)
    vmem = pltpu.VMEM
    dma = pltpu.SemaphoreType.DMA
    scratch = [
        vmem(_TABLES.shape, F32),
        vmem((D,), BF16), vmem((D,), BF16), vmem((D,), BF16), vmem((D,), BF16), vmem((D,), BF16),
        vmem((4, D), BF16),
        vmem((NG * L, 128), BF16),
        vmem((2 * D, D), BF16),
        vmem((2 * NG * D, 128), BF16),
        vmem((NG * L, 128), BF16),
        vmem((NG * L, 128), BF16),
        vmem((NG * L, 128), BF16),
        vmem((D, L), BF16),
        vmem((NG * P_ROWS * 8, 128), F32),
        vmem((2 * NG * D + 32, 128), BF16),
        vmem((2 * NG * NG * 64 + 16, 128), I32),
        vmem((SLOTS * 128 + 32, 128), BF16),
        vmem((SLOTS * 64 + 16, 128), I32),
        vmem((2 * 2 * NG * BU_PART, 128), F32),
        vmem((2 * NG * L + 32, 128), BF16),
        vmem((3 * NG * 8, 128), F32),
        vmem((NG * YS_ROWS, 128), F32),
        vmem((L + 16, D), F32),
        vmem((L // 2 + 16, 128), I32),
        vmem((KF_PAD + L + 16, 128), F32),
        vmem((2 * L + 16, 128), F32),
        vmem((2 * L + 16, 128), F32),
        vmem((2 * L + 8, 128), F32),
        vmem((32 * 128 + 32, 128), BF16),
        vmem((32 * 128 + 32, 128), BF16),
        vmem((8 * 128, 128), BF16),
        vmem((8 * 128, 128), BF16),
        vmem((NG * L + 16, 128), F32),
        dma((S_END,)),
    ]
    out = pl.pallas_call(
        _kernel,
        out_shape=jax.ShapeDtypeStruct((L, 2 * D), F32),
        in_specs=[pl.BlockSpec(memory_space=pl.ANY)] * 16,
        out_specs=pl.BlockSpec(memory_space=pl.ANY),
        scratch_shapes=scratch,
        compiler_params=pltpu.CompilerParams(vmem_limit_bytes=100 * 1024 * 1024, flags=CFG["flags"], disable_semaphore_checks=CFG["nosem"]),
        name="s5_h3",
    )(_TABLES, A_x.reshape(L, D), A_Lambda_re, A_Lambda_im, A_B_re, A_B_im, A_C_re, A_C_im,
      A_log_dt, A_Dskip, B_q.reshape(L, D), B_k.reshape(L, D), B_v.reshape(L, D),
      B_shift_k.T, B_ssm_k, B_ssm_D)
    return out.reshape(1, L, 2 * D)
```

```python
import math

import jax
import jax.numpy as jnp
import numpy as np
from jax import lax
from jax.experimental import pallas as pl
from jax.experimental.pallas import tpu as pltpu

F32, BF16, I32 = jnp.float32, jnp.bfloat16, jnp.int32

L = 2048
D = 640
NG = D // 128
UNIT = 256
SEG = 16
R = UNIT // SEG
LEAD = 4
HALF = UNIT // 2
BU_PART = 9 * 2 * R
YS_ROWS = SEG * (R // 2 + 1)
KF_PAD = 8


class _Signed:
    def __init__(self, v, neg=False):
        self.v, self.neg = v, neg

    def __neg__(self):
        return _Signed(self.v, not self.neg)

    def __add__(self, o):
        if self.neg == o.neg:
            return _Signed(self.v + o.v, self.neg)
        return _Signed(o.v - self.v if self.neg else self.v - o.v)

    def __sub__(self, o):
        return self + (-o)

    def __mul__(self, c):
        return _Signed(self.v * np.float32(-c if self.neg else c))

    def get(self):
        return -self.v if self.neg else self.v


def _rot(re, im, num, den):
    num %= den
    h = math.sqrt(0.5)
    if num == 0:
        return re, im
    if 4 * num == den:
        return -im, re
    if 4 * num == 3 * den:
        return im, -re
    if 8 * num == den:
        return (re - im) * h, (re + im) * h
    if 8 * num == 3 * den:
        return (re + im) * (-h), (re - im) * h
    if 8 * num == 5 * den:
        return (im - re) * h, (re + im) * (-h)
    if 8 * num == 7 * den:
        return (re + im) * h, (im - re) * h
    c = math.cos(2 * math.pi * num / den)
    s = math.sin(2 * math.pi * num / den)
    return re * c - im * s, re * s + im * c


def _dft4(z, sign):
    (r0, i0), (r1, i1), (r2, i2), (r3, i3) = z
    ar, ai, br, bi = r0 + r2, i0 + i2, r0 - r2, i0 - i2
    cr, ci, dr, di = r1 + r3, i1 + i3, r1 - r3, i1 - i3
    plus, minus = (br - di, bi + dr), (br + di, bi - dr)
    if sign < 0:
        plus, minus = minus, plus
    return [(ar + cr, ai + ci), plus, (ar - cr, ai - ci), minus]


def _fwd1(n, u):
    a0, a1, b0, b1 = u
    p, q = _rot(a0, b0, n, 32), _rot(a1, b1, n + 4, 32)
    s0, s1 = a0 + b0, a1 + b1
    return [(p[0] + q[0], p[1] + q[1]), _rot(p[0] - q[0], p[1] - q[1], n, 8),
            _rot(a0 - b0, a1 - b1, n, 16), (s0 + s1, s0 - s1)]


def _fwd2(grp, z):
    if grp < 3:
        return _dft4(z, 1)
    s4 = [t[0] for t in z]
    d4 = [t[1] for t in z]
    p = (d4[0], d4[2])
    q = _rot(d4[1], d4[3], 1, 8)
    s5 = [s4[0] + s4[2], s4[1] + s4[3]]
    return [
        (s5[0] + s5[1], s5[0] - s5[1]),
        (s4[0] - s4[2], s4[1] - s4[3]),
        (p[0] + q[0], p[1] + q[1]),
        (p[0] - q[0], p[1] - q[1]),
    ]


def _inv2(grp, w):
    if grp < 3:
        return _dft4(w, -1)
    s5 = [w[0][0] + w[0][1], w[0][0] - w[0][1]]
    s4 = [s5[0] + w[1][0], s5[1] + w[1][1], s5[0] - w[1][0], s5[1] - w[1][1]]
    p = (w[2][0] + w[3][0], w[2][1] + w[3][1])
    q = _rot(w[2][0] - w[3][0], w[2][1] - w[3][1], -1, 8)
    d4 = [p[0], q[0], p[1], q[1]]
    return [(s4[n], d4[n]) for n in range(4)]


def _inv1(n, z):
    e = _rot(*z[1], -n, 8)
    p = _rot(z[0][0] + e[0], z[0][1] + e[1], -n, 32)
    q = _rot(z[0][0] - e[0], z[0][1] - e[1], -(n + 4), 32)
    d0, d1 = _rot(*z[2], -n, 16)
    s0, s1 = z[3][0] + z[3][1], z[3][0] - z[3][1]
    return [p[0] + (s0 + d0), q[0] + (s1 + d1), p[1] + (s0 - d0), q[1] + (s1 - d1)]


_F1 = [4 * (g + 2 * k) + 1 for g in range(2) for k in range(4)]
_F1 += [2 * (4 * k + 1) for k in range(4)] + [0, 8, 4, 20]
_REAL_SLOT = 12
SLOTS = len(_F1)


def _dft_tables():
    kap = np.arange(128)
    j = 8 * (kap // 16) + kap % 8
    part = (kap // 8) % 2
    pr, pc, jr, jc = part[:, None], part[None, :], j[:, None], j[None, :]
    lo = 2 * np.pi * jr * jc / 64
    base = np.where(pr == pc, np.cos(lo), np.where(pr == 0, -np.sin(lo), np.sin(lo)))
    hi = 2 * np.pi * (16 + 32 * (jr - 32)) * jc / 2048
    v0 = np.where(pr == 0, np.cos(lo), np.where(jr == 0, np.cos(np.pi * jc), np.sin(lo)))
    v32 = np.where(pr == 0, np.cos(hi), np.sin(hi))
    real = np.where(jr < 32, np.where(pc == 0, v0, 0.0), np.where(pc == 1, v32, 0.0))
    th = 2 * np.pi * np.outer(np.array(_F1), j) / 2048
    zeros = np.zeros((8, 128))
    return np.concatenate([base, real, np.cos(th), np.sin(th), zeros]).astype(np.float32)


_TABLES = _dft_tables()
_FFT_SCALE = 2.0 ** -10

(P_MU, P_RHO, P_RHO1, P_RHO2, P_RHO4, P_TAP, P_SSMD, P_DSKIP, P_COEF, P_ROWS) = (
    0, 2, 4, 6, 8, 10, 14, 15, 16, 20)
S_SMALL, S_F0, S_K0, S_C, S_OUT, S_X0, S_B = range(7)
S_COL = S_B + NG
S_END = S_COL + NG - 1


def _cmul(a, b):
    return a[0] * b[0] - a[1] * b[1], a[0] * b[1] + a[1] * b[0]


def _pack(lo, hi):
    return jnp.concatenate([lo, hi], axis=0).astype(BF16)


def _unpack(w):
    v = pltpu.bitcast(w, BF16).astype(F32)
    return v[:8], v[8:]


CFG = dict(scan=22, u=24, k1=0, p2=0, inv=36, skip=30, tail=4, kconv=4, steps=2, p2n=2,
           u0w=350, kwin=(100, 216), tr=(60, 90), wid=(216, 330), scanw=(0, 350), invw=(220, 420),
           k2w=(230, 480), mf=128, mi=128, ord=(3, 4), sk0=12, when=(0, 1, 1, 2, 3, 4, 6), s2=380, retap=False, invend=290,
           Q=1, invsplit=False, kg=1, k0=1.0, u0=0.45, udir=True, kdir=True,
           flags=None, nosem=False, skipme=lambda n, rows: False)


class _Zeros:
    def __init__(self, v):
        self.v = v


class _Gate:
    def __init__(self, pred=None, seen=()):
        self.pred, self.seen = pred, seen

    def early(self, lag):
        old = [e for e in self.seen if e[0] <= -lag]
        return max(old, key=lambda e: e[0])[1] if lag and old else None

    def value(self, v, lag):
        early = self.early(lag)
        return v if early is None else jnp.where(self.pred, v, early)

    def loads(self, ref, lag):
        early = self.early(lag)
        if early is not None:
            ref[pl.ds(ref.shape[0] - 8, 8), :] = (
                early if ref.dtype == F32 else pltpu.bitcast(early, I32))


def _weave(passes, plan, pred):
    if CFG["skipme"](len(passes), sum(q[0] for q in passes)):
        return
    begin, clock = [], [0] * 4
    for i, (n, *_) in enumerate(passes):
        begin.append(clock[i % 4] / 16)
        clock[i % 4] += n

    def index(t):
        later = [i for i, b in enumerate(begin) if b >= t - 3.999]
        if not later:
            return len(passes)
        same = [i for i in later if begin[i] == min(begin[j] for j in later)]
        return same[min(max(int((t - begin[same[0]]) / 4 * len(same)), 0), len(same) - 1)]

    at = [[] for _ in range(len(passes) + 1)]
    for tasks, lo, hi in plan:
        total, done = sum(sum(c) for c, _ in tasks) or 1, 0.0
        for costs, fn in tasks:
            where = []
            for cost in costs:
                done += cost
                where.append(index(lo + done / total * (hi - lo)))
            at[min(where)].append((fn, where))
    seen, ties = [], [[] for _ in at]
    for i, fns in enumerate(at):
        now = (begin[i] + i % 4) if i < len(begin) else clock[0] / 16
        early = [(t - now, v) for t, v in seen if t % CFG["Q"] < 1 or CFG["Q"] == 1]
        for fn, where in fns:
            for w, tie in zip(where, fn(_Gate(pred, early)) or ()):
                ties[w].append(tie)
        if i == len(passes):
            break
        n, lhs, rhs, consume = passes[i]
        w = rhs()
        for tie in ties[i]:
            if isinstance(tie, _Zeros):
                v = tie.v
                w[-1] = w[-1] | (v if v.dtype == I32 else pltpu.bitcast(v, I32))
            else:
                w[-1] = jnp.where(pred, w[-1], pltpu.bitcast(tie, I32))
        d = jnp.dot(pltpu.bitcast(jnp.concatenate(lhs(), axis=0), BF16),
                    pltpu.bitcast(jnp.concatenate(w, axis=0), BF16), preferred_element_type=F32)
        seen += [(begin[i] + i % 4 + j // 16 - 4, d[j - 8:j]) for j in range(64, n + 1, 64)]
        consume(d)


def _now(tasks):
    for _, fn in tasks:
        fn(_Gate())


def _kernel(tab_hbm, x_hbm, lre_hbm, lim_hbm, bre_hbm, bim_hbm, cre_hbm, cim_hbm,
            ldt_hbm, dsk_hbm, q_hbm, k_hbm, v_hbm, tap_hbm, sk_hbm, sd_hbm,
            o_hbm,
            tab, lre_v, lim_v, ldt_v, dsk_v, sd_v, tap_v,
            xb, braw, craw, qb, kb, vb, skb,
            par, wb16, wc, mf16, mi, bu, hb16, carry, ys, oa,
            kt, kf, st_u, st_k, st_i, vu16, vk16, pb0, pb1, ob,
            sem):
    x32, q32, k32, v32, wb, mf, hb, vu, vk = (
        r.bitcast(I32) for r in (xb, qb, kb, vb, wb16, mf16, hb16, vu16, vk16))
    pb16 = (pb0, pb1)
    pb = (pb0.bitcast(I32), pb1.bitcast(I32))

    def rows(ref, start, n=8):
        return ref[pl.ds(start, n), :]

    def hint(v, n):
        return v if isinstance(v, int) or n == 1 else pl.multiple_of(v, n)

    def view(ref, start, n=None):
        return ref.at[pl.ds(hint(start, 16), n or ref.shape[0]), :]

    def after(ref):
        return _Zeros(view(ref, z8)[ref.shape[0] - 16:ref.shape[0] - 8, 0:128])

    small = [pltpu.make_async_copy(s, d, sem.at[S_SMALL]) for s, d in (
        (lre_hbm, lre_v), (lim_hbm, lim_v), (ldt_hbm, ldt_v),
        (dsk_hbm, dsk_v), (sd_hbm, sd_v), (tap_hbm, tap_v),
        (tab_hbm.at[pl.ds(288, 8), :], tab.at[pl.ds(288, 8), :]))]
    tab_dma = pltpu.make_async_copy(
        tab_hbm.at[pl.ds(0, 288), :], tab.at[pl.ds(0, 288), :], sem.at[S_B + 4])

    def x_dma(u):
        return [pltpu.make_async_copy(
            x_hbm.at[pl.ds(hint(u * UNIT, UNIT), UNIT), pl.ds(128 * n, 128)],
            xb.at[pl.ds(hint(n * L + u * UNIT, UNIT), UNIT), :], sem.at[(S_X0, S_B + 4, S_F0, S_K0)[u] if isinstance(u, int) and u < LEAD
                                                     else S_COL + u - LEAD])
            for n in range(NG)]

    def b_dma(p):
        return [pltpu.make_async_copy(
            src.at[pl.ds(128 * p, 128), :], braw.at[pl.ds(D * c + 128 * p, 128), :],
            sem.at[S_B + p]) for c, src in enumerate((bre_hbm, bim_hbm))]

    c_dma = [pltpu.make_async_copy(
        src.at[:, pl.ds(128 * p, 128)], craw.at[pl.ds(D * (NG * c + p), D), :],
        sem.at[S_C]) for c, src in enumerate((cre_hbm, cim_hbm)) for p in range(NG)]

    def col_dma(which, g, sem_at):
        src, dst = ((k_hbm, kb), (v_hbm, vb), (q_hbm, qb))[which]
        return pltpu.make_async_copy(
            src.at[:, pl.ds(hint(128 * g, 128), 128)],
            dst.at[pl.ds(hint(L * g, L), L), :], sem.at[sem_at])

    def sk_dma(g, sem_at):
        t = hint(128 * g, 128)
        return [pltpu.make_async_copy(
            sk_hbm.at[pl.ds(t, 128), :], skb.at[pl.ds(t, 128), :], sem.at[sem_at])]

    def oa_dma(u, n):
        t = hint(u * UNIT, UNIT)
        return pltpu.make_async_copy(
            oa.at[pl.ds(t, UNIT), pl.ds(128 * n, 128)],
            o_hbm.at[pl.ds(t, UNIT), pl.ds(128 * n, 128)], sem.at[S_OUT])

    def oa_unit_dma(u):
        t = hint(u * UNIT, UNIT)
        return pltpu.make_async_copy(
            oa.at[pl.ds(t, UNIT), :], o_hbm.at[pl.ds(t, UNIT), pl.ds(0, D)], sem.at[S_OUT])

    def ob_dma(g, half):
        h = L // 2
        return pltpu.make_async_copy(
            ob.at[pl.ds(hint(L * g + h * half, h), h), :],
            o_hbm.at[pl.ds(h * half, h), pl.ds(hint(D + 128 * g, 128), 128)], sem.at[S_OUT])

    def start(ds):
        for d in ds:
            d.start()

    def wait(ds):
        for d in ds:
            d.wait()

    def prm(g, row):
        return rows(view(par, g * (P_ROWS * 8), P_ROWS * 8), row * 8)

    def bu_passes(u, slot, z, shift):
        out = []
        xu, w = view(x32, u * (UNIT // 2), ((NG - 1) * L + UNIT) // 2), view(wb, z)
        order = [p + c * NG for p in range(NG) for c in range(2)]
        for n in order:
            sizes = [128, 128]
            if shift and n == order[0]:
                sizes = [32, 32, 96, 96]
            if shift and n == order[-1]:
                sizes = [96, 96, 32, 32]
            if shift is None:
                sizes = [64] * 4
            for m, MM in zip(np.cumsum([0] + sizes).tolist(), sizes):
                acc = []
                for kk in range(NG):
                    def lhs(m=m, kk=kk, MM=MM):
                        t = (kk * L + m) // 2
                        return [rows(xu, t + 8 * i) for i in range(MM // 16)]

                    def rhs(n=n, kk=kk):
                        return [rows(w, (n * NG + kk) * 64 + 8 * i) for i in range(8)]

                    def consume(d, m=m, n=n, kk=kk, acc=acc, MM=MM):
                        acc.append(d if kk == 0 else acc[-1] + d)
                        if kk == NG - 1:
                            for i in range(MM // 8):
                                seg, r = divmod(m + 8 * i, R)
                                row = 9 * (seg % 2 * R + r) + seg // 2
                                bu[pl.ds((slot * 2 * NG + n) * BU_PART + row, 8, stride=9), :] = (
                                    acc[-1][8 * i:8 * i + 8])
                    out.append((MM, lhs, rhs, consume))
        return out

    def scan_tasks(u, slot, z):
        steps = CFG["steps"]
        state = {}
        hu = view(hb16, u * UNIT, (2 * NG - 1) * L + UNIT)

        def b(p, ch, r):
            return tuple(rows(bu, (slot * 2 * NG + c * NG + p) * BU_PART + 9 * (ch * R + r))
                         for c in range(2))

        def step(mu, h, br):
            return (mu[0] * h[0] + br[0]) - mu[1] * h[1], (mu[0] * h[1] + br[1]) + mu[1] * h[0]

        def ends(p, gate):
            mu, ties = (gate.value(prm(p, P_MU), CFG["scan"]), prm(p, P_MU + 1)), []
            h = [b(p, ch, 0) for ch in range(2)]
            for r in range(1, R):
                h = [step(mu, h[ch], b(p, ch, r)) for ch in range(2)]
                if r % steps == 0:
                    ties.append(h[r // steps % 2][0])
            state[p] = starts(p, h)
            return ties + [state[p][1][0]]

        def starts(p, e):
            last = lax.broadcasted_iota(I32, (8, 128), 0) == 7
            rho = (prm(p, P_RHO), prm(p, P_RHO + 1))
            pair = step(rho, e[0], e[1])
            a = tuple(pltpu.roll(jnp.where(last, rows(carry, (2 * p + c) * 8), pair[c]), 1, 0)
                      for c in range(2))
            for sh, row in ((1, P_RHO1), (2, P_RHO2), (4, P_RHO4)):
                a = step((prm(p, row), prm(p, row + 1)), tuple(pltpu.roll(c, sh, 0) for c in a), a)
            return [a, step(rho, a, e[0])]

        def run(p, r0, gate):
            if r0 == 0:
                state["mu"] = (prm(p, P_MU), prm(p, P_MU + 1))
            mu, h = (gate.value(state["mu"][0], CFG["scan"]), state["mu"][1]), state[p]
            for r in range(r0, r0 + steps):
                h = [step(mu, h[ch], b(p, ch, r)) for ch in range(2)]
                for c in range(2):
                    hu[pl.ds((c * NG + p) * L + 16 * r, 16), :] = _pack(h[0][c], h[1][c])
            state[p] = h
            if r0 + steps == R:
                for c in range(2):
                    carry[pl.ds((2 * p + c) * 8, 8), :] = h[1][c]
            return [after(hb)]

        tasks = []
        for p in range(NG):
            tasks.append(([16 * steps] * ((R - 1) // steps) + [46 + 16 * steps],
                          lambda gate, p=p: ends(p, gate)))
            tasks += [([18 * steps], lambda gate, p=p, r0=r0: run(p, r0, gate))
                      for r0 in range(0, R, steps)]
        return tasks

    def y_passes(h, n, sizes=(HALF,), z=0):
        out, w, hu = [], view(wc, z), view(hb, h * (HALF // 2), ((2 * NG - 1) * L + HALF) // 2)
        for t0, MM in zip(np.cumsum((0,) + sizes).tolist(), sizes):
            acc = []
            for kk in range(2 * NG):
                def lhs(t0=t0, kk=kk, MM=MM):
                    return [rows(hu, (kk * L + t0) // 2 + 8 * i) for i in range(MM // 16)]

                def rhs(kk=kk):
                    return [rows(w, (kk * NG + n) * 64 + 8 * i) for i in range(8)]

                def consume(d, t0=t0, kk=kk, acc=acc, MM=MM):
                    acc.append(d if kk == 0 else acc[-1] + d)
                    if kk == 2 * NG - 1:
                        for i in range(MM // 8):
                            r, ch = divmod(t0 // 8 + i, 2)
                            ys[pl.ds(n * YS_ROWS + ch * (R // 2 + 1) + r, 8, stride=R + 2), :] = (
                                acc[-1][8 * i:8 * i + 8])
                out.append((MM, lhs, rhs, consume))
        return out

    def skip_task(h, n):
        def fn(gate):
            dsk, ties = gate.value(prm(n, P_DSKIP), CFG["skip"]), []
            t = h // 2 * UNIT + h % 2 * (R // 2)
            xu = x32.at[pl.ds(hint(t // 2 + n * (L // 2), 4), UNIT // 2 - 4 + 8 * (n < NG - 1 or not isinstance(h, int))), :]
            ou = oa.at[pl.ds(hint(t, 8), UNIT - R // 2), :]
            for g in range(SEG):
                if g == SEG - 1 and n == NG - 1 and isinstance(h, int):
                    xs = _unpack(rows(xu, 8 * g - 4))[1]
                else:
                    xs = _unpack(rows(xu, 8 * g))[0]
                y = rows(ys, n * YS_ROWS + g * (R // 2 + 1))
                ou[pl.ds(R * g, 8), pl.ds(128 * n, 128)] = y + xs * dsk
                if g % 8 == 7:
                    ties.append(after(oa))
            return ties
        return ([24, 24], fn)

    def widen_tasks(g, z, pieces=2):
        def fn(i0, i1):
            kg = view(k32, g * (L // 2), L // 2)
            for i in range(i0, i1):
                lo, hi = _unpack(rows(kg, 8 * i))
                kf[pl.ds(KF_PAD + 16 * i, 8), :] = lo
                kf[pl.ds(KF_PAD + 16 * i + 8, 8), :] = hi
            return [after(kf)]
        n = L // 16 // pieces
        return [([2 * n], lambda gate, i=i: fn(i * n, (i + 1) * n)) for i in range(pieces)]

    def transpose_tasks(g, z, pieces=8):
        def fn(c0, c1):
            for c in range(c0, c1):
                t = skb[pl.ds(hint(128 * g, 128), 128), pl.ds(128 * c, 128)]
                kt[pl.ds(64 * c, 64), :] = pltpu.bitcast(t.T, I32)
            return [after(kt)]
        n = L // 128 // pieces
        return [([8 * n], lambda gate, i=i: fn(i * n, (i + 1) * n)) for i in range(pieces)]

    def staged(s, half, n, grp, c):
        return (((s * 2 + half) * 4 + n) * 4 + grp) * 16 + 8 * c

    ops1 = (18, 36, 30, 36)

    def forward_tasks_of(st, s, half, z, chunk, chunk_cost, direct):
        dst16, dst = (vu16, vu) if st is st_u else (vk16, vk)

        def second(grp, zs):
            for k, pair in enumerate(_fwd2(grp, zs)):
                dst16[pl.ds(((4 * grp + k) * 2 + half) * 128 + 16 * s, 16), :] = (
                    _pack(pair[0].get(), pair[1].get()))
            return after(dst)

        kept = []

        def first(gate, n):
            load = chunk(gate, n)
            u = [load(16 * half + n + 4 * m) for m in range(4)]
            pairs = _fwd1(n, [_Signed(v) for v in u])
            kept.append(pairs)
            for grp in range(2 * direct, 4):
                for c in range(2):
                    st[pl.ds(staged(s, half, n, grp, c), 8), :] = pairs[grp][c].get()
            return [u[0] + u[2]] * (chunk_cost > 4) + [after(st)]

        def rest(grp):
            if direct and grp < 2:
                return [second(grp, [t[grp] for t in kept])]
            return [second(grp, [tuple(_Signed(rows(view(st, z), staged(s, half, n, grp, c)))
                                       for c in range(2)) for n in range(4)])]

        split = (chunk_cost > 4) * (chunk_cost // 2 + 1)
        one = [([split] * (split > 0) + [chunk_cost + ops1[n] - split], lambda gate, n=n: first(gate, n))
               for n in range(4)]
        if CFG["p2n"] == 4:
            two = [([20], lambda gate, grp=grp: rest(grp)) for grp in range(4)]
        else:
            two = [([40], lambda gate, grp=grp: rest(grp) and rest(grp + 1)) for grp in (0, 2)]
        h = len(two) // 2
        return (one + two[:h], two[h:]) if direct else (one, two)

    def u_tasks(g, s, half, z):
        loaded = []

        def chunk(gate, n):
            if n == 0 or CFG["retap"]:
                loaded[:] = [prm(g, P_TAP + t) for t in range(4)]
            taps = [gate.value(loaded[0], CFG["u"])] + loaded[1:]
            kz, vg = view(kf, z), view(v32, g * (L // 2), L // 2)

            def load(c):
                t = 64 * c + 8 * s
                ks = rows(kz, KF_PAD + t) * taps[0]
                for lag in range(1, 4):
                    ks = ks + rows(kz, KF_PAD + t - lag) * taps[lag]
                return ks * _unpack(rows(vg, (t // 16) * 8))[s % 2]
            return load
        return forward_tasks_of(st_u, s, half, z, chunk, 36, CFG["udir"])

    def k_tasks(g, s, half, z, direct):
        def chunk(gate, n):
            if n % CFG["kg"] == 0:
                gate.loads(kt, CFG["k1"])

            def load(c):
                v = _unpack(rows(view(kt, z), 32 * c + 8 * (s // 2)))[s % 2]
                if s == 0 and c == 0:
                    first = lax.broadcasted_iota(I32, (8, 128), 0) == 0
                    v = v + jnp.where(first, prm(g, P_SSMD), 0.0)
                return v
            return load
        return forward_tasks_of(st_k, s, half, z, chunk, 4, direct)

    def fwd_passes(grp, z):
        out, MM = [], CFG["mf"]
        for slot in range(4 * grp, 4 * grp + 4):
            for part in range(128 // MM):
                got = []
                for src, half in ((vu, 0), (vk, 0), (vu, 1), (vk, 1)):
                    def lhs(slot=slot, part=part):
                        return [rows(mf, slot * 64 + MM // 2 * part + 8 * i) for i in range(MM // 16)]

                    def rhs(slot=slot, src=src, half=half):
                        return [rows(view(src, z), (2 * slot + half) * 64 + 8 * i) for i in range(8)]

                    def consume(d, slot=slot, part=part, got=got):
                        got.append(d)
                        if len(got) < 4:
                            return
                        for i in range(MM // 16):
                            u0, k0, u1, k1 = ((t[16 * i:16 * i + 8], t[16 * i + 8:16 * i + 16]) for t in got)
                            lo, a, b = _cmul(u0, k0), _cmul(u0, k1), _cmul(u1, k0)
                            if slot == _REAL_SLOT and part == 0 and i == 0:
                                first = lax.broadcasted_iota(I32, (8, 128), 0) == 0
                                lo, a, b = (tuple(jnp.where(first, 0.5 * (x[c] * y[c]), p[c]) for c in range(2))
                                            for p, x, y in ((lo, u0, k0), (a, u0, k1), (b, u1, k0)))
                            if _F1[slot] % 2:
                                hi = ((a[0] + b[0]) - lo[0], (a[1] + b[1]) - lo[1])
                            else:
                                hi = ((a[0] + b[0]) + lo[0], (a[1] + b[1]) + lo[1])
                            for half, p in enumerate((lo, hi)):
                                at = (slot % 4 * 2 + half) * 128 + MM * part + 16 * i
                                pb16[grp % 2][pl.ds(at, 16), :] = _pack(*p)
                    out.append((MM, lhs, rhs, consume))
        return out

    def inv_passes(grp, half, z):
        out, MM = [], CFG["mi"]
        for part in range(128 // MM):
            got = []
            for slot in range(4 * grp, 4 * grp + 4):
                def lhs(slot=slot, part=part):
                    return [rows(mi, slot * 64 + MM // 2 * part + 8 * i) for i in range(MM // 16)]

                def rhs(slot=slot):
                    return [rows(view(pb[grp % 2], z), (slot % 4 * 2 + half) * 64 + 8 * i)
                            for i in range(8)]

                def consume(d, part=part, got=got):
                    got.append(d)
                    if len(got) < 4:
                        return
                    for i in range(MM // 16):
                        w = [(_Signed(t[16 * i:16 * i + 8]), _Signed(t[16 * i + 8:16 * i + 16]))
                             for t in got]
                        for n, pair in enumerate(_inv2(grp, w)):
                            for c in range(2):
                                at = staged(MM // 16 * part + i, half, n, grp, c)
                                st_i[pl.ds(at, 8), :] = pair[c].get()
                out.append((MM, lhs, rhs, consume))
        return out

    def inv1_task(g, s, half, z):
        def fn(gate, ns):
            gate.loads(st_i, CFG["inv"])
            qg, og, ties = view(q32, g * (L // 2), L // 2), view(ob, g * L, L), []
            for n in ns:
                zs = [tuple(_Signed(rows(view(st_i, z), staged(s, half, n, grp, c))) for c in range(2))
                      for grp in range(4)]
                for m, y in enumerate(_inv1(n, zs)):
                    t = 64 * (16 * half + n + 4 * m) + 8 * s
                    og[pl.ds(t, 8), :] = _unpack(rows(qg, (t // 16) * 8))[s % 2] * y.get()
                ties.append(after(ob))
            return ties
        if CFG["invsplit"]:
            return [([12 + ops1[n]], lambda gate, n=n: fn(gate, [n])) for n in range(4)]
        return [([12 + n for n in ops1], lambda gate: fn(gate, range(4)))]

    filter0 = x_dma(2) + sk_dma(0, S_F0)
    data0 = x_dma(3) + [col_dma(0, 0, S_K0), col_dma(1, 0, S_K0)]

    def group_dma(g):
        at = S_COL + g
        return ([col_dma(2, g, at)] + sk_dma(g + 1, at)
                + [col_dma(0, g + 1, at), col_dma(1, g + 1, at)] + x_dma(g + LEAD))

    last_dma = col_dma(2, NG - 1, S_SMALL)

    start(small + b_dma(0) + x_dma(0) + b_dma(1) + b_dma(2))
    wait(small)
    zeros = rows(tab, 288).astype(I32)
    z8 = pl.multiple_of(zeros[0, 0], 16)
    sub = lax.broadcasted_iota(I32, (8, 128), 0)
    pred = zeros == 0

    def stack(ref):
        v = ref[...].astype(F32).reshape(1, D)
        return jnp.concatenate([v[:, 128 * g:128 * (g + 1)] for g in range(NG)]
                               + [v[:, :128]] * (8 - NG), axis=0)

    lre, lim = stack(lre_v), stack(lim_v)
    dt = jnp.exp(stack(ldt_v)).astype(BF16).astype(F32)
    mag, ang = jnp.exp(dt * lre), dt * lim
    lam = (mag * jnp.cos(ang), mag * jnp.sin(ang))
    scale = jnp.maximum(jnp.abs(lre), jnp.abs(lim))
    nre, nim = lre / scale, lim / scale
    den = (nre * nre + nim * nim) * scale
    coef = _cmul(((lam[0] - 1.0) / den, lam[1] / den), (nre, -nim))
    mu = (lam[0], -lam[1])
    rho = [mu]
    for _ in range(R.bit_length() + 2):
        rho.append(_cmul(rho[-1], rho[-1]))
    dsk, ssd = stack(dsk_v), stack(sd_v)
    taps = tap_v[...].astype(F32) * _FFT_SCALE
    for g in range(NG):
        def put(row, v):
            par[pl.ds((g * P_ROWS + row) * 8, 8), :] = v

        def lanes(v):
            return jnp.broadcast_to(v[g:g + 1], (8, 128))
        for c in range(2):
            put(P_MU + c, lanes(mu[c]))
            put(P_RHO + c, lanes(rho[-4][c]))
            for n, row in enumerate((P_RHO1, P_RHO2, P_RHO4)):
                put(row + c, jnp.where(sub >= 1 << n, lanes(rho[n - 3][c]), 0.0))
        for t in range(4):
            put(P_TAP + t, jnp.broadcast_to(taps[t:t + 1, 128 * g:128 * (g + 1)], (8, 128)))
        put(P_COEF, lanes(2.0 * coef[0]))
        put(P_COEF + 1, lanes(-2.0 * coef[0]))
        put(P_COEF + 2, lanes(2.0 * coef[1]))
        put(P_SSMD, lanes(ssd))
        put(P_DSKIP, lanes(dsk))
    for ref in (hb, oa, kf, kt, vu, vk, st_u, st_k, ob, mf, mi, wb, wc):
        ref[pl.ds(ref.shape[0] - 16, 8), pl.ds(0, 128)] = jnp.zeros((8, 128), ref.dtype)
    for i in range(2 * NG):
        carry[pl.ds(8 * i, 8), :] = jnp.zeros((8, 128), F32)
    kf[pl.ds(0, KF_PAD), :] = jnp.zeros((KF_PAD, 128), F32)

    def matrix_task(slot):
        def fn(gate):
            if slot != _REAL_SLOT:
                c, s = tab[pl.ds(256 + slot, 1), :], tab[pl.ds(272 + slot, 1), :]
            for a in range(8):
                if slot == _REAL_SLOT:
                    re, im = rows(tab, 128 + 16 * a), rows(tab, 128 + 16 * a + 8)
                else:
                    br, bi = rows(tab, 16 * a), rows(tab, 16 * a + 8)
                    re, im = c * br - s * bi, s * br + c * bi
                mf16[pl.ds(slot * 128 + 16 * a, 16), :] = _pack(re, im)
            m = pltpu.bitcast(rows(view(mf, z8), slot * 64, 64), BF16)
            mi[pl.ds(slot * 64, 64), :] = pltpu.bitcast(m.T, I32)
            return [after(mf), after(mi)]
        return ([48, 8], fn)

    def scale_b(p, kk):
        cr, ncr, ci = prm(p, P_COEF), prm(p, P_COEF + 1), prm(p, P_COEF + 2)
        br, bi = (braw[pl.ds(D * c + 128 * p, 128), pl.ds(128 * kk, 128)].T.astype(F32)
                  for c in range(2))
        ties = []
        for i in range(8):
            r0, r1 = br[16 * i:16 * i + 8], br[16 * i + 8:16 * i + 16]
            i0, i1 = bi[16 * i:16 * i + 8], bi[16 * i + 8:16 * i + 16]
            wb16[pl.ds((p * NG + kk) * 128 + 16 * i, 16), :] = _pack(
                cr * r0 - ci * i0, cr * r1 - ci * i1)
            wb16[pl.ds(((NG + p) * NG + kk) * 128 + 16 * i, 16), :] = _pack(
                ncr * i0 - ci * r0, ncr * i1 - ci * r1)
            if i % 2:
                ties.append(after(wb))
        return ties

    def c_task(n, k0, k1):
        def fn(gate):
            for kk in range(k0, k1):
                t = craw[pl.ds(kk * D + 128 * n, 128), :]
                wc[pl.ds((kk * NG + n) * 64, 64), :] = pltpu.bitcast(t.T, I32)
            return [after(wc)]
        return ([16], fn)

    first = bu_passes(0, 1, z8, None)
    first = [first[len(first) // NG * p:len(first) // NG * (p + 1)] for p in range(NG)]

    mats = [matrix_task(slot) for slot in range(SLOTS)]

    def scale_tasks(p):
        return [([36] * 4, lambda gate, kk=kk: scale_b(p, kk)) for kk in range(NG)]

    def dma_task(ds):
        return ([1], lambda gate: start(ds))

    def filter_tasks(g, early):
        ts = [k_tasks(g, j // 2, j % 2, z8, j >= early and CFG["kdir"]) for j in range(16)]
        return (transpose_tasks(g, z8), [q for t in ts[:early] for q in t[0]],
                [q for t in ts[:early] for q in t[1]] + [q for t in ts[early:] for q in t[0] + t[1]])

    def forward_tasks(g):
        return [t for s in range(8) for half in range(2) for t in sum(u_tasks(g, s, half, z8), [])]

    def y_block(halves, t0, z=0, lead=True, even=None):
        tiles = [(h, n) for h in halves for n in range(NG)]
        passes, plan = [], []
        for j, (h, n) in enumerate(tiles):
            sizes = (HALF,)
            if j == 0:
                if not lead:
                    continue
                sizes = (32, 96)
            if j == even:
                sizes = (64, 64)
            if j == len(tiles) - 1:
                sizes = (96, 32)
            passes += y_passes(h, n, sizes, z)
            t0 += 20
            plan.append(([skip_task(h, n)], t0 + CFG["sk0"], t0 + CFG["sk0"] + 6))
        return passes, plan

    total = 2 * NG * NG * UNIT // 64

    def early(at):
        for when, ds in zip(CFG["when"], (filter0, data0, c_dma, group_dma(0), group_dma(1), group_dma(2),
                                          group_dma(3) + [last_dma])):
            if when == at:
                start(ds)

    wait(b_dma(0))
    start(b_dma(3) + b_dma(4) + x_dma(1) + [tab_dma])
    _now(scale_tasks(0))
    wait(x_dma(0))
    _weave(first[0], [], pred)
    early(0)
    wait(b_dma(1))
    _now(scale_tasks(1))
    _weave(first[1], [], pred)
    early(1)
    wait(b_dma(2) + b_dma(3))
    _now(scale_tasks(2))
    _weave(first[2] + first[3], [(scale_tasks(3), 0, 32)], pred)
    early(2)
    wait(b_dma(4) + x_dma(1) + [tab_dma])
    _now(scale_tasks(4))
    _weave(first[4] + bu_passes(1, 0, 0, True), [
        (scan_tasks(0, 1, z8), 40, 40 + total), (mats, 0, 160)], pred)
    early(3)
    wait(filter0)
    tr, _, k1 = filter_tasks(0, 0)
    nk, fwd = int(CFG["k0"] * len(k1)), forward_tasks(0)
    nu = int(CFG["u0"] * len(fwd))
    _weave(bu_passes(2, 1, 0, True), [
        (scan_tasks(1, 0, z8), 0, total), (tr, 8, 32), (k1[:nk], 36, total)], pred)
    early(4)
    wait(data0 + c_dma)
    cs = [c_task(n, k, k + 2) for n in range(NG) for k in range(0, 2 * NG, 2)]
    yp, plan = y_block((0, 1), total, z8, even=2)
    _weave(bu_passes(3, 0, 0, True) + yp, plan + [
        (scan_tasks(2, 1, z8), 0, CFG["s2"]), (k1[nk:], 0, total), (widen_tasks(0, z8, 16), 0, 40),
        (cs, 0, total - 16), (fwd[:-2], 40, 2 * total), (fwd[-2:], 2 * total, 2 * total)], pred)
    start([oa_unit_dma(0)])
    early(6)

    def conv_passes():
        passes = fwd_passes(0, z8)
        for grp in range(1, 4):
            f, n = fwd_passes(grp, z8), 4 * 128 // CFG["mf"]
            a, b = (n * j for j in CFG["ord"])
            passes += f[:a] + inv_passes(grp - 1, 0, z8) + f[a:b] + inv_passes(grp - 1, 1, z8) + f[b:]
        return passes

    def inverse_tasks(g):
        tasks = []
        for half in range(2):
            for s in range(8):
                tasks += inv1_task(g, s, half, z8)
            tasks.append(dma_task([ob_dma(g, half)]))
        return tasks

    def body(i, _):
        wait(group_dma(i))
        halves = [2 + 3 * i + j for j in range(3)]
        lead = y_passes(halves[0], 0, (32, 96))
        y0 = 192 + 20 + total
        yp, plan = y_block(halves, y0, lead=False, even=7)
        passes = (conv_passes() + lead[:8] + inv_passes(3, 0, z8) + inv_passes(3, 1, z8) + lead[8:]
                  + bu_passes(i + LEAD, 0, 0, False) + yp)
        tr, k1, k2 = filter_tasks(i + 1, CFG["kconv"])
        fwd, tail, end = forward_tasks(i + 1), CFG["tail"], y0 + 280
        done = (3 * i + 2) // 2
        _weave(passes, plan + [
            ([dma_task([oa_unit_dma(done)])], y0 + 210, y0 + 210),
            (scan_tasks(i + LEAD - 1, 0, z8), *CFG["scanw"]), (tr, *CFG["tr"]),
            ([skip_task(halves[0], 0)], 232, 238),
            (widen_tasks(i + 1, z8, 16), *CFG["wid"]), (k1, *CFG["kwin"]),
            (inverse_tasks(i), *CFG["invw"]), (k2, *CFG["k2w"]),
            (fwd[:-tail], CFG["u0w"], end), (fwd[-tail:], end, end)], pred)
        pl.when(i % 2 == 1)(lambda: start([oa_unit_dma(done + 1)]))
        return 0

    lax.fori_loop(0, NG - 1, body, 0)

    wait([last_dma])
    g, last = NG - 1, L // UNIT - 1
    yp, plan = y_block((2 * last, 2 * last + 1), 192, even=2)
    ends = [[dma_task([oa_dma(last, n)])] for n in range(NG)]
    plan += [(ends[n], t + 6, t + 6) for n, (_, _, t) in enumerate(plan[NG:])]
    _weave(conv_passes() + yp[:8] + inv_passes(3, 0, z8) + inv_passes(3, 1, z8) + yp[8:], plan + [
        (scan_tasks(last, 0, z8), 0, 170),
        (inverse_tasks(g), 216, CFG["invend"])], pred)
    wait([oa_unit_dma(u) for u in range(last)] + [oa_dma(last, n) for n in range(NG)]
         + [ob_dma(n, half) for n in range(NG) for half in range(2)])


@jax.jit
def pallas_concat_heads__ssm_conv_s5__ssm_conv_h3__prompt_kernel(
    A_x: jax.Array,
    A_Lambda_re: jax.Array,
    A_Lambda_im: jax.Array,
    A_B_re: jax.Array,
    A_B_im: jax.Array,
    A_C_re: jax.Array,
    A_C_im: jax.Array,
    A_log_dt: jax.Array,
    A_Dskip: jax.Array,
    B_q: jax.Array,
    B_k: jax.Array,
    B_v: jax.Array,
    B_shift_k: jax.Array,
    B_ssm_k: jax.Array,
    B_ssm_D: jax.Array,
):
    assert A_x.shape == (1, L, D) and B_shift_k.shape == (D, 4)
    vmem = pltpu.VMEM
    dma = pltpu.SemaphoreType.DMA
    scratch = [
        vmem(_TABLES.shape, F32),
        vmem((D,), BF16), vmem((D,), BF16), vmem((D,), BF16), vmem((D,), BF16), vmem((D,), BF16),
        vmem((4, D), BF16),
        vmem((NG * L, 128), BF16),
        vmem((2 * D, D), BF16),
        vmem((2 * NG * D, 128), BF16),
        vmem((NG * L, 128), BF16),
        vmem((NG * L, 128), BF16),
        vmem((NG * L, 128), BF16),
        vmem((D, L), BF16),
        vmem((NG * P_ROWS * 8, 128), F32),
        vmem((2 * NG * D + 32, 128), BF16),
        vmem((2 * NG * NG * 64 + 16, 128), I32),
        vmem((SLOTS * 128 + 32, 128), BF16),
        vmem((SLOTS * 64 + 16, 128), I32),
        vmem((2 * 2 * NG * BU_PART, 128), F32),
        vmem((2 * NG * L + 32, 128), BF16),
        vmem((3 * NG * 8, 128), F32),
        vmem((NG * YS_ROWS, 128), F32),
        vmem((L + 16, D), F32),
        vmem((L // 2 + 16, 128), I32),
        vmem((KF_PAD + L + 16, 128), F32),
        vmem((2 * L + 16, 128), F32),
        vmem((2 * L + 16, 128), F32),
        vmem((2 * L + 8, 128), F32),
        vmem((32 * 128 + 32, 128), BF16),
        vmem((32 * 128 + 32, 128), BF16),
        vmem((8 * 128, 128), BF16),
        vmem((8 * 128, 128), BF16),
        vmem((NG * L + 16, 128), F32),
        dma((S_END,)),
    ]
    out = pl.pallas_call(
        _kernel,
        out_shape=jax.ShapeDtypeStruct((L, 2 * D), F32),
        in_specs=[pl.BlockSpec(memory_space=pl.ANY)] * 16,
        out_specs=pl.BlockSpec(memory_space=pl.ANY),
        scratch_shapes=scratch,
        compiler_params=pltpu.CompilerParams(vmem_limit_bytes=100 * 1024 * 1024, flags=CFG["flags"], disable_semaphore_checks=CFG["nosem"]),
        name="s5_h3",
    )(_TABLES, A_x.reshape(L, D), A_Lambda_re, A_Lambda_im, A_B_re, A_B_im, A_C_re, A_C_im,
      A_log_dt, A_Dskip, B_q.reshape(L, D), B_k.reshape(L, D), B_v.reshape(L, D),
      B_shift_k.T, B_ssm_k, B_ssm_D)
    return out.reshape(1, L, 2 * D)
```

```python
import math

import jax
import jax.numpy as jnp
import numpy as np
from jax import lax
from jax.experimental import pallas as pl
from jax.experimental.pallas import tpu as pltpu

F32, BF16, I32 = jnp.float32, jnp.bfloat16, jnp.int32

L = 2048
D = 640
NG = D // 128
UNIT = 256
SEG = 16
R = UNIT // SEG
LEAD = 4
HALF = UNIT // 2
BU_PART = 9 * 2 * R
YS_ROWS = SEG * (R // 2 + 1)
KF_PAD = 8


class _Signed:
    def __init__(self, v, neg=False):
        self.v, self.neg = v, neg

    def __neg__(self):
        return _Signed(self.v, not self.neg)

    def __add__(self, o):
        if self.neg == o.neg:
            return _Signed(self.v + o.v, self.neg)
        return _Signed(o.v - self.v if self.neg else self.v - o.v)

    def __sub__(self, o):
        return self + (-o)

    def __mul__(self, c):
        return _Signed(self.v * np.float32(-c if self.neg else c))

    def get(self):
        return -self.v if self.neg else self.v


def _rot(re, im, num, den):
    num %= den
    h = math.sqrt(0.5)
    if num == 0:
        return re, im
    if 4 * num == den:
        return -im, re
    if 4 * num == 3 * den:
        return im, -re
    if 8 * num == den:
        return (re - im) * h, (re + im) * h
    if 8 * num == 3 * den:
        return (re + im) * (-h), (re - im) * h
    if 8 * num == 5 * den:
        return (im - re) * h, (re + im) * (-h)
    if 8 * num == 7 * den:
        return (re + im) * h, (im - re) * h
    c = math.cos(2 * math.pi * num / den)
    s = math.sin(2 * math.pi * num / den)
    return re * c - im * s, re * s + im * c


def _dft4(z, sign):
    (r0, i0), (r1, i1), (r2, i2), (r3, i3) = z
    ar, ai, br, bi = r0 + r2, i0 + i2, r0 - r2, i0 - i2
    cr, ci, dr, di = r1 + r3, i1 + i3, r1 - r3, i1 - i3
    plus, minus = (br - di, bi + dr), (br + di, bi - dr)
    if sign < 0:
        plus, minus = minus, plus
    return [(ar + cr, ai + ci), plus, (ar - cr, ai - ci), minus]


def _fwd1(n, u):
    a0, a1, b0, b1 = u
    p, q = _rot(a0, b0, n, 32), _rot(a1, b1, n + 4, 32)
    s0, s1 = a0 + b0, a1 + b1
    return [(p[0] + q[0], p[1] + q[1]), _rot(p[0] - q[0], p[1] - q[1], n, 8),
            _rot(a0 - b0, a1 - b1, n, 16), (s0 + s1, s0 - s1)]


def _fwd2(grp, z):
    if grp < 3:
        return _dft4(z, 1)
    s4 = [t[0] for t in z]
    d4 = [t[1] for t in z]
    p = (d4[0], d4[2])
    q = _rot(d4[1], d4[3], 1, 8)
    s5 = [s4[0] + s4[2], s4[1] + s4[3]]
    return [
        (s5[0] + s5[1], s5[0] - s5[1]),
        (s4[0] - s4[2], s4[1] - s4[3]),
        (p[0] + q[0], p[1] + q[1]),
        (p[0] - q[0], p[1] - q[1]),
    ]


def _inv2(grp, w):
    if grp < 3:
        return _dft4(w, -1)
    s5 = [w[0][0] + w[0][1], w[0][0] - w[0][1]]
    s4 = [s5[0] + w[1][0], s5[1] + w[1][1], s5[0] - w[1][0], s5[1] - w[1][1]]
    p = (w[2][0] + w[3][0], w[2][1] + w[3][1])
    q = _rot(w[2][0] - w[3][0], w[2][1] - w[3][1], -1, 8)
    d4 = [p[0], q[0], p[1], q[1]]
    return [(s4[n], d4[n]) for n in range(4)]


def _inv1(n, z):
    e = _rot(*z[1], -n, 8)
    p = _rot(z[0][0] + e[0], z[0][1] + e[1], -n, 32)
    q = _rot(z[0][0] - e[0], z[0][1] - e[1], -(n + 4), 32)
    d0, d1 = _rot(*z[2], -n, 16)
    s0, s1 = z[3][0] + z[3][1], z[3][0] - z[3][1]
    return [p[0] + (s0 + d0), q[0] + (s1 + d1), p[1] + (s0 - d0), q[1] + (s1 - d1)]


_F1 = [4 * (g + 2 * k) + 1 for g in range(2) for k in range(4)]
_F1 += [2 * (4 * k + 1) for k in range(4)] + [0, 8, 4, 20]
_REAL_SLOT = 12
SLOTS = len(_F1)


def _dft_tables():
    kap = np.arange(128)
    j = 8 * (kap // 16) + kap % 8
    part = (kap // 8) % 2
    pr, pc, jr, jc = part[:, None], part[None, :], j[:, None], j[None, :]
    lo = 2 * np.pi * jr * jc / 64
    base = np.where(pr == pc, np.cos(lo), np.where(pr == 0, -np.sin(lo), np.sin(lo)))
    hi = 2 * np.pi * (16 + 32 * (jr - 32)) * jc / 2048
    v0 = np.where(pr == 0, np.cos(lo), np.where(jr == 0, np.cos(np.pi * jc), np.sin(lo)))
    v32 = np.where(pr == 0, np.cos(hi), np.sin(hi))
    real = np.where(jr < 32, np.where(pc == 0, v0, 0.0), np.where(pc == 1, v32, 0.0))
    th = 2 * np.pi * np.outer(np.array(_F1), j) / 2048
    zeros = np.zeros((8, 128))
    return np.concatenate([base, real, np.cos(th), np.sin(th), zeros]).astype(np.float32)


_TABLES = _dft_tables()
_FFT_SCALE = 2.0 ** -10

(P_MU, P_RHO, P_RHO1, P_RHO2, P_RHO4, P_TAP, P_SSMD, P_DSKIP, P_COEF, P_ROWS) = (
    0, 2, 4, 6, 8, 10, 14, 15, 16, 20)
S_SMALL, S_F0, S_K0, S_C, S_OUT, S_X0, S_B = range(7)
S_COL = S_B + NG
S_END = S_COL + NG - 1


def _cmul(a, b):
    return a[0] * b[0] - a[1] * b[1], a[0] * b[1] + a[1] * b[0]


def _pack(lo, hi):
    return jnp.concatenate([lo, hi], axis=0).astype(BF16)


def _unpack(w):
    v = pltpu.bitcast(w, BF16).astype(F32)
    return v[:8], v[8:]


CFG = dict(scan=22, u=24, k1=0, p2=0, inv=36, skip=30, tail=4, kconv=4, steps=2, p2n=2,
           u0w=350, kwin=(100, 216), tr=(60, 90), wid=(216, 330), scanw=(0, 350), invw=(220, 420),
           k2w=(230, 480), mf=128, mi=128, ord=(2, 4), sk0=12, sh1=None, sh2=None, when=(0, 1, 1, 2, 3, 4, 6), s2=380, retap=False, invend=290,
           Q=1, invsplit=False, kg=1, k0=1.0, u0=0.45, udir=True, kdir=True,
           flags=None, nosem=False, skipme=lambda n, rows: False)


class _Zeros:
    def __init__(self, v):
        self.v = v


class _Gate:
    def __init__(self, pred=None, seen=()):
        self.pred, self.seen = pred, seen

    def early(self, lag):
        old = [e for e in self.seen if e[0] <= -lag]
        return max(old, key=lambda e: e[0])[1] if lag and old else None

    def value(self, v, lag):
        early = self.early(lag)
        return v if early is None else jnp.where(self.pred, v, early)

    def loads(self, ref, lag):
        early = self.early(lag)
        if early is not None:
            ref[pl.ds(ref.shape[0] - 8, 8), :] = (
                early if ref.dtype == F32 else pltpu.bitcast(early, I32))


def _weave(passes, plan, pred):
    if CFG["skipme"](len(passes), sum(q[0] for q in passes)):
        return
    begin, clock = [], [0] * 4
    for i, (n, *_) in enumerate(passes):
        begin.append(clock[i % 4] / 16)
        clock[i % 4] += n

    def index(t):
        later = [i for i, b in enumerate(begin) if b >= t - 3.999]
        if not later:
            return len(passes)
        same = [i for i in later if begin[i] == min(begin[j] for j in later)]
        return same[min(max(int((t - begin[same[0]]) / 4 * len(same)), 0), len(same) - 1)]

    at = [[] for _ in range(len(passes) + 1)]
    for tasks, lo, hi in plan:
        total, done = sum(sum(c) for c, _ in tasks) or 1, 0.0
        for costs, fn in tasks:
            where = []
            for cost in costs:
                done += cost
                where.append(index(lo + done / total * (hi - lo)))
            at[min(where)].append((fn, where))
    seen, ties = [], [[] for _ in at]
    for i, fns in enumerate(at):
        now = (begin[i] + i % 4) if i < len(begin) else clock[0] / 16
        early = [(t - now, v) for t, v in seen if t % CFG["Q"] < 1 or CFG["Q"] == 1]
        for fn, where in fns:
            for w, tie in zip(where, fn(_Gate(pred, early)) or ()):
                ties[w].append(tie)
        if i == len(passes):
            break
        n, lhs, rhs, consume = passes[i]
        w = rhs()
        for tie in ties[i]:
            if isinstance(tie, _Zeros):
                v = tie.v
                w[-1] = w[-1] | (v if v.dtype == I32 else pltpu.bitcast(v, I32))
            else:
                w[-1] = jnp.where(pred, w[-1], pltpu.bitcast(tie, I32))
        d = jnp.dot(pltpu.bitcast(jnp.concatenate(lhs(), axis=0), BF16),
                    pltpu.bitcast(jnp.concatenate(w, axis=0), BF16), preferred_element_type=F32)
        seen += [(begin[i] + i % 4 + j // 16 - 4, d[j - 8:j]) for j in range(64, n + 1, 64)]
        consume(d)


def _now(tasks):
    for _, fn in tasks:
        fn(_Gate())


def _kernel(tab_hbm, x_hbm, lre_hbm, lim_hbm, bre_hbm, bim_hbm, cre_hbm, cim_hbm,
            ldt_hbm, dsk_hbm, q_hbm, k_hbm, v_hbm, tap_hbm, sk_hbm, sd_hbm,
            o_hbm,
            tab, lre_v, lim_v, ldt_v, dsk_v, sd_v, tap_v,
            xb, braw, craw, qb, kb, vb, skb,
            par, wb16, wc, mf16, mi, bu, hb16, carry, ys, oa,
            kt, kf, st_u, st_k, st_i, vu16, vk16, pb0, pb1, ob,
            sem):
    x32, q32, k32, v32, wb, mf, hb, vu, vk = (
        r.bitcast(I32) for r in (xb, qb, kb, vb, wb16, mf16, hb16, vu16, vk16))
    pb16 = (pb0, pb1)
    pb = (pb0.bitcast(I32), pb1.bitcast(I32))

    def rows(ref, start, n=8):
        return ref[pl.ds(start, n), :]

    def hint(v, n):
        return v if isinstance(v, int) or n == 1 else pl.multiple_of(v, n)

    def view(ref, start, n=None):
        return ref.at[pl.ds(hint(start, 16), n or ref.shape[0]), :]

    def after(ref):
        return _Zeros(view(ref, z8)[ref.shape[0] - 16:ref.shape[0] - 8, 0:128])

    small = [pltpu.make_async_copy(s, d, sem.at[S_SMALL]) for s, d in (
        (lre_hbm, lre_v), (lim_hbm, lim_v), (ldt_hbm, ldt_v),
        (dsk_hbm, dsk_v), (sd_hbm, sd_v), (tap_hbm, tap_v),
        (tab_hbm.at[pl.ds(288, 8), :], tab.at[pl.ds(288, 8), :]))]
    tab_dma = pltpu.make_async_copy(
        tab_hbm.at[pl.ds(0, 288), :], tab.at[pl.ds(0, 288), :], sem.at[S_B + 4])

    def x_dma(u):
        return [pltpu.make_async_copy(
            x_hbm.at[pl.ds(hint(u * UNIT, UNIT), UNIT), pl.ds(128 * n, 128)],
            xb.at[pl.ds(hint(n * L + u * UNIT, UNIT), UNIT), :], sem.at[(S_X0, S_B + 4, S_F0, S_K0)[u] if isinstance(u, int) and u < LEAD
                                                     else S_COL + u - LEAD])
            for n in range(NG)]

    def b_dma(p):
        return [pltpu.make_async_copy(
            src.at[pl.ds(128 * p, 128), :], braw.at[pl.ds(D * c + 128 * p, 128), :],
            sem.at[S_B + p]) for c, src in enumerate((bre_hbm, bim_hbm))]

    c_dma = [pltpu.make_async_copy(
        src.at[:, pl.ds(128 * p, 128)], craw.at[pl.ds(D * (NG * c + p), D), :],
        sem.at[S_C]) for c, src in enumerate((cre_hbm, cim_hbm)) for p in range(NG)]

    def col_dma(which, g, sem_at):
        src, dst = ((k_hbm, kb), (v_hbm, vb), (q_hbm, qb))[which]
        return pltpu.make_async_copy(
            src.at[:, pl.ds(hint(128 * g, 128), 128)],
            dst.at[pl.ds(hint(L * g, L), L), :], sem.at[sem_at])

    def sk_dma(g, sem_at):
        t = hint(128 * g, 128)
        return [pltpu.make_async_copy(
            sk_hbm.at[pl.ds(t, 128), :], skb.at[pl.ds(t, 128), :], sem.at[sem_at])]

    def oa_dma(u, n):
        t = hint(u * UNIT, UNIT)
        return pltpu.make_async_copy(
            oa.at[pl.ds(t, UNIT), pl.ds(128 * n, 128)],
            o_hbm.at[pl.ds(t, UNIT), pl.ds(128 * n, 128)], sem.at[S_OUT])

    def oa_unit_dma(u):
        t = hint(u * UNIT, UNIT)
        return pltpu.make_async_copy(
            oa.at[pl.ds(t, UNIT), :], o_hbm.at[pl.ds(t, UNIT), pl.ds(0, D)], sem.at[S_OUT])

    def ob_dma(g, half):
        h = L // 2
        return pltpu.make_async_copy(
            ob.at[pl.ds(hint(L * g + h * half, h), h), :],
            o_hbm.at[pl.ds(h * half, h), pl.ds(hint(D + 128 * g, 128), 128)], sem.at[S_OUT])

    def start(ds):
        for d in ds:
            d.start()

    def wait(ds):
        for d in ds:
            d.wait()

    def prm(g, row):
        return rows(view(par, g * (P_ROWS * 8), P_ROWS * 8), row * 8)

    def bu_passes(u, slot, z, shift):
        out = []
        xu, w = view(x32, u * (UNIT // 2), ((NG - 1) * L + UNIT) // 2), view(wb, z)
        order = [p + c * NG for p in range(NG) for c in range(2)]
        for n in order:
            sizes = [128, 128]
            if shift and n == order[0]:
                sizes = [32, 32, 96, 96]
            if shift and n == order[-1]:
                sizes = [96, 96, 32, 32] if shift is True else [64] * 4
            if shift is None:
                sizes = [64] * 4
            for m, MM in zip(np.cumsum([0] + sizes).tolist(), sizes):
                acc = []
                for kk in range(NG):
                    def lhs(m=m, kk=kk, MM=MM):
                        t = (kk * L + m) // 2
                        return [rows(xu, t + 8 * i) for i in range(MM // 16)]

                    def rhs(n=n, kk=kk):
                        return [rows(w, (n * NG + kk) * 64 + 8 * i) for i in range(8)]

                    def consume(d, m=m, n=n, kk=kk, acc=acc, MM=MM):
                        acc.append(d if kk == 0 else acc[-1] + d)
                        if kk == NG - 1:
                            for i in range(MM // 8):
                                seg, r = divmod(m + 8 * i, R)
                                row = 9 * (seg % 2 * R + r) + seg // 2
                                bu[pl.ds((slot * 2 * NG + n) * BU_PART + row, 8, stride=9), :] = (
                                    acc[-1][8 * i:8 * i + 8])
                    out.append((MM, lhs, rhs, consume))
        return out

    def scan_tasks(u, slot, z):
        steps = CFG["steps"]
        state = {}
        hu = view(hb16, u * UNIT, (2 * NG - 1) * L + UNIT)

        def b(p, ch, r):
            return tuple(rows(bu, (slot * 2 * NG + c * NG + p) * BU_PART + 9 * (ch * R + r))
                         for c in range(2))

        def step(mu, h, br):
            return (mu[0] * h[0] + br[0]) - mu[1] * h[1], (mu[0] * h[1] + br[1]) + mu[1] * h[0]

        def ends(p, gate):
            mu, ties = (gate.value(prm(p, P_MU), CFG["scan"]), prm(p, P_MU + 1)), []
            h = [b(p, ch, 0) for ch in range(2)]
            for r in range(1, R):
                h = [step(mu, h[ch], b(p, ch, r)) for ch in range(2)]
                if r % steps == 0:
                    ties.append(h[r // steps % 2][0])
            state[p] = starts(p, h)
            return ties + [state[p][1][0]]

        def starts(p, e):
            last = lax.broadcasted_iota(I32, (8, 128), 0) == 7
            rho = (prm(p, P_RHO), prm(p, P_RHO + 1))
            pair = step(rho, e[0], e[1])
            a = tuple(pltpu.roll(jnp.where(last, rows(carry, (2 * p + c) * 8), pair[c]), 1, 0)
                      for c in range(2))
            for sh, row in ((1, P_RHO1), (2, P_RHO2), (4, P_RHO4)):
                a = step((prm(p, row), prm(p, row + 1)), tuple(pltpu.roll(c, sh, 0) for c in a), a)
            return [a, step(rho, a, e[0])]

        def run(p, r0, gate):
            if r0 == 0:
                state["mu"] = (prm(p, P_MU), prm(p, P_MU + 1))
            mu, h = (gate.value(state["mu"][0], CFG["scan"]), state["mu"][1]), state[p]
            for r in range(r0, r0 + steps):
                h = [step(mu, h[ch], b(p, ch, r)) for ch in range(2)]
                for c in range(2):
                    hu[pl.ds((c * NG + p) * L + 16 * r, 16), :] = _pack(h[0][c], h[1][c])
            state[p] = h
            if r0 + steps == R:
                for c in range(2):
                    carry[pl.ds((2 * p + c) * 8, 8), :] = h[1][c]
            return [after(hb)]

        tasks = []
        for p in range(NG):
            tasks.append(([16 * steps] * ((R - 1) // steps) + [46 + 16 * steps],
                          lambda gate, p=p: ends(p, gate)))
            tasks += [([18 * steps], lambda gate, p=p, r0=r0: run(p, r0, gate))
                      for r0 in range(0, R, steps)]
        return tasks

    def y_passes(h, n, sizes=(HALF,), z=0):
        out, w, hu = [], view(wc, z), view(hb, h * (HALF // 2), ((2 * NG - 1) * L + HALF) // 2)
        for t0, MM in zip(np.cumsum((0,) + sizes).tolist(), sizes):
            acc = []
            for kk in range(2 * NG):
                def lhs(t0=t0, kk=kk, MM=MM):
                    return [rows(hu, (kk * L + t0) // 2 + 8 * i) for i in range(MM // 16)]

                def rhs(kk=kk):
                    return [rows(w, (kk * NG + n) * 64 + 8 * i) for i in range(8)]

                def consume(d, t0=t0, kk=kk, acc=acc, MM=MM):
                    acc.append(d if kk == 0 else acc[-1] + d)
                    if kk == 2 * NG - 1:
                        for i in range(MM // 8):
                            r, ch = divmod(t0 // 8 + i, 2)
                            ys[pl.ds(n * YS_ROWS + ch * (R // 2 + 1) + r, 8, stride=R + 2), :] = (
                                acc[-1][8 * i:8 * i + 8])
                out.append((MM, lhs, rhs, consume))
        return out

    def skip_task(h, n):
        def fn(gate):
            dsk, ties = gate.value(prm(n, P_DSKIP), CFG["skip"]), []
            t = h // 2 * UNIT + h % 2 * (R // 2)
            xu = x32.at[pl.ds(hint(t // 2 + n * (L // 2), 4), UNIT // 2 - 4 + 8 * (n < NG - 1 or not isinstance(h, int))), :]
            ou = oa.at[pl.ds(hint(t, 8), UNIT - R // 2), :]
            for g in range(SEG):
                if g == SEG - 1 and n == NG - 1 and isinstance(h, int):
                    xs = _unpack(rows(xu, 8 * g - 4))[1]
                else:
                    xs = _unpack(rows(xu, 8 * g))[0]
                y = rows(ys, n * YS_ROWS + g * (R // 2 + 1))
                ou[pl.ds(R * g, 8), pl.ds(128 * n, 128)] = y + xs * dsk
                if g % 8 == 7:
                    ties.append(after(oa))
            return ties
        return ([24, 24], fn)

    def widen_tasks(g, z, pieces=2):
        def fn(i0, i1):
            kg = view(k32, g * (L // 2), L // 2)
            for i in range(i0, i1):
                lo, hi = _unpack(rows(kg, 8 * i))
                kf[pl.ds(KF_PAD + 16 * i, 8), :] = lo
                kf[pl.ds(KF_PAD + 16 * i + 8, 8), :] = hi
            return [after(kf)]
        n = L // 16 // pieces
        return [([2 * n], lambda gate, i=i: fn(i * n, (i + 1) * n)) for i in range(pieces)]

    def transpose_tasks(g, z, pieces=8):
        def fn(c0, c1):
            for c in range(c0, c1):
                t = skb[pl.ds(hint(128 * g, 128), 128), pl.ds(128 * c, 128)]
                kt[pl.ds(64 * c, 64), :] = pltpu.bitcast(t.T, I32)
            return [after(kt)]
        n = L // 128 // pieces
        return [([8 * n], lambda gate, i=i: fn(i * n, (i + 1) * n)) for i in range(pieces)]

    def staged(s, half, n, grp, c):
        return (((s * 2 + half) * 4 + n) * 4 + grp) * 16 + 8 * c

    ops1 = (18, 36, 30, 36)

    def forward_tasks_of(st, s, half, z, chunk, chunk_cost, direct):
        dst16, dst = (vu16, vu) if st is st_u else (vk16, vk)

        def second(grp, zs):
            for k, pair in enumerate(_fwd2(grp, zs)):
                dst16[pl.ds(((4 * grp + k) * 2 + half) * 128 + 16 * s, 16), :] = (
                    _pack(pair[0].get(), pair[1].get()))
            return after(dst)

        kept = []

        def first(gate, n):
            load = chunk(gate, n)
            u = [load(16 * half + n + 4 * m) for m in range(4)]
            pairs = _fwd1(n, [_Signed(v) for v in u])
            kept.append(pairs)
            for grp in range(2 * direct, 4):
                for c in range(2):
                    st[pl.ds(staged(s, half, n, grp, c), 8), :] = pairs[grp][c].get()
            return [u[0] + u[2]] * (chunk_cost > 4) + [after(st)]

        def rest(grp):
            if direct and grp < 2:
                return [second(grp, [t[grp] for t in kept])]
            return [second(grp, [tuple(_Signed(rows(view(st, z), staged(s, half, n, grp, c)))
                                       for c in range(2)) for n in range(4)])]

        split = (chunk_cost > 4) * (chunk_cost // 2 + 1)
        one = [([split] * (split > 0) + [chunk_cost + ops1[n] - split], lambda gate, n=n: first(gate, n))
               for n in range(4)]
        if CFG["p2n"] == 4:
            two = [([20], lambda gate, grp=grp: rest(grp)) for grp in range(4)]
        else:
            two = [([40], lambda gate, grp=grp: rest(grp) and rest(grp + 1)) for grp in (0, 2)]
        h = len(two) // 2
        return (one + two[:h], two[h:]) if direct else (one, two)

    def u_tasks(g, s, half, z):
        loaded = []

        def chunk(gate, n):
            if n == 0 or CFG["retap"]:
                loaded[:] = [prm(g, P_TAP + t) for t in range(4)]
            taps = [gate.value(loaded[0], CFG["u"])] + loaded[1:]
            kz, vg = view(kf, z), view(v32, g * (L // 2), L // 2)

            def load(c):
                t = 64 * c + 8 * s
                ks = rows(kz, KF_PAD + t) * taps[0]
                for lag in range(1, 4):
                    ks = ks + rows(kz, KF_PAD + t - lag) * taps[lag]
                return ks * _unpack(rows(vg, (t // 16) * 8))[s % 2]
            return load
        return forward_tasks_of(st_u, s, half, z, chunk, 36, CFG["udir"])

    def k_tasks(g, s, half, z, direct):
        def chunk(gate, n):
            if n % CFG["kg"] == 0:
                gate.loads(kt, CFG["k1"])

            def load(c):
                v = _unpack(rows(view(kt, z), 32 * c + 8 * (s // 2)))[s % 2]
                if s == 0 and c == 0:
                    first = lax.broadcasted_iota(I32, (8, 128), 0) == 0
                    v = v + jnp.where(first, prm(g, P_SSMD), 0.0)
                return v
            return load
        return forward_tasks_of(st_k, s, half, z, chunk, 4, direct)

    def fwd_passes(grp, z):
        out, MM = [], CFG["mf"]
        for slot in range(4 * grp, 4 * grp + 4):
            for part in range(128 // MM):
                got = []
                for src, half in ((vu, 0), (vk, 0), (vu, 1), (vk, 1)):
                    def lhs(slot=slot, part=part):
                        return [rows(mf, slot * 64 + MM // 2 * part + 8 * i) for i in range(MM // 16)]

                    def rhs(slot=slot, src=src, half=half):
                        return [rows(view(src, z), (2 * slot + half) * 64 + 8 * i) for i in range(8)]

                    def consume(d, slot=slot, part=part, got=got):
                        got.append(d)
                        if len(got) < 4:
                            return
                        for i in range(MM // 16):
                            u0, k0, u1, k1 = ((t[16 * i:16 * i + 8], t[16 * i + 8:16 * i + 16]) for t in got)
                            lo, a, b = _cmul(u0, k0), _cmul(u0, k1), _cmul(u1, k0)
                            if slot == _REAL_SLOT and part == 0 and i == 0:
                                first = lax.broadcasted_iota(I32, (8, 128), 0) == 0
                                lo, a, b = (tuple(jnp.where(first, 0.5 * (x[c] * y[c]), p[c]) for c in range(2))
                                            for p, x, y in ((lo, u0, k0), (a, u0, k1), (b, u1, k0)))
                            if _F1[slot] % 2:
                                hi = ((a[0] + b[0]) - lo[0], (a[1] + b[1]) - lo[1])
                            else:
                                hi = ((a[0] + b[0]) + lo[0], (a[1] + b[1]) + lo[1])
                            for half, p in enumerate((lo, hi)):
                                at = (slot % 4 * 2 + half) * 128 + MM * part + 16 * i
                                pb16[grp % 2][pl.ds(at, 16), :] = _pack(*p)
                    out.append((MM, lhs, rhs, consume))
        return out

    def inv_passes(grp, half, z):
        out, MM = [], CFG["mi"]
        for part in range(128 // MM):
            got = []
            for slot in range(4 * grp, 4 * grp + 4):
                def lhs(slot=slot, part=part):
                    return [rows(mi, slot * 64 + MM // 2 * part + 8 * i) for i in range(MM // 16)]

                def rhs(slot=slot):
                    return [rows(view(pb[grp % 2], z), (slot % 4 * 2 + half) * 64 + 8 * i)
                            for i in range(8)]

                def consume(d, part=part, got=got):
                    got.append(d)
                    if len(got) < 4:
                        return
                    for i in range(MM // 16):
                        w = [(_Signed(t[16 * i:16 * i + 8]), _Signed(t[16 * i + 8:16 * i + 16]))
                             for t in got]
                        for n, pair in enumerate(_inv2(grp, w)):
                            for c in range(2):
                                at = staged(MM // 16 * part + i, half, n, grp, c)
                                st_i[pl.ds(at, 8), :] = pair[c].get()
                out.append((MM, lhs, rhs, consume))
        return out

    def inv1_task(g, s, half, z):
        def fn(gate, ns):
            gate.loads(st_i, CFG["inv"])
            qg, og, ties = view(q32, g * (L // 2), L // 2), view(ob, g * L, L), []
            for n in ns:
                zs = [tuple(_Signed(rows(view(st_i, z), staged(s, half, n, grp, c))) for c in range(2))
                      for grp in range(4)]
                for m, y in enumerate(_inv1(n, zs)):
                    t = 64 * (16 * half + n + 4 * m) + 8 * s
                    og[pl.ds(t, 8), :] = _unpack(rows(qg, (t // 16) * 8))[s % 2] * y.get()
                ties.append(after(ob))
            return ties
        if CFG["invsplit"]:
            return [([12 + ops1[n]], lambda gate, n=n: fn(gate, [n])) for n in range(4)]
        return [([12 + n for n in ops1], lambda gate: fn(gate, range(4)))]

    filter0 = x_dma(2) + sk_dma(0, S_F0)
    data0 = x_dma(3) + [col_dma(0, 0, S_K0), col_dma(1, 0, S_K0)]

    def group_dma(g):
        at = S_COL + g
        return ([col_dma(2, g, at)] + sk_dma(g + 1, at)
                + [col_dma(0, g + 1, at), col_dma(1, g + 1, at)] + x_dma(g + LEAD))

    last_dma = col_dma(2, NG - 1, S_SMALL)

    start(small + b_dma(0) + x_dma(0) + b_dma(1) + b_dma(2))
    wait(small)
    zeros = rows(tab, 288).astype(I32)
    z8 = pl.multiple_of(zeros[0, 0], 16)
    sub = lax.broadcasted_iota(I32, (8, 128), 0)
    pred = zeros == 0

    def stack(ref):
        v = ref[...].astype(F32).reshape(1, D)
        return jnp.concatenate([v[:, 128 * g:128 * (g + 1)] for g in range(NG)]
                               + [v[:, :128]] * (8 - NG), axis=0)

    lre, lim = stack(lre_v), stack(lim_v)
    dt = jnp.exp(stack(ldt_v)).astype(BF16).astype(F32)
    mag, ang = jnp.exp(dt * lre), dt * lim
    lam = (mag * jnp.cos(ang), mag * jnp.sin(ang))
    scale = jnp.maximum(jnp.abs(lre), jnp.abs(lim))
    nre, nim = lre / scale, lim / scale
    den = (nre * nre + nim * nim) * scale
    coef = _cmul(((lam[0] - 1.0) / den, lam[1] / den), (nre, -nim))
    mu = (lam[0], -lam[1])
    rho = [mu]
    for _ in range(R.bit_length() + 2):
        rho.append(_cmul(rho[-1], rho[-1]))
    dsk, ssd = stack(dsk_v), stack(sd_v)
    taps = tap_v[...].astype(F32) * _FFT_SCALE
    for g in range(NG):
        def put(row, v):
            par[pl.ds((g * P_ROWS + row) * 8, 8), :] = v

        def lanes(v):
            return jnp.broadcast_to(v[g:g + 1], (8, 128))
        for c in range(2):
            put(P_MU + c, lanes(mu[c]))
            put(P_RHO + c, lanes(rho[-4][c]))
            for n, row in enumerate((P_RHO1, P_RHO2, P_RHO4)):
                put(row + c, jnp.where(sub >= 1 << n, lanes(rho[n - 3][c]), 0.0))
        for t in range(4):
            put(P_TAP + t, jnp.broadcast_to(taps[t:t + 1, 128 * g:128 * (g + 1)], (8, 128)))
        put(P_COEF, lanes(2.0 * coef[0]))
        put(P_COEF + 1, lanes(-2.0 * coef[0]))
        put(P_COEF + 2, lanes(2.0 * coef[1]))
        put(P_SSMD, lanes(ssd))
        put(P_DSKIP, lanes(dsk))
    for ref in (hb, oa, kf, kt, vu, vk, st_u, st_k, ob, mf, mi, wb, wc):
        ref[pl.ds(ref.shape[0] - 16, 8), pl.ds(0, 128)] = jnp.zeros((8, 128), ref.dtype)
    for i in range(2 * NG):
        carry[pl.ds(8 * i, 8), :] = jnp.zeros((8, 128), F32)
    kf[pl.ds(0, KF_PAD), :] = jnp.zeros((KF_PAD, 128), F32)

    def matrix_task(slot):
        def fn(gate):
            if slot != _REAL_SLOT:
                c, s = tab[pl.ds(256 + slot, 1), :], tab[pl.ds(272 + slot, 1), :]
            for a in range(8):
                if slot == _REAL_SLOT:
                    re, im = rows(tab, 128 + 16 * a), rows(tab, 128 + 16 * a + 8)
                else:
                    br, bi = rows(tab, 16 * a), rows(tab, 16 * a + 8)
                    re, im = c * br - s * bi, s * br + c * bi
                mf16[pl.ds(slot * 128 + 16 * a, 16), :] = _pack(re, im)
            m = pltpu.bitcast(rows(view(mf, z8), slot * 64, 64), BF16)
            mi[pl.ds(slot * 64, 64), :] = pltpu.bitcast(m.T, I32)
            return [after(mf), after(mi)]
        return ([48, 8], fn)

    def scale_b(p, kk):
        cr, ncr, ci = prm(p, P_COEF), prm(p, P_COEF + 1), prm(p, P_COEF + 2)
        br, bi = (braw[pl.ds(D * c + 128 * p, 128), pl.ds(128 * kk, 128)].T.astype(F32)
                  for c in range(2))
        ties = []
        for i in range(8):
            r0, r1 = br[16 * i:16 * i + 8], br[16 * i + 8:16 * i + 16]
            i0, i1 = bi[16 * i:16 * i + 8], bi[16 * i + 8:16 * i + 16]
            wb16[pl.ds((p * NG + kk) * 128 + 16 * i, 16), :] = _pack(
                cr * r0 - ci * i0, cr * r1 - ci * i1)
            wb16[pl.ds(((NG + p) * NG + kk) * 128 + 16 * i, 16), :] = _pack(
                ncr * i0 - ci * r0, ncr * i1 - ci * r1)
            if i % 2:
                ties.append(after(wb))
        return ties

    def c_task(n, k0, k1):
        def fn(gate):
            for kk in range(k0, k1):
                t = craw[pl.ds(kk * D + 128 * n, 128), :]
                wc[pl.ds((kk * NG + n) * 64, 64), :] = pltpu.bitcast(t.T, I32)
            return [after(wc)]
        return ([16], fn)

    first = bu_passes(0, 1, z8, None)
    first = [first[len(first) // NG * p:len(first) // NG * (p + 1)] for p in range(NG)]

    mats = [matrix_task(slot) for slot in range(SLOTS)]

    def scale_tasks(p):
        return [([36] * 4, lambda gate, kk=kk: scale_b(p, kk)) for kk in range(NG)]

    def dma_task(ds):
        return ([1], lambda gate: start(ds))

    def filter_tasks(g, early):
        ts = [k_tasks(g, j // 2, j % 2, z8, j >= early and CFG["kdir"]) for j in range(16)]
        return (transpose_tasks(g, z8), [q for t in ts[:early] for q in t[0]],
                [q for t in ts[:early] for q in t[1]] + [q for t in ts[early:] for q in t[0] + t[1]])

    def forward_tasks(g):
        return [t for s in range(8) for half in range(2) for t in sum(u_tasks(g, s, half, z8), [])]

    def y_block(halves, t0, z=0, lead=True, even=None):
        tiles = [(h, n) for h in halves for n in range(NG)]
        passes, plan = [], []
        for j, (h, n) in enumerate(tiles):
            sizes = (HALF,)
            if j == 0 and lead is not None:
                if not lead:
                    continue
                sizes = (32, 96)
            if j == even:
                sizes = (64, 64)
            if j == len(tiles) - 1:
                sizes = (96, 32)
            passes += y_passes(h, n, sizes, z)
            t0 += 20
            plan.append(([skip_task(h, n)], t0 + CFG["sk0"], t0 + CFG["sk0"] + 6))
        return passes, plan

    total = 2 * NG * NG * UNIT // 64

    def early(at):
        for when, ds in zip(CFG["when"], (filter0, data0, c_dma, group_dma(0), group_dma(1), group_dma(2),
                                          group_dma(3) + [last_dma])):
            if when == at:
                start(ds)

    wait(b_dma(0))
    start(b_dma(3) + b_dma(4) + x_dma(1) + [tab_dma])
    _now(scale_tasks(0))
    wait(x_dma(0))
    _weave(first[0], [], pred)
    early(0)
    wait(b_dma(1))
    _now(scale_tasks(1))
    _weave(first[1], [], pred)
    early(1)
    wait(b_dma(2) + b_dma(3))
    _now(scale_tasks(2))
    _weave(first[2] + first[3], [(scale_tasks(3), 0, 32)], pred)
    early(2)
    wait(b_dma(4) + x_dma(1) + [tab_dma])
    _now(scale_tasks(4))
    _weave(first[4] + bu_passes(1, 0, 0, CFG["sh1"]), [
        (scan_tasks(0, 1, z8), 40, 40 + total), (mats, 0, 160)], pred)
    early(3)
    wait(filter0)
    tr, _, k1 = filter_tasks(0, 0)
    nk, fwd = int(CFG["k0"] * len(k1)), forward_tasks(0)
    nu = int(CFG["u0"] * len(fwd))
    _weave(bu_passes(2, 1, 0, CFG["sh2"]), [
        (scan_tasks(1, 0, z8), 0, total), (tr, 8, 32), (k1[:nk], 36, total)], pred)
    early(4)
    wait(data0 + c_dma)
    cs = [c_task(n, k, k + 2) for n in range(NG) for k in range(0, 2 * NG, 2)]
    yp, plan = y_block((0, 1), total, z8, lead=None, even=2)
    _weave(bu_passes(3, 0, 0, "open") + yp, plan + [
        (scan_tasks(2, 1, z8), 0, CFG["s2"]), (k1[nk:], 0, total), (widen_tasks(0, z8, 16), 0, 40),
        (cs, 0, total - 16), (fwd[:-2], 40, 2 * total), (fwd[-2:], 2 * total, 2 * total)], pred)
    start([oa_unit_dma(0)])
    early(6)

    def conv_passes():
        passes = fwd_passes(0, z8)
        for grp in range(1, 4):
            f, n = fwd_passes(grp, z8), 4 * 128 // CFG["mf"]
            a, b = (n * j for j in CFG["ord"])
            passes += f[:a] + inv_passes(grp - 1, 0, z8) + f[a:b] + inv_passes(grp - 1, 1, z8) + f[b:]
        return passes

    def inverse_tasks(g):
        tasks = []
        for half in range(2):
            for s in range(8):
                tasks += inv1_task(g, s, half, z8)
            tasks.append(dma_task([ob_dma(g, half)]))
        return tasks

    def body(i, _):
        wait(group_dma(i))
        halves = [2 + 3 * i + j for j in range(3)]
        lead = y_passes(halves[0], 0, (32, 96))
        y0 = 192 + 20 + total
        yp, plan = y_block(halves, y0, lead=False, even=7)
        passes = (conv_passes() + lead[:8] + inv_passes(3, 0, z8) + inv_passes(3, 1, z8) + lead[8:]
                  + bu_passes(i + LEAD, 0, 0, False) + yp)
        tr, k1, k2 = filter_tasks(i + 1, CFG["kconv"])
        fwd, tail, end = forward_tasks(i + 1), CFG["tail"], y0 + 280
        done = (3 * i + 2) // 2
        _weave(passes, plan + [
            ([dma_task([oa_unit_dma(done)])], y0 + 210, y0 + 210),
            (scan_tasks(i + LEAD - 1, 0, z8), *CFG["scanw"]), (tr, *CFG["tr"]),
            ([skip_task(halves[0], 0)], 232, 238),
            (widen_tasks(i + 1, z8, 16), *CFG["wid"]), (k1, *CFG["kwin"]),
            (inverse_tasks(i), *CFG["invw"]), (k2, *CFG["k2w"]),
            (fwd[:-tail], CFG["u0w"], end), (fwd[-tail:], end, end)], pred)
        pl.when(i % 2 == 1)(lambda: start([oa_unit_dma(done + 1)]))
        return 0

    lax.fori_loop(0, NG - 1, body, 0)

    wait([last_dma])
    g, last = NG - 1, L // UNIT - 1
    yp, plan = y_block((2 * last, 2 * last + 1), 192, even=2)
    ends = [[dma_task([oa_dma(last, n)])] for n in range(NG)]
    plan += [(ends[n], t + 6, t + 6) for n, (_, _, t) in enumerate(plan[NG:])]
    _weave(conv_passes() + yp[:8] + inv_passes(3, 0, z8) + inv_passes(3, 1, z8) + yp[8:], plan + [
        (scan_tasks(last, 0, z8), 0, 170),
        (inverse_tasks(g), 216, CFG["invend"])], pred)
    wait([oa_unit_dma(u) for u in range(last)] + [oa_dma(last, n) for n in range(NG)]
         + [ob_dma(n, half) for n in range(NG) for half in range(2)])


@jax.jit
def pallas_concat_heads__ssm_conv_s5__ssm_conv_h3__prompt_kernel(
    A_x: jax.Array,
    A_Lambda_re: jax.Array,
    A_Lambda_im: jax.Array,
    A_B_re: jax.Array,
    A_B_im: jax.Array,
    A_C_re: jax.Array,
    A_C_im: jax.Array,
    A_log_dt: jax.Array,
    A_Dskip: jax.Array,
    B_q: jax.Array,
    B_k: jax.Array,
    B_v: jax.Array,
    B_shift_k: jax.Array,
    B_ssm_k: jax.Array,
    B_ssm_D: jax.Array,
):
    assert A_x.shape == (1, L, D) and B_shift_k.shape == (D, 4)
    vmem = pltpu.VMEM
    dma = pltpu.SemaphoreType.DMA
    scratch = [
        vmem(_TABLES.shape, F32),
        vmem((D,), BF16), vmem((D,), BF16), vmem((D,), BF16), vmem((D,), BF16), vmem((D,), BF16),
        vmem((4, D), BF16),
        vmem((NG * L, 128), BF16),
        vmem((2 * D, D), BF16),
        vmem((2 * NG * D, 128), BF16),
        vmem((NG * L, 128), BF16),
        vmem((NG * L, 128), BF16),
        vmem((NG * L, 128), BF16),
        vmem((D, L), BF16),
        vmem((NG * P_ROWS * 8, 128), F32),
        vmem((2 * NG * D + 32, 128), BF16),
        vmem((2 * NG * NG * 64 + 16, 128), I32),
        vmem((SLOTS * 128 + 32, 128), BF16),
        vmem((SLOTS * 64 + 16, 128), I32),
        vmem((2 * 2 * NG * BU_PART, 128), F32),
        vmem((2 * NG * L + 32, 128), BF16),
        vmem((3 * NG * 8, 128), F32),
        vmem((NG * YS_ROWS, 128), F32),
        vmem((L + 16, D), F32),
        vmem((L // 2 + 16, 128), I32),
        vmem((KF_PAD + L + 16, 128), F32),
        vmem((2 * L + 16, 128), F32),
        vmem((2 * L + 16, 128), F32),
        vmem((2 * L + 8, 128), F32),
        vmem((32 * 128 + 32, 128), BF16),
        vmem((32 * 128 + 32, 128), BF16),
        vmem((8 * 128, 128), BF16),
        vmem((8 * 128, 128), BF16),
        vmem((NG * L + 16, 128), F32),
        dma((S_END,)),
    ]
    out = pl.pallas_call(
        _kernel,
        out_shape=jax.ShapeDtypeStruct((L, 2 * D), F32),
        in_specs=[pl.BlockSpec(memory_space=pl.ANY)] * 16,
        out_specs=pl.BlockSpec(memory_space=pl.ANY),
        scratch_shapes=scratch,
        compiler_params=pltpu.CompilerParams(vmem_limit_bytes=100 * 1024 * 1024, flags=CFG["flags"], disable_semaphore_checks=CFG["nosem"]),
        name="s5_h3",
    )(_TABLES, A_x.reshape(L, D), A_Lambda_re, A_Lambda_im, A_B_re, A_B_im, A_C_re, A_C_im,
      A_log_dt, A_Dskip, B_q.reshape(L, D), B_k.reshape(L, D), B_v.reshape(L, D),
      B_shift_k.T, B_ssm_k, B_ssm_D)
    return out.reshape(1, L, 2 * D)
```

```python
import math

import jax
import jax.numpy as jnp
import numpy as np
from jax import lax
from jax.experimental import pallas as pl
from jax.experimental.pallas import tpu as pltpu

F32, BF16, I32 = jnp.float32, jnp.bfloat16, jnp.int32

L = 2048
D = 640
NG = D // 128
UNIT = 256
SEG = 16
R = UNIT // SEG
LEAD = 4
HALF = UNIT // 2
BU_PART = 9 * 2 * R
YS_ROWS = SEG * (R // 2 + 1)
KF_PAD = 8


class _Signed:
    def __init__(self, v, neg=False):
        self.v, self.neg = v, neg

    def __neg__(self):
        return _Signed(self.v, not self.neg)

    def __add__(self, o):
        if self.neg == o.neg:
            return _Signed(self.v + o.v, self.neg)
        return _Signed(o.v - self.v if self.neg else self.v - o.v)

    def __sub__(self, o):
        return self + (-o)

    def __mul__(self, c):
        return _Signed(self.v * np.float32(-c if self.neg else c))

    def get(self):
        return -self.v if self.neg else self.v


def _rot(re, im, num, den):
    num %= den
    h = math.sqrt(0.5)
    if num == 0:
        return re, im
    if 4 * num == den:
        return -im, re
    if 4 * num == 3 * den:
        return im, -re
    if 8 * num == den:
        return (re - im) * h, (re + im) * h
    if 8 * num == 3 * den:
        return (re + im) * (-h), (re - im) * h
    if 8 * num == 5 * den:
        return (im - re) * h, (re + im) * (-h)
    if 8 * num == 7 * den:
        return (re + im) * h, (im - re) * h
    c = math.cos(2 * math.pi * num / den)
    s = math.sin(2 * math.pi * num / den)
    return re * c - im * s, re * s + im * c


def _dft4(z, sign):
    (r0, i0), (r1, i1), (r2, i2), (r3, i3) = z
    ar, ai, br, bi = r0 + r2, i0 + i2, r0 - r2, i0 - i2
    cr, ci, dr, di = r1 + r3, i1 + i3, r1 - r3, i1 - i3
    plus, minus = (br - di, bi + dr), (br + di, bi - dr)
    if sign < 0:
        plus, minus = minus, plus
    return [(ar + cr, ai + ci), plus, (ar - cr, ai - ci), minus]


def _fwd1(n, u):
    a0, a1, b0, b1 = u
    p, q = _rot(a0, b0, n, 32), _rot(a1, b1, n + 4, 32)
    s0, s1 = a0 + b0, a1 + b1
    return [(p[0] + q[0], p[1] + q[1]), _rot(p[0] - q[0], p[1] - q[1], n, 8),
            _rot(a0 - b0, a1 - b1, n, 16), (s0 + s1, s0 - s1)]


def _fwd2(grp, z):
    if grp < 3:
        return _dft4(z, 1)
    s4 = [t[0] for t in z]
    d4 = [t[1] for t in z]
    p = (d4[0], d4[2])
    q = _rot(d4[1], d4[3], 1, 8)
    s5 = [s4[0] + s4[2], s4[1] + s4[3]]
    return [
        (s5[0] + s5[1], s5[0] - s5[1]),
        (s4[0] - s4[2], s4[1] - s4[3]),
        (p[0] + q[0], p[1] + q[1]),
        (p[0] - q[0], p[1] - q[1]),
    ]


def _inv2(grp, w):
    if grp < 3:
        return _dft4(w, -1)
    s5 = [w[0][0] + w[0][1], w[0][0] - w[0][1]]
    s4 = [s5[0] + w[1][0], s5[1] + w[1][1], s5[0] - w[1][0], s5[1] - w[1][1]]
    p = (w[2][0] + w[3][0], w[2][1] + w[3][1])
    q = _rot(w[2][0] - w[3][0], w[2][1] - w[3][1], -1, 8)
    d4 = [p[0], q[0], p[1], q[1]]
    return [(s4[n], d4[n]) for n in range(4)]


def _inv1(n, z):
    e = _rot(*z[1], -n, 8)
    p = _rot(z[0][0] + e[0], z[0][1] + e[1], -n, 32)
    q = _rot(z[0][0] - e[0], z[0][1] - e[1], -(n + 4), 32)
    d0, d1 = _rot(*z[2], -n, 16)
    s0, s1 = z[3][0] + z[3][1], z[3][0] - z[3][1]
    return [p[0] + (s0 + d0), q[0] + (s1 + d1), p[1] + (s0 - d0), q[1] + (s1 - d1)]


_F1 = [4 * (g + 2 * k) + 1 for g in range(2) for k in range(4)]
_F1 += [2 * (4 * k + 1) for k in range(4)] + [0, 8, 4, 20]
_REAL_SLOT = 12
SLOTS = len(_F1)


def _dft_tables():
    kap = np.arange(128)
    j = 8 * (kap // 16) + kap % 8
    part = (kap // 8) % 2
    pr, pc, jr, jc = part[:, None], part[None, :], j[:, None], j[None, :]
    lo = 2 * np.pi * jr * jc / 64
    base = np.where(pr == pc, np.cos(lo), np.where(pr == 0, -np.sin(lo), np.sin(lo)))
    hi = 2 * np.pi * (16 + 32 * (jr - 32)) * jc / 2048
    v0 = np.where(pr == 0, np.cos(lo), np.where(jr == 0, np.cos(np.pi * jc), np.sin(lo)))
    v32 = np.where(pr == 0, np.cos(hi), np.sin(hi))
    real = np.where(jr < 32, np.where(pc == 0, v0, 0.0), np.where(pc == 1, v32, 0.0))
    th = 2 * np.pi * np.outer(np.array(_F1), j) / 2048
    zeros = np.zeros((8, 128))
    return np.concatenate([base, real, np.cos(th), np.sin(th), zeros]).astype(np.float32)


_TABLES = _dft_tables()
_FFT_SCALE = 2.0 ** -10

(P_MU, P_RHO, P_RHO1, P_RHO2, P_RHO4, P_TAP, P_SSMD, P_DSKIP, P_COEF, P_ROWS) = (
    0, 2, 4, 6, 8, 10, 14, 15, 16, 20)
S_SMALL, S_F0, S_K0, S_C, S_OUT, S_X0, S_B = range(7)
S_COL = S_B + NG
S_END = S_COL + NG - 1


def _cmul(a, b):
    return a[0] * b[0] - a[1] * b[1], a[0] * b[1] + a[1] * b[0]


def _pack(lo, hi):
    return jnp.concatenate([lo, hi], axis=0).astype(BF16)


def _unpack_tile(w):
    return [_unpack(w[8 * i:8 * i + 8]) for i in range(w.shape[0] // 8)]


def _unpack(w):
    v = pltpu.bitcast(w, BF16).astype(F32)
    return v[:8], v[8:]


CFG = dict(scan=22, u=24, k1=0, p2=0, inv=44, skip=30, tail=3, kconv=4, steps=2, p2n=2,
           u0w=350, kwin=(100, 216), tr=(60, 90), wid=(216, 330), scanw=(0, 350), invw=(220, 380),
           k2w=(230, 480), mf=128, mi=128, ord=(2, 4), sk0=20, m0=[128, 128], sh1=None, sh2=None, when=(0, 1, 1, 2, 3, 4, 6), s2=380, retap=False, invend=290,
           Q=1, invsplit=False, kg=1, k0=1.0, u0=0.45, udir=True, kdir=True,
           flags=None, nosem=False, skipme=lambda n, rows: False)


class _Zeros:
    def __init__(self, v):
        self.v = v


class _Gate:
    def __init__(self, pred=None, seen=()):
        self.pred, self.seen = pred, seen

    def early(self, lag):
        old = [e for e in self.seen if e[0] <= -lag]
        return max(old, key=lambda e: e[0])[1] if lag and old else None

    def value(self, v, lag):
        early = self.early(lag)
        return v if early is None else jnp.where(self.pred, v, early)

    def loads(self, ref, lag):
        early = self.early(lag)
        if early is not None:
            ref[pl.ds(ref.shape[0] - 8, 8), :] = (
                early if ref.dtype == F32 else pltpu.bitcast(early, I32))


def _weave(passes, plan, pred):
    if CFG["skipme"](len(passes), sum(q[0] for q in passes)):
        return
    begin, clock = [], [0] * 4
    for i, (n, *_) in enumerate(passes):
        begin.append(clock[i % 4] / 16)
        clock[i % 4] += n

    def index(t):
        later = [i for i, b in enumerate(begin) if b >= t - 3.999]
        if not later:
            return len(passes)
        same = [i for i in later if begin[i] == min(begin[j] for j in later)]
        return same[min(max(int((t - begin[same[0]]) / 4 * len(same)), 0), len(same) - 1)]

    at = [[] for _ in range(len(passes) + 1)]
    for tasks, lo, hi in plan:
        total, done = sum(sum(c) for c, _ in tasks) or 1, 0.0
        for costs, fn in tasks:
            where = []
            for cost in costs:
                done += cost
                where.append(index(lo + done / total * (hi - lo)))
            at[min(where)].append((fn, where))
    seen, ties = [], [[] for _ in at]
    for i, fns in enumerate(at):
        now = (begin[i] + i % 4) if i < len(begin) else clock[0] / 16
        early = [(t - now, v) for t, v in seen if t % CFG["Q"] < 1 or CFG["Q"] == 1]
        for fn, where in fns:
            for w, tie in zip(where, fn(_Gate(pred, early)) or ()):
                ties[w].append(tie)
        if i == len(passes):
            break
        n, lhs, rhs, consume = passes[i]
        w = rhs()
        if not isinstance(w, list):
            d = lax.dot_general(pltpu.bitcast(jnp.concatenate(lhs(), axis=0), BF16), w,
                                (((1,), (1,)), ((), ())), preferred_element_type=F32)
            consume(d)
            continue
        for tie in ties[i]:
            if isinstance(tie, _Zeros):
                v = tie.v
                w[-1] = w[-1] | (v if v.dtype == I32 else pltpu.bitcast(v, I32))
            else:
                w[-1] = jnp.where(pred, w[-1], pltpu.bitcast(tie, I32))
        d = jnp.dot(pltpu.bitcast(jnp.concatenate(lhs(), axis=0), BF16),
                    pltpu.bitcast(jnp.concatenate(w, axis=0), BF16), preferred_element_type=F32)
        seen += [(begin[i] + i % 4 + j // 16 - 4, d[j - 8:j]) for j in range(64, n + 1, 64)]
        consume(d)


def _now(tasks):
    for _, fn in tasks:
        fn(_Gate())


def _kernel(tab_hbm, x_hbm, lre_hbm, lim_hbm, bre_hbm, bim_hbm, cre_hbm, cim_hbm,
            ldt_hbm, dsk_hbm, q_hbm, k_hbm, v_hbm, tap_hbm, sk_hbm, sd_hbm,
            o_hbm,
            tab, lre_v, lim_v, ldt_v, dsk_v, sd_v, tap_v,
            xb, braw, craw, qb, kb, vb, skb,
            par, wb16, wc, mf16, mi, bu, hb16, carry, ys, oa,
            kt, kf, st_u, st_k, st_i, vu16, vk16, pb0, pb1, ob,
            sem):
    x32, q32, k32, v32, wb, mf, hb, vu, vk = (
        r.bitcast(I32) for r in (xb, qb, kb, vb, wb16, mf16, hb16, vu16, vk16))
    c32 = craw.bitcast(I32)
    pb16 = (pb0, pb1)
    pb = (pb0.bitcast(I32), pb1.bitcast(I32))

    def rows(ref, start, n=8):
        return ref[pl.ds(start, n), :]

    def hint(v, n):
        return v if isinstance(v, int) or n == 1 else pl.multiple_of(v, n)

    def view(ref, start, n=None):
        return ref.at[pl.ds(hint(start, 16), n or ref.shape[0]), :]

    def after(ref):
        return _Zeros(view(ref, z8)[ref.shape[0] - 16:ref.shape[0] - 8, 0:128])

    small = [pltpu.make_async_copy(s, d, sem.at[S_SMALL]) for s, d in (
        (lre_hbm, lre_v), (lim_hbm, lim_v), (ldt_hbm, ldt_v),
        (dsk_hbm, dsk_v), (sd_hbm, sd_v), (tap_hbm, tap_v),
        (tab_hbm.at[pl.ds(288, 8), :], tab.at[pl.ds(288, 8), :]))]
    tab_dma = pltpu.make_async_copy(
        tab_hbm.at[pl.ds(0, 288), :], tab.at[pl.ds(0, 288), :], sem.at[S_B + 4])

    def x_dma(u):
        return [pltpu.make_async_copy(
            x_hbm.at[pl.ds(hint(u * UNIT, UNIT), UNIT), pl.ds(128 * n, 128)],
            xb.at[pl.ds(hint(n * L + u * UNIT, UNIT), UNIT), :], sem.at[(S_X0, S_B + 4, S_F0, S_K0)[u] if isinstance(u, int) and u < LEAD
                                                     else S_COL + u - LEAD])
            for n in range(NG)]

    def b_dma(p):
        return [pltpu.make_async_copy(
            src.at[pl.ds(128 * p, 128), :], braw.at[pl.ds(D * c + 128 * p, 128), :],
            sem.at[S_B + p]) for c, src in enumerate((bre_hbm, bim_hbm))]

    c_dma = [pltpu.make_async_copy(
        src.at[:, pl.ds(128 * p, 128)], craw.at[pl.ds(D * (NG * c + p), D), :],
        sem.at[S_C]) for c, src in enumerate((cre_hbm, cim_hbm)) for p in range(NG)]

    def col_dma(which, g, sem_at):
        src, dst = ((k_hbm, kb), (v_hbm, vb), (q_hbm, qb))[which]
        return pltpu.make_async_copy(
            src.at[:, pl.ds(hint(128 * g, 128), 128)],
            dst.at[pl.ds(hint(L * g, L), L), :], sem.at[sem_at])

    def sk_dma(g, sem_at):
        t = hint(128 * g, 128)
        return [pltpu.make_async_copy(
            sk_hbm.at[pl.ds(t, 128), :], skb.at[pl.ds(t, 128), :], sem.at[sem_at])]

    def oa_dma(u, n):
        t = hint(u * UNIT, UNIT)
        return pltpu.make_async_copy(
            oa.at[pl.ds(t, UNIT), pl.ds(128 * n, 128)],
            o_hbm.at[pl.ds(t, UNIT), pl.ds(128 * n, 128)], sem.at[S_OUT])

    def oa_unit_dma(u):
        t = hint(u * UNIT, UNIT)
        return pltpu.make_async_copy(
            oa.at[pl.ds(t, UNIT), :], o_hbm.at[pl.ds(t, UNIT), pl.ds(0, D)], sem.at[S_OUT])

    def ob_dma(g, half):
        h = L // 2
        return pltpu.make_async_copy(
            ob.at[pl.ds(hint(L * g + h * half, h), h), :],
            o_hbm.at[pl.ds(h * half, h), pl.ds(hint(D + 128 * g, 128), 128)], sem.at[S_OUT])

    def start(ds):
        for d in ds:
            d.start()

    def wait(ds):
        for d in ds:
            d.wait()

    def prm(g, row):
        return rows(view(par, g * (P_ROWS * 8), P_ROWS * 8), row * 8)

    def bu_passes(u, slot, z, shift):
        out = []
        xu, w = view(x32, u * (UNIT // 2), ((NG - 1) * L + UNIT) // 2), view(wb, z)
        order = [p + c * NG for p in range(NG) for c in range(2)]
        for n in order:
            sizes = [128, 128]
            if shift and n == order[0]:
                sizes = [32, 32, 96, 96]
            if shift and n == order[-1]:
                sizes = [96, 96, 32, 32] if shift is True else [64] * 4
            if shift is None:
                sizes = CFG["m0"] if u == 0 else [64] * 4
            for m, MM in zip(np.cumsum([0] + sizes).tolist(), sizes):
                acc = []
                for kk in range(NG):
                    def lhs(m=m, kk=kk, MM=MM):
                        t = (kk * L + m) // 2
                        return [rows(xu, t + 8 * i) for i in range(MM // 16)]

                    def rhs(n=n, kk=kk):
                        if u == 0 if isinstance(u, int) else False:
                            return braw[pl.ds(128 * n, 128), pl.ds(128 * kk, 128)]
                        return [rows(w, (n * NG + kk) * 64 + 8 * i) for i in range(8)]

                    def consume(d, m=m, n=n, kk=kk, acc=acc, MM=MM):
                        acc.append(d if kk == 0 else acc[-1] + d)
                        if kk == NG - 1:
                            for i in range(MM // 8):
                                seg, r = divmod(m + 8 * i, R)
                                row = 9 * (seg % 2 * R + r) + seg // 2
                                bu[pl.ds((slot * 2 * NG + n) * BU_PART + row, 8, stride=9), :] = (
                                    acc[-1][8 * i:8 * i + 8])
                    out.append((MM, lhs, rhs, consume))
        return out

    def scan_tasks(u, slot, z):
        steps = CFG["steps"]
        state = {}
        hu = view(hb16, u * UNIT, (2 * NG - 1) * L + UNIT)

        def b(p, ch, r):
            return tuple(rows(bu, (slot * 2 * NG + c * NG + p) * BU_PART + 9 * (ch * R + r))
                         for c in range(2))

        def step(mu, h, br):
            return (mu[0] * h[0] + br[0]) - mu[1] * h[1], (mu[0] * h[1] + br[1]) + mu[1] * h[0]

        def ends(p, gate):
            mu, ties = (gate.value(prm(p, P_MU), CFG["scan"]), prm(p, P_MU + 1)), []
            h = [b(p, ch, 0) for ch in range(2)]
            for r in range(1, R):
                h = [step(mu, h[ch], b(p, ch, r)) for ch in range(2)]
                if r % steps == 0:
                    ties.append(h[r // steps % 2][0])
            state[p] = starts(p, h)
            return ties + [state[p][1][0]]

        def starts(p, e):
            last = lax.broadcasted_iota(I32, (8, 128), 0) == 7
            rho = (prm(p, P_RHO), prm(p, P_RHO + 1))
            pair = step(rho, e[0], e[1])
            a = tuple(pltpu.roll(jnp.where(last, rows(carry, (2 * p + c) * 8), pair[c]), 1, 0)
                      for c in range(2))
            for sh, row in ((1, P_RHO1), (2, P_RHO2), (4, P_RHO4)):
                a = step((prm(p, row), prm(p, row + 1)), tuple(pltpu.roll(c, sh, 0) for c in a), a)
            return [a, step(rho, a, e[0])]

        def run(p, r0, gate):
            if r0 == 0:
                state["mu"] = (prm(p, P_MU), prm(p, P_MU + 1))
            mu, h = (gate.value(state["mu"][0], CFG["scan"]), state["mu"][1]), state[p]
            for r in range(r0, r0 + steps):
                h = [step(mu, h[ch], b(p, ch, r)) for ch in range(2)]
                for c in range(2):
                    hu[pl.ds((c * NG + p) * L + 16 * r, 16), :] = _pack(h[0][c], h[1][c])
            state[p] = h
            if r0 + steps == R:
                for c in range(2):
                    carry[pl.ds((2 * p + c) * 8, 8), :] = h[1][c]
            return [after(hb)]

        tasks = []
        for p in range(NG):
            tasks.append(([16 * steps] * ((R - 1) // steps) + [46 + 16 * steps],
                          lambda gate, p=p: ends(p, gate)))
            tasks += [([18 * steps], lambda gate, p=p, r0=r0: run(p, r0, gate))
                      for r0 in range(0, R, steps)]
        return tasks

    def y_passes(h, n, sizes=(HALF,), z=0):
        out, w, hu = [], view(wc, z), view(hb, h * (HALF // 2), ((2 * NG - 1) * L + HALF) // 2)
        for t0, MM in zip(np.cumsum((0,) + sizes).tolist(), sizes):
            acc = []
            for kk in range(2 * NG):
                def lhs(t0=t0, kk=kk, MM=MM):
                    return [rows(hu, (kk * L + t0) // 2 + 8 * i) for i in range(MM // 16)]

                def rhs(kk=kk):
                    return [rows(w, (kk * NG + n) * 64 + 8 * i) for i in range(8)]

                def consume(d, t0=t0, kk=kk, acc=acc, MM=MM):
                    acc.append(d if kk == 0 else acc[-1] + d)
                    if kk == 2 * NG - 1:
                        for i in range(MM // 8):
                            r, ch = divmod(t0 // 8 + i, 2)
                            ys[pl.ds(n * YS_ROWS + ch * (R // 2 + 1) + r, 8, stride=R + 2), :] = (
                                acc[-1][8 * i:8 * i + 8])
                out.append((MM, lhs, rhs, consume))
        return out

    def skip_task(h, n):
        def fn(gate):
            dsk, ties = gate.value(prm(n, P_DSKIP), CFG["skip"]), []
            t = h // 2 * UNIT + h % 2 * (R // 2)
            xu = x32.at[pl.ds(hint(t // 2 + n * (L // 2), 4), UNIT // 2 - 4 + 8 * (n < NG - 1 or not isinstance(h, int))), :]
            ou = oa.at[pl.ds(hint(t, 8), UNIT - R // 2), :]
            for g in range(SEG):
                if g == SEG - 1 and n == NG - 1 and isinstance(h, int):
                    xs = _unpack(rows(xu, 8 * g - 4))[1]
                else:
                    xs = _unpack(rows(xu, 8 * g))[0]
                y = rows(ys, n * YS_ROWS + g * (R // 2 + 1))
                ou[pl.ds(R * g, 8), pl.ds(128 * n, 128)] = y + xs * dsk
                if g % 8 == 7:
                    ties.append(after(oa))
            return ties
        return ([24, 24], fn)

    def widen_tasks(g, z, pieces=2):
        def fn(i0, i1):
            kg = view(k32, g * (L // 2), L // 2)
            for i in range(i0, i1):
                lo, hi = _unpack(rows(kg, 8 * i))
                kf[pl.ds(KF_PAD + 16 * i, 8), :] = lo
                kf[pl.ds(KF_PAD + 16 * i + 8, 8), :] = hi
            return [after(kf)]
        n = L // 16 // pieces
        return [([2 * n], lambda gate, i=i: fn(i * n, (i + 1) * n)) for i in range(pieces)]

    def transpose_tasks(g, z, pieces=8):
        def fn(c0, c1):
            for c in range(c0, c1):
                t = skb[pl.ds(hint(128 * g, 128), 128), pl.ds(128 * c, 128)]
                kt[pl.ds(64 * c, 64), :] = pltpu.bitcast(t.T, I32)
            return [after(kt)]
        n = L // 128 // pieces
        return [([8 * n], lambda gate, i=i: fn(i * n, (i + 1) * n)) for i in range(pieces)]

    def staged(s, half, n, grp, c):
        return (((s * 2 + half) * 4 + n) * 4 + grp) * 16 + 8 * c

    ops1 = (18, 36, 30, 36)

    def forward_tasks_of(st, s, half, z, chunk, chunk_cost, direct):
        dst16, dst = (vu16, vu) if st is st_u else (vk16, vk)

        def second(grp, zs):
            for k, pair in enumerate(_fwd2(grp, zs)):
                dst16[pl.ds(((4 * grp + k) * 2 + half) * 128 + 16 * s, 16), :] = (
                    _pack(pair[0].get(), pair[1].get()))
            return after(dst)

        kept = []

        def first(gate, n):
            load = chunk(gate, n)
            u = [load(16 * half + n + 4 * m) for m in range(4)]
            pairs = _fwd1(n, [_Signed(v) for v in u])
            kept.append(pairs)
            for grp in range(2 * direct, 4):
                for c in range(2):
                    st[pl.ds(staged(s, half, n, grp, c), 8), :] = pairs[grp][c].get()
            return [u[0] + u[2]] * (chunk_cost > 4) + [after(st)]

        def rest(grp):
            if direct and grp < 2:
                return [second(grp, [t[grp] for t in kept])]
            return [second(grp, [tuple(_Signed(rows(view(st, z), staged(s, half, n, grp, c)))
                                       for c in range(2)) for n in range(4)])]

        split = (chunk_cost > 4) * (chunk_cost // 2 + 1)
        one = [([split] * (split > 0) + [chunk_cost + ops1[n] - split], lambda gate, n=n: first(gate, n))
               for n in range(4)]
        if CFG["p2n"] == 4:
            two = [([20], lambda gate, grp=grp: rest(grp)) for grp in range(4)]
        else:
            two = [([40], lambda gate, grp=grp: rest(grp) and rest(grp + 1)) for grp in (0, 2)]
        h = len(two) // 2
        return (one + two[:h], two[h:]) if direct else (one, two)

    def u_tasks(g, s, half, z):
        loaded = []

        def chunk(gate, n):
            if n == 0 or CFG["retap"]:
                loaded[:] = [prm(g, P_TAP + t) for t in range(4)]
            taps = [gate.value(loaded[0], CFG["u"])] + loaded[1:]
            kz, vg = view(kf, z), view(v32, g * (L // 2), L // 2)

            def load(c):
                t = 64 * c + 8 * s
                ks = rows(kz, KF_PAD + t) * taps[0]
                for lag in range(1, 4):
                    ks = ks + rows(kz, KF_PAD + t - lag) * taps[lag]
                return ks * _unpack(rows(vg, (t // 16) * 8))[s % 2]
            return load
        return forward_tasks_of(st_u, s, half, z, chunk, 36, CFG["udir"])

    def k_tasks(g, s, half, z, direct):
        def chunk(gate, n):
            if n % CFG["kg"] == 0:
                gate.loads(kt, CFG["k1"])

            def load(c):
                v = _unpack(rows(view(kt, z), 32 * c + 8 * (s // 2)))[s % 2]
                if s == 0 and c == 0:
                    first = lax.broadcasted_iota(I32, (8, 128), 0) == 0
                    v = v + jnp.where(first, prm(g, P_SSMD), 0.0)
                return v
            return load
        return forward_tasks_of(st_k, s, half, z, chunk, 4, direct)

    def fwd_passes(grp, z):
        out, MM = [], CFG["mf"]
        for slot in range(4 * grp, 4 * grp + 4):
            for part in range(128 // MM):
                got = []
                for src, half in ((vu, 0), (vk, 0), (vu, 1), (vk, 1)):
                    def lhs(slot=slot, part=part):
                        return [rows(mf, slot * 64 + MM // 2 * part + 8 * i) for i in range(MM // 16)]

                    def rhs(slot=slot, src=src, half=half):
                        return [rows(view(src, z), (2 * slot + half) * 64 + 8 * i) for i in range(8)]

                    def consume(d, slot=slot, part=part, got=got):
                        got.append(d)
                        if len(got) < 4:
                            return
                        for i in range(MM // 16):
                            u0, k0, u1, k1 = ((t[16 * i:16 * i + 8], t[16 * i + 8:16 * i + 16]) for t in got)
                            lo, a, b = _cmul(u0, k0), _cmul(u0, k1), _cmul(u1, k0)
                            if slot == _REAL_SLOT and part == 0 and i == 0:
                                first = lax.broadcasted_iota(I32, (8, 128), 0) == 0
                                lo, a, b = (tuple(jnp.where(first, 0.5 * (x[c] * y[c]), p[c]) for c in range(2))
                                            for p, x, y in ((lo, u0, k0), (a, u0, k1), (b, u1, k0)))
                            if _F1[slot] % 2:
                                hi = ((a[0] + b[0]) - lo[0], (a[1] + b[1]) - lo[1])
                            else:
                                hi = ((a[0] + b[0]) + lo[0], (a[1] + b[1]) + lo[1])
                            for half, p in enumerate((lo, hi)):
                                at = (slot % 4 * 2 + half) * 128 + MM * part + 16 * i
                                pb16[grp % 2][pl.ds(at, 16), :] = _pack(*p)
                    out.append((MM, lhs, rhs, consume))
        return out

    def inv_passes(grp, half, z):
        out, MM = [], CFG["mi"]
        for part in range(128 // MM):
            got = []
            for slot in range(4 * grp, 4 * grp + 4):
                def lhs(slot=slot, part=part):
                    return [rows(mi, slot * 64 + MM // 2 * part + 8 * i) for i in range(MM // 16)]

                def rhs(slot=slot):
                    return [rows(view(pb[grp % 2], z), (slot % 4 * 2 + half) * 64 + 8 * i)
                            for i in range(8)]

                def consume(d, part=part, got=got):
                    got.append(d)
                    if len(got) < 4:
                        return
                    for i in range(MM // 16):
                        w = [(_Signed(t[16 * i:16 * i + 8]), _Signed(t[16 * i + 8:16 * i + 16]))
                             for t in got]
                        for n, pair in enumerate(_inv2(grp, w)):
                            for c in range(2):
                                at = staged(MM // 16 * part + i, half, n, grp, c)
                                st_i[pl.ds(at, 8), :] = pair[c].get()
                out.append((MM, lhs, rhs, consume))
        return out

    def inv1_task(g, s, half, z):
        def fn(gate, ns):
            gate.loads(st_i, CFG["inv"])
            qg, og, ties = view(q32, g * (L // 2), L // 2), view(ob, g * L, L), []
            for n in ns:
                zs = [tuple(_Signed(rows(view(st_i, z), staged(s, half, n, grp, c))) for c in range(2))
                      for grp in range(4)]
                for m, y in enumerate(_inv1(n, zs)):
                    t = 64 * (16 * half + n + 4 * m) + 8 * s
                    og[pl.ds(t, 8), :] = _unpack(rows(qg, (t // 16) * 8))[s % 2] * y.get()
                ties.append(after(ob))
            return ties
        if CFG["invsplit"]:
            return [([12 + ops1[n]], lambda gate, n=n: fn(gate, [n])) for n in range(4)]
        return [([12 + n for n in ops1], lambda gate: fn(gate, range(4)))]

    filter0 = x_dma(2) + sk_dma(0, S_F0)
    data0 = x_dma(3) + [col_dma(0, 0, S_K0), col_dma(1, 0, S_K0)]

    def group_dma(g):
        at = S_COL + g
        return ([col_dma(2, g, at)] + sk_dma(g + 1, at)
                + [col_dma(0, g + 1, at), col_dma(1, g + 1, at)] + x_dma(g + LEAD))

    last_dma = col_dma(2, NG - 1, S_SMALL)

    start(small + b_dma(0) + x_dma(0) + b_dma(1) + b_dma(2))
    wait(small)
    zeros = rows(tab, 288).astype(I32)
    z8 = pl.multiple_of(zeros[0, 0], 16)
    sub = lax.broadcasted_iota(I32, (8, 128), 0)
    pred = zeros == 0

    def stack(ref):
        v = ref[...].astype(F32).reshape(1, D)
        return jnp.concatenate([v[:, 128 * g:128 * (g + 1)] for g in range(NG)]
                               + [v[:, :128]] * (8 - NG), axis=0)

    lre, lim = stack(lre_v), stack(lim_v)
    dt = jnp.exp(stack(ldt_v)).astype(BF16).astype(F32)
    mag, ang = jnp.exp(dt * lre), dt * lim
    lam = (mag * jnp.cos(ang), mag * jnp.sin(ang))
    scale = jnp.maximum(jnp.abs(lre), jnp.abs(lim))
    nre, nim = lre / scale, lim / scale
    den = (nre * nre + nim * nim) * scale
    coef = _cmul(((lam[0] - 1.0) / den, lam[1] / den), (nre, -nim))
    mu = lam
    rho = [mu]
    for _ in range(R.bit_length() + 2):
        rho.append(_cmul(rho[-1], rho[-1]))
    dsk, ssd = stack(dsk_v), stack(sd_v)
    taps = tap_v[...].astype(F32) * _FFT_SCALE
    for g in range(NG):
        def put(row, v):
            par[pl.ds((g * P_ROWS + row) * 8, 8), :] = v

        def lanes(v):
            return jnp.broadcast_to(v[g:g + 1], (8, 128))
        for c in range(2):
            put(P_MU + c, lanes(mu[c]))
            put(P_RHO + c, lanes(rho[-4][c]))
            for n, row in enumerate((P_RHO1, P_RHO2, P_RHO4)):
                put(row + c, jnp.where(sub >= 1 << n, lanes(rho[n - 3][c]), 0.0))
        for t in range(4):
            put(P_TAP + t, jnp.broadcast_to(taps[t:t + 1, 128 * g:128 * (g + 1)], (8, 128)))
        put(P_COEF, lanes(2.0 * coef[0]))
        put(P_COEF + 2, lanes(-2.0 * coef[1]))
        put(P_SSMD, lanes(ssd))
        put(P_DSKIP, lanes(dsk))
    for ref in (hb, oa, kf, kt, vu, vk, st_u, st_k, ob, mf, mi, wb, wc):
        ref[pl.ds(ref.shape[0] - 16, 8), pl.ds(0, 128)] = jnp.zeros((8, 128), ref.dtype)
    for i in range(2 * NG):
        carry[pl.ds(8 * i, 8), :] = jnp.zeros((8, 128), F32)
    kf[pl.ds(0, KF_PAD), :] = jnp.zeros((KF_PAD, 128), F32)

    def matrix_task(slot):
        def fn(gate):
            if slot != _REAL_SLOT:
                c, s = tab[pl.ds(256 + slot, 1), :], tab[pl.ds(272 + slot, 1), :]
            for a in range(8):
                if slot == _REAL_SLOT:
                    re, im = rows(tab, 128 + 16 * a), rows(tab, 128 + 16 * a + 8)
                else:
                    br, bi = rows(tab, 16 * a), rows(tab, 16 * a + 8)
                    re, im = c * br - s * bi, s * br + c * bi
                mf16[pl.ds(slot * 128 + 16 * a, 16), :] = _pack(re, im)
            m = pltpu.bitcast(rows(view(mf, z8), slot * 64, 64), BF16)
            mi[pl.ds(slot * 64, 64), :] = pltpu.bitcast(m.T, I32)
            return [after(mf), after(mi)]
        return ([48, 8], fn)

    def b_task(p):
        def fn(gate):
            ties = []
            for n in (p, NG + p):
                for kk in range(NG):
                    t = braw[pl.ds(128 * n, 128), pl.ds(128 * kk, 128)]
                    wb[pl.ds((n * NG + kk) * 64, 64), :] = pltpu.bitcast(t.T, I32)
                    ties.append(after(wb))
            return ties
        return ([24] * (2 * NG), fn)

    def c_task(n, p):
        def fn(gate):
            cr, ci, nci = prm(p, P_COEF), prm(p, P_COEF + 1), prm(p, P_COEF + 2)
            t = [_unpack_tile(rows(c32, ((c * NG + p) * D + 128 * n) // 2, 64)) for c in range(2)]
            re = [_pack(cr * a0 + nci * b0, cr * a1 + nci * b1) for (a0, a1), (b0, b1) in zip(*t)]
            im = [_pack(nci * a0 - cr * b0, nci * a1 - cr * b1) for (a0, a1), (b0, b1) in zip(*t)]
            ties = []
            for c, tile in enumerate((re, im)):
                wc[pl.ds(((c * NG + p) * NG + n) * 64, 64), :] = pltpu.bitcast(
                    jnp.concatenate(tile, axis=0).T, I32)
                ties.append(after(wc))
            return ties
        return ([80, 80], fn)

    first = bu_passes(0, 1, z8, None)
    first = [first[len(first) // NG * p:len(first) // NG * (p + 1)] for p in range(NG)]

    mats = [matrix_task(slot) for slot in range(SLOTS)]

    def dma_task(ds):
        return ([1], lambda gate: start(ds))

    def filter_tasks(g, early):
        ts = [k_tasks(g, j // 2, j % 2, z8, j >= early and CFG["kdir"]) for j in range(16)]
        return (transpose_tasks(g, z8), [q for t in ts[:early] for q in t[0]],
                [q for t in ts[:early] for q in t[1]] + [q for t in ts[early:] for q in t[0] + t[1]])

    def forward_tasks(g):
        return [t for s in range(8) for half in range(2) for t in sum(u_tasks(g, s, half, z8), [])]

    def y_block(halves, t0, z=0, lead=True, even=None):
        tiles = [(h, n) for h in halves for n in range(NG)]
        passes, plan = [], []
        for j, (h, n) in enumerate(tiles):
            sizes = (HALF,)
            if j == 0 and lead is not None:
                if not lead:
                    continue
                sizes = (32, 96)
            if j == even:
                sizes = (64, 64)
            if j == len(tiles) - 1:
                sizes = (96, 32)
            passes += y_passes(h, n, sizes, z)
            t0 += 20
            plan.append(([skip_task(h, n)], t0 + CFG["sk0"], t0 + CFG["sk0"] + 6))
        return passes, plan

    total = 2 * NG * NG * UNIT // 64

    def early(at):
        for when, ds in zip(CFG["when"], (filter0, data0, c_dma, group_dma(0), group_dma(1), group_dma(2),
                                          group_dma(3) + [last_dma])):
            if when == at:
                start(ds)

    start(b_dma(3) + b_dma(4) + x_dma(1) + [tab_dma])
    wait(x_dma(0) + b_dma(0))
    _weave(first[0], [], pred)
    early(0)
    wait(b_dma(1))
    _weave(first[1], [], pred)
    early(1)
    wait(b_dma(2) + b_dma(3))
    _weave(first[2] + first[3], [([b_task(p) for p in range(4)], 0, 80)], pred)
    early(2)
    wait(b_dma(4) + x_dma(1) + [tab_dma])
    _weave(first[4] + bu_passes(1, 0, z8, CFG["sh1"]), [
        ([b_task(4)], 0, 36),
        (scan_tasks(0, 1, z8), 40, 40 + total), (mats, 60, 200)], pred)
    early(3)
    wait(filter0)
    tr, _, k1 = filter_tasks(0, 0)
    nk, fwd = int(CFG["k0"] * len(k1)), forward_tasks(0)
    nu = int(CFG["u0"] * len(fwd))
    _weave(bu_passes(2, 1, 0, CFG["sh2"]), [
        (scan_tasks(1, 0, z8), 0, total), (tr, 8, 32), (k1[:nk], 36, total)], pred)
    early(4)
    wait(data0 + c_dma)
    cs = [c_task(n, p) for n in range(NG) for p in range(NG)]
    yp, plan = y_block((0, 1), total, z8, lead=None, even=2)
    _weave(bu_passes(3, 0, 0, "open") + yp, plan + [
        (scan_tasks(2, 1, z8), 0, CFG["s2"]), (k1[nk:], 0, total), (widen_tasks(0, z8, 16), 0, 40),
        (cs[:2 * NG], 0, total - 16), (cs[2 * NG:], total - 100, total + 16), (fwd[:-2], 40, 2 * total), (fwd[-2:], 2 * total, 2 * total)], pred)
    start([oa_unit_dma(0)])
    early(6)

    def conv_passes():
        passes = fwd_passes(0, z8)
        for grp in range(1, 4):
            f, n = fwd_passes(grp, z8), 4 * 128 // CFG["mf"]
            a, b = (n * j for j in CFG["ord"])
            passes += f[:a] + inv_passes(grp - 1, 0, z8) + f[a:b] + inv_passes(grp - 1, 1, z8) + f[b:]
        return passes

    def inverse_tasks(g):
        tasks = []
        for half in range(2):
            for s in range(8):
                tasks += inv1_task(g, s, half, z8)
            tasks.append(dma_task([ob_dma(g, half)]))
        return tasks

    def body(i, _):
        wait(group_dma(i))
        halves = [2 + 3 * i + j for j in range(3)]
        lead = y_passes(halves[0], 0, (32, 96))
        y0 = 192 + 20 + total
        yp, plan = y_block(halves, y0, lead=False, even=7)
        passes = (conv_passes() + lead[:8] + inv_passes(3, 0, z8) + inv_passes(3, 1, z8) + lead[8:]
                  + bu_passes(i + LEAD, 0, 0, False) + yp)
        tr, k1, k2 = filter_tasks(i + 1, CFG["kconv"])
        fwd, tail, end = forward_tasks(i + 1), CFG["tail"], y0 + 280
        done = (3 * i + 2) // 2
        _weave(passes, plan + [
            ([dma_task([oa_unit_dma(done)])], y0 + 210, y0 + 210),
            (scan_tasks(i + LEAD - 1, 0, z8), *CFG["scanw"]), (tr, *CFG["tr"]),
            ([skip_task(halves[0], 0)], 232, 238),
            (widen_tasks(i + 1, z8, 16), *CFG["wid"]), (k1, *CFG["kwin"]),
            (inverse_tasks(i), *CFG["invw"]), (k2, *CFG["k2w"]),
            (fwd[:-tail], CFG["u0w"], end), (fwd[-tail:], end, end)], pred)
        pl.when(i % 2 == 1)(lambda: start([oa_unit_dma(done + 1)]))
        return 0

    lax.fori_loop(0, NG - 1, body, 0)

    wait([last_dma])
    g, last = NG - 1, L // UNIT - 1
    yp, plan = y_block((2 * last, 2 * last + 1), 192, even=2)
    ends = [[dma_task([oa_dma(last, n)])] for n in range(NG)]
    plan += [(ends[n], t + 6, t + 6) for n, (_, _, t) in enumerate(plan[NG:])]
    _weave(conv_passes() + yp[:8] + inv_passes(3, 0, z8) + inv_passes(3, 1, z8) + yp[8:], plan + [
        (scan_tasks(last, 0, z8), 0, 170),
        (inverse_tasks(g), 216, CFG["invend"])], pred)
    wait([oa_unit_dma(u) for u in range(last)] + [oa_dma(last, n) for n in range(NG)]
         + [ob_dma(n, half) for n in range(NG) for half in range(2)])


@jax.jit
def pallas_concat_heads__ssm_conv_s5__ssm_conv_h3__prompt_kernel(
    A_x: jax.Array,
    A_Lambda_re: jax.Array,
    A_Lambda_im: jax.Array,
    A_B_re: jax.Array,
    A_B_im: jax.Array,
    A_C_re: jax.Array,
    A_C_im: jax.Array,
    A_log_dt: jax.Array,
    A_Dskip: jax.Array,
    B_q: jax.Array,
    B_k: jax.Array,
    B_v: jax.Array,
    B_shift_k: jax.Array,
    B_ssm_k: jax.Array,
    B_ssm_D: jax.Array,
):
    assert A_x.shape == (1, L, D) and B_shift_k.shape == (D, 4)
    vmem = pltpu.VMEM
    dma = pltpu.SemaphoreType.DMA
    scratch = [
        vmem(_TABLES.shape, F32),
        vmem((D,), BF16), vmem((D,), BF16), vmem((D,), BF16), vmem((D,), BF16), vmem((D,), BF16),
        vmem((4, D), BF16),
        vmem((NG * L, 128), BF16),
        vmem((2 * D, D), BF16),
        vmem((2 * NG * D, 128), BF16),
        vmem((NG * L, 128), BF16),
        vmem((NG * L, 128), BF16),
        vmem((NG * L, 128), BF16),
        vmem((D, L), BF16),
        vmem((NG * P_ROWS * 8, 128), F32),
        vmem((2 * NG * D + 32, 128), BF16),
        vmem((2 * NG * NG * 64 + 16, 128), I32),
        vmem((SLOTS * 128 + 32, 128), BF16),
        vmem((SLOTS * 64 + 16, 128), I32),
        vmem((2 * 2 * NG * BU_PART, 128), F32),
        vmem((2 * NG * L + 32, 128), BF16),
        vmem((3 * NG * 8, 128), F32),
        vmem((NG * YS_ROWS, 128), F32),
        vmem((L + 16, D), F32),
        vmem((L // 2 + 16, 128), I32),
        vmem((KF_PAD + L + 16, 128), F32),
        vmem((2 * L + 16, 128), F32),
        vmem((2 * L + 16, 128), F32),
        vmem((2 * L + 8, 128), F32),
        vmem((32 * 128 + 32, 128), BF16),
        vmem((32 * 128 + 32, 128), BF16),
        vmem((8 * 128, 128), BF16),
        vmem((8 * 128, 128), BF16),
        vmem((NG * L + 16, 128), F32),
        dma((S_END,)),
    ]
    out = pl.pallas_call(
        _kernel,
        out_shape=jax.ShapeDtypeStruct((L, 2 * D), F32),
        in_specs=[pl.BlockSpec(memory_space=pl.ANY)] * 16,
        out_specs=pl.BlockSpec(memory_space=pl.ANY),
        scratch_shapes=scratch,
        compiler_params=pltpu.CompilerParams(vmem_limit_bytes=100 * 1024 * 1024, flags=CFG["flags"], disable_semaphore_checks=CFG["nosem"]),
        name="s5_h3",
    )(_TABLES, A_x.reshape(L, D), A_Lambda_re, A_Lambda_im, A_B_re, A_B_im, A_C_re, A_C_im,
      A_log_dt, A_Dskip, B_q.reshape(L, D), B_k.reshape(L, D), B_v.reshape(L, D),
      B_shift_k.T, B_ssm_k, B_ssm_D)
    return out.reshape(1, L, 2 * D)
```

```python
import math

import jax
import jax.numpy as jnp
import numpy as np
from jax import lax
from jax.experimental import pallas as pl
from jax.experimental.pallas import tpu as pltpu

F32, BF16, I32 = jnp.float32, jnp.bfloat16, jnp.int32

L = 2048
D = 640
NG = D // 128
UNIT = 256
SEG = 16
R = UNIT // SEG
LEAD = 4
HALF = UNIT // 2
BU_PART = 9 * 2 * R
YS_ROWS = SEG * (R // 2 + 1)
KF_PAD = 8


class _Signed:
    def __init__(self, v, neg=False):
        self.v, self.neg = v, neg

    def __neg__(self):
        return _Signed(self.v, not self.neg)

    def __add__(self, o):
        if self.neg == o.neg:
            return _Signed(self.v + o.v, self.neg)
        return _Signed(o.v - self.v if self.neg else self.v - o.v)

    def __sub__(self, o):
        return self + (-o)

    def __mul__(self, c):
        return _Signed(self.v * np.float32(-c if self.neg else c))

    def get(self):
        return -self.v if self.neg else self.v


def _rot(re, im, num, den):
    num %= den
    h = math.sqrt(0.5)
    if num == 0:
        return re, im
    if 4 * num == den:
        return -im, re
    if 4 * num == 3 * den:
        return im, -re
    if 8 * num == den:
        return (re - im) * h, (re + im) * h
    if 8 * num == 3 * den:
        return (re + im) * (-h), (re - im) * h
    if 8 * num == 5 * den:
        return (im - re) * h, (re + im) * (-h)
    if 8 * num == 7 * den:
        return (re + im) * h, (im - re) * h
    c = math.cos(2 * math.pi * num / den)
    s = math.sin(2 * math.pi * num / den)
    return re * c - im * s, re * s + im * c


def _dft4(z, sign):
    (r0, i0), (r1, i1), (r2, i2), (r3, i3) = z
    ar, ai, br, bi = r0 + r2, i0 + i2, r0 - r2, i0 - i2
    cr, ci, dr, di = r1 + r3, i1 + i3, r1 - r3, i1 - i3
    plus, minus = (br - di, bi + dr), (br + di, bi - dr)
    if sign < 0:
        plus, minus = minus, plus
    return [(ar + cr, ai + ci), plus, (ar - cr, ai - ci), minus]


def _fwd1(n, u):
    a0, a1, b0, b1 = u
    p, q = _rot(a0, b0, n, 32), _rot(a1, b1, n + 4, 32)
    s0, s1 = a0 + b0, a1 + b1
    return [(p[0] + q[0], p[1] + q[1]), _rot(p[0] - q[0], p[1] - q[1], n, 8),
            _rot(a0 - b0, a1 - b1, n, 16), (s0 + s1, s0 - s1)]


def _fwd2(grp, z):
    if grp < 3:
        return _dft4(z, 1)
    s4 = [t[0] for t in z]
    d4 = [t[1] for t in z]
    p = (d4[0], d4[2])
    q = _rot(d4[1], d4[3], 1, 8)
    s5 = [s4[0] + s4[2], s4[1] + s4[3]]
    return [
        (s5[0] + s5[1], s5[0] - s5[1]),
        (s4[0] - s4[2], s4[1] - s4[3]),
        (p[0] + q[0], p[1] + q[1]),
        (p[0] - q[0], p[1] - q[1]),
    ]


def _inv2(grp, w):
    if grp < 3:
        return _dft4(w, -1)
    s5 = [w[0][0] + w[0][1], w[0][0] - w[0][1]]
    s4 = [s5[0] + w[1][0], s5[1] + w[1][1], s5[0] - w[1][0], s5[1] - w[1][1]]
    p = (w[2][0] + w[3][0], w[2][1] + w[3][1])
    q = _rot(w[2][0] - w[3][0], w[2][1] - w[3][1], -1, 8)
    d4 = [p[0], q[0], p[1], q[1]]
    return [(s4[n], d4[n]) for n in range(4)]


def _inv1(n, z):
    e = _rot(*z[1], -n, 8)
    p = _rot(z[0][0] + e[0], z[0][1] + e[1], -n, 32)
    q = _rot(z[0][0] - e[0], z[0][1] - e[1], -(n + 4), 32)
    d0, d1 = _rot(*z[2], -n, 16)
    s0, s1 = z[3][0] + z[3][1], z[3][0] - z[3][1]
    return [p[0] + (s0 + d0), q[0] + (s1 + d1), p[1] + (s0 - d0), q[1] + (s1 - d1)]


_F1 = [4 * (g + 2 * k) + 1 for g in range(2) for k in range(4)]
_F1 += [2 * (4 * k + 1) for k in range(4)] + [0, 8, 4, 20]
_REAL_SLOT = 12
SLOTS = len(_F1)


def _dft_tables():
    kap = np.arange(128)
    j = 8 * (kap // 16) + kap % 8
    part = (kap // 8) % 2
    pr, pc, jr, jc = part[:, None], part[None, :], j[:, None], j[None, :]
    lo = 2 * np.pi * jr * jc / 64
    base = np.where(pr == pc, np.cos(lo), np.where(pr == 0, -np.sin(lo), np.sin(lo)))
    hi = 2 * np.pi * (16 + 32 * (jr - 32)) * jc / 2048
    v0 = np.where(pr == 0, np.cos(lo), np.where(jr == 0, np.cos(np.pi * jc), np.sin(lo)))
    v32 = np.where(pr == 0, np.cos(hi), np.sin(hi))
    real = np.where(jr < 32, np.where(pc == 0, v0, 0.0), np.where(pc == 1, v32, 0.0))
    th = 2 * np.pi * np.outer(np.array(_F1), j) / 2048
    zeros = np.zeros((8, 128))
    return np.concatenate([base, real, np.cos(th), np.sin(th), zeros]).astype(np.float32)


_TABLES = _dft_tables()
_FFT_SCALE = 2.0 ** -10

(P_MU, P_RHO, P_RHO1, P_RHO2, P_RHO4, P_TAP, P_SSMD, P_DSKIP, P_COEF, P_ROWS) = (
    0, 2, 4, 6, 8, 10, 14, 15, 16, 20)
S_SMALL, S_F0, S_K0, S_C, S_OUT, S_X0, S_B = range(7)
S_COL = S_B + NG
S_END = S_COL + NG - 1


def _cmul(a, b):
    return a[0] * b[0] - a[1] * b[1], a[0] * b[1] + a[1] * b[0]


def _pack(lo, hi):
    return jnp.concatenate([lo, hi], axis=0).astype(BF16)


def _unpack_tile(w):
    return [_unpack(w[8 * i:8 * i + 8]) for i in range(w.shape[0] // 8)]


def _unpack(w):
    v = pltpu.bitcast(w, BF16).astype(F32)
    return v[:8], v[8:]


CFG = dict(scan=22, u=24, k1=0, p2=0, inv=44, skip=30, tail=3, kconv=4, steps=2, p2n=2,
           u0w=350, kwin=(100, 216), tr=(60, 90), wid=(216, 330), scanw=(0, 350), invw=(220, 380),
           k2w=(230, 480), mf=128, mi=128, ord=(2, 4), sk0=20, ct=2, cw=(30, 260), f0=120, m0=[128, 128], sh1=None, sh2=None, when=(0, 1, 1, 2, 3, 4, 6), s2=(0, 390), retap=False, invend=290,
           Q=1, invsplit=False, kg=1, k0=1.0, u0=0.45, udir=True, kdir=True,
           flags=None, nosem=False, skipme=lambda n, rows: False)


class _Zeros:
    def __init__(self, v):
        self.v = v


class _Gate:
    def __init__(self, pred=None, seen=()):
        self.pred, self.seen = pred, seen

    def early(self, lag):
        old = [e for e in self.seen if e[0] <= -lag]
        return max(old, key=lambda e: e[0])[1] if lag and old else None

    def value(self, v, lag):
        early = self.early(lag)
        return v if early is None else jnp.where(self.pred, v, early)

    def loads(self, ref, lag):
        early = self.early(lag)
        if early is not None:
            ref[pl.ds(ref.shape[0] - 8, 8), :] = (
                early if ref.dtype == F32 else pltpu.bitcast(early, I32))


def _weave(passes, plan, pred):
    if CFG["skipme"](len(passes), sum(q[0] for q in passes)):
        return
    begin, clock = [], [0] * 4
    for i, (n, *_) in enumerate(passes):
        begin.append(clock[i % 4] / 16)
        clock[i % 4] += n

    def index(t):
        later = [i for i, b in enumerate(begin) if b >= t - 3.999]
        if not later:
            return len(passes)
        same = [i for i in later if begin[i] == min(begin[j] for j in later)]
        return same[min(max(int((t - begin[same[0]]) / 4 * len(same)), 0), len(same) - 1)]

    at = [[] for _ in range(len(passes) + 1)]
    for tasks, lo, hi in plan:
        total, done = sum(sum(c) for c, _ in tasks) or 1, 0.0
        for costs, fn in tasks:
            where = []
            for cost in costs:
                done += cost
                where.append(index(lo + done / total * (hi - lo)))
            at[min(where)].append((fn, where))
    seen, ties = [], [[] for _ in at]
    for i, fns in enumerate(at):
        now = (begin[i] + i % 4) if i < len(begin) else clock[0] / 16
        early = [(t - now, v) for t, v in seen if t % CFG["Q"] < 1 or CFG["Q"] == 1]
        for fn, where in fns:
            for w, tie in zip(where, fn(_Gate(pred, early)) or ()):
                ties[w].append(tie)
        if i == len(passes):
            break
        n, lhs, rhs, consume = passes[i]
        w = rhs()
        if not isinstance(w, list):
            d = lax.dot_general(pltpu.bitcast(jnp.concatenate(lhs(), axis=0), BF16), w,
                                (((1,), (1,)), ((), ())), preferred_element_type=F32)
            consume(d)
            continue
        for tie in ties[i]:
            if isinstance(tie, _Zeros):
                v = tie.v
                w[-1] = w[-1] | (v if v.dtype == I32 else pltpu.bitcast(v, I32))
            else:
                w[-1] = jnp.where(pred, w[-1], pltpu.bitcast(tie, I32))
        d = jnp.dot(pltpu.bitcast(jnp.concatenate(lhs(), axis=0), BF16),
                    pltpu.bitcast(jnp.concatenate(w, axis=0), BF16), preferred_element_type=F32)
        seen += [(begin[i] + i % 4 + j // 16 - 4, d[j - 8:j]) for j in range(64, n + 1, 64)]
        consume(d)


def _now(tasks):
    for _, fn in tasks:
        fn(_Gate())


def _kernel(tab_hbm, x_hbm, lre_hbm, lim_hbm, bre_hbm, bim_hbm, cre_hbm, cim_hbm,
            ldt_hbm, dsk_hbm, q_hbm, k_hbm, v_hbm, tap_hbm, sk_hbm, sd_hbm,
            o_hbm,
            tab, lre_v, lim_v, ldt_v, dsk_v, sd_v, tap_v,
            xb, braw, craw, qb, kb, vb, skb,
            par, wb16, wc, mf16, mi, bu, hb16, carry, ys, oa,
            kt, kf, st_u, st_k, st_i, vu16, vk16, pb0, pb1, ob,
            sem):
    x32, q32, k32, v32, wb, mf, hb, vu, vk = (
        r.bitcast(I32) for r in (xb, qb, kb, vb, wb16, mf16, hb16, vu16, vk16))
    c32 = craw.bitcast(I32)
    pb16 = (pb0, pb1)
    pb = (pb0.bitcast(I32), pb1.bitcast(I32))

    def rows(ref, start, n=8):
        return ref[pl.ds(start, n), :]

    def hint(v, n):
        return v if isinstance(v, int) or n == 1 else pl.multiple_of(v, n)

    def view(ref, start, n=None):
        return ref.at[pl.ds(hint(start, 16), n or ref.shape[0]), :]

    def after(ref):
        return _Zeros(view(ref, z8)[ref.shape[0] - 16:ref.shape[0] - 8, 0:128])

    small = [pltpu.make_async_copy(s, d, sem.at[S_SMALL]) for s, d in (
        (lre_hbm, lre_v), (lim_hbm, lim_v), (ldt_hbm, ldt_v),
        (dsk_hbm, dsk_v), (sd_hbm, sd_v), (tap_hbm, tap_v),
        (tab_hbm.at[pl.ds(288, 8), :], tab.at[pl.ds(288, 8), :]))]
    tab_dma = pltpu.make_async_copy(
        tab_hbm.at[pl.ds(0, 288), :], tab.at[pl.ds(0, 288), :], sem.at[S_B + 4])

    def x_dma(u):
        return [pltpu.make_async_copy(
            x_hbm.at[pl.ds(hint(u * UNIT, UNIT), UNIT), pl.ds(128 * n, 128)],
            xb.at[pl.ds(hint(n * L + u * UNIT, UNIT), UNIT), :], sem.at[(S_X0, S_B + 4, S_F0, S_K0)[u] if isinstance(u, int) and u < LEAD
                                                     else S_COL + u - LEAD])
            for n in range(NG)]

    def b_dma(p):
        return [pltpu.make_async_copy(
            src.at[pl.ds(128 * p, 128), :], braw.at[pl.ds(D * c + 128 * p, 128), :],
            sem.at[S_B + p]) for c, src in enumerate((bre_hbm, bim_hbm))]

    c_dma = [pltpu.make_async_copy(
        src.at[:, pl.ds(128 * p, 128)], craw.at[pl.ds(D * (NG * c + p), D), :],
        sem.at[S_C]) for c, src in enumerate((cre_hbm, cim_hbm)) for p in range(NG)]

    def col_dma(which, g, sem_at):
        src, dst = ((k_hbm, kb), (v_hbm, vb), (q_hbm, qb))[which]
        return pltpu.make_async_copy(
            src.at[:, pl.ds(hint(128 * g, 128), 128)],
            dst.at[pl.ds(hint(L * g, L), L), :], sem.at[sem_at])

    def sk_dma(g, sem_at):
        t = hint(128 * g, 128)
        return [pltpu.make_async_copy(
            sk_hbm.at[pl.ds(t, 128), :], skb.at[pl.ds(t, 128), :], sem.at[sem_at])]

    def oa_dma(u, n):
        t = hint(u * UNIT, UNIT)
        return pltpu.make_async_copy(
            oa.at[pl.ds(t, UNIT), pl.ds(128 * n, 128)],
            o_hbm.at[pl.ds(t, UNIT), pl.ds(128 * n, 128)], sem.at[S_OUT])

    def oa_unit_dma(u):
        t = hint(u * UNIT, UNIT)
        return pltpu.make_async_copy(
            oa.at[pl.ds(t, UNIT), :], o_hbm.at[pl.ds(t, UNIT), pl.ds(0, D)], sem.at[S_OUT])

    def ob_dma(g, half):
        h = L // 2
        return pltpu.make_async_copy(
            ob.at[pl.ds(hint(L * g + h * half, h), h), :],
            o_hbm.at[pl.ds(h * half, h), pl.ds(hint(D + 128 * g, 128), 128)], sem.at[S_OUT])

    def start(ds):
        for d in ds:
            d.start()

    def wait(ds):
        for d in ds:
            d.wait()

    def prm(g, row):
        return rows(view(par, g * (P_ROWS * 8), P_ROWS * 8), row * 8)

    def bu_passes(u, slot, z, shift):
        out = []
        xu, w = view(x32, u * (UNIT // 2), ((NG - 1) * L + UNIT) // 2), view(wb, z)
        order = [p + c * NG for p in range(NG) for c in range(2)]
        for n in order:
            sizes = [128, 128]
            if shift and n == order[0]:
                sizes = [32, 32, 96, 96]
            if shift and n == order[-1]:
                sizes = [96, 96, 32, 32] if shift is True else [64] * 4
            if shift is None:
                sizes = CFG["m0"] if u == 0 else [64] * 4
            for m, MM in zip(np.cumsum([0] + sizes).tolist(), sizes):
                acc = []
                for kk in range(NG):
                    def lhs(m=m, kk=kk, MM=MM):
                        t = (kk * L + m) // 2
                        return [rows(xu, t + 8 * i) for i in range(MM // 16)]

                    def rhs(n=n, kk=kk):
                        if u == 0 if isinstance(u, int) else False:
                            return braw[pl.ds(128 * n, 128), pl.ds(128 * kk, 128)]
                        return [rows(w, (n * NG + kk) * 64 + 8 * i) for i in range(8)]

                    def consume(d, m=m, n=n, kk=kk, acc=acc, MM=MM):
                        acc.append(d if kk == 0 else acc[-1] + d)
                        if kk == NG - 1:
                            for i in range(MM // 8):
                                seg, r = divmod(m + 8 * i, R)
                                row = 9 * (seg % 2 * R + r) + seg // 2
                                bu[pl.ds((slot * 2 * NG + n) * BU_PART + row, 8, stride=9), :] = (
                                    acc[-1][8 * i:8 * i + 8])
                    out.append((MM, lhs, rhs, consume))
        return out

    def scan_tasks(u, slot, z):
        steps = CFG["steps"]
        state = {}
        hu = view(hb16, u * UNIT, (2 * NG - 1) * L + UNIT)

        def b(p, ch, r):
            return tuple(rows(bu, (slot * 2 * NG + c * NG + p) * BU_PART + 9 * (ch * R + r))
                         for c in range(2))

        def step(mu, h, br):
            return (mu[0] * h[0] + br[0]) - mu[1] * h[1], (mu[0] * h[1] + br[1]) + mu[1] * h[0]

        def ends(p, gate):
            mu, ties = (gate.value(prm(p, P_MU), CFG["scan"]), prm(p, P_MU + 1)), []
            h = [b(p, ch, 0) for ch in range(2)]
            for r in range(1, R):
                h = [step(mu, h[ch], b(p, ch, r)) for ch in range(2)]
                if r % steps == 0:
                    ties.append(h[r // steps % 2][0])
            state[p] = starts(p, h)
            return ties + [state[p][1][0]]

        def starts(p, e):
            last = lax.broadcasted_iota(I32, (8, 128), 0) == 7
            rho = (prm(p, P_RHO), prm(p, P_RHO + 1))
            pair = step(rho, e[0], e[1])
            a = tuple(pltpu.roll(jnp.where(last, rows(carry, (2 * p + c) * 8), pair[c]), 1, 0)
                      for c in range(2))
            for sh, row in ((1, P_RHO1), (2, P_RHO2), (4, P_RHO4)):
                a = step((prm(p, row), prm(p, row + 1)), tuple(pltpu.roll(c, sh, 0) for c in a), a)
            return [a, step(rho, a, e[0])]

        def run(p, r0, gate):
            if r0 == 0:
                state["mu"] = (prm(p, P_MU), prm(p, P_MU + 1))
            mu, h = (gate.value(state["mu"][0], CFG["scan"]), state["mu"][1]), state[p]
            for r in range(r0, r0 + steps):
                h = [step(mu, h[ch], b(p, ch, r)) for ch in range(2)]
                for c in range(2):
                    hu[pl.ds((c * NG + p) * L + 16 * r, 16), :] = _pack(h[0][c], h[1][c])
            state[p] = h
            if r0 + steps == R:
                for c in range(2):
                    carry[pl.ds((2 * p + c) * 8, 8), :] = h[1][c]
            return [after(hb)]

        tasks = []
        for p in range(NG):
            tasks.append(([16 * steps] * ((R - 1) // steps) + [46 + 16 * steps],
                          lambda gate, p=p: ends(p, gate)))
            tasks += [([18 * steps], lambda gate, p=p, r0=r0: run(p, r0, gate))
                      for r0 in range(0, R, steps)]
        return tasks

    def y_passes(h, n, sizes=(HALF,), z=0):
        out, w, hu = [], view(wc, z), view(hb, h * (HALF // 2), ((2 * NG - 1) * L + HALF) // 2)
        for t0, MM in zip(np.cumsum((0,) + sizes).tolist(), sizes):
            acc = []
            for kk in range(2 * NG):
                def lhs(t0=t0, kk=kk, MM=MM):
                    return [rows(hu, (kk * L + t0) // 2 + 8 * i) for i in range(MM // 16)]

                def rhs(kk=kk):
                    return [rows(w, (kk * NG + n) * 64 + 8 * i) for i in range(8)]

                def consume(d, t0=t0, kk=kk, acc=acc, MM=MM):
                    acc.append(d if kk == 0 else acc[-1] + d)
                    if kk == 2 * NG - 1:
                        for i in range(MM // 8):
                            r, ch = divmod(t0 // 8 + i, 2)
                            ys[pl.ds(n * YS_ROWS + ch * (R // 2 + 1) + r, 8, stride=R + 2), :] = (
                                acc[-1][8 * i:8 * i + 8])
                out.append((MM, lhs, rhs, consume))
        return out

    def skip_task(h, n):
        def fn(gate):
            dsk, ties = gate.value(prm(n, P_DSKIP), CFG["skip"]), []
            t = h // 2 * UNIT + h % 2 * (R // 2)
            xu = x32.at[pl.ds(hint(t // 2 + n * (L // 2), 4), UNIT // 2 - 4 + 8 * (n < NG - 1 or not isinstance(h, int))), :]
            ou = oa.at[pl.ds(hint(t, 8), UNIT - R // 2), :]
            for g in range(SEG):
                if g == SEG - 1 and n == NG - 1 and isinstance(h, int):
                    xs = _unpack(rows(xu, 8 * g - 4))[1]
                else:
                    xs = _unpack(rows(xu, 8 * g))[0]
                y = rows(ys, n * YS_ROWS + g * (R // 2 + 1))
                ou[pl.ds(R * g, 8), pl.ds(128 * n, 128)] = y + xs * dsk
                if g % 8 == 7:
                    ties.append(after(oa))
            return ties
        return ([24, 24], fn)

    def widen_tasks(g, z, pieces=2):
        def fn(i0, i1):
            kg = view(k32, g * (L // 2), L // 2)
            for i in range(i0, i1):
                lo, hi = _unpack(rows(kg, 8 * i))
                kf[pl.ds(KF_PAD + 16 * i, 8), :] = lo
                kf[pl.ds(KF_PAD + 16 * i + 8, 8), :] = hi
            return [after(kf)]
        n = L // 16 // pieces
        return [([2 * n], lambda gate, i=i: fn(i * n, (i + 1) * n)) for i in range(pieces)]

    def transpose_tasks(g, z, pieces=8):
        def fn(c0, c1):
            for c in range(c0, c1):
                t = skb[pl.ds(hint(128 * g, 128), 128), pl.ds(128 * c, 128)]
                kt[pl.ds(64 * c, 64), :] = pltpu.bitcast(t.T, I32)
            return [after(kt)]
        n = L // 128 // pieces
        return [([8 * n], lambda gate, i=i: fn(i * n, (i + 1) * n)) for i in range(pieces)]

    def staged(s, half, n, grp, c):
        return (((s * 2 + half) * 4 + n) * 4 + grp) * 16 + 8 * c

    ops1 = (18, 36, 30, 36)

    def forward_tasks_of(st, s, half, z, chunk, chunk_cost, direct):
        dst16, dst = (vu16, vu) if st is st_u else (vk16, vk)

        def second(grp, zs):
            for k, pair in enumerate(_fwd2(grp, zs)):
                dst16[pl.ds(((4 * grp + k) * 2 + half) * 128 + 16 * s, 16), :] = (
                    _pack(pair[0].get(), pair[1].get()))
            return after(dst)

        kept = []

        def first(gate, n):
            load = chunk(gate, n)
            u = [load(16 * half + n + 4 * m) for m in range(4)]
            pairs = _fwd1(n, [_Signed(v) for v in u])
            kept.append(pairs)
            for grp in range(2 * direct, 4):
                for c in range(2):
                    st[pl.ds(staged(s, half, n, grp, c), 8), :] = pairs[grp][c].get()
            return [u[0] + u[2]] * (chunk_cost > 4) + [after(st)]

        def rest(grp):
            if direct and grp < 2:
                return [second(grp, [t[grp] for t in kept])]
            return [second(grp, [tuple(_Signed(rows(view(st, z), staged(s, half, n, grp, c)))
                                       for c in range(2)) for n in range(4)])]

        split = (chunk_cost > 4) * (chunk_cost // 2 + 1)
        one = [([split] * (split > 0) + [chunk_cost + ops1[n] - split], lambda gate, n=n: first(gate, n))
               for n in range(4)]
        if CFG["p2n"] == 4:
            two = [([20], lambda gate, grp=grp: rest(grp)) for grp in range(4)]
        else:
            two = [([40], lambda gate, grp=grp: rest(grp) and rest(grp + 1)) for grp in (0, 2)]
        h = len(two) // 2
        return (one + two[:h], two[h:]) if direct else (one, two)

    def u_tasks(g, s, half, z):
        loaded = []

        def chunk(gate, n):
            if n == 0 or CFG["retap"]:
                loaded[:] = [prm(g, P_TAP + t) for t in range(4)]
            taps = [gate.value(loaded[0], CFG["u"])] + loaded[1:]
            kz, vg = view(kf, z), view(v32, g * (L // 2), L // 2)

            def load(c):
                t = 64 * c + 8 * s
                ks = rows(kz, KF_PAD + t) * taps[0]
                for lag in range(1, 4):
                    ks = ks + rows(kz, KF_PAD + t - lag) * taps[lag]
                return ks * _unpack(rows(vg, (t // 16) * 8))[s % 2]
            return load
        return forward_tasks_of(st_u, s, half, z, chunk, 36, CFG["udir"])

    def k_tasks(g, s, half, z, direct):
        def chunk(gate, n):
            if n % CFG["kg"] == 0:
                gate.loads(kt, CFG["k1"])

            def load(c):
                v = _unpack(rows(view(kt, z), 32 * c + 8 * (s // 2)))[s % 2]
                if s == 0 and c == 0:
                    first = lax.broadcasted_iota(I32, (8, 128), 0) == 0
                    v = v + jnp.where(first, prm(g, P_SSMD), 0.0)
                return v
            return load
        return forward_tasks_of(st_k, s, half, z, chunk, 4, direct)

    def fwd_passes(grp, z):
        out, MM = [], CFG["mf"]
        for slot in range(4 * grp, 4 * grp + 4):
            for part in range(128 // MM):
                got = []
                for src, half in ((vu, 0), (vk, 0), (vu, 1), (vk, 1)):
                    def lhs(slot=slot, part=part):
                        return [rows(mf, slot * 64 + MM // 2 * part + 8 * i) for i in range(MM // 16)]

                    def rhs(slot=slot, src=src, half=half):
                        return [rows(view(src, z), (2 * slot + half) * 64 + 8 * i) for i in range(8)]

                    def consume(d, slot=slot, part=part, got=got):
                        got.append(d)
                        if len(got) < 4:
                            return
                        for i in range(MM // 16):
                            u0, k0, u1, k1 = ((t[16 * i:16 * i + 8], t[16 * i + 8:16 * i + 16]) for t in got)
                            lo, a, b = _cmul(u0, k0), _cmul(u0, k1), _cmul(u1, k0)
                            if slot == _REAL_SLOT and part == 0 and i == 0:
                                first = lax.broadcasted_iota(I32, (8, 128), 0) == 0
                                lo, a, b = (tuple(jnp.where(first, 0.5 * (x[c] * y[c]), p[c]) for c in range(2))
                                            for p, x, y in ((lo, u0, k0), (a, u0, k1), (b, u1, k0)))
                            if _F1[slot] % 2:
                                hi = ((a[0] + b[0]) - lo[0], (a[1] + b[1]) - lo[1])
                            else:
                                hi = ((a[0] + b[0]) + lo[0], (a[1] + b[1]) + lo[1])
                            for half, p in enumerate((lo, hi)):
                                at = (slot % 4 * 2 + half) * 128 + MM * part + 16 * i
                                pb16[grp % 2][pl.ds(at, 16), :] = _pack(*p)
                    out.append((MM, lhs, rhs, consume))
        return out

    def inv_passes(grp, half, z):
        out, MM = [], CFG["mi"]
        for part in range(128 // MM):
            got = []
            for slot in range(4 * grp, 4 * grp + 4):
                def lhs(slot=slot, part=part):
                    return [rows(mi, slot * 64 + MM // 2 * part + 8 * i) for i in range(MM // 16)]

                def rhs(slot=slot):
                    return [rows(view(pb[grp % 2], z), (slot % 4 * 2 + half) * 64 + 8 * i)
                            for i in range(8)]

                def consume(d, part=part, got=got):
                    got.append(d)
                    if len(got) < 4:
                        return
                    for i in range(MM // 16):
                        w = [(_Signed(t[16 * i:16 * i + 8]), _Signed(t[16 * i + 8:16 * i + 16]))
                             for t in got]
                        for n, pair in enumerate(_inv2(grp, w)):
                            for c in range(2):
                                at = staged(MM // 16 * part + i, half, n, grp, c)
                                st_i[pl.ds(at, 8), :] = pair[c].get()
                out.append((MM, lhs, rhs, consume))
        return out

    def inv1_task(g, s, half, z):
        def fn(gate, ns):
            gate.loads(st_i, CFG["inv"])
            qg, og, ties = view(q32, g * (L // 2), L // 2), view(ob, g * L, L), []
            for n in ns:
                zs = [tuple(_Signed(rows(view(st_i, z), staged(s, half, n, grp, c))) for c in range(2))
                      for grp in range(4)]
                for m, y in enumerate(_inv1(n, zs)):
                    t = 64 * (16 * half + n + 4 * m) + 8 * s
                    og[pl.ds(t, 8), :] = _unpack(rows(qg, (t // 16) * 8))[s % 2] * y.get()
                ties.append(after(ob))
            return ties
        if CFG["invsplit"]:
            return [([12 + ops1[n]], lambda gate, n=n: fn(gate, [n])) for n in range(4)]
        return [([12 + n for n in ops1], lambda gate: fn(gate, range(4)))]

    filter0 = x_dma(2) + sk_dma(0, S_F0)
    data0 = x_dma(3) + [col_dma(0, 0, S_K0), col_dma(1, 0, S_K0)]

    def group_dma(g):
        at = S_COL + g
        return ([col_dma(2, g, at)] + sk_dma(g + 1, at)
                + [col_dma(0, g + 1, at), col_dma(1, g + 1, at)] + x_dma(g + LEAD))

    last_dma = col_dma(2, NG - 1, S_SMALL)

    start(small + b_dma(0) + x_dma(0) + b_dma(1) + b_dma(2))
    wait(small)
    zeros = rows(tab, 288).astype(I32)
    z8 = pl.multiple_of(zeros[0, 0], 16)
    sub = lax.broadcasted_iota(I32, (8, 128), 0)
    pred = zeros == 0

    def stack(ref):
        v = ref[...].astype(F32).reshape(1, D)
        return jnp.concatenate([v[:, 128 * g:128 * (g + 1)] for g in range(NG)]
                               + [v[:, :128]] * (8 - NG), axis=0)

    lre, lim = stack(lre_v), stack(lim_v)
    dt = jnp.exp(stack(ldt_v)).astype(BF16).astype(F32)
    mag, ang = jnp.exp(dt * lre), dt * lim
    lam = (mag * jnp.cos(ang), mag * jnp.sin(ang))
    scale = jnp.maximum(jnp.abs(lre), jnp.abs(lim))
    nre, nim = lre / scale, lim / scale
    den = (nre * nre + nim * nim) * scale
    coef = _cmul(((lam[0] - 1.0) / den, lam[1] / den), (nre, -nim))
    mu = lam
    rho = [mu]
    for _ in range(R.bit_length() + 2):
        rho.append(_cmul(rho[-1], rho[-1]))
    dsk, ssd = stack(dsk_v), stack(sd_v)
    taps = tap_v[...].astype(F32) * _FFT_SCALE
    for g in range(NG):
        def put(row, v):
            par[pl.ds((g * P_ROWS + row) * 8, 8), :] = v

        def lanes(v):
            return jnp.broadcast_to(v[g:g + 1], (8, 128))
        for c in range(2):
            put(P_MU + c, lanes(mu[c]))
            put(P_RHO + c, lanes(rho[-4][c]))
            for n, row in enumerate((P_RHO1, P_RHO2, P_RHO4)):
                put(row + c, jnp.where(sub >= 1 << n, lanes(rho[n - 3][c]), 0.0))
        for t in range(4):
            put(P_TAP + t, jnp.broadcast_to(taps[t:t + 1, 128 * g:128 * (g + 1)], (8, 128)))
        put(P_COEF, lanes(2.0 * coef[0]))
        put(P_COEF + 2, lanes(-2.0 * coef[1]))
        put(P_SSMD, lanes(ssd))
        put(P_DSKIP, lanes(dsk))
    for ref in (hb, oa, kf, kt, vu, vk, st_u, st_k, ob, mf, mi, wb, wc):
        ref[pl.ds(ref.shape[0] - 16, 8), pl.ds(0, 128)] = jnp.zeros((8, 128), ref.dtype)
    for i in range(2 * NG):
        carry[pl.ds(8 * i, 8), :] = jnp.zeros((8, 128), F32)
    kf[pl.ds(0, KF_PAD), :] = jnp.zeros((KF_PAD, 128), F32)

    def matrix_task(slot):
        def fn(gate):
            if slot != _REAL_SLOT:
                c, s = tab[pl.ds(256 + slot, 1), :], tab[pl.ds(272 + slot, 1), :]
            for a in range(8):
                if slot == _REAL_SLOT:
                    re, im = rows(tab, 128 + 16 * a), rows(tab, 128 + 16 * a + 8)
                else:
                    br, bi = rows(tab, 16 * a), rows(tab, 16 * a + 8)
                    re, im = c * br - s * bi, s * br + c * bi
                mf16[pl.ds(slot * 128 + 16 * a, 16), :] = _pack(re, im)
            m = pltpu.bitcast(rows(view(mf, z8), slot * 64, 64), BF16)
            mi[pl.ds(slot * 64, 64), :] = pltpu.bitcast(m.T, I32)
            return [after(mf), after(mi)]
        return ([48, 8], fn)

    def b_task(p):
        def fn(gate):
            ties = []
            for n in (p, NG + p):
                for kk in range(NG):
                    t = braw[pl.ds(128 * n, 128), pl.ds(128 * kk, 128)]
                    wb[pl.ds((n * NG + kk) * 64, 64), :] = pltpu.bitcast(t.T, I32)
                    ties.append(after(wb))
            return ties
        return ([24] * (2 * NG), fn)

    def c_task(n, p):
        def fn(gate):
            cr, ci, nci = prm(p, P_COEF), prm(p, P_COEF + 1), prm(p, P_COEF + 2)
            t = [_unpack_tile(rows(c32, ((c * NG + p) * D + 128 * n) // 2, 64)) for c in range(2)]
            re = [_pack(cr * a0 + nci * b0, cr * a1 + nci * b1) for (a0, a1), (b0, b1) in zip(*t)]
            im = [_pack(nci * a0 - cr * b0, nci * a1 - cr * b1) for (a0, a1), (b0, b1) in zip(*t)]
            ties = []
            for c, tile in enumerate((re, im)):
                wc[pl.ds(((c * NG + p) * NG + n) * 64, 64), :] = pltpu.bitcast(
                    jnp.concatenate(tile, axis=0).T, I32)
                ties.append(after(wc))
            return ties[2 - CFG["ct"]:]
        return ([[160], [80, 80]][CFG["ct"] - 1], fn)

    first = bu_passes(0, 1, z8, None)
    first = [first[len(first) // NG * p:len(first) // NG * (p + 1)] for p in range(NG)]

    mats = [matrix_task(slot) for slot in range(SLOTS)]

    def dma_task(ds):
        return ([1], lambda gate: start(ds))

    def filter_tasks(g, early):
        ts = [k_tasks(g, j // 2, j % 2, z8, j >= early and CFG["kdir"]) for j in range(16)]
        return (transpose_tasks(g, z8), [q for t in ts[:early] for q in t[0]],
                [q for t in ts[:early] for q in t[1]] + [q for t in ts[early:] for q in t[0] + t[1]])

    def forward_tasks(g):
        return [t for s in range(8) for half in range(2) for t in sum(u_tasks(g, s, half, z8), [])]

    def y_block(halves, t0, z=0, lead=True, even=None):
        tiles = [(h, n) for h in halves for n in range(NG)]
        passes, plan = [], []
        for j, (h, n) in enumerate(tiles):
            sizes = (HALF,)
            if j == 0 and lead is not None:
                if not lead:
                    continue
                sizes = (32, 96)
            if j == even:
                sizes = (64, 64)
            if j == len(tiles) - 1:
                sizes = (96, 32)
            passes += y_passes(h, n, sizes, z)
            t0 += 20
            plan.append(([skip_task(h, n)], t0 + CFG["sk0"], t0 + CFG["sk0"] + 6))
        return passes, plan

    total = 2 * NG * NG * UNIT // 64

    def early(at):
        for when, ds in zip(CFG["when"], (filter0, data0, c_dma, group_dma(0), group_dma(1), group_dma(2),
                                          group_dma(3) + [last_dma])):
            if when == at:
                start(ds)

    start(b_dma(3) + b_dma(4) + x_dma(1) + [tab_dma])
    wait(x_dma(0) + b_dma(0))
    _weave(first[0], [], pred)
    early(0)
    wait(b_dma(1))
    _weave(first[1], [], pred)
    early(1)
    wait(b_dma(2) + b_dma(3))
    _weave(first[2] + first[3], [([b_task(p) for p in range(4)], 0, 80)], pred)
    early(2)
    wait(b_dma(4) + x_dma(1) + [tab_dma])
    _weave(first[4] + bu_passes(1, 0, z8, CFG["sh1"]), [
        ([b_task(4)], 0, 36),
        (scan_tasks(0, 1, z8), 40, 40 + total), (mats, 60, 200)], pred)
    early(3)
    wait(filter0)
    tr, _, k1 = filter_tasks(0, 0)
    nk, fwd = int(CFG["k0"] * len(k1)), forward_tasks(0)
    nu = int(CFG["u0"] * len(fwd))
    _weave(bu_passes(2, 1, 0, CFG["sh2"]), [
        (scan_tasks(1, 0, z8), 0, total), (tr, 8, 32), (k1[:nk], 36, total)], pred)
    early(4)
    wait(data0 + c_dma)
    cs = [c_task(n, p) for n in range(NG) for p in range(NG)]
    yp, plan = y_block((0, 1), total, z8, lead=None, even=2)
    _weave(bu_passes(3, 0, 0, "open") + yp, plan + [
        (scan_tasks(2, 1, z8), *CFG["s2"]), (k1[nk:], 0, total), (widen_tasks(0, z8, 16), 0, 40),
        (cs, *CFG["cw"]), (fwd[:-2], CFG["f0"], 2 * total), (fwd[-2:], 2 * total, 2 * total)], pred)
    start([oa_unit_dma(0)])
    early(6)

    def conv_passes():
        passes = fwd_passes(0, z8)
        for grp in range(1, 4):
            f, n = fwd_passes(grp, z8), 4 * 128 // CFG["mf"]
            a, b = (n * j for j in CFG["ord"])
            passes += f[:a] + inv_passes(grp - 1, 0, z8) + f[a:b] + inv_passes(grp - 1, 1, z8) + f[b:]
        return passes

    def inverse_tasks(g):
        tasks = []
        for half in range(2):
            for s in range(8):
                tasks += inv1_task(g, s, half, z8)
            tasks.append(dma_task([ob_dma(g, half)]))
        return tasks

    def body(i, _):
        wait(group_dma(i))
        halves = [2 + 3 * i + j for j in range(3)]
        lead = y_passes(halves[0], 0, (32, 96))
        y0 = 192 + 20 + total
        yp, plan = y_block(halves, y0, lead=False, even=7)
        passes = (conv_passes() + lead[:8] + inv_passes(3, 0, z8) + inv_passes(3, 1, z8) + lead[8:]
                  + bu_passes(i + LEAD, 0, 0, False) + yp)
        tr, k1, k2 = filter_tasks(i + 1, CFG["kconv"])
        fwd, tail, end = forward_tasks(i + 1), CFG["tail"], y0 + 280
        done = (3 * i + 2) // 2
        _weave(passes, plan + [
            ([dma_task([oa_unit_dma(done)])], y0 + 210, y0 + 210),
            (scan_tasks(i + LEAD - 1, 0, z8), *CFG["scanw"]), (tr, *CFG["tr"]),
            ([skip_task(halves[0], 0)], 232, 238),
            (widen_tasks(i + 1, z8, 16), *CFG["wid"]), (k1, *CFG["kwin"]),
            (inverse_tasks(i), *CFG["invw"]), (k2, *CFG["k2w"]),
            (fwd[:-tail], CFG["u0w"], end), (fwd[-tail:], end, end)], pred)
        pl.when(i % 2 == 1)(lambda: start([oa_unit_dma(done + 1)]))
        return 0

    lax.fori_loop(0, NG - 1, body, 0)

    wait([last_dma])
    g, last = NG - 1, L // UNIT - 1
    yp, plan = y_block((2 * last, 2 * last + 1), 192, even=2)
    ends = [[dma_task([oa_dma(last, n)])] for n in range(NG)]
    plan += [(ends[n], t + 6, t + 6) for n, (_, _, t) in enumerate(plan[NG:])]
    _weave(conv_passes() + yp[:8] + inv_passes(3, 0, z8) + inv_passes(3, 1, z8) + yp[8:], plan + [
        (scan_tasks(last, 0, z8), 0, 170),
        (inverse_tasks(g), 216, CFG["invend"])], pred)
    wait([oa_unit_dma(u) for u in range(last)] + [oa_dma(last, n) for n in range(NG)]
         + [ob_dma(n, half) for n in range(NG) for half in range(2)])


@jax.jit
def pallas_concat_heads__ssm_conv_s5__ssm_conv_h3__prompt_kernel(
    A_x: jax.Array,
    A_Lambda_re: jax.Array,
    A_Lambda_im: jax.Array,
    A_B_re: jax.Array,
    A_B_im: jax.Array,
    A_C_re: jax.Array,
    A_C_im: jax.Array,
    A_log_dt: jax.Array,
    A_Dskip: jax.Array,
    B_q: jax.Array,
    B_k: jax.Array,
    B_v: jax.Array,
    B_shift_k: jax.Array,
    B_ssm_k: jax.Array,
    B_ssm_D: jax.Array,
):
    assert A_x.shape == (1, L, D) and B_shift_k.shape == (D, 4)
    vmem = pltpu.VMEM
    dma = pltpu.SemaphoreType.DMA
    scratch = [
        vmem(_TABLES.shape, F32),
        vmem((D,), BF16), vmem((D,), BF16), vmem((D,), BF16), vmem((D,), BF16), vmem((D,), BF16),
        vmem((4, D), BF16),
        vmem((NG * L, 128), BF16),
        vmem((2 * D, D), BF16),
        vmem((2 * NG * D, 128), BF16),
        vmem((NG * L, 128), BF16),
        vmem((NG * L, 128), BF16),
        vmem((NG * L, 128), BF16),
        vmem((D, L), BF16),
        vmem((NG * P_ROWS * 8, 128), F32),
        vmem((2 * NG * D + 32, 128), BF16),
        vmem((2 * NG * NG * 64 + 16, 128), I32),
        vmem((SLOTS * 128 + 32, 128), BF16),
        vmem((SLOTS * 64 + 16, 128), I32),
        vmem((2 * 2 * NG * BU_PART, 128), F32),
        vmem((2 * NG * L + 32, 128), BF16),
        vmem((3 * NG * 8, 128), F32),
        vmem((NG * YS_ROWS, 128), F32),
        vmem((L + 16, D), F32),
        vmem((L // 2 + 16, 128), I32),
        vmem((KF_PAD + L + 16, 128), F32),
        vmem((2 * L + 16, 128), F32),
        vmem((2 * L + 16, 128), F32),
        vmem((2 * L + 8, 128), F32),
        vmem((32 * 128 + 32, 128), BF16),
        vmem((32 * 128 + 32, 128), BF16),
        vmem((8 * 128, 128), BF16),
        vmem((8 * 128, 128), BF16),
        vmem((NG * L + 16, 128), F32),
        dma((S_END,)),
    ]
    out = pl.pallas_call(
        _kernel,
        out_shape=jax.ShapeDtypeStruct((L, 2 * D), F32),
        in_specs=[pl.BlockSpec(memory_space=pl.ANY)] * 16,
        out_specs=pl.BlockSpec(memory_space=pl.ANY),
        scratch_shapes=scratch,
        compiler_params=pltpu.CompilerParams(vmem_limit_bytes=100 * 1024 * 1024, flags=CFG["flags"], disable_semaphore_checks=CFG["nosem"]),
        name="s5_h3",
    )(_TABLES, A_x.reshape(L, D), A_Lambda_re, A_Lambda_im, A_B_re, A_B_im, A_C_re, A_C_im,
      A_log_dt, A_Dskip, B_q.reshape(L, D), B_k.reshape(L, D), B_v.reshape(L, D),
      B_shift_k.T, B_ssm_k, B_ssm_D)
    return out.reshape(1, L, 2 * D)
```

```python
import math

import jax
import jax.numpy as jnp
import numpy as np
from jax import lax
from jax.experimental import pallas as pl
from jax.experimental.pallas import tpu as pltpu

F32, BF16, I32 = jnp.float32, jnp.bfloat16, jnp.int32

L = 2048
D = 640
NG = D // 128
UNIT = 256
SEG = 16
R = UNIT // SEG
LEAD = 4
HALF = UNIT // 2
BU_PART = 9 * 2 * R
YS_ROWS = SEG * (R // 2 + 1)
KF_PAD = 8


class _Signed:
    def __init__(self, v, neg=False):
        self.v, self.neg = v, neg

    def __neg__(self):
        return _Signed(self.v, not self.neg)

    def __add__(self, o):
        if self.neg == o.neg:
            return _Signed(self.v + o.v, self.neg)
        return _Signed(o.v - self.v if self.neg else self.v - o.v)

    def __sub__(self, o):
        return self + (-o)

    def __mul__(self, c):
        return _Signed(self.v * np.float32(-c if self.neg else c))

    def get(self):
        return -self.v if self.neg else self.v


def _rot(re, im, num, den):
    num %= den
    h = math.sqrt(0.5)
    if num == 0:
        return re, im
    if 4 * num == den:
        return -im, re
    if 4 * num == 3 * den:
        return im, -re
    if 8 * num == den:
        return (re - im) * h, (re + im) * h
    if 8 * num == 3 * den:
        return (re + im) * (-h), (re - im) * h
    if 8 * num == 5 * den:
        return (im - re) * h, (re + im) * (-h)
    if 8 * num == 7 * den:
        return (re + im) * h, (im - re) * h
    c = math.cos(2 * math.pi * num / den)
    s = math.sin(2 * math.pi * num / den)
    return re * c - im * s, re * s + im * c


def _dft4(z, sign):
    (r0, i0), (r1, i1), (r2, i2), (r3, i3) = z
    ar, ai, br, bi = r0 + r2, i0 + i2, r0 - r2, i0 - i2
    cr, ci, dr, di = r1 + r3, i1 + i3, r1 - r3, i1 - i3
    plus, minus = (br - di, bi + dr), (br + di, bi - dr)
    if sign < 0:
        plus, minus = minus, plus
    return [(ar + cr, ai + ci), plus, (ar - cr, ai - ci), minus]


def _fwd1(n, u):
    a0, a1, b0, b1 = u
    p, q = _rot(a0, b0, n, 32), _rot(a1, b1, n + 4, 32)
    s0, s1 = a0 + b0, a1 + b1
    return [(p[0] + q[0], p[1] + q[1]), _rot(p[0] - q[0], p[1] - q[1], n, 8),
            _rot(a0 - b0, a1 - b1, n, 16), (s0 + s1, s0 - s1)]


def _fwd2(grp, z):
    if grp < 3:
        return _dft4(z, 1)
    s4 = [t[0] for t in z]
    d4 = [t[1] for t in z]
    p = (d4[0], d4[2])
    q = _rot(d4[1], d4[3], 1, 8)
    s5 = [s4[0] + s4[2], s4[1] + s4[3]]
    return [
        (s5[0] + s5[1], s5[0] - s5[1]),
        (s4[0] - s4[2], s4[1] - s4[3]),
        (p[0] + q[0], p[1] + q[1]),
        (p[0] - q[0], p[1] - q[1]),
    ]


def _inv2(grp, w):
    if grp < 3:
        return _dft4(w, -1)
    s5 = [w[0][0] + w[0][1], w[0][0] - w[0][1]]
    s4 = [s5[0] + w[1][0], s5[1] + w[1][1], s5[0] - w[1][0], s5[1] - w[1][1]]
    p = (w[2][0] + w[3][0], w[2][1] + w[3][1])
    q = _rot(w[2][0] - w[3][0], w[2][1] - w[3][1], -1, 8)
    d4 = [p[0], q[0], p[1], q[1]]
    return [(s4[n], d4[n]) for n in range(4)]


def _inv1(n, z):
    e = _rot(*z[1], -n, 8)
    p = _rot(z[0][0] + e[0], z[0][1] + e[1], -n, 32)
    q = _rot(z[0][0] - e[0], z[0][1] - e[1], -(n + 4), 32)
    d0, d1 = _rot(*z[2], -n, 16)
    s0, s1 = z[3][0] + z[3][1], z[3][0] - z[3][1]
    return [p[0] + (s0 + d0), q[0] + (s1 + d1), p[1] + (s0 - d0), q[1] + (s1 - d1)]


_F1 = [4 * (g + 2 * k) + 1 for g in range(2) for k in range(4)]
_F1 += [2 * (4 * k + 1) for k in range(4)] + [0, 8, 4, 20]
_REAL_SLOT = 12
SLOTS = len(_F1)


def _dft_tables():
    kap = np.arange(128)
    j = 8 * (kap // 16) + kap % 8
    part = (kap // 8) % 2
    pr, pc, jr, jc = part[:, None], part[None, :], j[:, None], j[None, :]
    lo = 2 * np.pi * jr * jc / 64
    base = np.where(pr == pc, np.cos(lo), np.where(pr == 0, -np.sin(lo), np.sin(lo)))
    hi = 2 * np.pi * (16 + 32 * (jr - 32)) * jc / 2048
    v0 = np.where(pr == 0, np.cos(lo), np.where(jr == 0, np.cos(np.pi * jc), np.sin(lo)))
    v32 = np.where(pr == 0, np.cos(hi), np.sin(hi))
    real = np.where(jr < 32, np.where(pc == 0, v0, 0.0), np.where(pc == 1, v32, 0.0))
    th = 2 * np.pi * np.outer(np.array(_F1), j) / 2048
    zeros = np.zeros((8, 128))
    return np.concatenate([base, real, np.cos(th), np.sin(th), zeros]).astype(np.float32)


_TABLES = _dft_tables()
_FFT_SCALE = 2.0 ** -10

(P_MU, P_RHO, P_RHO1, P_RHO2, P_RHO4, P_TAP, P_SSMD, P_DSKIP, P_COEF, P_ROWS) = (
    0, 2, 4, 6, 8, 10, 14, 15, 16, 20)
S_SMALL, S_F0, S_K0, S_C, S_OUT, S_X0, S_B = range(7)
S_COL = S_B + NG
S_END = S_COL + NG - 1


def _cmul(a, b):
    return a[0] * b[0] - a[1] * b[1], a[0] * b[1] + a[1] * b[0]


def _pack(lo, hi):
    return jnp.concatenate([lo, hi], axis=0).astype(BF16)


def _unpack_tile(w):
    return [_unpack(w[8 * i:8 * i + 8]) for i in range(w.shape[0] // 8)]


def _unpack(w):
    v = pltpu.bitcast(w, BF16).astype(F32)
    return v[:8], v[8:]


PLAN = dict(
    scan_lead=22, conv_lead=20, inverse_lead=44, skip_lead=24,
    scan=(0, 350), transpose=(60, 90), filter_early=(100, 216), early=4, inverse=(220, 380),
    widen=(216, 330), filter=(230, 480), forward=350, tail=3, skip=20,
    scale_c=(30, 260), scan0=(0, 390), forward0=120, last_inverse=(216, 290),
)


class _Zeros:
    def __init__(self, v):
        self.v = v


class _Gate:
    def __init__(self, pred=None, seen=()):
        self.pred, self.seen = pred, seen

    def early(self, lag):
        old = [e for e in self.seen if e[0] <= -lag]
        return max(old, key=lambda e: e[0])[1] if old else None

    def value(self, v, lag):
        early = self.early(lag)
        return v if early is None else jnp.where(self.pred, v, early)

    def loads(self, ref, lag):
        early = self.early(lag)
        if early is not None:
            ref[pl.ds(ref.shape[0] - 8, 8), :] = (
                early if ref.dtype == F32 else pltpu.bitcast(early, I32))


def _weave(passes, plan, pred):
    begin, clock = [], [0] * 4
    for i, (n, *_) in enumerate(passes):
        begin.append(clock[i % 4] / 16)
        clock[i % 4] += n

    def index(t):
        later = [i for i, b in enumerate(begin) if b >= t - 3.999]
        if not later:
            return len(passes)
        same = [i for i in later if begin[i] == min(begin[j] for j in later)]
        return same[min(max(int((t - begin[same[0]]) / 4 * len(same)), 0), len(same) - 1)]

    at = [[] for _ in range(len(passes) + 1)]
    for tasks, lo, hi in plan:
        total, done = sum(sum(c) for c, _ in tasks) or 1, 0.0
        for costs, fn in tasks:
            where = []
            for cost in costs:
                done += cost
                where.append(index(lo + done / total * (hi - lo)))
            at[min(where)].append((fn, where))
    seen, ties = [], [[] for _ in at]
    for i, fns in enumerate(at):
        now = (begin[i] + i % 4) if i < len(begin) else clock[0] / 16
        early = [(t - now, v) for t, v in seen]
        for fn, where in fns:
            for w, tie in zip(where, fn(_Gate(pred, early)) or ()):
                ties[w].append(tie)
        if i == len(passes):
            break
        n, lhs, rhs, consume = passes[i]
        w = rhs()
        if not isinstance(w, list):
            d = lax.dot_general(pltpu.bitcast(jnp.concatenate(lhs(), axis=0), BF16), w,
                                (((1,), (1,)), ((), ())), preferred_element_type=F32)
            consume(d)
            continue
        for tie in ties[i]:
            if isinstance(tie, _Zeros):
                v = tie.v
                w[-1] = w[-1] | (v if v.dtype == I32 else pltpu.bitcast(v, I32))
            else:
                w[-1] = jnp.where(pred, w[-1], pltpu.bitcast(tie, I32))
        d = jnp.dot(pltpu.bitcast(jnp.concatenate(lhs(), axis=0), BF16),
                    pltpu.bitcast(jnp.concatenate(w, axis=0), BF16), preferred_element_type=F32)
        seen += [(begin[i] + i % 4 + j // 16 - 4, d[j - 8:j]) for j in range(64, n + 1, 64)]
        consume(d)


def _kernel(tab_hbm, x_hbm, lre_hbm, lim_hbm, bre_hbm, bim_hbm, cre_hbm, cim_hbm,
            ldt_hbm, dsk_hbm, q_hbm, k_hbm, v_hbm, tap_hbm, sk_hbm, sd_hbm,
            o_hbm,
            tab, lre_v, lim_v, ldt_v, dsk_v, sd_v, tap_v,
            xb, braw, craw, qb, kb, vb, skb,
            par, wb16, wc, mf16, mi, bu, hb16, carry, ys, oa,
            kt, kf, st_u, st_k, st_i, vu16, vk16, pb0, pb1, ob,
            sem):
    x32, q32, k32, v32, wb, mf, hb, vu, vk = (
        r.bitcast(I32) for r in (xb, qb, kb, vb, wb16, mf16, hb16, vu16, vk16))
    c32 = craw.bitcast(I32)
    pb16 = (pb0, pb1)
    pb = (pb0.bitcast(I32), pb1.bitcast(I32))

    def rows(ref, start, n=8):
        return ref[pl.ds(start, n), :]

    def hint(v, n):
        return v if isinstance(v, int) or n == 1 else pl.multiple_of(v, n)

    def view(ref, start, n=None):
        return ref.at[pl.ds(hint(start, 16), n or ref.shape[0]), :]

    def after(ref):
        return _Zeros(view(ref, z8)[ref.shape[0] - 16:ref.shape[0] - 8, 0:128])

    small = [pltpu.make_async_copy(s, d, sem.at[S_SMALL]) for s, d in (
        (lre_hbm, lre_v), (lim_hbm, lim_v), (ldt_hbm, ldt_v),
        (dsk_hbm, dsk_v), (sd_hbm, sd_v), (tap_hbm, tap_v),
        (tab_hbm.at[pl.ds(288, 8), :], tab.at[pl.ds(288, 8), :]))]
    tab_dma = pltpu.make_async_copy(
        tab_hbm.at[pl.ds(0, 288), :], tab.at[pl.ds(0, 288), :], sem.at[S_B + 4])

    def x_dma(u, at):
        return [pltpu.make_async_copy(
            x_hbm.at[pl.ds(hint(u * UNIT, UNIT), UNIT), pl.ds(128 * n, 128)],
            xb.at[pl.ds(hint(n * L + u * UNIT, UNIT), UNIT), :], sem.at[at])
            for n in range(NG)]

    def b_dma(p):
        return [pltpu.make_async_copy(
            src.at[pl.ds(128 * p, 128), :], braw.at[pl.ds(D * c + 128 * p, 128), :],
            sem.at[S_B + p]) for c, src in enumerate((bre_hbm, bim_hbm))]

    c_dma = [pltpu.make_async_copy(
        src.at[:, pl.ds(128 * p, 128)], craw.at[pl.ds(D * (NG * c + p), D), :],
        sem.at[S_C]) for c, src in enumerate((cre_hbm, cim_hbm)) for p in range(NG)]

    def col_dma(which, g, sem_at):
        src, dst = ((k_hbm, kb), (v_hbm, vb), (q_hbm, qb))[which]
        return pltpu.make_async_copy(
            src.at[:, pl.ds(hint(128 * g, 128), 128)],
            dst.at[pl.ds(hint(L * g, L), L), :], sem.at[sem_at])

    def sk_dma(g, sem_at):
        t = hint(128 * g, 128)
        return pltpu.make_async_copy(
            sk_hbm.at[pl.ds(t, 128), :], skb.at[pl.ds(t, 128), :], sem.at[sem_at])

    def oa_dma(u, n):
        t = hint(u * UNIT, UNIT)
        return pltpu.make_async_copy(
            oa.at[pl.ds(t, UNIT), pl.ds(128 * n, 128)],
            o_hbm.at[pl.ds(t, UNIT), pl.ds(128 * n, 128)], sem.at[S_OUT])

    def oa_unit_dma(u):
        t = hint(u * UNIT, UNIT)
        return pltpu.make_async_copy(
            oa.at[pl.ds(t, UNIT), :], o_hbm.at[pl.ds(t, UNIT), pl.ds(0, D)], sem.at[S_OUT])

    def ob_dma(g, half):
        h = L // 2
        return pltpu.make_async_copy(
            ob.at[pl.ds(hint(L * g + h * half, h), h), :],
            o_hbm.at[pl.ds(h * half, h), pl.ds(hint(D + 128 * g, 128), 128)], sem.at[S_OUT])

    def start(ds):
        for d in ds:
            d.start()

    def wait(ds):
        for d in ds:
            d.wait()

    def prm(g, row):
        return rows(view(par, g * (P_ROWS * 8), P_ROWS * 8), row * 8)

    def bu_passes(u, slot, size=128, z=0, shift=False, raw=False):
        out = []
        xu, w = view(x32, u * (UNIT // 2), ((NG - 1) * L + UNIT) // 2), view(wb, z)
        order = [p + c * NG for p in range(NG) for c in range(2)]
        for n in order:
            sizes = [size] * (UNIT // size)
            if shift and n == order[0]:
                sizes = [32, 32, 96, 96]
            if shift and n == order[-1]:
                sizes = [64] * 4
            for m, MM in zip(np.cumsum([0] + sizes).tolist(), sizes):
                acc = []
                for kk in range(NG):
                    def lhs(m=m, kk=kk, MM=MM):
                        t = (kk * L + m) // 2
                        return [rows(xu, t + 8 * i) for i in range(MM // 16)]

                    def rhs(n=n, kk=kk):
                        if raw:
                            return braw[pl.ds(128 * n, 128), pl.ds(128 * kk, 128)]
                        return [rows(w, (n * NG + kk) * 64 + 8 * i) for i in range(8)]

                    def consume(d, m=m, n=n, kk=kk, acc=acc, MM=MM):
                        acc.append(d if kk == 0 else acc[-1] + d)
                        if kk == NG - 1:
                            for i in range(MM // 8):
                                seg, r = divmod(m + 8 * i, R)
                                row = 9 * (seg % 2 * R + r) + seg // 2
                                bu[pl.ds((slot * 2 * NG + n) * BU_PART + row, 8, stride=9), :] = (
                                    acc[-1][8 * i:8 * i + 8])
                    out.append((MM, lhs, rhs, consume))
        return out

    def scan_tasks(u, slot):
        steps, state = 2, {}
        hu = view(hb16, u * UNIT, (2 * NG - 1) * L + UNIT)

        def b(p, ch, r):
            return tuple(rows(bu, (slot * 2 * NG + c * NG + p) * BU_PART + 9 * (ch * R + r))
                         for c in range(2))

        def step(mu, h, br):
            return (mu[0] * h[0] + br[0]) - mu[1] * h[1], (mu[0] * h[1] + br[1]) + mu[1] * h[0]

        def ends(p, gate):
            mu, ties = (gate.value(prm(p, P_MU), PLAN["scan_lead"]), prm(p, P_MU + 1)), []
            h = [b(p, ch, 0) for ch in range(2)]
            for r in range(1, R):
                h = [step(mu, h[ch], b(p, ch, r)) for ch in range(2)]
                if r % steps == 0:
                    ties.append(h[r // steps % 2][0])
            state[p] = starts(p, h)
            return ties + [state[p][1][0]]

        def starts(p, e):
            last = lax.broadcasted_iota(I32, (8, 128), 0) == 7
            rho = (prm(p, P_RHO), prm(p, P_RHO + 1))
            pair = step(rho, e[0], e[1])
            a = tuple(pltpu.roll(jnp.where(last, rows(carry, (2 * p + c) * 8), pair[c]), 1, 0)
                      for c in range(2))
            for sh, row in ((1, P_RHO1), (2, P_RHO2), (4, P_RHO4)):
                a = step((prm(p, row), prm(p, row + 1)), tuple(pltpu.roll(c, sh, 0) for c in a), a)
            return [a, step(rho, a, e[0])]

        def run(p, r0, gate):
            if r0 == 0:
                state["mu"] = (prm(p, P_MU), prm(p, P_MU + 1))
            mu, h = (gate.value(state["mu"][0], PLAN["scan_lead"]), state["mu"][1]), state[p]
            for r in range(r0, r0 + steps):
                h = [step(mu, h[ch], b(p, ch, r)) for ch in range(2)]
                for c in range(2):
                    hu[pl.ds((c * NG + p) * L + 16 * r, 16), :] = _pack(h[0][c], h[1][c])
            state[p] = h
            if r0 + steps == R:
                for c in range(2):
                    carry[pl.ds((2 * p + c) * 8, 8), :] = h[1][c]
            return [after(hb)]

        tasks = []
        for p in range(NG):
            tasks.append(([16 * steps] * ((R - 1) // steps) + [46 + 16 * steps],
                          lambda gate, p=p: ends(p, gate)))
            tasks += [([18 * steps], lambda gate, p=p, r0=r0: run(p, r0, gate))
                      for r0 in range(0, R, steps)]
        return tasks

    def y_passes(h, n, sizes=(HALF,), z=0):
        out, w, hu = [], view(wc, z), view(hb, h * (HALF // 2), ((2 * NG - 1) * L + HALF) // 2)
        for t0, MM in zip(np.cumsum((0,) + sizes).tolist(), sizes):
            acc = []
            for kk in range(2 * NG):
                def lhs(t0=t0, kk=kk, MM=MM):
                    return [rows(hu, (kk * L + t0) // 2 + 8 * i) for i in range(MM // 16)]

                def rhs(kk=kk):
                    return [rows(w, (kk * NG + n) * 64 + 8 * i) for i in range(8)]

                def consume(d, t0=t0, kk=kk, acc=acc, MM=MM):
                    acc.append(d if kk == 0 else acc[-1] + d)
                    if kk == 2 * NG - 1:
                        for i in range(MM // 8):
                            r, ch = divmod(t0 // 8 + i, 2)
                            ys[pl.ds(n * YS_ROWS + ch * (R // 2 + 1) + r, 8, stride=R + 2), :] = (
                                acc[-1][8 * i:8 * i + 8])
                out.append((MM, lhs, rhs, consume))
        return out

    def skip_task(h, n):
        def fn(gate):
            dsk, ties = gate.value(prm(n, P_DSKIP), PLAN["skip_lead"]), []
            t = h // 2 * UNIT + h % 2 * (R // 2)
            edge = n == NG - 1 and isinstance(h, int)
            xu = x32.at[pl.ds(hint(t // 2 + n * (L // 2), 4), UNIT // 2 + (-4 if edge else 4)), :]
            ou = oa.at[pl.ds(hint(t, 8), UNIT - R // 2), :]
            for g in range(SEG):
                if g == SEG - 1 and edge:
                    xs = _unpack(rows(xu, 8 * g - 4))[1]
                else:
                    xs = _unpack(rows(xu, 8 * g))[0]
                y = rows(ys, n * YS_ROWS + g * (R // 2 + 1))
                ou[pl.ds(R * g, 8), pl.ds(128 * n, 128)] = y + xs * dsk
                if g % 8 == 7:
                    ties.append(after(oa))
            return ties
        return ([24, 24], fn)

    def widen_tasks(g):
        def fn(i0):
            kg = view(k32, g * (L // 2), L // 2)
            for i in range(i0, i0 + 8):
                lo, hi = _unpack(rows(kg, 8 * i))
                kf[pl.ds(KF_PAD + 16 * i, 8), :] = lo
                kf[pl.ds(KF_PAD + 16 * i + 8, 8), :] = hi
            return [after(kf)]
        return [([16], lambda gate, i=i: fn(i)) for i in range(0, L // 16, 8)]

    def transpose_tasks(g):
        def fn(c0):
            for c in (c0, c0 + 1):
                t = skb[pl.ds(hint(128 * g, 128), 128), pl.ds(128 * c, 128)]
                kt[pl.ds(64 * c, 64), :] = pltpu.bitcast(t.T, I32)
            return [after(kt)]
        return [([16], lambda gate, c=c: fn(c)) for c in range(0, L // 128, 2)]

    def staged(s, half, n, grp, c):
        return (((s * 2 + half) * 4 + n) * 4 + grp) * 16 + 8 * c

    ops1 = (18, 36, 30, 36)

    def transform_tasks(st, s, half, chunk, chunk_cost, direct):
        dst16, dst = (vu16, vu) if st is st_u else (vk16, vk)
        kept = []

        def first(gate, n):
            load = chunk(gate, n)
            u = [load(16 * half + n + 4 * m) for m in range(4)]
            pairs = _fwd1(n, [_Signed(v) for v in u])
            kept.append(pairs)
            for grp in range(2 * direct, 4):
                for c in range(2):
                    st[pl.ds(staged(s, half, n, grp, c), 8), :] = pairs[grp][c].get()
            return [u[0] + u[2]] * (chunk_cost > 4) + [after(st)]

        def second(grps):
            for grp in grps:
                if direct and grp < 2:
                    zs = [t[grp] for t in kept]
                else:
                    zs = [tuple(_Signed(rows(view(st, z8), staged(s, half, n, grp, c)))
                                for c in range(2)) for n in range(4)]
                for k, pair in enumerate(_fwd2(grp, zs)):
                    dst16[pl.ds(((4 * grp + k) * 2 + half) * 128 + 16 * s, 16), :] = (
                        _pack(pair[0].get(), pair[1].get()))
            return [after(dst)]

        split = (chunk_cost > 4) * (chunk_cost // 2 + 1)
        one = [([split] * (split > 0) + [chunk_cost + ops1[n] - split],
                lambda gate, n=n: first(gate, n)) for n in range(4)]
        two = [([40], lambda gate, grp=grp: second((grp, grp + 1))) for grp in (0, 2)]
        return (one + two[:1], two[1:]) if direct else (one, two)

    def kv_tasks(g):
        tasks = []
        for s in range(8):
            for half in range(2):
                def chunk(gate, n, s=s, loaded=[]):
                    if n == 0:
                        loaded[:] = [prm(g, P_TAP + t) for t in range(4)]
                    taps = [gate.value(loaded[0], PLAN["conv_lead"])] + loaded[1:]
                    kz, vg = view(kf, z8), view(v32, g * (L // 2), L // 2)

                    def load(c):
                        t = 64 * c + 8 * s
                        ks = rows(kz, KF_PAD + t) * taps[0]
                        for lag in range(1, 4):
                            ks = ks + rows(kz, KF_PAD + t - lag) * taps[lag]
                        return ks * _unpack(rows(vg, (t // 16) * 8))[s % 2]
                    return load
                tasks += sum(transform_tasks(st_u, s, half, chunk, 36, True), [])
        return tasks

    def filter_tasks(g, early):
        before, after_use = [], []
        for j in range(16):
            def chunk(gate, n, s=j // 2):
                def load(c):
                    v = _unpack(rows(view(kt, z8), 32 * c + 8 * (s // 2)))[s % 2]
                    if s == 0 and c == 0:
                        first = lax.broadcasted_iota(I32, (8, 128), 0) == 0
                        v = v + jnp.where(first, prm(g, P_SSMD), 0.0)
                    return v
                return load
            one, two = transform_tasks(st_k, j // 2, j % 2, chunk, 4, j >= early)
            before += one if j < early else []
            after_use += two if j < early else one + two
        return before, after_use

    def fwd_passes(grp):
        out = []
        for slot in range(4 * grp, 4 * grp + 4):
            got = []
            for src, half in ((vu, 0), (vk, 0), (vu, 1), (vk, 1)):
                def lhs(slot=slot):
                    return [rows(mf, slot * 64 + 8 * i) for i in range(8)]

                def rhs(slot=slot, src=src, half=half):
                    return [rows(view(src, z8), (2 * slot + half) * 64 + 8 * i) for i in range(8)]

                def consume(d, slot=slot, got=got):
                    got.append(d)
                    if len(got) < 4:
                        return
                    for i in range(8):
                        u0, k0, u1, k1 = (
                            (t[16 * i:16 * i + 8], t[16 * i + 8:16 * i + 16]) for t in got)
                        lo, a, b = _cmul(u0, k0), _cmul(u0, k1), _cmul(u1, k0)
                        if slot == _REAL_SLOT and i == 0:
                            first = lax.broadcasted_iota(I32, (8, 128), 0) == 0
                            lo, a, b = (
                                tuple(jnp.where(first, 0.5 * (x[c] * y[c]), p[c]) for c in range(2))
                                for p, x, y in ((lo, u0, k0), (a, u0, k1), (b, u1, k0)))
                        if _F1[slot] % 2:
                            hi = ((a[0] + b[0]) - lo[0], (a[1] + b[1]) - lo[1])
                        else:
                            hi = ((a[0] + b[0]) + lo[0], (a[1] + b[1]) + lo[1])
                        for half, p in enumerate((lo, hi)):
                            at = (slot % 4 * 2 + half) * 128 + 16 * i
                            pb16[grp % 2][pl.ds(at, 16), :] = _pack(*p)
                out.append((128, lhs, rhs, consume))
        return out

    def inv_passes(grp, half):
        out, got = [], []
        for slot in range(4 * grp, 4 * grp + 4):
            def lhs(slot=slot):
                return [rows(mi, slot * 64 + 8 * i) for i in range(8)]

            def rhs(slot=slot):
                return [rows(view(pb[grp % 2], z8), (slot % 4 * 2 + half) * 64 + 8 * i)
                        for i in range(8)]

            def consume(d):
                got.append(d)
                if len(got) < 4:
                    return
                for s in range(8):
                    w = [(_Signed(t[16 * s:16 * s + 8]), _Signed(t[16 * s + 8:16 * s + 16]))
                         for t in got]
                    for n, pair in enumerate(_inv2(grp, w)):
                        for c in range(2):
                            st_i[pl.ds(staged(s, half, n, grp, c), 8), :] = pair[c].get()
            out.append((128, lhs, rhs, consume))
        return out

    def inverse_tasks(g):
        def fn(gate, s, half):
            gate.loads(st_i, PLAN["inverse_lead"])
            qg, og, ties = view(q32, g * (L // 2), L // 2), view(ob, g * L, L), []
            for n in range(4):
                zs = [tuple(_Signed(rows(view(st_i, z8), staged(s, half, n, grp, c)))
                            for c in range(2)) for grp in range(4)]
                for m, y in enumerate(_inv1(n, zs)):
                    t = 64 * (16 * half + n + 4 * m) + 8 * s
                    og[pl.ds(t, 8), :] = _unpack(rows(qg, (t // 16) * 8))[s % 2] * y.get()
                ties.append(after(ob))
            return ties

        tasks = []
        for half in range(2):
            tasks += [([12 + n for n in ops1], lambda gate, s=s, half=half: fn(gate, s, half))
                      for s in range(8)]
            tasks.append(dma_task(ob_dma(g, half)))
        return tasks

    def dma_task(copy):
        return [1], lambda gate: copy.start()

    filter0 = x_dma(2, S_F0) + [sk_dma(0, S_F0)]
    data0 = x_dma(3, S_K0) + [col_dma(0, 0, S_K0), col_dma(1, 0, S_K0)]
    x0, x1 = x_dma(0, S_X0), x_dma(1, S_B + 4)

    def group_dma(g):
        at = S_COL + g
        return [col_dma(2, g, at), sk_dma(g + 1, at), col_dma(0, g + 1, at),
                col_dma(1, g + 1, at)] + x_dma(g + LEAD, at)

    last_dma = col_dma(2, NG - 1, S_SMALL)

    start(small + b_dma(0) + x0 + b_dma(1) + b_dma(2))
    wait(small)
    zeros = rows(tab, 288).astype(I32)
    z8 = pl.multiple_of(zeros[0, 0], 16)
    sub = lax.broadcasted_iota(I32, (8, 128), 0)
    pred = zeros == 0

    def stack(ref):
        v = ref[...].astype(F32).reshape(1, D)
        return jnp.concatenate([v[:, 128 * g:128 * (g + 1)] for g in range(NG)]
                               + [v[:, :128]] * (8 - NG), axis=0)

    lre, lim = stack(lre_v), stack(lim_v)
    dt = jnp.exp(stack(ldt_v)).astype(BF16).astype(F32)
    mag, ang = jnp.exp(dt * lre), dt * lim
    lam = (mag * jnp.cos(ang), mag * jnp.sin(ang))
    scale = jnp.maximum(jnp.abs(lre), jnp.abs(lim))
    nre, nim = lre / scale, lim / scale
    den = (nre * nre + nim * nim) * scale
    coef = _cmul(((lam[0] - 1.0) / den, lam[1] / den), (nre, -nim))
    mu = lam
    rho = [mu]
    for _ in range(R.bit_length() + 2):
        rho.append(_cmul(rho[-1], rho[-1]))
    dsk, ssd = stack(dsk_v), stack(sd_v)
    taps = tap_v[...].astype(F32) * _FFT_SCALE
    for g in range(NG):
        def put(row, v):
            par[pl.ds((g * P_ROWS + row) * 8, 8), :] = v

        def lanes(v):
            return jnp.broadcast_to(v[g:g + 1], (8, 128))
        for c in range(2):
            put(P_MU + c, lanes(mu[c]))
            put(P_RHO + c, lanes(rho[-4][c]))
            for n, row in enumerate((P_RHO1, P_RHO2, P_RHO4)):
                put(row + c, jnp.where(sub >= 1 << n, lanes(rho[n - 3][c]), 0.0))
        for t in range(4):
            put(P_TAP + t, jnp.broadcast_to(taps[t:t + 1, 128 * g:128 * (g + 1)], (8, 128)))
        put(P_COEF, lanes(2.0 * coef[0]))
        put(P_COEF + 2, lanes(-2.0 * coef[1]))
        put(P_SSMD, lanes(ssd))
        put(P_DSKIP, lanes(dsk))
    for ref in (hb, oa, kf, kt, vu, vk, st_u, st_k, ob, mf, mi, wb, wc):
        ref[pl.ds(ref.shape[0] - 16, 8), pl.ds(0, 128)] = jnp.zeros((8, 128), ref.dtype)
    for i in range(2 * NG):
        carry[pl.ds(8 * i, 8), :] = jnp.zeros((8, 128), F32)
    kf[pl.ds(0, KF_PAD), :] = jnp.zeros((KF_PAD, 128), F32)

    def matrix_task(slot):
        def fn(gate):
            if slot != _REAL_SLOT:
                c, s = tab[pl.ds(256 + slot, 1), :], tab[pl.ds(272 + slot, 1), :]
            for a in range(8):
                if slot == _REAL_SLOT:
                    re, im = rows(tab, 128 + 16 * a), rows(tab, 128 + 16 * a + 8)
                else:
                    br, bi = rows(tab, 16 * a), rows(tab, 16 * a + 8)
                    re, im = c * br - s * bi, s * br + c * bi
                mf16[pl.ds(slot * 128 + 16 * a, 16), :] = _pack(re, im)
            m = pltpu.bitcast(rows(view(mf, z8), slot * 64, 64), BF16)
            mi[pl.ds(slot * 64, 64), :] = pltpu.bitcast(m.T, I32)
            return [after(mf), after(mi)]
        return ([48, 8], fn)

    def b_task(p):
        def fn(gate):
            ties = []
            for n in (p, NG + p):
                for kk in range(NG):
                    t = braw[pl.ds(128 * n, 128), pl.ds(128 * kk, 128)]
                    wb[pl.ds((n * NG + kk) * 64, 64), :] = pltpu.bitcast(t.T, I32)
                    ties.append(after(wb))
            return ties
        return ([24] * (2 * NG), fn)

    def c_task(n, p):
        def fn(gate):
            cr, ci, nci = prm(p, P_COEF), prm(p, P_COEF + 1), prm(p, P_COEF + 2)
            t = [_unpack_tile(rows(c32, ((c * NG + p) * D + 128 * n) // 2, 64)) for c in range(2)]
            re = [_pack(cr * a0 + nci * b0, cr * a1 + nci * b1) for (a0, a1), (b0, b1) in zip(*t)]
            im = [_pack(nci * a0 - cr * b0, nci * a1 - cr * b1) for (a0, a1), (b0, b1) in zip(*t)]
            ties = []
            for c, tile in enumerate((re, im)):
                wc[pl.ds(((c * NG + p) * NG + n) * 64, 64), :] = pltpu.bitcast(
                    jnp.concatenate(tile, axis=0).T, I32)
                ties.append(after(wc))
            return ties
        return ([80, 80], fn)

    def y_block(halves, t0, lead, even, z=0):
        tiles = [(h, n) for h in halves for n in range(NG)]
        passes, plan = [], []
        for j, (h, n) in enumerate(tiles):
            sizes = (HALF,)
            if j == 0 and lead is not None:
                if not lead:
                    continue
                sizes = (32, 96)
            if j == even:
                sizes = (64, 64)
            if j == len(tiles) - 1:
                sizes = (96, 32)
            passes += y_passes(h, n, sizes, z)
            t0 += 20
            plan.append(([skip_task(h, n)], t0 + PLAN["skip"], t0 + PLAN["skip"] + 6))
        return passes, plan

    def conv_passes(between):
        passes = fwd_passes(0)
        for grp in range(1, 4):
            f = fwd_passes(grp)
            passes += f[:8] + inv_passes(grp - 1, 0) + f[8:] + inv_passes(grp - 1, 1)
        return passes + between[:8] + inv_passes(3, 0) + inv_passes(3, 1) + between[8:]

    unit = 2 * NG * NG * UNIT // 64

    first = bu_passes(0, 1, raw=True)
    first = [first[20 * p:20 * (p + 1)] for p in range(NG)]
    start(b_dma(3) + b_dma(4) + x1 + [tab_dma])
    wait(x0 + b_dma(0))
    _weave(first[0], [], pred)
    start(filter0)
    wait(b_dma(1))
    _weave(first[1], [], pred)
    start(data0 + c_dma)
    wait(b_dma(2))
    _weave(first[2], [([b_task(p) for p in range(2)], 0, 40)], pred)
    wait(b_dma(3))
    _weave(first[3], [([b_task(p) for p in range(2, 4)], 0, 40)], pred)
    start(group_dma(0))
    wait(b_dma(4) + x1 + [tab_dma])
    _weave(first[4] + bu_passes(1, 0, 64, z8), [
        ([b_task(4)], 0, 36), (scan_tasks(0, 1), 40, 40 + unit),
        ([matrix_task(slot) for slot in range(SLOTS)], 60, 200)], pred)
    start(group_dma(1))
    wait(filter0)
    _weave(bu_passes(2, 1, 64), [
        (scan_tasks(1, 0), 0, unit), (transpose_tasks(0), 8, 32),
        (filter_tasks(0, 0)[1], 36, unit)], pred)
    start(group_dma(2))
    wait(data0 + c_dma)
    yp, plan = y_block((0, 1), unit, None, 2, z8)
    kv = kv_tasks(0)
    _weave(bu_passes(3, 0, shift=True) + yp, plan + [
        (scan_tasks(2, 1), *PLAN["scan0"]), (widen_tasks(0), 0, 40),
        ([c_task(n, p) for n in range(NG) for p in range(NG)], *PLAN["scale_c"]),
        (kv[:-2], PLAN["forward0"], 2 * unit), (kv[-2:], 2 * unit, 2 * unit)], pred)
    start([oa_unit_dma(0)] + group_dma(3) + [last_dma])

    def body(i, _):
        wait(group_dma(i))
        halves = [2 + 3 * i + j for j in range(3)]
        y0 = 192 + 20 + unit
        yp, plan = y_block(halves, y0, False, 7)
        passes = conv_passes(y_passes(halves[0], 0, (32, 96))) + bu_passes(i + LEAD, 0) + yp
        early, late = filter_tasks(i + 1, PLAN["early"])
        kv, tail, end = kv_tasks(i + 1), PLAN["tail"], y0 + 280
        done = (3 * i + 2) // 2
        _weave(passes, plan + [
            ([dma_task(oa_unit_dma(done))], y0 + 210, y0 + 210),
            (scan_tasks(i + LEAD - 1, 0), *PLAN["scan"]),
            (transpose_tasks(i + 1), *PLAN["transpose"]),
            ([skip_task(halves[0], 0)], 232, 238),
            (widen_tasks(i + 1), *PLAN["widen"]), (early, *PLAN["filter_early"]),
            (inverse_tasks(i), *PLAN["inverse"]), (late, *PLAN["filter"]),
            (kv[:-tail], PLAN["forward"], end), (kv[-tail:], end, end)], pred)
        pl.when(i % 2 == 1)(lambda: start([oa_unit_dma(done + 1)]))
        return 0

    lax.fori_loop(0, NG - 1, body, 0)

    wait([last_dma])
    last = L // UNIT - 1
    yp, plan = y_block((2 * last, 2 * last + 1), 192, True, 2)
    plan += [([dma_task(oa_dma(last, n))], t + 6, t + 6) for n, (_, _, t) in enumerate(plan[NG:])]
    _weave(conv_passes(yp), plan + [
        (scan_tasks(last, 0), 0, 170), (inverse_tasks(NG - 1), *PLAN["last_inverse"])], pred)
    wait([oa_unit_dma(u) for u in range(last)] + [oa_dma(last, n) for n in range(NG)]
         + [ob_dma(n, half) for n in range(NG) for half in range(2)])


@jax.jit
def pallas_concat_heads__ssm_conv_s5__ssm_conv_h3__prompt_kernel(
    A_x: jax.Array,
    A_Lambda_re: jax.Array,
    A_Lambda_im: jax.Array,
    A_B_re: jax.Array,
    A_B_im: jax.Array,
    A_C_re: jax.Array,
    A_C_im: jax.Array,
    A_log_dt: jax.Array,
    A_Dskip: jax.Array,
    B_q: jax.Array,
    B_k: jax.Array,
    B_v: jax.Array,
    B_shift_k: jax.Array,
    B_ssm_k: jax.Array,
    B_ssm_D: jax.Array,
):
    assert A_x.shape == (1, L, D) and B_shift_k.shape == (D, 4)
    vmem = pltpu.VMEM
    dma = pltpu.SemaphoreType.DMA
    scratch = [
        vmem(_TABLES.shape, F32),
        vmem((D,), BF16), vmem((D,), BF16), vmem((D,), BF16), vmem((D,), BF16), vmem((D,), BF16),
        vmem((4, D), BF16),
        vmem((NG * L, 128), BF16),
        vmem((2 * D, D), BF16),
        vmem((2 * NG * D, 128), BF16),
        vmem((NG * L, 128), BF16),
        vmem((NG * L, 128), BF16),
        vmem((NG * L, 128), BF16),
        vmem((D, L), BF16),
        vmem((NG * P_ROWS * 8, 128), F32),
        vmem((2 * NG * D + 32, 128), BF16),
        vmem((2 * NG * NG * 64 + 16, 128), I32),
        vmem((SLOTS * 128 + 32, 128), BF16),
        vmem((SLOTS * 64 + 16, 128), I32),
        vmem((2 * 2 * NG * BU_PART, 128), F32),
        vmem((2 * NG * L + 32, 128), BF16),
        vmem((3 * NG * 8, 128), F32),
        vmem((NG * YS_ROWS, 128), F32),
        vmem((L + 16, D), F32),
        vmem((L // 2 + 16, 128), I32),
        vmem((KF_PAD + L + 16, 128), F32),
        vmem((2 * L + 16, 128), F32),
        vmem((2 * L + 16, 128), F32),
        vmem((2 * L + 8, 128), F32),
        vmem((32 * 128 + 32, 128), BF16),
        vmem((32 * 128 + 32, 128), BF16),
        vmem((8 * 128, 128), BF16),
        vmem((8 * 128, 128), BF16),
        vmem((NG * L + 16, 128), F32),
        dma((S_END,)),
    ]
    out = pl.pallas_call(
        _kernel,
        out_shape=jax.ShapeDtypeStruct((L, 2 * D), F32),
        in_specs=[pl.BlockSpec(memory_space=pl.ANY)] * 16,
        out_specs=pl.BlockSpec(memory_space=pl.ANY),
        scratch_shapes=scratch,
        compiler_params=pltpu.CompilerParams(vmem_limit_bytes=100 * 1024 * 1024),
        name="s5_h3",
    )(_TABLES, A_x.reshape(L, D), A_Lambda_re, A_Lambda_im, A_B_re, A_B_im, A_C_re, A_C_im,
      A_log_dt, A_Dskip, B_q.reshape(L, D), B_k.reshape(L, D), B_v.reshape(L, D),
      B_shift_k.T, B_ssm_k, B_ssm_D)
    return out.reshape(1, L, 2 * D)
```

```python
import math

import jax
import jax.numpy as jnp
import numpy as np
from jax import lax
from jax.experimental import pallas as pl
from jax.experimental.pallas import tpu as pltpu

F32, BF16, I32 = jnp.float32, jnp.bfloat16, jnp.int32

L = 2048
D = 640
NG = D // 128
UNIT = 256
SEG = 16
R = UNIT // SEG
LEAD = 4
HALF = UNIT // 2
BU_PART = 9 * 2 * R
YS_ROWS = SEG * (R // 2 + 1)
KF_PAD = 8


class _Signed:
    def __init__(self, v, neg=False):
        self.v, self.neg = v, neg

    def __neg__(self):
        return _Signed(self.v, not self.neg)

    def __add__(self, o):
        if self.neg == o.neg:
            return _Signed(self.v + o.v, self.neg)
        return _Signed(o.v - self.v if self.neg else self.v - o.v)

    def __sub__(self, o):
        return self + (-o)

    def __mul__(self, c):
        return _Signed(self.v * np.float32(-c if self.neg else c))

    def get(self):
        return -self.v if self.neg else self.v


def _rot(re, im, num, den):
    num %= den
    h = math.sqrt(0.5)
    if num == 0:
        return re, im
    if 4 * num == den:
        return -im, re
    if 4 * num == 3 * den:
        return im, -re
    if 8 * num == den:
        return (re - im) * h, (re + im) * h
    if 8 * num == 3 * den:
        return (re + im) * (-h), (re - im) * h
    if 8 * num == 5 * den:
        return (im - re) * h, (re + im) * (-h)
    if 8 * num == 7 * den:
        return (re + im) * h, (im - re) * h
    c = math.cos(2 * math.pi * num / den)
    s = math.sin(2 * math.pi * num / den)
    return re * c - im * s, re * s + im * c


def _dft4(z, sign):
    (r0, i0), (r1, i1), (r2, i2), (r3, i3) = z
    ar, ai, br, bi = r0 + r2, i0 + i2, r0 - r2, i0 - i2
    cr, ci, dr, di = r1 + r3, i1 + i3, r1 - r3, i1 - i3
    plus, minus = (br - di, bi + dr), (br + di, bi - dr)
    if sign < 0:
        plus, minus = minus, plus
    return [(ar + cr, ai + ci), plus, (ar - cr, ai - ci), minus]


def _fwd1(n, u):
    a0, a1, b0, b1 = u
    p, q = _rot(a0, b0, n, 32), _rot(a1, b1, n + 4, 32)
    s0, s1 = a0 + b0, a1 + b1
    return [(p[0] + q[0], p[1] + q[1]), _rot(p[0] - q[0], p[1] - q[1], n, 8),
            _rot(a0 - b0, a1 - b1, n, 16), (s0 + s1, s0 - s1)]


def _fwd2(grp, z):
    if grp < 3:
        return _dft4(z, 1)
    s4 = [t[0] for t in z]
    d4 = [t[1] for t in z]
    p = (d4[0], d4[2])
    q = _rot(d4[1], d4[3], 1, 8)
    s5 = [s4[0] + s4[2], s4[1] + s4[3]]
    return [
        (s5[0] + s5[1], s5[0] - s5[1]),
        (s4[0] - s4[2], s4[1] - s4[3]),
        (p[0] + q[0], p[1] + q[1]),
        (p[0] - q[0], p[1] - q[1]),
    ]


def _inv2(grp, w):
    if grp < 3:
        return _dft4(w, -1)
    s5 = [w[0][0] + w[0][1], w[0][0] - w[0][1]]
    s4 = [s5[0] + w[1][0], s5[1] + w[1][1], s5[0] - w[1][0], s5[1] - w[1][1]]
    p = (w[2][0] + w[3][0], w[2][1] + w[3][1])
    q = _rot(w[2][0] - w[3][0], w[2][1] - w[3][1], -1, 8)
    d4 = [p[0], q[0], p[1], q[1]]
    return [(s4[n], d4[n]) for n in range(4)]


def _inv1(n, z):
    e = _rot(*z[1], -n, 8)
    p = _rot(z[0][0] + e[0], z[0][1] + e[1], -n, 32)
    q = _rot(z[0][0] - e[0], z[0][1] - e[1], -(n + 4), 32)
    d0, d1 = _rot(*z[2], -n, 16)
    s0, s1 = z[3][0] + z[3][1], z[3][0] - z[3][1]
    return [p[0] + (s0 + d0), q[0] + (s1 + d1), p[1] + (s0 - d0), q[1] + (s1 - d1)]


_F1 = [4 * (g + 2 * k) + 1 for g in range(2) for k in range(4)]
_F1 += [2 * (4 * k + 1) for k in range(4)] + [0, 8, 4, 20]
_REAL_SLOT = 12
SLOTS = len(_F1)


def _dft_tables():
    kap = np.arange(128)
    j = 8 * (kap // 16) + kap % 8
    part = (kap // 8) % 2
    pr, pc, jr, jc = part[:, None], part[None, :], j[:, None], j[None, :]
    lo = 2 * np.pi * jr * jc / 64
    base = np.where(pr == pc, np.cos(lo), np.where(pr == 0, -np.sin(lo), np.sin(lo)))
    hi = 2 * np.pi * (16 + 32 * (jr - 32)) * jc / 2048
    v0 = np.where(pr == 0, np.cos(lo), np.where(jr == 0, np.cos(np.pi * jc), np.sin(lo)))
    v32 = np.where(pr == 0, np.cos(hi), np.sin(hi))
    real = np.where(jr < 32, np.where(pc == 0, v0, 0.0), np.where(pc == 1, v32, 0.0))
    th = 2 * np.pi * np.outer(np.array(_F1), j) / 2048
    zeros = np.zeros((8, 128))
    return np.concatenate([base, real, np.cos(th), np.sin(th), zeros]).astype(np.float32)


_TABLES = _dft_tables()
_FFT_SCALE = 2.0 ** -10

(P_MU, P_RHO, P_RHO1, P_RHO2, P_RHO4, P_TAP, P_SSMD, P_DSKIP, P_COEF, P_ROWS) = (
    0, 2, 4, 6, 8, 10, 14, 15, 16, 20)
S_SMALL, S_F0, S_K0, S_C, S_OUT, S_X0, S_B = range(7)
S_COL = S_B + NG
S_END = S_COL + NG - 1


def _cmul(a, b):
    return a[0] * b[0] - a[1] * b[1], a[0] * b[1] + a[1] * b[0]


def _pack(lo, hi):
    return jnp.concatenate([lo, hi], axis=0).astype(BF16)


def _unpack_tile(w):
    return [_unpack(w[8 * i:8 * i + 8]) for i in range(w.shape[0] // 8)]


def _unpack(w):
    v = pltpu.bitcast(w, BF16).astype(F32)
    return v[:8], v[8:]


PLAN = dict(
    scan_lead=22, conv_lead=20, inverse_lead=44, skip_lead=24,
    tiles=2, bties=5, scan=(0, 350), transpose=(60, 90), filter_early=(100, 216), early=4, inverse=(220, 380),
    widen=(216, 330), filter=(230, 480), forward=350, tail=3, skip=20,
    scale_c=(10, 220), scan0=(0, 350), forward0=110, last_inverse=(216, 290),
)


class _Zeros:
    def __init__(self, v):
        self.v = v


class _Gate:
    def __init__(self, pred=None, seen=()):
        self.pred, self.seen = pred, seen

    def early(self, lag):
        old = [e for e in self.seen if e[0] <= -lag]
        return max(old, key=lambda e: e[0])[1] if old else None

    def value(self, v, lag):
        early = self.early(lag)
        return v if early is None else jnp.where(self.pred, v, early)

    def loads(self, ref, lag):
        early = self.early(lag)
        if early is not None:
            ref[pl.ds(ref.shape[0] - 8, 8), :] = (
                early if ref.dtype == F32 else pltpu.bitcast(early, I32))


def _weave(passes, plan, pred):
    begin, clock = [], [0] * 4
    for i, (n, *_) in enumerate(passes):
        begin.append(clock[i % 4] / 16)
        clock[i % 4] += n

    def index(t):
        later = [i for i, b in enumerate(begin) if b >= t - 3.999]
        if not later:
            return len(passes)
        same = [i for i in later if begin[i] == min(begin[j] for j in later)]
        return same[min(max(int((t - begin[same[0]]) / 4 * len(same)), 0), len(same) - 1)]

    at = [[] for _ in range(len(passes) + 1)]
    for tasks, lo, hi in plan:
        total, done = sum(sum(c) for c, _ in tasks) or 1, 0.0
        for costs, fn in tasks:
            where = []
            for cost in costs:
                done += cost
                where.append(index(lo + done / total * (hi - lo)))
            at[min(where)].append((fn, where))
    seen, ties = [], [[] for _ in at]
    for i, fns in enumerate(at):
        now = (begin[i] + i % 4) if i < len(begin) else clock[0] / 16
        early = [(t - now, v) for t, v in seen]
        for fn, where in fns:
            for w, tie in zip(where, fn(_Gate(pred, early)) or ()):
                ties[w].append(tie)
        if i == len(passes):
            break
        n, lhs, rhs, consume = passes[i]
        w = rhs()
        if not isinstance(w, list):
            d = lax.dot_general(pltpu.bitcast(jnp.concatenate(lhs(), axis=0), BF16), w,
                                (((1,), (1,)), ((), ())), preferred_element_type=F32)
            consume(d)
            continue
        for tie in ties[i]:
            if isinstance(tie, _Zeros):
                v = tie.v
                w[-1] = w[-1] | (v if v.dtype == I32 else pltpu.bitcast(v, I32))
            else:
                w[-1] = jnp.where(pred, w[-1], pltpu.bitcast(tie, I32))
        d = jnp.dot(pltpu.bitcast(jnp.concatenate(lhs(), axis=0), BF16),
                    pltpu.bitcast(jnp.concatenate(w, axis=0), BF16), preferred_element_type=F32)
        seen += [(begin[i] + i % 4 + j // 16 - 4, d[j - 8:j]) for j in range(64, n + 1, 64)]
        consume(d)


def _kernel(tab_hbm, x_hbm, lre_hbm, lim_hbm, bre_hbm, bim_hbm, cre_hbm, cim_hbm,
            ldt_hbm, dsk_hbm, q_hbm, k_hbm, v_hbm, tap_hbm, sk_hbm, sd_hbm,
            o_hbm,
            tab, lre_v, lim_v, ldt_v, dsk_v, sd_v, tap_v,
            xb, braw, craw, qb, kb, vb, skb,
            par, wb16, wc, mf16, mi, bu, hb16, carry, ys, oa,
            kt, kf, st_u, st_k, st_i, vu16, vk16, pb0, pb1, ob,
            sem):
    x32, q32, k32, v32, wb, mf, hb, vu, vk = (
        r.bitcast(I32) for r in (xb, qb, kb, vb, wb16, mf16, hb16, vu16, vk16))
    c32 = craw.bitcast(I32)
    pb16 = (pb0, pb1)
    pb = (pb0.bitcast(I32), pb1.bitcast(I32))

    def rows(ref, start, n=8):
        return ref[pl.ds(start, n), :]

    def hint(v, n):
        return v if isinstance(v, int) or n == 1 else pl.multiple_of(v, n)

    def view(ref, start, n=None):
        return ref.at[pl.ds(hint(start, 16), n or ref.shape[0]), :]

    def after(ref):
        return _Zeros(view(ref, z8)[ref.shape[0] - 16:ref.shape[0] - 8, 0:128])

    small = [pltpu.make_async_copy(s, d, sem.at[S_SMALL]) for s, d in (
        (lre_hbm, lre_v), (lim_hbm, lim_v), (ldt_hbm, ldt_v),
        (dsk_hbm, dsk_v), (sd_hbm, sd_v), (tap_hbm, tap_v),
        (tab_hbm.at[pl.ds(288, 8), :], tab.at[pl.ds(288, 8), :]))]
    tab_dma = pltpu.make_async_copy(
        tab_hbm.at[pl.ds(0, 288), :], tab.at[pl.ds(0, 288), :], sem.at[S_B + 4])

    def x_dma(u, at):
        return [pltpu.make_async_copy(
            x_hbm.at[pl.ds(hint(u * UNIT, UNIT), UNIT), pl.ds(128 * n, 128)],
            xb.at[pl.ds(hint(n * L + u * UNIT, UNIT), UNIT), :], sem.at[at])
            for n in range(NG)]

    def b_dma(p):
        return [pltpu.make_async_copy(
            src.at[pl.ds(128 * p, 128), :], braw.at[pl.ds(D * c + 128 * p, 128), :],
            sem.at[S_B + p]) for c, src in enumerate((bre_hbm, bim_hbm))]

    c_dma = [pltpu.make_async_copy(
        src.at[:, pl.ds(128 * p, 128)], craw.at[pl.ds(D * (NG * c + p), D), :],
        sem.at[S_C]) for c, src in enumerate((cre_hbm, cim_hbm)) for p in range(NG)]

    def col_dma(which, g, sem_at):
        src, dst = ((k_hbm, kb), (v_hbm, vb), (q_hbm, qb))[which]
        return pltpu.make_async_copy(
            src.at[:, pl.ds(hint(128 * g, 128), 128)],
            dst.at[pl.ds(hint(L * g, L), L), :], sem.at[sem_at])

    def sk_dma(g, sem_at):
        t = hint(128 * g, 128)
        return pltpu.make_async_copy(
            sk_hbm.at[pl.ds(t, 128), :], skb.at[pl.ds(t, 128), :], sem.at[sem_at])

    def oa_dma(u, n):
        t = hint(u * UNIT, UNIT)
        return pltpu.make_async_copy(
            oa.at[pl.ds(t, UNIT), pl.ds(128 * n, 128)],
            o_hbm.at[pl.ds(t, UNIT), pl.ds(128 * n, 128)], sem.at[S_OUT])

    def oa_unit_dma(u):
        t = hint(u * UNIT, UNIT)
        return pltpu.make_async_copy(
            oa.at[pl.ds(t, UNIT), :], o_hbm.at[pl.ds(t, UNIT), pl.ds(0, D)], sem.at[S_OUT])

    def ob_dma(g, half):
        h = L // 2
        return pltpu.make_async_copy(
            ob.at[pl.ds(hint(L * g + h * half, h), h), :],
            o_hbm.at[pl.ds(h * half, h), pl.ds(hint(D + 128 * g, 128), 128)], sem.at[S_OUT])

    def start(ds):
        for d in ds:
            d.start()

    def wait(ds):
        for d in ds:
            d.wait()

    def prm(g, row):
        return rows(view(par, g * (P_ROWS * 8), P_ROWS * 8), row * 8)

    def bu_passes(u, slot, size=128, z=0, shift=False, raw=False, groups=range(NG)):
        out = []
        xu, w = view(x32, u * (UNIT // 2), ((NG - 1) * L + UNIT) // 2), view(wb, z)
        order = [p + c * NG for p in groups for c in range(2)]
        for n in order:
            sizes = [size] * (UNIT // size)
            if shift and n == order[0]:
                sizes = [32, 32, 96, 96]
            if shift and n == order[-1]:
                sizes = [64] * 4
            for m, MM in zip(np.cumsum([0] + sizes).tolist(), sizes):
                acc = []
                for kk in range(NG):
                    def lhs(m=m, kk=kk, MM=MM):
                        t = (kk * L + m) // 2
                        return [rows(xu, t + 8 * i) for i in range(MM // 16)]

                    def rhs(n=n, kk=kk):
                        if raw:
                            return braw[pl.ds(128 * n, 128), pl.ds(128 * kk, 128)]
                        return [rows(w, (n * NG + kk) * 64 + 8 * i) for i in range(8)]

                    def consume(d, m=m, n=n, kk=kk, acc=acc, MM=MM):
                        acc.append(d if kk == 0 else acc[-1] + d)
                        if kk == NG - 1:
                            for i in range(MM // 8):
                                seg, r = divmod(m + 8 * i, R)
                                row = 9 * (seg % 2 * R + r) + seg // 2
                                bu[pl.ds((slot * 2 * NG + n) * BU_PART + row, 8, stride=9), :] = (
                                    acc[-1][8 * i:8 * i + 8])
                    out.append((MM, lhs, rhs, consume))
        return out

    def scan_tasks(u, slot):
        steps, state = 2, {}
        hu = view(hb16, u * UNIT, (2 * NG - 1) * L + UNIT)

        def b(p, ch, r):
            return tuple(rows(bu, (slot * 2 * NG + c * NG + p) * BU_PART + 9 * (ch * R + r))
                         for c in range(2))

        def step(mu, h, br):
            return (mu[0] * h[0] + br[0]) - mu[1] * h[1], (mu[0] * h[1] + br[1]) + mu[1] * h[0]

        def ends(p, gate):
            mu, ties = (gate.value(prm(p, P_MU), PLAN["scan_lead"]), prm(p, P_MU + 1)), []
            h = [b(p, ch, 0) for ch in range(2)]
            for r in range(1, R):
                h = [step(mu, h[ch], b(p, ch, r)) for ch in range(2)]
                if r % steps == 0:
                    ties.append(h[r // steps % 2][0])
            state[p] = starts(p, h)
            return ties + [state[p][1][0]]

        def starts(p, e):
            last = lax.broadcasted_iota(I32, (8, 128), 0) == 7
            rho = (prm(p, P_RHO), prm(p, P_RHO + 1))
            pair = step(rho, e[0], e[1])
            a = tuple(pltpu.roll(jnp.where(last, rows(carry, (2 * p + c) * 8), pair[c]), 1, 0)
                      for c in range(2))
            for sh, row in ((1, P_RHO1), (2, P_RHO2), (4, P_RHO4)):
                a = step((prm(p, row), prm(p, row + 1)), tuple(pltpu.roll(c, sh, 0) for c in a), a)
            return [a, step(rho, a, e[0])]

        def run(p, r0, gate):
            if r0 == 0:
                state["mu"] = (prm(p, P_MU), prm(p, P_MU + 1))
            mu, h = (gate.value(state["mu"][0], PLAN["scan_lead"]), state["mu"][1]), state[p]
            for r in range(r0, r0 + steps):
                h = [step(mu, h[ch], b(p, ch, r)) for ch in range(2)]
                for c in range(2):
                    hu[pl.ds((c * NG + p) * L + 16 * r, 16), :] = _pack(h[0][c], h[1][c])
            state[p] = h
            if r0 + steps == R:
                for c in range(2):
                    carry[pl.ds((2 * p + c) * 8, 8), :] = h[1][c]
            return [after(hb)]

        tasks = []
        for p in range(NG):
            tasks.append(([16 * steps] * ((R - 1) // steps) + [46 + 16 * steps],
                          lambda gate, p=p: ends(p, gate)))
            tasks += [([18 * steps], lambda gate, p=p, r0=r0: run(p, r0, gate))
                      for r0 in range(0, R, steps)]
        return tasks

    def y_passes(h, n, sizes=(HALF,), z=0):
        out, w, hu = [], view(wc, z), view(hb, h * (HALF // 2), ((2 * NG - 1) * L + HALF) // 2)
        for t0, MM in zip(np.cumsum((0,) + sizes).tolist(), sizes):
            acc = []
            for kk in range(2 * NG):
                def lhs(t0=t0, kk=kk, MM=MM):
                    return [rows(hu, (kk * L + t0) // 2 + 8 * i) for i in range(MM // 16)]

                def rhs(kk=kk):
                    return [rows(w, (kk * NG + n) * 64 + 8 * i) for i in range(8)]

                def consume(d, t0=t0, kk=kk, acc=acc, MM=MM):
                    acc.append(d if kk == 0 else acc[-1] + d)
                    if kk == 2 * NG - 1:
                        for i in range(MM // 8):
                            r, ch = divmod(t0 // 8 + i, 2)
                            ys[pl.ds(n * YS_ROWS + ch * (R // 2 + 1) + r, 8, stride=R + 2), :] = (
                                acc[-1][8 * i:8 * i + 8])
                out.append((MM, lhs, rhs, consume))
        return out

    def skip_task(h, n):
        def fn(gate):
            dsk, ties = gate.value(prm(n, P_DSKIP), PLAN["skip_lead"]), []
            t = h // 2 * UNIT + h % 2 * (R // 2)
            edge = n == NG - 1 and isinstance(h, int)
            xu = x32.at[pl.ds(hint(t // 2 + n * (L // 2), 4), UNIT // 2 + (-4 if edge else 4)), :]
            ou = oa.at[pl.ds(hint(t, 8), UNIT - R // 2), :]
            for g in range(SEG):
                if g == SEG - 1 and edge:
                    xs = _unpack(rows(xu, 8 * g - 4))[1]
                else:
                    xs = _unpack(rows(xu, 8 * g))[0]
                y = rows(ys, n * YS_ROWS + g * (R // 2 + 1))
                ou[pl.ds(R * g, 8), pl.ds(128 * n, 128)] = y + xs * dsk
                if g % 8 == 7:
                    ties.append(after(oa))
            return ties
        return ([24, 24], fn)

    def widen_tasks(g):
        def fn(i0):
            kg = view(k32, g * (L // 2), L // 2)
            for i in range(i0, i0 + 8):
                lo, hi = _unpack(rows(kg, 8 * i))
                kf[pl.ds(KF_PAD + 16 * i, 8), :] = lo
                kf[pl.ds(KF_PAD + 16 * i + 8, 8), :] = hi
            return [after(kf)]
        return [([16], lambda gate, i=i: fn(i)) for i in range(0, L // 16, 8)]

    def transpose_tasks(g):
        n = PLAN["tiles"]

        def fn(c0):
            for c in range(c0, c0 + n):
                t = skb[pl.ds(hint(128 * g, 128), 128), pl.ds(128 * c, 128)]
                kt[pl.ds(64 * c, 64), :] = pltpu.bitcast(t.T, I32)
            return [after(kt)]
        return [([8 * n], lambda gate, c=c: fn(c)) for c in range(0, L // 128, n)]

    def staged(s, half, n, grp, c):
        return (((s * 2 + half) * 4 + n) * 4 + grp) * 16 + 8 * c

    ops1 = (18, 36, 30, 36)

    def transform_tasks(st, s, half, chunk, chunk_cost, direct):
        dst16, dst = (vu16, vu) if st is st_u else (vk16, vk)
        kept = []

        def first(gate, n):
            load = chunk(gate, n)
            u = [load(16 * half + n + 4 * m) for m in range(4)]
            pairs = _fwd1(n, [_Signed(v) for v in u])
            kept.append(pairs)
            for grp in range(2 * direct, 4):
                for c in range(2):
                    st[pl.ds(staged(s, half, n, grp, c), 8), :] = pairs[grp][c].get()
            return [u[0] + u[2]] * (chunk_cost > 4) + [after(st)]

        def second(grps):
            for grp in grps:
                if direct and grp < 2:
                    zs = [t[grp] for t in kept]
                else:
                    zs = [tuple(_Signed(rows(view(st, z8), staged(s, half, n, grp, c)))
                                for c in range(2)) for n in range(4)]
                for k, pair in enumerate(_fwd2(grp, zs)):
                    dst16[pl.ds(((4 * grp + k) * 2 + half) * 128 + 16 * s, 16), :] = (
                        _pack(pair[0].get(), pair[1].get()))
            return [after(dst)]

        split = (chunk_cost > 4) * (chunk_cost // 2 + 1)
        one = [([split] * (split > 0) + [chunk_cost + ops1[n] - split],
                lambda gate, n=n: first(gate, n)) for n in range(4)]
        two = [([40], lambda gate, grp=grp: second((grp, grp + 1))) for grp in (0, 2)]
        return (one + two[:1], two[1:]) if direct else (one, two)

    def kv_tasks(g):
        tasks = []
        for s in range(8):
            for half in range(2):
                def chunk(gate, n, s=s, loaded=[]):
                    if n == 0:
                        loaded[:] = [prm(g, P_TAP + t) for t in range(4)]
                    taps = [gate.value(loaded[0], PLAN["conv_lead"])] + loaded[1:]
                    kz, vg = view(kf, z8), view(v32, g * (L // 2), L // 2)

                    def load(c):
                        t = 64 * c + 8 * s
                        ks = rows(kz, KF_PAD + t) * taps[0]
                        for lag in range(1, 4):
                            ks = ks + rows(kz, KF_PAD + t - lag) * taps[lag]
                        return ks * _unpack(rows(vg, (t // 16) * 8))[s % 2]
                    return load
                tasks += sum(transform_tasks(st_u, s, half, chunk, 36, True), [])
        return tasks

    def filter_tasks(g, early):
        before, after_use = [], []
        for j in range(16):
            def chunk(gate, n, s=j // 2):
                def load(c):
                    v = _unpack(rows(view(kt, z8), 32 * c + 8 * (s // 2)))[s % 2]
                    if s == 0 and c == 0:
                        first = lax.broadcasted_iota(I32, (8, 128), 0) == 0
                        v = v + jnp.where(first, prm(g, P_SSMD), 0.0)
                    return v
                return load
            one, two = transform_tasks(st_k, j // 2, j % 2, chunk, 4, j >= early)
            before += one if j < early else []
            after_use += two if j < early else one + two
        return before, after_use

    def fwd_passes(grp):
        out = []
        for slot in range(4 * grp, 4 * grp + 4):
            got = []
            for src, half in ((vu, 0), (vk, 0), (vu, 1), (vk, 1)):
                def lhs(slot=slot):
                    return [rows(mf, slot * 64 + 8 * i) for i in range(8)]

                def rhs(slot=slot, src=src, half=half):
                    return [rows(view(src, z8), (2 * slot + half) * 64 + 8 * i) for i in range(8)]

                def consume(d, slot=slot, got=got):
                    got.append(d)
                    if len(got) < 4:
                        return
                    for i in range(8):
                        u0, k0, u1, k1 = (
                            (t[16 * i:16 * i + 8], t[16 * i + 8:16 * i + 16]) for t in got)
                        lo, a, b = _cmul(u0, k0), _cmul(u0, k1), _cmul(u1, k0)
                        if slot == _REAL_SLOT and i == 0:
                            first = lax.broadcasted_iota(I32, (8, 128), 0) == 0
                            lo, a, b = (
                                tuple(jnp.where(first, 0.5 * (x[c] * y[c]), p[c]) for c in range(2))
                                for p, x, y in ((lo, u0, k0), (a, u0, k1), (b, u1, k0)))
                        if _F1[slot] % 2:
                            hi = ((a[0] + b[0]) - lo[0], (a[1] + b[1]) - lo[1])
                        else:
                            hi = ((a[0] + b[0]) + lo[0], (a[1] + b[1]) + lo[1])
                        for half, p in enumerate((lo, hi)):
                            at = (slot % 4 * 2 + half) * 128 + 16 * i
                            pb16[grp % 2][pl.ds(at, 16), :] = _pack(*p)
                out.append((128, lhs, rhs, consume))
        return out

    def inv_passes(grp, half):
        out, got = [], []
        for slot in range(4 * grp, 4 * grp + 4):
            def lhs(slot=slot):
                return [rows(mi, slot * 64 + 8 * i) for i in range(8)]

            def rhs(slot=slot):
                return [rows(view(pb[grp % 2], z8), (slot % 4 * 2 + half) * 64 + 8 * i)
                        for i in range(8)]

            def consume(d):
                got.append(d)
                if len(got) < 4:
                    return
                for s in range(8):
                    w = [(_Signed(t[16 * s:16 * s + 8]), _Signed(t[16 * s + 8:16 * s + 16]))
                         for t in got]
                    for n, pair in enumerate(_inv2(grp, w)):
                        for c in range(2):
                            st_i[pl.ds(staged(s, half, n, grp, c), 8), :] = pair[c].get()
            out.append((128, lhs, rhs, consume))
        return out

    def inverse_tasks(g):
        def fn(gate, s, half):
            gate.loads(st_i, PLAN["inverse_lead"])
            qg, og, ties = view(q32, g * (L // 2), L // 2), view(ob, g * L, L), []
            for n in range(4):
                zs = [tuple(_Signed(rows(view(st_i, z8), staged(s, half, n, grp, c)))
                            for c in range(2)) for grp in range(4)]
                for m, y in enumerate(_inv1(n, zs)):
                    t = 64 * (16 * half + n + 4 * m) + 8 * s
                    og[pl.ds(t, 8), :] = _unpack(rows(qg, (t // 16) * 8))[s % 2] * y.get()
                ties.append(after(ob))
            return ties

        tasks = []
        for half in range(2):
            tasks += [([12 + n for n in ops1], lambda gate, s=s, half=half: fn(gate, s, half))
                      for s in range(8)]
            tasks.append(dma_task(ob_dma(g, half)))
        return tasks

    def dma_task(copy):
        return [1], lambda gate: copy.start()

    filter0 = x_dma(2, S_F0) + [sk_dma(0, S_F0)] + x_dma(3, S_F0)
    data0 = [col_dma(0, 0, S_K0), col_dma(1, 0, S_K0)]
    x0, x1 = x_dma(0, S_X0), x_dma(1, S_B + 4)

    def group_dma(g):
        at = S_COL + g
        return [col_dma(2, g, at), sk_dma(g + 1, at), col_dma(0, g + 1, at),
                col_dma(1, g + 1, at)] + x_dma(g + LEAD, at)

    last_dma = col_dma(2, NG - 1, S_SMALL)

    start(small + b_dma(0) + x0 + b_dma(1) + b_dma(2))
    wait(small)
    zeros = rows(tab, 288).astype(I32)
    z8 = pl.multiple_of(zeros[0, 0], 16)
    sub = lax.broadcasted_iota(I32, (8, 128), 0)
    pred = zeros == 0

    def stack(ref):
        v = ref[...].astype(F32).reshape(1, D)
        return jnp.concatenate([v[:, 128 * g:128 * (g + 1)] for g in range(NG)]
                               + [v[:, :128]] * (8 - NG), axis=0)

    lre, lim = stack(lre_v), stack(lim_v)
    dt = jnp.exp(stack(ldt_v)).astype(BF16).astype(F32)
    mag, ang = jnp.exp(dt * lre), dt * lim
    lam = (mag * jnp.cos(ang), mag * jnp.sin(ang))
    scale = jnp.maximum(jnp.abs(lre), jnp.abs(lim))
    nre, nim = lre / scale, lim / scale
    den = (nre * nre + nim * nim) * scale
    coef = _cmul(((lam[0] - 1.0) / den, lam[1] / den), (nre, -nim))
    mu = lam
    rho = [mu]
    for _ in range(R.bit_length() + 2):
        rho.append(_cmul(rho[-1], rho[-1]))
    dsk, ssd = stack(dsk_v), stack(sd_v)
    taps = tap_v[...].astype(F32) * _FFT_SCALE
    for g in range(NG):
        def put(row, v):
            par[pl.ds((g * P_ROWS + row) * 8, 8), :] = v

        def lanes(v):
            return jnp.broadcast_to(v[g:g + 1], (8, 128))
        for c in range(2):
            put(P_MU + c, lanes(mu[c]))
            put(P_RHO + c, lanes(rho[-4][c]))
            for n, row in enumerate((P_RHO1, P_RHO2, P_RHO4)):
                put(row + c, jnp.where(sub >= 1 << n, lanes(rho[n - 3][c]), 0.0))
        for t in range(4):
            put(P_TAP + t, jnp.broadcast_to(taps[t:t + 1, 128 * g:128 * (g + 1)], (8, 128)))
        put(P_COEF, lanes(2.0 * coef[0]))
        put(P_COEF + 2, lanes(-2.0 * coef[1]))
        put(P_SSMD, lanes(ssd))
        put(P_DSKIP, lanes(dsk))
    for ref in (hb, oa, kf, kt, vu, vk, st_u, st_k, ob, mf, mi, wb, wc):
        ref[pl.ds(ref.shape[0] - 16, 8), pl.ds(0, 128)] = jnp.zeros((8, 128), ref.dtype)
    for i in range(2 * NG):
        carry[pl.ds(8 * i, 8), :] = jnp.zeros((8, 128), F32)
    kf[pl.ds(0, KF_PAD), :] = jnp.zeros((KF_PAD, 128), F32)

    def matrix_task(slot):
        def fn(gate):
            if slot != _REAL_SLOT:
                c, s = tab[pl.ds(256 + slot, 1), :], tab[pl.ds(272 + slot, 1), :]
            for a in range(8):
                if slot == _REAL_SLOT:
                    re, im = rows(tab, 128 + 16 * a), rows(tab, 128 + 16 * a + 8)
                else:
                    br, bi = rows(tab, 16 * a), rows(tab, 16 * a + 8)
                    re, im = c * br - s * bi, s * br + c * bi
                mf16[pl.ds(slot * 128 + 16 * a, 16), :] = _pack(re, im)
            m = pltpu.bitcast(rows(view(mf, z8), slot * 64, 64), BF16)
            mi[pl.ds(slot * 64, 64), :] = pltpu.bitcast(m.T, I32)
            return [after(mf), after(mi)]
        return ([48, 8], fn)

    def b_task(p):
        def fn(gate):
            ties = []
            for n in (p, NG + p):
                for kk in range(NG):
                    t = braw[pl.ds(128 * n, 128), pl.ds(128 * kk, 128)]
                    wb[pl.ds((n * NG + kk) * 64, 64), :] = pltpu.bitcast(t.T, I32)
                    if (kk + 1) % PLAN["bties"] == 0:
                        ties.append(after(wb))
            return ties
        return ([24] * (2 * NG // PLAN["bties"]), fn)

    def c_task(n, p):
        def fn(gate):
            cr, ci, nci = prm(p, P_COEF), prm(p, P_COEF + 1), prm(p, P_COEF + 2)
            t = [_unpack_tile(rows(c32, ((c * NG + p) * D + 128 * n) // 2, 64)) for c in range(2)]
            re = [_pack(cr * a0 + nci * b0, cr * a1 + nci * b1) for (a0, a1), (b0, b1) in zip(*t)]
            im = [_pack(nci * a0 - cr * b0, nci * a1 - cr * b1) for (a0, a1), (b0, b1) in zip(*t)]
            ties = []
            for c, tile in enumerate((re, im)):
                wc[pl.ds(((c * NG + p) * NG + n) * 64, 64), :] = pltpu.bitcast(
                    jnp.concatenate(tile, axis=0).T, I32)
                ties.append(after(wc))
            return ties
        return ([80, 80], fn)

    def y_block(halves, t0, lead, even, z=0):
        tiles = [(h, n) for h in halves for n in range(NG)]
        passes, plan = [], []
        for j, (h, n) in enumerate(tiles):
            sizes = (HALF,)
            if j == 0 and lead is not None:
                if not lead:
                    continue
                sizes = (32, 96)
            if j == even:
                sizes = (64, 64)
            if j == len(tiles) - 1:
                sizes = (96, 32)
            passes += y_passes(h, n, sizes, z)
            t0 += 20
            plan.append(([skip_task(h, n)], t0 + PLAN["skip"], t0 + PLAN["skip"] + 6))
        return passes, plan

    def conv_passes(between):
        passes = fwd_passes(0)
        for grp in range(1, 4):
            f = fwd_passes(grp)
            passes += f[:8] + inv_passes(grp - 1, 0) + f[8:] + inv_passes(grp - 1, 1)
        return passes + between[:8] + inv_passes(3, 0) + inv_passes(3, 1) + between[8:]

    unit = 2 * NG * NG * UNIT // 64

    first = bu_passes(0, 1, raw=True)
    first = [first[20 * p:20 * (p + 1)] for p in range(NG)]
    wait(x0 + b_dma(0))
    start(b_dma(3) + b_dma(4) + x1 + [tab_dma])
    _weave(first[0], [], pred)
    start(filter0)
    wait(b_dma(1))
    _weave(first[1], [], pred)
    start(data0 + c_dma)
    wait(b_dma(2))
    _weave(first[2], [([b_task(p) for p in range(2)], 0, 40)], pred)
    wait(b_dma(3))
    _weave(first[3], [([b_task(p) for p in range(2, 4)], 0, 40)], pred)
    start(group_dma(0))
    wait(b_dma(4) + x1 + [tab_dma])
    _weave(first[4] + bu_passes(1, 0, 64, z8), [
        ([b_task(4)], 0, 36), (scan_tasks(0, 1), 40, 40 + unit),
        ([matrix_task(slot) for slot in range(SLOTS)], 60, 200)], pred)
    start(group_dma(1))
    wait(filter0)
    _weave(bu_passes(2, 1, 64) + bu_passes(3, 0, 64, groups=[0]), [
        (scan_tasks(1, 0), 0, unit), (transpose_tasks(0), 8, 32),
        (filter_tasks(0, 0)[1], 36, unit + 40)], pred)
    start(group_dma(2))
    wait(data0 + c_dma)
    yp, plan = y_block((0, 1), unit - 40, None, 2, z8)
    kv = kv_tasks(0)
    end = 2 * unit - 40
    _weave(bu_passes(3, 0, shift=True, groups=range(1, NG)) + yp, plan + [
        (scan_tasks(2, 1), *PLAN["scan0"]), (widen_tasks(0), 0, 40),
        ([c_task(n, p) for n in range(NG) for p in range(NG)], *PLAN["scale_c"]),
        (kv[:-2], PLAN["forward0"], end), (kv[-2:], end, end)], pred)
    start([oa_unit_dma(0)] + group_dma(3) + [last_dma])

    def body(i, _):
        wait(group_dma(i))
        halves = [2 + 3 * i + j for j in range(3)]
        y0 = 192 + 20 + unit
        yp, plan = y_block(halves, y0, False, 7)
        passes = conv_passes(y_passes(halves[0], 0, (32, 96))) + bu_passes(i + LEAD, 0) + yp
        early, late = filter_tasks(i + 1, PLAN["early"])
        kv, tail, end = kv_tasks(i + 1), PLAN["tail"], y0 + 280
        done = (3 * i + 2) // 2
        _weave(passes, plan + [
            ([dma_task(oa_unit_dma(done))], y0 + 210, y0 + 210),
            (scan_tasks(i + LEAD - 1, 0), *PLAN["scan"]),
            (transpose_tasks(i + 1), *PLAN["transpose"]),
            ([skip_task(halves[0], 0)], 232, 238),
            (widen_tasks(i + 1), *PLAN["widen"]), (early, *PLAN["filter_early"]),
            (inverse_tasks(i), *PLAN["inverse"]), (late, *PLAN["filter"]),
            (kv[:-tail], PLAN["forward"], end), (kv[-tail:], end, end)], pred)
        pl.when(i % 2 == 1)(lambda: start([oa_unit_dma(done + 1)]))
        return 0

    lax.fori_loop(0, NG - 1, body, 0)

    wait([last_dma])
    last = L // UNIT - 1
    yp, plan = y_block((2 * last, 2 * last + 1), 192, True, 2)
    plan += [([dma_task(oa_dma(last, n))], t + 6, t + 6) for n, (_, _, t) in enumerate(plan[NG:])]
    _weave(conv_passes(yp), plan + [
        (scan_tasks(last, 0), 0, 170), (inverse_tasks(NG - 1), *PLAN["last_inverse"])], pred)
    wait([oa_unit_dma(u) for u in range(last)] + [oa_dma(last, n) for n in range(NG)]
         + [ob_dma(n, half) for n in range(NG) for half in range(2)])


@jax.jit
def pallas_concat_heads__ssm_conv_s5__ssm_conv_h3__prompt_kernel(
    A_x: jax.Array,
    A_Lambda_re: jax.Array,
    A_Lambda_im: jax.Array,
    A_B_re: jax.Array,
    A_B_im: jax.Array,
    A_C_re: jax.Array,
    A_C_im: jax.Array,
    A_log_dt: jax.Array,
    A_Dskip: jax.Array,
    B_q: jax.Array,
    B_k: jax.Array,
    B_v: jax.Array,
    B_shift_k: jax.Array,
    B_ssm_k: jax.Array,
    B_ssm_D: jax.Array,
):
    assert A_x.shape == (1, L, D) and B_shift_k.shape == (D, 4)
    vmem = pltpu.VMEM
    dma = pltpu.SemaphoreType.DMA
    scratch = [
        vmem(_TABLES.shape, F32),
        vmem((D,), BF16), vmem((D,), BF16), vmem((D,), BF16), vmem((D,), BF16), vmem((D,), BF16),
        vmem((4, D), BF16),
        vmem((NG * L, 128), BF16),
        vmem((2 * D, D), BF16),
        vmem((2 * NG * D, 128), BF16),
        vmem((NG * L, 128), BF16),
        vmem((NG * L, 128), BF16),
        vmem((NG * L, 128), BF16),
        vmem((D, L), BF16),
        vmem((NG * P_ROWS * 8, 128), F32),
        vmem((2 * NG * D + 32, 128), BF16),
        vmem((2 * NG * NG * 64 + 16, 128), I32),
        vmem((SLOTS * 128 + 32, 128), BF16),
        vmem((SLOTS * 64 + 16, 128), I32),
        vmem((2 * 2 * NG * BU_PART, 128), F32),
        vmem((2 * NG * L + 32, 128), BF16),
        vmem((3 * NG * 8, 128), F32),
        vmem((NG * YS_ROWS, 128), F32),
        vmem((L + 16, D), F32),
        vmem((L // 2 + 16, 128), I32),
        vmem((KF_PAD + L + 16, 128), F32),
        vmem((2 * L + 16, 128), F32),
        vmem((2 * L + 16, 128), F32),
        vmem((2 * L + 8, 128), F32),
        vmem((32 * 128 + 32, 128), BF16),
        vmem((32 * 128 + 32, 128), BF16),
        vmem((8 * 128, 128), BF16),
        vmem((8 * 128, 128), BF16),
        vmem((NG * L + 16, 128), F32),
        dma((S_END,)),
    ]
    out = pl.pallas_call(
        _kernel,
        out_shape=jax.ShapeDtypeStruct((L, 2 * D), F32),
        in_specs=[pl.BlockSpec(memory_space=pl.ANY)] * 16,
        out_specs=pl.BlockSpec(memory_space=pl.ANY),
        scratch_shapes=scratch,
        compiler_params=pltpu.CompilerParams(vmem_limit_bytes=100 * 1024 * 1024),
        name="s5_h3",
    )(_TABLES, A_x.reshape(L, D), A_Lambda_re, A_Lambda_im, A_B_re, A_B_im, A_C_re, A_C_im,
      A_log_dt, A_Dskip, B_q.reshape(L, D), B_k.reshape(L, D), B_v.reshape(L, D),
      B_shift_k.T, B_ssm_k, B_ssm_D)
    return out.reshape(1, L, 2 * D)
```

```python
import math

import jax
import jax.numpy as jnp
import numpy as np
from jax import lax
from jax.experimental import pallas as pl
from jax.experimental.pallas import tpu as pltpu

F32, BF16, I32 = jnp.float32, jnp.bfloat16, jnp.int32

L = 2048
D = 640
NG = D // 128
UNIT = 256
SEG = 16
R = UNIT // SEG
LEAD = 4
HALF = UNIT // 2
BU_PART = 9 * 2 * R
YS_ROWS = SEG * (R // 2 + 1)
KF_PAD = 8


class _Signed:
    def __init__(self, v, neg=False):
        self.v, self.neg = v, neg

    def __neg__(self):
        return _Signed(self.v, not self.neg)

    def __add__(self, o):
        if self.neg == o.neg:
            return _Signed(self.v + o.v, self.neg)
        return _Signed(o.v - self.v if self.neg else self.v - o.v)

    def __sub__(self, o):
        return self + (-o)

    def __mul__(self, c):
        return _Signed(self.v * np.float32(-c if self.neg else c))

    def get(self):
        return -self.v if self.neg else self.v


def _rot(re, im, num, den):
    num %= den
    h = math.sqrt(0.5)
    if num == 0:
        return re, im
    if 4 * num == den:
        return -im, re
    if 4 * num == 3 * den:
        return im, -re
    if 8 * num == den:
        return (re - im) * h, (re + im) * h
    if 8 * num == 3 * den:
        return (re + im) * (-h), (re - im) * h
    if 8 * num == 5 * den:
        return (im - re) * h, (re + im) * (-h)
    if 8 * num == 7 * den:
        return (re + im) * h, (im - re) * h
    c = math.cos(2 * math.pi * num / den)
    s = math.sin(2 * math.pi * num / den)
    return re * c - im * s, re * s + im * c


def _dft4(z, sign):
    (r0, i0), (r1, i1), (r2, i2), (r3, i3) = z
    ar, ai, br, bi = r0 + r2, i0 + i2, r0 - r2, i0 - i2
    cr, ci, dr, di = r1 + r3, i1 + i3, r1 - r3, i1 - i3
    plus, minus = (br - di, bi + dr), (br + di, bi - dr)
    if sign < 0:
        plus, minus = minus, plus
    return [(ar + cr, ai + ci), plus, (ar - cr, ai - ci), minus]


def _fwd1(n, u):
    a0, a1, b0, b1 = u
    p, q = _rot(a0, b0, n, 32), _rot(a1, b1, n + 4, 32)
    s0, s1 = a0 + b0, a1 + b1
    return [(p[0] + q[0], p[1] + q[1]), _rot(p[0] - q[0], p[1] - q[1], n, 8),
            _rot(a0 - b0, a1 - b1, n, 16), (s0 + s1, s0 - s1)]


def _fwd2(grp, z):
    if grp < 3:
        return _dft4(z, 1)
    s4 = [t[0] for t in z]
    d4 = [t[1] for t in z]
    p = (d4[0], d4[2])
    q = _rot(d4[1], d4[3], 1, 8)
    s5 = [s4[0] + s4[2], s4[1] + s4[3]]
    return [
        (s5[0] + s5[1], s5[0] - s5[1]),
        (s4[0] - s4[2], s4[1] - s4[3]),
        (p[0] + q[0], p[1] + q[1]),
        (p[0] - q[0], p[1] - q[1]),
    ]


def _inv2(grp, w):
    if grp < 3:
        return _dft4(w, -1)
    s5 = [w[0][0] + w[0][1], w[0][0] - w[0][1]]
    s4 = [s5[0] + w[1][0], s5[1] + w[1][1], s5[0] - w[1][0], s5[1] - w[1][1]]
    p = (w[2][0] + w[3][0], w[2][1] + w[3][1])
    q = _rot(w[2][0] - w[3][0], w[2][1] - w[3][1], -1, 8)
    d4 = [p[0], q[0], p[1], q[1]]
    return [(s4[n], d4[n]) for n in range(4)]


def _inv1(n, z):
    e = _rot(*z[1], -n, 8)
    p = _rot(z[0][0] + e[0], z[0][1] + e[1], -n, 32)
    q = _rot(z[0][0] - e[0], z[0][1] - e[1], -(n + 4), 32)
    d0, d1 = _rot(*z[2], -n, 16)
    s0, s1 = z[3][0] + z[3][1], z[3][0] - z[3][1]
    return [p[0] + (s0 + d0), q[0] + (s1 + d1), p[1] + (s0 - d0), q[1] + (s1 - d1)]


_F1 = [4 * (g + 2 * k) + 1 for g in range(2) for k in range(4)]
_F1 += [2 * (4 * k + 1) for k in range(4)] + [0, 8, 4, 20]
_REAL_SLOT = 12
SLOTS = len(_F1)


def _dft_tables():
    kap = np.arange(128)
    j = 8 * (kap // 16) + kap % 8
    part = (kap // 8) % 2
    pr, pc, jr, jc = part[:, None], part[None, :], j[:, None], j[None, :]
    lo = 2 * np.pi * jr * jc / 64
    base = np.where(pr == pc, np.cos(lo), np.where(pr == 0, -np.sin(lo), np.sin(lo)))
    hi = 2 * np.pi * (16 + 32 * (jr - 32)) * jc / 2048
    v0 = np.where(pr == 0, np.cos(lo), np.where(jr == 0, np.cos(np.pi * jc), np.sin(lo)))
    v32 = np.where(pr == 0, np.cos(hi), np.sin(hi))
    real = np.where(jr < 32, np.where(pc == 0, v0, 0.0), np.where(pc == 1, v32, 0.0))
    th = 2 * np.pi * np.outer(np.array(_F1), j) / 2048
    zeros = np.zeros((8, 128))
    return np.concatenate([base, real, np.cos(th), np.sin(th), zeros]).astype(np.float32)


_TABLES = _dft_tables()
_FFT_SCALE = 2.0 ** -10

(P_MU, P_RHO, P_RHO1, P_RHO2, P_RHO4, P_TAP, P_SSMD, P_DSKIP, P_COEF, P_ROWS) = (
    0, 2, 4, 6, 8, 10, 14, 15, 16, 20)
S_SMALL, S_F0, S_K0, S_C, S_OUT, S_X0, S_B = range(7)
S_COL = S_B + NG
S_END = S_COL + NG - 1


def _cmul(a, b):
    return a[0] * b[0] - a[1] * b[1], a[0] * b[1] + a[1] * b[0]


def _pack(lo, hi):
    return jnp.concatenate([lo, hi], axis=0).astype(BF16)


def _unpack_tile(w):
    return [_unpack(w[8 * i:8 * i + 8]) for i in range(w.shape[0] // 8)]


def _unpack(w):
    v = pltpu.bitcast(w, BF16).astype(F32)
    return v[:8], v[8:]


PLAN = dict(
    scan_lead=22, conv_lead=20, inverse_lead=44, skip_lead=24,
    scan=(0, 350), transpose=(60, 90), filter_early=(100, 216), early=4, inverse=(220, 380),
    widen=(216, 330), filter=(230, 480), forward=350, tail=3, skip=28,
    scale_c=(10, 220), scan0=(0, 350), forward0=110, last_inverse=(216, 290),
)


class _Zeros:
    def __init__(self, v):
        self.v = v


class _Gate:
    def __init__(self, pred=None, seen=()):
        self.pred, self.seen = pred, seen

    def early(self, lag):
        old = [e for e in self.seen if e[0] <= -lag]
        return max(old, key=lambda e: e[0])[1] if old else None

    def value(self, v, lag):
        early = self.early(lag)
        return v if early is None else jnp.where(self.pred, v, early)

    def loads(self, ref, lag):
        early = self.early(lag)
        if early is not None:
            ref[pl.ds(ref.shape[0] - 8, 8), :] = (
                early if ref.dtype == F32 else pltpu.bitcast(early, I32))


def _weave(passes, plan, pred):
    begin, clock = [], [0] * 4
    for i, (n, *_) in enumerate(passes):
        begin.append(clock[i % 4] / 16)
        clock[i % 4] += n

    def index(t):
        later = [i for i, b in enumerate(begin) if b >= t - 3.999]
        if not later:
            return len(passes)
        same = [i for i in later if begin[i] == min(begin[j] for j in later)]
        return same[min(max(int((t - begin[same[0]]) / 4 * len(same)), 0), len(same) - 1)]

    at = [[] for _ in range(len(passes) + 1)]
    for tasks, lo, hi in plan:
        total, done = sum(sum(c) for c, _ in tasks) or 1, 0.0
        for costs, fn in tasks:
            where = []
            for cost in costs:
                done += cost
                where.append(index(lo + done / total * (hi - lo)))
            at[min(where)].append((fn, where))
    seen, ties = [], [[] for _ in at]
    for i, fns in enumerate(at):
        now = (begin[i] + i % 4) if i < len(begin) else clock[0] / 16
        early = [(t - now, v) for t, v in seen]
        for fn, where in fns:
            for w, tie in zip(where, fn(_Gate(pred, early)) or ()):
                ties[w].append(tie)
        if i == len(passes):
            break
        n, lhs, rhs, consume = passes[i]
        w = rhs()
        if not isinstance(w, list):
            d = lax.dot_general(pltpu.bitcast(jnp.concatenate(lhs(), axis=0), BF16), w,
                                (((1,), (1,)), ((), ())), preferred_element_type=F32)
            consume(d)
            continue
        for tie in ties[i]:
            if isinstance(tie, _Zeros):
                v = tie.v
                w[-1] = w[-1] | (v if v.dtype == I32 else pltpu.bitcast(v, I32))
            else:
                w[-1] = jnp.where(pred, w[-1], pltpu.bitcast(tie, I32))
        d = jnp.dot(pltpu.bitcast(jnp.concatenate(lhs(), axis=0), BF16),
                    pltpu.bitcast(jnp.concatenate(w, axis=0), BF16), preferred_element_type=F32)
        seen += [(begin[i] + i % 4 + j // 16 - 4, d[j - 8:j]) for j in range(64, n + 1, 64)]
        consume(d)


def _kernel(tab_hbm, x_hbm, lre_hbm, lim_hbm, bre_hbm, bim_hbm, cre_hbm, cim_hbm,
            ldt_hbm, dsk_hbm, q_hbm, k_hbm, v_hbm, tap_hbm, sk_hbm, sd_hbm,
            o_hbm,
            tab, lre_v, lim_v, ldt_v, dsk_v, sd_v, tap_v,
            xb, braw, craw, qb, kb, vb, skb,
            par, wb16, wc, mf16, mi, bu, hb16, carry, ys, oa,
            kt, kf, st_u, st_k, st_i, vu16, vk16, pb0, pb1, ob,
            sem):
    x32, q32, k32, v32, wb, mf, hb, vu, vk = (
        r.bitcast(I32) for r in (xb, qb, kb, vb, wb16, mf16, hb16, vu16, vk16))
    c32 = craw.bitcast(I32)
    pb16 = (pb0, pb1)
    pb = (pb0.bitcast(I32), pb1.bitcast(I32))

    def rows(ref, start, n=8):
        return ref[pl.ds(start, n), :]

    def hint(v, n):
        return v if isinstance(v, int) or n == 1 else pl.multiple_of(v, n)

    def view(ref, start, n=None):
        return ref.at[pl.ds(hint(start, 16), n or ref.shape[0]), :]

    def after(ref):
        return _Zeros(view(ref, z8)[ref.shape[0] - 16:ref.shape[0] - 8, 0:128])

    small = [pltpu.make_async_copy(s, d, sem.at[S_SMALL]) for s, d in (
        (lre_hbm, lre_v), (lim_hbm, lim_v), (ldt_hbm, ldt_v),
        (dsk_hbm, dsk_v), (sd_hbm, sd_v), (tap_hbm, tap_v),
        (tab_hbm.at[pl.ds(288, 8), :], tab.at[pl.ds(288, 8), :]))]
    tab_dma = pltpu.make_async_copy(
        tab_hbm.at[pl.ds(0, 288), :], tab.at[pl.ds(0, 288), :], sem.at[S_B + 4])

    def x_dma(u, at):
        return [pltpu.make_async_copy(
            x_hbm.at[pl.ds(hint(u * UNIT, UNIT), UNIT), pl.ds(128 * n, 128)],
            xb.at[pl.ds(hint(n * L + u * UNIT, UNIT), UNIT), :], sem.at[at])
            for n in range(NG)]

    def b_dma(p):
        return [pltpu.make_async_copy(
            src.at[pl.ds(128 * p, 128), :], braw.at[pl.ds(D * c + 128 * p, 128), :],
            sem.at[S_B + p]) for c, src in enumerate((bre_hbm, bim_hbm))]

    c_dma = [pltpu.make_async_copy(
        src.at[:, pl.ds(128 * p, 128)], craw.at[pl.ds(D * (NG * c + p), D), :],
        sem.at[S_C]) for c, src in enumerate((cre_hbm, cim_hbm)) for p in range(NG)]

    def col_dma(which, g, sem_at):
        src, dst = ((k_hbm, kb), (v_hbm, vb), (q_hbm, qb))[which]
        return pltpu.make_async_copy(
            src.at[:, pl.ds(hint(128 * g, 128), 128)],
            dst.at[pl.ds(hint(L * g, L), L), :], sem.at[sem_at])

    def sk_dma(g, sem_at):
        t = hint(128 * g, 128)
        return pltpu.make_async_copy(
            sk_hbm.at[pl.ds(t, 128), :], skb.at[pl.ds(t, 128), :], sem.at[sem_at])

    def oa_dma(u, n):
        t = hint(u * UNIT, UNIT)
        return pltpu.make_async_copy(
            oa.at[pl.ds(t, UNIT), pl.ds(128 * n, 128)],
            o_hbm.at[pl.ds(t, UNIT), pl.ds(128 * n, 128)], sem.at[S_OUT])

    def oa_unit_dma(u):
        t = hint(u * UNIT, UNIT)
        return pltpu.make_async_copy(
            oa.at[pl.ds(t, UNIT), :], o_hbm.at[pl.ds(t, UNIT), pl.ds(0, D)], sem.at[S_OUT])

    def ob_dma(g, half):
        h = L // 2
        return pltpu.make_async_copy(
            ob.at[pl.ds(hint(L * g + h * half, h), h), :],
            o_hbm.at[pl.ds(h * half, h), pl.ds(hint(D + 128 * g, 128), 128)], sem.at[S_OUT])

    def start(ds):
        for d in ds:
            d.start()

    def wait(ds):
        for d in ds:
            d.wait()

    def prm(g, row):
        return rows(view(par, g * (P_ROWS * 8), P_ROWS * 8), row * 8)

    def bu_passes(u, slot, size=128, z=0, shift=False, raw=False, groups=range(NG)):
        out = []
        xu, w = view(x32, u * (UNIT // 2), ((NG - 1) * L + UNIT) // 2), view(wb, z)
        order = [p + c * NG for p in groups for c in range(2)]
        for n in order:
            sizes = [size] * (UNIT // size)
            if shift and n == order[0]:
                sizes = [32, 32, 96, 96]
            if shift and n == order[-1]:
                sizes = [64] * 4
            for m, MM in zip(np.cumsum([0] + sizes).tolist(), sizes):
                acc = []
                for kk in range(NG):
                    def lhs(m=m, kk=kk, MM=MM):
                        t = (kk * L + m) // 2
                        return [rows(xu, t + 8 * i) for i in range(MM // 16)]

                    def rhs(n=n, kk=kk):
                        if raw:
                            return braw[pl.ds(128 * n, 128), pl.ds(128 * kk, 128)]
                        return [rows(w, (n * NG + kk) * 64 + 8 * i) for i in range(8)]

                    def consume(d, m=m, n=n, kk=kk, acc=acc, MM=MM):
                        acc.append(d if kk == 0 else acc[-1] + d)
                        if kk == NG - 1:
                            for i in range(MM // 8):
                                seg, r = divmod(m + 8 * i, R)
                                row = 9 * (seg % 2 * R + r) + seg // 2
                                bu[pl.ds((slot * 2 * NG + n) * BU_PART + row, 8, stride=9), :] = (
                                    acc[-1][8 * i:8 * i + 8])
                    out.append((MM, lhs, rhs, consume))
        return out

    def scan_tasks(u, slot):
        steps, state = 2, {}
        hu = view(hb16, u * UNIT, (2 * NG - 1) * L + UNIT)

        def b(p, ch, r):
            return tuple(rows(bu, (slot * 2 * NG + c * NG + p) * BU_PART + 9 * (ch * R + r))
                         for c in range(2))

        def step(mu, h, br):
            return (mu[0] * h[0] + br[0]) - mu[1] * h[1], (mu[0] * h[1] + br[1]) + mu[1] * h[0]

        def ends(p, gate):
            mu, ties = (gate.value(prm(p, P_MU), PLAN["scan_lead"]), prm(p, P_MU + 1)), []
            h = [b(p, ch, 0) for ch in range(2)]
            for r in range(1, R):
                h = [step(mu, h[ch], b(p, ch, r)) for ch in range(2)]
                if r % steps == 0:
                    ties.append(h[r // steps % 2][0])
            state[p] = starts(p, h)
            return ties + [state[p][1][0]]

        def starts(p, e):
            last = lax.broadcasted_iota(I32, (8, 128), 0) == 7
            rho = (prm(p, P_RHO), prm(p, P_RHO + 1))
            pair = step(rho, e[0], e[1])
            a = tuple(pltpu.roll(jnp.where(last, rows(carry, (2 * p + c) * 8), pair[c]), 1, 0)
                      for c in range(2))
            for sh, row in ((1, P_RHO1), (2, P_RHO2), (4, P_RHO4)):
                a = step((prm(p, row), prm(p, row + 1)), tuple(pltpu.roll(c, sh, 0) for c in a), a)
            return [a, step(rho, a, e[0])]

        def run(p, r0, gate):
            if r0 == 0:
                state["mu"] = (prm(p, P_MU), prm(p, P_MU + 1))
            mu, h = (gate.value(state["mu"][0], PLAN["scan_lead"]), state["mu"][1]), state[p]
            for r in range(r0, r0 + steps):
                h = [step(mu, h[ch], b(p, ch, r)) for ch in range(2)]
                for c in range(2):
                    hu[pl.ds((c * NG + p) * L + 16 * r, 16), :] = _pack(h[0][c], h[1][c])
            state[p] = h
            if r0 + steps == R:
                for c in range(2):
                    carry[pl.ds((2 * p + c) * 8, 8), :] = h[1][c]
            return [after(hb)]

        tasks = []
        for p in range(NG):
            tasks.append(([16 * steps] * ((R - 1) // steps) + [46 + 16 * steps],
                          lambda gate, p=p: ends(p, gate)))
            tasks += [([18 * steps], lambda gate, p=p, r0=r0: run(p, r0, gate))
                      for r0 in range(0, R, steps)]
        return tasks

    def y_passes(h, n, sizes=(HALF,), z=0):
        out, w, hu = [], view(wc, z), view(hb, h * (HALF // 2), ((2 * NG - 1) * L + HALF) // 2)
        for t0, MM in zip(np.cumsum((0,) + sizes).tolist(), sizes):
            acc = []
            for kk in range(2 * NG):
                def lhs(t0=t0, kk=kk, MM=MM):
                    return [rows(hu, (kk * L + t0) // 2 + 8 * i) for i in range(MM // 16)]

                def rhs(kk=kk):
                    return [rows(w, (kk * NG + n) * 64 + 8 * i) for i in range(8)]

                def consume(d, t0=t0, kk=kk, acc=acc, MM=MM):
                    acc.append(d if kk == 0 else acc[-1] + d)
                    if kk == 2 * NG - 1:
                        for i in range(MM // 8):
                            r, ch = divmod(t0 // 8 + i, 2)
                            ys[pl.ds(n * YS_ROWS + ch * (R // 2 + 1) + r, 8, stride=R + 2), :] = (
                                acc[-1][8 * i:8 * i + 8])
                out.append((MM, lhs, rhs, consume))
        return out

    def skip_task(h, n):
        def fn(gate):
            dsk, ties = gate.value(prm(n, P_DSKIP), PLAN["skip_lead"]), []
            t = h // 2 * UNIT + h % 2 * (R // 2)
            edge = n == NG - 1 and isinstance(h, int)
            xu = x32.at[pl.ds(hint(t // 2 + n * (L // 2), 4), UNIT // 2 + (-4 if edge else 4)), :]
            ou = oa.at[pl.ds(hint(t, 8), UNIT - R // 2), :]
            for g in range(SEG):
                if g == SEG - 1 and edge:
                    xs = _unpack(rows(xu, 8 * g - 4))[1]
                else:
                    xs = _unpack(rows(xu, 8 * g))[0]
                y = rows(ys, n * YS_ROWS + g * (R // 2 + 1))
                ou[pl.ds(R * g, 8), pl.ds(128 * n, 128)] = y + xs * dsk
                if g % 8 == 7:
                    ties.append(after(oa))
            return ties
        return ([24, 24], fn)

    def widen_tasks(g):
        def fn(i0):
            kg = view(k32, g * (L // 2), L // 2)
            for i in range(i0, i0 + 8):
                lo, hi = _unpack(rows(kg, 8 * i))
                kf[pl.ds(KF_PAD + 16 * i, 8), :] = lo
                kf[pl.ds(KF_PAD + 16 * i + 8, 8), :] = hi
            return [after(kf)]
        return [([16], lambda gate, i=i: fn(i)) for i in range(0, L // 16, 8)]

    def transpose_tasks(g):
        n = 2

        def fn(c0):
            for c in range(c0, c0 + n):
                t = skb[pl.ds(hint(128 * g, 128), 128), pl.ds(128 * c, 128)]
                kt[pl.ds(64 * c, 64), :] = pltpu.bitcast(t.T, I32)
            return [after(kt)]
        return [([8 * n], lambda gate, c=c: fn(c)) for c in range(0, L // 128, n)]

    def staged(s, half, n, grp, c):
        return (((s * 2 + half) * 4 + n) * 4 + grp) * 16 + 8 * c

    ops1 = (18, 36, 30, 36)

    def transform_tasks(st, s, half, chunk, chunk_cost, direct):
        dst16, dst = (vu16, vu) if st is st_u else (vk16, vk)
        kept = []

        def first(gate, n):
            load = chunk(gate, n)
            u = [load(16 * half + n + 4 * m) for m in range(4)]
            pairs = _fwd1(n, [_Signed(v) for v in u])
            kept.append(pairs)
            for grp in range(2 * direct, 4):
                for c in range(2):
                    st[pl.ds(staged(s, half, n, grp, c), 8), :] = pairs[grp][c].get()
            return [u[0] + u[2]] * (chunk_cost > 4) + [after(st)]

        def second(grps):
            for grp in grps:
                if direct and grp < 2:
                    zs = [t[grp] for t in kept]
                else:
                    zs = [tuple(_Signed(rows(view(st, z8), staged(s, half, n, grp, c)))
                                for c in range(2)) for n in range(4)]
                for k, pair in enumerate(_fwd2(grp, zs)):
                    dst16[pl.ds(((4 * grp + k) * 2 + half) * 128 + 16 * s, 16), :] = (
                        _pack(pair[0].get(), pair[1].get()))
            return [after(dst)]

        split = (chunk_cost > 4) * (chunk_cost // 2 + 1)
        one = [([split] * (split > 0) + [chunk_cost + ops1[n] - split],
                lambda gate, n=n: first(gate, n)) for n in range(4)]
        two = [([40], lambda gate, grp=grp: second((grp, grp + 1))) for grp in (0, 2)]
        return (one + two[:1], two[1:]) if direct else (one, two)

    def kv_tasks(g):
        tasks = []
        for s in range(8):
            for half in range(2):
                def chunk(gate, n, s=s, loaded=[]):
                    if n == 0:
                        loaded[:] = [prm(g, P_TAP + t) for t in range(4)]
                    taps = [gate.value(loaded[0], PLAN["conv_lead"])] + loaded[1:]
                    kz, vg = view(kf, z8), view(v32, g * (L // 2), L // 2)

                    def load(c):
                        t = 64 * c + 8 * s
                        ks = rows(kz, KF_PAD + t) * taps[0]
                        for lag in range(1, 4):
                            ks = ks + rows(kz, KF_PAD + t - lag) * taps[lag]
                        return ks * _unpack(rows(vg, (t // 16) * 8))[s % 2]
                    return load
                tasks += sum(transform_tasks(st_u, s, half, chunk, 36, True), [])
        return tasks

    def filter_tasks(g, early):
        before, after_use = [], []
        for j in range(16):
            def chunk(gate, n, s=j // 2):
                def load(c):
                    v = _unpack(rows(view(kt, z8), 32 * c + 8 * (s // 2)))[s % 2]
                    if s == 0 and c == 0:
                        first = lax.broadcasted_iota(I32, (8, 128), 0) == 0
                        v = v + jnp.where(first, prm(g, P_SSMD), 0.0)
                    return v
                return load
            one, two = transform_tasks(st_k, j // 2, j % 2, chunk, 4, j >= early)
            before += one if j < early else []
            after_use += two if j < early else one + two
        return before, after_use

    def fwd_passes(grp):
        out = []
        for slot in range(4 * grp, 4 * grp + 4):
            got = []
            for src, half in ((vu, 0), (vk, 0), (vu, 1), (vk, 1)):
                def lhs(slot=slot):
                    return [rows(mf, slot * 64 + 8 * i) for i in range(8)]

                def rhs(slot=slot, src=src, half=half):
                    return [rows(view(src, z8), (2 * slot + half) * 64 + 8 * i) for i in range(8)]

                def consume(d, slot=slot, got=got):
                    got.append(d)
                    if len(got) < 4:
                        return
                    for i in range(8):
                        u0, k0, u1, k1 = (
                            (t[16 * i:16 * i + 8], t[16 * i + 8:16 * i + 16]) for t in got)
                        lo, a, b = _cmul(u0, k0), _cmul(u0, k1), _cmul(u1, k0)
                        if slot == _REAL_SLOT and i == 0:
                            first = lax.broadcasted_iota(I32, (8, 128), 0) == 0
                            lo, a, b = (
                                tuple(jnp.where(first, 0.5 * (x[c] * y[c]), p[c]) for c in range(2))
                                for p, x, y in ((lo, u0, k0), (a, u0, k1), (b, u1, k0)))
                        if _F1[slot] % 2:
                            hi = ((a[0] + b[0]) - lo[0], (a[1] + b[1]) - lo[1])
                        else:
                            hi = ((a[0] + b[0]) + lo[0], (a[1] + b[1]) + lo[1])
                        for half, p in enumerate((lo, hi)):
                            at = (slot % 4 * 2 + half) * 128 + 16 * i
                            pb16[grp % 2][pl.ds(at, 16), :] = _pack(*p)
                out.append((128, lhs, rhs, consume))
        return out

    def inv_passes(grp, half):
        out, got = [], []
        for slot in range(4 * grp, 4 * grp + 4):
            def lhs(slot=slot):
                return [rows(mi, slot * 64 + 8 * i) for i in range(8)]

            def rhs(slot=slot):
                return [rows(view(pb[grp % 2], z8), (slot % 4 * 2 + half) * 64 + 8 * i)
                        for i in range(8)]

            def consume(d):
                got.append(d)
                if len(got) < 4:
                    return
                for s in range(8):
                    w = [(_Signed(t[16 * s:16 * s + 8]), _Signed(t[16 * s + 8:16 * s + 16]))
                         for t in got]
                    for n, pair in enumerate(_inv2(grp, w)):
                        for c in range(2):
                            st_i[pl.ds(staged(s, half, n, grp, c), 8), :] = pair[c].get()
            out.append((128, lhs, rhs, consume))
        return out

    def inverse_tasks(g):
        def fn(gate, s, half):
            gate.loads(st_i, PLAN["inverse_lead"])
            qg, og, ties = view(q32, g * (L // 2), L // 2), view(ob, g * L, L), []
            for n in range(4):
                zs = [tuple(_Signed(rows(view(st_i, z8), staged(s, half, n, grp, c)))
                            for c in range(2)) for grp in range(4)]
                for m, y in enumerate(_inv1(n, zs)):
                    t = 64 * (16 * half + n + 4 * m) + 8 * s
                    og[pl.ds(t, 8), :] = _unpack(rows(qg, (t // 16) * 8))[s % 2] * y.get()
                ties.append(after(ob))
            return ties

        tasks = []
        for half in range(2):
            tasks += [([12 + n for n in ops1], lambda gate, s=s, half=half: fn(gate, s, half))
                      for s in range(8)]
            tasks.append(dma_task(ob_dma(g, half)))
        return tasks

    def dma_task(copy):
        return [1], lambda gate: copy.start()

    filter0 = x_dma(2, S_F0) + [sk_dma(0, S_F0)] + x_dma(3, S_F0)
    data0 = [col_dma(0, 0, S_K0), col_dma(1, 0, S_K0)]
    x0, x1 = x_dma(0, S_X0), x_dma(1, S_B + 4)

    def group_dma(g):
        at = S_COL + g
        return [col_dma(2, g, at), sk_dma(g + 1, at), col_dma(0, g + 1, at),
                col_dma(1, g + 1, at)] + x_dma(g + LEAD, at)

    last_dma = col_dma(2, NG - 1, S_SMALL)

    start(small + b_dma(0) + x0 + b_dma(1) + b_dma(2))
    wait(small + x0 + b_dma(0))
    zeros = rows(tab, 288).astype(I32)
    z8 = pl.multiple_of(zeros[0, 0], 16)
    sub = lax.broadcasted_iota(I32, (8, 128), 0)
    pred = zeros == 0

    def stack(ref):
        v = ref[...].astype(F32).reshape(1, D)
        return jnp.concatenate([v[:, 128 * g:128 * (g + 1)] for g in range(NG)]
                               + [v[:, :128]] * (8 - NG), axis=0)

    lre, lim = stack(lre_v), stack(lim_v)
    dt = jnp.exp(stack(ldt_v)).astype(BF16).astype(F32)
    mag, ang = jnp.exp(dt * lre), dt * lim
    lam = (mag * jnp.cos(ang), mag * jnp.sin(ang))
    scale = jnp.maximum(jnp.abs(lre), jnp.abs(lim))
    nre, nim = lre / scale, lim / scale
    den = (nre * nre + nim * nim) * scale
    coef = _cmul(((lam[0] - 1.0) / den, lam[1] / den), (nre, -nim))
    mu = lam
    rho = [mu]
    for _ in range(R.bit_length() + 2):
        rho.append(_cmul(rho[-1], rho[-1]))
    dsk, ssd = stack(dsk_v), stack(sd_v)
    taps = tap_v[...].astype(F32) * _FFT_SCALE
    for g in range(NG):
        def put(row, v):
            par[pl.ds((g * P_ROWS + row) * 8, 8), :] = v

        def lanes(v):
            return jnp.broadcast_to(v[g:g + 1], (8, 128))
        for c in range(2):
            put(P_MU + c, lanes(mu[c]))
            put(P_RHO + c, lanes(rho[-4][c]))
            for n, row in enumerate((P_RHO1, P_RHO2, P_RHO4)):
                put(row + c, jnp.where(sub >= 1 << n, lanes(rho[n - 3][c]), 0.0))
        for t in range(4):
            put(P_TAP + t, jnp.broadcast_to(taps[t:t + 1, 128 * g:128 * (g + 1)], (8, 128)))
        put(P_COEF, lanes(2.0 * coef[0]))
        put(P_COEF + 2, lanes(-2.0 * coef[1]))
        put(P_SSMD, lanes(ssd))
        put(P_DSKIP, lanes(dsk))
    for ref in (hb, oa, kf, kt, vu, vk, st_u, st_k, ob, mf, mi, wb, wc):
        ref[pl.ds(ref.shape[0] - 16, 8), pl.ds(0, 128)] = jnp.zeros((8, 128), ref.dtype)
    for i in range(2 * NG):
        carry[pl.ds(8 * i, 8), :] = jnp.zeros((8, 128), F32)
    kf[pl.ds(0, KF_PAD), :] = jnp.zeros((KF_PAD, 128), F32)

    def matrix_task(slot):
        def fn(gate):
            if slot != _REAL_SLOT:
                c, s = tab[pl.ds(256 + slot, 1), :], tab[pl.ds(272 + slot, 1), :]
            for a in range(8):
                if slot == _REAL_SLOT:
                    re, im = rows(tab, 128 + 16 * a), rows(tab, 128 + 16 * a + 8)
                else:
                    br, bi = rows(tab, 16 * a), rows(tab, 16 * a + 8)
                    re, im = c * br - s * bi, s * br + c * bi
                mf16[pl.ds(slot * 128 + 16 * a, 16), :] = _pack(re, im)
            m = pltpu.bitcast(rows(view(mf, z8), slot * 64, 64), BF16)
            mi[pl.ds(slot * 64, 64), :] = pltpu.bitcast(m.T, I32)
            return [after(mf), after(mi)]
        return ([48, 8], fn)

    def b_task(p):
        def fn(gate):
            ties = []
            for n in (p, NG + p):
                for kk in range(NG):
                    t = braw[pl.ds(128 * n, 128), pl.ds(128 * kk, 128)]
                    wb[pl.ds((n * NG + kk) * 64, 64), :] = pltpu.bitcast(t.T, I32)
                ties.append(after(wb))
            return ties
        return ([24, 24], fn)

    def c_task(n, p):
        def fn(gate):
            cr, ci, nci = prm(p, P_COEF), prm(p, P_COEF + 1), prm(p, P_COEF + 2)
            t = [_unpack_tile(rows(c32, ((c * NG + p) * D + 128 * n) // 2, 64)) for c in range(2)]
            re = [_pack(cr * a0 + nci * b0, cr * a1 + nci * b1) for (a0, a1), (b0, b1) in zip(*t)]
            im = [_pack(nci * a0 - cr * b0, nci * a1 - cr * b1) for (a0, a1), (b0, b1) in zip(*t)]
            ties = []
            for c, tile in enumerate((re, im)):
                wc[pl.ds(((c * NG + p) * NG + n) * 64, 64), :] = pltpu.bitcast(
                    jnp.concatenate(tile, axis=0).T, I32)
                ties.append(after(wc))
            return ties
        return ([80, 80], fn)

    def y_block(halves, t0, lead, even, z=0):
        tiles = [(h, n) for h in halves for n in range(NG)]
        passes, plan = [], []
        for j, (h, n) in enumerate(tiles):
            sizes = (HALF,)
            if j == 0 and lead is not None:
                if not lead:
                    continue
                sizes = (32, 96)
            if j == even:
                sizes = (64, 64)
            if j == len(tiles) - 1:
                sizes = (96, 32)
            passes += y_passes(h, n, sizes, z)
            t0 += 20
            plan.append(([skip_task(h, n)], t0 + PLAN["skip"], t0 + PLAN["skip"] + 6))
        return passes, plan

    def conv_passes(between):
        passes = fwd_passes(0)
        for grp in range(1, 4):
            f = fwd_passes(grp)
            passes += f[:8] + inv_passes(grp - 1, 0) + f[8:] + inv_passes(grp - 1, 1)
        return passes + between[:8] + inv_passes(3, 0) + inv_passes(3, 1) + between[8:]

    unit = 2 * NG * NG * UNIT // 64

    first = bu_passes(0, 1, raw=True)
    first = [first[20 * p:20 * (p + 1)] for p in range(NG)]
    start(b_dma(3) + b_dma(4) + x1 + [tab_dma])
    _weave(first[0], [], pred)
    start(filter0)
    wait(b_dma(1))
    _weave(first[1], [], pred)
    start(data0 + c_dma)
    wait(b_dma(2))
    _weave(first[2], [([b_task(p) for p in range(2)], 0, 40)], pred)
    wait(b_dma(3))
    _weave(first[3], [([b_task(p) for p in range(2, 4)], 0, 40)], pred)
    start(group_dma(0))
    wait(b_dma(4) + x1 + [tab_dma])
    _weave(first[4] + bu_passes(1, 0, 64, z8), [
        ([b_task(4)], 0, 36), (scan_tasks(0, 1), 40, 40 + unit),
        ([matrix_task(slot) for slot in range(SLOTS)], 60, 200)], pred)
    start(group_dma(1))
    wait(filter0)
    _weave(bu_passes(2, 1, 64) + bu_passes(3, 0, 64, groups=[0]), [
        (scan_tasks(1, 0), 0, unit), (transpose_tasks(0), 8, 32),
        (filter_tasks(0, 0)[1], 36, unit + 40)], pred)
    start(group_dma(2))
    wait(data0 + c_dma)
    yp, plan = y_block((0, 1), unit - 40, None, 2, z8)
    kv = kv_tasks(0)
    end = 2 * unit - 40
    _weave(bu_passes(3, 0, shift=True, groups=range(1, NG)) + yp, plan + [
        (scan_tasks(2, 1), *PLAN["scan0"]), (widen_tasks(0), 0, 40),
        ([c_task(n, p) for n in range(NG) for p in range(NG)], *PLAN["scale_c"]),
        (kv[:-2], PLAN["forward0"], end), (kv[-2:], end, end)], pred)
    start([oa_unit_dma(0)] + group_dma(3) + [last_dma])

    def body(i, _):
        wait(group_dma(i))
        halves = [2 + 3 * i + j for j in range(3)]
        y0 = 192 + 20 + unit
        yp, plan = y_block(halves, y0, False, 7)
        passes = conv_passes(y_passes(halves[0], 0, (32, 96))) + bu_passes(i + LEAD, 0) + yp
        early, late = filter_tasks(i + 1, PLAN["early"])
        kv, tail, end = kv_tasks(i + 1), PLAN["tail"], y0 + 280
        done = (3 * i + 2) // 2
        sent = y0 + 180 + PLAN["skip"] + 8
        _weave(passes, plan + [
            ([dma_task(oa_unit_dma(done))], sent, sent),
            (scan_tasks(i + LEAD - 1, 0), *PLAN["scan"]),
            (transpose_tasks(i + 1), *PLAN["transpose"]),
            ([skip_task(halves[0], 0)], 232, 238),
            (widen_tasks(i + 1), *PLAN["widen"]), (early, *PLAN["filter_early"]),
            (inverse_tasks(i), *PLAN["inverse"]), (late, *PLAN["filter"]),
            (kv[:-tail], PLAN["forward"], end), (kv[-tail:], end, end)], pred)
        pl.when(i % 2 == 1)(lambda: start([oa_unit_dma(done + 1)]))
        return 0

    lax.fori_loop(0, NG - 1, body, 0)

    wait([last_dma])
    last = L // UNIT - 1
    yp, plan = y_block((2 * last, 2 * last + 1), 192, True, 2)
    plan += [([dma_task(oa_dma(last, n))], t + 6, t + 6) for n, (_, _, t) in enumerate(plan[NG:])]
    _weave(conv_passes(yp), plan + [
        (scan_tasks(last, 0), 0, 170), (inverse_tasks(NG - 1), *PLAN["last_inverse"])], pred)
    wait([oa_unit_dma(u) for u in range(last)] + [oa_dma(last, n) for n in range(NG)]
         + [ob_dma(n, half) for n in range(NG) for half in range(2)])


@jax.jit
def pallas_concat_heads__ssm_conv_s5__ssm_conv_h3__prompt_kernel(
    A_x: jax.Array,
    A_Lambda_re: jax.Array,
    A_Lambda_im: jax.Array,
    A_B_re: jax.Array,
    A_B_im: jax.Array,
    A_C_re: jax.Array,
    A_C_im: jax.Array,
    A_log_dt: jax.Array,
    A_Dskip: jax.Array,
    B_q: jax.Array,
    B_k: jax.Array,
    B_v: jax.Array,
    B_shift_k: jax.Array,
    B_ssm_k: jax.Array,
    B_ssm_D: jax.Array,
):
    assert A_x.shape == (1, L, D) and B_shift_k.shape == (D, 4)
    vmem = pltpu.VMEM
    dma = pltpu.SemaphoreType.DMA
    scratch = [
        vmem(_TABLES.shape, F32),
        vmem((D,), BF16), vmem((D,), BF16), vmem((D,), BF16), vmem((D,), BF16), vmem((D,), BF16),
        vmem((4, D), BF16),
        vmem((NG * L, 128), BF16),
        vmem((2 * D, D), BF16),
        vmem((2 * NG * D, 128), BF16),
        vmem((NG * L, 128), BF16),
        vmem((NG * L, 128), BF16),
        vmem((NG * L, 128), BF16),
        vmem((D, L), BF16),
        vmem((NG * P_ROWS * 8, 128), F32),
        vmem((2 * NG * D + 32, 128), BF16),
        vmem((2 * NG * NG * 64 + 16, 128), I32),
        vmem((SLOTS * 128 + 32, 128), BF16),
        vmem((SLOTS * 64 + 16, 128), I32),
        vmem((2 * 2 * NG * BU_PART, 128), F32),
        vmem((2 * NG * L + 32, 128), BF16),
        vmem((3 * NG * 8, 128), F32),
        vmem((NG * YS_ROWS, 128), F32),
        vmem((L + 16, D), F32),
        vmem((L // 2 + 16, 128), I32),
        vmem((KF_PAD + L + 16, 128), F32),
        vmem((2 * L + 16, 128), F32),
        vmem((2 * L + 16, 128), F32),
        vmem((2 * L + 8, 128), F32),
        vmem((32 * 128 + 32, 128), BF16),
        vmem((32 * 128 + 32, 128), BF16),
        vmem((8 * 128, 128), BF16),
        vmem((8 * 128, 128), BF16),
        vmem((NG * L + 16, 128), F32),
        dma((S_END,)),
    ]
    out = pl.pallas_call(
        _kernel,
        out_shape=jax.ShapeDtypeStruct((L, 2 * D), F32),
        in_specs=[pl.BlockSpec(memory_space=pl.ANY)] * 16,
        out_specs=pl.BlockSpec(memory_space=pl.ANY),
        scratch_shapes=scratch,
        compiler_params=pltpu.CompilerParams(vmem_limit_bytes=100 * 1024 * 1024),
        name="s5_h3",
    )(_TABLES, A_x.reshape(L, D), A_Lambda_re, A_Lambda_im, A_B_re, A_B_im, A_C_re, A_C_im,
      A_log_dt, A_Dskip, B_q.reshape(L, D), B_k.reshape(L, D), B_v.reshape(L, D),
      B_shift_k.T, B_ssm_k, B_ssm_D)
    return out.reshape(1, L, 2 * D)
```

```python
import math

import jax
import jax.numpy as jnp
import numpy as np
from jax import lax
from jax.experimental import pallas as pl
from jax.experimental.pallas import tpu as pltpu

F32, BF16, I32 = jnp.float32, jnp.bfloat16, jnp.int32

L = 2048
D = 640
NG = D // 128
UNIT = 256
SEG = 16
R = UNIT // SEG
LEAD = 4
HALF = UNIT // 2
BU_PART = 9 * 2 * R
YS_ROWS = SEG * (R // 2 + 1)
KF_PAD = 8


class _Signed:
    def __init__(self, v, neg=False):
        self.v, self.neg = v, neg

    def __neg__(self):
        return _Signed(self.v, not self.neg)

    def __add__(self, o):
        if self.neg == o.neg:
            return _Signed(self.v + o.v, self.neg)
        return _Signed(o.v - self.v if self.neg else self.v - o.v)

    def __sub__(self, o):
        return self + (-o)

    def __mul__(self, c):
        return _Signed(self.v * np.float32(-c if self.neg else c))

    def get(self):
        return -self.v if self.neg else self.v


def _rot(re, im, num, den):
    num %= den
    h = math.sqrt(0.5)
    if num == 0:
        return re, im
    if 4 * num == den:
        return -im, re
    if 4 * num == 3 * den:
        return im, -re
    if 8 * num == den:
        return (re - im) * h, (re + im) * h
    if 8 * num == 3 * den:
        return (re + im) * (-h), (re - im) * h
    if 8 * num == 5 * den:
        return (im - re) * h, (re + im) * (-h)
    if 8 * num == 7 * den:
        return (re + im) * h, (im - re) * h
    c = math.cos(2 * math.pi * num / den)
    s = math.sin(2 * math.pi * num / den)
    return re * c - im * s, re * s + im * c


def _dft4(z, sign):
    (r0, i0), (r1, i1), (r2, i2), (r3, i3) = z
    ar, ai, br, bi = r0 + r2, i0 + i2, r0 - r2, i0 - i2
    cr, ci, dr, di = r1 + r3, i1 + i3, r1 - r3, i1 - i3
    plus, minus = (br - di, bi + dr), (br + di, bi - dr)
    if sign < 0:
        plus, minus = minus, plus
    return [(ar + cr, ai + ci), plus, (ar - cr, ai - ci), minus]


def _fwd1(n, u):
    a0, a1, b0, b1 = u
    p, q = _rot(a0, b0, n, 32), _rot(a1, b1, n + 4, 32)
    s0, s1 = a0 + b0, a1 + b1
    return [(p[0] + q[0], p[1] + q[1]), _rot(p[0] - q[0], p[1] - q[1], n, 8),
            _rot(a0 - b0, a1 - b1, n, 16), (s0 + s1, s0 - s1)]


def _fwd2(grp, z):
    if grp < 3:
        return _dft4(z, 1)
    s4 = [t[0] for t in z]
    d4 = [t[1] for t in z]
    p = (d4[0], d4[2])
    q = _rot(d4[1], d4[3], 1, 8)
    s5 = [s4[0] + s4[2], s4[1] + s4[3]]
    return [
        (s5[0] + s5[1], s5[0] - s5[1]),
        (s4[0] - s4[2], s4[1] - s4[3]),
        (p[0] + q[0], p[1] + q[1]),
        (p[0] - q[0], p[1] - q[1]),
    ]


def _inv2(grp, w):
    if grp < 3:
        return _dft4(w, -1)
    s5 = [w[0][0] + w[0][1], w[0][0] - w[0][1]]
    s4 = [s5[0] + w[1][0], s5[1] + w[1][1], s5[0] - w[1][0], s5[1] - w[1][1]]
    p = (w[2][0] + w[3][0], w[2][1] + w[3][1])
    q = _rot(w[2][0] - w[3][0], w[2][1] - w[3][1], -1, 8)
    d4 = [p[0], q[0], p[1], q[1]]
    return [(s4[n], d4[n]) for n in range(4)]


def _inv1(n, z):
    e = _rot(*z[1], -n, 8)
    p = _rot(z[0][0] + e[0], z[0][1] + e[1], -n, 32)
    q = _rot(z[0][0] - e[0], z[0][1] - e[1], -(n + 4), 32)
    d0, d1 = _rot(*z[2], -n, 16)
    s0, s1 = z[3][0] + z[3][1], z[3][0] - z[3][1]
    return [p[0] + (s0 + d0), q[0] + (s1 + d1), p[1] + (s0 - d0), q[1] + (s1 - d1)]


_F1 = [4 * (g + 2 * k) + 1 for g in range(2) for k in range(4)]
_F1 += [2 * (4 * k + 1) for k in range(4)] + [0, 8, 4, 20]
_REAL_SLOT = 12
SLOTS = len(_F1)


def _dft_tables():
    kap = np.arange(128)
    j = 8 * (kap // 16) + kap % 8
    part = (kap // 8) % 2
    pr, pc, jr, jc = part[:, None], part[None, :], j[:, None], j[None, :]
    lo = 2 * np.pi * jr * jc / 64
    base = np.where(pr == pc, np.cos(lo), np.where(pr == 0, -np.sin(lo), np.sin(lo)))
    hi = 2 * np.pi * (16 + 32 * (jr - 32)) * jc / 2048
    v0 = np.where(pr == 0, np.cos(lo), np.where(jr == 0, np.cos(np.pi * jc), np.sin(lo)))
    v32 = np.where(pr == 0, np.cos(hi), np.sin(hi))
    real = np.where(jr < 32, np.where(pc == 0, v0, 0.0), np.where(pc == 1, v32, 0.0))
    th = 2 * np.pi * np.outer(np.array(_F1), j) / 2048
    zeros = np.zeros((8, 128))
    return np.concatenate([base, real, np.cos(th), np.sin(th), zeros]).astype(np.float32)


_TABLES = _dft_tables()
_FFT_SCALE = 2.0 ** -10

(P_MU, P_RHO, P_RHO1, P_RHO2, P_RHO4, P_TAP, P_SSMD, P_DSKIP, P_COEF, P_ROWS) = (
    0, 2, 4, 6, 8, 10, 14, 15, 16, 20)
S_SMALL, S_F0, S_K0, S_C, S_OUT, S_X0, S_B = range(7)
S_COL = S_B + NG
S_END = S_COL + NG - 1


def _cmul(a, b):
    return a[0] * b[0] - a[1] * b[1], a[0] * b[1] + a[1] * b[0]


def _pack(lo, hi):
    return jnp.concatenate([lo, hi], axis=0).astype(BF16)


def _unpack_tile(w):
    return [_unpack(w[8 * i:8 * i + 8]) for i in range(w.shape[0] // 8)]


def _unpack(w):
    v = pltpu.bitcast(w, BF16).astype(F32)
    return v[:8], v[8:]


PLAN = dict(
    scan_lead=22, conv_lead=20, inverse_lead=44, skip_lead=24, scale_lead=40, filter_lead=30,
    scan=(0, 350), transpose=(60, 90), filter_early=(92, 200), early=4, inverse=(220, 380),
    widen=(216, 330), filter=(230, 480), forward=350, tail=3, skip=28,
    matrix=(60, 200), filter0=(36, 240),
    scale_c=(10, 220), scan0=(0, 350), forward0=110, last_inverse=(216, 290),
)


class _Zeros:
    def __init__(self, v):
        self.v = v


class _Gate:
    def __init__(self, pred=None, seen=()):
        self.pred, self.seen = pred, seen

    def early(self, lag):
        old = [e for e in self.seen if e[0] <= -lag]
        return max(old, key=lambda e: e[0])[1] if old else None

    def value(self, v, lag):
        early = self.early(lag)
        return v if early is None else jnp.where(self.pred, v, early)

    def loads(self, ref, lag):
        early = self.early(lag)
        if early is not None:
            ref[pl.ds(ref.shape[0] - 8, 8), :] = (
                early if ref.dtype == F32 else pltpu.bitcast(early, I32))


def _weave(passes, plan, pred):
    begin, clock = [], [0] * 4
    for i, (n, *_) in enumerate(passes):
        begin.append(clock[i % 4] / 16)
        clock[i % 4] += n

    def index(t):
        later = [i for i, b in enumerate(begin) if b >= t - 3.999]
        if not later:
            return len(passes)
        same = [i for i in later if begin[i] == min(begin[j] for j in later)]
        return same[min(max(int((t - begin[same[0]]) / 4 * len(same)), 0), len(same) - 1)]

    at = [[] for _ in range(len(passes) + 1)]
    for tasks, lo, hi in plan:
        total, done = sum(sum(c) for c, _ in tasks) or 1, 0.0
        for costs, fn in tasks:
            where = []
            for cost in costs:
                done += cost
                where.append(index(lo + done / total * (hi - lo)))
            at[min(where)].append((fn, where))
    seen, ties = [], [[] for _ in at]
    for i, fns in enumerate(at):
        now = (begin[i] + i % 4) if i < len(begin) else clock[0] / 16
        early = [(t - now, v) for t, v in seen]
        for fn, where in fns:
            for w, tie in zip(where, fn(_Gate(pred, early)) or ()):
                ties[w].append(tie)
        if i == len(passes):
            break
        n, lhs, rhs, consume = passes[i]
        w = rhs()
        if not isinstance(w, list):
            d = lax.dot_general(pltpu.bitcast(jnp.concatenate(lhs(), axis=0), BF16), w,
                                (((1,), (1,)), ((), ())), preferred_element_type=F32)
            consume(d)
            continue
        for tie in ties[i]:
            if isinstance(tie, _Zeros):
                v = tie.v
                w[-1] = w[-1] | (v if v.dtype == I32 else pltpu.bitcast(v, I32))
            else:
                w[-1] = jnp.where(pred, w[-1], pltpu.bitcast(tie, I32))
        d = jnp.dot(pltpu.bitcast(jnp.concatenate(lhs(), axis=0), BF16),
                    pltpu.bitcast(jnp.concatenate(w, axis=0), BF16), preferred_element_type=F32)
        seen += [(begin[i] + i % 4 + j // 16 - 4, d[j - 8:j]) for j in range(64, n + 1, 64)]
        consume(d)


def _kernel(tab_hbm, x_hbm, lre_hbm, lim_hbm, bre_hbm, bim_hbm, cre_hbm, cim_hbm,
            ldt_hbm, dsk_hbm, q_hbm, k_hbm, v_hbm, tap_hbm, sk_hbm, sd_hbm,
            o_hbm,
            tab, lre_v, lim_v, ldt_v, dsk_v, sd_v, tap_v,
            xb, braw, craw, qb, kb, vb, skb,
            par, wb16, wc, mf16, mi, bu, hb16, carry, ys, oa,
            kt, kf, st_u, st_k, st_i, vu16, vk16, pb0, pb1, ob,
            sem):
    x32, q32, k32, v32, wb, mf, hb, vu, vk = (
        r.bitcast(I32) for r in (xb, qb, kb, vb, wb16, mf16, hb16, vu16, vk16))
    c32 = craw.bitcast(I32)
    pb16 = (pb0, pb1)
    pb = (pb0.bitcast(I32), pb1.bitcast(I32))

    def rows(ref, start, n=8):
        return ref[pl.ds(start, n), :]

    def hint(v, n):
        return v if isinstance(v, int) or n == 1 else pl.multiple_of(v, n)

    def view(ref, start, n=None):
        return ref.at[pl.ds(hint(start, 16), n or ref.shape[0]), :]

    def after(ref):
        return _Zeros(view(ref, z8)[ref.shape[0] - 16:ref.shape[0] - 8, 0:128])

    small = [pltpu.make_async_copy(s, d, sem.at[S_SMALL]) for s, d in (
        (lre_hbm, lre_v), (lim_hbm, lim_v), (ldt_hbm, ldt_v),
        (dsk_hbm, dsk_v), (sd_hbm, sd_v), (tap_hbm, tap_v),
        (tab_hbm.at[pl.ds(288, 8), :], tab.at[pl.ds(288, 8), :]))]
    tab_dma = pltpu.make_async_copy(
        tab_hbm.at[pl.ds(0, 288), :], tab.at[pl.ds(0, 288), :], sem.at[S_B + 4])

    def x_dma(u, at):
        return [pltpu.make_async_copy(
            x_hbm.at[pl.ds(hint(u * UNIT, UNIT), UNIT), pl.ds(128 * n, 128)],
            xb.at[pl.ds(hint(n * L + u * UNIT, UNIT), UNIT), :], sem.at[at])
            for n in range(NG)]

    def b_dma(p):
        return [pltpu.make_async_copy(
            src.at[pl.ds(128 * p, 128), :], braw.at[pl.ds(D * c + 128 * p, 128), :],
            sem.at[S_B + p]) for c, src in enumerate((bre_hbm, bim_hbm))]

    c_dma = [pltpu.make_async_copy(
        src.at[:, pl.ds(128 * p, 128)], craw.at[pl.ds(D * (NG * c + p), D), :],
        sem.at[S_C]) for c, src in enumerate((cre_hbm, cim_hbm)) for p in range(NG)]

    def col_dma(which, g, sem_at):
        src, dst = ((k_hbm, kb), (v_hbm, vb), (q_hbm, qb))[which]
        return pltpu.make_async_copy(
            src.at[:, pl.ds(hint(128 * g, 128), 128)],
            dst.at[pl.ds(hint(L * g, L), L), :], sem.at[sem_at])

    def sk_dma(g, sem_at):
        t = hint(128 * g, 128)
        return pltpu.make_async_copy(
            sk_hbm.at[pl.ds(t, 128), :], skb.at[pl.ds(t, 128), :], sem.at[sem_at])

    def oa_dma(u, n):
        t = hint(u * UNIT, UNIT)
        return pltpu.make_async_copy(
            oa.at[pl.ds(t, UNIT), pl.ds(128 * n, 128)],
            o_hbm.at[pl.ds(t, UNIT), pl.ds(128 * n, 128)], sem.at[S_OUT])

    def oa_unit_dma(u):
        t = hint(u * UNIT, UNIT)
        return pltpu.make_async_copy(
            oa.at[pl.ds(t, UNIT), :], o_hbm.at[pl.ds(t, UNIT), pl.ds(0, D)], sem.at[S_OUT])

    def ob_dma(g, half):
        h = L // 2
        return pltpu.make_async_copy(
            ob.at[pl.ds(hint(L * g + h * half, h), h), :],
            o_hbm.at[pl.ds(h * half, h), pl.ds(hint(D + 128 * g, 128), 128)], sem.at[S_OUT])

    def start(ds):
        for d in ds:
            d.start()

    def wait(ds):
        for d in ds:
            d.wait()

    def prm(g, row):
        return rows(view(par, g * (P_ROWS * 8), P_ROWS * 8), row * 8)

    def bu_passes(u, slot, size=128, z=0, shift=False, raw=False, groups=range(NG)):
        out = []
        xu, w = view(x32, u * (UNIT // 2), ((NG - 1) * L + UNIT) // 2), view(wb, z)
        order = [p + c * NG for p in groups for c in range(2)]
        for n in order:
            sizes = [size] * (UNIT // size)
            if shift and n == order[0]:
                sizes = [32, 32, 96, 96]
            if shift and n == order[-1]:
                sizes = [64] * 4
            for m, MM in zip(np.cumsum([0] + sizes).tolist(), sizes):
                acc = []
                for kk in range(NG):
                    def lhs(m=m, kk=kk, MM=MM):
                        t = (kk * L + m) // 2
                        return [rows(xu, t + 8 * i) for i in range(MM // 16)]

                    def rhs(n=n, kk=kk):
                        if raw:
                            return braw[pl.ds(128 * n, 128), pl.ds(128 * kk, 128)]
                        return [rows(w, (n * NG + kk) * 64 + 8 * i) for i in range(8)]

                    def consume(d, m=m, n=n, kk=kk, acc=acc, MM=MM):
                        acc.append(d if kk == 0 else acc[-1] + d)
                        if kk == NG - 1:
                            for i in range(MM // 8):
                                seg, r = divmod(m + 8 * i, R)
                                row = 9 * (seg % 2 * R + r) + seg // 2
                                bu[pl.ds((slot * 2 * NG + n) * BU_PART + row, 8, stride=9), :] = (
                                    acc[-1][8 * i:8 * i + 8])
                    out.append((MM, lhs, rhs, consume))
        return out

    def scan_tasks(u, slot):
        steps, state = 2, {}
        hu = view(hb16, u * UNIT, (2 * NG - 1) * L + UNIT)

        def b(p, ch, r):
            return tuple(rows(bu, (slot * 2 * NG + c * NG + p) * BU_PART + 9 * (ch * R + r))
                         for c in range(2))

        def step(mu, h, br):
            return (mu[0] * h[0] + br[0]) - mu[1] * h[1], (mu[0] * h[1] + br[1]) + mu[1] * h[0]

        def ends(p, gate):
            mu, ties = (gate.value(prm(p, P_MU), PLAN["scan_lead"]), prm(p, P_MU + 1)), []
            h = [b(p, ch, 0) for ch in range(2)]
            for r in range(1, R):
                h = [step(mu, h[ch], b(p, ch, r)) for ch in range(2)]
                if r % steps == 0:
                    ties.append(h[r // steps % 2][0])
            state[p] = starts(p, h)
            return ties + [state[p][1][0]]

        def starts(p, e):
            last = lax.broadcasted_iota(I32, (8, 128), 0) == 7
            rho = (prm(p, P_RHO), prm(p, P_RHO + 1))
            pair = step(rho, e[0], e[1])
            a = tuple(pltpu.roll(jnp.where(last, rows(carry, (2 * p + c) * 8), pair[c]), 1, 0)
                      for c in range(2))
            for sh, row in ((1, P_RHO1), (2, P_RHO2), (4, P_RHO4)):
                a = step((prm(p, row), prm(p, row + 1)), tuple(pltpu.roll(c, sh, 0) for c in a), a)
            return [a, step(rho, a, e[0])]

        def run(p, r0, gate):
            if r0 == 0:
                state["mu"] = (prm(p, P_MU), prm(p, P_MU + 1))
            mu, h = (gate.value(state["mu"][0], PLAN["scan_lead"]), state["mu"][1]), state[p]
            for r in range(r0, r0 + steps):
                h = [step(mu, h[ch], b(p, ch, r)) for ch in range(2)]
                for c in range(2):
                    hu[pl.ds((c * NG + p) * L + 16 * r, 16), :] = _pack(h[0][c], h[1][c])
            state[p] = h
            if r0 + steps == R:
                for c in range(2):
                    carry[pl.ds((2 * p + c) * 8, 8), :] = h[1][c]
            return [after(hb)]

        tasks = []
        for p in range(NG):
            tasks.append(([16 * steps] * ((R - 1) // steps) + [46 + 16 * steps],
                          lambda gate, p=p: ends(p, gate)))
            tasks += [([18 * steps], lambda gate, p=p, r0=r0: run(p, r0, gate))
                      for r0 in range(0, R, steps)]
        return tasks

    def y_passes(h, n, sizes=(HALF,), z=0):
        out, w, hu = [], view(wc, z), view(hb, h * (HALF // 2), ((2 * NG - 1) * L + HALF) // 2)
        for t0, MM in zip(np.cumsum((0,) + sizes).tolist(), sizes):
            acc = []
            for kk in range(2 * NG):
                def lhs(t0=t0, kk=kk, MM=MM):
                    return [rows(hu, (kk * L + t0) // 2 + 8 * i) for i in range(MM // 16)]

                def rhs(kk=kk):
                    return [rows(w, (kk * NG + n) * 64 + 8 * i) for i in range(8)]

                def consume(d, t0=t0, kk=kk, acc=acc, MM=MM):
                    acc.append(d if kk == 0 else acc[-1] + d)
                    if kk == 2 * NG - 1:
                        for i in range(MM // 8):
                            r, ch = divmod(t0 // 8 + i, 2)
                            ys[pl.ds(n * YS_ROWS + ch * (R // 2 + 1) + r, 8, stride=R + 2), :] = (
                                acc[-1][8 * i:8 * i + 8])
                out.append((MM, lhs, rhs, consume))
        return out

    def skip_task(h, n):
        def fn(gate):
            dsk, ties = gate.value(prm(n, P_DSKIP), PLAN["skip_lead"]), []
            t = h // 2 * UNIT + h % 2 * (R // 2)
            edge = n == NG - 1 and isinstance(h, int)
            xu = x32.at[pl.ds(hint(t // 2 + n * (L // 2), 4), UNIT // 2 + (-4 if edge else 4)), :]
            ou = oa.at[pl.ds(hint(t, 8), UNIT - R // 2), :]
            for g in range(SEG):
                if g == SEG - 1 and edge:
                    xs = _unpack(rows(xu, 8 * g - 4))[1]
                else:
                    xs = _unpack(rows(xu, 8 * g))[0]
                y = rows(ys, n * YS_ROWS + g * (R // 2 + 1))
                ou[pl.ds(R * g, 8), pl.ds(128 * n, 128)] = y + xs * dsk
                if g % 8 == 7:
                    ties.append(after(oa))
            return ties
        return ([24, 24], fn)

    def widen_tasks(g):
        def fn(i0):
            kg = view(k32, g * (L // 2), L // 2)
            for i in range(i0, i0 + 8):
                lo, hi = _unpack(rows(kg, 8 * i))
                kf[pl.ds(KF_PAD + 16 * i, 8), :] = lo
                kf[pl.ds(KF_PAD + 16 * i + 8, 8), :] = hi
            return [after(kf)]
        return [([16], lambda gate, i=i: fn(i)) for i in range(0, L // 16, 8)]

    def transpose_tasks(g):
        n = 2

        def fn(c0):
            for c in range(c0, c0 + n):
                t = skb[pl.ds(hint(128 * g, 128), 128), pl.ds(128 * c, 128)]
                kt[pl.ds(64 * c, 64), :] = pltpu.bitcast(t.T, I32)
            return [after(kt)]
        return [([8 * n], lambda gate, c=c: fn(c)) for c in range(0, L // 128, n)]

    def staged(s, half, n, grp, c):
        return (((s * 2 + half) * 4 + n) * 4 + grp) * 16 + 8 * c

    ops1 = (18, 36, 30, 36)

    def transform_tasks(st, s, half, chunk, chunk_cost, direct):
        dst16, dst = (vu16, vu) if st is st_u else (vk16, vk)
        kept = []

        def first(gate, n):
            load = chunk(gate, n)
            u = [load(16 * half + n + 4 * m) for m in range(4)]
            pairs = _fwd1(n, [_Signed(v) for v in u])
            kept.append(pairs)
            for grp in range(2 * direct, 4):
                for c in range(2):
                    st[pl.ds(staged(s, half, n, grp, c), 8), :] = pairs[grp][c].get()
            return [u[0] + u[2]] * (chunk_cost > 4) + [after(st)]

        def second(grps):
            for grp in grps:
                if direct and grp < 2:
                    zs = [t[grp] for t in kept]
                else:
                    zs = [tuple(_Signed(rows(view(st, z8), staged(s, half, n, grp, c)))
                                for c in range(2)) for n in range(4)]
                for k, pair in enumerate(_fwd2(grp, zs)):
                    dst16[pl.ds(((4 * grp + k) * 2 + half) * 128 + 16 * s, 16), :] = (
                        _pack(pair[0].get(), pair[1].get()))
            return [after(dst)]

        split = (chunk_cost > 4) * (chunk_cost // 2 + 1)
        one = [([split] * (split > 0) + [chunk_cost + ops1[n] - split],
                lambda gate, n=n: first(gate, n)) for n in range(4)]
        two = [([40], lambda gate, grp=grp: second((grp, grp + 1))) for grp in (0, 2)]
        return (one + two[:1], two[1:]) if direct else (one, two)

    def kv_tasks(g):
        tasks = []
        for s in range(8):
            for half in range(2):
                def chunk(gate, n, s=s, loaded=[]):
                    if n == 0:
                        loaded[:] = [prm(g, P_TAP + t) for t in range(4)]
                    taps = [gate.value(loaded[0], PLAN["conv_lead"])] + loaded[1:]
                    kz, vg = view(kf, z8), view(v32, g * (L // 2), L // 2)

                    def load(c):
                        t = 64 * c + 8 * s
                        ks = rows(kz, KF_PAD + t) * taps[0]
                        for lag in range(1, 4):
                            ks = ks + rows(kz, KF_PAD + t - lag) * taps[lag]
                        return ks * _unpack(rows(vg, (t // 16) * 8))[s % 2]
                    return load
                tasks += sum(transform_tasks(st_u, s, half, chunk, 36, True), [])
        return tasks

    def filter_tasks(g, early, lead=None):
        before, after_use = [], []
        for j in range(16):
            def chunk(gate, n, s=j // 2):
                if lead:
                    gate.loads(kt, lead)

                def load(c):
                    v = _unpack(rows(view(kt, z8), 32 * c + 8 * (s // 2)))[s % 2]
                    if s == 0 and c == 0:
                        first = lax.broadcasted_iota(I32, (8, 128), 0) == 0
                        v = v + jnp.where(first, prm(g, P_SSMD), 0.0)
                    return v
                return load
            one, two = transform_tasks(st_k, j // 2, j % 2, chunk, 4, j >= early)
            before += one if j < early else []
            after_use += two if j < early else one + two
        return before, after_use

    def fwd_passes(grp):
        out = []
        for slot in range(4 * grp, 4 * grp + 4):
            got = []
            for src, half in ((vu, 0), (vk, 0), (vu, 1), (vk, 1)):
                def lhs(slot=slot):
                    return [rows(mf, slot * 64 + 8 * i) for i in range(8)]

                def rhs(slot=slot, src=src, half=half):
                    return [rows(view(src, z8), (2 * slot + half) * 64 + 8 * i) for i in range(8)]

                def consume(d, slot=slot, got=got):
                    got.append(d)
                    if len(got) < 4:
                        return
                    for i in range(8):
                        u0, k0, u1, k1 = (
                            (t[16 * i:16 * i + 8], t[16 * i + 8:16 * i + 16]) for t in got)
                        lo, a, b = _cmul(u0, k0), _cmul(u0, k1), _cmul(u1, k0)
                        if slot == _REAL_SLOT and i == 0:
                            first = lax.broadcasted_iota(I32, (8, 128), 0) == 0
                            lo, a, b = (
                                tuple(jnp.where(first, 0.5 * (x[c] * y[c]), p[c]) for c in range(2))
                                for p, x, y in ((lo, u0, k0), (a, u0, k1), (b, u1, k0)))
                        if _F1[slot] % 2:
                            hi = ((a[0] + b[0]) - lo[0], (a[1] + b[1]) - lo[1])
                        else:
                            hi = ((a[0] + b[0]) + lo[0], (a[1] + b[1]) + lo[1])
                        for half, p in enumerate((lo, hi)):
                            at = (slot % 4 * 2 + half) * 128 + 16 * i
                            pb16[grp % 2][pl.ds(at, 16), :] = _pack(*p)
                out.append((128, lhs, rhs, consume))
        return out

    def inv_passes(grp, half):
        out, got = [], []
        for slot in range(4 * grp, 4 * grp + 4):
            def lhs(slot=slot):
                return [rows(mi, slot * 64 + 8 * i) for i in range(8)]

            def rhs(slot=slot):
                return [rows(view(pb[grp % 2], z8), (slot % 4 * 2 + half) * 64 + 8 * i)
                        for i in range(8)]

            def consume(d):
                got.append(d)
                if len(got) < 4:
                    return
                for s in range(8):
                    w = [(_Signed(t[16 * s:16 * s + 8]), _Signed(t[16 * s + 8:16 * s + 16]))
                         for t in got]
                    for n, pair in enumerate(_inv2(grp, w)):
                        for c in range(2):
                            st_i[pl.ds(staged(s, half, n, grp, c), 8), :] = pair[c].get()
            out.append((128, lhs, rhs, consume))
        return out

    def inverse_tasks(g):
        def fn(gate, s, half):
            gate.loads(st_i, PLAN["inverse_lead"])
            qg, og, ties = view(q32, g * (L // 2), L // 2), view(ob, g * L, L), []
            for n in range(4):
                zs = [tuple(_Signed(rows(view(st_i, z8), staged(s, half, n, grp, c)))
                            for c in range(2)) for grp in range(4)]
                for m, y in enumerate(_inv1(n, zs)):
                    t = 64 * (16 * half + n + 4 * m) + 8 * s
                    og[pl.ds(t, 8), :] = _unpack(rows(qg, (t // 16) * 8))[s % 2] * y.get()
                ties.append(after(ob))
            return ties

        tasks = []
        for half in range(2):
            tasks += [([12 + n for n in ops1], lambda gate, s=s, half=half: fn(gate, s, half))
                      for s in range(8)]
            tasks.append(dma_task(ob_dma(g, half)))
        return tasks

    def dma_task(copy):
        return [1], lambda gate: copy.start()

    filter0 = x_dma(2, S_F0) + [sk_dma(0, S_F0)] + x_dma(3, S_F0)
    data0 = [col_dma(0, 0, S_K0), col_dma(1, 0, S_K0)]
    x0, x1 = x_dma(0, S_X0), x_dma(1, S_B + 4)

    def group_dma(g):
        at = S_COL + g
        return [col_dma(2, g, at), sk_dma(g + 1, at), col_dma(0, g + 1, at),
                col_dma(1, g + 1, at)] + x_dma(g + LEAD, at)

    last_dma = col_dma(2, NG - 1, S_SMALL)

    start(small + b_dma(0) + x0 + b_dma(1) + b_dma(2))
    wait(small + x0 + b_dma(0))
    zeros = rows(tab, 288).astype(I32)
    z8 = pl.multiple_of(zeros[0, 0], 16)
    sub = lax.broadcasted_iota(I32, (8, 128), 0)
    pred = zeros == 0

    def stack(ref):
        v = ref[...].astype(F32).reshape(1, D)
        return jnp.concatenate([v[:, 128 * g:128 * (g + 1)] for g in range(NG)]
                               + [v[:, :128]] * (8 - NG), axis=0)

    lre, lim = stack(lre_v), stack(lim_v)
    dt = jnp.exp(stack(ldt_v)).astype(BF16).astype(F32)
    mag, ang = jnp.exp(dt * lre), dt * lim
    lam = (mag * jnp.cos(ang), mag * jnp.sin(ang))
    scale = jnp.maximum(jnp.abs(lre), jnp.abs(lim))
    nre, nim = lre / scale, lim / scale
    den = (nre * nre + nim * nim) * scale
    coef = _cmul(((lam[0] - 1.0) / den, lam[1] / den), (nre, -nim))
    mu = lam
    rho = [mu]
    for _ in range(R.bit_length() + 2):
        rho.append(_cmul(rho[-1], rho[-1]))
    dsk, ssd = stack(dsk_v), stack(sd_v)
    taps = tap_v[...].astype(F32) * _FFT_SCALE
    for g in range(NG):
        def put(row, v):
            par[pl.ds((g * P_ROWS + row) * 8, 8), :] = v

        def lanes(v):
            return jnp.broadcast_to(v[g:g + 1], (8, 128))
        for c in range(2):
            put(P_MU + c, lanes(mu[c]))
            put(P_RHO + c, lanes(rho[-4][c]))
            for n, row in enumerate((P_RHO1, P_RHO2, P_RHO4)):
                put(row + c, jnp.where(sub >= 1 << n, lanes(rho[n - 3][c]), 0.0))
        for t in range(4):
            put(P_TAP + t, jnp.broadcast_to(taps[t:t + 1, 128 * g:128 * (g + 1)], (8, 128)))
        put(P_COEF, lanes(2.0 * coef[0]))
        put(P_COEF + 2, lanes(-2.0 * coef[1]))
        put(P_SSMD, lanes(ssd))
        put(P_DSKIP, lanes(dsk))
    for ref in (hb, oa, kf, kt, vu, vk, st_u, st_k, ob, mf, mi, wb, wc):
        ref[pl.ds(ref.shape[0] - 16, 8), pl.ds(0, 128)] = jnp.zeros((8, 128), ref.dtype)
    for i in range(2 * NG):
        carry[pl.ds(8 * i, 8), :] = jnp.zeros((8, 128), F32)
    kf[pl.ds(0, KF_PAD), :] = jnp.zeros((KF_PAD, 128), F32)

    def matrix_task(slot):
        def fn(gate):
            if slot != _REAL_SLOT:
                c, s = tab[pl.ds(256 + slot, 1), :], tab[pl.ds(272 + slot, 1), :]
            for a in range(8):
                if slot == _REAL_SLOT:
                    re, im = rows(tab, 128 + 16 * a), rows(tab, 128 + 16 * a + 8)
                else:
                    br, bi = rows(tab, 16 * a), rows(tab, 16 * a + 8)
                    re, im = c * br - s * bi, s * br + c * bi
                mf16[pl.ds(slot * 128 + 16 * a, 16), :] = _pack(re, im)
            m = pltpu.bitcast(rows(view(mf, z8), slot * 64, 64), BF16)
            mi[pl.ds(slot * 64, 64), :] = pltpu.bitcast(m.T, I32)
            return [after(mf), after(mi)]
        return ([48, 8], fn)

    def b_task(p):
        def fn(gate):
            ties = []
            for n in (p, NG + p):
                for kk in range(NG):
                    t = braw[pl.ds(128 * n, 128), pl.ds(128 * kk, 128)]
                    wb[pl.ds((n * NG + kk) * 64, 64), :] = pltpu.bitcast(t.T, I32)
                ties.append(after(wb))
            return ties
        return ([24, 24], fn)

    def c_task(n, p):
        def fn(gate):
            cr = gate.value(prm(p, P_COEF), PLAN["scale_lead"])
            nci = gate.value(prm(p, P_COEF + 2), PLAN["scale_lead"])
            t = [_unpack_tile(rows(c32, ((c * NG + p) * D + 128 * n) // 2, 64)) for c in range(2)]
            re = [_pack(cr * a0 + nci * b0, cr * a1 + nci * b1) for (a0, a1), (b0, b1) in zip(*t)]
            im = [_pack(nci * a0 - cr * b0, nci * a1 - cr * b1) for (a0, a1), (b0, b1) in zip(*t)]
            ties = []
            for c, tile in enumerate((re, im)):
                wc[pl.ds(((c * NG + p) * NG + n) * 64, 64), :] = pltpu.bitcast(
                    jnp.concatenate(tile, axis=0).T, I32)
                ties.append(after(wc))
            return ties
        return ([80, 80], fn)

    def y_block(halves, t0, lead, even, z=0):
        tiles = [(h, n) for h in halves for n in range(NG)]
        passes, plan = [], []
        for j, (h, n) in enumerate(tiles):
            sizes = (HALF,)
            if j == 0 and lead is not None:
                if not lead:
                    continue
                sizes = (32, 96)
            if j == even:
                sizes = (64, 64)
            if j == len(tiles) - 1:
                sizes = (96, 32)
            passes += y_passes(h, n, sizes, z)
            t0 += 20
            plan.append(([skip_task(h, n)], t0 + PLAN["skip"], t0 + PLAN["skip"] + 6))
        return passes, plan

    def conv_passes(between):
        passes = fwd_passes(0)
        for grp in range(1, 4):
            f = fwd_passes(grp)
            passes += f[:8] + inv_passes(grp - 1, 0) + f[8:] + inv_passes(grp - 1, 1)
        return passes + between[:8] + inv_passes(3, 0) + inv_passes(3, 1) + between[8:]

    unit = 2 * NG * NG * UNIT // 64

    first = bu_passes(0, 1, raw=True)
    first = [first[20 * p:20 * (p + 1)] for p in range(NG)]
    start(b_dma(3) + b_dma(4) + x1 + [tab_dma])
    _weave(first[0], [], pred)
    start(filter0)
    wait(b_dma(1))
    _weave(first[1], [], pred)
    start(data0 + c_dma)
    wait(b_dma(2))
    _weave(first[2], [([b_task(p) for p in range(2)], 0, 40)], pred)
    wait(b_dma(3))
    _weave(first[3], [([b_task(p) for p in range(2, 4)], 0, 40)], pred)
    start(group_dma(0))
    wait(b_dma(4) + x1 + [tab_dma])
    _weave(first[4] + bu_passes(1, 0, 64, z8), [
        ([b_task(4)], 0, 36), (scan_tasks(0, 1), 40, 40 + unit),
        ([matrix_task(slot) for slot in range(SLOTS)], *PLAN["matrix"])], pred)
    start(group_dma(1))
    wait(filter0)
    _weave(bu_passes(2, 1, 64) + bu_passes(3, 0, 64, groups=[0]), [
        (scan_tasks(1, 0), 0, unit), (transpose_tasks(0), 8, 32),
        (filter_tasks(0, 0, PLAN["filter_lead"])[1], *PLAN["filter0"])], pred)
    start(group_dma(2))
    wait(data0 + c_dma)
    yp, plan = y_block((0, 1), unit - 40, None, 2, z8)
    kv = kv_tasks(0)
    end = 2 * unit - 40
    _weave(bu_passes(3, 0, shift=True, groups=range(1, NG)) + yp, plan + [
        (scan_tasks(2, 1), *PLAN["scan0"]), (widen_tasks(0), 0, 40),
        ([c_task(n, p) for n in range(NG) for p in range(NG)], *PLAN["scale_c"]),
        (kv[:-2], PLAN["forward0"], end), (kv[-2:], end, end)], pred)
    start([oa_unit_dma(0)] + group_dma(3) + [last_dma])

    def body(i, _):
        wait(group_dma(i))
        halves = [2 + 3 * i + j for j in range(3)]
        y0 = 192 + 20 + unit
        yp, plan = y_block(halves, y0, False, 7)
        passes = conv_passes(y_passes(halves[0], 0, (32, 96))) + bu_passes(i + LEAD, 0) + yp
        early, late = filter_tasks(i + 1, PLAN["early"])
        kv, tail, end = kv_tasks(i + 1), PLAN["tail"], y0 + 280
        done = (3 * i + 2) // 2
        sent = y0 + 180 + PLAN["skip"] + 8
        _weave(passes, plan + [
            ([dma_task(oa_unit_dma(done))], sent, sent),
            (scan_tasks(i + LEAD - 1, 0), *PLAN["scan"]),
            (transpose_tasks(i + 1), *PLAN["transpose"]),
            ([skip_task(halves[0], 0)], 232, 238),
            (widen_tasks(i + 1), *PLAN["widen"]), (early, *PLAN["filter_early"]),
            (inverse_tasks(i), *PLAN["inverse"]), (late, *PLAN["filter"]),
            (kv[:-tail], PLAN["forward"], end), (kv[-tail:], end, end)], pred)
        pl.when(i % 2 == 1)(lambda: start([oa_unit_dma(done + 1)]))
        return 0

    lax.fori_loop(0, NG - 1, body, 0)

    wait([last_dma])
    last = L // UNIT - 1
    yp, plan = y_block((2 * last, 2 * last + 1), 192, True, 2)
    plan += [([dma_task(oa_dma(last, n))], t + 6, t + 6) for n, (_, _, t) in enumerate(plan[NG:])]
    _weave(conv_passes(yp), plan + [
        (scan_tasks(last, 0), 0, 170), (inverse_tasks(NG - 1), *PLAN["last_inverse"])], pred)
    wait([oa_unit_dma(u) for u in range(last)] + [oa_dma(last, n) for n in range(NG)]
         + [ob_dma(n, half) for n in range(NG) for half in range(2)])


@jax.jit
def pallas_concat_heads__ssm_conv_s5__ssm_conv_h3__prompt_kernel(
    A_x: jax.Array,
    A_Lambda_re: jax.Array,
    A_Lambda_im: jax.Array,
    A_B_re: jax.Array,
    A_B_im: jax.Array,
    A_C_re: jax.Array,
    A_C_im: jax.Array,
    A_log_dt: jax.Array,
    A_Dskip: jax.Array,
    B_q: jax.Array,
    B_k: jax.Array,
    B_v: jax.Array,
    B_shift_k: jax.Array,
    B_ssm_k: jax.Array,
    B_ssm_D: jax.Array,
):
    assert A_x.shape == (1, L, D) and B_shift_k.shape == (D, 4)
    vmem = pltpu.VMEM
    dma = pltpu.SemaphoreType.DMA
    scratch = [
        vmem(_TABLES.shape, F32),
        vmem((D,), BF16), vmem((D,), BF16), vmem((D,), BF16), vmem((D,), BF16), vmem((D,), BF16),
        vmem((4, D), BF16),
        vmem((NG * L, 128), BF16),
        vmem((2 * D, D), BF16),
        vmem((2 * NG * D, 128), BF16),
        vmem((NG * L, 128), BF16),
        vmem((NG * L, 128), BF16),
        vmem((NG * L, 128), BF16),
        vmem((D, L), BF16),
        vmem((NG * P_ROWS * 8, 128), F32),
        vmem((2 * NG * D + 32, 128), BF16),
        vmem((2 * NG * NG * 64 + 16, 128), I32),
        vmem((SLOTS * 128 + 32, 128), BF16),
        vmem((SLOTS * 64 + 16, 128), I32),
        vmem((2 * 2 * NG * BU_PART, 128), F32),
        vmem((2 * NG * L + 32, 128), BF16),
        vmem((3 * NG * 8, 128), F32),
        vmem((NG * YS_ROWS, 128), F32),
        vmem((L + 16, D), F32),
        vmem((L // 2 + 16, 128), I32),
        vmem((KF_PAD + L + 16, 128), F32),
        vmem((2 * L + 16, 128), F32),
        vmem((2 * L + 16, 128), F32),
        vmem((2 * L + 8, 128), F32),
        vmem((32 * 128 + 32, 128), BF16),
        vmem((32 * 128 + 32, 128), BF16),
        vmem((8 * 128, 128), BF16),
        vmem((8 * 128, 128), BF16),
        vmem((NG * L + 16, 128), F32),
        dma((S_END,)),
    ]
    out = pl.pallas_call(
        _kernel,
        out_shape=jax.ShapeDtypeStruct((L, 2 * D), F32),
        in_specs=[pl.BlockSpec(memory_space=pl.ANY)] * 16,
        out_specs=pl.BlockSpec(memory_space=pl.ANY),
        scratch_shapes=scratch,
        compiler_params=pltpu.CompilerParams(vmem_limit_bytes=100 * 1024 * 1024),
        name="s5_h3",
    )(_TABLES, A_x.reshape(L, D), A_Lambda_re, A_Lambda_im, A_B_re, A_B_im, A_C_re, A_C_im,
      A_log_dt, A_Dskip, B_q.reshape(L, D), B_k.reshape(L, D), B_v.reshape(L, D),
      B_shift_k.T, B_ssm_k, B_ssm_D)
    return out.reshape(1, L, 2 * D)
```

```python
import math

import jax
import jax.numpy as jnp
import numpy as np
from jax import lax
from jax.experimental import pallas as pl
from jax.experimental.pallas import tpu as pltpu

F32, BF16, I32 = jnp.float32, jnp.bfloat16, jnp.int32

L = 2048
D = 640
NG = D // 128
UNIT = 256
SEG = 16
R = UNIT // SEG
LEAD = 4
HALF = UNIT // 2
BU_PART = 9 * 2 * R
YS_ROWS = SEG * (R // 2 + 1)
KF_PAD = 8


class _Signed:
    def __init__(self, v, neg=False):
        self.v, self.neg = v, neg

    def __neg__(self):
        return _Signed(self.v, not self.neg)

    def __add__(self, o):
        if self.neg == o.neg:
            return _Signed(self.v + o.v, self.neg)
        return _Signed(o.v - self.v if self.neg else self.v - o.v)

    def __sub__(self, o):
        return self + (-o)

    def __mul__(self, c):
        return _Signed(self.v * np.float32(-c if self.neg else c))

    def get(self):
        return -self.v if self.neg else self.v


def _rot(re, im, num, den):
    num %= den
    h = math.sqrt(0.5)
    if num == 0:
        return re, im
    if 4 * num == den:
        return -im, re
    if 4 * num == 3 * den:
        return im, -re
    if 8 * num == den:
        return (re - im) * h, (re + im) * h
    if 8 * num == 3 * den:
        return (re + im) * (-h), (re - im) * h
    if 8 * num == 5 * den:
        return (im - re) * h, (re + im) * (-h)
    if 8 * num == 7 * den:
        return (re + im) * h, (im - re) * h
    c = math.cos(2 * math.pi * num / den)
    s = math.sin(2 * math.pi * num / den)
    return re * c - im * s, re * s + im * c


def _dft4(z, sign):
    (r0, i0), (r1, i1), (r2, i2), (r3, i3) = z
    ar, ai, br, bi = r0 + r2, i0 + i2, r0 - r2, i0 - i2
    cr, ci, dr, di = r1 + r3, i1 + i3, r1 - r3, i1 - i3
    plus, minus = (br - di, bi + dr), (br + di, bi - dr)
    if sign < 0:
        plus, minus = minus, plus
    return [(ar + cr, ai + ci), plus, (ar - cr, ai - ci), minus]


def _fwd1(n, u):
    a0, a1, b0, b1 = u
    p, q = _rot(a0, b0, n, 32), _rot(a1, b1, n + 4, 32)
    s0, s1 = a0 + b0, a1 + b1
    return [(p[0] + q[0], p[1] + q[1]), _rot(p[0] - q[0], p[1] - q[1], n, 8),
            _rot(a0 - b0, a1 - b1, n, 16), (s0 + s1, s0 - s1)]


def _fwd2(grp, z):
    if grp < 3:
        return _dft4(z, 1)
    s4 = [t[0] for t in z]
    d4 = [t[1] for t in z]
    p = (d4[0], d4[2])
    q = _rot(d4[1], d4[3], 1, 8)
    s5 = [s4[0] + s4[2], s4[1] + s4[3]]
    return [
        (s5[0] + s5[1], s5[0] - s5[1]),
        (s4[0] - s4[2], s4[1] - s4[3]),
        (p[0] + q[0], p[1] + q[1]),
        (p[0] - q[0], p[1] - q[1]),
    ]


def _inv2(grp, w):
    if grp < 3:
        return _dft4(w, -1)
    s5 = [w[0][0] + w[0][1], w[0][0] - w[0][1]]
    s4 = [s5[0] + w[1][0], s5[1] + w[1][1], s5[0] - w[1][0], s5[1] - w[1][1]]
    p = (w[2][0] + w[3][0], w[2][1] + w[3][1])
    q = _rot(w[2][0] - w[3][0], w[2][1] - w[3][1], -1, 8)
    d4 = [p[0], q[0], p[1], q[1]]
    return [(s4[n], d4[n]) for n in range(4)]


def _inv1(n, z):
    e = _rot(*z[1], -n, 8)
    p = _rot(z[0][0] + e[0], z[0][1] + e[1], -n, 32)
    q = _rot(z[0][0] - e[0], z[0][1] - e[1], -(n + 4), 32)
    d0, d1 = _rot(*z[2], -n, 16)
    s0, s1 = z[3][0] + z[3][1], z[3][0] - z[3][1]
    return [p[0] + (s0 + d0), q[0] + (s1 + d1), p[1] + (s0 - d0), q[1] + (s1 - d1)]


_F1 = [4 * (g + 2 * k) + 1 for g in range(2) for k in range(4)]
_F1 += [2 * (4 * k + 1) for k in range(4)] + [0, 8, 4, 20]
_REAL_SLOT = 12
SLOTS = len(_F1)


def _dft_tables():
    kap = np.arange(128)
    j = 8 * (kap // 16) + kap % 8
    part = (kap // 8) % 2
    pr, pc, jr, jc = part[:, None], part[None, :], j[:, None], j[None, :]
    lo = 2 * np.pi * jr * jc / 64
    base = np.where(pr == pc, np.cos(lo), np.where(pr == 0, -np.sin(lo), np.sin(lo)))
    hi = 2 * np.pi * (16 + 32 * (jr - 32)) * jc / 2048
    v0 = np.where(pr == 0, np.cos(lo), np.where(jr == 0, np.cos(np.pi * jc), np.sin(lo)))
    v32 = np.where(pr == 0, np.cos(hi), np.sin(hi))
    real = np.where(jr < 32, np.where(pc == 0, v0, 0.0), np.where(pc == 1, v32, 0.0))
    th = 2 * np.pi * np.outer(np.array(_F1), j) / 2048
    zeros = np.zeros((8, 128))
    return np.concatenate([base, real, np.cos(th), np.sin(th), zeros]).astype(np.float32)


_TABLES = _dft_tables()
_FFT_SCALE = 2.0 ** -10

(P_MU, P_RHO, P_RHO1, P_RHO2, P_RHO4, P_TAP, P_SSMD, P_DSKIP, P_COEF, P_ROWS) = (
    0, 2, 4, 6, 8, 10, 14, 15, 16, 20)
S_SMALL, S_F0, S_K0, S_C, S_OUT, S_X0, S_B = range(7)
S_COL = S_B + NG
S_END = S_COL + NG - 1


def _cmul(a, b):
    return a[0] * b[0] - a[1] * b[1], a[0] * b[1] + a[1] * b[0]


def _pack(lo, hi):
    return jnp.concatenate([lo, hi], axis=0).astype(BF16)


def _unpack_tile(w):
    return [_unpack(w[8 * i:8 * i + 8]) for i in range(w.shape[0] // 8)]


def _unpack(w):
    v = pltpu.bitcast(w, BF16).astype(F32)
    return v[:8], v[8:]


PLAN = dict(
    scan_lead=22, conv_lead=20, inverse_lead=44, skip_lead=24, scale_lead=40, filter_lead=36,
    scan=(0, 350), transpose=(60, 90), filter_early=(92, 200), early=4, inverse=(220, 380),
    widen=(216, 330), filter=(230, 480), forward=350, tail=3, skip=28,
    matrix=(60, 200), filter0=(36, 240),
    scale_c=(40, 290), scan0=(0, 350), forward0=60, last_inverse=(216, 290),
)


class _Zeros:
    def __init__(self, v):
        self.v = v


class _Gate:
    def __init__(self, pred=None, seen=()):
        self.pred, self.seen = pred, seen

    def early(self, lag):
        old = [e for e in self.seen if e[0] <= -lag]
        return max(old, key=lambda e: e[0])[1] if old else None

    def value(self, v, lag):
        early = self.early(lag)
        return v if early is None else jnp.where(self.pred, v, early)

    def loads(self, ref, lag):
        early = self.early(lag)
        if early is not None:
            ref[pl.ds(ref.shape[0] - 8, 8), :] = (
                early if ref.dtype == F32 else pltpu.bitcast(early, I32))


def _weave(passes, plan, pred):
    begin, clock = [], [0] * 4
    for i, (n, *_) in enumerate(passes):
        begin.append(clock[i % 4] / 16)
        clock[i % 4] += n

    def index(t):
        later = [i for i, b in enumerate(begin) if b >= t - 3.999]
        if not later:
            return len(passes)
        same = [i for i in later if begin[i] == min(begin[j] for j in later)]
        return same[min(max(int((t - begin[same[0]]) / 4 * len(same)), 0), len(same) - 1)]

    at = [[] for _ in range(len(passes) + 1)]
    for tasks, lo, hi in plan:
        total, done = sum(sum(c) for c, _ in tasks) or 1, 0.0
        for costs, fn in tasks:
            where = []
            for cost in costs:
                done += cost
                where.append(index(lo + done / total * (hi - lo)))
            at[min(where)].append((fn, where))
    seen, ties = [], [[] for _ in at]
    for i, fns in enumerate(at):
        now = (begin[i] + i % 4) if i < len(begin) else clock[0] / 16
        early = [(t - now, v) for t, v in seen]
        for fn, where in fns:
            for w, tie in zip(where, fn(_Gate(pred, early)) or ()):
                ties[w].append(tie)
        if i == len(passes):
            break
        n, lhs, rhs, consume = passes[i]
        w = rhs()
        if not isinstance(w, list):
            d = lax.dot_general(pltpu.bitcast(jnp.concatenate(lhs(), axis=0), BF16), w,
                                (((1,), (1,)), ((), ())), preferred_element_type=F32)
            consume(d)
            continue
        for tie in ties[i]:
            if isinstance(tie, _Zeros):
                v = tie.v
                w[-1] = w[-1] | (v if v.dtype == I32 else pltpu.bitcast(v, I32))
            else:
                w[-1] = jnp.where(pred, w[-1], pltpu.bitcast(tie, I32))
        d = jnp.dot(pltpu.bitcast(jnp.concatenate(lhs(), axis=0), BF16),
                    pltpu.bitcast(jnp.concatenate(w, axis=0), BF16), preferred_element_type=F32)
        seen += [(begin[i] + i % 4 + j // 16 - 4, d[j - 8:j]) for j in range(64, n + 1, 64)]
        consume(d)


def _kernel(tab_hbm, x_hbm, lre_hbm, lim_hbm, bre_hbm, bim_hbm, cre_hbm, cim_hbm,
            ldt_hbm, dsk_hbm, q_hbm, k_hbm, v_hbm, tap_hbm, sk_hbm, sd_hbm,
            o_hbm,
            tab, lre_v, lim_v, ldt_v, dsk_v, sd_v, tap_v,
            xb, braw, craw, qb, kb, vb, skb,
            par, wb16, wc, mf16, mi, bu, hb16, carry, ys, oa,
            kt, kf, st_u, st_k, st_i, vu16, vk16, pb0, pb1, ob,
            sem):
    x32, q32, k32, v32, wb, mf, hb, vu, vk = (
        r.bitcast(I32) for r in (xb, qb, kb, vb, wb16, mf16, hb16, vu16, vk16))
    c32 = craw.bitcast(I32)
    pb16 = (pb0, pb1)
    pb = (pb0.bitcast(I32), pb1.bitcast(I32))

    def rows(ref, start, n=8):
        return ref[pl.ds(start, n), :]

    def hint(v, n):
        return v if isinstance(v, int) or n == 1 else pl.multiple_of(v, n)

    def view(ref, start, n=None):
        return ref.at[pl.ds(hint(start, 16), n or ref.shape[0]), :]

    def after(ref):
        return _Zeros(view(ref, z8)[ref.shape[0] - 16:ref.shape[0] - 8, 0:128])

    small = [pltpu.make_async_copy(s, d, sem.at[S_SMALL]) for s, d in (
        (lre_hbm, lre_v), (lim_hbm, lim_v), (ldt_hbm, ldt_v),
        (dsk_hbm, dsk_v), (sd_hbm, sd_v), (tap_hbm, tap_v),
        (tab_hbm.at[pl.ds(288, 8), :], tab.at[pl.ds(288, 8), :]))]
    tab_dma = pltpu.make_async_copy(
        tab_hbm.at[pl.ds(0, 288), :], tab.at[pl.ds(0, 288), :], sem.at[S_B + 4])

    def x_dma(u, at):
        return [pltpu.make_async_copy(
            x_hbm.at[pl.ds(hint(u * UNIT, UNIT), UNIT), pl.ds(128 * n, 128)],
            xb.at[pl.ds(hint(n * L + u * UNIT, UNIT), UNIT), :], sem.at[at])
            for n in range(NG)]

    def b_dma(p):
        return [pltpu.make_async_copy(
            src.at[pl.ds(128 * p, 128), :], braw.at[pl.ds(D * c + 128 * p, 128), :],
            sem.at[S_B + p]) for c, src in enumerate((bre_hbm, bim_hbm))]

    c_dma = [pltpu.make_async_copy(
        src.at[:, pl.ds(128 * p, 128)], craw.at[pl.ds(D * (NG * c + p), D), :],
        sem.at[S_C]) for c, src in enumerate((cre_hbm, cim_hbm)) for p in range(NG)]

    def col_dma(which, g, sem_at):
        src, dst = ((k_hbm, kb), (v_hbm, vb), (q_hbm, qb))[which]
        return pltpu.make_async_copy(
            src.at[:, pl.ds(hint(128 * g, 128), 128)],
            dst.at[pl.ds(hint(L * g, L), L), :], sem.at[sem_at])

    def sk_dma(g, sem_at):
        t = hint(128 * g, 128)
        return pltpu.make_async_copy(
            sk_hbm.at[pl.ds(t, 128), :], skb.at[pl.ds(t, 128), :], sem.at[sem_at])

    def oa_dma(u, n):
        t = hint(u * UNIT, UNIT)
        return pltpu.make_async_copy(
            oa.at[pl.ds(t, UNIT), pl.ds(128 * n, 128)],
            o_hbm.at[pl.ds(t, UNIT), pl.ds(128 * n, 128)], sem.at[S_OUT])

    def oa_unit_dma(u):
        t = hint(u * UNIT, UNIT)
        return pltpu.make_async_copy(
            oa.at[pl.ds(t, UNIT), :], o_hbm.at[pl.ds(t, UNIT), pl.ds(0, D)], sem.at[S_OUT])

    def ob_dma(g, half):
        h = L // 2
        return pltpu.make_async_copy(
            ob.at[pl.ds(hint(L * g + h * half, h), h), :],
            o_hbm.at[pl.ds(h * half, h), pl.ds(hint(D + 128 * g, 128), 128)], sem.at[S_OUT])

    def start(ds):
        for d in ds:
            d.start()

    def wait(ds):
        for d in ds:
            d.wait()

    def prm(g, row):
        return rows(view(par, g * (P_ROWS * 8), P_ROWS * 8), row * 8)

    def bu_passes(u, slot, size=128, z=0, shift=False, raw=False, groups=range(NG)):
        out = []
        xu, w = view(x32, u * (UNIT // 2), ((NG - 1) * L + UNIT) // 2), view(wb, z)
        order = [p + c * NG for p in groups for c in range(2)]
        for n in order:
            sizes = [size] * (UNIT // size)
            if shift and n == order[0]:
                sizes = [32, 32, 96, 96]
            if shift and n == order[-1]:
                sizes = [64] * 4
            for m, MM in zip(np.cumsum([0] + sizes).tolist(), sizes):
                acc = []
                for kk in range(NG):
                    def lhs(m=m, kk=kk, MM=MM):
                        t = (kk * L + m) // 2
                        return [rows(xu, t + 8 * i) for i in range(MM // 16)]

                    def rhs(n=n, kk=kk):
                        if raw:
                            return braw[pl.ds(128 * n, 128), pl.ds(128 * kk, 128)]
                        return [rows(w, (n * NG + kk) * 64 + 8 * i) for i in range(8)]

                    def consume(d, m=m, n=n, kk=kk, acc=acc, MM=MM):
                        acc.append(d if kk == 0 else acc[-1] + d)
                        if kk == NG - 1:
                            for i in range(MM // 8):
                                seg, r = divmod(m + 8 * i, R)
                                row = 9 * (seg % 2 * R + r) + seg // 2
                                bu[pl.ds((slot * 2 * NG + n) * BU_PART + row, 8, stride=9), :] = (
                                    acc[-1][8 * i:8 * i + 8])
                    out.append((MM, lhs, rhs, consume))
        return out

    def scan_tasks(u, slot):
        steps, state = 2, {}
        hu = view(hb16, u * UNIT, (2 * NG - 1) * L + UNIT)

        def b(p, ch, r):
            return tuple(rows(bu, (slot * 2 * NG + c * NG + p) * BU_PART + 9 * (ch * R + r))
                         for c in range(2))

        def step(mu, h, br):
            return (mu[0] * h[0] + br[0]) - mu[1] * h[1], (mu[0] * h[1] + br[1]) + mu[1] * h[0]

        def ends(p, gate):
            mu, ties = (gate.value(prm(p, P_MU), PLAN["scan_lead"]), prm(p, P_MU + 1)), []
            h = [b(p, ch, 0) for ch in range(2)]
            for r in range(1, R):
                h = [step(mu, h[ch], b(p, ch, r)) for ch in range(2)]
                if r % steps == 0:
                    ties.append(h[r // steps % 2][0])
            state[p] = starts(p, h)
            return ties + [state[p][1][0]]

        def starts(p, e):
            last = lax.broadcasted_iota(I32, (8, 128), 0) == 7
            rho = (prm(p, P_RHO), prm(p, P_RHO + 1))
            pair = step(rho, e[0], e[1])
            a = tuple(pltpu.roll(jnp.where(last, rows(carry, (2 * p + c) * 8), pair[c]), 1, 0)
                      for c in range(2))
            for sh, row in ((1, P_RHO1), (2, P_RHO2), (4, P_RHO4)):
                a = step((prm(p, row), prm(p, row + 1)), tuple(pltpu.roll(c, sh, 0) for c in a), a)
            return [a, step(rho, a, e[0])]

        def run(p, r0, gate):
            if r0 == 0:
                state["mu"] = (prm(p, P_MU), prm(p, P_MU + 1))
            mu, h = (gate.value(state["mu"][0], PLAN["scan_lead"]), state["mu"][1]), state[p]
            for r in range(r0, r0 + steps):
                h = [step(mu, h[ch], b(p, ch, r)) for ch in range(2)]
                for c in range(2):
                    hu[pl.ds((c * NG + p) * L + 16 * r, 16), :] = _pack(h[0][c], h[1][c])
            state[p] = h
            if r0 + steps == R:
                for c in range(2):
                    carry[pl.ds((2 * p + c) * 8, 8), :] = h[1][c]
            return [after(hb)]

        tasks = []
        for p in range(NG):
            tasks.append(([16 * steps] * ((R - 1) // steps) + [46 + 16 * steps],
                          lambda gate, p=p: ends(p, gate)))
            tasks += [([18 * steps], lambda gate, p=p, r0=r0: run(p, r0, gate))
                      for r0 in range(0, R, steps)]
        return tasks

    def y_passes(h, n, sizes=(HALF,), z=0, slot=0):
        out, w, hu = [], view(wc, z), view(hb, h * (HALF // 2), ((2 * NG - 1) * L + HALF) // 2)
        for t0, MM in zip(np.cumsum((0,) + sizes).tolist(), sizes):
            acc = []
            for kk in range(2 * NG):
                def lhs(t0=t0, kk=kk, MM=MM):
                    return [rows(hu, (kk * L + t0) // 2 + 8 * i) for i in range(MM // 16)]

                def rhs(kk=kk):
                    return [rows(w, (kk * NG + n) * 64 + 8 * i) for i in range(8)]

                def consume(d, t0=t0, kk=kk, acc=acc, MM=MM):
                    acc.append(d if kk == 0 else acc[-1] + d)
                    if kk == 2 * NG - 1:
                        for i in range(MM // 8):
                            r, ch = divmod(t0 // 8 + i, 2)
                            at = (slot * NG + n) * YS_ROWS + ch * (R // 2 + 1) + r
                            ys[pl.ds(at, 8, stride=R + 2), :] = (
                                acc[-1][8 * i:8 * i + 8])
                out.append((MM, lhs, rhs, consume))
        return out

    def skip_task(h, n, slot=0):
        def fn(gate):
            dsk, ties = gate.value(prm(n, P_DSKIP), PLAN["skip_lead"]), []
            t = h // 2 * UNIT + h % 2 * (R // 2)
            edge = n == NG - 1 and isinstance(h, int)
            xu = x32.at[pl.ds(hint(t // 2 + n * (L // 2), 4), UNIT // 2 + (-4 if edge else 4)), :]
            ou = oa.at[pl.ds(hint(t, 8), UNIT - R // 2), :]
            for g in range(SEG):
                if g == SEG - 1 and edge:
                    xs = _unpack(rows(xu, 8 * g - 4))[1]
                else:
                    xs = _unpack(rows(xu, 8 * g))[0]
                y = rows(ys, (slot * NG + n) * YS_ROWS + g * (R // 2 + 1))
                ou[pl.ds(R * g, 8), pl.ds(128 * n, 128)] = y + xs * dsk
                if g % 8 == 7:
                    ties.append(after(oa))
            return ties
        return ([24, 24], fn)

    def widen_tasks(g):
        def fn(i0):
            kg = view(k32, g * (L // 2), L // 2)
            for i in range(i0, i0 + 8):
                lo, hi = _unpack(rows(kg, 8 * i))
                kf[pl.ds(KF_PAD + 16 * i, 8), :] = lo
                kf[pl.ds(KF_PAD + 16 * i + 8, 8), :] = hi
            return [after(kf)]
        return [([16], lambda gate, i=i: fn(i)) for i in range(0, L // 16, 8)]

    def transpose_tasks(g):
        n = 2

        def fn(c0):
            for c in range(c0, c0 + n):
                t = skb[pl.ds(hint(128 * g, 128), 128), pl.ds(128 * c, 128)]
                kt[pl.ds(64 * c, 64), :] = pltpu.bitcast(t.T, I32)
            return [after(kt)]
        return [([8 * n], lambda gate, c=c: fn(c)) for c in range(0, L // 128, n)]

    def staged(s, half, n, grp, c):
        return (((s * 2 + half) * 4 + n) * 4 + grp) * 16 + 8 * c

    ops1 = (18, 36, 30, 36)

    def transform_tasks(st, s, half, chunk, chunk_cost, direct):
        dst16, dst = (vu16, vu) if st is st_u else (vk16, vk)
        kept = []

        def first(gate, n):
            load = chunk(gate, n)
            u = [load(16 * half + n + 4 * m) for m in range(4)]
            pairs = _fwd1(n, [_Signed(v) for v in u])
            kept.append(pairs)
            for grp in range(2 * direct, 4):
                for c in range(2):
                    st[pl.ds(staged(s, half, n, grp, c), 8), :] = pairs[grp][c].get()
            return [u[0] + u[2]] * (chunk_cost > 4) + [after(st)]

        def second(grps):
            for grp in grps:
                if direct and grp < 2:
                    zs = [t[grp] for t in kept]
                else:
                    zs = [tuple(_Signed(rows(view(st, z8), staged(s, half, n, grp, c)))
                                for c in range(2)) for n in range(4)]
                for k, pair in enumerate(_fwd2(grp, zs)):
                    dst16[pl.ds(((4 * grp + k) * 2 + half) * 128 + 16 * s, 16), :] = (
                        _pack(pair[0].get(), pair[1].get()))
            return [after(dst)]

        split = (chunk_cost > 4) * (chunk_cost // 2 + 1)
        one = [([split] * (split > 0) + [chunk_cost + ops1[n] - split],
                lambda gate, n=n: first(gate, n)) for n in range(4)]
        two = [([40], lambda gate, grp=grp: second((grp, grp + 1))) for grp in (0, 2)]
        return (one + two[:1], two[1:]) if direct else (one, two)

    def kv_tasks(g):
        tasks = []
        for s in range(8):
            for half in range(2):
                def chunk(gate, n, s=s, loaded=[]):
                    if n == 0:
                        loaded[:] = [prm(g, P_TAP + t) for t in range(4)]
                    taps = [gate.value(loaded[0], PLAN["conv_lead"])] + loaded[1:]
                    kz, vg = view(kf, z8), view(v32, g * (L // 2), L // 2)

                    def load(c):
                        t = 64 * c + 8 * s
                        ks = rows(kz, KF_PAD + t) * taps[0]
                        for lag in range(1, 4):
                            ks = ks + rows(kz, KF_PAD + t - lag) * taps[lag]
                        return ks * _unpack(rows(vg, (t // 16) * 8))[s % 2]
                    return load
                tasks += sum(transform_tasks(st_u, s, half, chunk, 36, True), [])
        return tasks

    def filter_tasks(g, early, lead=None):
        before, after_use = [], []
        for j in range(16):
            def chunk(gate, n, s=j // 2):
                if lead:
                    gate.loads(kt, lead)

                def load(c):
                    v = _unpack(rows(view(kt, z8), 32 * c + 8 * (s // 2)))[s % 2]
                    if s == 0 and c == 0:
                        first = lax.broadcasted_iota(I32, (8, 128), 0) == 0
                        v = v + jnp.where(first, prm(g, P_SSMD), 0.0)
                    return v
                return load
            one, two = transform_tasks(st_k, j // 2, j % 2, chunk, 4, j >= early)
            before += one if j < early else []
            after_use += two if j < early else one + two
        return before, after_use

    def fwd_passes(grp):
        out = []
        for slot in range(4 * grp, 4 * grp + 4):
            got = []
            for src, half in ((vu, 0), (vk, 0), (vu, 1), (vk, 1)):
                def lhs(slot=slot):
                    return [rows(mf, slot * 64 + 8 * i) for i in range(8)]

                def rhs(slot=slot, src=src, half=half):
                    return [rows(view(src, z8), (2 * slot + half) * 64 + 8 * i) for i in range(8)]

                def consume(d, slot=slot, got=got):
                    got.append(d)
                    if len(got) < 4:
                        return
                    for i in range(8):
                        u0, k0, u1, k1 = (
                            (t[16 * i:16 * i + 8], t[16 * i + 8:16 * i + 16]) for t in got)
                        lo, a, b = _cmul(u0, k0), _cmul(u0, k1), _cmul(u1, k0)
                        if slot == _REAL_SLOT and i == 0:
                            first = lax.broadcasted_iota(I32, (8, 128), 0) == 0
                            lo, a, b = (
                                tuple(jnp.where(first, 0.5 * (x[c] * y[c]), p[c]) for c in range(2))
                                for p, x, y in ((lo, u0, k0), (a, u0, k1), (b, u1, k0)))
                        if _F1[slot] % 2:
                            hi = ((a[0] + b[0]) - lo[0], (a[1] + b[1]) - lo[1])
                        else:
                            hi = ((a[0] + b[0]) + lo[0], (a[1] + b[1]) + lo[1])
                        for half, p in enumerate((lo, hi)):
                            at = (slot % 4 * 2 + half) * 128 + 16 * i
                            pb16[grp % 2][pl.ds(at, 16), :] = _pack(*p)
                out.append((128, lhs, rhs, consume))
        return out

    def inv_passes(grp, half):
        out, got = [], []
        for slot in range(4 * grp, 4 * grp + 4):
            def lhs(slot=slot):
                return [rows(mi, slot * 64 + 8 * i) for i in range(8)]

            def rhs(slot=slot):
                return [rows(view(pb[grp % 2], z8), (slot % 4 * 2 + half) * 64 + 8 * i)
                        for i in range(8)]

            def consume(d):
                got.append(d)
                if len(got) < 4:
                    return
                for s in range(8):
                    w = [(_Signed(t[16 * s:16 * s + 8]), _Signed(t[16 * s + 8:16 * s + 16]))
                         for t in got]
                    for n, pair in enumerate(_inv2(grp, w)):
                        for c in range(2):
                            st_i[pl.ds(staged(s, half, n, grp, c), 8), :] = pair[c].get()
            out.append((128, lhs, rhs, consume))
        return out

    def inverse_tasks(g):
        def fn(gate, s, half):
            gate.loads(st_i, PLAN["inverse_lead"])
            qg, og, ties = view(q32, g * (L // 2), L // 2), view(ob, g * L, L), []
            for n in range(4):
                zs = [tuple(_Signed(rows(view(st_i, z8), staged(s, half, n, grp, c)))
                            for c in range(2)) for grp in range(4)]
                for m, y in enumerate(_inv1(n, zs)):
                    t = 64 * (16 * half + n + 4 * m) + 8 * s
                    og[pl.ds(t, 8), :] = _unpack(rows(qg, (t // 16) * 8))[s % 2] * y.get()
                ties.append(after(ob))
            return ties

        tasks = []
        for half in range(2):
            tasks += [([12 + n for n in ops1], lambda gate, s=s, half=half: fn(gate, s, half))
                      for s in range(8)]
            tasks.append(dma_task(ob_dma(g, half)))
        return tasks

    def dma_task(copy):
        return [1], lambda gate: copy.start()

    filter0 = x_dma(2, S_F0) + [sk_dma(0, S_F0)] + x_dma(3, S_F0)
    data0 = [col_dma(0, 0, S_K0), col_dma(1, 0, S_K0)]
    x0, x1 = x_dma(0, S_X0), x_dma(1, S_B + 4)

    def group_dma(g):
        at = S_COL + g
        return [col_dma(2, g, at), sk_dma(g + 1, at), col_dma(0, g + 1, at),
                col_dma(1, g + 1, at)] + x_dma(g + LEAD, at)

    last_dma = col_dma(2, NG - 1, S_SMALL)

    start(small + b_dma(0) + x0 + b_dma(1) + b_dma(2))
    wait(small + x0 + b_dma(0))
    zeros = rows(tab, 288).astype(I32)
    z8 = pl.multiple_of(zeros[0, 0], 16)
    sub = lax.broadcasted_iota(I32, (8, 128), 0)
    pred = zeros == 0

    def stack(ref):
        v = ref[...].astype(F32).reshape(1, D)
        return jnp.concatenate([v[:, 128 * g:128 * (g + 1)] for g in range(NG)]
                               + [v[:, :128]] * (8 - NG), axis=0)

    lre, lim = stack(lre_v), stack(lim_v)
    dt = jnp.exp(stack(ldt_v)).astype(BF16).astype(F32)
    mag, ang = jnp.exp(dt * lre), dt * lim
    lam = (mag * jnp.cos(ang), mag * jnp.sin(ang))
    scale = jnp.maximum(jnp.abs(lre), jnp.abs(lim))
    nre, nim = lre / scale, lim / scale
    den = (nre * nre + nim * nim) * scale
    coef = _cmul(((lam[0] - 1.0) / den, lam[1] / den), (nre, -nim))
    mu = lam
    rho = [mu]
    for _ in range(R.bit_length() + 2):
        rho.append(_cmul(rho[-1], rho[-1]))
    dsk, ssd = stack(dsk_v), stack(sd_v)
    taps = tap_v[...].astype(F32) * _FFT_SCALE
    for g in range(NG):
        def put(row, v):
            par[pl.ds((g * P_ROWS + row) * 8, 8), :] = v

        def lanes(v):
            return jnp.broadcast_to(v[g:g + 1], (8, 128))
        for c in range(2):
            put(P_MU + c, lanes(mu[c]))
            put(P_RHO + c, lanes(rho[-4][c]))
            for n, row in enumerate((P_RHO1, P_RHO2, P_RHO4)):
                put(row + c, jnp.where(sub >= 1 << n, lanes(rho[n - 3][c]), 0.0))
        for t in range(4):
            put(P_TAP + t, jnp.broadcast_to(taps[t:t + 1, 128 * g:128 * (g + 1)], (8, 128)))
        put(P_COEF, lanes(2.0 * coef[0]))
        put(P_COEF + 2, lanes(-2.0 * coef[1]))
        put(P_SSMD, lanes(ssd))
        put(P_DSKIP, lanes(dsk))
    for ref in (hb, oa, kf, kt, vu, vk, st_u, st_k, ob, mf, mi, wb, wc):
        ref[pl.ds(ref.shape[0] - 16, 8), pl.ds(0, 128)] = jnp.zeros((8, 128), ref.dtype)
    for i in range(2 * NG):
        carry[pl.ds(8 * i, 8), :] = jnp.zeros((8, 128), F32)
    kf[pl.ds(0, KF_PAD), :] = jnp.zeros((KF_PAD, 128), F32)

    def matrix_task(slot):
        def fn(gate):
            if slot != _REAL_SLOT:
                c, s = tab[pl.ds(256 + slot, 1), :], tab[pl.ds(272 + slot, 1), :]
            for a in range(8):
                if slot == _REAL_SLOT:
                    re, im = rows(tab, 128 + 16 * a), rows(tab, 128 + 16 * a + 8)
                else:
                    br, bi = rows(tab, 16 * a), rows(tab, 16 * a + 8)
                    re, im = c * br - s * bi, s * br + c * bi
                mf16[pl.ds(slot * 128 + 16 * a, 16), :] = _pack(re, im)
            m = pltpu.bitcast(rows(view(mf, z8), slot * 64, 64), BF16)
            mi[pl.ds(slot * 64, 64), :] = pltpu.bitcast(m.T, I32)
            return [after(mf), after(mi)]
        return ([48, 8], fn)

    def b_task(p):
        def fn(gate):
            ties = []
            for n in (p, NG + p):
                for kk in range(NG):
                    t = braw[pl.ds(128 * n, 128), pl.ds(128 * kk, 128)]
                    wb[pl.ds((n * NG + kk) * 64, 64), :] = pltpu.bitcast(t.T, I32)
                ties.append(after(wb))
            return ties
        return ([24, 24], fn)

    def c_task(n, p):
        def fn(gate):
            cr = gate.value(prm(p, P_COEF), PLAN["scale_lead"])
            nci = gate.value(prm(p, P_COEF + 2), PLAN["scale_lead"])
            t = [_unpack_tile(rows(c32, ((c * NG + p) * D + 128 * n) // 2, 64)) for c in range(2)]
            re = [_pack(cr * a0 + nci * b0, cr * a1 + nci * b1) for (a0, a1), (b0, b1) in zip(*t)]
            im = [_pack(nci * a0 - cr * b0, nci * a1 - cr * b1) for (a0, a1), (b0, b1) in zip(*t)]
            ties = []
            for c, tile in enumerate((re, im)):
                wc[pl.ds(((c * NG + p) * NG + n) * 64, 64), :] = pltpu.bitcast(
                    jnp.concatenate(tile, axis=0).T, I32)
                ties.append(after(wc))
            return ties
        return ([80, 80], fn)

    def y_block(halves, t0, lead, even, z=0, by_group=False):
        tiles = [(h, n) for h in halves for n in range(NG)]
        if by_group:
            tiles.sort(key=lambda tile: tile[1])
        passes, plan = [], []
        for j, (h, n) in enumerate(tiles):
            sizes = (HALF,)
            if j == 0 and lead is not None:
                if not lead:
                    continue
                sizes = (32, 96)
            if j == even:
                sizes = (64, 64)
            if j == len(tiles) - 1:
                sizes = (96, 32)
            slot = h if by_group else 0
            passes += y_passes(h, n, sizes, z, slot)
            t0 += 20
            plan.append(([skip_task(h, n, slot)], t0 + PLAN["skip"], t0 + PLAN["skip"] + 6))
        return passes, plan

    def conv_passes(between):
        passes = fwd_passes(0)
        for grp in range(1, 4):
            f = fwd_passes(grp)
            passes += f[:8] + inv_passes(grp - 1, 0) + f[8:] + inv_passes(grp - 1, 1)
        return passes + between[:8] + inv_passes(3, 0) + inv_passes(3, 1) + between[8:]

    unit = 2 * NG * NG * UNIT // 64

    first = bu_passes(0, 1, raw=True)
    first = [first[20 * p:20 * (p + 1)] for p in range(NG)]
    start(b_dma(3) + b_dma(4) + x1 + [tab_dma])
    _weave(first[0], [], pred)
    start(filter0)
    wait(b_dma(1))
    _weave(first[1], [], pred)
    start(data0 + c_dma)
    wait(b_dma(2))
    _weave(first[2], [([b_task(p) for p in range(2)], 0, 40)], pred)
    wait(b_dma(3))
    _weave(first[3], [([b_task(p) for p in range(2, 4)], 0, 40)], pred)
    start(group_dma(0))
    wait(b_dma(4) + x1 + [tab_dma])
    _weave(first[4] + bu_passes(1, 0, 64, z8), [
        ([b_task(4)], 0, 36), (scan_tasks(0, 1), 40, 40 + unit),
        ([matrix_task(slot) for slot in range(SLOTS)], *PLAN["matrix"])], pred)
    start(group_dma(1))
    wait(filter0)
    _weave(bu_passes(2, 1, 64) + bu_passes(3, 0, 64, groups=[0]), [
        (scan_tasks(1, 0), 0, unit), (transpose_tasks(0), 8, 32),
        (filter_tasks(0, 0, PLAN["filter_lead"])[1], *PLAN["filter0"])], pred)
    start(group_dma(2))
    wait(data0 + c_dma)
    yp, plan = y_block((0, 1), unit - 40, None, 2, z8, by_group=True)
    kv = kv_tasks(0)
    end = 2 * unit - 40
    _weave(bu_passes(3, 0, shift=True, groups=range(1, NG)) + yp, plan + [
        (scan_tasks(2, 1), *PLAN["scan0"]), (widen_tasks(0), 0, 40),
        ([c_task(n, p) for n in range(NG) for p in range(NG)], *PLAN["scale_c"]),
        (kv[:-2], PLAN["forward0"], end), (kv[-2:], end, end)], pred)
    start([oa_unit_dma(0)] + group_dma(3) + [last_dma])

    def body(i, _):
        wait(group_dma(i))
        halves = [2 + 3 * i + j for j in range(3)]
        y0 = 192 + 20 + unit
        yp, plan = y_block(halves, y0, False, 7)
        passes = conv_passes(y_passes(halves[0], 0, (32, 96))) + bu_passes(i + LEAD, 0) + yp
        early, late = filter_tasks(i + 1, PLAN["early"])
        kv, tail, end = kv_tasks(i + 1), PLAN["tail"], y0 + 280
        done = (3 * i + 2) // 2
        sent = y0 + 180 + PLAN["skip"] + 8
        _weave(passes, plan + [
            ([dma_task(oa_unit_dma(done))], sent, sent),
            (scan_tasks(i + LEAD - 1, 0), *PLAN["scan"]),
            (transpose_tasks(i + 1), *PLAN["transpose"]),
            ([skip_task(halves[0], 0)], 232, 238),
            (widen_tasks(i + 1), *PLAN["widen"]), (early, *PLAN["filter_early"]),
            (inverse_tasks(i), *PLAN["inverse"]), (late, *PLAN["filter"]),
            (kv[:-tail], PLAN["forward"], end), (kv[-tail:], end, end)], pred)
        pl.when(i % 2 == 1)(lambda: start([oa_unit_dma(done + 1)]))
        return 0

    lax.fori_loop(0, NG - 1, body, 0)

    wait([last_dma])
    last = L // UNIT - 1
    yp, plan = y_block((2 * last, 2 * last + 1), 192, True, 2)
    plan += [([dma_task(oa_dma(last, n))], t + 6, t + 6) for n, (_, _, t) in enumerate(plan[NG:])]
    _weave(conv_passes(yp), plan + [
        (scan_tasks(last, 0), 0, 170), (inverse_tasks(NG - 1), *PLAN["last_inverse"])], pred)
    wait([oa_unit_dma(u) for u in range(last)] + [oa_dma(last, n) for n in range(NG)]
         + [ob_dma(n, half) for n in range(NG) for half in range(2)])


@jax.jit
def pallas_concat_heads__ssm_conv_s5__ssm_conv_h3__prompt_kernel(
    A_x: jax.Array,
    A_Lambda_re: jax.Array,
    A_Lambda_im: jax.Array,
    A_B_re: jax.Array,
    A_B_im: jax.Array,
    A_C_re: jax.Array,
    A_C_im: jax.Array,
    A_log_dt: jax.Array,
    A_Dskip: jax.Array,
    B_q: jax.Array,
    B_k: jax.Array,
    B_v: jax.Array,
    B_shift_k: jax.Array,
    B_ssm_k: jax.Array,
    B_ssm_D: jax.Array,
):
    assert A_x.shape == (1, L, D) and B_shift_k.shape == (D, 4)
    vmem = pltpu.VMEM
    dma = pltpu.SemaphoreType.DMA
    scratch = [
        vmem(_TABLES.shape, F32),
        vmem((D,), BF16), vmem((D,), BF16), vmem((D,), BF16), vmem((D,), BF16), vmem((D,), BF16),
        vmem((4, D), BF16),
        vmem((NG * L, 128), BF16),
        vmem((2 * D, D), BF16),
        vmem((2 * NG * D, 128), BF16),
        vmem((NG * L, 128), BF16),
        vmem((NG * L, 128), BF16),
        vmem((NG * L, 128), BF16),
        vmem((D, L), BF16),
        vmem((NG * P_ROWS * 8, 128), F32),
        vmem((2 * NG * D + 32, 128), BF16),
        vmem((2 * NG * NG * 64 + 16, 128), I32),
        vmem((SLOTS * 128 + 32, 128), BF16),
        vmem((SLOTS * 64 + 16, 128), I32),
        vmem((2 * 2 * NG * BU_PART, 128), F32),
        vmem((2 * NG * L + 32, 128), BF16),
        vmem((3 * NG * 8, 128), F32),
        vmem((2 * NG * YS_ROWS, 128), F32),
        vmem((L + 16, D), F32),
        vmem((L // 2 + 16, 128), I32),
        vmem((KF_PAD + L + 16, 128), F32),
        vmem((2 * L + 16, 128), F32),
        vmem((2 * L + 16, 128), F32),
        vmem((2 * L + 8, 128), F32),
        vmem((32 * 128 + 32, 128), BF16),
        vmem((32 * 128 + 32, 128), BF16),
        vmem((8 * 128, 128), BF16),
        vmem((8 * 128, 128), BF16),
        vmem((NG * L + 16, 128), F32),
        dma((S_END,)),
    ]
    out = pl.pallas_call(
        _kernel,
        out_shape=jax.ShapeDtypeStruct((L, 2 * D), F32),
        in_specs=[pl.BlockSpec(memory_space=pl.ANY)] * 16,
        out_specs=pl.BlockSpec(memory_space=pl.ANY),
        scratch_shapes=scratch,
        compiler_params=pltpu.CompilerParams(vmem_limit_bytes=100 * 1024 * 1024),
        name="s5_h3",
    )(_TABLES, A_x.reshape(L, D), A_Lambda_re, A_Lambda_im, A_B_re, A_B_im, A_C_re, A_C_im,
      A_log_dt, A_Dskip, B_q.reshape(L, D), B_k.reshape(L, D), B_v.reshape(L, D),
      B_shift_k.T, B_ssm_k, B_ssm_D)
    return out.reshape(1, L, 2 * D)
```

```python
import math

import jax
import jax.numpy as jnp
import numpy as np
from jax import lax
from jax.experimental import pallas as pl
from jax.experimental.pallas import tpu as pltpu

F32, BF16, I32 = jnp.float32, jnp.bfloat16, jnp.int32

L = 2048
D = 640
NG = D // 128
UNIT = 256
SEG = 16
R = UNIT // SEG
LEAD = 4
HALF = UNIT // 2
BU_PART = 9 * 2 * R
YS_ROWS = SEG * (R // 2 + 1)
KF_PAD = 8


class _Signed:
    def __init__(self, v, neg=False):
        self.v, self.neg = v, neg

    def __neg__(self):
        return _Signed(self.v, not self.neg)

    def __add__(self, o):
        if self.neg == o.neg:
            return _Signed(self.v + o.v, self.neg)
        return _Signed(o.v - self.v if self.neg else self.v - o.v)

    def __sub__(self, o):
        return self + (-o)

    def __mul__(self, c):
        return _Signed(self.v * np.float32(-c if self.neg else c))

    def get(self):
        return -self.v if self.neg else self.v


def _rot(re, im, num, den):
    num %= den
    h = math.sqrt(0.5)
    if num == 0:
        return re, im
    if 4 * num == den:
        return -im, re
    if 4 * num == 3 * den:
        return im, -re
    if 8 * num == den:
        return (re - im) * h, (re + im) * h
    if 8 * num == 3 * den:
        return (re + im) * (-h), (re - im) * h
    if 8 * num == 5 * den:
        return (im - re) * h, (re + im) * (-h)
    if 8 * num == 7 * den:
        return (re + im) * h, (im - re) * h
    c = math.cos(2 * math.pi * num / den)
    s = math.sin(2 * math.pi * num / den)
    return re * c - im * s, re * s + im * c


def _dft4(z, sign):
    (r0, i0), (r1, i1), (r2, i2), (r3, i3) = z
    ar, ai, br, bi = r0 + r2, i0 + i2, r0 - r2, i0 - i2
    cr, ci, dr, di = r1 + r3, i1 + i3, r1 - r3, i1 - i3
    plus, minus = (br - di, bi + dr), (br + di, bi - dr)
    if sign < 0:
        plus, minus = minus, plus
    return [(ar + cr, ai + ci), plus, (ar - cr, ai - ci), minus]


def _fwd1(n, u):
    a0, a1, b0, b1 = u
    p, q = _rot(a0, b0, n, 32), _rot(a1, b1, n + 4, 32)
    s0, s1 = a0 + b0, a1 + b1
    return [(p[0] + q[0], p[1] + q[1]), _rot(p[0] - q[0], p[1] - q[1], n, 8),
            _rot(a0 - b0, a1 - b1, n, 16), (s0 + s1, s0 - s1)]


def _fwd2(grp, z):
    if grp < 3:
        return _dft4(z, 1)
    s4 = [t[0] for t in z]
    d4 = [t[1] for t in z]
    p = (d4[0], d4[2])
    q = _rot(d4[1], d4[3], 1, 8)
    s5 = [s4[0] + s4[2], s4[1] + s4[3]]
    return [
        (s5[0] + s5[1], s5[0] - s5[1]),
        (s4[0] - s4[2], s4[1] - s4[3]),
        (p[0] + q[0], p[1] + q[1]),
        (p[0] - q[0], p[1] - q[1]),
    ]


def _inv2(grp, w):
    if grp < 3:
        return _dft4(w, -1)
    s5 = [w[0][0] + w[0][1], w[0][0] - w[0][1]]
    s4 = [s5[0] + w[1][0], s5[1] + w[1][1], s5[0] - w[1][0], s5[1] - w[1][1]]
    p = (w[2][0] + w[3][0], w[2][1] + w[3][1])
    q = _rot(w[2][0] - w[3][0], w[2][1] - w[3][1], -1, 8)
    d4 = [p[0], q[0], p[1], q[1]]
    return [(s4[n], d4[n]) for n in range(4)]


def _inv1(n, z):
    e = _rot(*z[1], -n, 8)
    p = _rot(z[0][0] + e[0], z[0][1] + e[1], -n, 32)
    q = _rot(z[0][0] - e[0], z[0][1] - e[1], -(n + 4), 32)
    d0, d1 = _rot(*z[2], -n, 16)
    s0, s1 = z[3][0] + z[3][1], z[3][0] - z[3][1]
    return [p[0] + (s0 + d0), q[0] + (s1 + d1), p[1] + (s0 - d0), q[1] + (s1 - d1)]


_F1 = [4 * (g + 2 * k) + 1 for g in range(2) for k in range(4)]
_F1 += [2 * (4 * k + 1) for k in range(4)] + [0, 8, 4, 20]
_REAL_SLOT = 12
SLOTS = len(_F1)


def _dft_tables():
    kap = np.arange(128)
    j = 8 * (kap // 16) + kap % 8
    part = (kap // 8) % 2
    pr, pc, jr, jc = part[:, None], part[None, :], j[:, None], j[None, :]
    lo = 2 * np.pi * jr * jc / 64
    base = np.where(pr == pc, np.cos(lo), np.where(pr == 0, -np.sin(lo), np.sin(lo)))
    hi = 2 * np.pi * (16 + 32 * (jr - 32)) * jc / 2048
    v0 = np.where(pr == 0, np.cos(lo), np.where(jr == 0, np.cos(np.pi * jc), np.sin(lo)))
    v32 = np.where(pr == 0, np.cos(hi), np.sin(hi))
    real = np.where(jr < 32, np.where(pc == 0, v0, 0.0), np.where(pc == 1, v32, 0.0))
    th = 2 * np.pi * np.outer(np.array(_F1), j) / 2048
    zeros = np.zeros((8, 128))
    return np.concatenate([base, real, np.cos(th), np.sin(th), zeros]).astype(np.float32)


_TABLES = _dft_tables()
_FFT_SCALE = 2.0 ** -10

(P_MU, P_RHO, P_RHO1, P_RHO2, P_RHO4, P_TAP, P_SSMD, P_DSKIP, P_COEF, P_ROWS) = (
    0, 2, 4, 6, 8, 10, 14, 15, 16, 20)
S_SMALL, S_F0, S_K0, S_C, S_OUT, S_X0, S_B = range(7)
S_COL = S_B + NG
S_END = S_COL + NG - 1


def _cmul(a, b):
    return a[0] * b[0] - a[1] * b[1], a[0] * b[1] + a[1] * b[0]


def _pack(lo, hi):
    return jnp.concatenate([lo, hi], axis=0).astype(BF16)


def _unpack_tile(w):
    return [_unpack(w[8 * i:8 * i + 8]) for i in range(w.shape[0] // 8)]


def _unpack(w):
    v = pltpu.bitcast(w, BF16).astype(F32)
    return v[:8], v[8:]


PLAN = dict(
    scan_lead=22, conv_lead=20, inverse_lead=42, skip_lead=24, scale_lead=40, filter_lead=36,
    scan=(0, 350), transpose=(60, 90), filter_early=(92, 200), early=4, inverse=(220, 380),
    widen=(216, 330), filter=(230, 480), forward=350, tail=3, skip=28,
    matrix=(40, 200), filter0=(36, 240),
    scale_c=(40, 290), scan0=(0, 350), forward0=60, last_inverse=(216, 290),
)


class _Zeros:
    def __init__(self, v):
        self.v = v


class _Gate:
    def __init__(self, pred=None, seen=()):
        self.pred, self.seen = pred, seen

    def early(self, lag):
        old = [e for e in self.seen if e[0] <= -lag]
        return max(old, key=lambda e: e[0])[1] if old else None

    def value(self, v, lag):
        early = self.early(lag)
        return v if early is None else jnp.where(self.pred, v, early)

    def loads(self, ref, lag):
        early = self.early(lag)
        if early is not None:
            ref[pl.ds(ref.shape[0] - 8, 8), :] = (
                early if ref.dtype == F32 else pltpu.bitcast(early, I32))


def _weave(passes, plan, pred):
    begin, clock = [], [0] * 4
    for i, (n, *_) in enumerate(passes):
        begin.append(clock[i % 4] / 16)
        clock[i % 4] += n

    def index(t):
        later = [i for i, b in enumerate(begin) if b >= t - 3.999]
        if not later:
            return len(passes)
        same = [i for i in later if begin[i] == min(begin[j] for j in later)]
        return same[min(max(int((t - begin[same[0]]) / 4 * len(same)), 0), len(same) - 1)]

    at = [[] for _ in range(len(passes) + 1)]
    for tasks, lo, hi in plan:
        total, done = sum(sum(c) for c, _ in tasks) or 1, 0.0
        for costs, fn in tasks:
            where = []
            for cost in costs:
                done += cost
                where.append(index(lo + done / total * (hi - lo)))
            at[min(where)].append((fn, where))
    seen, ties = [], [[] for _ in at]
    for i, fns in enumerate(at):
        now = (begin[i] + i % 4) if i < len(begin) else clock[0] / 16
        early = [(t - now, v) for t, v in seen]
        for fn, where in fns:
            for w, tie in zip(where, fn(_Gate(pred, early)) or ()):
                ties[w].append(tie)
        if i == len(passes):
            break
        n, lhs, rhs, consume = passes[i]
        w = rhs()
        if not isinstance(w, list):
            d = lax.dot_general(pltpu.bitcast(jnp.concatenate(lhs(), axis=0), BF16), w,
                                (((1,), (1,)), ((), ())), preferred_element_type=F32)
            consume(d)
            continue
        for tie in ties[i]:
            if isinstance(tie, _Zeros):
                v = tie.v
                w[-1] = w[-1] | (v if v.dtype == I32 else pltpu.bitcast(v, I32))
            else:
                w[-1] = jnp.where(pred, w[-1], pltpu.bitcast(tie, I32))
        d = jnp.dot(pltpu.bitcast(jnp.concatenate(lhs(), axis=0), BF16),
                    pltpu.bitcast(jnp.concatenate(w, axis=0), BF16), preferred_element_type=F32)
        seen += [(begin[i] + i % 4 + j // 16 - 4, d[j - 8:j]) for j in range(64, n + 1, 64)]
        consume(d)


def _kernel(tab_hbm, x_hbm, lre_hbm, lim_hbm, bre_hbm, bim_hbm, cre_hbm, cim_hbm,
            ldt_hbm, dsk_hbm, q_hbm, k_hbm, v_hbm, tap_hbm, sk_hbm, sd_hbm,
            o_hbm,
            tab, lre_v, lim_v, ldt_v, dsk_v, sd_v, tap_v,
            xb, braw, craw, qb, kb, vb, skb,
            par, wb16, wc, mf16, mi, bu, hb16, carry, ys, oa,
            kt, kf, st_u, st_k, st_i, vu16, vk16, pb0, pb1, ob,
            sem):
    x32, q32, k32, v32, wb, mf, hb, vu, vk = (
        r.bitcast(I32) for r in (xb, qb, kb, vb, wb16, mf16, hb16, vu16, vk16))
    c32 = craw.bitcast(I32)
    pb16 = (pb0, pb1)
    pb = (pb0.bitcast(I32), pb1.bitcast(I32))

    def rows(ref, start, n=8):
        return ref[pl.ds(start, n), :]

    def hint(v, n):
        return v if isinstance(v, int) or n == 1 else pl.multiple_of(v, n)

    def view(ref, start, n=None):
        return ref.at[pl.ds(hint(start, 16), n or ref.shape[0]), :]

    def after(ref):
        return _Zeros(view(ref, z8)[ref.shape[0] - 16:ref.shape[0] - 8, 0:128])

    small = [pltpu.make_async_copy(s, d, sem.at[S_SMALL]) for s, d in (
        (lre_hbm, lre_v), (lim_hbm, lim_v), (ldt_hbm, ldt_v),
        (dsk_hbm, dsk_v), (sd_hbm, sd_v), (tap_hbm, tap_v),
        (tab_hbm.at[pl.ds(288, 8), :], tab.at[pl.ds(288, 8), :]))]
    tab_dma = pltpu.make_async_copy(
        tab_hbm.at[pl.ds(0, 288), :], tab.at[pl.ds(0, 288), :], sem.at[S_X0])

    def x_dma(u, at):
        return [pltpu.make_async_copy(
            x_hbm.at[pl.ds(hint(u * UNIT, UNIT), UNIT), pl.ds(128 * n, 128)],
            xb.at[pl.ds(hint(n * L + u * UNIT, UNIT), UNIT), :], sem.at[at])
            for n in range(NG)]

    def b_dma(p):
        return [pltpu.make_async_copy(
            src.at[pl.ds(128 * p, 128), :], braw.at[pl.ds(D * c + 128 * p, 128), :],
            sem.at[S_B + p]) for c, src in enumerate((bre_hbm, bim_hbm))]

    c_dma = [pltpu.make_async_copy(
        src.at[:, pl.ds(128 * p, 128)], craw.at[pl.ds(D * (NG * c + p), D), :],
        sem.at[S_C]) for c, src in enumerate((cre_hbm, cim_hbm)) for p in range(NG)]

    def col_dma(which, g, sem_at):
        src, dst = ((k_hbm, kb), (v_hbm, vb), (q_hbm, qb))[which]
        return pltpu.make_async_copy(
            src.at[:, pl.ds(hint(128 * g, 128), 128)],
            dst.at[pl.ds(hint(L * g, L), L), :], sem.at[sem_at])

    def sk_dma(g, sem_at):
        t = hint(128 * g, 128)
        return pltpu.make_async_copy(
            sk_hbm.at[pl.ds(t, 128), :], skb.at[pl.ds(t, 128), :], sem.at[sem_at])

    def oa_dma(u, n):
        t = hint(u * UNIT, UNIT)
        return pltpu.make_async_copy(
            oa.at[pl.ds(t, UNIT), pl.ds(128 * n, 128)],
            o_hbm.at[pl.ds(t, UNIT), pl.ds(128 * n, 128)], sem.at[S_OUT])

    def oa_unit_dma(u):
        t = hint(u * UNIT, UNIT)
        return pltpu.make_async_copy(
            oa.at[pl.ds(t, UNIT), :], o_hbm.at[pl.ds(t, UNIT), pl.ds(0, D)], sem.at[S_OUT])

    def ob_dma(g, half):
        h = L // 2
        return pltpu.make_async_copy(
            ob.at[pl.ds(hint(L * g + h * half, h), h), :],
            o_hbm.at[pl.ds(h * half, h), pl.ds(hint(D + 128 * g, 128), 128)], sem.at[S_OUT])

    def start(ds):
        for d in ds:
            d.start()

    def wait(ds):
        for d in ds:
            d.wait()

    def prm(g, row):
        return rows(view(par, g * (P_ROWS * 8), P_ROWS * 8), row * 8)

    def bu_passes(u, slot, size=128, z=0, shift=False, raw=False, groups=range(NG)):
        out = []
        xu, w = view(x32, u * (UNIT // 2), ((NG - 1) * L + UNIT) // 2), view(wb, z)
        order = [p + c * NG for p in groups for c in range(2)]
        for n in order:
            sizes = [size] * (UNIT // size)
            if shift and n == order[0]:
                sizes = [32, 32, 96, 96]
            if shift and n == order[-1]:
                sizes = [64] * 4
            for m, MM in zip(np.cumsum([0] + sizes).tolist(), sizes):
                acc = []
                for kk in range(NG):
                    def lhs(m=m, kk=kk, MM=MM):
                        t = (kk * L + m) // 2
                        return [rows(xu, t + 8 * i) for i in range(MM // 16)]

                    def rhs(n=n, kk=kk):
                        if raw:
                            return braw[pl.ds(128 * n, 128), pl.ds(128 * kk, 128)]
                        return [rows(w, (n * NG + kk) * 64 + 8 * i) for i in range(8)]

                    def consume(d, m=m, n=n, kk=kk, acc=acc, MM=MM):
                        acc.append(d if kk == 0 else acc[-1] + d)
                        if kk == NG - 1:
                            for i in range(MM // 8):
                                seg, r = divmod(m + 8 * i, R)
                                row = 9 * (seg % 2 * R + r) + seg // 2
                                bu[pl.ds((slot * 2 * NG + n) * BU_PART + row, 8, stride=9), :] = (
                                    acc[-1][8 * i:8 * i + 8])
                    out.append((MM, lhs, rhs, consume))
        return out

    def scan_tasks(u, slot):
        steps, state = 2, {}
        hu = view(hb16, u * UNIT, (2 * NG - 1) * L + UNIT)

        def b(p, ch, r):
            return tuple(rows(bu, (slot * 2 * NG + c * NG + p) * BU_PART + 9 * (ch * R + r))
                         for c in range(2))

        def step(mu, h, br):
            return (mu[0] * h[0] + br[0]) - mu[1] * h[1], (mu[0] * h[1] + br[1]) + mu[1] * h[0]

        def ends(p, gate):
            mu, ties = (gate.value(prm(p, P_MU), PLAN["scan_lead"]), prm(p, P_MU + 1)), []
            h = [b(p, ch, 0) for ch in range(2)]
            for r in range(1, R):
                h = [step(mu, h[ch], b(p, ch, r)) for ch in range(2)]
                if r % steps == 0:
                    ties.append(h[r // steps % 2][0])
            state[p] = starts(p, h)
            return ties + [state[p][1][0]]

        def starts(p, e):
            last = lax.broadcasted_iota(I32, (8, 128), 0) == 7
            rho = (prm(p, P_RHO), prm(p, P_RHO + 1))
            pair = step(rho, e[0], e[1])
            a = tuple(pltpu.roll(jnp.where(last, rows(carry, (2 * p + c) * 8), pair[c]), 1, 0)
                      for c in range(2))
            for sh, row in ((1, P_RHO1), (2, P_RHO2), (4, P_RHO4)):
                a = step((prm(p, row), prm(p, row + 1)), tuple(pltpu.roll(c, sh, 0) for c in a), a)
            return [a, step(rho, a, e[0])]

        def run(p, r0, gate):
            if r0 == 0:
                state["mu"] = (prm(p, P_MU), prm(p, P_MU + 1))
            mu, h = (gate.value(state["mu"][0], PLAN["scan_lead"]), state["mu"][1]), state[p]
            for r in range(r0, r0 + steps):
                h = [step(mu, h[ch], b(p, ch, r)) for ch in range(2)]
                for c in range(2):
                    hu[pl.ds((c * NG + p) * L + 16 * r, 16), :] = _pack(h[0][c], h[1][c])
            state[p] = h
            if r0 + steps == R:
                for c in range(2):
                    carry[pl.ds((2 * p + c) * 8, 8), :] = h[1][c]
            return [after(hb)]

        tasks = []
        for p in range(NG):
            tasks.append(([16 * steps] * ((R - 1) // steps) + [46 + 16 * steps],
                          lambda gate, p=p: ends(p, gate)))
            tasks += [([18 * steps], lambda gate, p=p, r0=r0: run(p, r0, gate))
                      for r0 in range(0, R, steps)]
        return tasks

    def y_passes(h, n, sizes=(HALF,), z=0, slot=0):
        out, w, hu = [], view(wc, z), view(hb, h * (HALF // 2), ((2 * NG - 1) * L + HALF) // 2)
        for t0, MM in zip(np.cumsum((0,) + sizes).tolist(), sizes):
            acc = []
            for kk in range(2 * NG):
                def lhs(t0=t0, kk=kk, MM=MM):
                    return [rows(hu, (kk * L + t0) // 2 + 8 * i) for i in range(MM // 16)]

                def rhs(kk=kk):
                    return [rows(w, (kk * NG + n) * 64 + 8 * i) for i in range(8)]

                def consume(d, t0=t0, kk=kk, acc=acc, MM=MM):
                    acc.append(d if kk == 0 else acc[-1] + d)
                    if kk == 2 * NG - 1:
                        for i in range(MM // 8):
                            r, ch = divmod(t0 // 8 + i, 2)
                            at = (slot * NG + n) * YS_ROWS + ch * (R // 2 + 1) + r
                            ys[pl.ds(at, 8, stride=R + 2), :] = (
                                acc[-1][8 * i:8 * i + 8])
                out.append((MM, lhs, rhs, consume))
        return out

    def skip_task(h, n, slot=0):
        def fn(gate):
            dsk, ties = gate.value(prm(n, P_DSKIP), PLAN["skip_lead"]), []
            t = h // 2 * UNIT + h % 2 * (R // 2)
            edge = n == NG - 1 and isinstance(h, int)
            xu = x32.at[pl.ds(hint(t // 2 + n * (L // 2), 4), UNIT // 2 + (-4 if edge else 4)), :]
            ou = oa.at[pl.ds(hint(t, 8), UNIT - R // 2), :]
            for g in range(SEG):
                if g == SEG - 1 and edge:
                    xs = _unpack(rows(xu, 8 * g - 4))[1]
                else:
                    xs = _unpack(rows(xu, 8 * g))[0]
                y = rows(ys, (slot * NG + n) * YS_ROWS + g * (R // 2 + 1))
                ou[pl.ds(R * g, 8), pl.ds(128 * n, 128)] = y + xs * dsk
                if g % 8 == 7:
                    ties.append(after(oa))
            return ties
        return ([24, 24], fn)

    def widen_tasks(g):
        def fn(i0):
            kg = view(k32, g * (L // 2), L // 2)
            for i in range(i0, i0 + 8):
                lo, hi = _unpack(rows(kg, 8 * i))
                kf[pl.ds(KF_PAD + 16 * i, 8), :] = lo
                kf[pl.ds(KF_PAD + 16 * i + 8, 8), :] = hi
            return [after(kf)]
        return [([16], lambda gate, i=i: fn(i)) for i in range(0, L // 16, 8)]

    def transpose_tasks(g):
        n = 2

        def fn(c0):
            for c in range(c0, c0 + n):
                t = skb[pl.ds(hint(128 * g, 128), 128), pl.ds(128 * c, 128)]
                kt[pl.ds(64 * c, 64), :] = pltpu.bitcast(t.T, I32)
            return [after(kt)]
        return [([8 * n], lambda gate, c=c: fn(c)) for c in range(0, L // 128, n)]

    def staged(s, half, n, grp, c):
        return (((s * 2 + half) * 4 + n) * 4 + grp) * 16 + 8 * c

    ops1 = (18, 36, 30, 36)

    def transform_tasks(st, s, half, chunk, chunk_cost, direct):
        dst16, dst = (vu16, vu) if st is st_u else (vk16, vk)
        kept = []

        def first(gate, n):
            load = chunk(gate, n)
            u = [load(16 * half + n + 4 * m) for m in range(4)]
            pairs = _fwd1(n, [_Signed(v) for v in u])
            kept.append(pairs)
            for grp in range(2 * direct, 4):
                for c in range(2):
                    st[pl.ds(staged(s, half, n, grp, c), 8), :] = pairs[grp][c].get()
            return [u[0] + u[2]] * (chunk_cost > 4) + [after(st)]

        def second(grps):
            for grp in grps:
                if direct and grp < 2:
                    zs = [t[grp] for t in kept]
                else:
                    zs = [tuple(_Signed(rows(view(st, z8), staged(s, half, n, grp, c)))
                                for c in range(2)) for n in range(4)]
                for k, pair in enumerate(_fwd2(grp, zs)):
                    dst16[pl.ds(((4 * grp + k) * 2 + half) * 128 + 16 * s, 16), :] = (
                        _pack(pair[0].get(), pair[1].get()))
            return [after(dst)]

        split = (chunk_cost > 4) * (chunk_cost // 2 + 1)
        one = [([split] * (split > 0) + [chunk_cost + ops1[n] - split],
                lambda gate, n=n: first(gate, n)) for n in range(4)]
        two = [([40], lambda gate, grp=grp: second((grp, grp + 1))) for grp in (0, 2)]
        return (one + two[:1], two[1:]) if direct else (one, two)

    def kv_tasks(g):
        tasks = []
        for s in range(8):
            for half in range(2):
                def chunk(gate, n, s=s, loaded=[]):
                    if n == 0:
                        loaded[:] = [prm(g, P_TAP + t) for t in range(4)]
                    taps = [gate.value(loaded[0], PLAN["conv_lead"])] + loaded[1:]
                    kz, vg = view(kf, z8), view(v32, g * (L // 2), L // 2)

                    def load(c):
                        t = 64 * c + 8 * s
                        ks = rows(kz, KF_PAD + t) * taps[0]
                        for lag in range(1, 4):
                            ks = ks + rows(kz, KF_PAD + t - lag) * taps[lag]
                        return ks * _unpack(rows(vg, (t // 16) * 8))[s % 2]
                    return load
                tasks += sum(transform_tasks(st_u, s, half, chunk, 36, True), [])
        return tasks

    def filter_tasks(g, early, lead=None):
        before, after_use = [], []
        for j in range(16):
            def chunk(gate, n, s=j // 2):
                if lead:
                    gate.loads(kt, lead)

                def load(c):
                    v = _unpack(rows(view(kt, z8), 32 * c + 8 * (s // 2)))[s % 2]
                    if s == 0 and c == 0:
                        first = lax.broadcasted_iota(I32, (8, 128), 0) == 0
                        v = v + jnp.where(first, prm(g, P_SSMD), 0.0)
                    return v
                return load
            one, two = transform_tasks(st_k, j // 2, j % 2, chunk, 4, j >= early)
            before += one if j < early else []
            after_use += two if j < early else one + two
        return before, after_use

    def fwd_passes(grp):
        out = []
        for slot in range(4 * grp, 4 * grp + 4):
            got = []
            for src, half in ((vu, 0), (vk, 0), (vu, 1), (vk, 1)):
                def lhs(slot=slot):
                    return [rows(mf, slot * 64 + 8 * i) for i in range(8)]

                def rhs(slot=slot, src=src, half=half):
                    return [rows(view(src, z8), (2 * slot + half) * 64 + 8 * i) for i in range(8)]

                def consume(d, slot=slot, got=got):
                    got.append(d)
                    if len(got) < 4:
                        return
                    for i in range(8):
                        u0, k0, u1, k1 = (
                            (t[16 * i:16 * i + 8], t[16 * i + 8:16 * i + 16]) for t in got)
                        lo, a, b = _cmul(u0, k0), _cmul(u0, k1), _cmul(u1, k0)
                        if slot == _REAL_SLOT and i == 0:
                            first = lax.broadcasted_iota(I32, (8, 128), 0) == 0
                            lo, a, b = (
                                tuple(jnp.where(first, 0.5 * (x[c] * y[c]), p[c]) for c in range(2))
                                for p, x, y in ((lo, u0, k0), (a, u0, k1), (b, u1, k0)))
                        if _F1[slot] % 2:
                            hi = ((a[0] + b[0]) - lo[0], (a[1] + b[1]) - lo[1])
                        else:
                            hi = ((a[0] + b[0]) + lo[0], (a[1] + b[1]) + lo[1])
                        for half, p in enumerate((lo, hi)):
                            at = (slot % 4 * 2 + half) * 128 + 16 * i
                            pb16[grp % 2][pl.ds(at, 16), :] = _pack(*p)
                out.append((128, lhs, rhs, consume))
        return out

    def inv_passes(grp, half):
        out, got = [], []
        for slot in range(4 * grp, 4 * grp + 4):
            def lhs(slot=slot):
                return [rows(mi, slot * 64 + 8 * i) for i in range(8)]

            def rhs(slot=slot):
                return [rows(view(pb[grp % 2], z8), (slot % 4 * 2 + half) * 64 + 8 * i)
                        for i in range(8)]

            def consume(d):
                got.append(d)
                if len(got) < 4:
                    return
                for s in range(8):
                    w = [(_Signed(t[16 * s:16 * s + 8]), _Signed(t[16 * s + 8:16 * s + 16]))
                         for t in got]
                    for n, pair in enumerate(_inv2(grp, w)):
                        for c in range(2):
                            st_i[pl.ds(staged(s, half, n, grp, c), 8), :] = pair[c].get()
            out.append((128, lhs, rhs, consume))
        return out

    def inverse_tasks(g):
        def fn(gate, s, half):
            gate.loads(st_i, PLAN["inverse_lead"])
            qg, og, ties = view(q32, g * (L // 2), L // 2), view(ob, g * L, L), []
            for n in range(4):
                zs = [tuple(_Signed(rows(view(st_i, z8), staged(s, half, n, grp, c)))
                            for c in range(2)) for grp in range(4)]
                for m, y in enumerate(_inv1(n, zs)):
                    t = 64 * (16 * half + n + 4 * m) + 8 * s
                    og[pl.ds(t, 8), :] = _unpack(rows(qg, (t // 16) * 8))[s % 2] * y.get()
                ties.append(after(ob))
            return ties

        tasks = []
        for half in range(2):
            tasks += [([12 + n for n in ops1], lambda gate, s=s, half=half: fn(gate, s, half))
                      for s in range(8)]
            tasks.append(dma_task(ob_dma(g, half)))
        return tasks

    def dma_task(copy):
        return [1], lambda gate: copy.start()

    filter0 = x_dma(2, S_F0) + [sk_dma(0, S_F0)] + x_dma(3, S_F0)
    data0 = [col_dma(0, 0, S_K0), col_dma(1, 0, S_K0)]
    x0, x1 = x_dma(0, S_X0), x_dma(1, S_X0)

    def group_dma(g):
        at = S_COL + g
        return [col_dma(2, g, at), sk_dma(g + 1, at), col_dma(0, g + 1, at),
                col_dma(1, g + 1, at)] + x_dma(g + LEAD, at)

    last_dma = col_dma(2, NG - 1, S_SMALL)

    start(small + b_dma(0) + x0 + b_dma(1) + b_dma(2))
    wait(small + x0 + b_dma(0))
    zeros = rows(tab, 288).astype(I32)
    z8 = pl.multiple_of(zeros[0, 0], 16)
    sub = lax.broadcasted_iota(I32, (8, 128), 0)
    pred = zeros == 0

    def stack(ref):
        v = ref[...].astype(F32).reshape(1, D)
        return jnp.concatenate([v[:, 128 * g:128 * (g + 1)] for g in range(NG)]
                               + [v[:, :128]] * (8 - NG), axis=0)

    lre, lim = stack(lre_v), stack(lim_v)
    dt = jnp.exp(stack(ldt_v)).astype(BF16).astype(F32)
    mag, ang = jnp.exp(dt * lre), dt * lim
    lam = (mag * jnp.cos(ang), mag * jnp.sin(ang))
    scale = jnp.maximum(jnp.abs(lre), jnp.abs(lim))
    nre, nim = lre / scale, lim / scale
    den = (nre * nre + nim * nim) * scale
    coef = _cmul(((lam[0] - 1.0) / den, lam[1] / den), (nre, -nim))
    mu = lam
    rho = [mu]
    for _ in range(R.bit_length() + 2):
        rho.append(_cmul(rho[-1], rho[-1]))
    dsk, ssd = stack(dsk_v), stack(sd_v)
    taps = tap_v[...].astype(F32) * _FFT_SCALE
    for g in range(NG):
        def put(row, v):
            par[pl.ds((g * P_ROWS + row) * 8, 8), :] = v

        def lanes(v):
            return jnp.broadcast_to(v[g:g + 1], (8, 128))
        for c in range(2):
            put(P_MU + c, lanes(mu[c]))
            put(P_RHO + c, lanes(rho[-4][c]))
            for n, row in enumerate((P_RHO1, P_RHO2, P_RHO4)):
                put(row + c, jnp.where(sub >= 1 << n, lanes(rho[n - 3][c]), 0.0))
        for t in range(4):
            put(P_TAP + t, jnp.broadcast_to(taps[t:t + 1, 128 * g:128 * (g + 1)], (8, 128)))
        put(P_COEF, lanes(2.0 * coef[0]))
        put(P_COEF + 2, lanes(-2.0 * coef[1]))
        put(P_SSMD, lanes(ssd))
        put(P_DSKIP, lanes(dsk))
    for ref in (hb, oa, kf, kt, vu, vk, st_u, st_k, ob, mf, mi, wb, wc):
        ref[pl.ds(ref.shape[0] - 16, 8), pl.ds(0, 128)] = jnp.zeros((8, 128), ref.dtype)
    for i in range(2 * NG):
        carry[pl.ds(8 * i, 8), :] = jnp.zeros((8, 128), F32)
    kf[pl.ds(0, KF_PAD), :] = jnp.zeros((KF_PAD, 128), F32)

    def matrix_task(slot):
        def fn(gate):
            if slot != _REAL_SLOT:
                c, s = tab[pl.ds(256 + slot, 1), :], tab[pl.ds(272 + slot, 1), :]
            for a in range(8):
                if slot == _REAL_SLOT:
                    re, im = rows(tab, 128 + 16 * a), rows(tab, 128 + 16 * a + 8)
                else:
                    br, bi = rows(tab, 16 * a), rows(tab, 16 * a + 8)
                    re, im = c * br - s * bi, s * br + c * bi
                mf16[pl.ds(slot * 128 + 16 * a, 16), :] = _pack(re, im)
            m = pltpu.bitcast(rows(view(mf, z8), slot * 64, 64), BF16)
            mi[pl.ds(slot * 64, 64), :] = pltpu.bitcast(m.T, I32)
            return [after(mf), after(mi)]
        return ([48, 8], fn)

    def b_task(p):
        def fn(gate):
            ties = []
            for n in (p, NG + p):
                for kk in range(NG):
                    t = braw[pl.ds(128 * n, 128), pl.ds(128 * kk, 128)]
                    wb[pl.ds((n * NG + kk) * 64, 64), :] = pltpu.bitcast(t.T, I32)
                ties.append(after(wb))
            return ties
        return ([24, 24], fn)

    def c_task(n, p):
        def fn(gate):
            cr = gate.value(prm(p, P_COEF), PLAN["scale_lead"])
            nci = gate.value(prm(p, P_COEF + 2), PLAN["scale_lead"])
            t = [_unpack_tile(rows(c32, ((c * NG + p) * D + 128 * n) // 2, 64)) for c in range(2)]
            re = [_pack(cr * a0 + nci * b0, cr * a1 + nci * b1) for (a0, a1), (b0, b1) in zip(*t)]
            im = [_pack(nci * a0 - cr * b0, nci * a1 - cr * b1) for (a0, a1), (b0, b1) in zip(*t)]
            ties = []
            for c, tile in enumerate((re, im)):
                wc[pl.ds(((c * NG + p) * NG + n) * 64, 64), :] = pltpu.bitcast(
                    jnp.concatenate(tile, axis=0).T, I32)
                ties.append(after(wc))
            return ties
        return ([80, 80], fn)

    def y_block(halves, t0, lead, even, z=0, by_group=False):
        tiles = [(h, n) for h in halves for n in range(NG)]
        if by_group:
            tiles.sort(key=lambda tile: tile[1])
        passes, plan = [], []
        for j, (h, n) in enumerate(tiles):
            sizes = (HALF,)
            if j == 0 and lead is not None:
                if not lead:
                    continue
                sizes = (32, 96)
            if j == even:
                sizes = (64, 64)
            if j == len(tiles) - 1:
                sizes = (96, 32)
            slot = h if by_group else 0
            passes += y_passes(h, n, sizes, z, slot)
            t0 += 20
            plan.append(([skip_task(h, n, slot)], t0 + PLAN["skip"], t0 + PLAN["skip"] + 6))
        return passes, plan

    def conv_passes(between):
        passes = fwd_passes(0)
        for grp in range(1, 4):
            f = fwd_passes(grp)
            passes += f[:8] + inv_passes(grp - 1, 0) + f[8:] + inv_passes(grp - 1, 1)
        return passes + between[:8] + inv_passes(3, 0) + inv_passes(3, 1) + between[8:]

    unit = 2 * NG * NG * UNIT // 64

    first = bu_passes(0, 1, raw=True)
    first = [first[20 * p:20 * (p + 1)] for p in range(NG)]
    start(b_dma(3) + b_dma(4) + x1 + [tab_dma])
    _weave(first[0], [], pred)
    start(filter0)
    wait(b_dma(1))
    _weave(first[1], [], pred)
    start(data0 + c_dma)
    wait(b_dma(2))
    _weave(first[2], [([b_task(p) for p in range(2)], 0, 40)], pred)
    wait(b_dma(3))
    _weave(first[3], [([b_task(p) for p in range(2, 4)], 0, 40)], pred)
    start(group_dma(0))
    wait(b_dma(4))
    _weave(first[4], [([b_task(4)], 0, 36)], pred)
    wait(x1 + [tab_dma])
    _weave(bu_passes(1, 0, 64), [
        (scan_tasks(0, 1), 0, unit),
        ([matrix_task(slot) for slot in range(SLOTS)], *PLAN["matrix"])], pred)
    start(group_dma(1))
    wait(filter0)
    _weave(bu_passes(2, 1, 64) + bu_passes(3, 0, 64, groups=[0]), [
        (scan_tasks(1, 0), 0, unit), (transpose_tasks(0), 8, 32),
        (filter_tasks(0, 0, PLAN["filter_lead"])[1], *PLAN["filter0"])], pred)
    start(group_dma(2))
    wait(data0 + c_dma)
    yp, plan = y_block((0, 1), unit - 40, None, 2, z8, by_group=True)
    kv = kv_tasks(0)
    end = 2 * unit - 40
    _weave(bu_passes(3, 0, shift=True, groups=range(1, NG)) + yp, plan + [
        (scan_tasks(2, 1), *PLAN["scan0"]), (widen_tasks(0), 0, 40),
        ([c_task(n, p) for n in range(NG) for p in range(NG)], *PLAN["scale_c"]),
        (kv[:-2], PLAN["forward0"], end), (kv[-2:], end, end)], pred)
    start([oa_unit_dma(0)] + group_dma(3) + [last_dma])

    def body(i, _):
        wait(group_dma(i))
        halves = [2 + 3 * i + j for j in range(3)]
        y0 = 192 + 20 + unit
        yp, plan = y_block(halves, y0, False, 7)
        passes = conv_passes(y_passes(halves[0], 0, (32, 96))) + bu_passes(i + LEAD, 0) + yp
        early, late = filter_tasks(i + 1, PLAN["early"])
        kv, tail, end = kv_tasks(i + 1), PLAN["tail"], y0 + 280
        done = (3 * i + 2) // 2
        sent = y0 + 180 + PLAN["skip"] + 8
        _weave(passes, plan + [
            ([dma_task(oa_unit_dma(done))], sent, sent),
            (scan_tasks(i + LEAD - 1, 0), *PLAN["scan"]),
            (transpose_tasks(i + 1), *PLAN["transpose"]),
            ([skip_task(halves[0], 0)], 232, 238),
            (widen_tasks(i + 1), *PLAN["widen"]), (early, *PLAN["filter_early"]),
            (inverse_tasks(i), *PLAN["inverse"]), (late, *PLAN["filter"]),
            (kv[:-tail], PLAN["forward"], end), (kv[-tail:], end, end)], pred)
        pl.when(i % 2 == 1)(lambda: start([oa_unit_dma(done + 1)]))
        return 0

    lax.fori_loop(0, NG - 1, body, 0)

    wait([last_dma])
    last = L // UNIT - 1
    yp, plan = y_block((2 * last, 2 * last + 1), 192, True, 2)
    plan += [([dma_task(oa_dma(last, n))], t + 6, t + 6) for n, (_, _, t) in enumerate(plan[NG:])]
    _weave(conv_passes(yp), plan + [
        (scan_tasks(last, 0), 0, 170), (inverse_tasks(NG - 1), *PLAN["last_inverse"])], pred)
    wait([oa_unit_dma(u) for u in range(last)] + [oa_dma(last, n) for n in range(NG)]
         + [ob_dma(n, half) for n in range(NG) for half in range(2)])


@jax.jit
def pallas_concat_heads__ssm_conv_s5__ssm_conv_h3__prompt_kernel(
    A_x: jax.Array,
    A_Lambda_re: jax.Array,
    A_Lambda_im: jax.Array,
    A_B_re: jax.Array,
    A_B_im: jax.Array,
    A_C_re: jax.Array,
    A_C_im: jax.Array,
    A_log_dt: jax.Array,
    A_Dskip: jax.Array,
    B_q: jax.Array,
    B_k: jax.Array,
    B_v: jax.Array,
    B_shift_k: jax.Array,
    B_ssm_k: jax.Array,
    B_ssm_D: jax.Array,
):
    assert A_x.shape == (1, L, D) and B_shift_k.shape == (D, 4)
    vmem = pltpu.VMEM
    dma = pltpu.SemaphoreType.DMA
    scratch = [
        vmem(_TABLES.shape, F32),
        vmem((D,), BF16), vmem((D,), BF16), vmem((D,), BF16), vmem((D,), BF16), vmem((D,), BF16),
        vmem((4, D), BF16),
        vmem((NG * L, 128), BF16),
        vmem((2 * D, D), BF16),
        vmem((2 * NG * D, 128), BF16),
        vmem((NG * L, 128), BF16),
        vmem((NG * L, 128), BF16),
        vmem((NG * L, 128), BF16),
        vmem((D, L), BF16),
        vmem((NG * P_ROWS * 8, 128), F32),
        vmem((2 * NG * D + 32, 128), BF16),
        vmem((2 * NG * NG * 64 + 16, 128), I32),
        vmem((SLOTS * 128 + 32, 128), BF16),
        vmem((SLOTS * 64 + 16, 128), I32),
        vmem((2 * 2 * NG * BU_PART, 128), F32),
        vmem((2 * NG * L + 32, 128), BF16),
        vmem((3 * NG * 8, 128), F32),
        vmem((2 * NG * YS_ROWS, 128), F32),
        vmem((L + 16, D), F32),
        vmem((L // 2 + 16, 128), I32),
        vmem((KF_PAD + L + 16, 128), F32),
        vmem((2 * L + 16, 128), F32),
        vmem((2 * L + 16, 128), F32),
        vmem((2 * L + 8, 128), F32),
        vmem((32 * 128 + 32, 128), BF16),
        vmem((32 * 128 + 32, 128), BF16),
        vmem((8 * 128, 128), BF16),
        vmem((8 * 128, 128), BF16),
        vmem((NG * L + 16, 128), F32),
        dma((S_END,)),
    ]
    out = pl.pallas_call(
        _kernel,
        out_shape=jax.ShapeDtypeStruct((L, 2 * D), F32),
        in_specs=[pl.BlockSpec(memory_space=pl.ANY)] * 16,
        out_specs=pl.BlockSpec(memory_space=pl.ANY),
        scratch_shapes=scratch,
        compiler_params=pltpu.CompilerParams(vmem_limit_bytes=100 * 1024 * 1024),
        name="s5_h3",
    )(_TABLES, A_x.reshape(L, D), A_Lambda_re, A_Lambda_im, A_B_re, A_B_im, A_C_re, A_C_im,
      A_log_dt, A_Dskip, B_q.reshape(L, D), B_k.reshape(L, D), B_v.reshape(L, D),
      B_shift_k.T, B_ssm_k, B_ssm_D)
    return out.reshape(1, L, 2 * D)
```
